```python
import jax
import jax.numpy as jnp

def _softmax(x, axis=-1):
    return jax.nn.softmax(x, axis=axis)

def _gelu(x):
    return jax.nn.gelu(x, approximate=True)

def _silu(x):
    return jax.nn.silu(x)

def _sigmoid(x):
    return jax.nn.sigmoid(x)

def _layernorm(x, axis=-1, eps=1e-05):
    m = jnp.mean(x, axis=axis, keepdims=True)
    v = jnp.var(x, axis=axis, keepdims=True)
    return (x - m) / jnp.sqrt(v + eps)

def _scatter_add(tgt, idx, src, axis=0):
    return tgt.at[idx].add(src)

def _segment_sum(src, seg, n):
    return jax.ops.segment_sum(src, seg, n)

class _Rng:

    def __init__(self, key):
        self._k = key

    def _next(self):
        self._k, sub = jax.random.split(self._k)
        return sub

    def normal(self, shape):
        return jax.random.normal(self._next(), shape, dtype=jnp.bfloat16)

    def randint(self, lo, hi, shape):
        return jax.random.randint(self._next(), shape, lo, hi, dtype=jnp.int32)

    def uniform(self, shape, lo=0.0, hi=1.0):
        return jax.random.uniform(self._next(), shape, jnp.bfloat16, lo, hi)

    def permutation(self, n):
        return jax.random.permutation(self._next(), n)
kernel_name = 'recurrent_scan__ssm_conv_h3__mixer_gmlp__prompt'

def setup_inputs():
    _rng = _Rng(jax.random.key(int.from_bytes(__import__("os").urandom(4), "little")))
    _w = lambda a: (lambda t: t.astype(jnp.bfloat16) if jnp.issubdtype(t.dtype, jnp.floating) else t)(jnp.asarray(a))

    def _A_setup():
        B, S, D = (1, 2048, 640)
        ks = 4
        return {'q': _w((lambda *s: _rng.normal(s) * 0.05)(B, S, D)), 'k': _w((lambda *s: _rng.normal(s) * 0.05)(B, S, D)), 'v': _w((lambda *s: _rng.normal(s) * 0.05)(B, S, D)), 'shift_k': _w((lambda *s: _rng.normal(s) * 0.05)(D, ks) * 0.5), 'ssm_k': _w((lambda *s: _rng.normal(s) * 0.05)(D, S) * (1.0 / S ** 0.5)), 'ssm_D': _w((lambda *s: _rng.normal(s) * 0.05)(D))}
    _A_in = _A_setup()

    def _B_setup():
        B, S, D, F = (1, 2048, 640, 1536)
        Fh = F // 2
        return {'x': _w((lambda *s: _rng.normal(s) * 0.05)(B, S, D)), 'w_in': _w((lambda *s: _rng.normal(s) * 0.05)(D, 2 * Fh)), 'w_sp': _w(0.01 * (lambda *s: _rng.normal(s) * 0.05)(S, S)), 'b_sp': _w(1.0 + 0.01 * (lambda *s: _rng.normal(s) * 0.05)(S)), 'w_out': _w((lambda *s: _rng.normal(s) * 0.05)(Fh, D))}
    _B_in = _B_setup()
    return {'A_q': _A_in['q'], 'A_k': _A_in['k'], 'A_v': _A_in['v'], 'A_shift_k': _A_in['shift_k'], 'A_ssm_k': _A_in['ssm_k'], 'A_ssm_D': _A_in['ssm_D'], 'B_x': _B_in['x'], 'B_w_in': _B_in['w_in'], 'B_w_sp': _B_in['w_sp'], 'B_b_sp': _B_in['b_sp'], 'B_w_out': _B_in['w_out']}

def reference(A_q, A_k, A_v, A_shift_k, A_ssm_k, A_ssm_D, B_x, B_w_in, B_w_sp, B_b_sp, B_w_out):

    def _A_ref(q, k, v, shift_k, ssm_k, ssm_D):
        B, S, D = q.shape
        ks = shift_k.shape[-1]
        k_pad = jnp.pad(k, ((0, 0), (ks - 1, 0), (0, 0)))
        k_shift = jnp.zeros_like(k)
        for t in range(ks):
            k_shift = k_shift + k_pad[:, t:t + S, :] * shift_k[:, ks - 1 - t][None, None, :]
        kv = k_shift * v
        L = 2 * S
        kv_pad = jnp.pad(kv, ((0, 0), (0, S), (0, 0)))
        kf_pad = jnp.pad(ssm_k, ((0, 0), (0, S)))
        kv_f = (lambda x, axes=(-2, -1): jnp.fft.rfft2(x.astype(jnp.float32), axes=axes))(kv_pad[:, None, :, :], axes=(1, 2))
        kf_f = (lambda x, axes=(-2, -1): jnp.fft.rfft2(x.astype(jnp.float32), axes=axes))(kf_pad[:, None, :], axes=(1, 2))
        kf_f = (lambda x, *d: x.transpose(*d))(kf_f, 1, 2, 0)
        y_f = kv_f * kf_f[None, :, :, :]
        y = (lambda x, s, axes=(-2, -1): jnp.fft.irfft2(x, s=s, axes=axes).astype(jnp.bfloat16))(y_f, (1, L), axes=(1, 2))[:, 0, :S, :]
        y = y + kv * ssm_D[None, None, :]
        return q * y

    def _B_ref(x, w_in, w_sp, b_sp, w_out):
        B, S, D = x.shape
        F = w_in.shape[-1]
        Fh = F // 2
        z = _gelu(jnp.einsum('bsd,df->bsf', x, w_in))
        z1 = z[..., :Fh].copy()
        z2 = _layernorm(z[..., Fh:], axis=-1)
        g = jnp.einsum('ts,bsf->btf', w_sp, z2) + b_sp[None, :, None]
        return jnp.einsum('bsf,fd->bsd', z1 * g, w_out)
    x = A_q
    xn = _layernorm(x, axis=-1)
    s = _A_ref(xn, A_k, A_v, A_shift_k, A_ssm_k, A_ssm_D)
    g = _silu(_B_ref(xn, B_w_in, B_w_sp, B_b_sp, B_w_out))
    return x + s * g
```

```python
import math

import jax
import jax.numpy as jnp
import jax.experimental.pallas as pl
import jax.experimental.pallas.tpu as pltpu

S = 2048
D = 640
FH = 768
P = 128
NB = S // P
TM = 256
NT = S // TM
EPS = 1e-5
F32 = jnp.float32
BF16 = jnp.bfloat16
GELU_C = math.sqrt(2.0 / math.pi)


def _dft_angle(shape, k_dim, n_dim):
    r = jax.lax.broadcasted_iota(jnp.int32, shape, k_dim)
    n = jax.lax.broadcasted_iota(jnp.int32, shape, n_dim)
    odd2 = jnp.where(r < 64, 4 * r + 1, 4 * r - 253)
    m = (odd2 * n) & 511
    return m.astype(F32) * (2.0 * math.pi / 512.0)


def _gelu2(z):
    u = z * (GELU_C + (GELU_C * 0.044715) * (z * z))
    return z + z * jnp.tanh(u)


def _ln(x, eps):
    n = x.shape[-1]
    m = jnp.sum(x, axis=-1, keepdims=True) * (1.0 / n)
    xc = x - m
    v = jnp.sum(xc * xc, axis=-1, keepdims=True) * (1.0 / n)
    return xc * jax.lax.rsqrt(v + eps)


def _blocks_of_step(i):
    return (i, NB - 1 - i)


def _kernel(q_hbm, k_hbm, v_hbm, sk_ref, h_hbm, d_ref, win_hbm, wsp_hbm, b_ref, wout_hbm,
            o_hbm,
            x_v, k_v, v_v, h_v, win_v, wsp_v, wout_v, o_v,
            xn_v, z1_v, z2_v, X_v, H_v, G_v, Z_v, F_v, Fi_v, bcol_v,
            sem_in, sem_w, sem_out):
    def cp_x(i):
        return pltpu.make_async_copy(q_hbm.at[0, pl.ds(i * TM, TM)], x_v.at[pl.ds(i * TM, TM)], sem_in.at[0, i])

    def cp_k(i):
        return pltpu.make_async_copy(k_hbm.at[0, pl.ds(i * TM, TM)], k_v.at[pl.ds(i * TM + 16, TM)], sem_in.at[1, i])

    def cp_v(i):
        return pltpu.make_async_copy(v_hbm.at[0, pl.ds(i * TM, TM)], v_v.at[pl.ds(i * TM, TM)], sem_in.at[2, i])

    def cp_h(i):
        return pltpu.make_async_copy(h_hbm.at[:, pl.ds(i * TM, TM)], h_v.at[i], sem_in.at[3, i])

    def cp_wsp(i, half):
        a = _blocks_of_step(i)[half]
        return pltpu.make_async_copy(wsp_hbm.at[pl.ds(a * P, P)], wsp_v.at[pl.ds(i * TM + half * P, P)],
                                     sem_in.at[4 + half, i])

    def cp_win():
        return pltpu.make_async_copy(win_hbm, win_v, sem_w.at[0])

    def cp_wout():
        return pltpu.make_async_copy(wout_hbm, wout_v, sem_w.at[1])

    def cp_out(a):
        return pltpu.make_async_copy(o_v.at[pl.ds(a * P, P)], o_hbm.at[0, pl.ds(a * P, P)], sem_out.at[a])

    def start_p1(i):
        cp_h(i).start()
        cp_x(i).start()
        cp_k(i).start()
        cp_v(i).start()

    start_p1(0)
    cp_win().start()
    start_p1(1)

    ang = _dft_angle((P, P), 0, 1)
    F_v[0:P, :] = jnp.cos(ang).astype(BF16)
    F_v[P:2 * P, :] = (-jnp.sin(ang)).astype(BF16)
    angt = _dft_angle((P, P), 1, 0)
    Fi_v[:, 0:P] = (jnp.cos(angt) * (1.0 / P)).astype(BF16)
    Fi_v[:, P:2 * P] = (jnp.sin(angt) * (-1.0 / P)).astype(BF16)

    brow = b_ref[...].astype(F32).reshape(1, S)
    for j in range(NB):
        bcol_v[j * P:(j + 1) * P, :] = jnp.broadcast_to(brow[:, j * P:(j + 1) * P], (P, P)).T
    drow = d_ref[...].astype(F32).reshape(1, D)
    sk = sk_ref[...].astype(F32)

    k_v[0:16, :] = jnp.zeros((16, D), BF16)
    H_v[0:P, :] = jnp.zeros((P, D), F32)
    H_v[P:P + 64, :] = jnp.broadcast_to(-drow, (64, D))
    H_v[P + 64:2 * P, :] = jnp.broadcast_to(drow, (64, D))
    cp_win().wait()

    def p1_step(i, carry):
        r0 = pl.multiple_of(i * TM, TM)
        rows = pl.ds(r0, TM)

        @pl.when(i + 2 < NT)
        def _():
            start_p1(i + 2)

        @pl.when(i >= 4)
        def _():
            for j in (0, 1):
                cp_wsp(2 * (i - 4) + j, 0).start()
                cp_wsp(2 * (i - 4) + j, 1).start()

        @pl.when(i == 3)
        def _():
            cp_wout().start()

        cp_h(i).wait()
        cp_x(i).wait()
        cp_k(i).wait()
        cp_v(i).wait()
        Fm = F_v[...]
        Hp = H_v[...]
        for half in range(2):
            j = 2 * i + half
            Hj = jax.lax.dot_general(Fm, h_v[i, :, half * P:(half + 1) * P], (((1,), (1,)), ((), ())),
                                     preferred_element_type=F32)
            G_v[j, 0:64, :] = Hj[0:64] - Hp[P:P + 64]
            G_v[j, 64:P, :] = Hj[64:P] + Hp[P + 64:2 * P]
            G_v[j, P:P + 64, :] = Hj[P:P + 64] + Hp[0:64]
            G_v[j, P + 64:2 * P, :] = Hj[P + 64:2 * P] - Hp[64:P]
            Hp = Hj
        H_v[...] = Hp

        xn = _ln(x_v[rows, :].astype(F32), EPS).astype(BF16)
        xn_v[rows, :] = xn
        z2 = _gelu2(jnp.dot(xn, win_v[:, FH:], preferred_element_type=F32))
        z2_v[rows, :] = _ln(z2, 4.0 * EPS).astype(BF16)
        z1_v[rows, :] = _gelu2(jnp.dot(xn, win_v[:, :FH], preferred_element_type=F32))

        kf = k_v[pl.ds(r0, TM + 16), :].astype(F32)
        ks = kf[16:16 + TM] * sk[0:1]
        for t in range(1, 4):
            ks = ks + kf[16 - t:16 - t + TM] * sk[t:t + 1]
        kv = (ks * v_v[rows, :].astype(F32)).astype(BF16)
        for half in range(2):
            X_v[2 * i + half] = jnp.dot(Fm, kv[half * P:(half + 1) * P], preferred_element_type=F32)
        return carry

    jax.lax.fori_loop(0, NT, p1_step, 0)

    cp_wout().wait()
    for i in range(NT):
        cp_wsp(i, 0).wait()
        cp_wsp(i, 1).wait()
    for i in range(NT):
        blocks = _blocks_of_step(i)
        for half, a in enumerate(blocks):
            for r in range(P // 16):
                re = pl.ds(r * 16, 16)
                im = pl.ds(P + r * 16, 16)
                accr = None
                acci = None
                for c in range(a + 1):
                    xr = X_v[c, re, :]
                    xi = X_v[c, im, :]
                    gr = G_v[a - c, re, :]
                    gi = G_v[a - c, im, :]
                    pr = xr * gr - xi * gi
                    pi = xr * gi + xi * gr
                    accr = pr if accr is None else accr + pr
                    acci = pi if acci is None else acci + pi
                Z_v[half, re, :] = accr.astype(BF16)
                Z_v[half, im, :] = acci.astype(BF16)

        g = jnp.dot(wsp_v[pl.ds(i * TM, TM), :], z2_v[...], preferred_element_type=F32)
        bc = jnp.concatenate([bcol_v[pl.ds(a * P, P), :] for a in blocks], axis=0)
        z1 = jnp.concatenate([z1_v[pl.ds(a * P, P), :] for a in blocks], axis=0)
        u = (z1 * (g + jnp.concatenate([bc] * (FH // 128), axis=1))).astype(BF16)
        hh = jnp.dot(u, wout_v[...], preferred_element_type=F32) * 0.25
        gate = hh + hh * jnp.tanh(hh)
        Fi = Fi_v[...]
        for half, a in enumerate(blocks):
            rows = pl.ds(a * P, P)
            y = jnp.dot(Fi, Z_v[half], preferred_element_type=F32)
            s = xn_v[rows, :].astype(F32) * y
            o_v[rows, :] = (x_v[rows, :].astype(F32) + s * gate[half * P:(half + 1) * P]).astype(BF16)
            cp_out(a).start()
    for a in range(NB):
        cp_out(a).wait()


@jax.jit
def pallas_recurrent_scan__ssm_conv_h3__mixer_gmlp__prompt_kernel(
    A_q: jax.Array,
    A_k: jax.Array,
    A_v: jax.Array,
    A_shift_k: jax.Array,
    A_ssm_k: jax.Array,
    A_ssm_D: jax.Array,
    B_x: jax.Array,
    B_w_in: jax.Array,
    B_w_sp: jax.Array,
    B_b_sp: jax.Array,
    B_w_out: jax.Array,
):
    del B_x
    hbm = pl.BlockSpec(memory_space=pl.ANY)
    vmem = pl.BlockSpec(memory_space=pltpu.VMEM)
    return pl.pallas_call(
        _kernel,
        out_shape=jax.ShapeDtypeStruct((1, S, D), BF16),
        in_specs=[hbm, hbm, hbm, vmem, hbm, vmem, hbm, hbm, vmem, hbm],
        out_specs=hbm,
        scratch_shapes=[
            pltpu.VMEM((S, D), BF16),
            pltpu.VMEM((S + 16, D), BF16),
            pltpu.VMEM((S, D), BF16),
            pltpu.VMEM((NT, D, TM), BF16),
            pltpu.VMEM((D, 2 * FH), BF16),
            pltpu.VMEM((S, S), BF16),
            pltpu.VMEM((FH, D), BF16),
            pltpu.VMEM((S, D), BF16),
            pltpu.VMEM((S, D), BF16),
            pltpu.VMEM((S, FH), F32),
            pltpu.VMEM((S, FH), BF16),
            pltpu.VMEM((NB, 2 * P, D), F32),
            pltpu.VMEM((2 * P, D), F32),
            pltpu.VMEM((NB, 2 * P, D), F32),
            pltpu.VMEM((2, 2 * P, D), BF16),
            pltpu.VMEM((2 * P, P), BF16),
            pltpu.VMEM((P, 2 * P), BF16),
            pltpu.VMEM((S, 128), F32),
            pltpu.SemaphoreType.DMA((6, NT)),
            pltpu.SemaphoreType.DMA((2,)),
            pltpu.SemaphoreType.DMA((NB,)),
        ],
        compiler_params=pltpu.CompilerParams(vmem_limit_bytes=100 * 1024 * 1024),
    )(A_q, A_k, A_v, A_shift_k.T, A_ssm_k, A_ssm_D, B_w_in, B_w_sp, B_b_sp, B_w_out)
```

```python
import math

import jax
import jax.numpy as jnp
import jax.experimental.pallas as pl
import jax.experimental.pallas.tpu as pltpu

S = 2048
D = 640
FH = 768
P = 128
NB = S // P
TM = 256
NT = S // TM
MC = 64
L = 128
EPS = 1e-5
F32 = jnp.float32
BF16 = jnp.bfloat16
U32 = jnp.uint32
GELU_C = math.sqrt(2.0 / math.pi)
NT_DIMS = (((1,), (1,)), ((), ()))


def _dot(a, b):
    return jnp.dot(a, b, preferred_element_type=F32)


def _dft_angle(shape, k_dim, n_dim):
    r = jax.lax.broadcasted_iota(jnp.int32, shape, k_dim)
    n = jax.lax.broadcasted_iota(jnp.int32, shape, n_dim)
    odd2 = jnp.where(r < 64, 4 * r + 1, 4 * r - 253)
    m = (odd2 * n) & 511
    return m.astype(F32) * (2.0 * math.pi / 512.0)


def _gelu2(z):
    u = z * (GELU_C + (GELU_C * 0.044715) * (z * z))
    return z + z * jnp.tanh(u)


def _ln(x, eps):
    n = x.shape[-1]
    m = jnp.sum(x, axis=-1, keepdims=True) * (1.0 / n)
    xc = x - m
    v = jnp.sum(xc * xc, axis=-1, keepdims=True) * (1.0 / n)
    return xc * jax.lax.rsqrt(v + eps)


def _blocks_of_step(i):
    return (i, NB - 1 - i)


class _Background:
    def __init__(self):
        self.q = []
        self.credit = 0.0

    def add(self, gen):
        self.q.append(gen)

    def run(self, budget):
        self.credit += budget
        while self.q and self.credit > 0:
            try:
                self.credit -= next(self.q[0])
            except StopIteration:
                self.q.pop(0)
        if not self.q:
            self.credit = 0.0

    def drain(self):
        while self.q:
            self.run(1e9)


def _kernel(one_ref, q_hbm, k_hbm, v_hbm, sk_ref, h_hbm, d_ref, win_hbm, wsp_hbm, b_ref, wout_hbm,
            o_hbm,
            x_u, k_u, v_u, h_u, win_u, wsp_u, wout_u, o_v,
            xn_u, z1_v, z2_u, kv_u, u_u, X_v, H_v, G_v, Z_u, F_u, Fi_u, bcol_v, sk_v,
            sem_in, sem_w, sem_out):
    x_v, k_v, v_v, h_v, win_v, wsp_v, wout_v, xn_v, z2_v, kv_v, u_v, Z_v, F_v, Fi_v = [
        r.bitcast(BF16) for r in (x_u, k_u, v_u, h_u, win_u, wsp_u, wout_u, xn_u, z2_u, kv_u, u_u, Z_u, F_u, Fi_u)]

    def cp_x(i):
        return pltpu.make_async_copy(q_hbm.at[0, pl.ds(i * TM, TM)], x_v.at[pl.ds(i * TM, TM)], sem_in.at[0, i])

    def cp_k(i):
        return pltpu.make_async_copy(k_hbm.at[0, pl.ds(i * TM, TM)], k_v.at[pl.ds(i * TM + 16, TM)],
                                     sem_in.at[1, i])

    def cp_v(i):
        return pltpu.make_async_copy(v_hbm.at[0, pl.ds(i * TM, TM)], v_v.at[pl.ds(i * TM, TM)], sem_in.at[2, i])

    def cp_h(i):
        return pltpu.make_async_copy(h_hbm.at[:, pl.ds(i * TM, TM)], h_v.at[i], sem_in.at[3, i])

    def cp_wsp(i, half):
        a = _blocks_of_step(i)[half]
        return pltpu.make_async_copy(wsp_hbm.at[pl.ds(a * P, P)], wsp_v.at[pl.ds(i * TM + half * P, P)],
                                     sem_in.at[4 + half, i])

    def cp_win():
        return pltpu.make_async_copy(win_hbm, win_v, sem_w.at[0])

    def cp_wout():
        return pltpu.make_async_copy(wout_hbm, wout_v, sem_w.at[1])

    def cp_out(a):
        return pltpu.make_async_copy(o_v.at[pl.ds(a * P, P)], o_hbm.at[0, pl.ds(a * P, P)], sem_out.at[a])

    def block(fn):
        pl.when(one_ref[0] == 1)(fn)

    def ln_x(i):
        for s in range(TM // 16):
            rows = pl.ds(i * TM + s * 16, 16)
            xn_v[rows, :] = _ln(x_v[rows, :].astype(F32), EPS).astype(BF16)
            yield 80

    def x_dft(i):
        Fm = F_v[...]
        for half in range(2):
            j = 2 * i + half
            X_v[j] = _dot(Fm, kv_v[j * P:(j + 1) * P, :])

    cp_x(0).start()
    cp_h(0).start()
    cp_win().start()
    cp_x(1).start()
    cp_k(0).start()
    cp_v(0).start()

    ang = _dft_angle((P, P), 0, 1)
    F_v[0:P, :] = jnp.cos(ang).astype(BF16)
    F_v[P:2 * P, :] = (-jnp.sin(ang)).astype(BF16)
    angt = _dft_angle((P, P), 1, 0)
    Fi_v[:, 0:P] = (jnp.cos(angt) * (1.0 / P)).astype(BF16)
    Fi_v[:, P:2 * P] = (jnp.sin(angt) * (-1.0 / P)).astype(BF16)

    brow = b_ref[...].astype(F32).reshape(1, S)
    for j in range(NB):
        bcol_v[j * P:(j + 1) * P, :] = jnp.broadcast_to(brow[:, j * P:(j + 1) * P], (P, P)).T
    drow = d_ref[...].astype(F32).reshape(1, D)
    sk = sk_ref[...].astype(F32)
    for t in range(4):
        sk_v[t] = jnp.broadcast_to(sk[t:t + 1], (8, D))

    k_v[0:16, :] = jnp.zeros((16, D), BF16)
    H_v[0:P, :] = jnp.zeros((P, D), F32)
    H_v[P:P + 64, :] = jnp.broadcast_to(-drow, (64, D))
    H_v[P + 64:2 * P, :] = jnp.broadcast_to(drow, (64, D))
    cp_x(0).wait()
    for _ in ln_x(0):
        pass

    def p1_dma(i):
        if i + 1 < NT:
            cp_h(i + 1).start()
            cp_k(i + 1).start()
            cp_v(i + 1).start()
        if i + 2 < NT:
            cp_x(i + 2).start()
        if i >= 4:
            for j in (0, 1):
                cp_wsp(2 * (i - 4) + j, 0).start()
                cp_wsp(2 * (i - 4) + j, 1).start()
        if i == 3:
            cp_wout().start()
        if i == 0:
            cp_win().wait()
        cp_h(i).wait()
        cp_k(i).wait()
        cp_v(i).wait()
        if i + 1 < NT:
            cp_x(i + 1).wait()

    def p1_step(i):
        r0 = i * TM
        bg = _Background()

        def kv_gen():
            for m in range(TM // MC):
                for l in range(D // L):
                    lanes = slice(l * L, (l + 1) * L)
                    kf = k_v[pl.ds(r0 + m * MC, MC + 16), lanes].astype(F32)
                    ks = None
                    for t in range(4):
                        w = sk_v[t, 0:1, lanes]
                        term = kf[16 - t:16 - t + MC] * w
                        ks = term if ks is None else ks + term
                    kv = ks * v_v[pl.ds(r0 + m * MC, MC), lanes].astype(F32)
                    kv_v[pl.ds(r0 + m * MC, MC), lanes] = kv.astype(BF16)
                    yield 115

        def ln_z2(m, tiles, s1, s2):
            mean = jnp.sum(s1, axis=-1, keepdims=True) * (1.0 / FH)
            ex2 = jnp.sum(s2, axis=-1, keepdims=True) * (1.0 / FH)
            var = jnp.maximum(ex2 - mean * mean, 0.0)
            rs = jax.lax.rsqrt(var + 4.0 * EPS)
            yield 50
            for n in range(FH // L):
                z2_v[pl.ds(r0 + m * MC, MC), n * L:(n + 1) * L] = ((tiles[n] - mean) * rs).astype(BF16)
                yield 20

        if i + 1 < NT:
            bg.add(ln_x(i + 1))
        bg.add(kv_gen())

        prev = [H_v[qd * 64:(qd + 1) * 64, :] for qd in range(4)]
        for half in range(2):
            j = 2 * i + half
            cur = []
            for qd in range(4):
                hq = jax.lax.dot_general(F_v[qd * 64:(qd + 1) * 64, :], h_v[i, :, half * P:(half + 1) * P],
                                         NT_DIMS, preferred_element_type=F32)
                cur.append(hq)
                other = prev[(qd + 2) % 4]
                G_v[j, qd * 64:(qd + 1) * 64, :] = hq - other if qd in (0, 3) else hq + other
                bg.run(100)
            prev = cur
        if i + 1 < NT:
            for qd in range(4):
                H_v[qd * 64:(qd + 1) * 64, :] = prev[qd]

        for m in range(TM // MC):
            rows = pl.ds(r0 + m * MC, MC)
            tiles = []
            s1 = s2 = None
            for n in range(FH // L):
                z = _gelu2(_dot(xn_v[rows, :], win_v[:, FH + n * L:FH + (n + 1) * L]))
                tiles.append(z)
                s1 = z if s1 is None else s1 + z
                s2 = z * z if s2 is None else s2 + z * z
                bg.run(55)
            bg.q.insert(0, ln_z2(m, tiles, s1, s2))
            for n in range(FH // L):
                z1_v[rows, n * L:(n + 1) * L] = _gelu2(_dot(xn_v[rows, :], win_v[:, n * L:(n + 1) * L]))
                bg.run(90)
        bg.drain()
        if i > 0:
            x_dft(i - 1)

    for i in range(NT):
        p1_dma(i)
        block(lambda i=i: p1_step(i))

    def p2_dma(i):
        if i == 0:
            cp_wout().wait()
        if i >= 2:
            for a in _blocks_of_step(i - 2):
                cp_out(a).start()
        if i < NT:
            cp_wsp(i, 0).wait()
            cp_wsp(i, 1).wait()

    def p2_step(i):
        bg = _Background()

        def freq_gen(half, a):
            for r in range(P // 16):
                re = pl.ds(r * 16, 16)
                im = pl.ds(P + r * 16, 16)
                for l in range(D // L):
                    lanes = slice(l * L, (l + 1) * L)
                    ar = ai = None
                    for c in range(a + 1):
                        xr = X_v[c, re, lanes]
                        xi = X_v[c, im, lanes]
                        gr = G_v[a - c, re, lanes]
                        gi = G_v[a - c, im, lanes]
                        pr = xr * gr - xi * gi
                        pi = xr * gi + xi * gr
                        ar = pr if ar is None else ar + pr
                        ai = pi if ai is None else ai + pi
                        if c == a:
                            Z_v[a, re, lanes] = ar.astype(BF16)
                            Z_v[a, im, lanes] = ai.astype(BF16)
                        yield 16

        def tail_piece(m, n):
            a = _blocks_of_step(i - 1)[m // 2]
            sub = (m % 2) * MC
            rows = pl.ds(a * P + sub, MC)
            lanes = slice(n * L, (n + 1) * L)
            hh = _dot(u_v[rows, :], wout_v[:, lanes]) * 0.25
            y = _dot(Fi_v[sub:sub + MC, :], Z_v[a, :, lanes])
            gate = hh + hh * jnp.tanh(hh)
            s = xn_v[rows, lanes].astype(F32) * y
            o_v[rows, lanes] = (x_v[rows, lanes].astype(F32) + s * gate).astype(BF16)

        pending = [(m, n) for m in range(TM // MC) for n in range(D // L)] if i > 0 else []
        if i == 0:
            x_dft(NT - 1)
        if i < NT:
            blocks = _blocks_of_step(i)
            for half, a in enumerate(blocks):
                bg.add(freq_gen(half, a))
            KG = 512
            big_budget = 96.0 if i > 0 else 114.0
            t = 0
            for m in range(TM // MC):
                rows = pl.ds(blocks[m // 2] * P + (m % 2) * MC, MC)
                for n in range(FH // L):
                    acc = None
                    for kg in range(S // KG):
                        p = _dot(wsp_v[i * TM + m * MC:i * TM + (m + 1) * MC, kg * KG:(kg + 1) * KG],
                                 z2_v[kg * KG:(kg + 1) * KG, n * L:(n + 1) * L])
                        acc = p if acc is None else acc + p
                        bg.run(big_budget)
                    u_v[rows, n * L:(n + 1) * L] = (
                        z1_v[rows, n * L:(n + 1) * L] * (acc + bcol_v[rows, :])).astype(BF16)
                    t += 1
                    if pending and t >= 2:
                        tail_piece(*pending.pop(0))
                        bg.run(90)
        bg.drain()
        for t_ in pending:
            tail_piece(*t_)

    for i in range(NT + 1):
        p2_dma(i)
        block(lambda i=i: p2_step(i))
    for a in _blocks_of_step(NT - 1):
        cp_out(a).start()
    for a in range(NB):
        cp_out(a).wait()


@jax.jit
def pallas_recurrent_scan__ssm_conv_h3__mixer_gmlp__prompt_kernel(
    A_q: jax.Array,
    A_k: jax.Array,
    A_v: jax.Array,
    A_shift_k: jax.Array,
    A_ssm_k: jax.Array,
    A_ssm_D: jax.Array,
    B_x: jax.Array,
    B_w_in: jax.Array,
    B_w_sp: jax.Array,
    B_b_sp: jax.Array,
    B_w_out: jax.Array,
):
    del B_x
    hbm = pl.BlockSpec(memory_space=pl.ANY)
    vmem = pl.BlockSpec(memory_space=pltpu.VMEM)

    def bf16_buf(*shape):
        return pltpu.VMEM(shape[:-2] + (shape[-2] // 2, shape[-1]), U32)

    return pl.pallas_call(
        _kernel,
        out_shape=jax.ShapeDtypeStruct((1, S, D), BF16),
        in_specs=[pl.BlockSpec(memory_space=pltpu.SMEM), hbm, hbm, hbm, vmem, hbm, vmem, hbm, hbm, vmem, hbm],
        out_specs=hbm,
        scratch_shapes=[
            bf16_buf(S, D),
            bf16_buf(S + 16, D),
            bf16_buf(S, D),
            bf16_buf(NT, D, TM),
            bf16_buf(D, 2 * FH),
            bf16_buf(S, S),
            bf16_buf(FH, D),
            pltpu.VMEM((S, D), BF16),
            bf16_buf(S, D),
            pltpu.VMEM((S, FH), F32),
            bf16_buf(S, FH),
            bf16_buf(S, D),
            bf16_buf(S, FH),
            pltpu.VMEM((NB, 2 * P, D), F32),
            pltpu.VMEM((2 * P, D), F32),
            pltpu.VMEM((NB, 2 * P, D), F32),
            bf16_buf(NB, 2 * P, D),
            bf16_buf(2 * P, P),
            bf16_buf(P, 2 * P),
            pltpu.VMEM((S, L), F32),
            pltpu.VMEM((4, 8, D), F32),
            pltpu.SemaphoreType.DMA((6, NT)),
            pltpu.SemaphoreType.DMA((2,)),
            pltpu.SemaphoreType.DMA((NB,)),
        ],
        compiler_params=pltpu.CompilerParams(vmem_limit_bytes=100 * 1024 * 1024),
    )(jnp.ones((1,), jnp.int32), A_q, A_k, A_v, A_shift_k.T, A_ssm_k, A_ssm_D, B_w_in, B_w_sp, B_b_sp, B_w_out)
```

```python
import math

import jax
import jax.numpy as jnp
import jax.experimental.pallas as pl
import jax.experimental.pallas.tpu as pltpu

S = 2048
D = 640
FH = 768
P = 128
NB = S // P
TM = 256
NT = S // TM
MC = 64
L = 128
EPS = 1e-5
F32 = jnp.float32
BF16 = jnp.bfloat16
U32 = jnp.uint32
GELU_C = math.sqrt(2.0 / math.pi)
NT_DIMS = (((1,), (1,)), ((), ()))


def _dot(a, b):
    return jnp.dot(a, b, preferred_element_type=F32)


def _dft_angle(shape, k_dim, n_dim):
    r = jax.lax.broadcasted_iota(jnp.int32, shape, k_dim)
    n = jax.lax.broadcasted_iota(jnp.int32, shape, n_dim)
    odd2 = jnp.where(r < 64, 4 * r + 1, 4 * r - 253)
    m = (odd2 * n) & 511
    return m.astype(F32) * (2.0 * math.pi / 512.0)


def _gelu2(z):
    u = z * (GELU_C + (GELU_C * 0.044715) * (z * z))
    return z + z * jnp.tanh(u)


def _ln(x, eps):
    n = x.shape[-1]
    m = jnp.sum(x, axis=-1, keepdims=True) * (1.0 / n)
    xc = x - m
    v = jnp.sum(xc * xc, axis=-1, keepdims=True) * (1.0 / n)
    return xc * jax.lax.rsqrt(v + eps)


def _blocks_of_step(i):
    return (NT - 1 - i, NT + i)


class _Background:
    def __init__(self):
        self.q = []
        self.credit = 0.0

    def add(self, gen):
        self.q.append(gen)

    def run(self, budget):
        self.credit += budget
        while self.q and self.credit > 0:
            try:
                self.credit -= next(self.q[0])
            except StopIteration:
                self.q.pop(0)
        if not self.q:
            self.credit = 0.0

    def drain(self):
        while self.q:
            self.run(1e9)


def _kernel(one_ref, q_hbm, k_hbm, v_hbm, sk_ref, h_hbm, d_ref, win_hbm, wsp_hbm, b_ref, wout_hbm,
            o_hbm,
            x_u, k_u, v_u, h_u, win_u, wsp_u, wout_u, o_v,
            xn_u, z1_v, z2_u, kv_u, u_u, X_v, H_v, G_v, Z_u, F_u, Fi_u, bcol_v, sk_v, kf_v,
            sem_in, sem_w, sem_out):
    x_v, k_v, v_v, h_v, win_v, wsp_v, wout_v, xn_v, z2_v, kv_v, u_v, Z_v, F_v, Fi_v = [
        r.bitcast(BF16) for r in (x_u, k_u, v_u, h_u, win_u, wsp_u, wout_u, xn_u, z2_u, kv_u, u_u, Z_u, F_u, Fi_u)]

    def cp_x(i):
        return pltpu.make_async_copy(q_hbm.at[0, pl.ds(i * TM, TM)], x_v.at[pl.ds(i * TM, TM)], sem_in.at[0, i])

    def cp_k(i):
        return pltpu.make_async_copy(k_hbm.at[0, pl.ds(i * TM, TM)], k_v.at[pl.ds(i * TM, TM)], sem_in.at[1, i])

    def cp_v(i):
        return pltpu.make_async_copy(v_hbm.at[0, pl.ds(i * TM, TM)], v_v.at[pl.ds(i * TM, TM)], sem_in.at[2, i])

    def cp_h(i):
        return pltpu.make_async_copy(h_hbm.at[:, pl.ds(i * TM, TM)], h_v.at[i], sem_in.at[3, i])

    def cp_wsp(i, half):
        a = _blocks_of_step(i)[half]
        return pltpu.make_async_copy(wsp_hbm.at[pl.ds(a * P, P)], wsp_v.at[pl.ds(i * TM + half * P, P)],
                                     sem_in.at[4 + half, i])

    def cp_win():
        return pltpu.make_async_copy(win_hbm, win_v, sem_w.at[0])

    def cp_wout():
        return pltpu.make_async_copy(wout_hbm, wout_v, sem_w.at[1])

    def cp_out(a):
        return pltpu.make_async_copy(o_v.at[pl.ds(a * P, P)], o_hbm.at[0, pl.ds(a * P, P)], sem_out.at[a])

    def block(fn):
        pl.when(one_ref[0] == 1)(fn)

    def ln_x(i):
        for s in range(TM // 16):
            rows = pl.ds(i * TM + s * 16, 16)
            xn_v[rows, :] = _ln(x_v[rows, :].astype(F32), EPS).astype(BF16)
            yield 80

    def x_dft(i, bg):
        for half in range(2):
            j = 2 * i + half
            for part in range(2):
                X_v[j, part * P:(part + 1) * P, :] = _dot(F_v[part * P:(part + 1) * P, 0:P],
                                                          kv_v[j * P:(j + 1) * P, :])
                bg.run(150)

    cp_x(0).start()
    cp_h(0).start()
    cp_win().start()
    cp_x(1).start()
    cp_k(0).start()
    cp_v(0).start()

    ang = _dft_angle((P, P), 0, 1)
    F_v[0:P, 0:P] = jnp.cos(ang).astype(BF16)
    F_v[P:2 * P, 0:P] = (-jnp.sin(ang)).astype(BF16)
    angt = _dft_angle((P, P), 1, 0)
    Fi_v[:, 0:P] = (jnp.cos(angt) * (1.0 / P)).astype(BF16)
    Fi_v[:, P:2 * P] = (jnp.sin(angt) * (-1.0 / P)).astype(BF16)

    brow = b_ref[...].astype(F32).reshape(1, S)
    for j in range(NB):
        bcol_v[j * P:(j + 1) * P, :] = jnp.broadcast_to(brow[:, j * P:(j + 1) * P], (P, P)).T
    drow = d_ref[...].astype(F32).reshape(1, D)
    sk = sk_ref[...].astype(F32)
    for t in range(4):
        sk_v[t] = jnp.broadcast_to(sk[t:t + 1], (8, D))

    kf_v[:, 0:8, :] = jnp.zeros((D // L, 8, L), F32)
    H_v[0:P, :] = jnp.zeros((P, D), F32)
    H_v[P:P + 64, :] = jnp.broadcast_to(-drow, (64, D))
    H_v[P + 64:2 * P, :] = jnp.broadcast_to(drow, (64, D))
    cp_x(0).wait()
    for _ in ln_x(0):
        pass

    def p1_dma(i):
        if i + 1 < NT:
            cp_h(i + 1).start()
            cp_k(i + 1).start()
            cp_v(i + 1).start()
        if i + 2 < NT:
            cp_x(i + 2).start()
        if i >= 5:
            cp_wsp(i - 5, 0).start()
            cp_wsp(i - 5, 1).start()
        if i == 3:
            cp_wout().start()
        if i == 0:
            cp_win().wait()
        cp_h(i).wait()
        cp_k(i).wait()
        cp_v(i).wait()
        if i + 1 < NT:
            cp_x(i + 1).wait()

    def p1_step(i):
        r0 = i * TM
        bg = _Background()

        def kv_gen():
            for m in range(TM // MC):
                r = r0 + m * MC
                for l in range(D // L):
                    lanes = slice(l * L, (l + 1) * L)
                    kf = k_v[pl.ds(r, MC), lanes].astype(F32)
                    kf_v[l, pl.ds(r + 8, MC), :] = kf
                    ks = kf * sk_v[0, 0:1, lanes]
                    for t in range(1, 4):
                        ks = ks + kf_v[l, pl.ds(r + 8 - t, MC), :] * sk_v[t, 0:1, lanes]
                    kv = ks * v_v[pl.ds(r, MC), lanes].astype(F32)
                    kv_v[pl.ds(r, MC), lanes] = kv.astype(BF16)
                    yield 90

        def ln_z2(m, tiles, s1, s2):
            mean = jnp.sum(s1, axis=-1, keepdims=True) * (1.0 / FH)
            ex2 = jnp.sum(s2, axis=-1, keepdims=True) * (1.0 / FH)
            var = jnp.maximum(ex2 - mean * mean, 0.0)
            rs = jax.lax.rsqrt(var + 4.0 * EPS)
            for n in range(FH // L):
                z2_v[pl.ds(r0 + m * MC, MC), n * L:(n + 1) * L] = ((tiles[n] - mean) * rs).astype(BF16)

        if i + 1 < NT:
            bg.add(ln_x(i + 1))
        bg.add(kv_gen())

        prev = [H_v[qd * 64:(qd + 1) * 64, :] for qd in range(4)]
        for half in range(2):
            j = 2 * i + half
            cur = []
            for part in range(2):
                hp = jax.lax.dot_general(F_v[part * P:(part + 1) * P, 0:P], h_v[i, :, half * P:(half + 1) * P],
                                         NT_DIMS, preferred_element_type=F32)
                for qd in (2 * part, 2 * part + 1):
                    hq = hp[(qd % 2) * 64:(qd % 2 + 1) * 64]
                    cur.append(hq)
                    other = prev[(qd + 2) % 4]
                    G_v[j, qd * 64:(qd + 1) * 64, :] = hq - other if qd in (0, 3) else hq + other
                bg.run(150)
            prev = cur
        if i + 1 < NT:
            for qd in range(4):
                H_v[qd * 64:(qd + 1) * 64, :] = prev[qd]

        for m in range(TM // MC):
            rows = pl.ds(r0 + m * MC, MC)
            tiles = []
            s1 = s2 = None
            for n in range(FH // L):
                z = _gelu2(_dot(xn_v[rows, :], win_v[:, FH + n * L:FH + (n + 1) * L]))
                tiles.append(z)
                s1 = z if s1 is None else s1 + z
                s2 = z * z if s2 is None else s2 + z * z
                bg.run(75)
            ln_z2(m, tiles, s1, s2)
            for n in range(FH // L):
                z1_v[rows, n * L:(n + 1) * L] = _gelu2(_dot(xn_v[rows, :], win_v[:, n * L:(n + 1) * L]))
                bg.run((0, 0, 0, 40, 75, 75)[n])
        if i > 0:
            x_dft(i - 1, bg)
        bg.drain()

    for i in range(NT):
        p1_dma(i)
        block(lambda i=i: p1_step(i))

    def p2_dma(i):
        if i == 0:
            cp_wout().wait()
        if i >= 2:
            for a in _blocks_of_step(i - 2):
                cp_out(a).start()
        if i + 3 < NT:
            cp_wsp(i + 3, 0).start()
            cp_wsp(i + 3, 1).start()
        if i < NT:
            cp_wsp(i, 0).wait()
            cp_wsp(i, 1).wait()

    def p2_step(i):
        bg = _Background()

        def freq_gen(half, a):
            for r in range(P // 16):
                re = pl.ds(r * 16, 16)
                im = pl.ds(P + r * 16, 16)
                for l in range(D // L):
                    lanes = slice(l * L, (l + 1) * L)
                    ar = ai = None
                    for c in range(a + 1):
                        xr = X_v[c, re, lanes]
                        xi = X_v[c, im, lanes]
                        gr = G_v[a - c, re, lanes]
                        gi = G_v[a - c, im, lanes]
                        pr = xr * gr - xi * gi
                        pi = xr * gi + xi * gr
                        ar = pr if ar is None else ar + pr
                        ai = pi if ai is None else ai + pi
                        if c == a:
                            Z_v[a, re, lanes] = ar.astype(BF16)
                            Z_v[a, im, lanes] = ai.astype(BF16)
                        yield 16

        def tail_piece(m, n):
            a = _blocks_of_step(i - 1)[m // 2]
            sub = (m % 2) * MC
            rows = pl.ds(a * P + sub, MC)
            lanes = slice(n * L, (n + 1) * L)
            hh = _dot(u_v[rows, :], wout_v[:, lanes]) * 0.25
            y = _dot(Fi_v[sub:sub + MC, :], Z_v[a, :, lanes])
            gate = hh + hh * jnp.tanh(hh)
            s = xn_v[rows, lanes].astype(F32) * y
            o_v[rows, lanes] = (x_v[rows, lanes].astype(F32) + s * gate).astype(BF16)

        pending = [(m, n) for m in range(TM // MC) for n in range(D // L)] if i > 0 else []
        if i < NT:
            blocks = _blocks_of_step(i)
            for half, a in enumerate(blocks):
                bg.add(freq_gen(half, a))
            if i == 0:
                x_dft(NT - 1, bg)
            KG = 512
            big_budget = 96.0 if i > 0 else 108.0
            t = 0
            for m in range(TM // MC):
                rows = pl.ds(blocks[m // 2] * P + (m % 2) * MC, MC)
                for n in range(FH // L):
                    acc = None
                    for kg in range(S // KG):
                        p = _dot(wsp_v[i * TM + m * MC:i * TM + (m + 1) * MC, kg * KG:(kg + 1) * KG],
                                 z2_v[kg * KG:(kg + 1) * KG, n * L:(n + 1) * L])
                        acc = p if acc is None else acc + p
                        bg.run(big_budget)
                    u_v[rows, n * L:(n + 1) * L] = (
                        z1_v[rows, n * L:(n + 1) * L] * (acc + bcol_v[rows, :])).astype(BF16)
                    t += 1
                    if pending and t >= 2:
                        tail_piece(*pending.pop(0))
                        bg.run(90)
        bg.drain()
        for t_ in pending:
            tail_piece(*t_)

    for i in range(NT + 1):
        p2_dma(i)
        block(lambda i=i: p2_step(i))
    for a in _blocks_of_step(NT - 1):
        cp_out(a).start()
    for a in range(NB):
        cp_out(a).wait()


@jax.jit
def pallas_recurrent_scan__ssm_conv_h3__mixer_gmlp__prompt_kernel(
    A_q: jax.Array,
    A_k: jax.Array,
    A_v: jax.Array,
    A_shift_k: jax.Array,
    A_ssm_k: jax.Array,
    A_ssm_D: jax.Array,
    B_x: jax.Array,
    B_w_in: jax.Array,
    B_w_sp: jax.Array,
    B_b_sp: jax.Array,
    B_w_out: jax.Array,
):
    del B_x
    hbm = pl.BlockSpec(memory_space=pl.ANY)
    vmem = pl.BlockSpec(memory_space=pltpu.VMEM)

    def bf16_buf(*shape):
        return pltpu.VMEM(shape[:-2] + (shape[-2] // 2, shape[-1]), U32)

    return pl.pallas_call(
        _kernel,
        out_shape=jax.ShapeDtypeStruct((1, S, D), BF16),
        in_specs=[pl.BlockSpec(memory_space=pltpu.SMEM), hbm, hbm, hbm, vmem, hbm, vmem, hbm, hbm, vmem, hbm],
        out_specs=hbm,
        scratch_shapes=[
            bf16_buf(S, D),
            bf16_buf(S, D),
            bf16_buf(S, D),
            bf16_buf(NT, D, TM),
            bf16_buf(D, 2 * FH),
            bf16_buf(S, S),
            bf16_buf(FH, D),
            pltpu.VMEM((S, D), BF16),
            bf16_buf(S, D),
            pltpu.VMEM((S, FH), F32),
            bf16_buf(S, FH),
            bf16_buf(S, D),
            bf16_buf(S, FH),
            pltpu.VMEM((NB, 2 * P, D), F32),
            pltpu.VMEM((2 * P, D), F32),
            pltpu.VMEM((NB, 2 * P, D), F32),
            bf16_buf(NB, 2 * P, D),
            bf16_buf(2 * P, 2 * P),
            bf16_buf(P, 2 * P),
            pltpu.VMEM((S, L), F32),
            pltpu.VMEM((4, 8, D), F32),
            pltpu.VMEM((D // L, S + 8, L), F32),
            pltpu.SemaphoreType.DMA((6, NT)),
            pltpu.SemaphoreType.DMA((2,)),
            pltpu.SemaphoreType.DMA((NB,)),
        ],
        compiler_params=pltpu.CompilerParams(vmem_limit_bytes=100 * 1024 * 1024),
    )(jnp.ones((1,), jnp.int32), A_q, A_k, A_v, A_shift_k.T, A_ssm_k, A_ssm_D, B_w_in, B_w_sp, B_b_sp, B_w_out)
```

```python
import math

import jax
import jax.numpy as jnp
import jax.experimental.pallas as pl
import jax.experimental.pallas.tpu as pltpu

S = 2048
D = 640
FH = 768
P = 128
NB = S // P
TM = 256
NT = S // TM
MC = 64
L = 128
EPS = 1e-5
F32 = jnp.float32
BF16 = jnp.bfloat16
U32 = jnp.uint32
GELU_C = math.sqrt(2.0 / math.pi)
NT_DIMS = (((1,), (1,)), ((), ()))


def _dot(a, b):
    return jnp.dot(a, b, preferred_element_type=F32)


def _dft_angle(shape, k_dim, n_dim):
    r = jax.lax.broadcasted_iota(jnp.int32, shape, k_dim)
    n = jax.lax.broadcasted_iota(jnp.int32, shape, n_dim)
    odd2 = jnp.where(r < 64, 4 * r + 1, 4 * r - 253)
    m = (odd2 * n) & 511
    return m.astype(F32) * (2.0 * math.pi / 512.0)


def _gelu2(z):
    u = z * (GELU_C + (GELU_C * 0.044715) * (z * z))
    return z + z * jnp.tanh(u)


def _ln(x, eps):
    n = x.shape[-1]
    m = jnp.sum(x, axis=-1, keepdims=True) * (1.0 / n)
    xc = x - m
    v = jnp.sum(xc * xc, axis=-1, keepdims=True) * (1.0 / n)
    return xc * jax.lax.rsqrt(v + eps)


def _blocks_of_step(i):
    return (NT - 1 - i, NT + i)


class _Background:
    def __init__(self):
        self.q = []
        self.credit = 0.0

    def add(self, gen):
        self.q.append(gen)

    def run(self, budget):
        self.credit += budget
        while self.q and self.credit > 0:
            try:
                self.credit -= next(self.q[0])
            except StopIteration:
                self.q.pop(0)
        if not self.q:
            self.credit = 0.0

    def drain(self):
        while self.q:
            self.run(1e9)


def _kernel(one_ref, q_hbm, k_hbm, v_hbm, sk_ref, h_hbm, d_ref, win_hbm, wsp_hbm, b_ref, wout_hbm,
            o_hbm,
            x_u, k_u, v_u, h_u, win_u, wsp_u, wout_u, o_v,
            xn_u, z1_v, z2_u, kv_u, u_u, X_v, H_v, G_v, Z_u, F_u, Fi_u, bcol_v, sk_v, kf_v,
            sem_in, sem_w, sem_out):
    x_v, k_v, v_v, h_v, win_v, wsp_v, wout_v, xn_v, z2_v, kv_v, u_v, Z_v, F_v, Fi_v = [
        r.bitcast(BF16) for r in (x_u, k_u, v_u, h_u, win_u, wsp_u, wout_u, xn_u, z2_u, kv_u, u_u, Z_u, F_u, Fi_u)]

    def cp_x(i):
        return pltpu.make_async_copy(q_hbm.at[0, pl.ds(i * TM, TM)], x_v.at[pl.ds(i * TM, TM)], sem_in.at[0, i])

    def cp_k(i):
        return pltpu.make_async_copy(k_hbm.at[0, pl.ds(i * TM, TM)], k_v.at[pl.ds(i * TM, TM)], sem_in.at[1, i])

    def cp_v(i):
        return pltpu.make_async_copy(v_hbm.at[0, pl.ds(i * TM, TM)], v_v.at[pl.ds(i * TM, TM)], sem_in.at[2, i])

    def cp_h(i):
        return pltpu.make_async_copy(h_hbm.at[:, pl.ds(i * TM, TM)], h_v.at[i], sem_in.at[3, i])

    def cp_wsp(i, half):
        a = _blocks_of_step(i)[half]
        return pltpu.make_async_copy(wsp_hbm.at[pl.ds(a * P, P)], wsp_v.at[pl.ds(i * TM + half * P, P)],
                                     sem_in.at[4 + half, i])

    def cp_win(half):
        cols = pl.ds(half * FH, FH)
        return pltpu.make_async_copy(win_hbm.at[:, cols], win_v.at[:, cols], sem_w.at[half])

    def cp_wout():
        return pltpu.make_async_copy(wout_hbm, wout_v, sem_w.at[2])

    def cp_out(a):
        return pltpu.make_async_copy(o_v.at[pl.ds(a * P, P)], o_hbm.at[0, pl.ds(a * P, P)], sem_out.at[a])

    def block(fn):
        pl.when(one_ref[0] == 1)(fn)

    def ln_x(t):
        for s in range(TM // 16):
            rows = pl.ds(t * TM + s * 16, 16)
            xn_v[rows, :] = _ln(x_v[rows, :].astype(F32), EPS).astype(BF16)
            yield 80

    def kv_gen(t):
        for m in range(TM // MC):
            r = t * TM + m * MC
            for l in range(D // L):
                lanes = slice(l * L, (l + 1) * L)
                kf = k_v[pl.ds(r, MC), lanes].astype(F32)
                kf_v[l, pl.ds(r + 8, MC), :] = kf
                ks = kf * sk_v[0, 0:1, lanes]
                for tap in range(1, 4):
                    ks = ks + kf_v[l, pl.ds(r + 8 - tap, MC), :] * sk_v[tap, 0:1, lanes]
                kv = ks * v_v[pl.ds(r, MC), lanes].astype(F32)
                kv_v[pl.ds(r, MC), lanes] = kv.astype(BF16)
                yield 90

    def freq_gen(a):
        for r in range(P // 16):
            re = pl.ds(r * 16, 16)
            im = pl.ds(P + r * 16, 16)
            for l in range(D // L):
                lanes = slice(l * L, (l + 1) * L)
                ar = ai = None
                for c in range(a + 1):
                    xr = X_v[c, re, lanes]
                    xi = X_v[c, im, lanes]
                    gr = G_v[a - c, re, lanes]
                    gi = G_v[a - c, im, lanes]
                    pr = xr * gr - xi * gi
                    pi = xr * gi + xi * gr
                    ar = pr if ar is None else ar + pr
                    ai = pi if ai is None else ai + pi
                    if c == a:
                        Z_v[a, re, lanes] = ar.astype(BF16)
                        Z_v[a, im, lanes] = ai.astype(BF16)
                    yield 16

    def job_h(t, bg, budget):
        prev = [H_v[qd * 64:(qd + 1) * 64, :] for qd in range(4)]
        for half in range(2):
            j = 2 * t + half
            cur = []
            for part in range(2):
                hp = jax.lax.dot_general(F_v[part * P:(part + 1) * P, 0:P], h_v[t, :, half * P:(half + 1) * P],
                                         NT_DIMS, preferred_element_type=F32)
                for qd in (2 * part, 2 * part + 1):
                    hq = hp[(qd % 2) * 64:(qd % 2 + 1) * 64]
                    cur.append(hq)
                    other = prev[(qd + 2) % 4]
                    G_v[j, qd * 64:(qd + 1) * 64, :] = hq - other if qd in (0, 3) else hq + other
                bg.run(budget)
            prev = cur
        if t + 1 < NT:
            for qd in range(4):
                H_v[qd * 64:(qd + 1) * 64, :] = prev[qd]

    def job_x(t, bg, budget):
        for half in range(2):
            j = 2 * t + half
            for part in range(2):
                X_v[j, part * P:(part + 1) * P, :] = _dot(F_v[part * P:(part + 1) * P, 0:P],
                                                          kv_v[j * P:(j + 1) * P, :])
                bg.run(budget)

    def job_z2(t, m, bg, budgets):
        rows = pl.ds(t * TM + m * MC, MC)
        tiles = []
        s1 = s2 = None
        for n in range(FH // L):
            z = _gelu2(_dot(xn_v[rows, :], win_v[:, FH + n * L:FH + (n + 1) * L]))
            tiles.append(z)
            s1 = z if s1 is None else s1 + z
            s2 = z * z if s2 is None else s2 + z * z
            bg.run(budgets[n])
        mean = jnp.sum(s1, axis=-1, keepdims=True) * (1.0 / FH)
        ex2 = jnp.sum(s2, axis=-1, keepdims=True) * (1.0 / FH)
        var = jnp.maximum(ex2 - mean * mean, 0.0)
        rs = jax.lax.rsqrt(var + 4.0 * EPS)
        for n in range(FH // L):
            z2_v[rows, n * L:(n + 1) * L] = ((tiles[n] - mean) * rs).astype(BF16)

    def job_z1(t, m, bg, budgets):
        rows = pl.ds(t * TM + m * MC, MC)
        for n in range(FH // L):
            z1_v[rows, n * L:(n + 1) * L] = _gelu2(_dot(xn_v[rows, :], win_v[:, n * L:(n + 1) * L]))
            bg.run(budgets[n])

    def tail_piece(a, sub, n):
        rows = pl.ds(a * P + sub, MC)
        lanes = slice(n * L, (n + 1) * L)
        hh = _dot(u_v[rows, :], wout_v[:, lanes]) * 0.25
        y = _dot(Fi_v[sub:sub + MC, :], Z_v[a, :, lanes])
        gate = hh + hh * jnp.tanh(hh)
        s = xn_v[rows, lanes].astype(F32) * y
        o_v[rows, lanes] = (x_v[rows, lanes].astype(F32) + s * gate).astype(BF16)

    def job_big(i, bg, pending, budget):
        blocks = _blocks_of_step(i)
        KG = 512
        t = 0
        for m in range(TM // MC):
            rows = pl.ds(blocks[m // 2] * P + (m % 2) * MC, MC)
            for n in range(FH // L):
                acc = None
                for kg in range(S // KG):
                    p = _dot(wsp_v[i * TM + m * MC:i * TM + (m + 1) * MC, kg * KG:(kg + 1) * KG],
                             z2_v[kg * KG:(kg + 1) * KG, n * L:(n + 1) * L])
                    acc = p if acc is None else acc + p
                    bg.run(budget)
                u_v[rows, n * L:(n + 1) * L] = (
                    z1_v[rows, n * L:(n + 1) * L] * (acc + bcol_v[rows, :])).astype(BF16)
                t += 1
                if pending and t >= 2:
                    tail_piece(*pending.pop(0))
                    bg.run(budget)

    cp_x(0).start()
    cp_win(1).start()

    ang = _dft_angle((P, P), 0, 1)
    F_v[0:P, 0:P] = jnp.cos(ang).astype(BF16)
    F_v[P:2 * P, 0:P] = (-jnp.sin(ang)).astype(BF16)
    angt = _dft_angle((P, P), 1, 0)
    Fi_v[:, 0:P] = (jnp.cos(angt) * (1.0 / P)).astype(BF16)
    Fi_v[:, P:2 * P] = (jnp.sin(angt) * (-1.0 / P)).astype(BF16)

    brow = b_ref[...].astype(F32).reshape(1, S)
    for j in range(NB):
        bcol_v[j * P:(j + 1) * P, :] = jnp.broadcast_to(brow[:, j * P:(j + 1) * P], (P, P)).T
    drow = d_ref[...].astype(F32).reshape(1, D)
    sk = sk_ref[...].astype(F32)
    for t in range(4):
        sk_v[t] = jnp.broadcast_to(sk[t:t + 1], (8, D))
    kf_v[:, 0:8, :] = jnp.zeros((D // L, 8, L), F32)
    H_v[0:P, :] = jnp.zeros((P, D), F32)
    H_v[P:P + 64, :] = jnp.broadcast_to(-drow, (64, D))
    H_v[P + 64:2 * P, :] = jnp.broadcast_to(drow, (64, D))

    cp_x(0).wait()
    cp_win(0).start()
    cp_x(1).start()
    for _ in ln_x(0):
        pass

    LAG = 2

    def conv_dma(g):
        t = g - LAG
        if 0 <= t + 1 < NT:
            cp_h(t + 1).start()
            cp_k(t + 1).start()
            cp_v(t + 1).start()
        if 0 <= t < NT:
            cp_h(t).wait()
            cp_k(t).wait()
            cp_v(t).wait()

    def p1_first_a():
        bg = _Background()
        for m in range(TM // MC):
            job_z2(0, m, bg, (0,) * 6)

    def p1_first_b():
        bg = _Background()
        bg.add(ln_x(1))
        for m in range(TM // MC):
            job_z1(0, m, bg, (60,) * 6)
        bg.drain()

    cp_win(1).wait()
    cp_x(2).start()
    block(p1_first_a)
    cp_win(0).wait()
    cp_x(1).wait()
    block(p1_first_b)

    def p1_dma(i):
        if i + 2 < NT:
            cp_x(i + 2).start()
        if i >= 5:
            cp_wsp(i - 5, 0).start()
            cp_wsp(i - 5, 1).start()
        if i == 3:
            cp_wout().start()
        conv_dma(i)
        if i + 1 < NT:
            cp_x(i + 1).wait()

    def p1_step(i):
        bg = _Background()
        if i + 1 < NT:
            bg.add(ln_x(i + 1))
        t = i - LAG
        if t >= 0:
            bg.add(kv_gen(t))
            job_h(t, bg, 150)
        for m in range(TM // MC):
            job_z2(i, m, bg, (75,) * 6)
            job_z1(i, m, bg, (0, 0, 0, 40, 75, 75))
        if t >= 1:
            job_x(t - 1, bg, 150)
        bg.drain()

    for i in range(1, NT):
        p1_dma(i)
        block(lambda i=i: p1_step(i))

    def p2_dma(i):
        if i == 0:
            cp_wout().wait()
        if i >= 2:
            for a in _blocks_of_step(i - 2):
                cp_out(a).start()
        if i >= 3:
            for a in _blocks_of_step(i - 3):
                cp_out(a).wait()
        if i + 3 < NT:
            cp_wsp(i + 3, 0).start()
            cp_wsp(i + 3, 1).start()
        conv_dma(NT + i)
        if i < NT:
            cp_wsp(i, 0).wait()
            cp_wsp(i, 1).wait()

    def tails_of(i):
        return [(a, sub, n) for a in _blocks_of_step(i) for sub in (0, MC) for n in range(D // L)]

    def p2_step(i):
        bg = _Background()
        pending = tails_of(i - 1) if i > 0 else []
        total = 17 * 40 * 16
        slots = 96 + len(pending)
        t = NT + i - LAG
        if t < NT:
            bg.add(kv_gen(t))
            total += 20 * 90
            slots += 8
        if t - 1 < NT:
            slots += 8
        for a in _blocks_of_step(i):
            bg.add(freq_gen(a))
        budget = total / (slots - 2.0)
        if t < NT:
            job_h(t, bg, 2 * budget)
        if t - 1 < NT:
            job_x(t - 1, bg, 2 * budget)
        job_big(i, bg, pending, budget)
        bg.drain()
        for t_ in pending:
            tail_piece(*t_)

    for i in range(NT):
        p2_dma(i)
        block(lambda i=i: p2_step(i))

    def p2_last():
        a0, a1 = _blocks_of_step(NT - 1)
        for t_ in tails_of(NT - 1):
            tail_piece(*t_)
            if t_ == (a0, MC, D // L - 1):
                cp_out(a0).start()

    p2_dma(NT)
    block(p2_last)
    cp_out(_blocks_of_step(NT - 1)[1]).start()
    for i in (NT - 2, NT - 1):
        for a in _blocks_of_step(i):
            cp_out(a).wait()


@jax.jit
def pallas_recurrent_scan__ssm_conv_h3__mixer_gmlp__prompt_kernel(
    A_q: jax.Array,
    A_k: jax.Array,
    A_v: jax.Array,
    A_shift_k: jax.Array,
    A_ssm_k: jax.Array,
    A_ssm_D: jax.Array,
    B_x: jax.Array,
    B_w_in: jax.Array,
    B_w_sp: jax.Array,
    B_b_sp: jax.Array,
    B_w_out: jax.Array,
):
    del B_x
    hbm = pl.BlockSpec(memory_space=pl.ANY)
    vmem = pl.BlockSpec(memory_space=pltpu.VMEM)

    def bf16_buf(*shape):
        return pltpu.VMEM(shape[:-2] + (shape[-2] // 2, shape[-1]), U32)

    return pl.pallas_call(
        _kernel,
        out_shape=jax.ShapeDtypeStruct((1, S, D), BF16),
        in_specs=[pl.BlockSpec(memory_space=pltpu.SMEM), hbm, hbm, hbm, vmem, hbm, vmem, hbm, hbm, vmem, hbm],
        out_specs=hbm,
        scratch_shapes=[
            bf16_buf(S, D),
            bf16_buf(S, D),
            bf16_buf(S, D),
            bf16_buf(NT, D, TM),
            bf16_buf(D, 2 * FH),
            bf16_buf(S, S),
            bf16_buf(FH, D),
            pltpu.VMEM((S, D), BF16),
            bf16_buf(S, D),
            pltpu.VMEM((S, FH), F32),
            bf16_buf(S, FH),
            bf16_buf(S, D),
            bf16_buf(S, FH),
            pltpu.VMEM((NB, 2 * P, D), F32),
            pltpu.VMEM((2 * P, D), F32),
            pltpu.VMEM((NB, 2 * P, D), F32),
            bf16_buf(NB, 2 * P, D),
            bf16_buf(2 * P, 2 * P),
            bf16_buf(P, 2 * P),
            pltpu.VMEM((S, L), F32),
            pltpu.VMEM((4, 8, D), F32),
            pltpu.VMEM((D // L, S + 8, L), F32),
            pltpu.SemaphoreType.DMA((6, NT)),
            pltpu.SemaphoreType.DMA((3,)),
            pltpu.SemaphoreType.DMA((NB,)),
        ],
        compiler_params=pltpu.CompilerParams(vmem_limit_bytes=100 * 1024 * 1024),
    )(jnp.ones((1,), jnp.int32), A_q, A_k, A_v, A_shift_k.T, A_ssm_k, A_ssm_D, B_w_in, B_w_sp, B_b_sp, B_w_out)
```

```python
import math

import jax
import jax.numpy as jnp
import jax.experimental.pallas as pl
import jax.experimental.pallas.tpu as pltpu

S = 2048
D = 640
FH = 768
P = 128
NB = S // P
TM = 256
NT = S // TM
MC = 64
L = 128
WC = 384
EPS = 1e-5
F32 = jnp.float32
BF16 = jnp.bfloat16
U32 = jnp.uint32
GELU_C = math.sqrt(2.0 / math.pi)
NT_DIMS = (((1,), (1,)), ((), ()))


def _dot(a, b):
    return jnp.dot(a, b, preferred_element_type=F32)


def _cos_sin(m):
    q = (m + 256) >> 9
    x = (m - (q << 9)).astype(F32) * (2.0 * math.pi / 2048.0)
    x2 = x * x
    s = x * (1.0 + x2 * (-1.0 / 6 + x2 * (1.0 / 120 + x2 * (-1.0 / 5040 + x2 * (1.0 / 362880)))))
    c = 1.0 + x2 * (-0.5 + x2 * (1.0 / 24 + x2 * (-1.0 / 720 + x2 * (1.0 / 40320 - x2 * (1.0 / 3628800)))))
    swap = (q & 1) == 1
    c0 = jnp.where(swap, s, c)
    s0 = jnp.where(swap, c, s)
    cos = jnp.where(((q + 1) & 2) == 2, -c0, c0)
    sin = jnp.where((q & 2) == 2, -s0, s0)
    return cos, sin


def _odd_freq(r):
    return jnp.where(r < 64, 4 * r + 1, 4 * r - 253)


def _gelu2(z):
    u = z * (GELU_C + (GELU_C * 0.044715) * (z * z))
    return z + z * jnp.tanh(u)


def _ln(x, eps):
    n = x.shape[-1]
    m = jnp.sum(x, axis=-1, keepdims=True) * (1.0 / n)
    xc = x - m
    v = jnp.sum(xc * xc, axis=-1, keepdims=True) * (1.0 / n)
    return xc * jax.lax.rsqrt(v + eps)


def _blocks_of_step(i):
    return (NT - 1 - i, NT + i)


class _Background:
    def __init__(self):
        self.q = []
        self.credit = 0.0

    def add(self, gen):
        self.q.append(gen)

    def run(self, budget):
        self.credit += budget
        while self.q and self.credit > 0:
            try:
                self.credit -= next(self.q[0])
            except StopIteration:
                self.q.pop(0)
        if not self.q:
            self.credit = 0.0

    def drain(self):
        while self.q:
            self.run(1e9)


def _kernel(one_ref, q_hbm, k_hbm, v_hbm, sk_hbm, h_hbm, d_hbm, win_hbm, wsp_hbm, b_hbm, wout_hbm,
            o_hbm,
            x_u, k_u, v_u, h_u, win_u, wsp_u, wout_u, o_v, sk_in, d_in, b_in,
            xn_u, z1_v, z2_u, zt_v, kv_u, u_u, X_v, H_v, G_v, Z_u, yl_v, F_u, Fi_u, bcol_v, sk_v, kf_v,
            sem_small, sem_x, sem_conv, sem_wsp, sem_w, sem_out):
    x_v, k_v, v_v, h_v, win_v, wsp_v, wout_v, xn_v, z2_v, kv_v, u_v, Z_v, F_v, Fi_v = [
        r.bitcast(BF16) for r in (x_u, k_u, v_u, h_u, win_u, wsp_u, wout_u, xn_u, z2_u, kv_u, u_u, Z_u, F_u,
                                  Fi_u)]

    def cp_small():
        return [pltpu.make_async_copy(s_, d_, sem_small.at[0])
                for s_, d_ in ((d_hbm, d_in), (sk_hbm, sk_in), (b_hbm, b_in))]

    def cp_x(t):
        return pltpu.make_async_copy(q_hbm.at[0, pl.ds(t * TM, TM)], x_v.at[pl.ds(t * TM, TM)], sem_x.at[t % 3])

    def cp_conv(t):
        rows = pl.ds(t * TM, TM)
        sem = sem_conv.at[t % 2]
        return [pltpu.make_async_copy(h_hbm.at[:, rows], h_v.at[t], sem),
                pltpu.make_async_copy(k_hbm.at[0, rows], k_v.at[rows], sem),
                pltpu.make_async_copy(v_hbm.at[0, rows], v_v.at[rows], sem)]

    def cp_wsp(i):
        return [pltpu.make_async_copy(wsp_hbm.at[pl.ds(a * P, P)], wsp_v.at[pl.ds(i * TM + half * P, P)],
                                      sem_wsp.at[i % 4]) for half, a in enumerate(_blocks_of_step(i))]

    def cp_win(c):
        cols = pl.ds(c * WC, WC)
        return pltpu.make_async_copy(win_hbm.at[:, cols], win_v.at[:, cols], sem_w.at[c])

    def cp_wout():
        return pltpu.make_async_copy(wout_hbm, wout_v, sem_w.at[4])

    def cp_out(i):
        return [pltpu.make_async_copy(o_v.at[pl.ds(a * P, P)], o_hbm.at[0, pl.ds(a * P, P)], sem_out.at[i % 3])
                for a in _blocks_of_step(i)]

    def start(cs):
        for c in cs:
            c.start()

    def wait(cs):
        for c in cs:
            c.wait()

    always = one_ref[0] == 1

    def block(fn):
        pl.when(always)(fn)

    def ln_x(t):
        for s in range(TM // 16):
            rows = pl.ds(t * TM + s * 16, 16)
            xn_v[rows, :] = _ln(x_v[rows, :].astype(F32), EPS).astype(BF16)
            yield 80

    def kv_gen(t):
        for m in range(TM // MC):
            r = t * TM + m * MC
            for l in range(D // L):
                lanes = slice(l * L, (l + 1) * L)
                kf = k_v[pl.ds(r, MC), lanes].astype(F32)
                kf_v[l, pl.ds(r + 8, MC), :] = kf
                ks = kf * sk_v[0, 0:1, lanes]
                for tap in range(1, 4):
                    ks = ks + kf_v[l, pl.ds(r + 8 - tap, MC), :] * sk_v[tap, 0:1, lanes]
                kv = ks * v_v[pl.ds(r, MC), lanes].astype(F32)
                kv_v[pl.ds(r, MC), lanes] = kv.astype(BF16)
                yield 90

    def freq_gen(a):
        for r in range(P // 16):
            re = pl.ds(r * 16, 16)
            im = pl.ds(P + r * 16, 16)
            for l in range(D // L):
                lanes = slice(l * L, (l + 1) * L)
                ar = ai = None
                for c in range(a + 1):
                    xr = X_v[c, re, lanes]
                    xi = X_v[c, im, lanes]
                    gr = G_v[a - c, re, lanes]
                    gi = G_v[a - c, im, lanes]
                    pr = xr * gr - xi * gi
                    pi = xr * gi + xi * gr
                    ar = pr if ar is None else ar + pr
                    ai = pi if ai is None else ai + pi
                    if c == a:
                        Z_v[a, re, lanes] = ar.astype(BF16)
                        Z_v[a, im, lanes] = ai.astype(BF16)
                    yield 16

    def job_h(t, bg, budget):
        prev = [H_v[qd * 64:(qd + 1) * 64, :] for qd in range(4)]
        for half in range(2):
            j = 2 * t + half
            cur = []
            for part in range(2):
                hp = jax.lax.dot_general(F_v[part * P:(part + 1) * P, 0:P], h_v[t, :, half * P:(half + 1) * P],
                                         NT_DIMS, preferred_element_type=F32)
                for qd in (2 * part, 2 * part + 1):
                    hq = hp[(qd % 2) * 64:(qd % 2 + 1) * 64]
                    cur.append(hq)
                    other = prev[(qd + 2) % 4]
                    G_v[j, qd * 64:(qd + 1) * 64, :] = hq - other if qd in (0, 3) else hq + other
                bg.run(budget)
            prev = cur
        if t + 1 < NT:
            for qd in range(4):
                H_v[qd * 64:(qd + 1) * 64, :] = prev[qd]

    def job_x(t, bg, budget):
        for half in range(2):
            j = 2 * t + half
            for part in range(2):
                X_v[j, part * P:(part + 1) * P, :] = _dot(F_v[part * P:(part + 1) * P, 0:P],
                                                          kv_v[j * P:(j + 1) * P, :])
                bg.run(budget)

    def z2_tile(t, m, n):
        return _gelu2(_dot(xn_v[pl.ds(t * TM + m * MC, MC), :], win_v[:, FH + n * L:FH + (n + 1) * L]))

    def job_z2(t, m, bg, budgets, first=0):
        rows = pl.ds(t * TM + m * MC, MC)
        tiles = []
        s1 = s2 = None
        for n in range(FH // L):
            z = z2_tile(t, m, n) if n >= first else zt_v[m * MC:(m + 1) * MC, n * L:(n + 1) * L]
            tiles.append(z)
            s1 = z if s1 is None else s1 + z
            s2 = z * z if s2 is None else s2 + z * z
            if n >= first:
                bg.run(budgets[n])
        mean = jnp.sum(s1, axis=-1, keepdims=True) * (1.0 / FH)
        ex2 = jnp.sum(s2, axis=-1, keepdims=True) * (1.0 / FH)
        var = jnp.maximum(ex2 - mean * mean, 0.0)
        rs = jax.lax.rsqrt(var + 4.0 * EPS)
        for n in range(FH // L):
            z2_v[rows, n * L:(n + 1) * L] = ((tiles[n] - mean) * rs).astype(BF16)

    def job_z1(t, m, bg, budgets):
        rows = pl.ds(t * TM + m * MC, MC)
        for n in range(FH // L):
            z1_v[rows, n * L:(n + 1) * L] = _gelu2(_dot(xn_v[rows, :], win_v[:, n * L:(n + 1) * L]))
            bg.run(budgets[n])

    rev8 = 7 - jax.lax.broadcasted_iota(jnp.int32, (8, L), 0)

    def tail_piece(a, upper, n):
        rows = pl.ds(a * P + (MC if upper else 0), MC)
        lanes = slice(n * L, (n + 1) * L)
        hh = _dot(u_v[rows, :], wout_v[:, lanes]) * 0.25
        if upper:
            ya = _dot(Fi_v[:, 0:P], Z_v[a, 0:P, lanes])
            yb = _dot(Fi_v[:, P:2 * P], Z_v[a, P:2 * P, lanes])
            y = ya - yb
            lo = ya + yb
            for j in range(MC // 8):
                yl_v[n, (7 - j) * 8:(8 - j) * 8, :] = jnp.take_along_axis(lo[j * 8:(j + 1) * 8], rev8, axis=0)
        else:
            y = yl_v[n]
        gate = hh + hh * jnp.tanh(hh)
        s = xn_v[rows, lanes].astype(F32) * y
        o_v[rows, lanes] = (x_v[rows, lanes].astype(F32) + s * gate).astype(BF16)

    def job_big(i, bg, pending, budget):
        blocks = _blocks_of_step(i)
        KG = 512
        t = 0
        for m in range(TM // MC):
            rows = pl.ds(blocks[m // 2] * P + (m % 2) * MC, MC)
            for n in range(FH // L):
                acc = None
                for kg in range(S // KG):
                    p = _dot(wsp_v[i * TM + m * MC:i * TM + (m + 1) * MC, kg * KG:(kg + 1) * KG],
                             z2_v[kg * KG:(kg + 1) * KG, n * L:(n + 1) * L])
                    acc = p if acc is None else acc + p
                    bg.run(budget)
                u_v[rows, n * L:(n + 1) * L] = (
                    z1_v[rows, n * L:(n + 1) * L] * (acc + bcol_v[rows, :])).astype(BF16)
                t += 1
                if pending and t >= 2:
                    tail_piece(*pending.pop(0))
                    bg.run(budget)

    start(cp_small())
    cp_x(0).start()
    cp_win(2).start()

    kk = _odd_freq(jax.lax.broadcasted_iota(jnp.int32, (P, P), 0))
    nn = jax.lax.broadcasted_iota(jnp.int32, (P, P), 1)
    fc, fs = _cos_sin((kk * (4 * nn - 127)) & 2047)
    F_v[0:P, 0:P] = fc.astype(BF16)
    F_v[P:2 * P, 0:P] = (-fs).astype(BF16)
    kk = _odd_freq(jax.lax.broadcasted_iota(jnp.int32, (MC, P), 1))
    mm = jax.lax.broadcasted_iota(jnp.int32, (MC, P), 0)
    ic, is_ = _cos_sin((kk * (4 * mm + 2)) & 2047)
    Fi_v[:, 0:P] = (ic * (1.0 / P)).astype(BF16)
    Fi_v[:, P:2 * P] = (is_ * (1.0 / P)).astype(BF16)
    cp_x(1).start()
    cp_win(3).start()

    wait(cp_small())
    brow = b_in[...].astype(F32).reshape(1, S)
    for j in range(NB):
        bcol_v[j * P:(j + 1) * P, :] = jnp.broadcast_to(brow[:, j * P:(j + 1) * P], (P, P)).T
    sk = sk_in[...].astype(F32)
    for t in range(4):
        sk_v[t] = jnp.broadcast_to(sk[t:t + 1], (8, D))
    kf_v[:, 0:8, :] = jnp.zeros((D // L, 8, L), F32)
    drow = d_in[...].astype(F32).reshape(1, D)
    dre = fc[:, 0:1] * drow
    dim = fs[:, 0:1] * drow
    H_v[0:64, :] = -dim[0:64]
    H_v[64:P, :] = dim[64:P]
    H_v[P:P + 64, :] = -dre[0:64]
    H_v[P + 64:2 * P, :] = dre[64:P]

    cp_x(0).wait()
    for _ in ln_x(0):
        pass

    LAG = 2

    def conv_dma(g):
        t = g - LAG
        if 0 <= t + 1 < NT:
            start(cp_conv(t + 1))
        if 0 <= t < NT:
            wait(cp_conv(t))

    def p1_a():
        for m in range(TM // MC):
            for n in range(WC // L):
                zt_v[m * MC:(m + 1) * MC, n * L:(n + 1) * L] = z2_tile(0, m, n)

    def p1_b():
        bg = _Background()
        bg.add(ln_x(1))
        for m in range(TM // MC):
            job_z2(0, m, bg, (110,) * 6, first=WC // L)
        bg.drain()

    def p1_c():
        bg = _Background()
        bg.add(ln_x(2))
        for m in range(TM // MC):
            job_z2(1, m, bg, (0, 0, 80, 80, 80, 80))
        bg.drain()

    def p1_d():
        bg = _Background()
        for t in range(2):
            for m in range(TM // MC):
                job_z1(t, m, bg, (0,) * 6)

    cp_win(2).wait()
    cp_x(2).start()
    cp_win(0).start()
    cp_win(1).start()
    block(p1_a)
    cp_x(1).wait()
    cp_win(3).wait()
    block(p1_b)
    cp_x(3).start()
    start(cp_conv(0))
    cp_x(2).wait()
    block(p1_c)
    cp_win(0).wait()
    cp_win(1).wait()
    block(p1_d)

    def p1_dma(i):
        if i + 2 < NT:
            cp_x(i + 2).start()
        if i >= 5:
            start(cp_wsp(i - 5))
        if i == 3:
            cp_wout().start()
        conv_dma(i)
        if i + 1 < NT:
            cp_x(i + 1).wait()

    def p1_step(i):
        bg = _Background()
        if i + 1 < NT:
            bg.add(ln_x(i + 1))
        t = i - LAG
        bg.add(kv_gen(t))
        bg.run(100)
        if t >= 1:
            job_x(t - 1, bg, 150)
        job_h(t, bg, 150)
        for m in range(TM // MC):
            job_z2(i, m, bg, (70,) * 6)
            job_z1(i, m, bg, (0, 0, 0, 40, 70, 70))
        bg.drain()

    for i in range(2, NT):
        p1_dma(i)
        block(lambda i=i: p1_step(i))

    def p2_dma(i):
        if i == 0:
            cp_wout().wait()
        if i >= 2:
            start(cp_out(i - 2))
        if i >= 3:
            wait(cp_out(i - 3))
        if i + 3 < NT:
            start(cp_wsp(i + 3))
        conv_dma(NT + i)
        if i < NT:
            wait(cp_wsp(i))

    def tails_of(i):
        return [(a, upper, n) for a in _blocks_of_step(i) for upper in (True, False) for n in range(D // L)]

    def p2_step(i):
        bg = _Background()
        pending = tails_of(i - 1) if i > 0 else []
        total = 17 * 40 * 16
        slots = 96 + len(pending)
        t = NT + i - LAG
        if t < NT:
            bg.add(kv_gen(t))
            total += 20 * 90
            slots += 8
        if t - 1 < NT:
            slots += 8
        for a in _blocks_of_step(i):
            bg.add(freq_gen(a))
        budget = total / (slots + 1.0)
        bg.run(budget)
        if t - 1 < NT:
            job_x(t - 1, bg, 2 * budget)
        if t < NT:
            job_h(t, bg, 2 * budget)
        job_big(i, bg, pending, budget)
        for t_ in pending:
            tail_piece(*t_)
        bg.drain()

    for i in range(NT):
        p2_dma(i)
        block(lambda i=i: p2_step(i))

    def p2_last():
        a0, a1 = _blocks_of_step(NT - 1)
        for t_ in tails_of(NT - 1):
            tail_piece(*t_)
            if t_ == (a0, False, D // L - 1):
                cp_out(NT - 1)[0].start()

    p2_dma(NT)
    block(p2_last)
    cp_out(NT - 1)[1].start()
    wait(cp_out(NT - 2))
    wait(cp_out(NT - 1))


@jax.jit
def pallas_recurrent_scan__ssm_conv_h3__mixer_gmlp__prompt_kernel(
    A_q: jax.Array,
    A_k: jax.Array,
    A_v: jax.Array,
    A_shift_k: jax.Array,
    A_ssm_k: jax.Array,
    A_ssm_D: jax.Array,
    B_x: jax.Array,
    B_w_in: jax.Array,
    B_w_sp: jax.Array,
    B_b_sp: jax.Array,
    B_w_out: jax.Array,
):
    del B_x
    hbm = pl.BlockSpec(memory_space=pl.ANY)

    def bf16_buf(*shape):
        return pltpu.VMEM(shape[:-2] + (shape[-2] // 2, shape[-1]), U32)

    return pl.pallas_call(
        _kernel,
        out_shape=jax.ShapeDtypeStruct((1, S, D), BF16),
        in_specs=[pl.BlockSpec(memory_space=pltpu.SMEM)] + [hbm] * 10,
        out_specs=hbm,
        scratch_shapes=[
            bf16_buf(S, D),
            bf16_buf(S, D),
            bf16_buf(S, D),
            bf16_buf(NT, D, TM),
            bf16_buf(D, 2 * FH),
            bf16_buf(S, S),
            bf16_buf(FH, D),
            pltpu.VMEM((S, D), BF16),
            pltpu.VMEM((4, D), BF16),
            pltpu.VMEM((D,), BF16),
            pltpu.VMEM((S,), BF16),
            bf16_buf(S, D),
            pltpu.VMEM((S, FH), F32),
            bf16_buf(S, FH),
            pltpu.VMEM((TM, WC), F32),
            bf16_buf(S, D),
            bf16_buf(S, FH),
            pltpu.VMEM((NB, 2 * P, D), F32),
            pltpu.VMEM((2 * P, D), F32),
            pltpu.VMEM((NB, 2 * P, D), F32),
            bf16_buf(NB, 2 * P, D),
            pltpu.VMEM((D // L, MC, L), F32),
            bf16_buf(2 * P, 2 * P),
            bf16_buf(MC, 2 * P),
            pltpu.VMEM((S, L), F32),
            pltpu.VMEM((4, 8, D), F32),
            pltpu.VMEM((D // L, S + 8, L), F32),
            pltpu.SemaphoreType.DMA((1,)),
            pltpu.SemaphoreType.DMA((3,)),
            pltpu.SemaphoreType.DMA((2,)),
            pltpu.SemaphoreType.DMA((4,)),
            pltpu.SemaphoreType.DMA((5,)),
            pltpu.SemaphoreType.DMA((3,)),
        ],
        compiler_params=pltpu.CompilerParams(vmem_limit_bytes=100 * 1024 * 1024),
    )(jnp.ones((1,), jnp.int32), A_q, A_k, A_v, A_shift_k.T, A_ssm_k, A_ssm_D, B_w_in, B_w_sp, B_b_sp, B_w_out)
```

```python
import math

import jax
import jax.numpy as jnp
import jax.experimental.pallas as pl
import jax.experimental.pallas.tpu as pltpu

S = 2048
D = 640
FH = 768
P = 128
NB = S // P
TM = 256
NT = S // TM
MC = 64
L = 128
WC = 384
EPS = 1e-5
F32 = jnp.float32
BF16 = jnp.bfloat16
U32 = jnp.uint32
GELU_C = math.sqrt(2.0 / math.pi)
NT_DIMS = (((1,), (1,)), ((), ()))
_ONLY = None


def _dot(a, b):
    return jnp.dot(a, b, preferred_element_type=F32)


def _cos_sin(m):
    q = (m + 256) >> 9
    x = (m - (q << 9)).astype(F32) * (2.0 * math.pi / 2048.0)
    x2 = x * x
    s = x * (1.0 + x2 * (-1.0 / 6 + x2 * (1.0 / 120 + x2 * (-1.0 / 5040 + x2 * (1.0 / 362880)))))
    c = 1.0 + x2 * (-0.5 + x2 * (1.0 / 24 + x2 * (-1.0 / 720 + x2 * (1.0 / 40320 - x2 * (1.0 / 3628800)))))
    swap = (q & 1) == 1
    c0 = jnp.where(swap, s, c)
    s0 = jnp.where(swap, c, s)
    cos = jnp.where(((q + 1) & 2) == 2, -c0, c0)
    sin = jnp.where((q & 2) == 2, -s0, s0)
    return cos, sin


def _odd_freq(r):
    return jnp.where(r < 64, 4 * r + 1, 4 * r - 253)


def _gelu2(z):
    u = z * (GELU_C + (GELU_C * 0.044715) * (z * z))
    return z + z * jnp.tanh(u)


def _signzero(z):
    bits = jax.lax.bitcast_convert_type(z, U32) & jnp.uint32(0x80000000)
    return jax.lax.bitcast_convert_type(bits, F32)


def _ln(x, eps, tie=None):
    n = x.shape[-1]
    part = x[:, 0:L]
    for j in range(1, n // L):
        part = part + x[:, j * L:(j + 1) * L]
    if tie is not None:
        part = part + tie
    m = jnp.sum(part, axis=-1, keepdims=True) * (1.0 / n)
    xc = x - m
    v = jnp.sum(xc * xc, axis=-1, keepdims=True) * (1.0 / n)
    return xc * jax.lax.rsqrt(v + eps)


def _blocks_of_step(i):
    return (NT - 1 - i, NT + i)


class _Background:
    def __init__(self):
        self.q = []
        self.credit = 0.0

    def add(self, gen):
        self.q.append(gen)

    def run(self, budget):
        self.credit += budget
        while self.q and self.credit > 0:
            try:
                self.credit -= next(self.q[0])
            except StopIteration:
                self.q.pop(0)
        if not self.q:
            self.credit = 0.0

    def drain(self):
        while self.q:
            self.run(1e9)


def _kernel(one_ref, q_hbm, k_hbm, v_hbm, sk_hbm, h_hbm, d_hbm, win_hbm, wsp_hbm, b_hbm, wout_hbm,
            o_hbm,
            x_u, k_u, v_u, h_u, win_u, wsp_u, wout_u, o_v, sk_in, d_in, b_in,
            xn_u, z1_v, z2_u, zg_v, kv_u, u_u, X_v, H_v, G_v, Z_u, yl_v, F_u, Fi_u, bcol_v, sk_v, kf_v,
            sem_small, sem_x, sem_conv, sem_wsp, sem_w, sem_out):
    x_v, k_v, v_v, h_v, win_v, wsp_v, wout_v, xn_v, z2_v, kv_v, u_v, Z_v, F_v, Fi_v = [
        r.bitcast(BF16) for r in (x_u, k_u, v_u, h_u, win_u, wsp_u, wout_u, xn_u, z2_u, kv_u, u_u, Z_u, F_u,
                                  Fi_u)]

    def cp_small():
        return [pltpu.make_async_copy(s_, d_, sem_small.at[0])
                for s_, d_ in ((d_hbm, d_in), (sk_hbm, sk_in), (b_hbm, b_in))]

    def cp_x(t):
        return pltpu.make_async_copy(q_hbm.at[0, pl.ds(t * TM, TM)], x_v.at[pl.ds(t * TM, TM)], sem_x.at[t % 3])

    def cp_conv(t):
        rows = pl.ds(t * TM, TM)
        sem = sem_conv.at[t % 2]
        return [pltpu.make_async_copy(h_hbm.at[:, rows], h_v.at[t], sem),
                pltpu.make_async_copy(k_hbm.at[0, rows], k_v.at[rows], sem),
                pltpu.make_async_copy(v_hbm.at[0, rows], v_v.at[rows], sem)]

    def cp_wsp(i):
        return [pltpu.make_async_copy(wsp_hbm.at[pl.ds(a * P, P)], wsp_v.at[pl.ds(i * TM + half * P, P)],
                                      sem_wsp.at[i % 4]) for half, a in enumerate(_blocks_of_step(i))]

    def cp_win(c):
        cols = pl.ds(c * WC, WC)
        return pltpu.make_async_copy(win_hbm.at[:, cols], win_v.at[:, cols], sem_w.at[c])

    def cp_wout():
        return pltpu.make_async_copy(wout_hbm, wout_v, sem_w.at[4])

    def cp_out(i, which=(0, 1)):
        return [pltpu.make_async_copy(o_v.at[pl.ds(a * P, P)], o_hbm.at[0, pl.ds(a * P, P)], sem_out.at[i % 3])
                for a in [_blocks_of_step(i)[w] for w in which]]

    def start(cs):
        for c in cs:
            c.start()

    def wait(cs):
        for c in cs:
            c.wait()

    always = one_ref[0] == 1

    def block(fn, name):
        if _ONLY is None or name in _ONLY:
            pl.when(always)(fn)

    def ln_x(t, s, tie=None):
        rows = pl.ds(t * TM + s * 16, 16)
        xn_v[rows, :] = _ln(x_v[rows, :].astype(F32), EPS, tie).astype(BF16)

    def ln_z2(t, s, tie=None):
        z2_v[pl.ds(t * TM + s * 16, 16), :] = _ln(zg_v[t % 2, s * 16:(s + 1) * 16, :], 4.0 * EPS, tie).astype(BF16)

    def tasks(fn, t):
        return [lambda tie, s=s: fn(t, s, tie) for s in range(TM // 16)]

    def kv_gen(t):
        for m in range(TM // MC):
            r = t * TM + m * MC
            for l in range(D // L):
                lanes = slice(l * L, (l + 1) * L)
                kf = k_v[pl.ds(r, MC), lanes].astype(F32)
                kf_v[l, pl.ds(r + 8, MC), :] = kf
                ks = kf * sk_v[0, 0:1, lanes]
                for tap in range(1, 4):
                    ks = ks + kf_v[l, pl.ds(r + 8 - tap, MC), :] * sk_v[tap, 0:1, lanes]
                kv = ks * v_v[pl.ds(r, MC), lanes].astype(F32)
                kv_v[pl.ds(r, MC), lanes] = kv.astype(BF16)
                yield 90

    def freq_gen(a):
        for r in range(P // 16):
            re = pl.ds(r * 16, 16)
            im = pl.ds(P + r * 16, 16)
            for l in range(D // L):
                lanes = slice(l * L, (l + 1) * L)
                ar = ai = None
                for c in range(a + 1):
                    xr = X_v[c, re, lanes]
                    xi = X_v[c, im, lanes]
                    gr = G_v[a - c, re, lanes]
                    gi = G_v[a - c, im, lanes]
                    pr = xr * gr - xi * gi
                    pi = xr * gi + xi * gr
                    ar = pr if ar is None else ar + pr
                    ai = pi if ai is None else ai + pi
                    if c == a:
                        Z_v[a, re, lanes] = ar.astype(BF16)
                        Z_v[a, im, lanes] = ai.astype(BF16)
                    yield 16

    def job_h(t, bg, budget):
        prev = [H_v[qd * 64:(qd + 1) * 64, :] for qd in range(4)]
        for half in range(2):
            j = 2 * t + half
            cur = []
            for part in range(2):
                hp = jax.lax.dot_general(F_v[part * P:(part + 1) * P, 0:P], h_v[t, :, half * P:(half + 1) * P],
                                         NT_DIMS, preferred_element_type=F32)
                for qd in (2 * part, 2 * part + 1):
                    hq = hp[(qd % 2) * 64:(qd % 2 + 1) * 64]
                    cur.append(hq)
                    other = prev[(qd + 2) % 4]
                    G_v[j, qd * 64:(qd + 1) * 64, :] = hq - other if qd in (0, 3) else hq + other
                bg.run(budget)
            prev = cur
        if t + 1 < NT:
            for qd in range(4):
                H_v[qd * 64:(qd + 1) * 64, :] = prev[qd]

    def job_x(t, bg, budget):
        for half in range(2):
            j = 2 * t + half
            for part in range(2):
                X_v[j, part * P:(part + 1) * P, :] = _dot(F_v[part * P:(part + 1) * P, 0:P],
                                                          kv_v[j * P:(j + 1) * P, :])
                bg.run(budget)

    def job_z(t, m, cols, bg=None, budgets=None, tied=None, ntied=None, inline_ln=False):
        rows = pl.ds(t * TM + m * MC, MC)
        for j, n in enumerate(cols):
            z = _gelu2(_dot(xn_v[rows, :], win_v[:, n * L:(n + 1) * L]))
            if n < FH // L:
                z1_v[rows, n * L:(n + 1) * L] = z
            else:
                zg_v[t % 2, m * MC:(m + 1) * MC, n * L - FH:(n + 1) * L - FH] = z
            if tied and ntied[j]:
                tie = _signzero(z[0:16])
                for _ in range(ntied[j]):
                    if tied:
                        tied.pop(0)(tie)
            if inline_ln and n == 2 * FH // L - 1:
                for s in range(4 * m, 4 * m + 4):
                    ln_z2(t, s)
            if bg is not None:
                bg.run(budgets[j])

    rev8 = 7 - jax.lax.broadcasted_iota(jnp.int32, (8, L), 0)

    def tail_piece(a, upper, n):
        rows = pl.ds(a * P + (MC if upper else 0), MC)
        lanes = slice(n * L, (n + 1) * L)
        hh = _dot(u_v[rows, :], wout_v[:, lanes]) * 0.25
        if upper:
            ya = _dot(Fi_v[:, 0:P], Z_v[a, 0:P, lanes])
            yb = _dot(Fi_v[:, P:2 * P], Z_v[a, P:2 * P, lanes])
            y = ya - yb
            lo = ya + yb
            for j in range(MC // 8):
                yl_v[n, (7 - j) * 8:(8 - j) * 8, :] = jnp.take_along_axis(lo[j * 8:(j + 1) * 8], rev8, axis=0)
        else:
            y = yl_v[n]
        gate = hh + hh * jnp.tanh(hh)
        s = xn_v[rows, lanes].astype(F32) * y
        o_v[rows, lanes] = (x_v[rows, lanes].astype(F32) + s * gate).astype(BF16)

    def job_big(i, bg, pending, budget):
        blocks = _blocks_of_step(i)
        KG = 512
        t = 0
        for m in range(TM // MC):
            rows = pl.ds(blocks[m // 2] * P + (m % 2) * MC, MC)
            for n in range(FH // L):
                acc = None
                for kg in range(S // KG):
                    p = _dot(wsp_v[i * TM + m * MC:i * TM + (m + 1) * MC, kg * KG:(kg + 1) * KG],
                             z2_v[kg * KG:(kg + 1) * KG, n * L:(n + 1) * L])
                    acc = p if acc is None else acc + p
                    bg.run(budget)
                u_v[rows, n * L:(n + 1) * L] = (
                    z1_v[rows, n * L:(n + 1) * L] * (acc + bcol_v[rows, :])).astype(BF16)
                t += 1
                if pending and t >= 2:
                    tail_piece(*pending.pop(0))
                    bg.run(budget)

    if _ONLY is not None:
        for r_ in (xn_u, z1_v, z2_u, zg_v, kv_u, u_u, X_v, H_v, G_v, Z_u, kf_v):
            c_ = pltpu.make_async_copy(r_, r_, sem_small.at[0])
            c_.start()
            c_.wait()

    start(cp_small())
    cp_x(0).start()
    cp_win(2).start()

    kk = _odd_freq(jax.lax.broadcasted_iota(jnp.int32, (P, P), 0))
    nn = jax.lax.broadcasted_iota(jnp.int32, (P, P), 1)
    fc, fs = _cos_sin((kk * (4 * nn - 127)) & 2047)
    F_v[0:P, 0:P] = fc.astype(BF16)
    F_v[P:2 * P, 0:P] = (-fs).astype(BF16)
    kk = _odd_freq(jax.lax.broadcasted_iota(jnp.int32, (MC, P), 1))
    mm = jax.lax.broadcasted_iota(jnp.int32, (MC, P), 0)
    ic, is_ = _cos_sin((kk * (4 * mm + 2)) & 2047)
    Fi_v[:, 0:P] = (ic * (1.0 / P)).astype(BF16)
    Fi_v[:, P:2 * P] = (is_ * (1.0 / P)).astype(BF16)
    cp_x(1).start()
    cp_win(3).start()

    wait(cp_small())
    brow = b_in[...].astype(F32).reshape(1, S)
    for j in range(NB):
        bcol_v[j * P:(j + 1) * P, :] = jnp.broadcast_to(brow[:, j * P:(j + 1) * P], (P, P)).T
    sk = sk_in[...].astype(F32)
    for t in range(4):
        sk_v[t] = jnp.broadcast_to(sk[t:t + 1], (8, D))
    kf_v[:, 0:8, :] = jnp.zeros((D // L, 8, L), F32)
    drow = d_in[...].astype(F32).reshape(1, D)
    dre = fc[:, 0:1] * drow
    dim = fs[:, 0:1] * drow
    H_v[0:64, :] = -dim[0:64]
    H_v[64:P, :] = dim[64:P]
    H_v[P:P + 64, :] = -dre[0:64]
    H_v[P + 64:2 * P, :] = dre[64:P]

    cp_x(0).wait()
    for s in range(TM // 16):
        ln_x(0, s)

    LAG = 2

    def conv_dma(g):
        t = g - LAG
        if 0 <= t + 1 < NT:
            start(cp_conv(t + 1))
        if 0 <= t < NT:
            wait(cp_conv(t))

    def interleave(a, b):
        out = []
        for j in range(max(len(a), len(b))):
            out += a[j:j + 1] + b[j:j + 1]
        return out

    def p1_a():
        for m in range(TM // MC):
            job_z(0, m, range(6, 9))

    def p1_b():
        tied = tasks(ln_x, 1)
        for m in range(TM // MC):
            job_z(0, m, range(9, 12), tied=tied, ntied=(2, 2, 2))

    def p1_c():
        tied = interleave(tasks(ln_x, 2), tasks(ln_z2, 0))
        for m in range(TM // MC):
            job_z(1, m, range(6, 12), tied=tied, ntied=(2, 1, 2, 1, 2, 1))

    def p1_d():
        tied = tasks(ln_z2, 1)
        for t in range(2):
            for m in range(TM // MC):
                job_z(t, m, range(6), tied=tied, ntied=(1, 0, 1, 0, 1, 0))

    cp_win(2).wait()
    cp_x(2).start()
    cp_win(0).start()
    cp_win(1).start()
    block(p1_a, 'p1_a')
    cp_x(1).wait()
    cp_win(3).wait()
    block(p1_b, 'p1_b')
    start(cp_conv(0))
    cp_x(3).start()
    cp_x(2).wait()
    block(p1_c, 'p1_c')
    cp_win(0).wait()
    cp_win(1).wait()
    block(p1_d, 'p1_d')

    def p1_dma(i):
        if i + 2 < NT:
            cp_x(i + 2).start()
        if i >= 5:
            start(cp_wsp(i - 5))
        if i == 3:
            cp_wout().start()
        conv_dma(i)
        if i + 1 < NT:
            cp_x(i + 1).wait()

    def p1_step(i):
        bg = _Background()
        t = i - LAG
        bg.add(kv_gen(t))
        tied = interleave(tasks(ln_x, i + 1) if i + 1 < NT else [], tasks(ln_z2, i - 1) if i > 2 else [])
        last = i == NT - 1
        ntied = (1, 1, 1, 1, 1, 0, 0, 0, 0, 0, 0, 0) if last else (1, 1, 0, 1, 1, 0) * 2
        for m in range(TM // MC):
            job_z(i, m, list(range(6, 12)) + list(range(6)), bg, (0, 0, 60, 0, 0, 60) * 2, tied, ntied, last)
            if m == 0:
                job_h(t, bg, 90)
        assert not tied
        if t >= 1:
            job_x(t - 1, bg, 180)
        bg.drain()

    for i in range(2, NT):
        p1_dma(i)
        block(lambda i=i: p1_step(i), f'p1_{i}')

    def p2_dma(i):
        if i == 0:
            cp_wout().wait()
        if i >= 2:
            start(cp_out(i - 2))
        if i >= 3:
            wait(cp_out(i - 3))
        if i + 3 < NT:
            start(cp_wsp(i + 3))
        conv_dma(NT + i)
        if i < NT:
            wait(cp_wsp(i))

    def tails_of(i):
        return [(a, upper, n) for a in _blocks_of_step(i) for upper in (True, False) for n in range(D // L)]

    def p2_step(i):
        bg = _Background()
        pending = tails_of(i - 1) if i > 0 else []
        total = 17 * 40 * 16
        slots = 96 + len(pending)
        t = NT + i - LAG
        if t < NT:
            bg.add(kv_gen(t))
            total += 20 * 90
            slots += 8
        if t - 1 < NT:
            slots += 8
        for a in _blocks_of_step(i):
            bg.add(freq_gen(a))
        budget = total / (slots + 1.0)
        bg.run(budget)
        if t - 1 < NT:
            job_x(t - 1, bg, 2 * budget)
        if t < NT:
            job_h(t, bg, 2 * budget)
        job_big(i, bg, pending, budget)
        for t_ in pending:
            tail_piece(*t_)
        bg.drain()

    for i in range(NT):
        p2_dma(i)
        block(lambda i=i: p2_step(i), f'p2_{i}')

    def p2_last():
        a0, a1 = _blocks_of_step(NT - 1)
        for t_ in tails_of(NT - 1):
            tail_piece(*t_)
            if t_ == (a0, False, D // L - 1):
                start(cp_out(NT - 1, (0,)))

    p2_dma(NT)
    block(p2_last, 'p2_last')
    start(cp_out(NT - 1, (1,)))
    wait(cp_out(NT - 2))
    wait(cp_out(NT - 1))
    if _ONLY is not None:
        for r_ in (xn_u, z1_v, z2_u, zg_v, kv_u, u_u, X_v, H_v, G_v, Z_u, kf_v):
            c_ = pltpu.make_async_copy(r_, r_, sem_small.at[0])
            c_.start()
            c_.wait()


@jax.jit
def pallas_recurrent_scan__ssm_conv_h3__mixer_gmlp__prompt_kernel(
    A_q: jax.Array,
    A_k: jax.Array,
    A_v: jax.Array,
    A_shift_k: jax.Array,
    A_ssm_k: jax.Array,
    A_ssm_D: jax.Array,
    B_x: jax.Array,
    B_w_in: jax.Array,
    B_w_sp: jax.Array,
    B_b_sp: jax.Array,
    B_w_out: jax.Array,
):
    del B_x
    hbm = pl.BlockSpec(memory_space=pl.ANY)

    def bf16_buf(*shape):
        return pltpu.VMEM(shape[:-2] + (shape[-2] // 2, shape[-1]), U32)

    return pl.pallas_call(
        _kernel,
        out_shape=jax.ShapeDtypeStruct((1, S, D), BF16),
        in_specs=[pl.BlockSpec(memory_space=pltpu.SMEM)] + [hbm] * 10,
        out_specs=hbm,
        scratch_shapes=[
            bf16_buf(S, D),
            bf16_buf(S, D),
            bf16_buf(S, D),
            bf16_buf(NT, D, TM),
            bf16_buf(D, 2 * FH),
            bf16_buf(S, S),
            bf16_buf(FH, D),
            pltpu.VMEM((S, D), BF16),
            pltpu.VMEM((4, D), BF16),
            pltpu.VMEM((D,), BF16),
            pltpu.VMEM((S,), BF16),
            bf16_buf(S, D),
            pltpu.VMEM((S, FH), F32),
            bf16_buf(S, FH),
            pltpu.VMEM((2, TM, FH), F32),
            bf16_buf(S, D),
            bf16_buf(S, FH),
            pltpu.VMEM((NB, 2 * P, D), F32),
            pltpu.VMEM((2 * P, D), F32),
            pltpu.VMEM((NB, 2 * P, D), F32),
            bf16_buf(NB, 2 * P, D),
            pltpu.VMEM((D // L, MC, L), F32),
            bf16_buf(2 * P, 2 * P),
            bf16_buf(MC, 2 * P),
            pltpu.VMEM((S, L), F32),
            pltpu.VMEM((4, 8, D), F32),
            pltpu.VMEM((D // L, S + 8, L), F32),
            pltpu.SemaphoreType.DMA((1,)),
            pltpu.SemaphoreType.DMA((3,)),
            pltpu.SemaphoreType.DMA((2,)),
            pltpu.SemaphoreType.DMA((4,)),
            pltpu.SemaphoreType.DMA((5,)),
            pltpu.SemaphoreType.DMA((3,)),
        ],
        compiler_params=pltpu.CompilerParams(vmem_limit_bytes=100 * 1024 * 1024),
    )(jnp.ones((1,), jnp.int32), A_q, A_k, A_v, A_shift_k.T, A_ssm_k, A_ssm_D, B_w_in, B_w_sp, B_b_sp, B_w_out)
```

```python
import math

import jax
import jax.numpy as jnp
import jax.experimental.pallas as pl
import jax.experimental.pallas.tpu as pltpu

S = 2048
D = 640
FH = 768
P = 128
NB = S // P
TM = 256
NT = S // TM
MC = 64
L = 128
HK = S // 2
HN = FH // 2
WC = 384
EPS = 1e-5
F32 = jnp.float32
BF16 = jnp.bfloat16
U32 = jnp.uint32
GELU_C = math.sqrt(2.0 / math.pi)
NT_DIMS = (((1,), (1,)), ((), ()))
_ONLY = None


def _dot(a, b):
    return jnp.dot(a, b, preferred_element_type=F32)


def _cos_sin(m):
    q = (m + 256) >> 9
    x = (m - (q << 9)).astype(F32) * (2.0 * math.pi / 2048.0)
    x2 = x * x
    s = x * (1.0 + x2 * (-1.0 / 6 + x2 * (1.0 / 120 + x2 * (-1.0 / 5040 + x2 * (1.0 / 362880)))))
    c = 1.0 + x2 * (-0.5 + x2 * (1.0 / 24 + x2 * (-1.0 / 720 + x2 * (1.0 / 40320 - x2 * (1.0 / 3628800)))))
    swap = (q & 1) == 1
    c0 = jnp.where(swap, s, c)
    s0 = jnp.where(swap, c, s)
    cos = jnp.where(((q + 1) & 2) == 2, -c0, c0)
    sin = jnp.where((q & 2) == 2, -s0, s0)
    return cos, sin


def _odd_freq(r):
    return jnp.where(r < 64, 4 * r + 1, 4 * r - 253)


def _gelu2(z):
    u = z * (GELU_C + (GELU_C * 0.044715) * (z * z))
    return z + z * jnp.tanh(u)


def _signzero(z):
    bits = jax.lax.bitcast_convert_type(z, U32) & jnp.uint32(0x80000000)
    return jax.lax.bitcast_convert_type(bits, F32)


def _ln(x, eps, tie=None):
    n = x.shape[-1]
    part = x[:, 0:L]
    for j in range(1, n // L):
        part = part + x[:, j * L:(j + 1) * L]
    if tie is not None:
        part = part + tie
    m = jnp.sum(part, axis=-1, keepdims=True) * (1.0 / n)
    xc = x - m
    v = jnp.sum(xc * xc, axis=-1, keepdims=True) * (1.0 / n)
    return xc * jax.lax.rsqrt(v + eps)


def _blocks_of_step(i):
    return (NT - 1 - i, NT + i)


class _Background:
    def __init__(self):
        self.q = []
        self.credit = 0.0

    def add(self, gen):
        self.q.append(gen)

    def run(self, budget):
        self.credit += budget
        while self.q and self.credit > 0:
            try:
                self.credit -= next(self.q[0])
            except StopIteration:
                self.q.pop(0)
        if not self.q:
            self.credit = 0.0

    def drain(self):
        while self.q:
            self.run(1e9)


def _kernel(one_ref, q_hbm, k_hbm, v_hbm, sk_hbm, h_hbm, d_hbm, win_hbm, wsp_hbm, b_hbm, wout_hbm,
            o_hbm,
            x_u, k_u, v_u, h_u, win_u, wsp_u, wout_u, o_v, sk_in, d_in, b_in,
            xn_u, z1_v, R_u, Lc_u, zf_v, zg_v, kv_u, u_u, X_v, H_v, G_v, Z_u, yl_v, F_u, Fi_u, bcol_v, sk_v, kf_v,
            sem_small, sem_x, sem_conv, sem_wsp, sem_w, sem_out):
    x_v, k_v, v_v, h_v, win_v, wsp_v, wout_v, xn_v, R_v, Lc_v, kv_v, u_v, Z_v, F_v, Fi_v = [
        r.bitcast(BF16) for r in (x_u, k_u, v_u, h_u, win_u, wsp_u, wout_u, xn_u, R_u, Lc_u, kv_u, u_u, Z_u, F_u,
                                  Fi_u)]

    def cp_small():
        return [pltpu.make_async_copy(s_, d_, sem_small.at[0])
                for s_, d_ in ((d_hbm, d_in), (sk_hbm, sk_in), (b_hbm, b_in))]

    def cp_x(t):
        return pltpu.make_async_copy(q_hbm.at[0, pl.ds(t * TM, TM)], x_v.at[pl.ds(t * TM, TM)], sem_x.at[t % 3])

    def cp_conv(t):
        rows = pl.ds(t * TM, TM)
        sem = sem_conv.at[t % 2]
        return [pltpu.make_async_copy(h_hbm.at[:, rows], h_v.at[t], sem),
                pltpu.make_async_copy(k_hbm.at[0, rows], k_v.at[rows], sem),
                pltpu.make_async_copy(v_hbm.at[0, rows], v_v.at[rows], sem)]

    def cp_wsp(i):
        return [pltpu.make_async_copy(wsp_hbm.at[pl.ds(a * P, P)], wsp_v.at[pl.ds(i * TM + half * P, P)],
                                      sem_wsp.at[i % 4]) for half, a in enumerate(_blocks_of_step(i))]

    def cp_win(c):
        cols = pl.ds(c * WC, WC)
        return pltpu.make_async_copy(win_hbm.at[:, cols], win_v.at[:, cols], sem_w.at[c])

    def cp_wout():
        return pltpu.make_async_copy(wout_hbm, wout_v, sem_w.at[4])

    def cp_out(i, which=(0, 1)):
        return [pltpu.make_async_copy(o_v.at[pl.ds(a * P, P)], o_hbm.at[0, pl.ds(a * P, P)], sem_out.at[i % 3])
                for a in [_blocks_of_step(i)[w] for w in which]]

    def start(cs):
        for c in cs:
            c.start()

    def wait(cs):
        for c in cs:
            c.wait()

    always = one_ref[0] == 1

    def block(fn, name):
        if _ONLY is None or name in _ONLY:
            pl.when(always)(fn)

    def ln_x(t, s, tie=None):
        rows = pl.ds(t * TM + s * 16, 16)
        xn_v[rows, :] = _ln(x_v[rows, :].astype(F32), EPS, tie).astype(BF16)

    def ln_z2(t, s, tie=None):
        y = _ln(zg_v[t % 2, s * 16:(s + 1) * 16, :], 4.0 * EPS, tie)
        lo, hi = y[:, :HN], y[:, HN:]
        r = (t * TM + s * 16) % HK
        rows = pl.ds(r, 16)
        if t < NT // 2:
            zf_v[rows, :] = y
            R_v[pl.ds(1 * HK + r, 16), :] = lo.astype(BF16)
            R_v[pl.ds(5 * HK + r, 16), :] = (lo + hi).astype(BF16)
        else:
            b11 = zf_v[rows, :HN]
            R_v[pl.ds(0 * HK + r, 16), :] = (b11 + hi).astype(BF16)
            R_v[pl.ds(2 * HK + r, 16), :] = (zf_v[rows, HN:] - hi).astype(BF16)
            R_v[pl.ds(3 * HK + r, 16), :] = (lo - b11).astype(BF16)
            R_v[pl.ds(4 * HK + r, 16), :] = hi.astype(BF16)
            R_v[pl.ds(6 * HK + r, 16), :] = (lo + hi).astype(BF16)

    def acomb_gen(i):
        for r in range(P // 16):
            for c in range(HK // 256):
                top = pl.ds(i * TM + r * 16, 16)
                bot = pl.ds(i * TM + P + r * 16, 16)
                c1 = slice(c * 256, (c + 1) * 256)
                c2 = slice(HK + c * 256, HK + (c + 1) * 256)
                a11 = wsp_v[top, c1].astype(F32)
                a12 = wsp_v[top, c2].astype(F32)
                a21 = wsp_v[bot, c1].astype(F32)
                a22 = wsp_v[bot, c2].astype(F32)
                r0 = (i % 2) * 5 * P + r * 16
                Lc_v[pl.ds(r0 + 0 * P, 16), c1] = (a11 + a22).astype(BF16)
                Lc_v[pl.ds(r0 + 1 * P, 16), c1] = (a21 + a22).astype(BF16)
                Lc_v[pl.ds(r0 + 2 * P, 16), c1] = (a11 + a12).astype(BF16)
                Lc_v[pl.ds(r0 + 3 * P, 16), c1] = (a21 - a11).astype(BF16)
                Lc_v[pl.ds(r0 + 4 * P, 16), c1] = (a12 - a22).astype(BF16)
                yield 46

    def tasks(fn, t):
        return [lambda tie, s=s: fn(t, s, tie) for s in range(TM // 16)]

    def kv_gen(t):
        for m in range(TM // MC):
            r = t * TM + m * MC
            for l in range(D // L):
                lanes = slice(l * L, (l + 1) * L)
                kf = k_v[pl.ds(r, MC), lanes].astype(F32)
                kf_v[l, pl.ds(r + 8, MC), :] = kf
                ks = kf * sk_v[0, 0:1, lanes]
                for tap in range(1, 4):
                    ks = ks + kf_v[l, pl.ds(r + 8 - tap, MC), :] * sk_v[tap, 0:1, lanes]
                kv = ks * v_v[pl.ds(r, MC), lanes].astype(F32)
                kv_v[pl.ds(r, MC), lanes] = kv.astype(BF16)
                yield 90

    def freq_gen(a):
        for r in range(P // 16):
            re = pl.ds(r * 16, 16)
            im = pl.ds(P + r * 16, 16)
            for l in range(D // L):
                lanes = slice(l * L, (l + 1) * L)
                ar = ai = None
                for c in range(a + 1):
                    xr = X_v[c, re, lanes]
                    xi = X_v[c, im, lanes]
                    gr = G_v[a - c, re, lanes]
                    gi = G_v[a - c, im, lanes]
                    pr = xr * gr - xi * gi
                    pi = xr * gi + xi * gr
                    ar = pr if ar is None else ar + pr
                    ai = pi if ai is None else ai + pi
                    if c == a:
                        Z_v[pl.ds(a * 2 * P + r * 16, 16), lanes] = ar.astype(BF16)
                        Z_v[pl.ds(a * 2 * P + P + r * 16, 16), lanes] = ai.astype(BF16)
                    yield 16

    def job_h(t, bg, budget):
        prev = [H_v[qd * 64:(qd + 1) * 64, :] for qd in range(4)]
        for half in range(2):
            j = 2 * t + half
            cur = []
            for part in range(2):
                hp = jax.lax.dot_general(F_v[part * P:(part + 1) * P, 0:P], h_v[t, :, half * P:(half + 1) * P],
                                         NT_DIMS, preferred_element_type=F32)
                for qd in (2 * part, 2 * part + 1):
                    hq = hp[(qd % 2) * 64:(qd % 2 + 1) * 64]
                    cur.append(hq)
                    other = prev[(qd + 2) % 4]
                    G_v[j, qd * 64:(qd + 1) * 64, :] = hq - other if qd in (0, 3) else hq + other
                bg.run(budget)
            prev = cur
        if t + 1 < NT:
            for qd in range(4):
                H_v[qd * 64:(qd + 1) * 64, :] = prev[qd]

    def job_x(t, bg, budget):
        for half in range(2):
            j = 2 * t + half
            for part in range(2):
                X_v[j, part * P:(part + 1) * P, :] = _dot(F_v[part * P:(part + 1) * P, 0:P],
                                                          kv_v[j * P:(j + 1) * P, :])
                bg.run(budget)

    def job_z(t, m, cols, bg=None, budgets=None, tied=None, ntied=None, inline_ln=False):
        rows = pl.ds(t * TM + m * MC, MC)
        for j, n in enumerate(cols):
            z = _gelu2(_dot(xn_v[rows, :], win_v[:, n * L:(n + 1) * L]))
            if n < FH // L:
                z1_v[rows, n * L:(n + 1) * L] = z
            else:
                zg_v[t % 2, m * MC:(m + 1) * MC, n * L - FH:(n + 1) * L - FH] = z
            if tied and ntied[j]:
                tie = _signzero(z[0:16])
                for _ in range(ntied[j]):
                    if tied:
                        tied.pop(0)(tie)
            if inline_ln and n == 2 * FH // L - 1:
                for s in range(4 * m, 4 * m + 4):
                    ln_z2(t, s)
            if bg is not None:
                bg.run(budgets[j])

    rev8 = 7 - jax.lax.broadcasted_iota(jnp.int32, (8, L), 0)

    def tail_piece(a, upper, n):
        rows = pl.ds(a * P + (MC if upper else 0), MC)
        lanes = slice(n * L, (n + 1) * L)
        hh = _dot(u_v[rows, :], wout_v[:, lanes]) * 0.25
        if upper:
            ya = _dot(Fi_v[:, 0:P], Z_v[a * 2 * P:a * 2 * P + P, lanes])
            yb = _dot(Fi_v[:, P:2 * P], Z_v[a * 2 * P + P:(a + 1) * 2 * P, lanes])
            y = ya - yb
            lo = ya + yb
            for j in range(MC // 8):
                yl_v[n, (7 - j) * 8:(8 - j) * 8, :] = jnp.take_along_axis(lo[j * 8:(j + 1) * 8], rev8, axis=0)
        else:
            y = yl_v[n]
        gate = hh + hh * jnp.tanh(hh)
        s = xn_v[rows, lanes].astype(F32) * y
        o_v[rows, lanes] = (x_v[rows, lanes].astype(F32) + s * gate).astype(BF16)

    def job_big(i, bg, pending, budget):
        a0, a1 = _blocks_of_step(i)
        KG = 512
        count = [0]

        def lhs(j, sub, cols):
            if j == 2:
                return wsp_v[i * TM + sub:i * TM + sub + MC, cols]
            if j == 3:
                return wsp_v[i * TM + P + sub:i * TM + P + sub + MC, HK + cols.start:HK + cols.stop]
            r0 = ((i % 2) * 5 + {0: 0, 1: 1, 4: 2, 5: 3, 6: 4}[j]) * P + sub
            return Lc_v[r0:r0 + MC, cols]

        def prod(j, sub, n, acc=None):
            for kg in range(HK // KG):
                ks = slice(kg * KG, (kg + 1) * KG)
                p = _dot(lhs(j, sub, ks), R_v[j * HK + kg * KG:j * HK + (kg + 1) * KG, n * L:(n + 1) * L])
                acc = p if acc is None else acc + p
                bg.run(budget)
            count[0] += 1
            return acc

        def maybe_tail():
            if pending and count[0] >= 3:
                tail_piece(*pending.pop(0))
                bg.run(budget)

        def emit(a, sub, n, g):
            rows = pl.ds(a * P + sub, MC)
            lanes = slice(n * L, (n + 1) * L)
            u_v[rows, lanes] = (z1_v[rows, lanes] * (g + bcol_v[rows, :])).astype(BF16)

        for sub in (0, MC):
            for n in range(HN // L):
                m2 = prod(1, sub, n)
                m4 = prod(3, sub, n)
                emit(a1, sub, n, m2 + m4)
                maybe_tail()
                m3 = prod(2, sub, n)
                t22 = m3 - m2
                m5 = prod(4, sub, n)
                emit(a0, sub, n + HN // L, m3 + m5)
                t11 = m4 - m5
                maybe_tail()
                m1 = prod(0, sub, n)
                maybe_tail()
                emit(a0, sub, n, prod(6, sub, n, t11 + m1))
                emit(a1, sub, n + HN // L, prod(5, sub, n, t22 + m1))
                maybe_tail()

    if _ONLY is not None:
        for r_ in (xn_u, z1_v, R_u, Lc_u, zf_v, zg_v, kv_u, u_u, X_v, H_v, G_v, Z_u, kf_v):
            c_ = pltpu.make_async_copy(r_, r_, sem_small.at[0])
            c_.start()
            c_.wait()

    start(cp_small())
    cp_x(0).start()
    cp_win(2).start()

    kk = _odd_freq(jax.lax.broadcasted_iota(jnp.int32, (P, P), 0))
    nn = jax.lax.broadcasted_iota(jnp.int32, (P, P), 1)
    fc, fs = _cos_sin((kk * (4 * nn - 127)) & 2047)
    F_v[0:P, 0:P] = fc.astype(BF16)
    F_v[P:2 * P, 0:P] = (-fs).astype(BF16)
    kk = _odd_freq(jax.lax.broadcasted_iota(jnp.int32, (MC, P), 1))
    mm = jax.lax.broadcasted_iota(jnp.int32, (MC, P), 0)
    ic, is_ = _cos_sin((kk * (4 * mm + 2)) & 2047)
    Fi_v[:, 0:P] = (ic * (1.0 / P)).astype(BF16)
    Fi_v[:, P:2 * P] = (is_ * (1.0 / P)).astype(BF16)
    cp_x(1).start()
    cp_win(3).start()

    wait(cp_small())
    brow = b_in[...].astype(F32).reshape(1, S)
    for j in range(NB):
        bcol_v[j * P:(j + 1) * P, :] = jnp.broadcast_to(brow[:, j * P:(j + 1) * P], (P, P)).T
    sk = sk_in[...].astype(F32)
    for t in range(4):
        sk_v[t] = jnp.broadcast_to(sk[t:t + 1], (8, D))
    kf_v[:, 0:8, :] = jnp.zeros((D // L, 8, L), F32)
    drow = d_in[...].astype(F32).reshape(1, D)
    dre = fc[:, 0:1] * drow
    dim = fs[:, 0:1] * drow
    H_v[0:64, :] = -dim[0:64]
    H_v[64:P, :] = dim[64:P]
    H_v[P:P + 64, :] = -dre[0:64]
    H_v[P + 64:2 * P, :] = dre[64:P]

    cp_x(0).wait()
    for s in range(TM // 16):
        ln_x(0, s)

    LAG = 2

    def conv_dma(g):
        t = g - LAG
        if 0 <= t + 1 < NT:
            start(cp_conv(t + 1))
        if 0 <= t < NT:
            wait(cp_conv(t))

    def interleave(a, b):
        out = []
        for j in range(max(len(a), len(b))):
            out += a[j:j + 1] + b[j:j + 1]
        return out

    def p1_a():
        for m in range(TM // MC):
            job_z(0, m, range(6, 9))

    def p1_b():
        tied = tasks(ln_x, 1)
        for m in range(TM // MC):
            job_z(0, m, range(9, 12), tied=tied, ntied=(2, 2, 2))

    def p1_c():
        tied = interleave(tasks(ln_x, 2), tasks(ln_z2, 0))
        for m in range(TM // MC):
            job_z(1, m, range(6, 12), tied=tied, ntied=(2, 1, 2, 1, 2, 1))

    def p1_d():
        tied = tasks(ln_z2, 1)
        for t in range(2):
            for m in range(TM // MC):
                job_z(t, m, range(6), tied=tied, ntied=(1, 0, 1, 0, 1, 0))

    cp_win(2).wait()
    cp_x(2).start()
    cp_win(0).start()
    cp_win(1).start()
    block(p1_a, 'p1_a')
    cp_x(1).wait()
    cp_win(3).wait()
    block(p1_b, 'p1_b')
    start(cp_conv(0))
    cp_x(3).start()
    cp_x(2).wait()
    block(p1_c, 'p1_c')
    cp_win(0).wait()
    cp_win(1).wait()
    block(p1_d, 'p1_d')

    def p1_dma(i):
        if i + 2 < NT:
            cp_x(i + 2).start()
        if i >= 5:
            start(cp_wsp(i - 5))
        if i == 3:
            cp_wout().start()
        conv_dma(i)
        if i + 1 < NT:
            cp_x(i + 1).wait()
        else:
            wait(cp_wsp(0))

    def p1_step(i):
        bg = _Background()
        t = i - LAG
        bg.add(kv_gen(t))
        if i == NT - 1:
            bg.add(acomb_gen(0))
        tied = interleave(tasks(ln_x, i + 1) if i + 1 < NT else [], tasks(ln_z2, i - 1) if i > 2 else [])
        last = i == NT - 1
        ntied = (1, 1, 1, 1, 1, 0, 0, 0, 0, 0, 0, 0) if last else (1, 1, 0, 1, 1, 0) * 2
        for m in range(TM // MC):
            job_z(i, m, list(range(6, 12)) + list(range(6)), bg, (0, 0, 0, 0, 0, 90, 0, 0, 0, 90, 90, 90) if last else (0, 0, 60, 0, 0, 60) * 2,
                  tied, ntied, last)
            if m == 0:
                job_h(t, bg, 90)
        assert not tied
        if t >= 1:
            job_x(t - 1, bg, 180)
        bg.drain()

    for i in range(2, NT):
        p1_dma(i)
        block(lambda i=i: p1_step(i), f'p1_{i}')

    def p2_dma(i):
        if i == 0:
            cp_wout().wait()
        if i >= 2:
            start(cp_out(i - 2))
        if i >= 3:
            wait(cp_out(i - 3))
        if i + 3 < NT:
            start(cp_wsp(i + 3))
        conv_dma(NT + i)
        if i + 1 < NT:
            wait(cp_wsp(i + 1))

    def tails_of(i):
        return [(a, upper, n) for a in _blocks_of_step(i) for upper in (True, False) for n in range(D // L)]

    def p2_step(i):
        bg = _Background()
        pending = tails_of(i - 1) if i > 0 else []
        total = 17 * 40 * 16
        slots = 84 + len(pending)
        if i + 1 < NT:
            bg.add(acomb_gen(i + 1))
            total += 32 * 46
        t = NT + i - LAG
        if t < NT:
            bg.add(kv_gen(t))
            total += 20 * 90
            slots += 8
        if t - 1 < NT:
            slots += 8
        for a in _blocks_of_step(i):
            bg.add(freq_gen(a))
        budget = total / (slots + 1.0)
        bg.run(budget)
        if t - 1 < NT:
            job_x(t - 1, bg, 2 * budget)
        if t < NT:
            job_h(t, bg, 2 * budget)
        job_big(i, bg, pending, budget)
        for t_ in pending:
            tail_piece(*t_)
        bg.drain()

    for i in range(NT):
        p2_dma(i)
        block(lambda i=i: p2_step(i), f'p2_{i}')

    def p2_last():
        a0, a1 = _blocks_of_step(NT - 1)
        for t_ in tails_of(NT - 1):
            tail_piece(*t_)
            if t_ == (a0, False, D // L - 1):
                start(cp_out(NT - 1, (0,)))

    p2_dma(NT)
    block(p2_last, 'p2_last')
    start(cp_out(NT - 1, (1,)))
    wait(cp_out(NT - 2))
    wait(cp_out(NT - 1))
    if _ONLY is not None:
        for r_ in (xn_u, z1_v, R_u, Lc_u, zf_v, zg_v, kv_u, u_u, X_v, H_v, G_v, Z_u, kf_v):
            c_ = pltpu.make_async_copy(r_, r_, sem_small.at[0])
            c_.start()
            c_.wait()


@jax.jit
def pallas_recurrent_scan__ssm_conv_h3__mixer_gmlp__prompt_kernel(
    A_q: jax.Array,
    A_k: jax.Array,
    A_v: jax.Array,
    A_shift_k: jax.Array,
    A_ssm_k: jax.Array,
    A_ssm_D: jax.Array,
    B_x: jax.Array,
    B_w_in: jax.Array,
    B_w_sp: jax.Array,
    B_b_sp: jax.Array,
    B_w_out: jax.Array,
):
    del B_x
    hbm = pl.BlockSpec(memory_space=pl.ANY)

    def bf16_buf(*shape):
        return pltpu.VMEM(shape[:-2] + (shape[-2] // 2, shape[-1]), U32)

    return pl.pallas_call(
        _kernel,
        out_shape=jax.ShapeDtypeStruct((1, S, D), BF16),
        in_specs=[pl.BlockSpec(memory_space=pltpu.SMEM)] + [hbm] * 10,
        out_specs=hbm,
        scratch_shapes=[
            bf16_buf(S, D),
            bf16_buf(S, D),
            bf16_buf(S, D),
            bf16_buf(NT, D, TM),
            bf16_buf(D, 2 * FH),
            bf16_buf(S, S),
            bf16_buf(FH, D),
            pltpu.VMEM((S, D), BF16),
            pltpu.VMEM((4, D), BF16),
            pltpu.VMEM((D,), BF16),
            pltpu.VMEM((S,), BF16),
            bf16_buf(S, D),
            pltpu.VMEM((S, FH), F32),
            bf16_buf(7 * HK, HN),
            bf16_buf(2 * 5 * P, HK),
            pltpu.VMEM((HK, FH), F32),
            pltpu.VMEM((2, TM, FH), F32),
            bf16_buf(S, D),
            bf16_buf(S, FH),
            pltpu.VMEM((NB, 2 * P, D), F32),
            pltpu.VMEM((2 * P, D), F32),
            pltpu.VMEM((NB, 2 * P, D), F32),
            bf16_buf(NB * 2 * P, D),
            pltpu.VMEM((D // L, MC, L), F32),
            bf16_buf(2 * P, 2 * P),
            bf16_buf(MC, 2 * P),
            pltpu.VMEM((S, L), F32),
            pltpu.VMEM((4, 8, D), F32),
            pltpu.VMEM((D // L, S + 8, L), F32),
            pltpu.SemaphoreType.DMA((1,)),
            pltpu.SemaphoreType.DMA((3,)),
            pltpu.SemaphoreType.DMA((2,)),
            pltpu.SemaphoreType.DMA((4,)),
            pltpu.SemaphoreType.DMA((5,)),
            pltpu.SemaphoreType.DMA((3,)),
        ],
        compiler_params=pltpu.CompilerParams(vmem_limit_bytes=100 * 1024 * 1024),
    )(jnp.ones((1,), jnp.int32), A_q, A_k, A_v, A_shift_k.T, A_ssm_k, A_ssm_D, B_w_in, B_w_sp, B_b_sp, B_w_out)
```

```python
import math

import jax
import jax.numpy as jnp
import jax.experimental.pallas as pl
import jax.experimental.pallas.tpu as pltpu

S = 2048
D = 640
FH = 768
P = 128
NB = S // P
TM = 256
NT = S // TM
MC = 64
L = 128
HK = S // 2
HN = FH // 2
WIN_CHUNKS = ((6, 7), (7, 9), (9, 12), (0, 3), (3, 6))
EPS = 1e-5
F32 = jnp.float32
BF16 = jnp.bfloat16
U32 = jnp.uint32
GELU_C = math.sqrt(2.0 / math.pi)
NT_DIMS = (((1,), (1,)), ((), ()))
_ONLY = None


def _dot(a, b):
    return jnp.dot(a, b, preferred_element_type=F32)


def _cos_sin(m):
    q = (m + 256) >> 9
    x = (m - (q << 9)).astype(F32) * (2.0 * math.pi / 2048.0)
    x2 = x * x
    s = x * (1.0 + x2 * (-1.0 / 6 + x2 * (1.0 / 120 + x2 * (-1.0 / 5040 + x2 * (1.0 / 362880)))))
    c = 1.0 + x2 * (-0.5 + x2 * (1.0 / 24 + x2 * (-1.0 / 720 + x2 * (1.0 / 40320 - x2 * (1.0 / 3628800)))))
    swap = (q & 1) == 1
    c0 = jnp.where(swap, s, c)
    s0 = jnp.where(swap, c, s)
    cos = jnp.where(((q + 1) & 2) == 2, -c0, c0)
    sin = jnp.where((q & 2) == 2, -s0, s0)
    return cos, sin


def _odd_freq(r):
    return jnp.where(r < 64, 4 * r + 1, 4 * r - 253)


def _gelu2(z):
    u = z * (GELU_C + (GELU_C * 0.044715) * (z * z))
    return z + z * jnp.tanh(u)


def _signzero(z):
    bits = jax.lax.bitcast_convert_type(z, U32) & jnp.uint32(0x80000000)
    return jax.lax.bitcast_convert_type(bits, F32)


def _ln(x, eps, tie=None):
    n = x.shape[-1]
    part = x[:, 0:L]
    for j in range(1, n // L):
        part = part + x[:, j * L:(j + 1) * L]
    if tie is not None:
        part = part + tie
    m = jnp.sum(part, axis=-1, keepdims=True) * (1.0 / n)
    xc = x - m
    v = jnp.sum(xc * xc, axis=-1, keepdims=True) * (1.0 / n)
    return xc * jax.lax.rsqrt(v + eps)


def _blocks_of_step(i):
    return (NT - 1 - i, NT + i)


class _Background:
    def __init__(self):
        self.q = []
        self.credit = 0.0

    def add(self, gen):
        self.q.append(gen)

    def run(self, budget):
        self.credit += budget
        while self.q and self.credit > 0:
            try:
                self.credit -= next(self.q[0])
            except StopIteration:
                self.q.pop(0)
        if not self.q:
            self.credit = 0.0

    def drain(self):
        while self.q:
            self.run(1e9)


def _kernel(one_ref, q_hbm, k_hbm, v_hbm, sk_hbm, h_hbm, d_hbm, win_hbm, wsp_hbm, b_hbm, wout_hbm,
            o_hbm,
            x_u, k_u, v_u, h_u, win_u, wsp_u, wout_u, o_v, sk_in, d_in, b_in,
            xn_u, z1_v, R_u, Lc_u, zf_v, zg_v, kv_u, u_u, X_v, H_v, G_v, Z_u, yl_v, F_u, Fi_u, bcol_v, ph_v, sk_v, kf_v,
            sem_small, sem_x, sem_conv, sem_wsp, sem_w, sem_out):
    x_v, k_v, v_v, h_v, win_v, wsp_v, wout_v, xn_v, R_v, Lc_v, kv_v, u_v, Z_v, F_v, Fi_v = [
        r.bitcast(BF16) for r in (x_u, k_u, v_u, h_u, win_u, wsp_u, wout_u, xn_u, R_u, Lc_u, kv_u, u_u, Z_u, F_u,
                                  Fi_u)]

    def cp_small():
        return [pltpu.make_async_copy(s_, d_, sem_small.at[0])
                for s_, d_ in ((d_hbm, d_in), (sk_hbm, sk_in), (b_hbm, b_in))]

    def cp_x(t):
        return pltpu.make_async_copy(q_hbm.at[0, pl.ds(t * TM, TM)], x_v.at[pl.ds(t * TM, TM)], sem_x.at[t % 3])

    def cp_conv(t):
        rows = pl.ds(t * TM, TM)
        sem = sem_conv.at[t % 2]
        return [pltpu.make_async_copy(h_hbm.at[:, rows], h_v.at[t], sem),
                pltpu.make_async_copy(k_hbm.at[0, rows], k_v.at[rows], sem),
                pltpu.make_async_copy(v_hbm.at[0, rows], v_v.at[rows], sem)]

    def cp_wsp(i):
        return [pltpu.make_async_copy(wsp_hbm.at[pl.ds(a * P, P)], wsp_v.at[pl.ds(i * TM + half * P, P)],
                                      sem_wsp.at[i % 4]) for half, a in enumerate(_blocks_of_step(i))]

    def cp_win(c):
        lo, hi = WIN_CHUNKS[c]
        cols = pl.ds(lo * L, (hi - lo) * L)
        return pltpu.make_async_copy(win_hbm.at[:, cols], win_v.at[:, cols], sem_w.at[c])

    def cp_wout():
        return pltpu.make_async_copy(wout_hbm, wout_v, sem_w.at[0])

    def cp_out(i, which=(0, 1)):
        return [pltpu.make_async_copy(o_v.at[pl.ds(a * P, P)], o_hbm.at[0, pl.ds(a * P, P)], sem_out.at[i % 3])
                for a in [_blocks_of_step(i)[w] for w in which]]

    def start(cs):
        for c in cs:
            c.start()

    def wait(cs):
        for c in cs:
            c.wait()

    always = one_ref[0] == 1

    def block(fn, name):
        if _ONLY is None or name in _ONLY:
            pl.when(always)(fn)

    def ln_x(t, s, tie=None):
        rows = pl.ds(t * TM + s * 16, 16)
        xn_v[rows, :] = _ln(x_v[rows, :].astype(F32), EPS, tie).astype(BF16)

    def ln_z2(t, s, tie=None):
        y = _ln(zg_v[t % 2, s * 16:(s + 1) * 16, :], 4.0 * EPS, tie)
        lo, hi = y[:, :HN], y[:, HN:]
        r = (t * TM + s * 16) % HK
        rows = pl.ds(r, 16)
        if t < NT // 2:
            zf_v[rows, :] = y
            R_v[pl.ds(1 * HK + r, 16), :] = lo.astype(BF16)
            R_v[pl.ds(5 * HK + r, 16), :] = (lo + hi).astype(BF16)
        else:
            b11 = zf_v[rows, :HN]
            R_v[pl.ds(0 * HK + r, 16), :] = (b11 + hi).astype(BF16)
            R_v[pl.ds(2 * HK + r, 16), :] = (zf_v[rows, HN:] - hi).astype(BF16)
            R_v[pl.ds(3 * HK + r, 16), :] = (lo - b11).astype(BF16)
            R_v[pl.ds(4 * HK + r, 16), :] = hi.astype(BF16)
            R_v[pl.ds(6 * HK + r, 16), :] = (lo + hi).astype(BF16)

    def acomb_gen(i):
        for r in range(P // 16):
            for c in range(HK // 256):
                top = pl.ds(i * TM + r * 16, 16)
                bot = pl.ds(i * TM + P + r * 16, 16)
                c1 = slice(c * 256, (c + 1) * 256)
                c2 = slice(HK + c * 256, HK + (c + 1) * 256)
                a11 = wsp_v[top, c1].astype(F32)
                a12 = wsp_v[top, c2].astype(F32)
                a21 = wsp_v[bot, c1].astype(F32)
                a22 = wsp_v[bot, c2].astype(F32)
                r0 = (i % 2) * 5 * P + r * 16
                Lc_v[pl.ds(r0 + 0 * P, 16), c1] = (a11 + a22).astype(BF16)
                Lc_v[pl.ds(r0 + 1 * P, 16), c1] = (a21 + a22).astype(BF16)
                Lc_v[pl.ds(r0 + 2 * P, 16), c1] = (a11 + a12).astype(BF16)
                Lc_v[pl.ds(r0 + 3 * P, 16), c1] = (a21 - a11).astype(BF16)
                Lc_v[pl.ds(r0 + 4 * P, 16), c1] = (a12 - a22).astype(BF16)
                yield 46

    def tasks(fn, t):
        return [lambda tie, s=s: fn(t, s, tie) for s in range(TM // 16)]

    def kv_gen(t):
        for m in range(TM // MC):
            r = t * TM + m * MC
            for l in range(D // L):
                lanes = slice(l * L, (l + 1) * L)
                kf = k_v[pl.ds(r, MC), lanes].astype(F32)
                kf_v[l, pl.ds(r + 8, MC), :] = kf
                ks = kf * sk_v[0, 0:1, lanes]
                for tap in range(1, 4):
                    ks = ks + kf_v[l, pl.ds(r + 8 - tap, MC), :] * sk_v[tap, 0:1, lanes]
                kv = ks * v_v[pl.ds(r, MC), lanes].astype(F32)
                kv_v[pl.ds(r, MC), lanes] = kv.astype(BF16)
                yield 90

    def freq_gen(a):
        for r in range(P // 16):
            re = pl.ds(r * 16, 16)
            im = pl.ds(P + r * 16, 16)
            for l in range(D // L):
                lanes = slice(l * L, (l + 1) * L)
                ar = ai = None
                for c in range(a + 1):
                    xr = X_v[c, re, lanes]
                    xi = X_v[c, im, lanes]
                    gr = G_v[a - c, re, lanes]
                    gi = G_v[a - c, im, lanes]
                    pr = xr * gr - xi * gi
                    pi = xr * gi + xi * gr
                    ar = pr if ar is None else ar + pr
                    ai = pi if ai is None else ai + pi
                    if c == a:
                        Z_v[pl.ds(a * 2 * P + r * 16, 16), lanes] = ar.astype(BF16)
                        Z_v[pl.ds(a * 2 * P + P + r * 16, 16), lanes] = ai.astype(BF16)
                    yield 16

    def job_h(t, bg, budget):
        prev = [H_v[qd * 64:(qd + 1) * 64, :] for qd in range(4)]
        for half in range(2):
            j = 2 * t + half
            cur = []
            for part in range(2):
                hp = jax.lax.dot_general(F_v[part * P:(part + 1) * P, 0:P], h_v[t, :, half * P:(half + 1) * P],
                                         NT_DIMS, preferred_element_type=F32)
                for qd in (2 * part, 2 * part + 1):
                    hq = hp[(qd % 2) * 64:(qd % 2 + 1) * 64]
                    cur.append(hq)
                    other = prev[(qd + 2) % 4]
                    G_v[j, qd * 64:(qd + 1) * 64, :] = hq - other if qd in (0, 3) else hq + other
                bg.run(budget)
            prev = cur
        if t + 1 < NT:
            for qd in range(4):
                H_v[qd * 64:(qd + 1) * 64, :] = prev[qd]

    def job_x(t, bg, budget):
        for half in range(2):
            j = 2 * t + half
            for part in range(2):
                X_v[j, part * P:(part + 1) * P, :] = _dot(F_v[part * P:(part + 1) * P, 0:P],
                                                          kv_v[j * P:(j + 1) * P, :])
                bg.run(budget)

    def job_z(t, m, cols, bg=None, budgets=None, tied=None, ntied=None, inline_ln=False):
        rows = pl.ds(t * TM + m * MC, MC)
        for j, n in enumerate(cols):
            z = _gelu2(_dot(xn_v[rows, :], win_v[:, n * L:(n + 1) * L]))
            if n < FH // L:
                z1_v[rows, n * L:(n + 1) * L] = z
            else:
                zg_v[t % 2, m * MC:(m + 1) * MC, n * L - FH:(n + 1) * L - FH] = z
            if tied and ntied[j]:
                tie = _signzero(z[0:16])
                for _ in range(ntied[j]):
                    if tied:
                        tied.pop(0)(tie)
            if inline_ln and n == 2 * FH // L - 1:
                for s in range(4 * m, 4 * m + 4):
                    ln_z2(t, s)
            if bg is not None:
                bg.run(budgets[j])

    rev8 = 7 - jax.lax.broadcasted_iota(jnp.int32, (8, L), 0)

    def tail_piece(a, upper, n):
        rows = pl.ds(a * P + (MC if upper else 0), MC)
        lanes = slice(n * L, (n + 1) * L)
        hh = _dot(u_v[rows, :], wout_v[:, lanes]) * 0.25
        if upper:
            ya = _dot(Fi_v[:, 0:P], Z_v[a * 2 * P:a * 2 * P + P, lanes])
            yb = _dot(Fi_v[:, P:2 * P], Z_v[a * 2 * P + P:(a + 1) * 2 * P, lanes])
            y = ya - yb
            lo = ya + yb
            for j in range(MC // 8):
                yl_v[n, (7 - j) * 8:(8 - j) * 8, :] = jnp.take_along_axis(lo[j * 8:(j + 1) * 8], rev8, axis=0)
        else:
            y = yl_v[n]
        gate = hh + hh * jnp.tanh(hh)
        s = xn_v[rows, lanes].astype(F32) * y
        o_v[rows, lanes] = (x_v[rows, lanes].astype(F32) + s * gate).astype(BF16)

    def job_big(i, bg, pending, budget):
        a0, a1 = _blocks_of_step(i)
        KG = 512
        count = [0]

        def lhs(j, sub, cols):
            if j == 2:
                return wsp_v[i * TM + sub:i * TM + sub + MC, cols]
            if j == 3:
                return wsp_v[i * TM + P + sub:i * TM + P + sub + MC, HK + cols.start:HK + cols.stop]
            r0 = ((i % 2) * 5 + {0: 0, 1: 1, 4: 2, 5: 3, 6: 4}[j]) * P + sub
            return Lc_v[r0:r0 + MC, cols]

        def prod(j, sub, n, acc=None):
            for kg in range(HK // KG):
                ks = slice(kg * KG, (kg + 1) * KG)
                p = _dot(lhs(j, sub, ks), R_v[j * HK + kg * KG:j * HK + (kg + 1) * KG, n * L:(n + 1) * L])
                acc = p if acc is None else acc + p
                bg.run(budget)
            count[0] += 1
            return acc

        def maybe_tail():
            if pending and count[0] >= 3:
                tail_piece(*pending.pop(0))
                bg.run(budget)

        def emit(a, sub, n, g):
            rows = pl.ds(a * P + sub, MC)
            lanes = slice(n * L, (n + 1) * L)
            u_v[rows, lanes] = (z1_v[rows, lanes] * (g + bcol_v[rows, :])).astype(BF16)

        for sub in (0, MC):
            for n in range(HN // L):
                m2 = prod(1, sub, n)
                m4 = prod(3, sub, n)
                emit(a1, sub, n, m2 + m4)
                maybe_tail()
                m3 = prod(2, sub, n)
                t22 = m3 - m2
                m5 = prod(4, sub, n)
                emit(a0, sub, n + HN // L, m3 + m5)
                t11 = m4 - m5
                maybe_tail()
                m1 = prod(0, sub, n)
                maybe_tail()
                emit(a0, sub, n, prod(6, sub, n, t11 + m1))
                emit(a1, sub, n + HN // L, prod(5, sub, n, t22 + m1))
                maybe_tail()

    if _ONLY is not None:
        for r_ in (xn_u, z1_v, R_u, Lc_u, zf_v, zg_v, kv_u, u_u, X_v, H_v, G_v, Z_u, kf_v):
            c_ = pltpu.make_async_copy(r_, r_, sem_small.at[0])
            c_.start()
            c_.wait()

    cp_x(0).start()
    cp_x(1).start()
    for c in range(5):
        cp_win(c).start()
    cp_x(2).start()
    start(cp_small())

    kk = _odd_freq(jax.lax.broadcasted_iota(jnp.int32, (P, P), 0))
    nn = jax.lax.broadcasted_iota(jnp.int32, (P, P), 1)
    fc, fs = _cos_sin((kk * (4 * nn - 127)) & 2047)
    F_v[0:P, 0:P] = fc.astype(BF16)
    F_v[P:2 * P, 0:P] = (-fs).astype(BF16)
    fc, fs = _cos_sin((kk * (-127)) & 2047)
    ph_v[0] = fc
    ph_v[1] = fs
    kk = _odd_freq(jax.lax.broadcasted_iota(jnp.int32, (MC, P), 1))
    mm = jax.lax.broadcasted_iota(jnp.int32, (MC, P), 0)
    ic, is_ = _cos_sin((kk * (4 * mm + 2)) & 2047)
    Fi_v[:, 0:P] = (ic * (1.0 / P)).astype(BF16)
    Fi_v[:, P:2 * P] = (is_ * (1.0 / P)).astype(BF16)
    kf_v[:, 0:8, :] = jnp.zeros((D // L, 8, L), F32)

    for t in range(2):
        cp_x(t).wait()
        for s in range(TM // 16):
            ln_x(t, s)

    def small_setup():
        sk = sk_in[...].astype(F32)
        for t in range(4):
            sk_v[t] = jnp.broadcast_to(sk[t:t + 1], (8, D))
        drow = d_in[...].astype(F32).reshape(1, D)
        for l in range(D // L):
            lanes = slice(l * L, (l + 1) * L)
            dre = ph_v[0] * drow[:, lanes]
            dim = ph_v[1] * drow[:, lanes]
            H_v[0:64, lanes] = -dim[0:64]
            H_v[64:P, lanes] = dim[64:P]
            H_v[P:P + 64, lanes] = -dre[0:64]
            H_v[P + 64:2 * P, lanes] = dre[64:P]
        brow = b_in[...].astype(F32).reshape(1, S)
        for j in range(NB):
            bcol_v[j * P:(j + 1) * P, :] = jnp.broadcast_to(brow[:, j * P:(j + 1) * P], (P, P)).T

    LAG = 2

    def conv_dma(g):
        t = g - LAG
        if 0 <= t + 1 < NT:
            start(cp_conv(t + 1))
        if 0 <= t < NT:
            wait(cp_conv(t))

    def interleave(*lists):
        out = []
        for j in range(max(len(a) for a in lists)):
            for a in lists:
                out += a[j:j + 1]
        return out

    def p1_first(c):
        tied = []
        if c == 3:
            tied = tasks(ln_z2, 0) + tasks(ln_z2, 1)[:6]
        if c == 4:
            tied = interleave(tasks(ln_x, 2), tasks(ln_z2, 1)[6:])
            small_setup()
        for t in range(2):
            for m in range(TM // MC):
                job_z(t, m, range(*WIN_CHUNKS[c]), tied=tied, ntied=(2 if m == 0 else 1, 1, 1))
        assert not tied

    for c in range(5):
        cp_win(c).wait()
        if c == 2:
            start(cp_conv(0))
            cp_x(3).start()
        if c == 4:
            cp_x(2).wait()
            wait(cp_small())
        block(lambda c=c: p1_first(c), f'p1_f{c}')

    def p1_dma(i):
        if i + 2 < NT:
            cp_x(i + 2).start()
        if i >= 5:
            start(cp_wsp(i - 5))
        if i == 3:
            cp_wout().start()
        conv_dma(i)
        if i + 1 < NT:
            cp_x(i + 1).wait()
        else:
            wait(cp_wsp(0))

    def p1_step(i):
        bg = _Background()
        t = i - LAG
        bg.add(kv_gen(t))
        if i == NT - 1:
            bg.add(acomb_gen(0))
        tied = interleave(tasks(ln_x, i + 1) if i + 1 < NT else [], tasks(ln_z2, i - 1) if i > 2 else [])
        last = i == NT - 1
        ntied = (1, 1, 1, 1, 1, 0, 0, 0, 0, 0, 0, 0) if last else (1, 1, 0, 1, 1, 0) * 2
        for m in range(TM // MC):
            job_z(i, m, list(range(6, 12)) + list(range(6)), bg, (0, 0, 0, 0, 0, 90, 0, 0, 0, 90, 90, 90) if last else (0, 0, 60, 0, 0, 60) * 2,
                  tied, ntied, last)
            if m == 0:
                job_h(t, bg, 90)
        assert not tied
        if t >= 1:
            job_x(t - 1, bg, 180)
        bg.drain()

    for i in range(2, NT):
        p1_dma(i)
        block(lambda i=i: p1_step(i), f'p1_{i}')

    def p2_dma(i):
        if i == 0:
            cp_wout().wait()
        if i >= 2:
            start(cp_out(i - 2))
        if i >= 3:
            wait(cp_out(i - 3))
        if i + 3 < NT:
            start(cp_wsp(i + 3))
        conv_dma(NT + i)
        if i + 1 < NT:
            wait(cp_wsp(i + 1))

    def tails_of(i):
        return [(a, upper, n) for a in _blocks_of_step(i) for upper in (True, False) for n in range(D // L)]

    def p2_step(i):
        bg = _Background()
        pending = tails_of(i - 1) if i > 0 else []
        total = 17 * 40 * 16
        slots = 84 + len(pending)
        if i + 1 < NT:
            bg.add(acomb_gen(i + 1))
            total += 32 * 46
        t = NT + i - LAG
        if t < NT:
            bg.add(kv_gen(t))
            total += 20 * 90
            slots += 8
        if t - 1 < NT:
            slots += 8
        for a in _blocks_of_step(i):
            bg.add(freq_gen(a))
        budget = total / (slots + 1.0)
        bg.run(budget)
        if t - 1 < NT:
            job_x(t - 1, bg, 2 * budget)
        if t < NT:
            job_h(t, bg, 2 * budget)
        job_big(i, bg, pending, budget)
        for t_ in pending:
            tail_piece(*t_)
        bg.drain()

    for i in range(NT):
        p2_dma(i)
        block(lambda i=i: p2_step(i), f'p2_{i}')

    def p2_last():
        a0, a1 = _blocks_of_step(NT - 1)
        for t_ in tails_of(NT - 1):
            tail_piece(*t_)
            if t_ == (a0, False, D // L - 1):
                start(cp_out(NT - 1, (0,)))

    p2_dma(NT)
    block(p2_last, 'p2_last')
    start(cp_out(NT - 1, (1,)))
    wait(cp_out(NT - 2))
    wait(cp_out(NT - 1))
    if _ONLY is not None:
        for r_ in (xn_u, z1_v, R_u, Lc_u, zf_v, zg_v, kv_u, u_u, X_v, H_v, G_v, Z_u, kf_v):
            c_ = pltpu.make_async_copy(r_, r_, sem_small.at[0])
            c_.start()
            c_.wait()


@jax.jit
def pallas_recurrent_scan__ssm_conv_h3__mixer_gmlp__prompt_kernel(
    A_q: jax.Array,
    A_k: jax.Array,
    A_v: jax.Array,
    A_shift_k: jax.Array,
    A_ssm_k: jax.Array,
    A_ssm_D: jax.Array,
    B_x: jax.Array,
    B_w_in: jax.Array,
    B_w_sp: jax.Array,
    B_b_sp: jax.Array,
    B_w_out: jax.Array,
):
    del B_x
    hbm = pl.BlockSpec(memory_space=pl.ANY)

    def bf16_buf(*shape):
        return pltpu.VMEM(shape[:-2] + (shape[-2] // 2, shape[-1]), U32)

    return pl.pallas_call(
        _kernel,
        out_shape=jax.ShapeDtypeStruct((1, S, D), BF16),
        in_specs=[pl.BlockSpec(memory_space=pltpu.SMEM)] + [hbm] * 10,
        out_specs=hbm,
        scratch_shapes=[
            bf16_buf(S, D),
            bf16_buf(S, D),
            bf16_buf(S, D),
            bf16_buf(NT, D, TM),
            bf16_buf(D, 2 * FH),
            bf16_buf(S, S),
            bf16_buf(FH, D),
            pltpu.VMEM((S, D), BF16),
            pltpu.VMEM((4, D), BF16),
            pltpu.VMEM((D,), BF16),
            pltpu.VMEM((S,), BF16),
            bf16_buf(S, D),
            pltpu.VMEM((S, FH), F32),
            bf16_buf(7 * HK, HN),
            bf16_buf(2 * 5 * P, HK),
            pltpu.VMEM((HK, FH), F32),
            pltpu.VMEM((2, TM, FH), F32),
            bf16_buf(S, D),
            bf16_buf(S, FH),
            pltpu.VMEM((NB, 2 * P, D), F32),
            pltpu.VMEM((2 * P, D), F32),
            pltpu.VMEM((NB, 2 * P, D), F32),
            bf16_buf(NB * 2 * P, D),
            pltpu.VMEM((D // L, MC, L), F32),
            bf16_buf(2 * P, 2 * P),
            bf16_buf(MC, 2 * P),
            pltpu.VMEM((S, L), F32),
            pltpu.VMEM((2, P, L), F32),
            pltpu.VMEM((4, 8, D), F32),
            pltpu.VMEM((D // L, S + 8, L), F32),
            pltpu.SemaphoreType.DMA((1,)),
            pltpu.SemaphoreType.DMA((3,)),
            pltpu.SemaphoreType.DMA((2,)),
            pltpu.SemaphoreType.DMA((4,)),
            pltpu.SemaphoreType.DMA((5,)),
            pltpu.SemaphoreType.DMA((3,)),
        ],
        compiler_params=pltpu.CompilerParams(vmem_limit_bytes=100 * 1024 * 1024),
    )(jnp.ones((1,), jnp.int32), A_q, A_k, A_v, A_shift_k.T, A_ssm_k, A_ssm_D, B_w_in, B_w_sp, B_b_sp, B_w_out)
```

```python
import math

import jax
import jax.numpy as jnp
import jax.experimental.pallas as pl
import jax.experimental.pallas.tpu as pltpu

S = 2048
D = 640
FH = 768
P = 128
NB = S // P
TM = 256
NT = S // TM
MC = 64
L = 128
HK = S // 2
HN = FH // 2
P2_GROUPS = ((0,), (1, 2), (3, 4), (5, 6), (7,))
STEP_BLOCKS = ((4, 5), (10, 11), (2, 3), (12, 13), (6, 7), (14, 15), (0, 1), (8, 9))
KV_COST, G_COST, A_COST = 110, 36, 56
WIN_CHUNKS = ((6, 7), (7, 9), (9, 12), (0, 3), (3, 6))
EPS = 1e-5
F32 = jnp.float32
BF16 = jnp.bfloat16
U32 = jnp.uint32
GELU_C = math.sqrt(2.0 / math.pi)
NT_DIMS = (((1,), (1,)), ((), ()))
_ONLY = None


def _dot(a, b):
    return jnp.dot(a, b, preferred_element_type=F32)


def _cos_sin(m):
    q = (m + 256) >> 9
    x = (m - (q << 9)).astype(F32) * (2.0 * math.pi / 2048.0)
    x2 = x * x
    s = x * (1.0 + x2 * (-1.0 / 6 + x2 * (1.0 / 120 + x2 * (-1.0 / 5040 + x2 * (1.0 / 362880)))))
    c = 1.0 + x2 * (-0.5 + x2 * (1.0 / 24 + x2 * (-1.0 / 720 + x2 * (1.0 / 40320 - x2 * (1.0 / 3628800)))))
    swap = (q & 1) == 1
    c0 = jnp.where(swap, s, c)
    s0 = jnp.where(swap, c, s)
    cos = jnp.where(((q + 1) & 2) == 2, -c0, c0)
    sin = jnp.where((q & 2) == 2, -s0, s0)
    return cos, sin


def _odd_freq(r):
    return jnp.where(r < 64, 4 * r + 1, 4 * r - 253)


def _gelu2(z):
    u = z * (GELU_C + (GELU_C * 0.044715) * (z * z))
    return z + z * jnp.tanh(u)


def _signzero(z):
    bits = jax.lax.bitcast_convert_type(z, U32) & jnp.uint32(0x80000000)
    return jax.lax.bitcast_convert_type(bits, F32)


def _ln(x, eps, tie=None, scale=None):
    n = x.shape[-1]
    part = x[:, 0:L]
    for j in range(1, n // L):
        part = part + x[:, j * L:(j + 1) * L]
    if tie is not None:
        part = part + tie
    m = jnp.sum(part, axis=-1, keepdims=True) * (1.0 / n)
    xc = x - m
    v = jnp.sum(xc * xc, axis=-1, keepdims=True) * (1.0 / n)
    rs = jax.lax.rsqrt(v + eps)
    if scale is not None:
        rs = rs * scale
    return xc * rs


def _blocks_of_step(i):
    return STEP_BLOCKS[i]


class _Background:
    def __init__(self):
        self.q = []
        self.credit = 0.0

    def add(self, gen):
        self.q.append(gen)

    def run(self, budget):
        self.credit += budget
        while self.q and self.credit > 0:
            try:
                self.credit -= next(self.q[0])
            except StopIteration:
                self.q.pop(0)
        if not self.q:
            self.credit = 0.0

    def drain(self):
        while self.q:
            self.run(1e9)


def _kernel(one_ref, q_hbm, k_hbm, v_hbm, sk_hbm, h_hbm, d_hbm, win_hbm, wsp_hbm, b_hbm, wout_hbm,
            o_hbm,
            x_u, k_u, v_u, h_u, win_u, wsp_u, wout_u, o_v, sk_in, d_in, b_in,
            xn_u, z1_v, R_u, Lc_u, zf_v, zg_v, kv_u, u_u, X_v, H_v, G_v, Z_u, yl_v, F_u, Fi_u, bcol_v, ph_v, sk_v, kf_v,
            sem_small, sem_x, sem_conv, sem_wsp, sem_w, sem_out):
    x_v, k_v, v_v, h_v, win_v, wsp_v, wout_v, xn_v, R_v, Lc_v, kv_v, u_v, Z_v, F_v, Fi_v = [
        r.bitcast(BF16) for r in (x_u, k_u, v_u, h_u, win_u, wsp_u, wout_u, xn_u, R_u, Lc_u, kv_u, u_u, Z_u, F_u,
                                  Fi_u)]

    def cp_small():
        return [pltpu.make_async_copy(s_, d_, sem_small.at[0])
                for s_, d_ in ((d_hbm, d_in), (sk_hbm, sk_in), (b_hbm, b_in))]

    def cp_x(t):
        return pltpu.make_async_copy(q_hbm.at[0, pl.ds(t * TM, TM)], x_v.at[pl.ds(t * TM, TM)], sem_x.at[t % 3])

    def cp_conv(t):
        rows = pl.ds(t * TM, TM)
        sem = sem_conv.at[t % 2]
        return [pltpu.make_async_copy(h_hbm.at[:, rows], h_v.at[t], sem),
                pltpu.make_async_copy(k_hbm.at[0, rows], k_v.at[rows], sem),
                pltpu.make_async_copy(v_hbm.at[0, rows], v_v.at[rows], sem)]

    def cp_wsp(i, which=(0, 1)):
        return [pltpu.make_async_copy(wsp_hbm.at[pl.ds(_blocks_of_step(i)[half] * P, P)],
                                      wsp_v.at[pl.ds(i * TM + half * P, P)], sem_wsp.at[i % 5]) for half in which]

    def cp_win(c):
        lo, hi = WIN_CHUNKS[c]
        cols = pl.ds(lo * L, (hi - lo) * L)
        return pltpu.make_async_copy(win_hbm.at[:, cols], win_v.at[:, cols], sem_w.at[c])

    def cp_wout():
        return pltpu.make_async_copy(wout_hbm, wout_v, sem_w.at[0])

    def cp_out(i, which=(0, 1)):
        return [pltpu.make_async_copy(o_v.at[pl.ds(a * P, P)], o_hbm.at[0, pl.ds(a * P, P)], sem_out.at[i % 5])
                for a in [_blocks_of_step(i)[w] for w in which]]

    def start(cs):
        for c in cs:
            c.start()

    def wait(cs):
        for c in cs:
            c.wait()

    always = one_ref[0] == 1

    def block(fn, name):
        if _ONLY is None or name in _ONLY:
            pl.when(always)(fn)

    def ln_x(t, s, tie=None):
        rows = pl.ds(t * TM + s * 16, 16)
        xn_v[rows, :] = _ln(x_v[rows, :].astype(F32), EPS, tie).astype(BF16)

    def ln_z2(t, s, tie=None):
        y = _ln(zg_v[t % 2, s * 16:(s + 1) * 16, :], 4.0 * EPS, tie, 0.25)
        lo, hi = y[:, :HN], y[:, HN:]
        r = (t * TM + s * 16) % HK
        rows = pl.ds(r, 16)
        if t < NT // 2:
            zf_v[rows, :] = y
            R_v[pl.ds(1 * HK + r, 16), :] = lo.astype(BF16)
            R_v[pl.ds(5 * HK + r, 16), :] = (lo + hi).astype(BF16)
        else:
            b11 = zf_v[rows, :HN]
            R_v[pl.ds(0 * HK + r, 16), :] = (b11 + hi).astype(BF16)
            R_v[pl.ds(2 * HK + r, 16), :] = (zf_v[rows, HN:] - hi).astype(BF16)
            R_v[pl.ds(3 * HK + r, 16), :] = (lo - b11).astype(BF16)
            R_v[pl.ds(4 * HK + r, 16), :] = hi.astype(BF16)
            R_v[pl.ds(6 * HK + r, 16), :] = (lo + hi).astype(BF16)

    def acomb_gen(i):
        for r in range(P // 16):
            for c in range(HK // 256):
                top = pl.ds(i * TM + r * 16, 16)
                bot = pl.ds(i * TM + P + r * 16, 16)
                c1 = slice(c * 256, (c + 1) * 256)
                c2 = slice(HK + c * 256, HK + (c + 1) * 256)
                a11 = wsp_v[top, c1].astype(F32)
                a12 = wsp_v[top, c2].astype(F32)
                a21 = wsp_v[bot, c1].astype(F32)
                a22 = wsp_v[bot, c2].astype(F32)
                r0 = (i % 4) * 5 * P + r * 16
                Lc_v[pl.ds(r0 + 0 * P, 16), c1] = (a11 + a22).astype(BF16)
                Lc_v[pl.ds(r0 + 1 * P, 16), c1] = (a21 + a22).astype(BF16)
                Lc_v[pl.ds(r0 + 2 * P, 16), c1] = (a11 + a12).astype(BF16)
                Lc_v[pl.ds(r0 + 3 * P, 16), c1] = (a21 - a11).astype(BF16)
                Lc_v[pl.ds(r0 + 4 * P, 16), c1] = (a12 - a22).astype(BF16)
                yield A_COST

    def tasks(fn, t):
        return [lambda tie, s=s: fn(t, s, tie) for s in range(TM // 16)]

    def kv_gen(t):
        for m in range(TM // MC):
            r = t * TM + m * MC
            for l in range(D // L):
                lanes = slice(l * L, (l + 1) * L)
                kf = k_v[pl.ds(r, MC), lanes].astype(F32)
                kf_v[l, pl.ds(r + 8, MC), :] = kf
                ks = kf * sk_v[0, 0:1, lanes]
                for tap in range(1, 4):
                    ks = ks + kf_v[l, pl.ds(r + 8 - tap, MC), :] * sk_v[tap, 0:1, lanes]
                kv = ks * v_v[pl.ds(r, MC), lanes].astype(F32)
                kv_v[pl.ds(r, MC), lanes] = kv.astype(BF16)
                yield KV_COST

    def g_gen(t):
        for r in range(P // 16):
            rows = pl.ds(r * 16, 16)
            for l in range(D // L):
                lanes = slice(l * L, (l + 1) * L)
                h = [(H_v[(2 * t + w) % 6, 0, rows, lanes], H_v[(2 * t + w) % 6, 1, rows, lanes]) for w in range(3)]
                for w in range(2):
                    (pr, pi), (cr, ci) = h[w], h[w + 1]
                    G_v[2 * t + w, 0, rows, lanes] = cr - pi if r < P // 32 else cr + pi
                    G_v[2 * t + w, 1, rows, lanes] = ci + pr if r < P // 32 else ci - pr
                yield G_COST

    def freq_gen(a):
        def cmac(acc, x, g):
            pr = x[0] * g[0] - x[1] * g[1]
            pi = x[0] * g[1] + x[1] * g[0]
            return (pr, pi) if acc is None else (acc[0] + pr, acc[1] + pi)

        for r in range(P // 16):
            for l in range(D // L):
                lanes = slice(l * L, (l + 1) * L)
                res = []
                for sub in range(2):
                    rows = pl.ds(r * 16 + sub * 8, 8)
                    lo = hi = None
                    g = (G_v[a + 1, 0, rows, lanes], G_v[a + 1, 1, rows, lanes])
                    for c in range(a + 2):
                        x = (X_v[c, 0, rows, lanes], X_v[c, 1, rows, lanes])
                        hi = cmac(hi, x, g)
                        if c <= a:
                            g = (G_v[a - c, 0, rows, lanes], G_v[a - c, 1, rows, lanes])
                            lo = cmac(lo, x, g)
                            yield 16
                    res.append((lo, hi))
                for w in range(2):
                    for part in range(2):
                        Z_v[pl.ds((a + w) * 2 * P + part * P + r * 16, 16), lanes] = jnp.concatenate(
                            [res[0][w][part], res[1][w][part]], axis=0).astype(BF16)
                yield 20

    def job_h(t, bg, budget):
        for j in (2 * t, 2 * t + 1):
            for part in range(2):
                hp = jax.lax.dot_general(F_v[part * P:(part + 1) * P, 0:P],
                                         h_v[t, :, (j % 2) * P:(j % 2 + 1) * P],
                                         NT_DIMS, preferred_element_type=F32)
                for g in range(8):
                    rows = pl.ds(part * 64 + g * 8, 8)
                    H_v[(j + 1) % 6, 0, rows, :] = hp[g * 16:g * 16 + 8]
                    H_v[(j + 1) % 6, 1, rows, :] = hp[g * 16 + 8:g * 16 + 16]
                bg.run(budget)

    def job_x(t, bg, budget):
        for j in (2 * t, 2 * t + 1):
            for part in range(2):
                xp = _dot(F_v[part * P:(part + 1) * P, 0:P], kv_v[j * P:(j + 1) * P, :])
                for g in range(8):
                    rows = pl.ds(part * 64 + g * 8, 8)
                    X_v[j, 0, rows, :] = xp[g * 16:g * 16 + 8]
                    X_v[j, 1, rows, :] = xp[g * 16 + 8:g * 16 + 16]
                bg.run(budget)

    def job_z(t, m, cols, bg=None, budgets=None, tied=None, ntied=None, inline_ln=False):
        rows = pl.ds(t * TM + m * MC, MC)
        for j, n in enumerate(cols):
            z = _gelu2(_dot(xn_v[rows, :], win_v[:, n * L:(n + 1) * L]))
            if n < FH // L:
                z1_v[rows, n * L:(n + 1) * L] = z
            else:
                zg_v[t % 2, m * MC:(m + 1) * MC, n * L - FH:(n + 1) * L - FH] = z
            if tied and ntied[j]:
                tie = _signzero(z[0:16])
                for _ in range(ntied[j]):
                    if tied:
                        tied.pop(0)(tie)
            if inline_ln and n == 2 * FH // L - 1:
                for s in range(4 * m, 4 * m + 4):
                    ln_z2(t, s)
            if bg is not None:
                bg.run(budgets[j])

    rev8 = 7 - jax.lax.broadcasted_iota(jnp.int32, (8, L), 0)

    def tail_piece(a, upper, n):
        rows = pl.ds(a * P + (MC if upper else 0), MC)
        lanes = slice(n * L, (n + 1) * L)
        hh = _dot(u_v[rows, :], wout_v[:, lanes])
        if upper:
            ya = _dot(Fi_v[:, 0:P], Z_v[a * 2 * P:a * 2 * P + P, lanes])
            yb = _dot(Fi_v[:, P:2 * P], Z_v[a * 2 * P + P:(a + 1) * 2 * P, lanes])
            y = ya - yb
            lo = ya + yb
            for j in range(MC // 8):
                yl_v[n, (7 - j) * 8:(8 - j) * 8, :] = jnp.take_along_axis(lo[j * 8:(j + 1) * 8], rev8, axis=0)
        else:
            y = yl_v[n]
        gate = hh + hh * jnp.tanh(hh)
        s = xn_v[rows, lanes].astype(F32) * y
        o_v[rows, lanes] = (x_v[rows, lanes].astype(F32) + s * gate).astype(BF16)

    def job_big(i, bg, pending, budget, every):
        a0, a1 = _blocks_of_step(i)
        KG = 512
        count = [0, 0]

        def lhs(j, sub, cols):
            if j == 2:
                return wsp_v[i * TM + sub:i * TM + sub + MC, cols]
            if j == 3:
                return wsp_v[i * TM + P + sub:i * TM + P + sub + MC, HK + cols.start:HK + cols.stop]
            r0 = ((i % 4) * 5 + {0: 0, 1: 1, 4: 2, 5: 3, 6: 4}[j]) * P + sub
            return Lc_v[r0:r0 + MC, cols]

        def prod(j, sub, n, acc=None):
            for kg in range(HK // KG):
                ks = slice(kg * KG, (kg + 1) * KG)
                p = _dot(lhs(j, sub, ks), R_v[j * HK + kg * KG:j * HK + (kg + 1) * KG, n * L:(n + 1) * L])
                acc = p if acc is None else acc + p
                bg.run(budget)
            count[0] += 1
            return acc

        def maybe_tail():
            count[1] += 1
            if pending and count[0] >= 3 and count[1] % every == 0:
                tail_piece(*pending.pop(0))
                bg.run(budget)

        def emit(a, sub, n, g):
            rows = pl.ds(a * P + sub, MC)
            lanes = slice(n * L, (n + 1) * L)
            u_v[rows, lanes] = (z1_v[rows, lanes] * (g + bcol_v[rows, :])).astype(BF16)

        for sub in (0, MC):
            for n in range(HN // L):
                m2 = prod(1, sub, n)
                m4 = prod(3, sub, n)
                emit(a1, sub, n, m2 + m4)
                maybe_tail()
                m3 = prod(2, sub, n)
                t22 = m3 - m2
                m5 = prod(4, sub, n)
                emit(a0, sub, n + HN // L, m3 + m5)
                t11 = m4 - m5
                maybe_tail()
                m1 = prod(0, sub, n)
                maybe_tail()
                emit(a0, sub, n, prod(6, sub, n, t11 + m1))
                emit(a1, sub, n + HN // L, prod(5, sub, n, t22 + m1))
                maybe_tail()

    if _ONLY is not None:
        for r_ in (xn_u, z1_v, R_u, Lc_u, zf_v, zg_v, kv_u, u_u, X_v, H_v, G_v, Z_u, kf_v):
            c_ = pltpu.make_async_copy(r_, r_, sem_small.at[0])
            c_.start()
            c_.wait()

    cp_x(0).start()
    cp_x(1).start()
    for c in range(5):
        cp_win(c).start()
    cp_x(2).start()
    start(cp_small())

    kk = _odd_freq(jax.lax.broadcasted_iota(jnp.int32, (P, P), 0))
    nn = jax.lax.broadcasted_iota(jnp.int32, (P, P), 1)
    fc, fs = _cos_sin((kk * (4 * nn - 127)) & 2047)
    for g in range(P // 8):
        F_v[g * 16:(g + 1) * 16, 0:P] = jnp.concatenate(
            [fc[g * 8:(g + 1) * 8], -fs[g * 8:(g + 1) * 8]], axis=0).astype(BF16)
    fc, fs = _cos_sin((kk * (-127)) & 2047)
    ph_v[0] = fc
    ph_v[1] = fs
    kk = _odd_freq(jax.lax.broadcasted_iota(jnp.int32, (MC, P), 1))
    mm = jax.lax.broadcasted_iota(jnp.int32, (MC, P), 0)
    ic, is_ = _cos_sin((kk * (4 * mm + 2)) & 2047)
    Fi_v[:, 0:P] = (ic * (1.0 / P)).astype(BF16)
    Fi_v[:, P:2 * P] = (is_ * (1.0 / P)).astype(BF16)
    kf_v[:, 0:8, :] = jnp.zeros((D // L, 8, L), F32)

    for t in range(2):
        cp_x(t).wait()
        for s in range(TM // 16):
            ln_x(t, s)

    def small_setup():
        sk = sk_in[...].astype(F32)
        for t in range(4):
            sk_v[t] = jnp.broadcast_to(sk[t:t + 1], (8, D))
        drow = d_in[...].astype(F32).reshape(1, D)
        for l in range(D // L):
            lanes = slice(l * L, (l + 1) * L)
            dre = ph_v[0] * drow[:, lanes]
            dim = ph_v[1] * drow[:, lanes]
            H_v[0, 0, 0:64, lanes] = -dim[0:64]
            H_v[0, 0, 64:P, lanes] = dim[64:P]
            H_v[0, 1, 0:64, lanes] = -dre[0:64]
            H_v[0, 1, 64:P, lanes] = dre[64:P]
        brow = b_in[...].astype(F32).reshape(1, S) * 0.25
        for j in range(NB):
            bcol_v[j * P:(j + 1) * P, :] = jnp.broadcast_to(brow[:, j * P:(j + 1) * P], (P, P)).T

    LAG = 2

    def interleave(*lists):
        out = []
        for j in range(max(len(a) for a in lists)):
            for a in lists:
                out += a[j:j + 1]
        return out

    def p1_first(c):
        tied = []
        if c == 3:
            tied = tasks(ln_z2, 0) + tasks(ln_z2, 1)[:6]
        if c == 4:
            tied = interleave(tasks(ln_x, 2), tasks(ln_z2, 1)[6:])
            small_setup()
        for t in range(2):
            for m in range(TM // MC):
                job_z(t, m, range(*WIN_CHUNKS[c]), tied=tied, ntied=(2 if m == 0 else 1, 1, 1))
        assert not tied

    for c in range(5):
        cp_win(c).wait()
        if c == 2:
            start(cp_conv(0))
            cp_x(3).start()
        if c == 4:
            cp_x(2).wait()
            wait(cp_small())
        block(lambda c=c: p1_first(c), f'p1_f{c}')

    def p1_dma(i):
        wait(cp_conv(i - LAG))
        if i + 1 < NT:
            cp_x(i + 1).wait()
        if i == NT - 3:
            wait(cp_wsp(0))
        if i + 2 < NT:
            cp_x(i + 2).start()
        start(cp_conv(i - LAG + 1))
        if i == NT - 1:
            start(cp_conv(NT - 1))
        start(cp_wsp((i - 2) // 2, ((i - 2) % 2,)))
        if i == 2:
            cp_wout().start()

    acomb0 = acomb_gen(0)

    def p1_step(i):
        bg = _Background()
        t = i - LAG
        bg.add(kv_gen(t))
        if t >= 1:
            bg.add(g_gen(t - 1))
        side = _Background()
        if i in (NT - 3, NT - 2):
            side.add(acomb0)
        tied = interleave(tasks(ln_x, i + 1) if i + 1 < NT else [], tasks(ln_z2, i - 1) if i > 2 else [])
        last = i == NT - 1
        ntied = (1, 0, 1, 0, 1, 0, 0, 0, 0, 0, 1, 0) if last else (1, 1, 0, 1, 1, 0) * 2
        budgets = (45, 120, 45, 120, 45, 120, 30, 30, 30, 120, 45, 120) if last else (45, 45, 140, 45, 45, 140) * 2
        for m in range(TM // MC):
            job_z(i, m, list(range(6, 12)) + list(range(6)), bg, budgets, tied, ntied, last)
            if m == 0:
                job_h(t, side, 2 * A_COST)
        assert not tied
        if t >= 1:
            job_x(t - 1, side, 2 * A_COST)
        bg.drain()
        if i == NT - 2:
            side.drain()

    for i in range(2, NT):
        p1_dma(i)
        block(lambda i=i: p1_step(i), f'p1_{i}')

    groups = P2_GROUPS
    NG = len(groups)

    def p2_dma(gi):
        if gi == 0:
            cp_wout().wait()
        if gi >= 2:
            for i in groups[gi - 2]:
                start(cp_out(i))
        if gi >= 3:
            for i in groups[gi - 3]:
                wait(cp_out(i))
        if gi + 2 < NG:
            for i in groups[gi + 2]:
                start(cp_wsp(i))
        if gi < 2:
            wait(cp_conv(NT - 2 + gi))
        if gi + 1 < NG:
            for i in groups[gi + 1]:
                wait(cp_wsp(i))

    def tails_of(i):
        return [(a, upper, n) for a in _blocks_of_step(i) for upper in (True, False) for n in range(D // L)]

    def p2_block(gi):
        bg = _Background()
        steps = groups[gi]
        pending = [t_ for i in (groups[gi - 1] if gi > 0 else []) for t_ in tails_of(i)]
        total = sum(a + 1 for i in steps for a in _blocks_of_step(i)) * 40 * 16
        slots = 84 * len(steps) + len(pending)
        bg.add(freq_gen(_blocks_of_step(steps[0])[0]))
        if gi < 2:
            bg.add(kv_gen(NT - 2 + gi))
            total += 20 * KV_COST
            slots += 8
        if gi < 3:
            slots += 8
            bg.add(g_gen(NT - 3 + gi))
            total += 40 * G_COST
        if gi + 1 < NG:
            for i in groups[gi + 1]:
                bg.add(acomb_gen(i))
                total += 32 * A_COST
        for i in steps[1:]:
            bg.add(freq_gen(_blocks_of_step(i)[0]))
        budget = total / (slots + 1.0)
        bg.run(budget)
        if gi < 3:
            job_x(NT - 3 + gi, bg, 2 * budget)
        if gi < 2:
            job_h(NT - 2 + gi, bg, 2 * budget)
        every = max(1, (24 * len(steps) - 2) // max(1, len(pending)))
        for i in steps:
            job_big(i, bg, pending, budget, every)
        for t_ in pending:
            tail_piece(*t_)
            bg.run(budget)
        bg.drain()

    for gi in range(NG):
        p2_dma(gi)
        block(lambda gi=gi: p2_block(gi), f'p2_{gi}')

    def p2_last():
        a0, a1 = _blocks_of_step(NT - 1)
        for t_ in tails_of(NT - 1):
            tail_piece(*t_)
            if t_ == (a0, False, D // L - 1):
                start(cp_out(NT - 1, (0,)))

    p2_dma(NG)
    block(p2_last, 'p2_last')
    start(cp_out(NT - 1, (1,)))
    for i in groups[NG - 2]:
        wait(cp_out(i))
    wait(cp_out(NT - 1))
    if _ONLY is not None:
        for r_ in (xn_u, z1_v, R_u, Lc_u, zf_v, zg_v, kv_u, u_u, X_v, H_v, G_v, Z_u, kf_v):
            c_ = pltpu.make_async_copy(r_, r_, sem_small.at[0])
            c_.start()
            c_.wait()


@jax.jit
def pallas_recurrent_scan__ssm_conv_h3__mixer_gmlp__prompt_kernel(
    A_q: jax.Array,
    A_k: jax.Array,
    A_v: jax.Array,
    A_shift_k: jax.Array,
    A_ssm_k: jax.Array,
    A_ssm_D: jax.Array,
    B_x: jax.Array,
    B_w_in: jax.Array,
    B_w_sp: jax.Array,
    B_b_sp: jax.Array,
    B_w_out: jax.Array,
):
    del B_x
    hbm = pl.BlockSpec(memory_space=pl.ANY)

    def bf16_buf(*shape):
        return pltpu.VMEM(shape[:-2] + (shape[-2] // 2, shape[-1]), U32)

    return pl.pallas_call(
        _kernel,
        out_shape=jax.ShapeDtypeStruct((1, S, D), BF16),
        in_specs=[pl.BlockSpec(memory_space=pltpu.SMEM)] + [hbm] * 10,
        out_specs=hbm,
        scratch_shapes=[
            bf16_buf(S, D),
            bf16_buf(S, D),
            bf16_buf(S, D),
            bf16_buf(NT, D, TM),
            bf16_buf(D, 2 * FH),
            bf16_buf(S, S),
            bf16_buf(FH, D),
            pltpu.VMEM((S, D), BF16),
            pltpu.VMEM((4, D), BF16),
            pltpu.VMEM((D,), BF16),
            pltpu.VMEM((S,), BF16),
            bf16_buf(S, D),
            pltpu.VMEM((S, FH), F32),
            bf16_buf(7 * HK, HN),
            bf16_buf(4 * 5 * P, HK),
            pltpu.VMEM((HK, FH), F32),
            pltpu.VMEM((2, TM, FH), F32),
            bf16_buf(S, D),
            bf16_buf(S, FH),
            pltpu.VMEM((NB, 2, P, D), F32),
            pltpu.VMEM((6, 2, P, D), F32),
            pltpu.VMEM((NB, 2, P, D), F32),
            bf16_buf(NB * 2 * P, D),
            pltpu.VMEM((D // L, MC, L), F32),
            bf16_buf(2 * P, 2 * P),
            bf16_buf(MC, 2 * P),
            pltpu.VMEM((S, L), F32),
            pltpu.VMEM((2, P, L), F32),
            pltpu.VMEM((4, 8, D), F32),
            pltpu.VMEM((D // L, S + 8, L), F32),
            pltpu.SemaphoreType.DMA((1,)),
            pltpu.SemaphoreType.DMA((3,)),
            pltpu.SemaphoreType.DMA((2,)),
            pltpu.SemaphoreType.DMA((5,)),
            pltpu.SemaphoreType.DMA((5,)),
            pltpu.SemaphoreType.DMA((5,)),
        ],
        compiler_params=pltpu.CompilerParams(vmem_limit_bytes=116 * 1024 * 1024),
    )(jnp.ones((1,), jnp.int32), A_q, A_k, A_v, A_shift_k.T, A_ssm_k, A_ssm_D, B_w_in, B_w_sp, B_b_sp, B_w_out)
```

```python
import math

import jax
import jax.numpy as jnp
import jax.experimental.pallas as pl
import jax.experimental.pallas.tpu as pltpu

S = 2048
D = 640
FH = 768
P = 128
NB = S // P
TM = 256
NT = S // TM
MC = 64
L = 128
HK = S // 2
KH = 256
HN = FH // 2
P2_GROUPS = ((0,), (1, 2), (3, 4), (5, 6), (7,))
STEP_BLOCKS = ((2, 3), (10, 11), (0, 1), (8, 9), (6, 7), (14, 15), (4, 5), (12, 13))
KV_COST, G_COST, A_COST = 110, 36, 56
WIN_CHUNKS = ((6, 7), (7, 9), (9, 12), (0, 3), (3, 6))
EPS = 1e-5
F32 = jnp.float32
BF16 = jnp.bfloat16
U32 = jnp.uint32
GELU_C = math.sqrt(2.0 / math.pi)
NT_DIMS = (((1,), (1,)), ((), ()))
_ONLY = None


def _dot(a, b):
    return jnp.dot(a, b, preferred_element_type=F32)


def _cos_sin(m):
    q = (m + 256) >> 9
    x = (m - (q << 9)).astype(F32) * (2.0 * math.pi / 2048.0)
    x2 = x * x
    s = x * (1.0 + x2 * (-1.0 / 6 + x2 * (1.0 / 120 + x2 * (-1.0 / 5040 + x2 * (1.0 / 362880)))))
    c = 1.0 + x2 * (-0.5 + x2 * (1.0 / 24 + x2 * (-1.0 / 720 + x2 * (1.0 / 40320 - x2 * (1.0 / 3628800)))))
    swap = (q & 1) == 1
    c0 = jnp.where(swap, s, c)
    s0 = jnp.where(swap, c, s)
    cos = jnp.where(((q + 1) & 2) == 2, -c0, c0)
    sin = jnp.where((q & 2) == 2, -s0, s0)
    return cos, sin


def _odd_freq(r):
    return jnp.where(r < 64, 4 * r + 1, 4 * r - 253)


def _gelu2(z):
    u = z * (GELU_C + (GELU_C * 0.044715) * (z * z))
    return z + z * jnp.tanh(u)


def _signzero(z):
    bits = jax.lax.bitcast_convert_type(z, U32) & jnp.uint32(0x80000000)
    return jax.lax.bitcast_convert_type(bits, F32)


def _ln(x, eps, tie=None, scale=None):
    n = x.shape[-1]
    part = x[:, 0:L]
    for j in range(1, n // L):
        part = part + x[:, j * L:(j + 1) * L]
    if tie is not None:
        part = part + tie
    m = jnp.sum(part, axis=-1, keepdims=True) * (1.0 / n)
    xc = x - m
    v = jnp.sum(xc * xc, axis=-1, keepdims=True) * (1.0 / n)
    rs = jax.lax.rsqrt(v + eps)
    if scale is not None:
        rs = rs * scale
    return xc * rs


def _blocks_of_step(i):
    return STEP_BLOCKS[i]


class _Background:
    def __init__(self):
        self.q = []
        self.credit = 0.0

    def add(self, gen):
        self.q.append(gen)

    def run(self, budget):
        self.credit += budget
        while self.q and self.credit > 0:
            try:
                self.credit -= next(self.q[0])
            except StopIteration:
                self.q.pop(0)
        if not self.q:
            self.credit = 0.0

    def drain(self):
        while self.q:
            self.run(1e9)


class _Tied:
    def __init__(self, tasks, npieces):
        self.tasks = list(tasks)
        self.rate = len(self.tasks) / float(npieces)
        self.credit = 0.999

    def run(self, z):
        self.credit += self.rate
        n = 0
        while self.tasks and self.credit >= 1.0:
            self.tasks.pop(0)(_signzero(z[0:16]))
            self.credit -= 1.0
            n += 1
        return n


def _kernel(one_ref, q_hbm, k_hbm, v_hbm, sk_hbm, h_hbm, d_hbm, win_hbm, wsp_hbm, b_hbm, wout_hbm,
            o_hbm,
            x_u, k_u, v_u, h_u, win_u, wsp_u, wout_u, o_v, sk_in, d_in, b_in,
            xn_u, XL_u, WB_u, z1_v, R_u, Lc_u, zf_v, zg_v, kv_u, u_u, X_v, H_v, G_v, Z_u, yl_v, F_u, Fi_u, bcol_v, ph_v, sk_v, kf_v,
            sem_small, sem_x, sem_conv, sem_wsp, sem_w, sem_out):
    x_v, k_v, v_v, h_v, win_v, wsp_v, wout_v, xn_v, XL_v, WB_v, R_v, Lc_v, kv_v, u_v, Z_v, F_v, Fi_v = [
        r.bitcast(BF16) for r in (x_u, k_u, v_u, h_u, win_u, wsp_u, wout_u, xn_u, XL_u, WB_u, R_u, Lc_u, kv_u, u_u, Z_u, F_u,
                                  Fi_u)]

    def cp_small():
        return [pltpu.make_async_copy(s_, d_, sem_small.at[0])
                for s_, d_ in ((d_hbm, d_in), (sk_hbm, sk_in), (b_hbm, b_in))]

    def cp_x(t):
        return pltpu.make_async_copy(q_hbm.at[0, pl.ds(t * TM, TM)], x_v.at[pl.ds(t * TM, TM)], sem_x.at[t % 3])

    def cp_conv(t):
        rows = pl.ds(t * TM, TM)
        sem = sem_conv.at[t % 2]
        return [pltpu.make_async_copy(h_hbm.at[:, rows], h_v.at[t], sem),
                pltpu.make_async_copy(k_hbm.at[0, rows], k_v.at[rows], sem),
                pltpu.make_async_copy(v_hbm.at[0, rows], v_v.at[rows], sem)]

    def cp_wsp(i, which=(0, 1)):
        return [pltpu.make_async_copy(wsp_hbm.at[pl.ds(_blocks_of_step(i)[half] * P, P)],
                                      wsp_v.at[pl.ds(i * TM + half * P, P)], sem_wsp.at[i % 5]) for half in which]

    def cp_win(c):
        lo, hi = WIN_CHUNKS[c]
        cols = pl.ds(lo * L, (hi - lo) * L)
        return pltpu.make_async_copy(win_hbm.at[:, cols], win_v.at[:, cols], sem_w.at[c])

    def cp_wout():
        return pltpu.make_async_copy(wout_hbm, wout_v, sem_w.at[0])

    def cp_out(i, which=(0, 1)):
        return [pltpu.make_async_copy(o_v.at[pl.ds(a * P, P)], o_hbm.at[0, pl.ds(a * P, P)], sem_out.at[i % 5])
                for a in [_blocks_of_step(i)[w] for w in which]]

    def start(cs):
        for c in cs:
            c.start()

    def wait(cs):
        for c in cs:
            c.wait()

    always = one_ref[0] == 1

    def block(fn, name):
        if _ONLY is None or name in _ONLY:
            pl.when(always)(fn)

    def ln_x(t, s, tie=None):
        rows = pl.ds(t * TM + s * 16, 16)
        y = _ln(x_v[rows, :].astype(F32), EPS, tie)
        xn_v[rows, :] = y.astype(BF16)
        return y

    def ln_x2(t, s, tie):
        p, q = s // 4, s % 4
        y1 = ln_x(t, 8 * p + q, tie)
        y2 = ln_x(t, 8 * p + 4 + q, tie)
        a11, a12, a21, a22 = y1[:, :KH], y1[:, KH:2 * KH], y2[:, :KH], y2[:, KH:2 * KH]
        r0 = (t % 2) * 5 * P + p * MC + q * 16
        for j, c in enumerate((a11 + a22, a21 + a22, a11 + a12, a21 - a11, a12 - a22)):
            XL_v[pl.ds(r0 + j * P, 16), :] = c.astype(BF16)

    def wcomb_gen(cols):
        for j in cols:
            c1 = slice(j * L, (j + 1) * L)
            c2 = slice(FH + j * L, FH + (j + 1) * L)
            for r in range(KH // 32):
                top = pl.ds(r * 32, 32)
                bot = pl.ds(KH + r * 32, 32)
                b11, b12 = win_v[top, c1].astype(F32), win_v[top, c2].astype(F32)
                b21, b22 = win_v[bot, c1].astype(F32), win_v[bot, c2].astype(F32)
                for w, c in enumerate((b11 + b22, b12 - b22, b21 - b11, b11 + b12, b21 + b22)):
                    WB_v[pl.ds(w * KH + r * 32, 32), c1] = c.astype(BF16)
                yield A_COST

    def ln_z2(t, s, tie=None):
        y = _ln(zg_v[t % 2, s * 16:(s + 1) * 16, :], 4.0 * EPS, tie, 0.25)
        lo, hi = y[:, :HN], y[:, HN:]
        r = (t * TM + s * 16) % HK
        rows = pl.ds(r, 16)
        if t < NT // 2:
            zf_v[rows, :] = y
            R_v[pl.ds(1 * HK + r, 16), :] = lo.astype(BF16)
            R_v[pl.ds(5 * HK + r, 16), :] = (lo + hi).astype(BF16)
        else:
            b11 = zf_v[rows, :HN]
            R_v[pl.ds(0 * HK + r, 16), :] = (b11 + hi).astype(BF16)
            R_v[pl.ds(2 * HK + r, 16), :] = (zf_v[rows, HN:] - hi).astype(BF16)
            R_v[pl.ds(3 * HK + r, 16), :] = (lo - b11).astype(BF16)
            R_v[pl.ds(4 * HK + r, 16), :] = hi.astype(BF16)
            R_v[pl.ds(6 * HK + r, 16), :] = (lo + hi).astype(BF16)

    def acomb_gen(i):
        for r in range(P // 16):
            for c in range(HK // 256):
                top = pl.ds(i * TM + r * 16, 16)
                bot = pl.ds(i * TM + P + r * 16, 16)
                c1 = slice(c * 256, (c + 1) * 256)
                c2 = slice(HK + c * 256, HK + (c + 1) * 256)
                a11 = wsp_v[top, c1].astype(F32)
                a12 = wsp_v[top, c2].astype(F32)
                a21 = wsp_v[bot, c1].astype(F32)
                a22 = wsp_v[bot, c2].astype(F32)
                r0 = (i % 4) * 5 * P + r * 16
                Lc_v[pl.ds(r0 + 0 * P, 16), c1] = (a11 + a22).astype(BF16)
                Lc_v[pl.ds(r0 + 1 * P, 16), c1] = (a21 + a22).astype(BF16)
                Lc_v[pl.ds(r0 + 2 * P, 16), c1] = (a11 + a12).astype(BF16)
                Lc_v[pl.ds(r0 + 3 * P, 16), c1] = (a21 - a11).astype(BF16)
                Lc_v[pl.ds(r0 + 4 * P, 16), c1] = (a12 - a22).astype(BF16)
                yield A_COST

    def tasks(fn, t, n=TM // 16):
        return [lambda tie, s=s: fn(t, s, tie) for s in range(n)]

    def kv_gen(t):
        for m in range(TM // MC):
            r = t * TM + m * MC
            for l in range(D // L):
                lanes = slice(l * L, (l + 1) * L)
                kf = k_v[pl.ds(r, MC), lanes].astype(F32)
                kf_v[l, pl.ds(r + 8, MC), :] = kf
                ks = kf * sk_v[0, 0:1, lanes]
                for tap in range(1, 4):
                    ks = ks + kf_v[l, pl.ds(r + 8 - tap, MC), :] * sk_v[tap, 0:1, lanes]
                kv = ks * v_v[pl.ds(r, MC), lanes].astype(F32)
                kv_v[pl.ds(r, MC), lanes] = kv.astype(BF16)
                yield KV_COST

    def g_gen(t):
        for r in range(P // 16):
            rows = pl.ds(r * 16, 16)
            for l in range(D // L):
                lanes = slice(l * L, (l + 1) * L)
                h = [(H_v[(2 * t + w) % 6, 0, rows, lanes], H_v[(2 * t + w) % 6, 1, rows, lanes]) for w in range(3)]
                for w in range(2):
                    (pr, pi), (cr, ci) = h[w], h[w + 1]
                    G_v[2 * t + w, 0, rows, lanes] = cr - pi if r < P // 32 else cr + pi
                    G_v[2 * t + w, 1, rows, lanes] = ci + pr if r < P // 32 else ci - pr
                yield G_COST

    def freq_gen(a):
        def cmac(acc, x, g):
            pr = x[0] * g[0] - x[1] * g[1]
            pi = x[0] * g[1] + x[1] * g[0]
            return (pr, pi) if acc is None else (acc[0] + pr, acc[1] + pi)

        for r in range(P // 16):
            rows = pl.ds(r * 16, 16)
            for l in range(D // L):
                lanes = slice(l * L, (l + 1) * L)
                lo = hi = None
                g = (G_v[a + 1, 0, rows, lanes], G_v[a + 1, 1, rows, lanes])
                for c in range(a + 2):
                    x = (X_v[c, 0, rows, lanes], X_v[c, 1, rows, lanes])
                    hi = cmac(hi, x, g)
                    if c <= a:
                        g = (G_v[a - c, 0, rows, lanes], G_v[a - c, 1, rows, lanes])
                        lo = cmac(lo, x, g)
                        yield 32
                for w, z in enumerate((lo, hi)):
                    for part in range(2):
                        Z_v[pl.ds((a + w) * 2 * P + part * P + r * 16, 16), lanes] = z[part].astype(BF16)
                yield 20

    def job_h(t, bg, budget):
        for j in (2 * t, 2 * t + 1):
            for part in range(2):
                hp = jax.lax.dot_general(F_v[part * P:(part + 1) * P, 0:P],
                                         h_v[t, :, (j % 2) * P:(j % 2 + 1) * P],
                                         NT_DIMS, preferred_element_type=F32)
                for g in range(8):
                    rows = pl.ds(part * 64 + g * 8, 8)
                    H_v[(j + 1) % 6, 0, rows, :] = hp[g * 16:g * 16 + 8]
                    H_v[(j + 1) % 6, 1, rows, :] = hp[g * 16 + 8:g * 16 + 16]
                bg.run(budget)

    def job_x(t, bg, budget):
        for j in (2 * t, 2 * t + 1):
            for part in range(2):
                xp = _dot(F_v[part * P:(part + 1) * P, 0:P], kv_v[j * P:(j + 1) * P, :])
                for g in range(8):
                    rows = pl.ds(part * 64 + g * 8, 8)
                    X_v[j, 0, rows, :] = xp[g * 16:g * 16 + 8]
                    X_v[j, 1, rows, :] = xp[g * 16 + 8:g * 16 + 16]
                bg.run(budget)

    def z_out(t, m, n, pre, bg, budget, tied):
        z = _gelu2(pre)
        if n < FH // L:
            z1_v[pl.ds(t * TM + m * MC, MC), n * L:(n + 1) * L] = z
        else:
            zg_v[t % 2, m * MC:(m + 1) * MC, n * L - FH:(n + 1) * L - FH] = z
        ntask = tied.run(z)
        bg.run(budget[1] if ntask else budget[0])

    def job_z(t, m, cols, bg, budget, tied):
        for n in cols:
            z_out(t, m, n, _dot(xn_v[pl.ds(t * TM + m * MC, MC), :], win_v[:, n * L:(n + 1) * L]), bg, budget, tied)

    def job_zs(t, p, j, bg, budget, tied):
        r1 = pl.ds(t * TM + p * P, MC)
        r2 = pl.ds(t * TM + p * P + MC, MC)
        c1 = slice(j * L, (j + 1) * L)
        c2 = slice(FH + j * L, FH + (j + 1) * L)

        def xl(w):
            r0 = (t % 2) * 5 * P + w * P + p * MC
            return XL_v[r0:r0 + MC, :]

        def wb(w):
            return WB_v[w * KH:(w + 1) * KH, c1]

        def rem(rows, cols):
            return _dot(xn_v[rows, 2 * KH:], win_v[2 * KH:, cols])

        m2 = _dot(xl(1), win_v[0:KH, c1])
        m4 = _dot(xn_v[r2, KH:2 * KH], wb(2))
        z_out(t, 2 * p + 1, j, m2 + m4 + rem(r2, c1), bg, budget, tied)
        m3 = _dot(xn_v[r1, 0:KH], wb(1))
        m5 = _dot(xl(2), win_v[KH:2 * KH, c2])
        z_out(t, 2 * p, 6 + j, m3 + m5 + rem(r1, c2), bg, budget, tied)
        m1 = _dot(xl(0), wb(0))
        z_out(t, 2 * p, j, (m4 - m5) + m1 + _dot(xl(4), wb(4)) + rem(r1, c1), bg, budget, tied)
        z_out(t, 2 * p + 1, 6 + j, (m3 - m2) + m1 + _dot(xl(3), wb(3)) + rem(r2, c2), bg, budget, tied)

    rev8 = 7 - jax.lax.broadcasted_iota(jnp.int32, (8, L), 0)

    def tail_piece(a, upper, n):
        rows = pl.ds(a * P + (MC if upper else 0), MC)
        lanes = slice(n * L, (n + 1) * L)
        hh = _dot(u_v[rows, :], wout_v[:, lanes])
        if upper:
            ya = _dot(Fi_v[:, 0:P], Z_v[a * 2 * P:a * 2 * P + P, lanes])
            yb = _dot(Fi_v[:, P:2 * P], Z_v[a * 2 * P + P:(a + 1) * 2 * P, lanes])
            y = ya - yb
            lo = ya + yb
            for j in range(MC // 8):
                yl_v[n, (7 - j) * 8:(8 - j) * 8, :] = jnp.take_along_axis(lo[j * 8:(j + 1) * 8], rev8, axis=0)
        else:
            y = yl_v[n]
        gate = hh + hh * jnp.tanh(hh)
        s = xn_v[rows, lanes].astype(F32) * y
        o_v[rows, lanes] = (x_v[rows, lanes].astype(F32) + s * gate).astype(BF16)

    def job_big(i, bg, pending, budget, every):
        a0, a1 = _blocks_of_step(i)
        KG = 512
        count = [0, 0]

        def lhs(j, sub, cols):
            if j == 2:
                return wsp_v[i * TM + sub:i * TM + sub + MC, cols]
            if j == 3:
                return wsp_v[i * TM + P + sub:i * TM + P + sub + MC, HK + cols.start:HK + cols.stop]
            r0 = ((i % 4) * 5 + {0: 0, 1: 1, 4: 2, 5: 3, 6: 4}[j]) * P + sub
            return Lc_v[r0:r0 + MC, cols]

        def prod(j, sub, n, acc=None):
            for kg in range(HK // KG):
                ks = slice(kg * KG, (kg + 1) * KG)
                p = _dot(lhs(j, sub, ks), R_v[j * HK + kg * KG:j * HK + (kg + 1) * KG, n * L:(n + 1) * L])
                acc = p if acc is None else acc + p
                bg.run(budget)
            count[0] += 1
            return acc

        def maybe_tail():
            count[1] += 1
            if pending and count[0] >= 3 and count[1] % every == 0:
                tail_piece(*pending.pop(0))
                bg.run(budget)

        def emit(a, sub, n, g):
            rows = pl.ds(a * P + sub, MC)
            lanes = slice(n * L, (n + 1) * L)
            u_v[rows, lanes] = (z1_v[rows, lanes] * (g + bcol_v[rows, :])).astype(BF16)

        for sub in (0, MC):
            for n in range(HN // L):
                m2 = prod(1, sub, n)
                m4 = prod(3, sub, n)
                emit(a1, sub, n, m2 + m4)
                maybe_tail()
                m3 = prod(2, sub, n)
                t22 = m3 - m2
                m5 = prod(4, sub, n)
                emit(a0, sub, n + HN // L, m3 + m5)
                t11 = m4 - m5
                maybe_tail()
                m1 = prod(0, sub, n)
                maybe_tail()
                emit(a0, sub, n, prod(6, sub, n, t11 + m1))
                emit(a1, sub, n + HN // L, prod(5, sub, n, t22 + m1))
                maybe_tail()

    if _ONLY is not None:
        for r_ in (xn_u, XL_u, WB_u, z1_v, R_u, Lc_u, zf_v, zg_v, kv_u, u_u, X_v, H_v, G_v, Z_u, kf_v):
            c_ = pltpu.make_async_copy(r_, r_, sem_small.at[0])
            c_.start()
            c_.wait()

    cp_x(0).start()
    cp_x(1).start()
    for c in range(5):
        cp_win(c).start()
    cp_x(2).start()
    start(cp_small())

    kk = _odd_freq(jax.lax.broadcasted_iota(jnp.int32, (P, P), 0))
    nn = jax.lax.broadcasted_iota(jnp.int32, (P, P), 1)
    fc, fs = _cos_sin((kk * (4 * nn - 127)) & 2047)
    for g in range(P // 8):
        F_v[g * 16:(g + 1) * 16, 0:P] = jnp.concatenate(
            [fc[g * 8:(g + 1) * 8], -fs[g * 8:(g + 1) * 8]], axis=0).astype(BF16)
    fc, fs = _cos_sin((kk * (-127)) & 2047)
    ph_v[0] = fc
    ph_v[1] = fs
    kk = _odd_freq(jax.lax.broadcasted_iota(jnp.int32, (MC, P), 1))
    mm = jax.lax.broadcasted_iota(jnp.int32, (MC, P), 0)
    ic, is_ = _cos_sin((kk * (4 * mm + 2)) & 2047)
    Fi_v[:, 0:P] = (ic * (1.0 / P)).astype(BF16)
    Fi_v[:, P:2 * P] = (is_ * (1.0 / P)).astype(BF16)
    kf_v[:, 0:8, :] = jnp.zeros((D // L, 8, L), F32)

    for t in range(2):
        cp_x(t).wait()
        for s in range(TM // 16):
            ln_x(t, s)

    def small_setup():
        sk = sk_in[...].astype(F32)
        for t in range(4):
            sk_v[t] = jnp.broadcast_to(sk[t:t + 1], (8, D))
        drow = d_in[...].astype(F32).reshape(1, D)
        for l in range(D // L):
            lanes = slice(l * L, (l + 1) * L)
            dre = ph_v[0] * drow[:, lanes]
            dim = ph_v[1] * drow[:, lanes]
            H_v[0, 0, 0:64, lanes] = -dim[0:64]
            H_v[0, 0, 64:P, lanes] = dim[64:P]
            H_v[0, 1, 0:64, lanes] = -dre[0:64]
            H_v[0, 1, 64:P, lanes] = dre[64:P]

    def bcol_task(t, j, tie):
        brow = b_in[...].astype(F32).reshape(1, S)[:, j * P:(j + 1) * P] * 0.25 + tie[0:1]
        bcol_v[j * P:(j + 1) * P, :] = jnp.broadcast_to(brow, (P, P)).T

    LAG = 2

    def interleave(*lists):
        out = []
        for j in range(max(len(a) for a in lists)):
            for a in lists:
                out += a[j:j + 1]
        return out

    def p1_first(c):
        bg = _Background()
        todo = []
        if c == 3:
            todo = tasks(ln_z2, 0)
            bg.add(wcomb_gen(range(3)))
        if c == 4:
            todo = tasks(ln_x2, 2, 8)
            bg.add(wcomb_gen(range(3, 6)))
            small_setup()
        tied = _Tied(todo, 20)
        for t in range(2):
            for m in range(TM // MC):
                job_z(t, m, range(*WIN_CHUNKS[c]), bg, (80, 40), tied)
        bg.drain()
        assert not tied.tasks

    for c in range(5):
        cp_win(c).wait()
        if c == 2:
            start(cp_conv(0))
            cp_x(3).start()
        if c == 4:
            cp_x(2).wait()
            wait(cp_small())
        block(lambda c=c: p1_first(c), f'p1_f{c}')

    def p1_dma(i):
        wait(cp_conv(i - LAG))
        if i + 1 < NT:
            cp_x(i + 1).wait()
        if i == NT - 3:
            wait(cp_wsp(0))
        if i + 2 < NT:
            cp_x(i + 2).start()
        start(cp_conv(i - LAG + 1))
        if i == NT - 1:
            start(cp_conv(NT - 1))
        start(cp_wsp((i - 2) // 2, ((i - 2) % 2,)))
        if i == 2:
            cp_wout().start()

    acomb0 = acomb_gen(0)

    def take(gen, n):
        for _ in range(n):
            yield next(gen)

    def p1_step(i):
        bg = _Background()
        dft = _Background()
        t = i - LAG
        kv = kv_gen(t)
        dft.add(take(kv, 20 if t >= 1 else 10))
        if t >= 1:
            bg.add(g_gen(t - 1))
        else:
            bg.add(take(kv, 10))
        extra = 0
        if i in (NT - 3, NT - 2):
            bg.add(take(acomb0, 16))
            extra = 20
        last = i == NT - 1
        z2t = tasks(ln_z2, i - 1)
        todo = interleave(tasks(ln_x2, i + 1, 8) if not last else [], z2t[0::2], z2t[1::2],
                          tasks(bcol_task, 0) if i == 2 else [])
        tied = _Tied(todo, 24 if last else 42)
        if t >= 1:
            dft.run(110)
            job_x(t - 1, dft, 250)
        for p in range(2):
            for j in range(FH // L):
                job_zs(i, p, j, bg, (60 + extra, 10 + extra), tied)
            if p == 0 and last:
                tied = _Tied(tasks(ln_z2, i, 8), 22)
        assert not tied.tasks
        if last:
            for s in range(8, 16):
                ln_z2(i, s)
        job_h(t, dft, 275)
        bg.drain()
        dft.drain()

    for i in range(2, NT):
        p1_dma(i)
        block(lambda i=i: p1_step(i), f'p1_{i}')

    groups = P2_GROUPS
    NG = len(groups)

    def p2_dma(gi):
        if gi == 0:
            cp_wout().wait()
        if gi >= 2:
            for i in groups[gi - 2]:
                start(cp_out(i))
        if gi >= 3:
            for i in groups[gi - 3]:
                wait(cp_out(i))
        if gi + 2 < NG:
            for i in groups[gi + 2]:
                start(cp_wsp(i))
        if gi < 2:
            wait(cp_conv(NT - 2 + gi))
        if gi + 1 < NG:
            for i in groups[gi + 1]:
                wait(cp_wsp(i))

    def tails_of(i):
        return [(a, upper, n) for a in _blocks_of_step(i) for upper in (True, False) for n in range(D // L)]

    def p2_block(gi):
        bg = _Background()
        steps = groups[gi]
        pending = [t_ for i in (groups[gi - 1] if gi > 0 else []) for t_ in tails_of(i)]
        total = sum(a + 1 for i in steps for a in _blocks_of_step(i)) * 40 * 16
        slots = 84 * len(steps) + len(pending)
        bg.add(freq_gen(_blocks_of_step(steps[0])[0]))
        if gi < 2:
            bg.add(kv_gen(NT - 2 + gi))
            total += 20 * KV_COST
            slots += 8
        if gi < 3:
            slots += 8
            bg.add(g_gen(NT - 3 + gi))
            total += 40 * G_COST
        if gi + 1 < NG:
            for i in groups[gi + 1]:
                bg.add(acomb_gen(i))
                total += 32 * A_COST
        for i in steps[1:]:
            bg.add(freq_gen(_blocks_of_step(i)[0]))
        budget = total / (slots + 1.0)
        bg.run(budget)
        if gi < 3:
            job_x(NT - 3 + gi, bg, 2 * budget)
        if gi < 2:
            job_h(NT - 2 + gi, bg, 2 * budget)
        every = max(1, (24 * len(steps) - 2) // max(1, len(pending)))
        for i in steps:
            job_big(i, bg, pending, budget, every)
        for t_ in pending:
            tail_piece(*t_)
            bg.run(budget)
        bg.drain()

    for gi in range(NG):
        p2_dma(gi)
        block(lambda gi=gi: p2_block(gi), f'p2_{gi}')

    def p2_last():
        a0, a1 = _blocks_of_step(NT - 1)
        for t_ in tails_of(NT - 1):
            tail_piece(*t_)
            if t_ == (a0, False, D // L - 1):
                start(cp_out(NT - 1, (0,)))

    p2_dma(NG)
    block(p2_last, 'p2_last')
    start(cp_out(NT - 1, (1,)))
    for i in groups[NG - 2]:
        wait(cp_out(i))
    wait(cp_out(NT - 1))
    if _ONLY is not None:
        for r_ in (xn_u, XL_u, WB_u, z1_v, R_u, Lc_u, zf_v, zg_v, kv_u, u_u, X_v, H_v, G_v, Z_u, kf_v):
            c_ = pltpu.make_async_copy(r_, r_, sem_small.at[0])
            c_.start()
            c_.wait()


@jax.jit
def pallas_recurrent_scan__ssm_conv_h3__mixer_gmlp__prompt_kernel(
    A_q: jax.Array,
    A_k: jax.Array,
    A_v: jax.Array,
    A_shift_k: jax.Array,
    A_ssm_k: jax.Array,
    A_ssm_D: jax.Array,
    B_x: jax.Array,
    B_w_in: jax.Array,
    B_w_sp: jax.Array,
    B_b_sp: jax.Array,
    B_w_out: jax.Array,
):
    del B_x
    hbm = pl.BlockSpec(memory_space=pl.ANY)

    def bf16_buf(*shape):
        return pltpu.VMEM(shape[:-2] + (shape[-2] // 2, shape[-1]), U32)

    return pl.pallas_call(
        _kernel,
        out_shape=jax.ShapeDtypeStruct((1, S, D), BF16),
        in_specs=[pl.BlockSpec(memory_space=pltpu.SMEM)] + [hbm] * 10,
        out_specs=hbm,
        scratch_shapes=[
            bf16_buf(S, D),
            bf16_buf(S, D),
            bf16_buf(S, D),
            bf16_buf(NT, D, TM),
            bf16_buf(D, 2 * FH),
            bf16_buf(S, S),
            bf16_buf(FH, D),
            pltpu.VMEM((S, D), BF16),
            pltpu.VMEM((4, D), BF16),
            pltpu.VMEM((D,), BF16),
            pltpu.VMEM((S,), BF16),
            bf16_buf(S, D),
            bf16_buf(2 * 5 * P, KH),
            bf16_buf(5 * KH, FH),
            pltpu.VMEM((S, FH), F32),
            bf16_buf(7 * HK, HN),
            bf16_buf(4 * 5 * P, HK),
            pltpu.VMEM((HK, FH), F32),
            pltpu.VMEM((2, TM, FH), F32),
            bf16_buf(S, D),
            bf16_buf(S, FH),
            pltpu.VMEM((NB, 2, P, D), F32),
            pltpu.VMEM((6, 2, P, D), F32),
            pltpu.VMEM((NB, 2, P, D), F32),
            bf16_buf(NB * 2 * P, D),
            pltpu.VMEM((D // L, MC, L), F32),
            bf16_buf(2 * P, 2 * P),
            bf16_buf(MC, 2 * P),
            pltpu.VMEM((S, L), F32),
            pltpu.VMEM((2, P, L), F32),
            pltpu.VMEM((4, 8, D), F32),
            pltpu.VMEM((D // L, S + 8, L), F32),
            pltpu.SemaphoreType.DMA((1,)),
            pltpu.SemaphoreType.DMA((3,)),
            pltpu.SemaphoreType.DMA((2,)),
            pltpu.SemaphoreType.DMA((5,)),
            pltpu.SemaphoreType.DMA((5,)),
            pltpu.SemaphoreType.DMA((5,)),
        ],
        compiler_params=pltpu.CompilerParams(vmem_limit_bytes=116 * 1024 * 1024),
    )(jnp.ones((1,), jnp.int32), A_q, A_k, A_v, A_shift_k.T, A_ssm_k, A_ssm_D, B_w_in, B_w_sp, B_b_sp, B_w_out)
```

```python
import math

import jax
import jax.numpy as jnp
import jax.experimental.pallas as pl
import jax.experimental.pallas.tpu as pltpu

S = 2048
D = 640
FH = 768
P = 128
NB = S // P
TM = 256
NT = S // TM
MC = 64
L = 128
HK = S // 2
KH = 256
HN = FH // 2
P2_GROUPS = ((0,), (1, 2), (3, 4), (5, 6), (7,))
STEP_BLOCKS = ((6, 7), (8, 9), (4, 5), (12, 13), (2, 3), (14, 15), (0, 1), (10, 11))
KV_COST, G_COST, A_COST = 110, 36, 56
WIN_CHUNKS = ((6, 7), (7, 9), (9, 12), (0, 3), (3, 6))
EPS = 1e-5
F32 = jnp.float32
BF16 = jnp.bfloat16
U32 = jnp.uint32
GELU_C = math.sqrt(2.0 / math.pi)
NT_DIMS = (((1,), (1,)), ((), ()))
_ONLY = None


def _dot(a, b):
    return jnp.dot(a, b, preferred_element_type=F32)


def _cos_sin(m):
    q = (m + 256) >> 9
    x = (m - (q << 9)).astype(F32) * (2.0 * math.pi / 2048.0)
    x2 = x * x
    s = x * (1.0 + x2 * (-1.0 / 6 + x2 * (1.0 / 120 + x2 * (-1.0 / 5040 + x2 * (1.0 / 362880)))))
    c = 1.0 + x2 * (-0.5 + x2 * (1.0 / 24 + x2 * (-1.0 / 720 + x2 * (1.0 / 40320 - x2 * (1.0 / 3628800)))))
    swap = (q & 1) == 1
    c0 = jnp.where(swap, s, c)
    s0 = jnp.where(swap, c, s)
    cos = jnp.where(((q + 1) & 2) == 2, -c0, c0)
    sin = jnp.where((q & 2) == 2, -s0, s0)
    return cos, sin


def _odd_freq(r):
    return jnp.where(r < 64, 4 * r + 1, 4 * r - 253)


def _gelu2(z):
    u = z * (GELU_C + (GELU_C * 0.044715) * (z * z))
    return z + z * jnp.tanh(u)


def _signzero(z):
    bits = jax.lax.bitcast_convert_type(z, U32) & jnp.uint32(0x80000000)
    return jax.lax.bitcast_convert_type(bits, F32)


def _ln(x, eps, tie=None, scale=None):
    n = x.shape[-1]
    part = x[:, 0:L]
    for j in range(1, n // L):
        part = part + x[:, j * L:(j + 1) * L]
    if tie is not None:
        part = part + tie
    m = jnp.sum(part, axis=-1, keepdims=True) * (1.0 / n)
    xc = x - m
    v = jnp.sum(xc * xc, axis=-1, keepdims=True) * (1.0 / n)
    rs = jax.lax.rsqrt(v + eps)
    if scale is not None:
        rs = rs * scale
    return xc * rs


def _blocks_of_step(i):
    return STEP_BLOCKS[i]


class _Background:
    def __init__(self):
        self.q = []
        self.credit = 0.0

    def add(self, gen):
        self.q.append(gen)

    def run(self, budget):
        self.credit += budget
        while self.q and self.credit > 0:
            try:
                self.credit -= next(self.q[0])
            except StopIteration:
                self.q.pop(0)
        if not self.q:
            self.credit = 0.0

    def drain(self):
        while self.q:
            self.run(1e9)


class _Tied:
    def __init__(self, tasks, npieces):
        self.tasks = list(tasks)
        self.rate = len(self.tasks) / float(npieces)
        self.credit = 0.999

    def run(self, z):
        self.credit += self.rate
        n = 0
        while self.tasks and self.credit >= 1.0:
            self.tasks.pop(0)(_signzero(z[0:16]))
            self.credit -= 1.0
            n += 1
        return n


def _kernel(one_ref, q_hbm, k_hbm, v_hbm, sk_hbm, h_hbm, d_hbm, win_hbm, wsp_hbm, b_hbm, wout_hbm,
            o_hbm,
            x_u, k_u, v_u, h_u, win_u, wsp_u, wout_u, o_v, sk_in, d_in, b_in,
            xn_u, XL_u, WB_u, UL_u, WO_u, z1_v, R_u, Lc_u, zf_v, zg_v, kv_u, u_u, X_v, H_v, G_v, Z_u, yl_v, F_u, Fi_u, bcol_v, ph_v, sk_v, kf_v,
            sem_small, sem_x, sem_conv, sem_wsp, sem_w, sem_out):
    x_v, k_v, v_v, h_v, win_v, wsp_v, wout_v, xn_v, XL_v, WB_v, UL_v, WO_v, R_v, Lc_v, kv_v, u_v, Z_v, F_v, Fi_v = [
        r.bitcast(BF16) for r in (x_u, k_u, v_u, h_u, win_u, wsp_u, wout_u, xn_u, XL_u, WB_u, UL_u, WO_u, R_u, Lc_u, kv_u, u_u, Z_u, F_u,
                                  Fi_u)]

    def cp_small():
        return [pltpu.make_async_copy(s_, d_, sem_small.at[0])
                for s_, d_ in ((d_hbm, d_in), (sk_hbm, sk_in), (b_hbm, b_in))]

    def cp_x(t):
        return pltpu.make_async_copy(q_hbm.at[0, pl.ds(t * TM, TM)], x_v.at[pl.ds(t * TM, TM)], sem_x.at[t % 3])

    def cp_conv(t):
        rows = pl.ds(t * TM, TM)
        sem = sem_conv.at[t % 2]
        return [pltpu.make_async_copy(h_hbm.at[:, rows], h_v.at[t], sem),
                pltpu.make_async_copy(k_hbm.at[0, rows], k_v.at[rows], sem),
                pltpu.make_async_copy(v_hbm.at[0, rows], v_v.at[rows], sem)]

    def cp_wsp(i, which=(0, 1)):
        return [pltpu.make_async_copy(wsp_hbm.at[pl.ds(_blocks_of_step(i)[half] * P, P)],
                                      wsp_v.at[pl.ds(i * TM + half * P, P)], sem_wsp.at[i % 5]) for half in which]

    def cp_win(c):
        lo, hi = WIN_CHUNKS[c]
        cols = pl.ds(lo * L, (hi - lo) * L)
        return pltpu.make_async_copy(win_hbm.at[:, cols], win_v.at[:, cols], sem_w.at[c])

    def cp_wout():
        return pltpu.make_async_copy(wout_hbm, wout_v, sem_w.at[0])

    def cp_out(i):
        rows = pl.ds(_blocks_of_step(i)[0] * P, TM)
        return [pltpu.make_async_copy(o_v.at[rows], o_hbm.at[0, rows], sem_out.at[i % 5])]

    def start(cs):
        for c in cs:
            c.start()

    def wait(cs):
        for c in cs:
            c.wait()

    always = one_ref[0] == 1

    def block(fn, name):
        if _ONLY is None or name in _ONLY:
            pl.when(always)(fn)

    def ln_x(t, s, tie=None):
        rows = pl.ds(t * TM + s * 16, 16)
        y = _ln(x_v[rows, :].astype(F32), EPS, tie)
        xn_v[rows, :] = y.astype(BF16)
        return y

    def ln_x2(t, s, tie):
        p, q = s // 4, s % 4
        y1 = ln_x(t, 8 * p + q, tie)
        y2 = ln_x(t, 8 * p + 4 + q, tie)
        a11, a12, a21, a22 = y1[:, :KH], y1[:, KH:2 * KH], y2[:, :KH], y2[:, KH:2 * KH]
        r0 = (t % 2) * 5 * P + p * MC + q * 16
        for j, c in enumerate((a11 + a22, a21 + a22, a11 + a12, a21 - a11, a12 - a22)):
            XL_v[pl.ds(r0 + j * P, 16), :] = c.astype(BF16)

    def wcomb_gen(cols):
        for j in cols:
            c1 = slice(j * L, (j + 1) * L)
            c2 = slice(FH + j * L, FH + (j + 1) * L)
            for r in range(KH // 32):
                top = pl.ds(r * 32, 32)
                bot = pl.ds(KH + r * 32, 32)
                b11, b12 = win_v[top, c1].astype(F32), win_v[top, c2].astype(F32)
                b21, b22 = win_v[bot, c1].astype(F32), win_v[bot, c2].astype(F32)
                for w, c in enumerate((b11 + b22, b12 - b22, b21 - b11, b11 + b12, b21 + b22)):
                    WB_v[pl.ds(w * KH + r * 32, 32), c1] = c.astype(BF16)
                yield A_COST

    def ln_z2(t, s, tie=None):
        y = _ln(zg_v[t % 2, s * 16:(s + 1) * 16, :], 4.0 * EPS, tie, 0.25)
        lo, hi = y[:, :HN], y[:, HN:]
        r = (t * TM + s * 16) % HK
        rows = pl.ds(r, 16)
        if t < NT // 2:
            zf_v[rows, :] = y
            R_v[pl.ds(1 * HK + r, 16), :] = lo.astype(BF16)
            R_v[pl.ds(5 * HK + r, 16), :] = (lo + hi).astype(BF16)
        else:
            b11 = zf_v[rows, :HN]
            R_v[pl.ds(0 * HK + r, 16), :] = (b11 + hi).astype(BF16)
            R_v[pl.ds(2 * HK + r, 16), :] = (zf_v[rows, HN:] - hi).astype(BF16)
            R_v[pl.ds(3 * HK + r, 16), :] = (lo - b11).astype(BF16)
            R_v[pl.ds(4 * HK + r, 16), :] = hi.astype(BF16)
            R_v[pl.ds(6 * HK + r, 16), :] = (lo + hi).astype(BF16)

    def acomb_gen(i):
        for r in range(P // 16):
            for c in range(HK // 256):
                top = pl.ds(i * TM + r * 16, 16)
                bot = pl.ds(i * TM + P + r * 16, 16)
                c1 = slice(c * 256, (c + 1) * 256)
                c2 = slice(HK + c * 256, HK + (c + 1) * 256)
                a11 = wsp_v[top, c1].astype(F32)
                a12 = wsp_v[top, c2].astype(F32)
                a21 = wsp_v[bot, c1].astype(F32)
                a22 = wsp_v[bot, c2].astype(F32)
                r0 = (i % 4) * 5 * P + r * 16
                Lc_v[pl.ds(r0 + 0 * P, 16), c1] = (a11 + a22).astype(BF16)
                Lc_v[pl.ds(r0 + 1 * P, 16), c1] = (a21 + a22).astype(BF16)
                Lc_v[pl.ds(r0 + 2 * P, 16), c1] = (a11 + a12).astype(BF16)
                Lc_v[pl.ds(r0 + 3 * P, 16), c1] = (a21 - a11).astype(BF16)
                Lc_v[pl.ds(r0 + 4 * P, 16), c1] = (a12 - a22).astype(BF16)
                yield A_COST

    def tasks(fn, t, n=TM // 16):
        return [lambda tie, s=s: fn(t, s, tie) for s in range(n)]

    def kv_gen(t):
        for m in range(TM // MC):
            r = t * TM + m * MC
            for l in range(D // L):
                lanes = slice(l * L, (l + 1) * L)
                kf = k_v[pl.ds(r, MC), lanes].astype(F32)
                kf_v[l, pl.ds(r + 8, MC), :] = kf
                ks = kf * sk_v[0, 0:1, lanes]
                for tap in range(1, 4):
                    ks = ks + kf_v[l, pl.ds(r + 8 - tap, MC), :] * sk_v[tap, 0:1, lanes]
                kv = ks * v_v[pl.ds(r, MC), lanes].astype(F32)
                kv_v[pl.ds(r, MC), lanes] = kv.astype(BF16)
                yield KV_COST

    def g_gen(t):
        for r in range(P // 16):
            rows = pl.ds(r * 16, 16)
            for l in range(D // L):
                lanes = slice(l * L, (l + 1) * L)
                h = [(H_v[(2 * t + w) % 6, 0, rows, lanes], H_v[(2 * t + w) % 6, 1, rows, lanes]) for w in range(3)]
                for w in range(2):
                    (pr, pi), (cr, ci) = h[w], h[w + 1]
                    G_v[2 * t + w, 0, rows, lanes] = cr - pi if r < P // 32 else cr + pi
                    G_v[2 * t + w, 1, rows, lanes] = ci + pr if r < P // 32 else ci - pr
                yield G_COST

    def freq_gen(a):
        def cmac(acc, x, g):
            pr = x[0] * g[0] - x[1] * g[1]
            pi = x[0] * g[1] + x[1] * g[0]
            return (pr, pi) if acc is None else (acc[0] + pr, acc[1] + pi)

        for r in range(P // 16):
            rows = pl.ds(r * 16, 16)
            for l in range(D // L):
                lanes = slice(l * L, (l + 1) * L)
                lo = hi = None
                g = (G_v[a + 1, 0, rows, lanes], G_v[a + 1, 1, rows, lanes])
                for c in range(a + 2):
                    x = (X_v[c, 0, rows, lanes], X_v[c, 1, rows, lanes])
                    hi = cmac(hi, x, g)
                    if c <= a:
                        g = (G_v[a - c, 0, rows, lanes], G_v[a - c, 1, rows, lanes])
                        lo = cmac(lo, x, g)
                        yield 32
                for w, z in enumerate((lo, hi)):
                    for part in range(2):
                        Z_v[pl.ds((a + w) * 2 * P + part * P + r * 16, 16), lanes] = z[part].astype(BF16)
                yield 20

    def job_h(t, bg, budget):
        for j in (2 * t, 2 * t + 1):
            for part in range(2):
                hp = jax.lax.dot_general(F_v[part * P:(part + 1) * P, 0:P],
                                         h_v[t, :, (j % 2) * P:(j % 2 + 1) * P],
                                         NT_DIMS, preferred_element_type=F32)
                for g in range(8):
                    rows = pl.ds(part * 64 + g * 8, 8)
                    H_v[(j + 1) % 6, 0, rows, :] = hp[g * 16:g * 16 + 8]
                    H_v[(j + 1) % 6, 1, rows, :] = hp[g * 16 + 8:g * 16 + 16]
                bg.run(budget)

    def job_x(t, bg, budget):
        for j in (2 * t, 2 * t + 1):
            for part in range(2):
                xp = _dot(F_v[part * P:(part + 1) * P, 0:P], kv_v[j * P:(j + 1) * P, :])
                for g in range(8):
                    rows = pl.ds(part * 64 + g * 8, 8)
                    X_v[j, 0, rows, :] = xp[g * 16:g * 16 + 8]
                    X_v[j, 1, rows, :] = xp[g * 16 + 8:g * 16 + 16]
                bg.run(budget)

    def z_out(t, m, n, pre, bg, budget, tied):
        z = _gelu2(pre)
        if n < FH // L:
            z1_v[pl.ds(t * TM + m * MC, MC), n * L:(n + 1) * L] = z
        else:
            zg_v[t % 2, m * MC:(m + 1) * MC, n * L - FH:(n + 1) * L - FH] = z
        ntask = tied.run(z)
        bg.run(budget[1] if ntask else budget[0])

    def job_z(t, m, cols, bg, budget, tied):
        for n in cols:
            z_out(t, m, n, _dot(xn_v[pl.ds(t * TM + m * MC, MC), :], win_v[:, n * L:(n + 1) * L]), bg, budget, tied)

    def job_zs(t, p, j, bg, budget, tied):
        r1 = pl.ds(t * TM + p * P, MC)
        r2 = pl.ds(t * TM + p * P + MC, MC)
        c1 = slice(j * L, (j + 1) * L)
        c2 = slice(FH + j * L, FH + (j + 1) * L)

        def xl(w):
            r0 = (t % 2) * 5 * P + w * P + p * MC
            return XL_v[r0:r0 + MC, :]

        def wb(w):
            return WB_v[w * KH:(w + 1) * KH, c1]

        def rem(rows, cols):
            return _dot(xn_v[rows, 2 * KH:], win_v[2 * KH:, cols])

        m2 = _dot(xl(1), win_v[0:KH, c1])
        m4 = _dot(xn_v[r2, KH:2 * KH], wb(2))
        z_out(t, 2 * p + 1, j, m2 + m4 + rem(r2, c1), bg, budget, tied)
        m3 = _dot(xn_v[r1, 0:KH], wb(1))
        m5 = _dot(xl(2), win_v[KH:2 * KH, c2])
        z_out(t, 2 * p, 6 + j, m3 + m5 + rem(r1, c2), bg, budget, tied)
        m1 = _dot(xl(0), wb(0))
        z_out(t, 2 * p, j, (m4 - m5) + m1 + _dot(xl(4), wb(4)) + rem(r1, c1), bg, budget, tied)
        z_out(t, 2 * p + 1, 6 + j, (m3 - m2) + m1 + _dot(xl(3), wb(3)) + rem(r2, c2), bg, budget, tied)

    rev8 = 7 - jax.lax.broadcasted_iota(jnp.int32, (8, L), 0)

    def finish(a, upper, n, hh):
        rows = pl.ds(a * P + (MC if upper else 0), MC)
        lanes = slice(n * L, (n + 1) * L)
        if upper:
            ya = _dot(Fi_v[:, 0:P], Z_v[a * 2 * P:a * 2 * P + P, lanes])
            yb = _dot(Fi_v[:, P:2 * P], Z_v[a * 2 * P + P:(a + 1) * 2 * P, lanes])
            y = ya - yb
            lo = ya + yb
            for j in range(MC // 8):
                yl_v[a % 2, n, (7 - j) * 8:(8 - j) * 8, :] = jnp.take_along_axis(lo[j * 8:(j + 1) * 8], rev8, axis=0)
        else:
            y = yl_v[a % 2, n]
        gate = hh + hh * jnp.tanh(hh)
        s = xn_v[rows, lanes].astype(F32) * y
        o_v[rows, lanes] = (x_v[rows, lanes].astype(F32) + s * gate).astype(BF16)

    def tail_gen(i):
        a0, a1 = _blocks_of_step(i)
        for upper in (True, False):
            sub = MC if upper else 0
            r1 = pl.ds(a0 * P + sub, MC)
            r2 = pl.ds(a1 * P + sub, MC)

            def ul(w):
                r0 = ((i % 4) * 5 + w) * P + sub
                return UL_v[r0:r0 + MC, :]

            for j in range(2):
                c1 = slice(j * L, (j + 1) * L)
                c2 = slice((2 + j) * L, (3 + j) * L)

                def wo(w):
                    return WO_v[w * HN:(w + 1) * HN, c1]

                m2 = _dot(ul(1), wout_v[0:HN, c1])
                m4 = _dot(u_v[r2, HN:], wo(2))
                finish(a1, upper, j, m2 + m4)
                yield
                m3 = _dot(u_v[r1, 0:HN], wo(1))
                m5 = _dot(ul(2), wout_v[HN:, c2])
                finish(a0, upper, 2 + j, m3 + m5)
                yield
                m1 = _dot(ul(0), wo(0))
                finish(a0, upper, j, (m4 - m5) + m1 + _dot(ul(4), wo(4)))
                yield
                finish(a1, upper, 2 + j, (m3 - m2) + m1 + _dot(ul(3), wo(3)))
                yield
            finish(a0, upper, 4, _dot(u_v[r1, :], wout_v[:, 4 * L:]))
            yield
            finish(a1, upper, 4, _dot(u_v[r2, :], wout_v[:, 4 * L:]))
            yield

    def wocomb_gen():
        for j in range(2):
            c1 = slice(j * L, (j + 1) * L)
            c2 = slice((2 + j) * L, (3 + j) * L)
            for r in range(HN // 32):
                top = pl.ds(r * 32, 32)
                bot = pl.ds(HN + r * 32, 32)
                b11, b12 = wout_v[top, c1].astype(F32), wout_v[top, c2].astype(F32)
                b21, b22 = wout_v[bot, c1].astype(F32), wout_v[bot, c2].astype(F32)
                for w, c in enumerate((b11 + b22, b12 - b22, b21 - b11, b11 + b12, b21 + b22)):
                    WO_v[pl.ds(w * HN + r * 32, 32), c1] = c.astype(BF16)
                yield A_COST

    def job_big(i, bg, pending, budget, every):
        a0, a1 = _blocks_of_step(i)
        KG = 512
        count = [0, 0]

        def lhs(j, sub, cols):
            if j == 2:
                return wsp_v[i * TM + sub:i * TM + sub + MC, cols]
            if j == 3:
                return wsp_v[i * TM + P + sub:i * TM + P + sub + MC, HK + cols.start:HK + cols.stop]
            r0 = ((i % 4) * 5 + {0: 0, 1: 1, 4: 2, 5: 3, 6: 4}[j]) * P + sub
            return Lc_v[r0:r0 + MC, cols]

        def prod(j, sub, n, acc=None):
            for kg in range(HK // KG):
                ks = slice(kg * KG, (kg + 1) * KG)
                p = _dot(lhs(j, sub, ks), R_v[j * HK + kg * KG:j * HK + (kg + 1) * KG, n * L:(n + 1) * L])
                acc = p if acc is None else acc + p
                bg.run(budget)
            count[0] += 1
            return acc

        def maybe_tail():
            count[1] += 1
            if pending and count[0] >= 3 and count[1] % every == 0:
                next(pending.pop(0))
                bg.run(budget)

        def emit(a, sub, n, g):
            rows = pl.ds(a * P + sub, MC)
            lanes = slice(n * L, (n + 1) * L)
            u = z1_v[rows, lanes] * (g + bcol_v[rows, :])
            u_v[rows, lanes] = u.astype(BF16)
            return u

        for sub in (0, MC):
            for n in range(HN // L):
                m2 = prod(1, sub, n)
                m4 = prod(3, sub, n)
                u21 = emit(a1, sub, n, m2 + m4)
                maybe_tail()
                m3 = prod(2, sub, n)
                t22 = m3 - m2
                m5 = prod(4, sub, n)
                u12 = emit(a0, sub, n + HN // L, m3 + m5)
                t11 = m4 - m5
                maybe_tail()
                m1 = prod(0, sub, n)
                maybe_tail()
                u11 = emit(a0, sub, n, prod(6, sub, n, t11 + m1))
                u22 = emit(a1, sub, n + HN // L, prod(5, sub, n, t22 + m1))
                for w, c in enumerate((u11 + u22, u21 + u22, u11 + u12, u21 - u11, u12 - u22)):
                    UL_v[pl.ds(((i % 4) * 5 + w) * P + sub, MC), n * L:(n + 1) * L] = c.astype(BF16)
                maybe_tail()

    if _ONLY is not None:
        for r_ in (xn_u, XL_u, WB_u, UL_u, WO_u, z1_v, R_u, Lc_u, zf_v, zg_v, kv_u, u_u, X_v, H_v, G_v, Z_u, kf_v):
            c_ = pltpu.make_async_copy(r_, r_, sem_small.at[0])
            c_.start()
            c_.wait()

    cp_x(0).start()
    cp_x(1).start()
    for c in range(5):
        cp_win(c).start()
    cp_x(2).start()
    start(cp_small())

    kk = _odd_freq(jax.lax.broadcasted_iota(jnp.int32, (P, P), 0))
    nn = jax.lax.broadcasted_iota(jnp.int32, (P, P), 1)
    fc, fs = _cos_sin((kk * (4 * nn - 127)) & 2047)
    for g in range(P // 8):
        F_v[g * 16:(g + 1) * 16, 0:P] = jnp.concatenate(
            [fc[g * 8:(g + 1) * 8], -fs[g * 8:(g + 1) * 8]], axis=0).astype(BF16)
    fc, fs = _cos_sin((kk * (-127)) & 2047)
    ph_v[0] = fc
    ph_v[1] = fs
    kk = _odd_freq(jax.lax.broadcasted_iota(jnp.int32, (MC, P), 1))
    mm = jax.lax.broadcasted_iota(jnp.int32, (MC, P), 0)
    ic, is_ = _cos_sin((kk * (4 * mm + 2)) & 2047)
    Fi_v[:, 0:P] = (ic * (1.0 / P)).astype(BF16)
    Fi_v[:, P:2 * P] = (is_ * (1.0 / P)).astype(BF16)
    kf_v[:, 0:8, :] = jnp.zeros((D // L, 8, L), F32)

    for t in range(2):
        cp_x(t).wait()
        for s in range(TM // 16):
            ln_x(t, s)

    def small_setup():
        sk = sk_in[...].astype(F32)
        for t in range(4):
            sk_v[t] = jnp.broadcast_to(sk[t:t + 1], (8, D))
        drow = d_in[...].astype(F32).reshape(1, D)
        for l in range(D // L):
            lanes = slice(l * L, (l + 1) * L)
            dre = ph_v[0] * drow[:, lanes]
            dim = ph_v[1] * drow[:, lanes]
            H_v[0, 0, 0:64, lanes] = -dim[0:64]
            H_v[0, 0, 64:P, lanes] = dim[64:P]
            H_v[0, 1, 0:64, lanes] = -dre[0:64]
            H_v[0, 1, 64:P, lanes] = dre[64:P]

    def bcol_task(t, j, tie):
        brow = b_in[...].astype(F32).reshape(1, S)[:, j * P:(j + 1) * P] * 0.25 + tie[0:1]
        bcol_v[j * P:(j + 1) * P, :] = jnp.broadcast_to(brow, (P, P)).T

    LAG = 2

    def interleave(*lists):
        out = []
        for j in range(max(len(a) for a in lists)):
            for a in lists:
                out += a[j:j + 1]
        return out

    def p1_first(c):
        bg = _Background()
        todo = []
        if c == 3:
            todo = tasks(ln_z2, 0)
            bg.add(wcomb_gen(range(3)))
        if c == 4:
            todo = tasks(ln_x2, 2, 8)
            bg.add(wcomb_gen(range(3, 6)))
            small_setup()
        tied = _Tied(todo, 20)
        for t in range(2):
            for m in range(TM // MC):
                job_z(t, m, range(*WIN_CHUNKS[c]), bg, (80, 40), tied)
        bg.drain()
        assert not tied.tasks

    for c in range(5):
        cp_win(c).wait()
        if c == 2:
            start(cp_conv(0))
            cp_x(3).start()
        if c == 4:
            cp_x(2).wait()
            wait(cp_small())
        block(lambda c=c: p1_first(c), f'p1_f{c}')

    def p1_dma(i):
        wait(cp_conv(i - LAG))
        if i + 1 < NT:
            cp_x(i + 1).wait()
        if i == 4:
            cp_wout().wait()
        if i == NT - 3:
            wait(cp_wsp(0))
        if i + 2 < NT:
            cp_x(i + 2).start()
        start(cp_conv(i - LAG + 1))
        if i == NT - 1:
            start(cp_conv(NT - 1))
        start(cp_wsp((i - 2) // 2, ((i - 2) % 2,)))
        if i == 2:
            cp_wout().start()

    acomb0 = acomb_gen(0)

    def take(gen, n):
        for _ in range(n):
            yield next(gen)

    def p1_step(i):
        bg = _Background()
        dft = _Background()
        t = i - LAG
        kv = kv_gen(t)
        dft.add(take(kv, 20 if t >= 1 else 10))
        if t >= 1:
            bg.add(g_gen(t - 1))
        else:
            bg.add(take(kv, 10))
        extra = 0
        if i == 4:
            bg.add(wocomb_gen())
            extra = 30
        if i in (NT - 3, NT - 2):
            bg.add(take(acomb0, 16))
            extra = 20
        last = i == NT - 1
        z2t = tasks(ln_z2, i - 1)
        todo = interleave(tasks(ln_x2, i + 1, 8) if not last else [], z2t[0::2], z2t[1::2],
                          tasks(bcol_task, 0) if i == 2 else [])
        tied = _Tied(todo, 24 if last else 42)
        if t >= 1:
            dft.run(110)
            job_x(t - 1, dft, 250)
        for p in range(2):
            for j in range(FH // L):
                job_zs(i, p, j, bg, (60 + extra, 10 + extra), tied)
            if p == 0 and last:
                tied = _Tied(tasks(ln_z2, i, 8), 22)
        assert not tied.tasks
        if last:
            for s in range(8, 16):
                ln_z2(i, s)
        job_h(t, dft, 275)
        bg.drain()
        dft.drain()

    for i in range(2, NT):
        p1_dma(i)
        block(lambda i=i: p1_step(i), f'p1_{i}')

    groups = P2_GROUPS
    NG = len(groups)

    def p2_dma(gi):
        if gi >= 2:
            for i in groups[gi - 2]:
                start(cp_out(i))
        if gi >= 3:
            for i in groups[gi - 3]:
                wait(cp_out(i))
        if gi + 2 < NG:
            for i in groups[gi + 2]:
                start(cp_wsp(i))
        if gi < 2:
            wait(cp_conv(NT - 2 + gi))
        if gi + 1 < NG:
            for i in groups[gi + 1]:
                wait(cp_wsp(i))

    def tails_of(i):
        return [tail_gen(i)] * 20

    def p2_block(gi):
        bg = _Background()
        steps = groups[gi]
        pending = [t_ for i in (groups[gi - 1] if gi > 0 else []) for t_ in tails_of(i)]
        total = sum(a + 1 for i in steps for a in _blocks_of_step(i)) * 40 * 16
        slots = 84 * len(steps) + len(pending)
        bg.add(freq_gen(_blocks_of_step(steps[0])[0]))
        if gi < 2:
            bg.add(kv_gen(NT - 2 + gi))
            total += 20 * KV_COST
            slots += 8
        if gi < 3:
            slots += 8
            bg.add(g_gen(NT - 3 + gi))
            total += 40 * G_COST
        if gi + 1 < NG:
            for i in groups[gi + 1]:
                bg.add(acomb_gen(i))
                total += 32 * A_COST
        for i in steps[1:]:
            bg.add(freq_gen(_blocks_of_step(i)[0]))
        budget = total / (slots + 1.0)
        bg.run(budget)
        if gi < 3:
            job_x(NT - 3 + gi, bg, 2 * budget)
        if gi < 2:
            job_h(NT - 2 + gi, bg, 2 * budget)
        every = max(1, (24 * len(steps) - 2) // max(1, len(pending)))
        for i in steps:
            job_big(i, bg, pending, budget, every)
        for t_ in pending:
            next(t_)
            bg.run(budget)
        bg.drain()

    for gi in range(NG):
        p2_dma(gi)
        block(lambda gi=gi: p2_block(gi), f'p2_{gi}')

    def cp_last(upper):
        a0 = _blocks_of_step(NT - 1)[0]
        return [pltpu.make_async_copy(o_v.at[pl.ds(r, MC)], o_hbm.at[0, pl.ds(r, MC)], sem_out.at[(NT - 1) % 5])
                for r in ((a0 + w) * P + (MC if upper else 0) for w in range(2))]

    def p2_last():
        for j, t_ in enumerate(tails_of(NT - 1)):
            next(t_)
            if j == 9:
                start(cp_last(True))

    p2_dma(NG)
    block(p2_last, 'p2_last')
    start(cp_last(False))
    for i in groups[NG - 2]:
        wait(cp_out(i))
    wait(cp_last(True))
    wait(cp_last(False))
    if _ONLY is not None:
        for r_ in (xn_u, XL_u, WB_u, UL_u, WO_u, z1_v, R_u, Lc_u, zf_v, zg_v, kv_u, u_u, X_v, H_v, G_v, Z_u, kf_v):
            c_ = pltpu.make_async_copy(r_, r_, sem_small.at[0])
            c_.start()
            c_.wait()


@jax.jit
def pallas_recurrent_scan__ssm_conv_h3__mixer_gmlp__prompt_kernel(
    A_q: jax.Array,
    A_k: jax.Array,
    A_v: jax.Array,
    A_shift_k: jax.Array,
    A_ssm_k: jax.Array,
    A_ssm_D: jax.Array,
    B_x: jax.Array,
    B_w_in: jax.Array,
    B_w_sp: jax.Array,
    B_b_sp: jax.Array,
    B_w_out: jax.Array,
):
    del B_x
    hbm = pl.BlockSpec(memory_space=pl.ANY)

    def bf16_buf(*shape):
        return pltpu.VMEM(shape[:-2] + (shape[-2] // 2, shape[-1]), U32)

    return pl.pallas_call(
        _kernel,
        out_shape=jax.ShapeDtypeStruct((1, S, D), BF16),
        in_specs=[pl.BlockSpec(memory_space=pltpu.SMEM)] + [hbm] * 10,
        out_specs=hbm,
        scratch_shapes=[
            bf16_buf(S, D),
            bf16_buf(S, D),
            bf16_buf(S, D),
            bf16_buf(NT, D, TM),
            bf16_buf(D, 2 * FH),
            bf16_buf(S, S),
            bf16_buf(FH, D),
            pltpu.VMEM((S, D), BF16),
            pltpu.VMEM((4, D), BF16),
            pltpu.VMEM((D,), BF16),
            pltpu.VMEM((S,), BF16),
            bf16_buf(S, D),
            bf16_buf(2 * 5 * P, KH),
            bf16_buf(5 * KH, FH),
            bf16_buf(4 * 5 * P, HN),
            bf16_buf(5 * HN, 2 * L),
            pltpu.VMEM((S, FH), F32),
            bf16_buf(7 * HK, HN),
            bf16_buf(4 * 5 * P, HK),
            pltpu.VMEM((HK, FH), F32),
            pltpu.VMEM((2, TM, FH), F32),
            bf16_buf(S, D),
            bf16_buf(S, FH),
            pltpu.VMEM((NB, 2, P, D), F32),
            pltpu.VMEM((6, 2, P, D), F32),
            pltpu.VMEM((NB, 2, P, D), F32),
            bf16_buf(NB * 2 * P, D),
            pltpu.VMEM((2, D // L, MC, L), F32),
            bf16_buf(2 * P, 2 * P),
            bf16_buf(MC, 2 * P),
            pltpu.VMEM((S, L), F32),
            pltpu.VMEM((2, P, L), F32),
            pltpu.VMEM((4, 8, D), F32),
            pltpu.VMEM((D // L, S + 8, L), F32),
            pltpu.SemaphoreType.DMA((1,)),
            pltpu.SemaphoreType.DMA((3,)),
            pltpu.SemaphoreType.DMA((2,)),
            pltpu.SemaphoreType.DMA((5,)),
            pltpu.SemaphoreType.DMA((5,)),
            pltpu.SemaphoreType.DMA((5,)),
        ],
        compiler_params=pltpu.CompilerParams(vmem_limit_bytes=116 * 1024 * 1024),
    )(jnp.ones((1,), jnp.int32), A_q, A_k, A_v, A_shift_k.T, A_ssm_k, A_ssm_D, B_w_in, B_w_sp, B_b_sp, B_w_out)
```

```python
import math

import jax
import jax.numpy as jnp
import jax.experimental.pallas as pl
import jax.experimental.pallas.tpu as pltpu

S = 2048
D = 640
FH = 768
P = 128
NB = S // P
TM = 256
NT = S // TM
MC = 64
L = 128
HK = S // 2
KH = 256
HN = FH // 2
P2_GROUPS = ((0,), (1, 2), (3, 4), (5, 6), (7,))
STEP_BLOCKS = ((6, 7), (8, 9), (4, 5), (12, 13), (2, 3), (14, 15), (0, 1), (10, 11))
KV_COST, G_COST, A_COST = 110, 36, 56
E_COST, U_COST, T_COST, TAIL_W = 24, 90, 90, 1.6
BIG_KG = 512
H_FIRST = True
TIED_N = 44
FR = 16
DFT_SPLIT = ((0, 5),)
KV_ROWS = 64
WIN_CHUNKS = ((6, 7), (7, 9), (9, 12), (0, 3), (3, 6))
EPS = 1e-5
F32 = jnp.float32
BF16 = jnp.bfloat16
U32 = jnp.uint32
GELU_C = math.sqrt(2.0 / math.pi)
NT_DIMS = (((1,), (1,)), ((), ()))
_ONLY = None


def _dot(a, b):
    return jnp.dot(a, b, preferred_element_type=F32)


def _cos_sin(m):
    q = (m + 256) >> 9
    x = (m - (q << 9)).astype(F32) * (2.0 * math.pi / 2048.0)
    x2 = x * x
    s = x * (1.0 + x2 * (-1.0 / 6 + x2 * (1.0 / 120 + x2 * (-1.0 / 5040 + x2 * (1.0 / 362880)))))
    c = 1.0 + x2 * (-0.5 + x2 * (1.0 / 24 + x2 * (-1.0 / 720 + x2 * (1.0 / 40320 - x2 * (1.0 / 3628800)))))
    swap = (q & 1) == 1
    c0 = jnp.where(swap, s, c)
    s0 = jnp.where(swap, c, s)
    cos = jnp.where(((q + 1) & 2) == 2, -c0, c0)
    sin = jnp.where((q & 2) == 2, -s0, s0)
    return cos, sin


def _odd_freq(r):
    return jnp.where(r < 64, 4 * r + 1, 4 * r - 253)


def _gelu2(z):
    u = z * (GELU_C + (GELU_C * 0.044715) * (z * z))
    return z + z * jnp.tanh(u)


def _signzero(z):
    bits = jax.lax.bitcast_convert_type(z, U32) & jnp.uint32(0x80000000)
    return jax.lax.bitcast_convert_type(bits, F32)


def _ln(x, eps, tie=None, scale=None):
    n = x.shape[-1]
    part = x[:, 0:L]
    for j in range(1, n // L):
        part = part + x[:, j * L:(j + 1) * L]
    if tie is not None:
        part = part + tie
    m = jnp.sum(part, axis=-1, keepdims=True) * (1.0 / n)
    xc = x - m
    v = jnp.sum(xc * xc, axis=-1, keepdims=True) * (1.0 / n)
    rs = jax.lax.rsqrt(v + eps)
    if scale is not None:
        rs = rs * scale
    return xc * rs


def _blocks_of_step(i):
    return STEP_BLOCKS[i]


class _Background:
    def __init__(self):
        self.q = []
        self.credit = 0.0

    def add(self, gen):
        self.q.append(gen)

    def run(self, budget):
        self.credit += budget
        while self.q and self.credit > 0:
            try:
                self.credit -= next(self.q[0])
            except StopIteration:
                self.q.pop(0)
        if not self.q:
            self.credit = 0.0

    def charge(self, cost):
        self.credit -= cost

    def drain(self):
        while self.q:
            self.run(1e9)


class _Tied:
    def __init__(self, tasks, npieces):
        self.tasks = list(tasks)
        self.rate = len(self.tasks) / float(npieces)
        self.credit = 0.999

    def run(self, z):
        self.credit += self.rate
        n = 0
        while self.tasks and self.credit >= 1.0:
            self.tasks.pop(0)(_signzero(z[0:16]))
            self.credit -= 1.0
            n += 1
        return n


def _kernel(q_hbm, k_hbm, v_hbm, sk_hbm, h_hbm, d_hbm, win_hbm, wsp_hbm, b_hbm, wout_hbm,
            o_hbm,
            x_u, k_u, v_u, h_u, win_u, wsp_u, wout_u, o_v, sk_in, d_in, b_in,
            xn_u, XL_u, WB_u, UL_u, WO_u, z1_v, R_u, Lc_u, zf_v, zg_v, kv_u, u_u, X_v, H_v, G_v, Z_u, yl_v, F_u, Fi_u, bcol_v, ph_v, sk_v, kf_v,
            sem_small, sem_x, sem_conv, sem_wsp, sem_w, sem_out):
    x_v, k_v, v_v, h_v, win_v, wsp_v, wout_v, xn_v, XL_v, WB_v, UL_v, WO_v, R_v, Lc_v, kv_v, u_v, Z_v, F_v, Fi_v = [
        r.bitcast(BF16) for r in (x_u, k_u, v_u, h_u, win_u, wsp_u, wout_u, xn_u, XL_u, WB_u, UL_u, WO_u, R_u, Lc_u, kv_u, u_u, Z_u, F_u,
                                  Fi_u)]

    def cp_small():
        return [pltpu.make_async_copy(s_, d_, sem_small.at[0])
                for s_, d_ in ((d_hbm, d_in), (sk_hbm, sk_in), (b_hbm, b_in))]

    def cp_x(t):
        return pltpu.make_async_copy(q_hbm.at[0, pl.ds(t * TM, TM)], x_v.at[pl.ds(t * TM, TM)], sem_x.at[t % 3])

    def cp_conv(t):
        rows = pl.ds(t * TM, TM)
        sem = sem_conv.at[t % 2]
        return [pltpu.make_async_copy(h_hbm.at[:, rows], h_v.at[t], sem),
                pltpu.make_async_copy(k_hbm.at[0, rows], k_v.at[rows], sem),
                pltpu.make_async_copy(v_hbm.at[0, rows], v_v.at[rows], sem)]

    def cp_wsp(i, which=(0, 1)):
        return [pltpu.make_async_copy(wsp_hbm.at[pl.ds(_blocks_of_step(i)[half] * P, P)],
                                      wsp_v.at[pl.ds(i * TM + half * P, P)], sem_wsp.at[i % 5]) for half in which]

    def cp_win(c):
        lo, hi = WIN_CHUNKS[c]
        cols = pl.ds(lo * L, (hi - lo) * L)
        return pltpu.make_async_copy(win_hbm.at[:, cols], win_v.at[:, cols], sem_w.at[c])

    def cp_wout():
        return pltpu.make_async_copy(wout_hbm, wout_v, sem_w.at[0])

    def cp_out(i):
        rows = pl.ds(_blocks_of_step(i)[0] * P, TM)
        return [pltpu.make_async_copy(o_v.at[rows], o_hbm.at[0, rows], sem_out.at[i % 5])]

    def start(cs):
        for c in cs:
            c.start()

    def wait(cs):
        for c in cs:
            c.wait()

    def block(fn, name):
        def body(it):
            fn()
            return it + 1

        if _ONLY is None or name in _ONLY:
            jax.lax.while_loop(lambda it: it < 1, body, jnp.int32(0))

    def ln_x(t, s, tie=None):
        rows = pl.ds(t * TM + s * 16, 16)
        y = _ln(x_v[rows, :].astype(F32), EPS, tie)
        xn_v[rows, :] = y.astype(BF16)
        return y

    def ln_x2(t, s, tie):
        p, q = s // 4, s % 4
        y1 = ln_x(t, 8 * p + q, tie)
        y2 = ln_x(t, 8 * p + 4 + q, tie)
        a11, a12, a21, a22 = y1[:, :KH], y1[:, KH:2 * KH], y2[:, :KH], y2[:, KH:2 * KH]
        r0 = (t % 2) * 5 * P + p * MC + q * 16
        for j, c in enumerate((a11 + a22, a21 + a22, a11 + a12, a21 - a11, a12 - a22)):
            XL_v[pl.ds(r0 + j * P, 16), :] = c.astype(BF16)

    def wcomb_gen(cols):
        for j in cols:
            c1 = slice(j * L, (j + 1) * L)
            c2 = slice(FH + j * L, FH + (j + 1) * L)
            for r in range(KH // 32):
                top = pl.ds(r * 32, 32)
                bot = pl.ds(KH + r * 32, 32)
                b11, b12 = win_v[top, c1].astype(F32), win_v[top, c2].astype(F32)
                b21, b22 = win_v[bot, c1].astype(F32), win_v[bot, c2].astype(F32)
                for w, c in enumerate((b11 + b22, b12 - b22, b21 - b11, b11 + b12, b21 + b22)):
                    WB_v[pl.ds(w * KH + r * 32, 32), c1] = c.astype(BF16)
                yield A_COST

    def ln_z2(t, s, tie=None):
        y = _ln(zg_v[t % 2, s * 16:(s + 1) * 16, :], 4.0 * EPS, tie, 0.25)
        lo, hi = y[:, :HN], y[:, HN:]
        r = (t * TM + s * 16) % HK
        rows = pl.ds(r, 16)
        if t < NT // 2:
            zf_v[rows, :] = y
            R_v[pl.ds(1 * HK + r, 16), :] = lo.astype(BF16)
            R_v[pl.ds(5 * HK + r, 16), :] = (lo + hi).astype(BF16)
        else:
            b11 = zf_v[rows, :HN]
            R_v[pl.ds(0 * HK + r, 16), :] = (b11 + hi).astype(BF16)
            R_v[pl.ds(2 * HK + r, 16), :] = (zf_v[rows, HN:] - hi).astype(BF16)
            R_v[pl.ds(3 * HK + r, 16), :] = (lo - b11).astype(BF16)
            R_v[pl.ds(4 * HK + r, 16), :] = hi.astype(BF16)
            R_v[pl.ds(6 * HK + r, 16), :] = (lo + hi).astype(BF16)

    def acomb_gen(i, groups=range(P // 16)):
        for r in groups:
            for c in range(HK // 256):
                top = pl.ds(i * TM + r * 16, 16)
                bot = pl.ds(i * TM + P + r * 16, 16)
                c1 = slice(c * 256, (c + 1) * 256)
                c2 = slice(HK + c * 256, HK + (c + 1) * 256)
                a11 = wsp_v[top, c1].astype(F32)
                a12 = wsp_v[top, c2].astype(F32)
                a21 = wsp_v[bot, c1].astype(F32)
                a22 = wsp_v[bot, c2].astype(F32)
                r0 = (i % 4) * 5 * P + r * 16
                Lc_v[pl.ds(r0 + 0 * P, 16), c1] = (a11 + a22).astype(BF16)
                Lc_v[pl.ds(r0 + 1 * P, 16), c1] = (a21 + a22).astype(BF16)
                Lc_v[pl.ds(r0 + 2 * P, 16), c1] = (a11 + a12).astype(BF16)
                Lc_v[pl.ds(r0 + 3 * P, 16), c1] = (a21 - a11).astype(BF16)
                Lc_v[pl.ds(r0 + 4 * P, 16), c1] = (a12 - a22).astype(BF16)
                yield A_COST

    def tasks(fn, t, n=TM // 16):
        return [lambda tie, s=s: fn(t, s, tie) for s in range(n)]

    def kv_gen(t):
        for m in range(TM // KV_ROWS):
            r = t * TM + m * KV_ROWS
            for l in range(D // L):
                lanes = slice(l * L, (l + 1) * L)
                kf = k_v[pl.ds(r, KV_ROWS), lanes].astype(F32)
                kf_v[l, pl.ds(r + 8, KV_ROWS), :] = kf
                ks = kf * sk_v[0, 0:1, lanes]
                for tap in range(1, 4):
                    ks = ks + kf_v[l, pl.ds(r + 8 - tap, KV_ROWS), :] * sk_v[tap, 0:1, lanes]
                kv = ks * v_v[pl.ds(r, KV_ROWS), lanes].astype(F32)
                kv_v[pl.ds(r, KV_ROWS), lanes] = kv.astype(BF16)
                yield KV_COST * KV_ROWS / 64

    def g_gen(t):
        for r in range(P // 16):
            rows = pl.ds(r * 16, 16)
            for l in range(D // L):
                lanes = slice(l * L, (l + 1) * L)
                h = [(H_v[(2 * t + w) % 6, 0, rows, lanes], H_v[(2 * t + w) % 6, 1, rows, lanes]) for w in range(3)]
                for w in range(2):
                    (pr, pi), (cr, ci) = h[w], h[w + 1]
                    G_v[2 * t + w, 0, rows, lanes] = cr - pi if r < P // 32 else cr + pi
                    G_v[2 * t + w, 1, rows, lanes] = ci + pr if r < P // 32 else ci - pr
                yield G_COST

    def freq_gen(a):
        def cmac(acc, x, g):
            pr = x[0] * g[0] - x[1] * g[1]
            pi = x[0] * g[1] + x[1] * g[0]
            return (pr, pi) if acc is None else (acc[0] + pr, acc[1] + pi)

        for r in range(P // 16):
            for l in range(D // L):
                lanes = slice(l * L, (l + 1) * L)
                res = []
                for sub in range(16 // FR):
                    rows = pl.ds(r * 16 + sub * FR, FR)
                    lo = hi = None
                    g = (G_v[a + 1, 0, rows, lanes], G_v[a + 1, 1, rows, lanes])
                    for c in range(a + 2):
                        x = (X_v[c, 0, rows, lanes], X_v[c, 1, rows, lanes])
                        hi = cmac(hi, x, g)
                        if c <= a:
                            g = (G_v[a - c, 0, rows, lanes], G_v[a - c, 1, rows, lanes])
                            lo = cmac(lo, x, g)
                            yield 2 * FR
                    res.append((lo, hi))
                for w in range(2):
                    for part in range(2):
                        Z_v[pl.ds((a + w) * 2 * P + part * P + r * 16, 16), lanes] = jnp.concatenate(
                            [z[w][part] for z in res], axis=0).astype(BF16)
                yield 20

    def dft_job(rhs, dst, bg, budget):
        for j in range(2):
            for half in range(2):
                for l0, l1 in DFT_SPLIT:
                    lanes = slice(l0 * L, l1 * L)
                    r = rhs(F_v[half * P:(half + 1) * P, 0:P], j, lanes).reshape(8, 2, 8, (l1 - l0) * L)
                    for part in range(2):
                        dst(j, part, pl.ds(half * 64, 64), lanes, r[:, part].reshape(64, (l1 - l0) * L))
                    bg.run(budget * (l1 - l0) / 2)

    def job_h(t, bg, budget):
        def dst(j, part, rows, lanes, val):
            H_v[(2 * t + j + 1) % 6, part, rows, lanes] = val
        dft_job(lambda f, j, lanes: jax.lax.dot_general(f, h_v[t, lanes, j * P:(j + 1) * P], NT_DIMS,
                                                        preferred_element_type=F32), dst, bg, budget)

    def job_x(t, bg, budget):
        def dst(j, part, rows, lanes, val):
            X_v[2 * t + j, part, rows, lanes] = val
        dft_job(lambda f, j, lanes: _dot(f, kv_v[(2 * t + j) * P:(2 * t + j + 1) * P, lanes]), dst, bg, budget)

    def z_out(t, m, n, pre, bg, budget, tied):
        z = _gelu2(pre)
        if n < FH // L:
            z1_v[pl.ds(t * TM + m * MC, MC), n * L:(n + 1) * L] = z
        else:
            zg_v[t % 2, m * MC:(m + 1) * MC, n * L - FH:(n + 1) * L - FH] = z
        ntask = tied.run(z)
        bg.run(budget[1] if ntask else budget[0])

    def job_z(t, m, cols, bg, budget, tied):
        for n in cols:
            z_out(t, m, n, _dot(xn_v[pl.ds(t * TM + m * MC, MC), :], win_v[:, n * L:(n + 1) * L]), bg, budget, tied)

    def job_zs(t, p, j, bg, budget, tied):
        r1 = pl.ds(t * TM + p * P, MC)
        r2 = pl.ds(t * TM + p * P + MC, MC)
        c1 = slice(j * L, (j + 1) * L)
        c2 = slice(FH + j * L, FH + (j + 1) * L)

        def xl(w):
            r0 = (t % 2) * 5 * P + w * P + p * MC
            return XL_v[r0:r0 + MC, :]

        def wb(w):
            return WB_v[w * KH:(w + 1) * KH, c1]

        def rem(rows, cols):
            return _dot(xn_v[rows, 2 * KH:], win_v[2 * KH:, cols])

        m2 = _dot(xl(1), win_v[0:KH, c1])
        m4 = _dot(xn_v[r2, KH:2 * KH], wb(2))
        z_out(t, 2 * p + 1, j, m2 + m4 + rem(r2, c1), bg, budget, tied)
        m3 = _dot(xn_v[r1, 0:KH], wb(1))
        m5 = _dot(xl(2), win_v[KH:2 * KH, c2])
        z_out(t, 2 * p, 6 + j, m3 + m5 + rem(r1, c2), bg, budget, tied)
        m1 = _dot(xl(0), wb(0))
        z_out(t, 2 * p, j, (m4 - m5) + m1 + _dot(xl(4), wb(4)) + rem(r1, c1), bg, budget, tied)
        z_out(t, 2 * p + 1, 6 + j, (m3 - m2) + m1 + _dot(xl(3), wb(3)) + rem(r2, c2), bg, budget, tied)

    rev8 = 7 - jax.lax.broadcasted_iota(jnp.int32, (8, L), 0)

    def finish(a, upper, n, hh, slot):
        rows = pl.ds(a * P + (MC if upper else 0), MC)
        lanes = slice(n * L, (n + 1) * L)
        if upper:
            ya = _dot(Fi_v[:, 0:P], Z_v[a * 2 * P:a * 2 * P + P, lanes])
            yb = _dot(Fi_v[:, P:2 * P], Z_v[a * 2 * P + P:(a + 1) * 2 * P, lanes])
            slot(0.5)
            y = ya - yb
            lo = ya + yb
            for j in range(MC // 8):
                yl_v[a % 2, n, (7 - j) * 8:(8 - j) * 8, :] = jnp.take_along_axis(lo[j * 8:(j + 1) * 8], rev8, axis=0)
        else:
            y = yl_v[a % 2, n]
        gate = hh + hh * jnp.tanh(hh)
        s = xn_v[rows, lanes].astype(F32) * y
        o_v[rows, lanes] = (x_v[rows, lanes].astype(F32) + s * gate).astype(BF16)

    def tail_gen(i, bg, budget):
        a0, a1 = _blocks_of_step(i)

        def slot(w):
            bg.run(w * budget[0])

        def dot3(a, b):
            r = _dot(a, b)
            slot(0.75)
            return r

        for upper in (True, False):
            sub = MC if upper else 0
            r1 = pl.ds(a0 * P + sub, MC)
            r2 = pl.ds(a1 * P + sub, MC)

            def ul(w):
                r0 = ((i % 4) * 5 + w) * P + sub
                return UL_v[r0:r0 + MC, :]

            for j in range(2):
                c1 = slice(j * L, (j + 1) * L)
                c2 = slice((2 + j) * L, (3 + j) * L)

                def wo(w):
                    return WO_v[w * HN:(w + 1) * HN, c1]

                m2 = dot3(ul(1), wout_v[0:HN, c1])
                m4 = dot3(u_v[r2, HN:], wo(2))
                finish(a1, upper, j, m2 + m4, slot)
                bg.charge(T_COST)
                yield
                m3 = dot3(u_v[r1, 0:HN], wo(1))
                m5 = dot3(ul(2), wout_v[HN:, c2])
                finish(a0, upper, 2 + j, m3 + m5, slot)
                bg.charge(T_COST)
                yield
                m1 = dot3(ul(0), wo(0))
                finish(a0, upper, j, (m4 - m5) + m1 + dot3(ul(4), wo(4)), slot)
                bg.charge(T_COST)
                yield
                finish(a1, upper, 2 + j, (m3 - m2) + m1 + dot3(ul(3), wo(3)), slot)
                bg.charge(T_COST)
                yield
            finish(a0, upper, 4, dot3(u_v[r1, 0:HN], wout_v[0:HN, 4 * L:]) + dot3(u_v[r1, HN:], wout_v[HN:, 4 * L:]), slot)
            bg.charge(T_COST)
            yield
            finish(a1, upper, 4, dot3(u_v[r2, 0:HN], wout_v[0:HN, 4 * L:]) + dot3(u_v[r2, HN:], wout_v[HN:, 4 * L:]), slot)
            bg.charge(T_COST)
            yield

    def wocomb_gen():
        for j in range(2):
            c1 = slice(j * L, (j + 1) * L)
            c2 = slice((2 + j) * L, (3 + j) * L)
            for r in range(HN // 32):
                top = pl.ds(r * 32, 32)
                bot = pl.ds(HN + r * 32, 32)
                b11, b12 = wout_v[top, c1].astype(F32), wout_v[top, c2].astype(F32)
                b21, b22 = wout_v[bot, c1].astype(F32), wout_v[bot, c2].astype(F32)
                for w, c in enumerate((b11 + b22, b12 - b22, b21 - b11, b11 + b12, b21 + b22)):
                    WO_v[pl.ds(w * HN + r * 32, 32), c1] = c.astype(BF16)
                yield A_COST

    def job_big(i, bg, pending, budget, every):
        a0, a1 = _blocks_of_step(i)
        KG = BIG_KG

        def lhs(j, sub, cols):
            if j == 2:
                return wsp_v[i * TM + sub:i * TM + sub + MC, cols]
            if j == 3:
                return wsp_v[i * TM + P + sub:i * TM + P + sub + MC, HK + cols.start:HK + cols.stop]
            r0 = ((i % 4) * 5 + {0: 0, 1: 1, 4: 2, 5: 3, 6: 4}[j]) * P + sub
            return Lc_v[r0:r0 + MC, cols]

        def prod(j, sub, n, acc=None):
            for kg in range(HK // KG):
                ks = slice(kg * KG, (kg + 1) * KG)
                p = _dot(lhs(j, sub, ks), R_v[j * HK + kg * KG:j * HK + (kg + 1) * KG, n * L:(n + 1) * L])
                acc = p if acc is None else acc + p
                bg.run(budget * KG / 512)
            return acc

        def tails(n):
            for _ in range(n):
                if pending:
                    next(pending.pop(0))

        def emit(a, sub, n, g):
            rows = pl.ds(a * P + sub, MC)
            lanes = slice(n * L, (n + 1) * L)
            u = z1_v[rows, lanes] * (g + bcol_v[rows, :])
            u_v[rows, lanes] = u.astype(BF16)
            bg.charge(E_COST)
            return u

        for sub in (0, MC):
            for n in range(HN // L):
                m2 = prod(1, sub, n)
                m4 = prod(3, sub, n)
                u21 = emit(a1, sub, n, m2 + m4)
                m3 = prod(2, sub, n)
                t22 = m3 - m2
                m5 = prod(4, sub, n)
                u12 = emit(a0, sub, n + HN // L, m3 + m5)
                t11 = m4 - m5
                m1 = prod(0, sub, n)
                u11 = emit(a0, sub, n, prod(6, sub, n, t11 + m1))
                u22 = emit(a1, sub, n + HN // L, prod(5, sub, n, t22 + m1))
                for w, c in enumerate((u11 + u22, u21 + u22, u11 + u12, u21 - u11, u12 - u22)):
                    UL_v[pl.ds(((i % 4) * 5 + w) * P + sub, MC), n * L:(n + 1) * L] = c.astype(BF16)
                bg.charge(U_COST)
                tails(every.pop(0))

    if _ONLY is not None:
        for r_ in (xn_u, XL_u, WB_u, UL_u, WO_u, z1_v, R_u, Lc_u, zf_v, zg_v, kv_u, u_u, X_v, H_v, G_v, Z_u, kf_v):
            c_ = pltpu.make_async_copy(r_, r_, sem_small.at[0])
            c_.start()
            c_.wait()

    cp_x(0).start()
    cp_x(1).start()
    for c in range(5):
        cp_win(c).start()
    cp_x(2).start()
    start(cp_small())

    kk = _odd_freq(jax.lax.broadcasted_iota(jnp.int32, (P, P), 0))
    nn = jax.lax.broadcasted_iota(jnp.int32, (P, P), 1)
    fc, fs = _cos_sin((kk * (4 * nn - 127)) & 2047)
    for g in range(P // 8):
        F_v[g * 16:(g + 1) * 16, 0:P] = jnp.concatenate(
            [fc[g * 8:(g + 1) * 8], -fs[g * 8:(g + 1) * 8]], axis=0).astype(BF16)
    fc, fs = _cos_sin((kk * (-127)) & 2047)
    ph_v[0] = fc
    ph_v[1] = fs
    kk = _odd_freq(jax.lax.broadcasted_iota(jnp.int32, (MC, P), 1))
    mm = jax.lax.broadcasted_iota(jnp.int32, (MC, P), 0)
    ic, is_ = _cos_sin((kk * (4 * mm + 2)) & 2047)
    Fi_v[:, 0:P] = (ic * (1.0 / P)).astype(BF16)
    Fi_v[:, P:2 * P] = (is_ * (1.0 / P)).astype(BF16)
    kf_v[:, 0:8, :] = jnp.zeros((D // L, 8, L), F32)

    for t in range(2):
        cp_x(t).wait()
        for s in range(TM // 16):
            ln_x(t, s)

    def small_setup():
        sk = sk_in[...].astype(F32)
        for t in range(4):
            sk_v[t] = jnp.broadcast_to(sk[t:t + 1], (8, D))
        drow = d_in[...].astype(F32).reshape(1, D)
        for l in range(D // L):
            lanes = slice(l * L, (l + 1) * L)
            dre = ph_v[0] * drow[:, lanes]
            dim = ph_v[1] * drow[:, lanes]
            H_v[0, 0, 0:64, lanes] = -dim[0:64]
            H_v[0, 0, 64:P, lanes] = dim[64:P]
            H_v[0, 1, 0:64, lanes] = -dre[0:64]
            H_v[0, 1, 64:P, lanes] = dre[64:P]

    def bcol_task(t, j, tie):
        brow = b_in[...].astype(F32).reshape(1, S)[:, j * P:(j + 1) * P] * 0.25 + tie[0:1]
        bcol_v[j * P:(j + 1) * P, :] = jnp.broadcast_to(brow, (P, P)).T

    LAG = 2

    def interleave(*lists):
        out = []
        for j in range(max(len(a) for a in lists)):
            for a in lists:
                out += a[j:j + 1]
        return out

    def p1_first(c):
        bg = _Background()
        todo = []
        if c == 3:
            todo = tasks(ln_z2, 0)
            bg.add(wcomb_gen(range(3)))
        if c == 4:
            todo = tasks(ln_x2, 2, 8)
            bg.add(wcomb_gen(range(3, 6)))
            small_setup()
        tied = _Tied(todo, 20)
        for t in range(2):
            for m in range(TM // MC):
                job_z(t, m, range(*WIN_CHUNKS[c]), bg, (80, 40), tied)
        bg.drain()
        assert not tied.tasks

    for c in range(5):
        cp_win(c).wait()
        if c == 2:
            start(cp_conv(0))
            cp_x(3).start()
        if c == 4:
            cp_x(2).wait()
            wait(cp_small())
        block(lambda c=c: p1_first(c), f'p1_f{c}')

    def p1_wait(i):
        wait(cp_conv(i - LAG))
        if i + 1 < NT:
            cp_x(i + 1).wait()
        if i == 4:
            cp_wout().wait()
        if i == NT - 3:
            wait(cp_wsp(0))

    def p1_start(i):
        if i + 2 < NT:
            cp_x(i + 2).start()
        start(cp_conv(i - LAG + 1))
        if i == NT - 1:
            start(cp_conv(NT - 1))
        start(cp_wsp((i - 2) // 2, ((i - 2) % 2,)))
        if i == 2:
            cp_wout().start()

    def take(gen, n):
        for _ in range(n):
            yield next(gen)

    def p1_step(i):
        bg = _Background()
        dft = _Background()
        t = i - LAG
        kv = kv_gen(t)
        dft.add(take(kv, (20 if t >= 1 else 10) * 64 // KV_ROWS))
        if t >= 1:
            bg.add(g_gen(t - 1))
        else:
            bg.add(take(kv, 10 * 64 // KV_ROWS))
        extra = 0
        if i == 4:
            bg.add(wocomb_gen())
            extra = 30
        if i in (NT - 3, NT - 2):
            bg.add(acomb_gen(0, range(4) if i == NT - 3 else range(4, 8)))
            extra = 20
        last = i == NT - 1
        z2t = tasks(ln_z2, i - 1)
        todo = interleave(tasks(ln_x2, i + 1, 8) if not last else [], z2t[0::2], z2t[1::2],
                          tasks(bcol_task, 0) if i == 2 else [])
        tied = _Tied(todo, 24 if last else TIED_N)
        if t >= 1:
            dft.run(110)
            job_x(t - 1, dft, 100)
        if H_FIRST and not last:
            job_h(t, dft, 110)
        for p in range(2):
            for j in range(FH // L):
                job_zs(i, p, j, bg, (60 + extra, 10 + extra), tied)
            if p == 0 and last:
                tied = _Tied(tasks(ln_z2, i, 8), 22)
        assert not tied.tasks
        if last:
            for s in range(8, 16):
                ln_z2(i, s)
        if last or not H_FIRST:
            job_h(t, dft, 110)
        bg.drain()
        dft.drain()

    for i in range(2, NT):
        p1_wait(i)
        p1_start(i)
        block(lambda i=i: p1_step(i), f'p1_{i}')

    groups = P2_GROUPS
    NG = len(groups)

    def p2_dma(gi):
        if gi >= 2:
            for i in groups[gi - 2]:
                start(cp_out(i))
        if gi >= 3:
            for i in groups[gi - 3]:
                wait(cp_out(i))
        if gi + 2 < NG:
            for i in groups[gi + 2]:
                start(cp_wsp(i))
        if gi < 2:
            wait(cp_conv(NT - 2 + gi))
        if gi + 1 < NG:
            for i in groups[gi + 1]:
                wait(cp_wsp(i))

    def tails_of(i, bg, budget):
        return [tail_gen(i, bg, budget)] * 20

    def p2_block(gi):
        bg = _Background()
        steps = groups[gi]
        tb = [0.0]
        pending = [t_ for i in (groups[gi - 1] if gi > 0 else []) for t_ in tails_of(i, bg, tb)]
        total = sum(a + 1 for i in steps for a in _blocks_of_step(i)) * 40 * 16
        total += len(steps) * (24 * E_COST + 6 * U_COST) + len(pending) * T_COST
        slots = 84 * len(steps) + TAIL_W * len(pending)
        bg.add(freq_gen(_blocks_of_step(steps[0])[0]))
        if gi < 2:
            bg.add(kv_gen(NT - 2 + gi))
            total += 20 * KV_COST
            slots += 10
        if gi < 3:
            slots += 10
            bg.add(g_gen(NT - 3 + gi))
            total += 40 * G_COST
        if gi + 1 < NG:
            for i in groups[gi + 1]:
                bg.add(acomb_gen(i))
                total += 32 * A_COST
        for i in steps[1:]:
            bg.add(freq_gen(_blocks_of_step(i)[0]))
        budget = tb[0] = total / (slots + 1.0)
        bg.run(budget)
        if gi < 3:
            job_x(NT - 3 + gi, bg, budget)
        if gi < 2:
            job_h(NT - 2 + gi, bg, budget)
        units = [4, 4, 2, 4, 4, 2] * (len(pending) // 20)
        every = [0] * (6 * len(steps))
        for j, n in enumerate(units):
            every[min(len(every) - 1, j * len(every) // len(units))] += n
        for i in steps:
            job_big(i, bg, pending, budget, every)
        for t_ in pending:
            next(t_)
        bg.drain()

    for gi in range(NG):
        p2_dma(gi)
        block(lambda gi=gi: p2_block(gi), f'p2_{gi}')

    def cp_last(upper):
        a0 = _blocks_of_step(NT - 1)[0]
        return [pltpu.make_async_copy(o_v.at[pl.ds(r, MC)], o_hbm.at[0, pl.ds(r, MC)], sem_out.at[(NT - 1) % 5])
                for r in ((a0 + w) * P + (MC if upper else 0) for w in range(2))]

    def p2_last():
        for j, t_ in enumerate(tails_of(NT - 1, _Background(), [0.0])):
            next(t_)
            if j == 9:
                start(cp_last(True))

    p2_dma(NG)
    block(p2_last, 'p2_last')
    start(cp_last(False))
    for i in groups[NG - 2]:
        wait(cp_out(i))
    wait(cp_last(True))
    wait(cp_last(False))
    if _ONLY is not None:
        for r_ in (xn_u, XL_u, WB_u, UL_u, WO_u, z1_v, R_u, Lc_u, zf_v, zg_v, kv_u, u_u, X_v, H_v, G_v, Z_u, kf_v):
            c_ = pltpu.make_async_copy(r_, r_, sem_small.at[0])
            c_.start()
            c_.wait()


@jax.jit
def pallas_recurrent_scan__ssm_conv_h3__mixer_gmlp__prompt_kernel(
    A_q: jax.Array,
    A_k: jax.Array,
    A_v: jax.Array,
    A_shift_k: jax.Array,
    A_ssm_k: jax.Array,
    A_ssm_D: jax.Array,
    B_x: jax.Array,
    B_w_in: jax.Array,
    B_w_sp: jax.Array,
    B_b_sp: jax.Array,
    B_w_out: jax.Array,
):
    del B_x
    hbm = pl.BlockSpec(memory_space=pl.ANY)

    def bf16_buf(*shape):
        return pltpu.VMEM(shape[:-2] + (shape[-2] // 2, shape[-1]), U32)

    return pl.pallas_call(
        _kernel,
        out_shape=jax.ShapeDtypeStruct((1, S, D), BF16),
        in_specs=[hbm] * 10,
        out_specs=hbm,
        scratch_shapes=[
            bf16_buf(S, D),
            bf16_buf(S, D),
            bf16_buf(S, D),
            bf16_buf(NT, D, TM),
            bf16_buf(D, 2 * FH),
            bf16_buf(S, S),
            bf16_buf(FH, D),
            pltpu.VMEM((S, D), BF16),
            pltpu.VMEM((4, D), BF16),
            pltpu.VMEM((D,), BF16),
            pltpu.VMEM((S,), BF16),
            bf16_buf(S, D),
            bf16_buf(2 * 5 * P, KH),
            bf16_buf(5 * KH, FH),
            bf16_buf(4 * 5 * P, HN),
            bf16_buf(5 * HN, 2 * L),
            pltpu.VMEM((S, FH), F32),
            bf16_buf(7 * HK, HN),
            bf16_buf(4 * 5 * P, HK),
            pltpu.VMEM((HK, FH), F32),
            pltpu.VMEM((2, TM, FH), F32),
            bf16_buf(S, D),
            bf16_buf(S, FH),
            pltpu.VMEM((NB, 2, P, D), F32),
            pltpu.VMEM((6, 2, P, D), F32),
            pltpu.VMEM((NB, 2, P, D), F32),
            bf16_buf(NB * 2 * P, D),
            pltpu.VMEM((2, D // L, MC, L), F32),
            bf16_buf(2 * P, 2 * P),
            bf16_buf(MC, 2 * P),
            pltpu.VMEM((S, L), F32),
            pltpu.VMEM((2, P, L), F32),
            pltpu.VMEM((4, 8, D), F32),
            pltpu.VMEM((D // L, S + 8, L), F32),
            pltpu.SemaphoreType.DMA((1,)),
            pltpu.SemaphoreType.DMA((3,)),
            pltpu.SemaphoreType.DMA((2,)),
            pltpu.SemaphoreType.DMA((5,)),
            pltpu.SemaphoreType.DMA((5,)),
            pltpu.SemaphoreType.DMA((5,)),
        ],
        compiler_params=pltpu.CompilerParams(vmem_limit_bytes=116 * 1024 * 1024, disable_semaphore_checks=True),
    )(A_q, A_k, A_v, A_shift_k.T, A_ssm_k, A_ssm_D, B_w_in, B_w_sp, B_b_sp, B_w_out)
```

```python
import math

import jax
import jax.numpy as jnp
import jax.experimental.pallas as pl
import jax.experimental.pallas.tpu as pltpu

S = 2048
D = 640
FH = 768
P = 128
NB = S // P
TM = 256
NT = S // TM
MC = 64
L = 128
HK = S // 2
KH = 256
HN = FH // 2
P2_GROUPS = ((0,), (1, 2), (3, 4), (5, 6), (7,))
STEP_BLOCKS = ((6, 7), (8, 9), (4, 5), (12, 13), (2, 3), (14, 15), (0, 1), (10, 11))
KV_COST, G_COST, A_COST = 110, 36, 56
E_COST, U_COST, T_COST, TAIL_W = 24, 90, 90, 1.6
BIG_KG = 512
TIE_X = False
DFT_B = (130, 80)
Z_B0, Z_B1 = 60, 10
TIED_N = 42
ORDER = 1
FR = 16
KV_ROWS = 64
WIN_CHUNKS = ((6, 7), (7, 9), (9, 12), (0, 3), (3, 6))
EPS = 1e-5
F32 = jnp.float32
BF16 = jnp.bfloat16
U32 = jnp.uint32
GELU_C = math.sqrt(2.0 / math.pi)
NT_DIMS = (((1,), (1,)), ((), ()))
_ONLY = None


def _dot(a, b):
    return jnp.dot(a, b, preferred_element_type=F32)


def _cos_sin(m):
    q = (m + 256) >> 9
    x = (m - (q << 9)).astype(F32) * (2.0 * math.pi / 2048.0)
    x2 = x * x
    s = x * (1.0 + x2 * (-1.0 / 6 + x2 * (1.0 / 120 + x2 * (-1.0 / 5040 + x2 * (1.0 / 362880)))))
    c = 1.0 + x2 * (-0.5 + x2 * (1.0 / 24 + x2 * (-1.0 / 720 + x2 * (1.0 / 40320 - x2 * (1.0 / 3628800)))))
    swap = (q & 1) == 1
    c0 = jnp.where(swap, s, c)
    s0 = jnp.where(swap, c, s)
    cos = jnp.where(((q + 1) & 2) == 2, -c0, c0)
    sin = jnp.where((q & 2) == 2, -s0, s0)
    return cos, sin


def _odd_freq(r):
    return jnp.where(r < 64, 4 * r + 1, 4 * r - 253)


def _gelu2(z):
    u = z * (GELU_C + (GELU_C * 0.044715) * (z * z))
    return z + z * jnp.tanh(u)


def _signzero(z):
    bits = jax.lax.bitcast_convert_type(z, U32) & jnp.uint32(0x80000000)
    return jax.lax.bitcast_convert_type(bits, F32)


def _ln(x, eps, tie=None, scale=None):
    n = x.shape[-1]
    cols = [x[:, j * L:(j + 1) * L] for j in range(n // L)]
    s1 = cols[0]
    s2 = cols[0] * cols[0]
    for c in cols[1:]:
        s1 = s1 + c
        s2 = s2 + c * c
    if tie is not None:
        s1 = s1 + tie
        s2 = s2 + tie
    m = jnp.sum(s1, axis=-1, keepdims=True) * (1.0 / n)
    v = jnp.maximum(jnp.sum(s2, axis=-1, keepdims=True) * (1.0 / n) - m * m, 0.0)
    rs = jax.lax.rsqrt(v + eps)
    if scale is not None:
        rs = rs * scale
    return (x - m) * rs


def _blocks_of_step(i):
    return STEP_BLOCKS[i]


class _Background:
    def __init__(self):
        self.q = []
        self.credit = 0.0

    def add(self, gen):
        self.q.append(gen)

    def run(self, budget):
        self.credit += budget
        while self.q and self.credit > 0:
            try:
                self.credit -= next(self.q[0])
            except StopIteration:
                self.q.pop(0)
        if not self.q:
            self.credit = 0.0

    def charge(self, cost):
        self.credit -= cost

    def drain(self):
        while self.q:
            self.run(1e9)


class _Tied:
    def __init__(self, tasks, npieces):
        self.tasks = list(tasks)
        self.rate = len(self.tasks) / float(npieces)
        self.credit = 0.999

    def run(self, z):
        self.credit += self.rate
        n = 0
        while self.tasks and self.credit >= 1.0:
            self.tasks.pop(0)(_signzero(z[0:16]))
            self.credit -= 1.0
            n += 1
        return n


def _kernel(q_hbm, k_hbm, v_hbm, sk_hbm, h_hbm, d_hbm, win_hbm, wsp_hbm, b_hbm, wout_hbm,
            o_hbm,
            x_u, k_u, v_u, h_u, win_u, wsp_u, wout_u, o_v, sk_in, d_in, b_in,
            xn_u, XL_u, WB_u, UL_u, WO_u, z1_v, R_u, Lc_u, zf_v, zg_v, kv_u, u_u, X_v, H_v, G_v, Z_u, yl_v, F_u, Fi_u, bcol_v, ph_v, sk_v, kf_v,
            sem_small, sem_x, sem_conv, sem_wsp, sem_w, sem_out):
    x_v, k_v, v_v, h_v, win_v, wsp_v, wout_v, xn_v, XL_v, WB_v, UL_v, WO_v, R_v, Lc_v, kv_v, u_v, Z_v, F_v, Fi_v = [
        r.bitcast(BF16) for r in (x_u, k_u, v_u, h_u, win_u, wsp_u, wout_u, xn_u, XL_u, WB_u, UL_u, WO_u, R_u, Lc_u, kv_u, u_u, Z_u, F_u,
                                  Fi_u)]

    def cp_small():
        return [pltpu.make_async_copy(s_, d_, sem_small.at[0])
                for s_, d_ in ((d_hbm, d_in), (sk_hbm, sk_in), (b_hbm, b_in))]

    def cp_x(t):
        return pltpu.make_async_copy(q_hbm.at[0, pl.ds(t * TM, TM)], x_v.at[pl.ds(t * TM, TM)], sem_x.at[t % 3])

    def cp_conv(t):
        rows = pl.ds(t * TM, TM)
        sem = sem_conv.at[t % 2]
        return [pltpu.make_async_copy(h_hbm.at[:, rows], h_v.at[t], sem),
                pltpu.make_async_copy(k_hbm.at[0, rows], k_v.at[rows], sem),
                pltpu.make_async_copy(v_hbm.at[0, rows], v_v.at[rows], sem)]

    def cp_wsp(i, which=(0, 1)):
        return [pltpu.make_async_copy(wsp_hbm.at[pl.ds(_blocks_of_step(i)[half] * P, P)],
                                      wsp_v.at[pl.ds(i * TM + half * P, P)], sem_wsp.at[i % 5]) for half in which]

    def cp_win(c):
        lo, hi = WIN_CHUNKS[c]
        cols = pl.ds(lo * L, (hi - lo) * L)
        return pltpu.make_async_copy(win_hbm.at[:, cols], win_v.at[:, cols], sem_w.at[c])

    def cp_wout():
        return pltpu.make_async_copy(wout_hbm, wout_v, sem_w.at[0])

    def cp_out(i):
        rows = pl.ds(_blocks_of_step(i)[0] * P, TM)
        return [pltpu.make_async_copy(o_v.at[rows], o_hbm.at[0, rows], sem_out.at[i % 5])]

    def start(cs):
        for c in cs:
            c.start()

    def wait(cs):
        for c in cs:
            c.wait()

    def block(fn, name):
        def body(it):
            fn()
            return it + 1

        if _ONLY is None or name in _ONLY:
            jax.lax.while_loop(lambda it: it < 1, body, jnp.int32(0))

    def ln_x(t, s, tie=None):
        rows = pl.ds(t * TM + s * 16, 16)
        y = _ln(x_v[rows, :].astype(F32), EPS, tie)
        xn_v[rows, :] = y.astype(BF16)
        return y

    def ln_x2(t, s, tie):
        p, q = s // 4, s % 4
        y1 = ln_x(t, 8 * p + q, tie)
        y2 = ln_x(t, 8 * p + 4 + q, tie)
        a11, a12, a21, a22 = y1[:, :KH], y1[:, KH:2 * KH], y2[:, :KH], y2[:, KH:2 * KH]
        r0 = (t % 2) * 5 * P + p * MC + q * 16
        for j, c in enumerate((a11 + a22, a21 + a22, a11 + a12, a21 - a11, a12 - a22)):
            XL_v[pl.ds(r0 + j * P, 16), :] = c.astype(BF16)

    def wcomb_gen(cols):
        for j in cols:
            c1 = slice(j * L, (j + 1) * L)
            c2 = slice(FH + j * L, FH + (j + 1) * L)
            for r in range(KH // 32):
                top = pl.ds(r * 32, 32)
                bot = pl.ds(KH + r * 32, 32)
                b11, b12 = win_v[top, c1].astype(F32), win_v[top, c2].astype(F32)
                b21, b22 = win_v[bot, c1].astype(F32), win_v[bot, c2].astype(F32)
                for w, c in enumerate((b11 + b22, b12 - b22, b21 - b11, b11 + b12, b21 + b22)):
                    WB_v[pl.ds(w * KH + r * 32, 32), c1] = c.astype(BF16)
                yield A_COST

    def ln_z2(t, s, tie=None):
        y = _ln(zg_v[t % 2, s * 16:(s + 1) * 16, :], 4.0 * EPS, tie, 0.25)
        lo, hi = y[:, :HN], y[:, HN:]
        r = (t * TM + s * 16) % HK
        rows = pl.ds(r, 16)
        if t < NT // 2:
            zf_v[rows, :] = y
            R_v[pl.ds(1 * HK + r, 16), :] = lo.astype(BF16)
            R_v[pl.ds(5 * HK + r, 16), :] = (lo + hi).astype(BF16)
        else:
            b11 = zf_v[rows, :HN]
            R_v[pl.ds(0 * HK + r, 16), :] = (b11 + hi).astype(BF16)
            R_v[pl.ds(2 * HK + r, 16), :] = (zf_v[rows, HN:] - hi).astype(BF16)
            R_v[pl.ds(3 * HK + r, 16), :] = (lo - b11).astype(BF16)
            R_v[pl.ds(4 * HK + r, 16), :] = hi.astype(BF16)
            R_v[pl.ds(6 * HK + r, 16), :] = (lo + hi).astype(BF16)

    def acomb_gen(i, groups=range(P // 16)):
        for r in groups:
            for c in range(HK // 256):
                top = pl.ds(i * TM + r * 16, 16)
                bot = pl.ds(i * TM + P + r * 16, 16)
                c1 = slice(c * 256, (c + 1) * 256)
                c2 = slice(HK + c * 256, HK + (c + 1) * 256)
                a11 = wsp_v[top, c1].astype(F32)
                a12 = wsp_v[top, c2].astype(F32)
                a21 = wsp_v[bot, c1].astype(F32)
                a22 = wsp_v[bot, c2].astype(F32)
                r0 = (i % 4) * 5 * P + r * 16
                Lc_v[pl.ds(r0 + 0 * P, 16), c1] = (a11 + a22).astype(BF16)
                Lc_v[pl.ds(r0 + 1 * P, 16), c1] = (a21 + a22).astype(BF16)
                Lc_v[pl.ds(r0 + 2 * P, 16), c1] = (a11 + a12).astype(BF16)
                Lc_v[pl.ds(r0 + 3 * P, 16), c1] = (a21 - a11).astype(BF16)
                Lc_v[pl.ds(r0 + 4 * P, 16), c1] = (a12 - a22).astype(BF16)
                yield A_COST

    def tasks(fn, t, n=TM // 16):
        return [lambda tie, s=s: fn(t, s, tie) for s in range(n)]

    def kv_gen(t):
        for m in range(TM // KV_ROWS):
            r = t * TM + m * KV_ROWS
            for l in range(D // L):
                lanes = slice(l * L, (l + 1) * L)
                kf = k_v[pl.ds(r, KV_ROWS), lanes].astype(F32)
                kf_v[l, pl.ds(r + 8, KV_ROWS), :] = kf
                ks = kf * sk_v[0, 0:1, lanes]
                for tap in range(1, 4):
                    ks = ks + kf_v[l, pl.ds(r + 8 - tap, KV_ROWS), :] * sk_v[tap, 0:1, lanes]
                kv = ks * v_v[pl.ds(r, KV_ROWS), lanes].astype(F32)
                kv_v[pl.ds(r, KV_ROWS), lanes] = kv.astype(BF16)
                yield KV_COST * KV_ROWS / 64

    def g_gen(t):
        for r in range(P // 16):
            rows = pl.ds(r * 16, 16)
            for l in range(D // L):
                lanes = slice(l * L, (l + 1) * L)
                h = [(H_v[(2 * t + w) % 6, 0, rows, lanes], H_v[(2 * t + w) % 6, 1, rows, lanes]) for w in range(3)]
                for w in range(2):
                    (pr, pi), (cr, ci) = h[w], h[w + 1]
                    G_v[2 * t + w, 0, rows, lanes] = cr - pi if r < P // 32 else cr + pi
                    G_v[2 * t + w, 1, rows, lanes] = ci + pr if r < P // 32 else ci - pr
                yield G_COST

    def freq_gen(a):
        def cmac(acc, x, g):
            pr = x[0] * g[0] - x[1] * g[1]
            pi = x[0] * g[1] + x[1] * g[0]
            return (pr, pi) if acc is None else (acc[0] + pr, acc[1] + pi)

        for r in range(P // 16):
            for l in range(D // L):
                lanes = slice(l * L, (l + 1) * L)
                res = []
                for sub in range(16 // FR):
                    rows = pl.ds(r * 16 + sub * FR, FR)
                    lo = hi = None
                    g = (G_v[a + 1, 0, rows, lanes], G_v[a + 1, 1, rows, lanes])
                    for c in range(a + 2):
                        x = (X_v[c, 0, rows, lanes], X_v[c, 1, rows, lanes])
                        hi = cmac(hi, x, g)
                        if c <= a:
                            g = (G_v[a - c, 0, rows, lanes], G_v[a - c, 1, rows, lanes])
                            lo = cmac(lo, x, g)
                            yield 2 * FR
                    res.append((lo, hi))
                for w in range(2):
                    for part in range(2):
                        Z_v[pl.ds((a + w) * 2 * P + part * P + r * 16, 16), lanes] = jnp.concatenate(
                            [z[w][part] for z in res], axis=0).astype(BF16)
                yield 20

    def dft_piece(kind, t, q, bg, budget, tied=None):
        j, half = q // 2, q % 2
        f = F_v[half * P:(half + 1) * P, 0:P]
        if kind == 'H':
            r = jax.lax.dot_general(f, h_v[t, :, j * P:(j + 1) * P], NT_DIMS, preferred_element_type=F32)
            dst, idx = H_v, (2 * t + j + 1) % 6
        else:
            r = _dot(f, kv_v[(2 * t + j) * P:(2 * t + j + 1) * P, :])
            dst, idx = X_v, 2 * t + j
        r4 = r.reshape(8, 2, 8, D)
        for part in range(2):
            dst[idx, part, half * 64:(half + 1) * 64, :] = r4[:, part].reshape(64, D)
        if tied is not None:
            tied.run(r[:, 0:L])
            tied.run(r[:, 2 * L:3 * L])
        bg.run(budget * 2.5)

    def job_h(t, bg, budget):
        for q in range(4):
            dft_piece('H', t, q, bg, budget)

    def job_x(t, bg, budget):
        for q in range(4):
            dft_piece('X', t, q, bg, budget)

    def z_out(t, m, n, pre, bg, budget, tied):
        z = _gelu2(pre)
        if n < FH // L:
            z1_v[pl.ds(t * TM + m * MC, MC), n * L:(n + 1) * L] = z
        else:
            zg_v[t % 2, m * MC:(m + 1) * MC, n * L - FH:(n + 1) * L - FH] = z
        ntask = tied.run(z)
        bg.run(budget[1] if ntask else budget[0])

    def job_z(t, m, cols, bg, budget, tied):
        for n in cols:
            z_out(t, m, n, _dot(xn_v[pl.ds(t * TM + m * MC, MC), :], win_v[:, n * L:(n + 1) * L]), bg, budget, tied)

    def job_zs(t, p, j, bg, budget, tied):
        r1 = pl.ds(t * TM + p * P, MC)
        r2 = pl.ds(t * TM + p * P + MC, MC)
        c1 = slice(j * L, (j + 1) * L)
        c2 = slice(FH + j * L, FH + (j + 1) * L)

        def xl(w):
            r0 = (t % 2) * 5 * P + w * P + p * MC
            return XL_v[r0:r0 + MC, :]

        def wb(w):
            return WB_v[w * KH:(w + 1) * KH, c1]

        def rem(rows, cols):
            return _dot(xn_v[rows, 2 * KH:], win_v[2 * KH:, cols])

        m2 = _dot(xl(1), win_v[0:KH, c1])
        m4 = _dot(xn_v[r2, KH:2 * KH], wb(2))
        z_out(t, 2 * p + 1, j, m2 + m4 + rem(r2, c1), bg, budget, tied)
        m3 = _dot(xn_v[r1, 0:KH], wb(1))
        m5 = _dot(xl(2), win_v[KH:2 * KH, c2])
        z_out(t, 2 * p, 6 + j, m3 + m5 + rem(r1, c2), bg, budget, tied)
        m1 = _dot(xl(0), wb(0))
        z_out(t, 2 * p, j, (m4 - m5) + m1 + _dot(xl(4), wb(4)) + rem(r1, c1), bg, budget, tied)
        z_out(t, 2 * p + 1, 6 + j, (m3 - m2) + m1 + _dot(xl(3), wb(3)) + rem(r2, c2), bg, budget, tied)

    rev8 = 7 - jax.lax.broadcasted_iota(jnp.int32, (8, L), 0)

    def finish(a, upper, n, hh, slot):
        rows = pl.ds(a * P + (MC if upper else 0), MC)
        lanes = slice(n * L, (n + 1) * L)
        if upper:
            ya = _dot(Fi_v[:, 0:P], Z_v[a * 2 * P:a * 2 * P + P, lanes])
            yb = _dot(Fi_v[:, P:2 * P], Z_v[a * 2 * P + P:(a + 1) * 2 * P, lanes])
            slot(0.5)
            y = ya - yb
            lo = ya + yb
            for j in range(MC // 8):
                yl_v[a % 2, n, (7 - j) * 8:(8 - j) * 8, :] = jnp.take_along_axis(lo[j * 8:(j + 1) * 8], rev8, axis=0)
        else:
            y = yl_v[a % 2, n]
        gate = hh + hh * jnp.tanh(hh)
        s = xn_v[rows, lanes].astype(F32) * y
        o_v[rows, lanes] = (x_v[rows, lanes].astype(F32) + s * gate).astype(BF16)

    def tail_gen(i, bg, budget):
        a0, a1 = _blocks_of_step(i)

        def slot(w):
            bg.run(w * budget[0])

        def dot3(a, b):
            r = _dot(a, b)
            slot(0.75)
            return r

        for upper in (True, False):
            sub = MC if upper else 0
            r1 = pl.ds(a0 * P + sub, MC)
            r2 = pl.ds(a1 * P + sub, MC)

            def ul(w):
                r0 = ((i % 4) * 5 + w) * P + sub
                return UL_v[r0:r0 + MC, :]

            for j in range(2):
                c1 = slice(j * L, (j + 1) * L)
                c2 = slice((2 + j) * L, (3 + j) * L)

                def wo(w):
                    return WO_v[w * HN:(w + 1) * HN, c1]

                m2 = dot3(ul(1), wout_v[0:HN, c1])
                m4 = dot3(u_v[r2, HN:], wo(2))
                finish(a1, upper, j, m2 + m4, slot)
                bg.charge(T_COST)
                yield
                m3 = dot3(u_v[r1, 0:HN], wo(1))
                m5 = dot3(ul(2), wout_v[HN:, c2])
                finish(a0, upper, 2 + j, m3 + m5, slot)
                bg.charge(T_COST)
                yield
                m1 = dot3(ul(0), wo(0))
                finish(a0, upper, j, (m4 - m5) + m1 + dot3(ul(4), wo(4)), slot)
                bg.charge(T_COST)
                yield
                finish(a1, upper, 2 + j, (m3 - m2) + m1 + dot3(ul(3), wo(3)), slot)
                bg.charge(T_COST)
                yield
            finish(a0, upper, 4, dot3(u_v[r1, 0:HN], wout_v[0:HN, 4 * L:]) + dot3(u_v[r1, HN:], wout_v[HN:, 4 * L:]), slot)
            bg.charge(T_COST)
            yield
            finish(a1, upper, 4, dot3(u_v[r2, 0:HN], wout_v[0:HN, 4 * L:]) + dot3(u_v[r2, HN:], wout_v[HN:, 4 * L:]), slot)
            bg.charge(T_COST)
            yield

    def wocomb_gen():
        for j in range(2):
            c1 = slice(j * L, (j + 1) * L)
            c2 = slice((2 + j) * L, (3 + j) * L)
            for r in range(HN // 32):
                top = pl.ds(r * 32, 32)
                bot = pl.ds(HN + r * 32, 32)
                b11, b12 = wout_v[top, c1].astype(F32), wout_v[top, c2].astype(F32)
                b21, b22 = wout_v[bot, c1].astype(F32), wout_v[bot, c2].astype(F32)
                for w, c in enumerate((b11 + b22, b12 - b22, b21 - b11, b11 + b12, b21 + b22)):
                    WO_v[pl.ds(w * HN + r * 32, 32), c1] = c.astype(BF16)
                yield A_COST

    def job_big(i, bg, pending, budget, every):
        a0, a1 = _blocks_of_step(i)
        KG = BIG_KG

        def lhs(j, sub, cols):
            if j == 2:
                return wsp_v[i * TM + sub:i * TM + sub + MC, cols]
            if j == 3:
                return wsp_v[i * TM + P + sub:i * TM + P + sub + MC, HK + cols.start:HK + cols.stop]
            r0 = ((i % 4) * 5 + {0: 0, 1: 1, 4: 2, 5: 3, 6: 4}[j]) * P + sub
            return Lc_v[r0:r0 + MC, cols]

        def prod(j, sub, n, acc=None):
            for kg in range(HK // KG):
                ks = slice(kg * KG, (kg + 1) * KG)
                p = _dot(lhs(j, sub, ks), R_v[j * HK + kg * KG:j * HK + (kg + 1) * KG, n * L:(n + 1) * L])
                acc = p if acc is None else acc + p
                bg.run(budget * KG / 512)
            return acc

        def tails(n):
            for _ in range(n):
                if pending:
                    next(pending.pop(0))

        def emit(a, sub, n, g):
            rows = pl.ds(a * P + sub, MC)
            lanes = slice(n * L, (n + 1) * L)
            u = z1_v[rows, lanes] * (g + bcol_v[rows, :])
            u_v[rows, lanes] = u.astype(BF16)
            bg.charge(E_COST)
            return u

        for sub in (0, MC):
            for n in range(HN // L):
                def put(w, c):
                    UL_v[pl.ds(((i % 4) * 5 + w) * P + sub, MC), n * L:(n + 1) * L] = c.astype(BF16)

                if ORDER == 0:
                    m2 = prod(1, sub, n)
                    m4 = prod(3, sub, n)
                    u21 = emit(a1, sub, n, m2 + m4)
                    m3 = prod(2, sub, n)
                    t22 = m3 - m2
                    m5 = prod(4, sub, n)
                    u12 = emit(a0, sub, n + HN // L, m3 + m5)
                    t11 = m4 - m5
                    m1 = prod(0, sub, n)
                    u11 = emit(a0, sub, n, prod(6, sub, n, t11 + m1))
                    u22 = emit(a1, sub, n + HN // L, prod(5, sub, n, t22 + m1))
                    for w, c in enumerate((u11 + u22, u21 + u22, u11 + u12, u21 - u11, u12 - u22)):
                        put(w, c)
                else:
                    m1 = prod(0, sub, n)
                    t11 = prod(6, sub, n, m1)
                    m4 = prod(3, sub, n)
                    t11 = t11 + m4
                    m5 = prod(4, sub, n)
                    u11 = emit(a0, sub, n, t11 - m5)
                    m2 = prod(1, sub, n)
                    u21 = emit(a1, sub, n, m2 + m4)
                    put(3, u21 - u11)
                    t22 = m1 - m2
                    m3 = prod(2, sub, n)
                    u12 = emit(a0, sub, n + HN // L, m3 + m5)
                    put(2, u11 + u12)
                    u22 = emit(a1, sub, n + HN // L, prod(5, sub, n, t22 + m3))
                    put(0, u11 + u22)
                    put(1, u21 + u22)
                    put(4, u12 - u22)
                bg.charge(U_COST)
                tails(every.pop(0))

    if _ONLY is not None:
        for r_ in (xn_u, XL_u, WB_u, UL_u, WO_u, z1_v, R_u, Lc_u, zf_v, zg_v, kv_u, u_u, X_v, H_v, G_v, Z_u, kf_v):
            c_ = pltpu.make_async_copy(r_, r_, sem_small.at[0])
            c_.start()
            c_.wait()

    cp_x(0).start()
    cp_x(1).start()
    for c in range(5):
        cp_win(c).start()
    cp_x(2).start()
    start(cp_small())

    kk = _odd_freq(jax.lax.broadcasted_iota(jnp.int32, (P, P), 0))
    nn = jax.lax.broadcasted_iota(jnp.int32, (P, P), 1)
    fc, fs = _cos_sin((kk * (4 * nn - 127)) & 2047)
    for g in range(P // 8):
        F_v[g * 16:(g + 1) * 16, 0:P] = jnp.concatenate(
            [fc[g * 8:(g + 1) * 8], -fs[g * 8:(g + 1) * 8]], axis=0).astype(BF16)
    fc, fs = _cos_sin((kk * (-127)) & 2047)
    ph_v[0] = fc
    ph_v[1] = fs
    kk = _odd_freq(jax.lax.broadcasted_iota(jnp.int32, (MC, P), 1))
    mm = jax.lax.broadcasted_iota(jnp.int32, (MC, P), 0)
    ic, is_ = _cos_sin((kk * (4 * mm + 2)) & 2047)
    Fi_v[:, 0:P] = (ic * (1.0 / P)).astype(BF16)
    Fi_v[:, P:2 * P] = (is_ * (1.0 / P)).astype(BF16)
    kf_v[:, 0:8, :] = jnp.zeros((D // L, 8, L), F32)

    for t in range(2):
        cp_x(t).wait()
        for s in range(TM // 16):
            ln_x(t, s)

    def small_setup():
        sk = sk_in[...].astype(F32)
        for t in range(4):
            sk_v[t] = jnp.broadcast_to(sk[t:t + 1], (8, D))
        drow = d_in[...].astype(F32).reshape(1, D)
        for l in range(D // L):
            lanes = slice(l * L, (l + 1) * L)
            dre = ph_v[0] * drow[:, lanes]
            dim = ph_v[1] * drow[:, lanes]
            H_v[0, 0, 0:64, lanes] = -dim[0:64]
            H_v[0, 0, 64:P, lanes] = dim[64:P]
            H_v[0, 1, 0:64, lanes] = -dre[0:64]
            H_v[0, 1, 64:P, lanes] = dre[64:P]

    def bcol_task(t, j, tie):
        brow = b_in[...].astype(F32).reshape(1, S)[:, j * P:(j + 1) * P] * 0.25 + tie[0:1]
        bcol_v[j * P:(j + 1) * P, :] = jnp.broadcast_to(brow, (P, P)).T

    LAG = 2

    def interleave(*lists):
        out = []
        for j in range(max(len(a) for a in lists)):
            for a in lists:
                out += a[j:j + 1]
        return out

    def p1_first(c):
        bg = _Background()
        todo = []
        if c == 3:
            todo = tasks(ln_z2, 0)
            bg.add(wcomb_gen(range(3)))
        if c == 4:
            todo = tasks(ln_x2, 2, 8)
            bg.add(wcomb_gen(range(3, 6)))
            small_setup()
        tied = _Tied(todo, 20)
        for t in range(2):
            for m in range(TM // MC):
                job_z(t, m, range(*WIN_CHUNKS[c]), bg, (80, 40), tied)
        bg.drain()
        assert not tied.tasks

    for c in range(5):
        cp_win(c).wait()
        if c == 2:
            start(cp_conv(0))
            cp_x(3).start()
        if c == 4:
            cp_x(2).wait()
            wait(cp_small())
        block(lambda c=c: p1_first(c), f'p1_f{c}')

    def p1_wait(i):
        wait(cp_conv(i - LAG))
        if i + 1 < NT:
            cp_x(i + 1).wait()
        if i == 4:
            cp_wout().wait()
        if i == NT - 3:
            wait(cp_wsp(0))

    def p1_start(i):
        if i + 2 < NT:
            cp_x(i + 2).start()
        start(cp_conv(i - LAG + 1))
        start(cp_wsp((i - 2) // 2, ((i - 2) % 2,)))
        if i == NT - 1:
            start(cp_conv(NT - 1))
        if i == 2:
            cp_wout().start()

    def take(gen, n):
        for _ in range(n):
            yield next(gen)

    def p1_step(i):
        bg = _Background()
        dft = _Background()
        t = i - LAG
        kv = kv_gen(t)
        dft.add(take(kv, (20 if t >= 1 else 10) * 64 // KV_ROWS))
        if t >= 1:
            bg.add(g_gen(t - 1))
        else:
            bg.add(take(kv, 10 * 64 // KV_ROWS))
        extra = 0
        if i == 4:
            bg.add(wocomb_gen())
            extra = 30
        if i in (NT - 3, NT - 2):
            bg.add(acomb_gen(0, range(4) if i == NT - 3 else range(4, 8)))
            extra = 20
        last = i == NT - 1
        z2t = tasks(ln_z2, i - 1)
        todo = interleave(tasks(ln_x2, i + 1, 8) if not last else [], z2t[0::2], z2t[1::2],
                          tasks(bcol_task, 0) if i == 2 else [])
        nx = 8 if (t >= 1 and TIE_X) else 0
        tied = _Tied(todo, (24 if last else TIED_N) + nx)
        dft.run(110)
        if t >= 1:
            for q in range(4):
                dft_piece('X', t - 1, q, dft, DFT_B[0], tied if TIE_X else None)
        for p in range(2):
            for j in range(FH // L):
                job_zs(i, p, j, bg, (Z_B0 + extra, Z_B1 + extra), tied)
            assert not tied.tasks or (p == 0 and not last)
            if p == 0 and last:
                tied = _Tied(tasks(ln_z2, i, 8), 22)
        if last:
            for s in range(8, 16):
                ln_z2(i, s)
        for q in range(4):
            dft_piece('H', t, q, dft, DFT_B[1])
        bg.drain()
        dft.drain()

    for i in range(2, NT):
        p1_wait(i)
        p1_start(i)
        block(lambda i=i: p1_step(i), f'p1_{i}')

    groups = P2_GROUPS
    NG = len(groups)

    def p2_dma(gi):
        if gi >= 2:
            for i in groups[gi - 2]:
                start(cp_out(i))
        if gi >= 3:
            for i in groups[gi - 3]:
                wait(cp_out(i))
        if gi + 2 < NG:
            for i in groups[gi + 2]:
                start(cp_wsp(i))
        if gi < 2:
            wait(cp_conv(NT - 2 + gi))
        if gi + 1 < NG:
            for i in groups[gi + 1]:
                wait(cp_wsp(i))

    def tails_of(i, bg, budget):
        return [tail_gen(i, bg, budget)] * 20

    def p2_block(gi):
        bg = _Background()
        steps = groups[gi]
        tb = [0.0]
        pending = [t_ for i in (groups[gi - 1] if gi > 0 else []) for t_ in tails_of(i, bg, tb)]
        total = sum(a + 1 for i in steps for a in _blocks_of_step(i)) * 40 * 16
        total += len(steps) * (24 * E_COST + 6 * U_COST) + len(pending) * T_COST
        slots = 84 * len(steps) + TAIL_W * len(pending)
        bg.add(freq_gen(_blocks_of_step(steps[0])[0]))
        if gi < 2:
            bg.add(kv_gen(NT - 2 + gi))
            total += 20 * KV_COST
            slots += 10
        if gi < 3:
            slots += 10
            bg.add(g_gen(NT - 3 + gi))
            total += 40 * G_COST
        if gi + 1 < NG:
            for i in groups[gi + 1]:
                bg.add(acomb_gen(i))
                total += 32 * A_COST
        for i in steps[1:]:
            bg.add(freq_gen(_blocks_of_step(i)[0]))
        budget = tb[0] = total / (slots + 1.0)
        bg.run(budget)
        if gi < 3:
            job_x(NT - 3 + gi, bg, budget)
        if gi < 2:
            job_h(NT - 2 + gi, bg, budget)
        units = [4, 4, 2, 4, 4, 2] * (len(pending) // 20)
        every = [0] * (6 * len(steps))
        for j, n in enumerate(units):
            every[min(len(every) - 1, j * len(every) // len(units))] += n
        for i in steps:
            job_big(i, bg, pending, budget, every)
        for t_ in pending:
            next(t_)
        bg.drain()

    for gi in range(NG):
        p2_dma(gi)
        block(lambda gi=gi: p2_block(gi), f'p2_{gi}')

    def cp_last(upper):
        a0 = _blocks_of_step(NT - 1)[0]
        return [pltpu.make_async_copy(o_v.at[pl.ds(r, MC)], o_hbm.at[0, pl.ds(r, MC)], sem_out.at[(NT - 1) % 5])
                for r in ((a0 + w) * P + (MC if upper else 0) for w in range(2))]

    def p2_last():
        for j, t_ in enumerate(tails_of(NT - 1, _Background(), [0.0])):
            next(t_)
            if j == 9:
                start(cp_last(True))

    p2_dma(NG)
    block(p2_last, 'p2_last')
    start(cp_last(False))
    for i in groups[NG - 2]:
        wait(cp_out(i))
    wait(cp_last(True))
    wait(cp_last(False))
    if _ONLY is not None:
        for r_ in (xn_u, XL_u, WB_u, UL_u, WO_u, z1_v, R_u, Lc_u, zf_v, zg_v, kv_u, u_u, X_v, H_v, G_v, Z_u, kf_v):
            c_ = pltpu.make_async_copy(r_, r_, sem_small.at[0])
            c_.start()
            c_.wait()


@jax.jit
def pallas_recurrent_scan__ssm_conv_h3__mixer_gmlp__prompt_kernel(
    A_q: jax.Array,
    A_k: jax.Array,
    A_v: jax.Array,
    A_shift_k: jax.Array,
    A_ssm_k: jax.Array,
    A_ssm_D: jax.Array,
    B_x: jax.Array,
    B_w_in: jax.Array,
    B_w_sp: jax.Array,
    B_b_sp: jax.Array,
    B_w_out: jax.Array,
):
    del B_x
    hbm = pl.BlockSpec(memory_space=pl.ANY)

    def bf16_buf(*shape):
        return pltpu.VMEM(shape[:-2] + (shape[-2] // 2, shape[-1]), U32)

    return pl.pallas_call(
        _kernel,
        out_shape=jax.ShapeDtypeStruct((1, S, D), BF16),
        in_specs=[hbm] * 10,
        out_specs=hbm,
        scratch_shapes=[
            bf16_buf(S, D),
            bf16_buf(S, D),
            bf16_buf(S, D),
            bf16_buf(NT, D, TM),
            bf16_buf(D, 2 * FH),
            bf16_buf(S, S),
            bf16_buf(FH, D),
            pltpu.VMEM((S, D), BF16),
            pltpu.VMEM((4, D), BF16),
            pltpu.VMEM((D,), BF16),
            pltpu.VMEM((S,), BF16),
            bf16_buf(S, D),
            bf16_buf(2 * 5 * P, KH),
            bf16_buf(5 * KH, FH),
            bf16_buf(4 * 5 * P, HN),
            bf16_buf(5 * HN, 2 * L),
            pltpu.VMEM((S, FH), F32),
            bf16_buf(7 * HK, HN),
            bf16_buf(4 * 5 * P, HK),
            pltpu.VMEM((HK, FH), F32),
            pltpu.VMEM((2, TM, FH), F32),
            bf16_buf(S, D),
            bf16_buf(S, FH),
            pltpu.VMEM((NB, 2, P, D), F32),
            pltpu.VMEM((6, 2, P, D), F32),
            pltpu.VMEM((NB, 2, P, D), F32),
            bf16_buf(NB * 2 * P, D),
            pltpu.VMEM((2, D // L, MC, L), F32),
            bf16_buf(2 * P, 2 * P),
            bf16_buf(MC, 2 * P),
            pltpu.VMEM((S, L), F32),
            pltpu.VMEM((2, P, L), F32),
            pltpu.VMEM((4, 8, D), F32),
            pltpu.VMEM((D // L, S + 8, L), F32),
            pltpu.SemaphoreType.DMA((1,)),
            pltpu.SemaphoreType.DMA((3,)),
            pltpu.SemaphoreType.DMA((2,)),
            pltpu.SemaphoreType.DMA((5,)),
            pltpu.SemaphoreType.DMA((5,)),
            pltpu.SemaphoreType.DMA((5,)),
        ],
        compiler_params=pltpu.CompilerParams(vmem_limit_bytes=116 * 1024 * 1024, disable_semaphore_checks=True),
    )(A_q, A_k, A_v, A_shift_k.T, A_ssm_k, A_ssm_D, B_w_in, B_w_sp, B_b_sp, B_w_out)
```

```python
import math

import jax
import jax.numpy as jnp
import jax.experimental.pallas as pl
import jax.experimental.pallas.tpu as pltpu

S = 2048
D = 640
FH = 768
P = 128
NB = S // P
TM = 256
NT = S // TM
MC = 64
L = 128
HK = S // 2
KH = 256
HN = FH // 2
P2_GROUPS = ((0,), (1, 2), (3, 4), (5, 6), (7,))
STEP_BLOCKS = ((6, 7), (8, 9), (4, 5), (12, 13), (2, 3), (14, 15), (0, 1), (10, 11))
KV_COST, G_COST, A_COST = 110, 36, 56
E_COST, U_COST, T_COST, TAIL_W = 24, 90, 90, 1.6
BIG_KG = 512
TIE_X = False
DFT_B = (130, 80)
Z_B0, Z_B1 = 60, 10
TIED_N = 42
ORDER = 1
FR = 16
KV_ROWS = 64
WIN_CHUNKS = ((6, 7), (7, 9), (9, 12), (0, 3), (3, 6))
EPS = 1e-5
F32 = jnp.float32
BF16 = jnp.bfloat16
U32 = jnp.uint32
GELU_C = math.sqrt(2.0 / math.pi)
GA = (GELU_C * 0.044715) ** (1.0 / 3.0)
NT_DIMS = (((1,), (1,)), ((), ()))
_ONLY = None


def _dot(a, b):
    return jnp.dot(a, b, preferred_element_type=F32)


def _cos_sin(m):
    q = (m + 256) >> 9
    x = (m - (q << 9)).astype(F32) * (2.0 * math.pi / 2048.0)
    x2 = x * x
    s = x * (1.0 + x2 * (-1.0 / 6 + x2 * (1.0 / 120 + x2 * (-1.0 / 5040 + x2 * (1.0 / 362880)))))
    c = 1.0 + x2 * (-0.5 + x2 * (1.0 / 24 + x2 * (-1.0 / 720 + x2 * (1.0 / 40320 - x2 * (1.0 / 3628800)))))
    swap = (q & 1) == 1
    c0 = jnp.where(swap, s, c)
    s0 = jnp.where(swap, c, s)
    cos = jnp.where(((q + 1) & 2) == 2, -c0, c0)
    sin = jnp.where((q & 2) == 2, -s0, s0)
    return cos, sin


def _odd_freq(r):
    return jnp.where(r < 64, 4 * r + 1, 4 * r - 253)


def _gelu_scaled(z):
    return z + z * jnp.tanh(z * (GELU_C / GA + z * z))


def _signzero(z):
    bits = jax.lax.bitcast_convert_type(z, U32) & jnp.uint32(0x80000000)
    return jax.lax.bitcast_convert_type(bits, F32)


def _ln(x, eps, tie=None, scale=None):
    n = x.shape[-1]
    cols = [x[:, j * L:(j + 1) * L] for j in range(n // L)]
    s1 = cols[0]
    s2 = cols[0] * cols[0]
    for c in cols[1:]:
        s1 = s1 + c
        s2 = s2 + c * c
    if tie is not None:
        s1 = s1 + tie
        s2 = s2 + tie
    m = jnp.sum(s1, axis=-1, keepdims=True) * (1.0 / n)
    v = jnp.maximum(jnp.sum(s2, axis=-1, keepdims=True) * (1.0 / n) - m * m, 0.0)
    rs = jax.lax.rsqrt(v + eps)
    if scale is not None:
        rs = rs * scale
    return (x - m) * rs


def _blocks_of_step(i):
    return STEP_BLOCKS[i]


class _Background:
    def __init__(self):
        self.q = []
        self.credit = 0.0

    def add(self, gen):
        self.q.append(gen)

    def run(self, budget):
        self.credit += budget
        while self.q and self.credit > 0:
            try:
                self.credit -= next(self.q[0])
            except StopIteration:
                self.q.pop(0)
        if not self.q:
            self.credit = 0.0

    def charge(self, cost):
        self.credit -= cost

    def drain(self):
        while self.q:
            self.run(1e9)


class _Tied:
    def __init__(self, tasks, npieces):
        self.tasks = list(tasks)
        self.rate = len(self.tasks) / float(npieces)
        self.credit = 0.999

    def run(self, z):
        self.credit += self.rate
        n = 0
        while self.tasks and self.credit >= 1.0:
            self.tasks.pop(0)(_signzero(z[0:16]))
            self.credit -= 1.0
            n += 1
        return n


def _kernel(q_hbm, k_hbm, v_hbm, sk_hbm, h_hbm, d_hbm, win_hbm, wsp_hbm, b_hbm, wout_hbm,
            o_hbm,
            x_u, k_u, v_u, h_u, win_u, wsp_u, wout_u, o_v, sk_in, d_in, b_in,
            xn_u, XL_u, WB_u, UL_u, WO_u, z1_v, R_u, Lc_u, zf_v, zg_v, kv_u, u_u, X_v, H_v, G_v, Z_u, yl_v, F_u, Fi_u, bcol_v, ph_v, sk_v, kf_v,
            sem_small, sem_x, sem_conv, sem_wsp, sem_w, sem_out):
    x_v, k_v, v_v, h_v, win_v, wsp_v, wout_v, xn_v, XL_v, WB_v, UL_v, WO_v, R_v, Lc_v, kv_v, u_v, Z_v, F_v, Fi_v = [
        r.bitcast(BF16) for r in (x_u, k_u, v_u, h_u, win_u, wsp_u, wout_u, xn_u, XL_u, WB_u, UL_u, WO_u, R_u, Lc_u, kv_u, u_u, Z_u, F_u,
                                  Fi_u)]

    def cp_small():
        return [pltpu.make_async_copy(s_, d_, sem_small.at[0])
                for s_, d_ in ((d_hbm, d_in), (sk_hbm, sk_in), (b_hbm, b_in))]

    def cp_x(t):
        return pltpu.make_async_copy(q_hbm.at[0, pl.ds(t * TM, TM)], x_v.at[pl.ds(t * TM, TM)], sem_x.at[t % 3])

    def cp_conv(t):
        rows = pl.ds(t * TM, TM)
        sem = sem_conv.at[t % 2]
        return [pltpu.make_async_copy(h_hbm.at[:, rows], h_v.at[t], sem),
                pltpu.make_async_copy(k_hbm.at[0, rows], k_v.at[rows], sem),
                pltpu.make_async_copy(v_hbm.at[0, rows], v_v.at[rows], sem)]

    def cp_wsp(i, which=(0, 1)):
        return [pltpu.make_async_copy(wsp_hbm.at[pl.ds(_blocks_of_step(i)[half] * P, P)],
                                      wsp_v.at[pl.ds(i * TM + half * P, P)], sem_wsp.at[i % 5]) for half in which]

    def cp_win(c):
        lo, hi = WIN_CHUNKS[c]
        cols = pl.ds(lo * L, (hi - lo) * L)
        return pltpu.make_async_copy(win_hbm.at[:, cols], win_v.at[:, cols], sem_w.at[c])

    def cp_wout():
        return pltpu.make_async_copy(wout_hbm, wout_v, sem_w.at[0])

    def cp_out(i):
        rows = pl.ds(_blocks_of_step(i)[0] * P, TM)
        return [pltpu.make_async_copy(o_v.at[rows], o_hbm.at[0, rows], sem_out.at[i % 5])]

    def start(cs):
        for c in cs:
            c.start()

    def wait(cs):
        for c in cs:
            c.wait()

    def block(fn, name):
        def body(it):
            fn()
            return it + 1

        if _ONLY is None or name in _ONLY:
            jax.lax.while_loop(lambda it: it < 1, body, jnp.int32(0))

    def ln_x(t, s, tie=None):
        rows = pl.ds(t * TM + s * 16, 16)
        y = _ln(x_v[rows, :].astype(F32), EPS, tie, GA)
        xn_v[rows, :] = y.astype(BF16)
        return y

    def ln_x2(t, s, tie):
        p, q = s // 4, s % 4
        y1 = ln_x(t, 8 * p + q, tie)
        y2 = ln_x(t, 8 * p + 4 + q, tie)
        a11, a12, a21, a22 = y1[:, :KH], y1[:, KH:2 * KH], y2[:, :KH], y2[:, KH:2 * KH]
        r0 = (t % 2) * 5 * P + p * MC + q * 16
        for j, c in enumerate((a11 + a22, a21 + a22, a11 + a12, a21 - a11, a12 - a22)):
            XL_v[pl.ds(r0 + j * P, 16), :] = c.astype(BF16)

    def wcomb_gen(cols):
        for j in cols:
            c1 = slice(j * L, (j + 1) * L)
            c2 = slice(FH + j * L, FH + (j + 1) * L)
            for r in range(KH // 32):
                top = pl.ds(r * 32, 32)
                bot = pl.ds(KH + r * 32, 32)
                b11, b12 = win_v[top, c1].astype(F32), win_v[top, c2].astype(F32)
                b21, b22 = win_v[bot, c1].astype(F32), win_v[bot, c2].astype(F32)
                for w, c in enumerate((b11 + b22, b12 - b22, b21 - b11, b11 + b12, b21 + b22)):
                    WB_v[pl.ds(w * KH + r * 32, 32), c1] = c.astype(BF16)
                yield A_COST

    def ln_z2(t, s, tie=None):
        y = _ln(zg_v[t % 2, s * 16:(s + 1) * 16, :], 4.0 * GA * GA * EPS, tie, 0.25 / GA)
        lo, hi = y[:, :HN], y[:, HN:]
        r = (t * TM + s * 16) % HK
        rows = pl.ds(r, 16)
        if t < NT // 2:
            zf_v[rows, :] = y
            R_v[pl.ds(1 * HK + r, 16), :] = lo.astype(BF16)
            R_v[pl.ds(5 * HK + r, 16), :] = (lo + hi).astype(BF16)
        else:
            b11 = zf_v[rows, :HN]
            R_v[pl.ds(0 * HK + r, 16), :] = (b11 + hi).astype(BF16)
            R_v[pl.ds(2 * HK + r, 16), :] = (zf_v[rows, HN:] - hi).astype(BF16)
            R_v[pl.ds(3 * HK + r, 16), :] = (lo - b11).astype(BF16)
            R_v[pl.ds(4 * HK + r, 16), :] = hi.astype(BF16)
            R_v[pl.ds(6 * HK + r, 16), :] = (lo + hi).astype(BF16)

    def acomb_gen(i, groups=range(P // 16)):
        for r in groups:
            for c in range(HK // 256):
                top = pl.ds(i * TM + r * 16, 16)
                bot = pl.ds(i * TM + P + r * 16, 16)
                c1 = slice(c * 256, (c + 1) * 256)
                c2 = slice(HK + c * 256, HK + (c + 1) * 256)
                a11 = wsp_v[top, c1].astype(F32)
                a12 = wsp_v[top, c2].astype(F32)
                a21 = wsp_v[bot, c1].astype(F32)
                a22 = wsp_v[bot, c2].astype(F32)
                r0 = (i % 4) * 5 * P + r * 16
                Lc_v[pl.ds(r0 + 0 * P, 16), c1] = (a11 + a22).astype(BF16)
                Lc_v[pl.ds(r0 + 1 * P, 16), c1] = (a21 + a22).astype(BF16)
                Lc_v[pl.ds(r0 + 2 * P, 16), c1] = (a11 + a12).astype(BF16)
                Lc_v[pl.ds(r0 + 3 * P, 16), c1] = (a21 - a11).astype(BF16)
                Lc_v[pl.ds(r0 + 4 * P, 16), c1] = (a12 - a22).astype(BF16)
                yield A_COST

    def tasks(fn, t, n=TM // 16):
        return [lambda tie, s=s: fn(t, s, tie) for s in range(n)]

    def kv_gen(t):
        for m in range(TM // KV_ROWS):
            r = t * TM + m * KV_ROWS
            for l in range(D // L):
                lanes = slice(l * L, (l + 1) * L)
                kf = k_v[pl.ds(r, KV_ROWS), lanes].astype(F32)
                kf_v[l, pl.ds(r + 8, KV_ROWS), :] = kf
                ks = kf * sk_v[0, 0:1, lanes]
                for tap in range(1, 4):
                    ks = ks + kf_v[l, pl.ds(r + 8 - tap, KV_ROWS), :] * sk_v[tap, 0:1, lanes]
                kv = ks * v_v[pl.ds(r, KV_ROWS), lanes].astype(F32)
                kv_v[pl.ds(r, KV_ROWS), lanes] = kv.astype(BF16)
                yield KV_COST * KV_ROWS / 64

    def g_gen(t):
        for r in range(P // 16):
            rows = pl.ds(r * 16, 16)
            for l in range(D // L):
                lanes = slice(l * L, (l + 1) * L)
                h = [(H_v[(2 * t + w) % 6, 0, rows, lanes], H_v[(2 * t + w) % 6, 1, rows, lanes]) for w in range(3)]
                for w in range(2):
                    (pr, pi), (cr, ci) = h[w], h[w + 1]
                    G_v[2 * t + w, 0, rows, lanes] = cr - pi if r < P // 32 else cr + pi
                    G_v[2 * t + w, 1, rows, lanes] = ci + pr if r < P // 32 else ci - pr
                yield G_COST

    def freq_gen(a):
        def cmac(acc, x, g):
            pr = x[0] * g[0] - x[1] * g[1]
            pi = x[0] * g[1] + x[1] * g[0]
            return (pr, pi) if acc is None else (acc[0] + pr, acc[1] + pi)

        for r in range(P // 16):
            for l in range(D // L):
                lanes = slice(l * L, (l + 1) * L)
                res = []
                for sub in range(16 // FR):
                    rows = pl.ds(r * 16 + sub * FR, FR)
                    lo = hi = None
                    g = (G_v[a + 1, 0, rows, lanes], G_v[a + 1, 1, rows, lanes])
                    for c in range(a + 2):
                        x = (X_v[c, 0, rows, lanes], X_v[c, 1, rows, lanes])
                        hi = cmac(hi, x, g)
                        if c <= a:
                            g = (G_v[a - c, 0, rows, lanes], G_v[a - c, 1, rows, lanes])
                            lo = cmac(lo, x, g)
                            yield 2 * FR
                    res.append((lo, hi))
                for w in range(2):
                    for part in range(2):
                        Z_v[pl.ds((a + w) * 2 * P + part * P + r * 16, 16), lanes] = jnp.concatenate(
                            [z[w][part] for z in res], axis=0).astype(BF16)
                yield 20

    def dft_piece(kind, t, q, bg, budget, tied=None):
        j, half = q // 2, q % 2
        f = F_v[half * P:(half + 1) * P, 0:P]
        if kind == 'H':
            r = jax.lax.dot_general(f, h_v[t, :, j * P:(j + 1) * P], NT_DIMS, preferred_element_type=F32)
            dst, idx = H_v, (2 * t + j + 1) % 6
        else:
            r = _dot(f, kv_v[(2 * t + j) * P:(2 * t + j + 1) * P, :])
            dst, idx = X_v, 2 * t + j
        r4 = r.reshape(8, 2, 8, D)
        for part in range(2):
            dst[idx, part, half * 64:(half + 1) * 64, :] = r4[:, part].reshape(64, D)
        if tied is not None:
            tied.run(r[:, 0:L])
            tied.run(r[:, 2 * L:3 * L])
        bg.run(budget * 2.5)

    def job_h(t, bg, budget):
        for q in range(4):
            dft_piece('H', t, q, bg, budget)

    def job_x(t, bg, budget):
        for q in range(4):
            dft_piece('X', t, q, bg, budget)

    def z_out(t, m, n, pre, bg, budget, tied):
        z = _gelu_scaled(pre)
        if n < FH // L:
            z1_v[pl.ds(t * TM + m * MC, MC), n * L:(n + 1) * L] = z
        else:
            zg_v[t % 2, m * MC:(m + 1) * MC, n * L - FH:(n + 1) * L - FH] = z
        ntask = tied.run(z)
        bg.run(budget[1] if ntask else budget[0])

    def job_z(t, m, cols, bg, budget, tied):
        for n in cols:
            z_out(t, m, n, _dot(xn_v[pl.ds(t * TM + m * MC, MC), :], win_v[:, n * L:(n + 1) * L]), bg, budget, tied)

    def job_zs(t, p, j, bg, budget, tied):
        r1 = pl.ds(t * TM + p * P, MC)
        r2 = pl.ds(t * TM + p * P + MC, MC)
        c1 = slice(j * L, (j + 1) * L)
        c2 = slice(FH + j * L, FH + (j + 1) * L)

        def xl(w):
            r0 = (t % 2) * 5 * P + w * P + p * MC
            return XL_v[r0:r0 + MC, :]

        def wb(w):
            return WB_v[w * KH:(w + 1) * KH, c1]

        def rem(rows, cols):
            return _dot(xn_v[rows, 2 * KH:], win_v[2 * KH:, cols])

        m2 = _dot(xl(1), win_v[0:KH, c1])
        m4 = _dot(xn_v[r2, KH:2 * KH], wb(2))
        z_out(t, 2 * p + 1, j, m2 + m4 + rem(r2, c1), bg, budget, tied)
        m3 = _dot(xn_v[r1, 0:KH], wb(1))
        m5 = _dot(xl(2), win_v[KH:2 * KH, c2])
        z_out(t, 2 * p, 6 + j, m3 + m5 + rem(r1, c2), bg, budget, tied)
        m1 = _dot(xl(0), wb(0))
        z_out(t, 2 * p, j, (m4 - m5) + m1 + _dot(xl(4), wb(4)) + rem(r1, c1), bg, budget, tied)
        z_out(t, 2 * p + 1, 6 + j, (m3 - m2) + m1 + _dot(xl(3), wb(3)) + rem(r2, c2), bg, budget, tied)

    rev8 = 7 - jax.lax.broadcasted_iota(jnp.int32, (8, L), 0)

    def finish(a, upper, n, hh, slot):
        rows = pl.ds(a * P + (MC if upper else 0), MC)
        lanes = slice(n * L, (n + 1) * L)
        if upper:
            ya = _dot(Fi_v[:, 0:P], Z_v[a * 2 * P:a * 2 * P + P, lanes])
            yb = _dot(Fi_v[:, P:2 * P], Z_v[a * 2 * P + P:(a + 1) * 2 * P, lanes])
            slot(0.5)
            y = ya - yb
            lo = ya + yb
            for j in range(MC // 8):
                yl_v[a % 2, n, (7 - j) * 8:(8 - j) * 8, :] = jnp.take_along_axis(lo[j * 8:(j + 1) * 8], rev8, axis=0)
        else:
            y = yl_v[a % 2, n]
        gate = hh + hh * jnp.tanh(hh)
        s = xn_v[rows, lanes].astype(F32) * y
        o_v[rows, lanes] = (x_v[rows, lanes].astype(F32) + s * gate).astype(BF16)

    def tail_gen(i, bg, budget):
        a0, a1 = _blocks_of_step(i)

        def slot(w):
            bg.run(w * budget[0])

        def dot3(a, b):
            r = _dot(a, b)
            slot(0.75)
            return r

        for upper in (True, False):
            sub = MC if upper else 0
            r1 = pl.ds(a0 * P + sub, MC)
            r2 = pl.ds(a1 * P + sub, MC)

            def ul(w):
                r0 = ((i % 4) * 5 + w) * P + sub
                return UL_v[r0:r0 + MC, :]

            for j in range(2):
                c1 = slice(j * L, (j + 1) * L)
                c2 = slice((2 + j) * L, (3 + j) * L)

                def wo(w):
                    return WO_v[w * HN:(w + 1) * HN, c1]

                m2 = dot3(ul(1), wout_v[0:HN, c1])
                m4 = dot3(u_v[r2, HN:], wo(2))
                finish(a1, upper, j, m2 + m4, slot)
                bg.charge(T_COST)
                yield
                m3 = dot3(u_v[r1, 0:HN], wo(1))
                m5 = dot3(ul(2), wout_v[HN:, c2])
                finish(a0, upper, 2 + j, m3 + m5, slot)
                bg.charge(T_COST)
                yield
                m1 = dot3(ul(0), wo(0))
                finish(a0, upper, j, (m4 - m5) + m1 + dot3(ul(4), wo(4)), slot)
                bg.charge(T_COST)
                yield
                finish(a1, upper, 2 + j, (m3 - m2) + m1 + dot3(ul(3), wo(3)), slot)
                bg.charge(T_COST)
                yield
            finish(a0, upper, 4, dot3(u_v[r1, 0:HN], wout_v[0:HN, 4 * L:]) + dot3(u_v[r1, HN:], wout_v[HN:, 4 * L:]), slot)
            bg.charge(T_COST)
            yield
            finish(a1, upper, 4, dot3(u_v[r2, 0:HN], wout_v[0:HN, 4 * L:]) + dot3(u_v[r2, HN:], wout_v[HN:, 4 * L:]), slot)
            bg.charge(T_COST)
            yield

    def wocomb_gen():
        for j in range(2):
            c1 = slice(j * L, (j + 1) * L)
            c2 = slice((2 + j) * L, (3 + j) * L)
            for r in range(HN // 32):
                top = pl.ds(r * 32, 32)
                bot = pl.ds(HN + r * 32, 32)
                b11, b12 = wout_v[top, c1].astype(F32), wout_v[top, c2].astype(F32)
                b21, b22 = wout_v[bot, c1].astype(F32), wout_v[bot, c2].astype(F32)
                for w, c in enumerate((b11 + b22, b12 - b22, b21 - b11, b11 + b12, b21 + b22)):
                    WO_v[pl.ds(w * HN + r * 32, 32), c1] = c.astype(BF16)
                yield A_COST

    def job_big(i, bg, pending, budget, every):
        a0, a1 = _blocks_of_step(i)
        KG = BIG_KG

        def lhs(j, sub, cols):
            if j == 2:
                return wsp_v[i * TM + sub:i * TM + sub + MC, cols]
            if j == 3:
                return wsp_v[i * TM + P + sub:i * TM + P + sub + MC, HK + cols.start:HK + cols.stop]
            r0 = ((i % 4) * 5 + {0: 0, 1: 1, 4: 2, 5: 3, 6: 4}[j]) * P + sub
            return Lc_v[r0:r0 + MC, cols]

        def prod(j, sub, n, acc=None):
            for kg in range(HK // KG):
                ks = slice(kg * KG, (kg + 1) * KG)
                p = _dot(lhs(j, sub, ks), R_v[j * HK + kg * KG:j * HK + (kg + 1) * KG, n * L:(n + 1) * L])
                acc = p if acc is None else acc + p
                bg.run(budget * KG / 512)
            return acc

        def tails(n):
            for _ in range(n):
                if pending:
                    next(pending.pop(0))

        def emit(a, sub, n, g):
            rows = pl.ds(a * P + sub, MC)
            lanes = slice(n * L, (n + 1) * L)
            u = z1_v[rows, lanes] * (g + bcol_v[rows, :])
            u_v[rows, lanes] = u.astype(BF16)
            bg.charge(E_COST)
            return u

        for sub in (0, MC):
            for n in range(HN // L):
                def put(w, c):
                    UL_v[pl.ds(((i % 4) * 5 + w) * P + sub, MC), n * L:(n + 1) * L] = c.astype(BF16)

                if ORDER == 0:
                    m2 = prod(1, sub, n)
                    m4 = prod(3, sub, n)
                    u21 = emit(a1, sub, n, m2 + m4)
                    m3 = prod(2, sub, n)
                    t22 = m3 - m2
                    m5 = prod(4, sub, n)
                    u12 = emit(a0, sub, n + HN // L, m3 + m5)
                    t11 = m4 - m5
                    m1 = prod(0, sub, n)
                    u11 = emit(a0, sub, n, prod(6, sub, n, t11 + m1))
                    u22 = emit(a1, sub, n + HN // L, prod(5, sub, n, t22 + m1))
                    for w, c in enumerate((u11 + u22, u21 + u22, u11 + u12, u21 - u11, u12 - u22)):
                        put(w, c)
                else:
                    m1 = prod(0, sub, n)
                    t11 = prod(6, sub, n, m1)
                    m4 = prod(3, sub, n)
                    t11 = t11 + m4
                    m5 = prod(4, sub, n)
                    u11 = emit(a0, sub, n, t11 - m5)
                    m2 = prod(1, sub, n)
                    u21 = emit(a1, sub, n, m2 + m4)
                    put(3, u21 - u11)
                    t22 = m1 - m2
                    m3 = prod(2, sub, n)
                    u12 = emit(a0, sub, n + HN // L, m3 + m5)
                    put(2, u11 + u12)
                    u22 = emit(a1, sub, n + HN // L, prod(5, sub, n, t22 + m3))
                    put(0, u11 + u22)
                    put(1, u21 + u22)
                    put(4, u12 - u22)
                bg.charge(U_COST)
                tails(every.pop(0))

    if _ONLY is not None:
        for r_ in (xn_u, XL_u, WB_u, UL_u, WO_u, z1_v, R_u, Lc_u, zf_v, zg_v, kv_u, u_u, X_v, H_v, G_v, Z_u, kf_v):
            c_ = pltpu.make_async_copy(r_, r_, sem_small.at[0])
            c_.start()
            c_.wait()

    cp_x(0).start()
    cp_win(0).start()
    cp_x(1).start()
    for c in range(1, 5):
        cp_win(c).start()
    cp_x(2).start()
    start(cp_small())

    kk = _odd_freq(jax.lax.broadcasted_iota(jnp.int32, (P, P), 0))
    nn = jax.lax.broadcasted_iota(jnp.int32, (P, P), 1)
    fc, fs = _cos_sin((kk * (4 * nn - 127)) & 2047)
    for g in range(P // 8):
        F_v[g * 16:(g + 1) * 16, 0:P] = jnp.concatenate(
            [fc[g * 8:(g + 1) * 8], -fs[g * 8:(g + 1) * 8]], axis=0).astype(BF16)
    fc, fs = _cos_sin((kk * (-127)) & 2047)
    ph_v[0] = fc
    ph_v[1] = fs
    kk = _odd_freq(jax.lax.broadcasted_iota(jnp.int32, (MC, P), 1))
    mm = jax.lax.broadcasted_iota(jnp.int32, (MC, P), 0)
    ic, is_ = _cos_sin((kk * (4 * mm + 2)) & 2047)
    Fi_v[:, 0:P] = (ic * (1.0 / (P * GA))).astype(BF16)
    Fi_v[:, P:2 * P] = (is_ * (1.0 / (P * GA))).astype(BF16)
    kf_v[:, 0:8, :] = jnp.zeros((D // L, 8, L), F32)

    cp_x(0).wait()
    for s in range(TM // 16):
        ln_x(0, s)

    def small_setup():
        sk = sk_in[...].astype(F32)
        for t in range(4):
            sk_v[t] = jnp.broadcast_to(sk[t:t + 1], (8, D))
        drow = d_in[...].astype(F32).reshape(1, D)
        for l in range(D // L):
            lanes = slice(l * L, (l + 1) * L)
            dre = ph_v[0] * drow[:, lanes]
            dim = ph_v[1] * drow[:, lanes]
            H_v[0, 0, 0:64, lanes] = -dim[0:64]
            H_v[0, 0, 64:P, lanes] = dim[64:P]
            H_v[0, 1, 0:64, lanes] = -dre[0:64]
            H_v[0, 1, 64:P, lanes] = dre[64:P]

    def bcol_task(t, j, tie):
        brow = b_in[...].astype(F32).reshape(1, S)[:, j * P:(j + 1) * P] * (0.25 / GA) + tie[0:1]
        bcol_v[j * P:(j + 1) * P, :] = jnp.broadcast_to(brow, (P, P)).T

    LAG = 2

    def interleave(*lists):
        out = []
        for j in range(max(len(a) for a in lists)):
            for a in lists:
                out += a[j:j + 1]
        return out

    def p1_first(c):
        bg = _Background()
        todo = []
        if c == 3:
            todo = tasks(ln_z2, 0)
            bg.add(wcomb_gen(range(3)))
        if c == 4:
            todo = tasks(ln_x2, 2, 8)
            bg.add(wcomb_gen(range(3, 6)))
            small_setup()
        tied = _Tied(todo, 20)
        if c == 0:
            for s in range(TM // 16):
                ln_x(1, s)
        for t in range(2):
            for m in range(TM // MC):
                job_z(t, m, range(*WIN_CHUNKS[c]), bg, (80, 40), tied)
        bg.drain()
        assert not tied.tasks

    for c in range(5):
        cp_win(c).wait()
        if c == 0:
            cp_x(1).wait()
        if c == 2:
            start(cp_conv(0))
            cp_x(3).start()
        if c == 4:
            cp_x(2).wait()
            wait(cp_small())
        block(lambda c=c: p1_first(c), f'p1_f{c}')

    def p1_wait(i):
        wait(cp_conv(i - LAG))
        if i + 1 < NT:
            cp_x(i + 1).wait()
        if i == 4:
            cp_wout().wait()
        if i == NT - 3:
            wait(cp_wsp(0))

    def p1_start(i):
        if i + 2 < NT:
            cp_x(i + 2).start()
        start(cp_conv(i - LAG + 1))
        start(cp_wsp((i - 2) // 2, ((i - 2) % 2,)))
        if i == NT - 1:
            start(cp_conv(NT - 1))
        if i == 2:
            cp_wout().start()

    def take(gen, n):
        for _ in range(n):
            yield next(gen)

    def p1_step(i):
        bg = _Background()
        dft = _Background()
        t = i - LAG
        kv = kv_gen(t)
        dft.add(take(kv, (20 if t >= 1 else 10) * 64 // KV_ROWS))
        if t >= 1:
            bg.add(g_gen(t - 1))
        else:
            bg.add(take(kv, 10 * 64 // KV_ROWS))
        extra = 0
        if i == 4:
            bg.add(wocomb_gen())
            extra = 30
        if i in (NT - 3, NT - 2):
            bg.add(acomb_gen(0, range(4) if i == NT - 3 else range(4, 8)))
            extra = 20
        last = i == NT - 1
        z2t = tasks(ln_z2, i - 1)
        todo = interleave(tasks(ln_x2, i + 1, 8) if not last else [], z2t[0::2], z2t[1::2],
                          tasks(bcol_task, 0) if i == 2 else [])
        nx = 8 if (t >= 1 and TIE_X) else 0
        tied = _Tied(todo, (24 if last else TIED_N) + nx)
        dft.run(110)
        if t >= 1:
            for q in range(4):
                dft_piece('X', t - 1, q, dft, DFT_B[0], tied if TIE_X else None)
        for p in range(2):
            for j in range(FH // L):
                job_zs(i, p, j, bg, (Z_B0 + extra, Z_B1 + extra), tied)
            assert not tied.tasks or (p == 0 and not last)
            if p == 0 and last:
                tied = _Tied(tasks(ln_z2, i, 8), 22)
        if last:
            for s in range(8, 16):
                ln_z2(i, s)
        for q in range(4):
            dft_piece('H', t, q, dft, DFT_B[1])
        bg.drain()
        dft.drain()

    for i in range(2, NT):
        p1_wait(i)
        p1_start(i)
        block(lambda i=i: p1_step(i), f'p1_{i}')

    groups = P2_GROUPS
    NG = len(groups)

    def p2_dma(gi):
        if gi >= 2:
            for i in groups[gi - 2]:
                start(cp_out(i))
        if gi >= 3:
            for i in groups[gi - 3]:
                wait(cp_out(i))
        if gi + 2 < NG:
            for i in groups[gi + 2]:
                start(cp_wsp(i))
        if gi < 2:
            wait(cp_conv(NT - 2 + gi))
        if gi + 1 < NG:
            for i in groups[gi + 1]:
                wait(cp_wsp(i))

    def tails_of(i, bg, budget):
        return [tail_gen(i, bg, budget)] * 20

    def p2_block(gi):
        bg = _Background()
        steps = groups[gi]
        tb = [0.0]
        pending = [t_ for i in (groups[gi - 1] if gi > 0 else []) for t_ in tails_of(i, bg, tb)]
        total = sum(a + 1 for i in steps for a in _blocks_of_step(i)) * 40 * 16
        total += len(steps) * (24 * E_COST + 6 * U_COST) + len(pending) * T_COST
        slots = 84 * len(steps) + TAIL_W * len(pending)
        bg.add(freq_gen(_blocks_of_step(steps[0])[0]))
        if gi < 2:
            bg.add(kv_gen(NT - 2 + gi))
            total += 20 * KV_COST
            slots += 10
        if gi < 3:
            slots += 10
            bg.add(g_gen(NT - 3 + gi))
            total += 40 * G_COST
        if gi + 1 < NG:
            for i in groups[gi + 1]:
                bg.add(acomb_gen(i))
                total += 32 * A_COST
        for i in steps[1:]:
            bg.add(freq_gen(_blocks_of_step(i)[0]))
        budget = tb[0] = total / (slots + 1.0)
        bg.run(budget)
        if gi < 3:
            job_x(NT - 3 + gi, bg, budget)
        if gi < 2:
            job_h(NT - 2 + gi, bg, budget)
        units = [4, 4, 2, 4, 4, 2] * (len(pending) // 20)
        every = [0] * (6 * len(steps))
        for j, n in enumerate(units):
            every[min(len(every) - 1, j * len(every) // len(units))] += n
        for i in steps:
            job_big(i, bg, pending, budget, every)
        for t_ in pending:
            next(t_)
        bg.drain()

    for gi in range(NG):
        p2_dma(gi)
        block(lambda gi=gi: p2_block(gi), f'p2_{gi}')

    def cp_last(upper):
        a0 = _blocks_of_step(NT - 1)[0]
        return [pltpu.make_async_copy(o_v.at[pl.ds(r, MC)], o_hbm.at[0, pl.ds(r, MC)], sem_out.at[(NT - 1) % 5])
                for r in ((a0 + w) * P + (MC if upper else 0) for w in range(2))]

    def p2_last():
        for j, t_ in enumerate(tails_of(NT - 1, _Background(), [0.0])):
            next(t_)
            if j == 9:
                start(cp_last(True))

    p2_dma(NG)
    block(p2_last, 'p2_last')
    start(cp_last(False))
    for i in groups[NG - 2]:
        wait(cp_out(i))
    wait(cp_last(True))
    wait(cp_last(False))
    if _ONLY is not None:
        for r_ in (xn_u, XL_u, WB_u, UL_u, WO_u, z1_v, R_u, Lc_u, zf_v, zg_v, kv_u, u_u, X_v, H_v, G_v, Z_u, kf_v):
            c_ = pltpu.make_async_copy(r_, r_, sem_small.at[0])
            c_.start()
            c_.wait()


@jax.jit
def pallas_recurrent_scan__ssm_conv_h3__mixer_gmlp__prompt_kernel(
    A_q: jax.Array,
    A_k: jax.Array,
    A_v: jax.Array,
    A_shift_k: jax.Array,
    A_ssm_k: jax.Array,
    A_ssm_D: jax.Array,
    B_x: jax.Array,
    B_w_in: jax.Array,
    B_w_sp: jax.Array,
    B_b_sp: jax.Array,
    B_w_out: jax.Array,
):
    del B_x
    hbm = pl.BlockSpec(memory_space=pl.ANY)

    def bf16_buf(*shape):
        return pltpu.VMEM(shape[:-2] + (shape[-2] // 2, shape[-1]), U32)

    return pl.pallas_call(
        _kernel,
        out_shape=jax.ShapeDtypeStruct((1, S, D), BF16),
        in_specs=[hbm] * 10,
        out_specs=hbm,
        scratch_shapes=[
            bf16_buf(S, D),
            bf16_buf(S, D),
            bf16_buf(S, D),
            bf16_buf(NT, D, TM),
            bf16_buf(D, 2 * FH),
            bf16_buf(S, S),
            bf16_buf(FH, D),
            pltpu.VMEM((S, D), BF16),
            pltpu.VMEM((4, D), BF16),
            pltpu.VMEM((D,), BF16),
            pltpu.VMEM((S,), BF16),
            bf16_buf(S, D),
            bf16_buf(2 * 5 * P, KH),
            bf16_buf(5 * KH, FH),
            bf16_buf(4 * 5 * P, HN),
            bf16_buf(5 * HN, 2 * L),
            pltpu.VMEM((S, FH), F32),
            bf16_buf(7 * HK, HN),
            bf16_buf(4 * 5 * P, HK),
            pltpu.VMEM((HK, FH), F32),
            pltpu.VMEM((2, TM, FH), F32),
            bf16_buf(S, D),
            bf16_buf(S, FH),
            pltpu.VMEM((NB, 2, P, D), F32),
            pltpu.VMEM((6, 2, P, D), F32),
            pltpu.VMEM((NB, 2, P, D), F32),
            bf16_buf(NB * 2 * P, D),
            pltpu.VMEM((2, D // L, MC, L), F32),
            bf16_buf(2 * P, 2 * P),
            bf16_buf(MC, 2 * P),
            pltpu.VMEM((S, L), F32),
            pltpu.VMEM((2, P, L), F32),
            pltpu.VMEM((4, 8, D), F32),
            pltpu.VMEM((D // L, S + 8, L), F32),
            pltpu.SemaphoreType.DMA((1,)),
            pltpu.SemaphoreType.DMA((3,)),
            pltpu.SemaphoreType.DMA((2,)),
            pltpu.SemaphoreType.DMA((5,)),
            pltpu.SemaphoreType.DMA((5,)),
            pltpu.SemaphoreType.DMA((5,)),
        ],
        compiler_params=pltpu.CompilerParams(vmem_limit_bytes=116 * 1024 * 1024, disable_semaphore_checks=True),
    )(A_q, A_k, A_v, A_shift_k.T, A_ssm_k, A_ssm_D, B_w_in, B_w_sp, B_b_sp, B_w_out)
```

```python
import math

import jax
import jax.numpy as jnp
import jax.experimental.pallas as pl
import jax.experimental.pallas.tpu as pltpu

S = 2048
D = 640
FH = 768
P = 128
NB = S // P
TM = 256
NT = S // TM
MC = 64
L = 128
HK = S // 2
KH = 256
HN = FH // 2
P1_GROUPS = ((2,), (3,), (4, 5), (6, 7))
P1_XG = {2: None, 3: 0, 4: 1, 5: None, 6: 2, 7: 3}
P1_LNX = {2: (3,), 3: (4, 5), 4: (6,), 5: (7,), 6: (), 7: ()}
P2_XG = ((4, 5), (6,), (7,), (), ())
P2_GROUPS = ((0,), (1, 2), (3, 4), (5, 6), (7,))
STEP_BLOCKS = ((6, 7), (8, 9), (4, 5), (12, 13), (2, 3), (14, 15), (0, 1), (10, 11))
KV_COST, G_COST, A_COST = 110, 36, 56
E_COST, U_COST, T_COST, TAIL_W = 24, 90, 90, 1.6
BIG_KG = 512
TIE_X = False
DFT_B = (130, 80)
Z_B0, Z_B1 = 60, 10
TIED_N = 42
ORDER = 1
FR = 16
KV_ROWS = 64
WIN_CHUNKS = ((6, 7), (7, 9), (9, 12), (0, 3), (3, 6))
EPS = 1e-5
F32 = jnp.float32
BF16 = jnp.bfloat16
U32 = jnp.uint32
GELU_C = math.sqrt(2.0 / math.pi)
GA = (GELU_C * 0.044715) ** (1.0 / 3.0)
NT_DIMS = (((1,), (1,)), ((), ()))
_ONLY = None


def _dot(a, b):
    return jnp.dot(a, b, preferred_element_type=F32)


def _cos_sin(m):
    q = (m + 256) >> 9
    x = (m - (q << 9)).astype(F32) * (2.0 * math.pi / 2048.0)
    x2 = x * x
    s = x * (1.0 + x2 * (-1.0 / 6 + x2 * (1.0 / 120 + x2 * (-1.0 / 5040 + x2 * (1.0 / 362880)))))
    c = 1.0 + x2 * (-0.5 + x2 * (1.0 / 24 + x2 * (-1.0 / 720 + x2 * (1.0 / 40320 - x2 * (1.0 / 3628800)))))
    swap = (q & 1) == 1
    c0 = jnp.where(swap, s, c)
    s0 = jnp.where(swap, c, s)
    cos = jnp.where(((q + 1) & 2) == 2, -c0, c0)
    sin = jnp.where((q & 2) == 2, -s0, s0)
    return cos, sin


def _odd_freq(r):
    return jnp.where(r < 64, 4 * r + 1, 4 * r - 253)


def _gelu_scaled(z):
    return z + z * jnp.tanh(z * (GELU_C / GA + z * z))


def _signzero(z):
    bits = jax.lax.bitcast_convert_type(z, U32) & jnp.uint32(0x80000000)
    return jax.lax.bitcast_convert_type(bits, F32)


def _ln(x, eps, tie=None, scale=None):
    n = x.shape[-1]
    cols = [x[:, j * L:(j + 1) * L] for j in range(n // L)]
    s1 = cols[0]
    s2 = cols[0] * cols[0]
    for c in cols[1:]:
        s1 = s1 + c
        s2 = s2 + c * c
    if tie is not None:
        s1 = s1 + tie
        s2 = s2 + tie
    m = jnp.sum(s1, axis=-1, keepdims=True) * (1.0 / n)
    v = jnp.maximum(jnp.sum(s2, axis=-1, keepdims=True) * (1.0 / n) - m * m, 0.0)
    rs = jax.lax.rsqrt(v + eps)
    if scale is not None:
        rs = rs * scale
    return (x - m) * rs


def _blocks_of_step(i):
    return STEP_BLOCKS[i]


class _Background:
    def __init__(self):
        self.q = []
        self.credit = 0.0

    def add(self, gen):
        self.q.append(gen)

    def run(self, budget):
        self.credit += budget
        while self.q and self.credit > 0:
            try:
                self.credit -= next(self.q[0])
            except StopIteration:
                self.q.pop(0)
        if not self.q:
            self.credit = 0.0

    def charge(self, cost):
        self.credit -= cost

    def drain(self):
        while self.q:
            self.run(1e9)


class _Tied:
    def __init__(self, tasks, npieces):
        self.tasks = list(tasks)
        self.rate = len(self.tasks) / float(npieces)
        self.credit = 0.999

    def run(self, z):
        self.credit += self.rate
        n = 0
        while self.tasks and self.credit >= 1.0:
            self.tasks.pop(0)(_signzero(z[0:16]))
            self.credit -= 1.0
            n += 1
        return n


def _kernel(q_hbm, k_hbm, v_hbm, sk_hbm, h_hbm, d_hbm, win_hbm, wsp_hbm, b_hbm, wout_hbm,
            o_hbm,
            x_u, k_u, v_u, h_u, win_u, wsp_u, wout_u, o_v, sk_in, d_in, b_in,
            xn_u, XL_u, WB_u, UL_u, WO_u, z1_v, R_u, Lc_u, zf_v, zg_v, kv_u, u_u, X_v, H_v, G_v, Z_u, yl_v, F_u, Fi_u, bcol_v, ph_v, sk_v, kf_v,
            sem_small, sem_x, sem_conv, sem_wsp, sem_w, sem_out):
    x_v, k_v, v_v, h_v, win_v, wsp_v, wout_v, xn_v, XL_v, WB_v, UL_v, WO_v, R_v, Lc_v, kv_v, u_v, Z_v, F_v, Fi_v = [
        r.bitcast(BF16) for r in (x_u, k_u, v_u, h_u, win_u, wsp_u, wout_u, xn_u, XL_u, WB_u, UL_u, WO_u, R_u, Lc_u, kv_u, u_u, Z_u, F_u,
                                  Fi_u)]

    def cp_small():
        return [pltpu.make_async_copy(s_, d_, sem_small.at[0])
                for s_, d_ in ((d_hbm, d_in), (sk_hbm, sk_in), (b_hbm, b_in))]

    def cp_x(t):
        return pltpu.make_async_copy(q_hbm.at[0, pl.ds(t * TM, TM)], x_v.at[pl.ds(t * TM, TM)], sem_x.at[t % 5])

    def cp_conv(t):
        rows = pl.ds(t * TM, TM)
        sem = sem_conv.at[t % 4]
        return [pltpu.make_async_copy(h_hbm.at[:, rows], h_v.at[t], sem),
                pltpu.make_async_copy(k_hbm.at[0, rows], k_v.at[rows], sem),
                pltpu.make_async_copy(v_hbm.at[0, rows], v_v.at[rows], sem)]

    def cp_wsp(i, which=(0, 1)):
        return [pltpu.make_async_copy(wsp_hbm.at[pl.ds(_blocks_of_step(i)[half] * P, P)],
                                      wsp_v.at[pl.ds(i * TM + half * P, P)], sem_wsp.at[i % 5]) for half in which]

    def cp_win(c):
        lo, hi = WIN_CHUNKS[c]
        cols = pl.ds(lo * L, (hi - lo) * L)
        return pltpu.make_async_copy(win_hbm.at[:, cols], win_v.at[:, cols], sem_w.at[c])

    def cp_wout():
        return pltpu.make_async_copy(wout_hbm, wout_v, sem_w.at[0])

    def cp_out(i):
        rows = pl.ds(_blocks_of_step(i)[0] * P, TM)
        return [pltpu.make_async_copy(o_v.at[rows], o_hbm.at[0, rows], sem_out.at[i % 5])]

    def start(cs):
        for c in cs:
            c.start()

    def wait(cs):
        for c in cs:
            c.wait()

    def block(fn, name):
        def body(it):
            fn()
            return it + 1

        if _ONLY is None or name in _ONLY:
            jax.lax.while_loop(lambda it: it < 1, body, jnp.int32(0))

    def ln_x(t, s, tie=None):
        rows = pl.ds(t * TM + s * 16, 16)
        y = _ln(x_v[rows, :].astype(F32), EPS, tie, GA)
        xn_v[rows, :] = y.astype(BF16)
        return y

    def ln_x2(t, s, tie):
        p, q = s // 4, s % 4
        y1 = ln_x(t, 8 * p + q, tie)
        y2 = ln_x(t, 8 * p + 4 + q, tie)
        a11, a12, a21, a22 = y1[:, :KH], y1[:, KH:2 * KH], y2[:, :KH], y2[:, KH:2 * KH]
        r0 = (t % 4) * 5 * P + p * MC + q * 16
        for j, c in enumerate((a11 + a22, a21 + a22, a11 + a12, a21 - a11, a12 - a22)):
            XL_v[pl.ds(r0 + j * P, 16), :] = c.astype(BF16)

    def wcomb_gen(cols):
        for j in cols:
            c1 = slice(j * L, (j + 1) * L)
            c2 = slice(FH + j * L, FH + (j + 1) * L)
            for r in range(KH // 32):
                top = pl.ds(r * 32, 32)
                bot = pl.ds(KH + r * 32, 32)
                b11, b12 = win_v[top, c1].astype(F32), win_v[top, c2].astype(F32)
                b21, b22 = win_v[bot, c1].astype(F32), win_v[bot, c2].astype(F32)
                for w, c in enumerate((b11 + b22, b12 - b22, b21 - b11, b11 + b12, b21 + b22)):
                    WB_v[pl.ds(w * KH + r * 32, 32), c1] = c.astype(BF16)
                yield A_COST

    def ln_z2(t, s, tie=None):
        y = _ln(zg_v[t % 3, s * 16:(s + 1) * 16, :], 4.0 * GA * GA * EPS, tie, 0.25 / GA)
        lo, hi = y[:, :HN], y[:, HN:]
        r = (t * TM + s * 16) % HK
        rows = pl.ds(r, 16)
        if t < NT // 2:
            zf_v[rows, :] = y
            R_v[pl.ds(1 * HK + r, 16), :] = lo.astype(BF16)
            R_v[pl.ds(5 * HK + r, 16), :] = (lo + hi).astype(BF16)
        else:
            b11 = zf_v[rows, :HN]
            R_v[pl.ds(0 * HK + r, 16), :] = (b11 + hi).astype(BF16)
            R_v[pl.ds(2 * HK + r, 16), :] = (zf_v[rows, HN:] - hi).astype(BF16)
            R_v[pl.ds(3 * HK + r, 16), :] = (lo - b11).astype(BF16)
            R_v[pl.ds(4 * HK + r, 16), :] = hi.astype(BF16)
            R_v[pl.ds(6 * HK + r, 16), :] = (lo + hi).astype(BF16)

    def acomb_gen(i, groups=range(P // 16)):
        for r in groups:
            for c in range(HK // 256):
                top = pl.ds(i * TM + r * 16, 16)
                bot = pl.ds(i * TM + P + r * 16, 16)
                c1 = slice(c * 256, (c + 1) * 256)
                c2 = slice(HK + c * 256, HK + (c + 1) * 256)
                a11 = wsp_v[top, c1].astype(F32)
                a12 = wsp_v[top, c2].astype(F32)
                a21 = wsp_v[bot, c1].astype(F32)
                a22 = wsp_v[bot, c2].astype(F32)
                r0 = (i % 4) * 5 * P + r * 16
                Lc_v[pl.ds(r0 + 0 * P, 16), c1] = (a11 + a22).astype(BF16)
                Lc_v[pl.ds(r0 + 1 * P, 16), c1] = (a21 + a22).astype(BF16)
                Lc_v[pl.ds(r0 + 2 * P, 16), c1] = (a11 + a12).astype(BF16)
                Lc_v[pl.ds(r0 + 3 * P, 16), c1] = (a21 - a11).astype(BF16)
                Lc_v[pl.ds(r0 + 4 * P, 16), c1] = (a12 - a22).astype(BF16)
                yield A_COST

    def tasks(fn, t, n=TM // 16):
        return [lambda tie, s=s: fn(t, s, tie) for s in range(n)]

    def kv_gen(t):
        for m in range(TM // KV_ROWS):
            r = t * TM + m * KV_ROWS
            for l in range(D // L):
                lanes = slice(l * L, (l + 1) * L)
                kf = k_v[pl.ds(r, KV_ROWS), lanes].astype(F32)
                kf_v[l, pl.ds(r + 8, KV_ROWS), :] = kf
                ks = kf * sk_v[0, 0:1, lanes]
                for tap in range(1, 4):
                    ks = ks + kf_v[l, pl.ds(r + 8 - tap, KV_ROWS), :] * sk_v[tap, 0:1, lanes]
                kv = ks * v_v[pl.ds(r, KV_ROWS), lanes].astype(F32)
                kv_v[pl.ds(r, KV_ROWS), lanes] = kv.astype(BF16)
                yield KV_COST * KV_ROWS / 64

    def g_gen(t):
        for r in range(P // 16):
            rows = pl.ds(r * 16, 16)
            for l in range(D // L):
                lanes = slice(l * L, (l + 1) * L)
                h = [(H_v[(2 * t + w) % 10, 0, rows, lanes], H_v[(2 * t + w) % 10, 1, rows, lanes]) for w in range(3)]
                for w in range(2):
                    (pr, pi), (cr, ci) = h[w], h[w + 1]
                    G_v[2 * t + w, 0, rows, lanes] = cr - pi if r < P // 32 else cr + pi
                    G_v[2 * t + w, 1, rows, lanes] = ci + pr if r < P // 32 else ci - pr
                yield G_COST

    def freq_gen(a):
        def cmac(acc, x, g):
            pr = x[0] * g[0] - x[1] * g[1]
            pi = x[0] * g[1] + x[1] * g[0]
            return (pr, pi) if acc is None else (acc[0] + pr, acc[1] + pi)

        for r in range(P // 16):
            for l in range(D // L):
                lanes = slice(l * L, (l + 1) * L)
                res = []
                for sub in range(16 // FR):
                    rows = pl.ds(r * 16 + sub * FR, FR)
                    lo = hi = None
                    g = (G_v[a + 1, 0, rows, lanes], G_v[a + 1, 1, rows, lanes])
                    for c in range(a + 2):
                        x = (X_v[c, 0, rows, lanes], X_v[c, 1, rows, lanes])
                        hi = cmac(hi, x, g)
                        if c <= a:
                            g = (G_v[a - c, 0, rows, lanes], G_v[a - c, 1, rows, lanes])
                            lo = cmac(lo, x, g)
                            yield 2 * FR
                    res.append((lo, hi))
                for w in range(2):
                    for part in range(2):
                        Z_v[pl.ds((a + w) * 2 * P + part * P + r * 16, 16), lanes] = jnp.concatenate(
                            [z[w][part] for z in res], axis=0).astype(BF16)
                yield 20

    def dft_piece(kind, t, q, bg, budget, tied=None):
        j, half = q // 2, q % 2
        f = F_v[half * P:(half + 1) * P, 0:P]
        if kind == 'H':
            r = jax.lax.dot_general(f, h_v[t, :, j * P:(j + 1) * P], NT_DIMS, preferred_element_type=F32)
            dst, idx = H_v, (2 * t + j + 1) % 10
        else:
            r = _dot(f, kv_v[(2 * t + j) * P:(2 * t + j + 1) * P, :])
            dst, idx = X_v, 2 * t + j
        r4 = r.reshape(8, 2, 8, D)
        for part in range(2):
            dst[idx, part, half * 64:(half + 1) * 64, :] = r4[:, part].reshape(64, D)
        if tied is not None:
            tied.run(r[:, 0:L])
            tied.run(r[:, 2 * L:3 * L])
        bg.run(budget * 2.5)

    def job_h(t, bg, budget):
        for q in range(4):
            dft_piece('H', t, q, bg, budget)

    def job_x(t, bg, budget):
        for q in range(4):
            dft_piece('X', t, q, bg, budget)

    def z_out(t, m, n, pre, bg, budget, tied):
        z = _gelu_scaled(pre)
        if n < FH // L:
            z1_v[pl.ds(t * TM + m * MC, MC), n * L:(n + 1) * L] = z
        else:
            zg_v[t % 3, m * MC:(m + 1) * MC, n * L - FH:(n + 1) * L - FH] = z
        ntask = tied.run(z)
        bg.run(budget[1] if ntask else budget[0])

    def job_z(t, m, cols, bg, budget, tied):
        for n in cols:
            z_out(t, m, n, _dot(xn_v[pl.ds(t * TM + m * MC, MC), :], win_v[:, n * L:(n + 1) * L]), bg, budget, tied)

    def job_zs(t, p, j, bg, budget, tied):
        r1 = pl.ds(t * TM + p * P, MC)
        r2 = pl.ds(t * TM + p * P + MC, MC)
        c1 = slice(j * L, (j + 1) * L)
        c2 = slice(FH + j * L, FH + (j + 1) * L)

        def xl(w):
            r0 = (t % 4) * 5 * P + w * P + p * MC
            return XL_v[r0:r0 + MC, :]

        def wb(w):
            return WB_v[w * KH:(w + 1) * KH, c1]

        def rem(rows, cols):
            return _dot(xn_v[rows, 2 * KH:], win_v[2 * KH:, cols])

        m2 = _dot(xl(1), win_v[0:KH, c1])
        m4 = _dot(xn_v[r2, KH:2 * KH], wb(2))
        z_out(t, 2 * p + 1, j, m2 + m4 + rem(r2, c1), bg, budget, tied)
        m3 = _dot(xn_v[r1, 0:KH], wb(1))
        m5 = _dot(xl(2), win_v[KH:2 * KH, c2])
        z_out(t, 2 * p, 6 + j, m3 + m5 + rem(r1, c2), bg, budget, tied)
        m1 = _dot(xl(0), wb(0))
        z_out(t, 2 * p, j, (m4 - m5) + m1 + _dot(xl(4), wb(4)) + rem(r1, c1), bg, budget, tied)
        z_out(t, 2 * p + 1, 6 + j, (m3 - m2) + m1 + _dot(xl(3), wb(3)) + rem(r2, c2), bg, budget, tied)

    rev8 = 7 - jax.lax.broadcasted_iota(jnp.int32, (8, L), 0)

    def finish(a, upper, n, hh, slot):
        rows = pl.ds(a * P + (MC if upper else 0), MC)
        lanes = slice(n * L, (n + 1) * L)
        if upper:
            ya = _dot(Fi_v[:, 0:P], Z_v[a * 2 * P:a * 2 * P + P, lanes])
            yb = _dot(Fi_v[:, P:2 * P], Z_v[a * 2 * P + P:(a + 1) * 2 * P, lanes])
            slot(0.5)
            y = ya - yb
            lo = ya + yb
            for j in range(MC // 8):
                yl_v[a % 2, n, (7 - j) * 8:(8 - j) * 8, :] = jnp.take_along_axis(lo[j * 8:(j + 1) * 8], rev8, axis=0)
        else:
            y = yl_v[a % 2, n]
        gate = hh + hh * jnp.tanh(hh)
        s = xn_v[rows, lanes].astype(F32) * y
        o_v[rows, lanes] = (x_v[rows, lanes].astype(F32) + s * gate).astype(BF16)

    def tail_gen(i, bg, budget):
        a0, a1 = _blocks_of_step(i)

        def slot(w):
            bg.run(w * budget[0])

        def dot3(a, b):
            r = _dot(a, b)
            slot(0.75)
            return r

        for upper in (True, False):
            sub = MC if upper else 0
            r1 = pl.ds(a0 * P + sub, MC)
            r2 = pl.ds(a1 * P + sub, MC)

            def ul(w):
                r0 = ((i % 4) * 5 + w) * P + sub
                return UL_v[r0:r0 + MC, :]

            for j in range(2):
                c1 = slice(j * L, (j + 1) * L)
                c2 = slice((2 + j) * L, (3 + j) * L)

                def wo(w):
                    return WO_v[w * HN:(w + 1) * HN, c1]

                m2 = dot3(ul(1), wout_v[0:HN, c1])
                m4 = dot3(u_v[r2, HN:], wo(2))
                finish(a1, upper, j, m2 + m4, slot)
                bg.charge(T_COST)
                yield
                m3 = dot3(u_v[r1, 0:HN], wo(1))
                m5 = dot3(ul(2), wout_v[HN:, c2])
                finish(a0, upper, 2 + j, m3 + m5, slot)
                bg.charge(T_COST)
                yield
                m1 = dot3(ul(0), wo(0))
                finish(a0, upper, j, (m4 - m5) + m1 + dot3(ul(4), wo(4)), slot)
                bg.charge(T_COST)
                yield
                finish(a1, upper, 2 + j, (m3 - m2) + m1 + dot3(ul(3), wo(3)), slot)
                bg.charge(T_COST)
                yield
            finish(a0, upper, 4, dot3(u_v[r1, 0:HN], wout_v[0:HN, 4 * L:]) + dot3(u_v[r1, HN:], wout_v[HN:, 4 * L:]), slot)
            bg.charge(T_COST)
            yield
            finish(a1, upper, 4, dot3(u_v[r2, 0:HN], wout_v[0:HN, 4 * L:]) + dot3(u_v[r2, HN:], wout_v[HN:, 4 * L:]), slot)
            bg.charge(T_COST)
            yield

    def wocomb_gen():
        for j in range(2):
            c1 = slice(j * L, (j + 1) * L)
            c2 = slice((2 + j) * L, (3 + j) * L)
            for r in range(HN // 32):
                top = pl.ds(r * 32, 32)
                bot = pl.ds(HN + r * 32, 32)
                b11, b12 = wout_v[top, c1].astype(F32), wout_v[top, c2].astype(F32)
                b21, b22 = wout_v[bot, c1].astype(F32), wout_v[bot, c2].astype(F32)
                for w, c in enumerate((b11 + b22, b12 - b22, b21 - b11, b11 + b12, b21 + b22)):
                    WO_v[pl.ds(w * HN + r * 32, 32), c1] = c.astype(BF16)
                yield A_COST

    def job_big(i, bg, pending, budget, every):
        a0, a1 = _blocks_of_step(i)
        KG = BIG_KG

        def lhs(j, sub, cols):
            if j == 2:
                return wsp_v[i * TM + sub:i * TM + sub + MC, cols]
            if j == 3:
                return wsp_v[i * TM + P + sub:i * TM + P + sub + MC, HK + cols.start:HK + cols.stop]
            r0 = ((i % 4) * 5 + {0: 0, 1: 1, 4: 2, 5: 3, 6: 4}[j]) * P + sub
            return Lc_v[r0:r0 + MC, cols]

        def prod(j, sub, n, acc=None):
            for kg in range(HK // KG):
                ks = slice(kg * KG, (kg + 1) * KG)
                p = _dot(lhs(j, sub, ks), R_v[j * HK + kg * KG:j * HK + (kg + 1) * KG, n * L:(n + 1) * L])
                acc = p if acc is None else acc + p
                bg.run(budget * KG / 512)
            return acc

        def tails(n):
            for _ in range(n):
                if pending:
                    next(pending.pop(0))

        def emit(a, sub, n, g):
            rows = pl.ds(a * P + sub, MC)
            lanes = slice(n * L, (n + 1) * L)
            u = z1_v[rows, lanes] * (g + bcol_v[rows, :])
            u_v[rows, lanes] = u.astype(BF16)
            bg.charge(E_COST)
            return u

        for sub in (0, MC):
            for n in range(HN // L):
                def put(w, c):
                    UL_v[pl.ds(((i % 4) * 5 + w) * P + sub, MC), n * L:(n + 1) * L] = c.astype(BF16)

                if ORDER == 0:
                    m2 = prod(1, sub, n)
                    m4 = prod(3, sub, n)
                    u21 = emit(a1, sub, n, m2 + m4)
                    m3 = prod(2, sub, n)
                    t22 = m3 - m2
                    m5 = prod(4, sub, n)
                    u12 = emit(a0, sub, n + HN // L, m3 + m5)
                    t11 = m4 - m5
                    m1 = prod(0, sub, n)
                    u11 = emit(a0, sub, n, prod(6, sub, n, t11 + m1))
                    u22 = emit(a1, sub, n + HN // L, prod(5, sub, n, t22 + m1))
                    for w, c in enumerate((u11 + u22, u21 + u22, u11 + u12, u21 - u11, u12 - u22)):
                        put(w, c)
                else:
                    m1 = prod(0, sub, n)
                    t11 = prod(6, sub, n, m1)
                    m4 = prod(3, sub, n)
                    t11 = t11 + m4
                    m5 = prod(4, sub, n)
                    u11 = emit(a0, sub, n, t11 - m5)
                    m2 = prod(1, sub, n)
                    u21 = emit(a1, sub, n, m2 + m4)
                    put(3, u21 - u11)
                    t22 = m1 - m2
                    m3 = prod(2, sub, n)
                    u12 = emit(a0, sub, n + HN // L, m3 + m5)
                    put(2, u11 + u12)
                    u22 = emit(a1, sub, n + HN // L, prod(5, sub, n, t22 + m3))
                    put(0, u11 + u22)
                    put(1, u21 + u22)
                    put(4, u12 - u22)
                bg.charge(U_COST)
                tails(every.pop(0))

    if _ONLY is not None:
        for r_ in (xn_u, XL_u, WB_u, UL_u, WO_u, z1_v, R_u, Lc_u, zf_v, zg_v, kv_u, u_u, X_v, H_v, G_v, Z_u, kf_v):
            c_ = pltpu.make_async_copy(r_, r_, sem_small.at[0])
            c_.start()
            c_.wait()

    cp_x(0).start()
    cp_win(0).start()
    cp_x(1).start()
    for c in range(1, 5):
        cp_win(c).start()
    cp_x(2).start()
    start(cp_small())

    kk = _odd_freq(jax.lax.broadcasted_iota(jnp.int32, (P, P), 0))
    nn = jax.lax.broadcasted_iota(jnp.int32, (P, P), 1)
    fc, fs = _cos_sin((kk * (4 * nn - 127)) & 2047)
    for g in range(P // 8):
        F_v[g * 16:(g + 1) * 16, 0:P] = jnp.concatenate(
            [fc[g * 8:(g + 1) * 8], -fs[g * 8:(g + 1) * 8]], axis=0).astype(BF16)
    fc, fs = _cos_sin((kk * (-127)) & 2047)
    ph_v[0] = fc
    ph_v[1] = fs
    kk = _odd_freq(jax.lax.broadcasted_iota(jnp.int32, (MC, P), 1))
    mm = jax.lax.broadcasted_iota(jnp.int32, (MC, P), 0)
    ic, is_ = _cos_sin((kk * (4 * mm + 2)) & 2047)
    Fi_v[:, 0:P] = (ic * (1.0 / (P * GA))).astype(BF16)
    Fi_v[:, P:2 * P] = (is_ * (1.0 / (P * GA))).astype(BF16)
    kf_v[:, 0:8, :] = jnp.zeros((D // L, 8, L), F32)

    cp_x(0).wait()
    for s in range(TM // 16):
        ln_x(0, s)

    def small_setup():
        sk = sk_in[...].astype(F32)
        for t in range(4):
            sk_v[t] = jnp.broadcast_to(sk[t:t + 1], (8, D))
        drow = d_in[...].astype(F32).reshape(1, D)
        for l in range(D // L):
            lanes = slice(l * L, (l + 1) * L)
            dre = ph_v[0] * drow[:, lanes]
            dim = ph_v[1] * drow[:, lanes]
            H_v[0, 0, 0:64, lanes] = -dim[0:64]
            H_v[0, 0, 64:P, lanes] = dim[64:P]
            H_v[0, 1, 0:64, lanes] = -dre[0:64]
            H_v[0, 1, 64:P, lanes] = dre[64:P]

    def bcol_task(t, j, tie):
        brow = b_in[...].astype(F32).reshape(1, S)[:, j * P:(j + 1) * P] * (0.25 / GA) + tie[0:1]
        bcol_v[j * P:(j + 1) * P, :] = jnp.broadcast_to(brow, (P, P)).T

    LAG = 2

    def interleave(*lists):
        out = []
        for j in range(max(len(a) for a in lists)):
            for a in lists:
                out += a[j:j + 1]
        return out

    def p1_first(c):
        bg = _Background()
        todo = []
        if c == 3:
            todo = tasks(ln_z2, 0)
            bg.add(wcomb_gen(range(3)))
        if c == 4:
            todo = tasks(ln_x2, 2, 8)
            bg.add(wcomb_gen(range(3, 6)))
            small_setup()
        tied = _Tied(todo, 20)
        if c == 0:
            for s in range(TM // 16):
                ln_x(1, s)
        for t in range(2):
            for m in range(TM // MC):
                job_z(t, m, range(*WIN_CHUNKS[c]), bg, (80, 40), tied)
        bg.drain()
        assert not tied.tasks

    for c in range(5):
        cp_win(c).wait()
        if c == 0:
            cp_x(1).wait()
        if c == 2:
            start(cp_conv(0))
            cp_x(3).start()
        if c == 4:
            cp_x(2).wait()
            wait(cp_small())
            cp_x(4).start()
            cp_x(5).start()
        block(lambda c=c: p1_first(c), f'p1_f{c}')

    def p1_dma(g):
        if g == 0:
            wait(cp_conv(0))
            cp_x(3).wait()
            start(cp_conv(1))
            cp_x(6).start()
            cp_x(7).start()
            start(cp_conv(2))
        if g == 1:
            wait(cp_conv(1))
            cp_x(4).wait()
            cp_x(5).wait()
            start(cp_conv(3))
            start(cp_conv(4))
        if g == 2:
            wait(cp_conv(2))
            wait(cp_conv(3))
            cp_x(6).wait()
            cp_x(7).wait()
            start(cp_conv(5))
            cp_wout().start()
            start(cp_wsp(0))
            start(cp_wsp(1))
        if g == 3:
            wait(cp_conv(4))
            wait(cp_conv(5))
            cp_wout().wait()
            wait(cp_wsp(0))
            start(cp_conv(6))
            start(cp_wsp(2))
            start(cp_conv(7))

    def take(gen, n):
        for _ in range(n):
            yield next(gen)

    def p1_step(i):
        bg = _Background()
        dft = _Background()
        t = i - LAG
        xg = P1_XG[i]
        kv = kv_gen(t)
        dft.add(take(kv, (10 if xg is None else 20) * 64 // KV_ROWS))
        if xg is not None:
            bg.add(g_gen(xg))
        else:
            bg.add(take(kv, 10 * 64 // KV_ROWS))
        extra = 0
        if i == 6:
            bg.add(wocomb_gen())
            bg.add(acomb_gen(0, range(3)))
            extra = 42
        if i == 7:
            bg.add(acomb_gen(0, range(3, 8)))
            extra = 24
        last = i == NT - 1
        z2t = tasks(ln_z2, i - 1)
        todo = interleave(*([tasks(ln_x2, t_, 8) for t_ in P1_LNX[i]] + [z2t[0::2], z2t[1::2]] +
                            [tasks(bcol_task, 0) if i == 2 else []]))
        nx = 8 if (t >= 1 and TIE_X) else 0
        tied = _Tied(todo, (24 if last else TIED_N) + nx)
        dft.run(110)
        if xg is not None:
            for q in range(4):
                dft_piece('X', xg, q, dft, DFT_B[0], tied if TIE_X else None)
        for p in range(2):
            for j in range(FH // L):
                job_zs(i, p, j, bg, (Z_B0 + extra, Z_B1 + extra), tied)
            assert not tied.tasks or (p == 0 and not last)
            if p == 0 and last:
                tied = _Tied(tasks(ln_z2, i, 8), 22)
        if last:
            for s in range(8, 16):
                ln_z2(i, s)
        for q in range(4):
            dft_piece('H', t, q, dft, DFT_B[1])
        bg.drain()
        dft.drain()

    def p1_block(g):
        for i in P1_GROUPS[g]:
            p1_step(i)

    for g in range(len(P1_GROUPS)):
        p1_dma(g)
        block(lambda g=g: p1_block(g), f'p1_g{g}')

    groups = P2_GROUPS
    NG = len(groups)

    def p2_dma(gi):
        if gi >= 2:
            for i in groups[gi - 2]:
                start(cp_out(i))
        if gi >= 3:
            for i in groups[gi - 3]:
                wait(cp_out(i))
        if gi + 2 < NG:
            for i in groups[gi + 2]:
                start(cp_wsp(i))
        if gi < 2:
            wait(cp_conv(NT - 2 + gi))
        if gi + 1 < NG:
            for i in groups[gi + 1]:
                wait(cp_wsp(i))

    def tails_of(i, bg, budget):
        return [tail_gen(i, bg, budget)] * 20

    def p2_block(gi):
        bg = _Background()
        steps = groups[gi]
        tb = [0.0]
        pending = [t_ for i in (groups[gi - 1] if gi > 0 else []) for t_ in tails_of(i, bg, tb)]
        total = sum(a + 1 for i in steps for a in _blocks_of_step(i)) * 40 * 16
        total += len(steps) * (24 * E_COST + 6 * U_COST) + len(pending) * T_COST
        slots = 84 * len(steps) + TAIL_W * len(pending)
        bg.add(freq_gen(_blocks_of_step(steps[0])[0]))
        if gi < 2:
            bg.add(kv_gen(NT - 2 + gi))
            total += 20 * KV_COST
            slots += 10
        for t in P2_XG[gi]:
            slots += 10
            bg.add(g_gen(t))
            total += 40 * G_COST
        if gi + 1 < NG:
            for i in groups[gi + 1]:
                bg.add(acomb_gen(i))
                total += 32 * A_COST
        for i in steps[1:]:
            bg.add(freq_gen(_blocks_of_step(i)[0]))
        budget = tb[0] = total / (slots + 1.0)
        bg.run(budget)
        for t in P2_XG[gi]:
            job_x(t, bg, budget)
        if gi < 2:
            job_h(NT - 2 + gi, bg, budget)
        units = [4, 4, 2, 4, 4, 2] * (len(pending) // 20)
        every = [0] * (6 * len(steps))
        for j, n in enumerate(units):
            every[min(len(every) - 1, j * len(every) // len(units))] += n
        for i in steps:
            job_big(i, bg, pending, budget, every)
        for t_ in pending:
            next(t_)
        bg.drain()

    for gi in range(NG):
        p2_dma(gi)
        block(lambda gi=gi: p2_block(gi), f'p2_{gi}')

    def cp_last(upper):
        a0 = _blocks_of_step(NT - 1)[0]
        return [pltpu.make_async_copy(o_v.at[pl.ds(r, MC)], o_hbm.at[0, pl.ds(r, MC)], sem_out.at[(NT - 1) % 5])
                for r in ((a0 + w) * P + (MC if upper else 0) for w in range(2))]

    def p2_last():
        for j, t_ in enumerate(tails_of(NT - 1, _Background(), [0.0])):
            next(t_)
            if j == 9:
                start(cp_last(True))

    p2_dma(NG)
    block(p2_last, 'p2_last')
    start(cp_last(False))
    for i in groups[NG - 2]:
        wait(cp_out(i))
    wait(cp_last(True))
    wait(cp_last(False))
    if _ONLY is not None:
        for r_ in (xn_u, XL_u, WB_u, UL_u, WO_u, z1_v, R_u, Lc_u, zf_v, zg_v, kv_u, u_u, X_v, H_v, G_v, Z_u, kf_v):
            c_ = pltpu.make_async_copy(r_, r_, sem_small.at[0])
            c_.start()
            c_.wait()


@jax.jit
def pallas_recurrent_scan__ssm_conv_h3__mixer_gmlp__prompt_kernel(
    A_q: jax.Array,
    A_k: jax.Array,
    A_v: jax.Array,
    A_shift_k: jax.Array,
    A_ssm_k: jax.Array,
    A_ssm_D: jax.Array,
    B_x: jax.Array,
    B_w_in: jax.Array,
    B_w_sp: jax.Array,
    B_b_sp: jax.Array,
    B_w_out: jax.Array,
):
    del B_x
    hbm = pl.BlockSpec(memory_space=pl.ANY)

    def bf16_buf(*shape):
        return pltpu.VMEM(shape[:-2] + (shape[-2] // 2, shape[-1]), U32)

    return pl.pallas_call(
        _kernel,
        out_shape=jax.ShapeDtypeStruct((1, S, D), BF16),
        in_specs=[hbm] * 10,
        out_specs=hbm,
        scratch_shapes=[
            bf16_buf(S, D),
            bf16_buf(S, D),
            bf16_buf(S, D),
            bf16_buf(NT, D, TM),
            bf16_buf(D, 2 * FH),
            bf16_buf(S, S),
            bf16_buf(FH, D),
            pltpu.VMEM((S, D), BF16),
            pltpu.VMEM((4, D), BF16),
            pltpu.VMEM((D,), BF16),
            pltpu.VMEM((S,), BF16),
            bf16_buf(S, D),
            bf16_buf(4 * 5 * P, KH),
            bf16_buf(5 * KH, FH),
            bf16_buf(4 * 5 * P, HN),
            bf16_buf(5 * HN, 2 * L),
            pltpu.VMEM((S, FH), F32),
            bf16_buf(7 * HK, HN),
            bf16_buf(4 * 5 * P, HK),
            pltpu.VMEM((HK, FH), F32),
            pltpu.VMEM((3, TM, FH), F32),
            bf16_buf(S, D),
            bf16_buf(S, FH),
            pltpu.VMEM((NB, 2, P, D), F32),
            pltpu.VMEM((10, 2, P, D), F32),
            pltpu.VMEM((NB, 2, P, D), F32),
            bf16_buf(NB * 2 * P, D),
            pltpu.VMEM((2, D // L, MC, L), F32),
            bf16_buf(2 * P, 2 * P),
            bf16_buf(MC, 2 * P),
            pltpu.VMEM((S, L), F32),
            pltpu.VMEM((2, P, L), F32),
            pltpu.VMEM((4, 8, D), F32),
            pltpu.VMEM((D // L, S + 8, L), F32),
            pltpu.SemaphoreType.DMA((1,)),
            pltpu.SemaphoreType.DMA((5,)),
            pltpu.SemaphoreType.DMA((4,)),
            pltpu.SemaphoreType.DMA((5,)),
            pltpu.SemaphoreType.DMA((5,)),
            pltpu.SemaphoreType.DMA((5,)),
        ],
        compiler_params=pltpu.CompilerParams(vmem_limit_bytes=116 * 1024 * 1024, disable_semaphore_checks=True),
    )(A_q, A_k, A_v, A_shift_k.T, A_ssm_k, A_ssm_D, B_w_in, B_w_sp, B_b_sp, B_w_out)
```

```python
import math

import jax
import jax.numpy as jnp
import jax.experimental.pallas as pl
import jax.experimental.pallas.tpu as pltpu

S = 2048
D = 640
FH = 768
P = 128
NB = S // P
TM = 256
NT = S // TM
MC = 64
L = 128
HK = S // 2
KH = 256
HN = FH // 2
P1_GROUPS = ((2,), (3,), (4, 5), (6, 7))
P1_XG = {2: None, 3: 0, 4: 1, 5: None, 6: 2, 7: 3}
P1_LNX = {2: (3,), 3: (4, 5), 4: (6,), 5: (7,), 6: (), 7: ()}
P2_XG = ((4, 5), (6,), (7,), (), ())
P2_GROUPS = ((0,), (1, 2), (3, 4), (5, 6), (7,))
STEP_BLOCKS = ((6, 7), (8, 9), (4, 5), (12, 13), (2, 3), (14, 15), (0, 1), (10, 11))
KV_COST, G_COST, A_COST = 110, 36, 56
E_COST, U_COST, T_COST, TAIL_W = 24, 90, 90, 1.6
BIG_KG = 512
TIE_X = False
DFT_B = (130, 80)
Z_B0, Z_B1 = 60, 10
TIED_N = 42
ORDER = 1
ZS_MID = 0.0
H_SPLIT = ((0, 2), (2, 4), (4, 5))
KV_SPLIT = (12, 4, 4)
FR = 16
KV_ROWS = 64
WIN_CHUNKS = ((6, 7), (7, 9), (9, 12), (0, 3), (3, 6))
EPS = 1e-5
F32 = jnp.float32
BF16 = jnp.bfloat16
U32 = jnp.uint32
GELU_C = math.sqrt(2.0 / math.pi)
GA = (GELU_C * 0.044715) ** (1.0 / 3.0)
NT_DIMS = (((1,), (1,)), ((), ()))
_ONLY = None


def _dot(a, b):
    return jnp.dot(a, b, preferred_element_type=F32)


def _cos_sin(m):
    q = (m + 256) >> 9
    x = (m - (q << 9)).astype(F32) * (2.0 * math.pi / 2048.0)
    x2 = x * x
    s = x * (1.0 + x2 * (-1.0 / 6 + x2 * (1.0 / 120 + x2 * (-1.0 / 5040 + x2 * (1.0 / 362880)))))
    c = 1.0 + x2 * (-0.5 + x2 * (1.0 / 24 + x2 * (-1.0 / 720 + x2 * (1.0 / 40320 - x2 * (1.0 / 3628800)))))
    swap = (q & 1) == 1
    c0 = jnp.where(swap, s, c)
    s0 = jnp.where(swap, c, s)
    cos = jnp.where(((q + 1) & 2) == 2, -c0, c0)
    sin = jnp.where((q & 2) == 2, -s0, s0)
    return cos, sin


def _odd_freq(r):
    return jnp.where(r < 64, 4 * r + 1, 4 * r - 253)


def _gelu_scaled(z):
    return z + z * jnp.tanh(z * (GELU_C / GA + z * z))


def _signzero(z):
    bits = jax.lax.bitcast_convert_type(z, U32) & jnp.uint32(0x80000000)
    return jax.lax.bitcast_convert_type(bits, F32)


def _ln(x, eps, tie=None, scale=None):
    n = x.shape[-1]
    cols = [x[:, j * L:(j + 1) * L] for j in range(n // L)]
    s1 = cols[0]
    s2 = cols[0] * cols[0]
    for c in cols[1:]:
        s1 = s1 + c
        s2 = s2 + c * c
    if tie is not None:
        s1 = s1 + tie
        s2 = s2 + tie
    m = jnp.sum(s1, axis=-1, keepdims=True) * (1.0 / n)
    v = jnp.maximum(jnp.sum(s2, axis=-1, keepdims=True) * (1.0 / n) - m * m, 0.0)
    rs = jax.lax.rsqrt(v + eps)
    if scale is not None:
        rs = rs * scale
    return (x - m) * rs


def _blocks_of_step(i):
    return STEP_BLOCKS[i]


class _Background:
    def __init__(self):
        self.q = []
        self.credit = 0.0

    def add(self, gen):
        self.q.append(gen)

    def run(self, budget):
        self.credit += budget
        while self.q and self.credit > 0:
            try:
                self.credit -= next(self.q[0])
            except StopIteration:
                self.q.pop(0)
        if not self.q:
            self.credit = 0.0

    def charge(self, cost):
        self.credit -= cost

    def drain(self):
        while self.q:
            self.run(1e9)


class _Tied:
    def __init__(self, tasks, npieces):
        self.tasks = list(tasks)
        self.rate = len(self.tasks) / float(npieces)
        self.credit = 0.999

    def run(self, z):
        self.credit += self.rate
        n = 0
        while self.tasks and self.credit >= 1.0:
            self.tasks.pop(0)(_signzero(z[0:16]))
            self.credit -= 1.0
            n += 1
        return n


def _kernel(q_hbm, k_hbm, v_hbm, sk_hbm, h_hbm, d_hbm, win_hbm, wsp_hbm, b_hbm, wout_hbm,
            o_hbm,
            x_u, k_u, v_u, h_u, win_u, wsp_u, wout_u, o_v, sk_in, d_in, b_in,
            xn_u, XL_u, WB_u, UL_u, WO_u, z1_v, R_u, Lc_u, zf_v, zg_v, kv_u, u_u, X_v, H_v, G_v, Z_u, yl_v, F_u, Fi_u, bcol_v, ph_v, sk_v, kf_v,
            sem_small, sem_x, sem_conv, sem_wsp, sem_w, sem_out):
    x_v, k_v, v_v, h_v, win_v, wsp_v, wout_v, xn_v, XL_v, WB_v, UL_v, WO_v, R_v, Lc_v, kv_v, u_v, Z_v, F_v, Fi_v = [
        r.bitcast(BF16) for r in (x_u, k_u, v_u, h_u, win_u, wsp_u, wout_u, xn_u, XL_u, WB_u, UL_u, WO_u, R_u, Lc_u, kv_u, u_u, Z_u, F_u,
                                  Fi_u)]

    def cp_small():
        return [pltpu.make_async_copy(s_, d_, sem_small.at[0])
                for s_, d_ in ((d_hbm, d_in), (sk_hbm, sk_in), (b_hbm, b_in))]

    def cp_x(t):
        return pltpu.make_async_copy(q_hbm.at[0, pl.ds(t * TM, TM)], x_v.at[pl.ds(t * TM, TM)], sem_x.at[t % 5])

    def cp_conv(t):
        rows = pl.ds(t * TM, TM)
        sem = sem_conv.at[t % 4]
        return [pltpu.make_async_copy(h_hbm.at[:, rows], h_v.at[t], sem),
                pltpu.make_async_copy(k_hbm.at[0, rows], k_v.at[rows], sem),
                pltpu.make_async_copy(v_hbm.at[0, rows], v_v.at[rows], sem)]

    def cp_wsp(i, which=(0, 1)):
        return [pltpu.make_async_copy(wsp_hbm.at[pl.ds(_blocks_of_step(i)[half] * P, P)],
                                      wsp_v.at[pl.ds(i * TM + half * P, P)], sem_wsp.at[i % 5]) for half in which]

    def cp_win(c):
        lo, hi = WIN_CHUNKS[c]
        cols = pl.ds(lo * L, (hi - lo) * L)
        return pltpu.make_async_copy(win_hbm.at[:, cols], win_v.at[:, cols], sem_w.at[c])

    def cp_wout():
        return pltpu.make_async_copy(wout_hbm, wout_v, sem_w.at[0])

    def cp_out(i):
        rows = pl.ds(_blocks_of_step(i)[0] * P, TM)
        return [pltpu.make_async_copy(o_v.at[rows], o_hbm.at[0, rows], sem_out.at[i % 5])]

    def start(cs):
        for c in cs:
            c.start()

    def wait(cs):
        for c in cs:
            c.wait()

    def block(fn, name):
        def body(it):
            fn()
            return it + 1

        if _ONLY is None or name in _ONLY:
            jax.lax.while_loop(lambda it: it < 1, body, jnp.int32(0))

    def ln_x(t, s, tie=None):
        rows = pl.ds(t * TM + s * 16, 16)
        y = _ln(x_v[rows, :].astype(F32), EPS, tie, GA)
        xn_v[rows, :] = y.astype(BF16)
        return y

    def ln_x2(t, s, tie):
        p, q = s // 4, s % 4
        y1 = ln_x(t, 8 * p + q, tie)
        y2 = ln_x(t, 8 * p + 4 + q, tie)
        a11, a12, a21, a22 = y1[:, :KH], y1[:, KH:2 * KH], y2[:, :KH], y2[:, KH:2 * KH]
        r0 = (t % 4) * 5 * P + p * MC + q * 16
        for j, c in enumerate((a11 + a22, a21 + a22, a11 + a12, a21 - a11, a12 - a22)):
            XL_v[pl.ds(r0 + j * P, 16), :] = c.astype(BF16)

    def wcomb_gen(cols):
        for j in cols:
            c1 = slice(j * L, (j + 1) * L)
            c2 = slice(FH + j * L, FH + (j + 1) * L)
            for r in range(KH // 32):
                top = pl.ds(r * 32, 32)
                bot = pl.ds(KH + r * 32, 32)
                b11, b12 = win_v[top, c1].astype(F32), win_v[top, c2].astype(F32)
                b21, b22 = win_v[bot, c1].astype(F32), win_v[bot, c2].astype(F32)
                for w, c in enumerate((b11 + b22, b12 - b22, b21 - b11, b11 + b12, b21 + b22)):
                    WB_v[pl.ds(w * KH + r * 32, 32), c1] = c.astype(BF16)
                yield A_COST

    def ln_z2(t, s, tie=None):
        y = _ln(zg_v[t % 3, s * 16:(s + 1) * 16, :], 4.0 * GA * GA * EPS, tie, 0.25 / GA)
        lo, hi = y[:, :HN], y[:, HN:]
        r = (t * TM + s * 16) % HK
        rows = pl.ds(r, 16)
        if t < NT // 2:
            zf_v[rows, :] = y
            R_v[pl.ds(1 * HK + r, 16), :] = lo.astype(BF16)
            R_v[pl.ds(5 * HK + r, 16), :] = (lo + hi).astype(BF16)
        else:
            b11, b12 = zf_v[rows, :HN], zf_v[rows, HN:]
            R_v[pl.ds(0 * HK + r, 16), :] = (b11 + hi).astype(BF16)
            R_v[pl.ds(2 * HK + r, 16), :] = (b12 - hi).astype(BF16)
            R_v[pl.ds(3 * HK + r, 16), :] = (lo - b11).astype(BF16)
            R_v[pl.ds(4 * HK + r, 16), :] = hi.astype(BF16)
            R_v[pl.ds(6 * HK + r, 16), :] = (lo + hi).astype(BF16)

    def acomb_gen(i, groups=range(P // 16)):
        for r in groups:
            for c in range(HK // 256):
                top = pl.ds(i * TM + r * 16, 16)
                bot = pl.ds(i * TM + P + r * 16, 16)
                c1 = slice(c * 256, (c + 1) * 256)
                c2 = slice(HK + c * 256, HK + (c + 1) * 256)
                a11 = wsp_v[top, c1].astype(F32)
                a12 = wsp_v[top, c2].astype(F32)
                a21 = wsp_v[bot, c1].astype(F32)
                a22 = wsp_v[bot, c2].astype(F32)
                r0 = (i % 4) * 5 * P + r * 16
                Lc_v[pl.ds(r0 + 0 * P, 16), c1] = (a11 + a22).astype(BF16)
                Lc_v[pl.ds(r0 + 1 * P, 16), c1] = (a21 + a22).astype(BF16)
                Lc_v[pl.ds(r0 + 2 * P, 16), c1] = (a11 + a12).astype(BF16)
                Lc_v[pl.ds(r0 + 3 * P, 16), c1] = (a21 - a11).astype(BF16)
                Lc_v[pl.ds(r0 + 4 * P, 16), c1] = (a12 - a22).astype(BF16)
                yield A_COST

    def tasks(fn, t, n=TM // 16):
        return [lambda tie, s=s: fn(t, s, tie) for s in range(n)]

    def kv_gen(t):
        for m in range(TM // KV_ROWS):
            r = t * TM + m * KV_ROWS
            for l in range(D // L):
                lanes = slice(l * L, (l + 1) * L)
                kf = k_v[pl.ds(r, KV_ROWS), lanes].astype(F32)
                kf_v[l, pl.ds(r + 8, KV_ROWS), :] = kf
                ks = kf * sk_v[0, 0:1, lanes]
                for tap in range(1, 4):
                    ks = ks + kf_v[l, pl.ds(r + 8 - tap, KV_ROWS), :] * sk_v[tap, 0:1, lanes]
                kv = ks * v_v[pl.ds(r, KV_ROWS), lanes].astype(F32)
                kv_v[pl.ds(r, KV_ROWS), lanes] = kv.astype(BF16)
                yield KV_COST * KV_ROWS / 64

    def freq_gen(a):
        def cmac(acc, x, g):
            pr = x[0] * g[0] - x[1] * g[1]
            pi = x[0] * g[1] + x[1] * g[0]
            return (pr, pi) if acc is None else (acc[0] + pr, acc[1] + pi)

        for r in range(P // 16):
            for l in range(D // L):
                lanes = slice(l * L, (l + 1) * L)
                res = []
                for sub in range(16 // FR):
                    rows = pl.ds(r * 16 + sub * FR, FR)
                    lo = hi = None
                    g = (G_v[a + 1, 0, rows, lanes], G_v[a + 1, 1, rows, lanes])
                    for c in range(a + 2):
                        x = (X_v[c, 0, rows, lanes], X_v[c, 1, rows, lanes])
                        hi = cmac(hi, x, g)
                        if c <= a:
                            g = (G_v[a - c, 0, rows, lanes], G_v[a - c, 1, rows, lanes])
                            lo = cmac(lo, x, g)
                            yield 2 * FR
                    res.append((lo, hi))
                for w in range(2):
                    for part in range(2):
                        Z_v[pl.ds((a + w) * 2 * P + part * P + r * 16, 16), lanes] = jnp.concatenate(
                            [z[w][part] for z in res], axis=0).astype(BF16)
                yield 20

    def job_x(t, bg, budget):
        for j in (2 * t, 2 * t + 1):
            for half in range(2):
                r = _dot(F_v[half * P:(half + 1) * P, 0:P], kv_v[j * P:(j + 1) * P, :]).reshape(8, 2, 8, D)
                for part in range(2):
                    X_v[j, part, half * 64:(half + 1) * 64, :] = r[:, part].reshape(64, D)
                bg.run(budget * 2.5)

    def job_h(t, bg, budget):
        for half in range(2):
            rows = pl.ds(half * 64, 64)
            for l0, l1 in H_SPLIT:
                w = (l1 - l0) * L
                lanes = slice(l0 * L, l1 * L)
                rhs = jnp.concatenate([h_v[t, lanes, 0:P], h_v[t, lanes, P:2 * P]], axis=0)
                r = jax.lax.dot_general(F_v[half * P:(half + 1) * P, 0:P], rhs, NT_DIMS,
                                        preferred_element_type=F32).reshape(8, 2, 8, 2 * w)
                re, im = r[:, 0].reshape(64, 2 * w), r[:, 1].reshape(64, 2 * w)
                prev = (H_v[t % 2, 0, rows, lanes], H_v[t % 2, 1, rows, lanes])
                for j in range(2):
                    cur = (re[:, j * w:(j + 1) * w], im[:, j * w:(j + 1) * w])
                    G_v[2 * t + j, 0, rows, lanes] = cur[0] + prev[1] if half else cur[0] - prev[1]
                    G_v[2 * t + j, 1, rows, lanes] = cur[1] - prev[0] if half else cur[1] + prev[0]
                    prev = cur
                if t + 1 < NT:
                    H_v[(t + 1) % 2, 0, rows, lanes] = prev[0]
                    H_v[(t + 1) % 2, 1, rows, lanes] = prev[1]
                bg.run(budget * (l1 - l0))

    def z_out(t, m, n, pre, bg, budget, tied):
        z = _gelu_scaled(pre)
        if n < FH // L:
            z1_v[pl.ds(t * TM + m * MC, MC), n * L:(n + 1) * L] = z
        else:
            zg_v[t % 3, m * MC:(m + 1) * MC, n * L - FH:(n + 1) * L - FH] = z
        ntask = tied.run(z)
        bg.run(budget[1] if ntask else budget[0])

    def job_z(t, m, cols, bg, budget, tied):
        for n in cols:
            z_out(t, m, n, _dot(xn_v[pl.ds(t * TM + m * MC, MC), :], win_v[:, n * L:(n + 1) * L]), bg, budget, tied)

    def job_zs(t, p, j, bg, budget, tied):
        r1 = pl.ds(t * TM + p * P, MC)
        r2 = pl.ds(t * TM + p * P + MC, MC)
        c1 = slice(j * L, (j + 1) * L)
        c2 = slice(FH + j * L, FH + (j + 1) * L)

        def xl(w):
            r0 = (t % 4) * 5 * P + w * P + p * MC
            return XL_v[r0:r0 + MC, :]

        def wb(w):
            return WB_v[w * KH:(w + 1) * KH, c1]

        def rem(rows, cols):
            return _dot(xn_v[rows, 2 * KH:], win_v[2 * KH:, cols])

        def dot2(a, b):
            r = _dot(a, b)
            bg.run(mid)
            return r

        mid = ZS_MID * budget[0]
        budget = (budget[0] - 1.75 * mid, budget[1] - 1.75 * mid)
        m2 = dot2(xl(1), win_v[0:KH, c1])
        m4 = dot2(xn_v[r2, KH:2 * KH], wb(2))
        z_out(t, 2 * p + 1, j, m2 + m4 + rem(r2, c1), bg, budget, tied)
        m3 = dot2(xn_v[r1, 0:KH], wb(1))
        m5 = dot2(xl(2), win_v[KH:2 * KH, c2])
        z_out(t, 2 * p, 6 + j, m3 + m5 + rem(r1, c2), bg, budget, tied)
        t11, t22 = m4 - m5, m3 - m2
        m1 = dot2(xl(0), wb(0))
        t11, t22 = t11 + m1, t22 + m1
        z_out(t, 2 * p, j, t11 + dot2(xl(4), wb(4)) + rem(r1, c1), bg, budget, tied)
        z_out(t, 2 * p + 1, 6 + j, t22 + dot2(xl(3), wb(3)) + rem(r2, c2), bg, budget, tied)

    rev8 = 7 - jax.lax.broadcasted_iota(jnp.int32, (8, L), 0)

    def finish(a, upper, n, hh, slot):
        rows = pl.ds(a * P + (MC if upper else 0), MC)
        lanes = slice(n * L, (n + 1) * L)
        if upper:
            ya = _dot(Fi_v[:, 0:P], Z_v[a * 2 * P:a * 2 * P + P, lanes])
            yb = _dot(Fi_v[:, P:2 * P], Z_v[a * 2 * P + P:(a + 1) * 2 * P, lanes])
            slot(0.5)
            y = ya - yb
            lo = ya + yb
            for j in range(MC // 8):
                yl_v[a % 2, n, (7 - j) * 8:(8 - j) * 8, :] = jnp.take_along_axis(lo[j * 8:(j + 1) * 8], rev8, axis=0)
        else:
            y = yl_v[a % 2, n]
        gate = hh + hh * jnp.tanh(hh)
        s = xn_v[rows, lanes].astype(F32) * y
        o_v[rows, lanes] = (x_v[rows, lanes].astype(F32) + s * gate).astype(BF16)

    def tail_gen(i, bg, budget):
        a0, a1 = _blocks_of_step(i)

        def slot(w):
            bg.run(w * budget[0])

        def dot3(a, b):
            r = _dot(a, b)
            slot(0.75)
            return r

        for upper in (True, False):
            sub = MC if upper else 0
            r1 = pl.ds(a0 * P + sub, MC)
            r2 = pl.ds(a1 * P + sub, MC)

            def ul(w):
                r0 = ((i % 4) * 5 + w) * P + sub
                return UL_v[r0:r0 + MC, :]

            for j in range(2):
                c1 = slice(j * L, (j + 1) * L)
                c2 = slice((2 + j) * L, (3 + j) * L)

                def wo(w):
                    return WO_v[w * HN:(w + 1) * HN, c1]

                m2 = dot3(ul(1), wout_v[0:HN, c1])
                m4 = dot3(u_v[r2, HN:], wo(2))
                finish(a1, upper, j, m2 + m4, slot)
                bg.charge(T_COST)
                yield
                m3 = dot3(u_v[r1, 0:HN], wo(1))
                m5 = dot3(ul(2), wout_v[HN:, c2])
                finish(a0, upper, 2 + j, m3 + m5, slot)
                bg.charge(T_COST)
                yield
                m1 = dot3(ul(0), wo(0))
                finish(a0, upper, j, (m4 - m5) + m1 + dot3(ul(4), wo(4)), slot)
                bg.charge(T_COST)
                yield
                finish(a1, upper, 2 + j, (m3 - m2) + m1 + dot3(ul(3), wo(3)), slot)
                bg.charge(T_COST)
                yield
            finish(a0, upper, 4, dot3(u_v[r1, 0:HN], wout_v[0:HN, 4 * L:]) + dot3(u_v[r1, HN:], wout_v[HN:, 4 * L:]), slot)
            bg.charge(T_COST)
            yield
            finish(a1, upper, 4, dot3(u_v[r2, 0:HN], wout_v[0:HN, 4 * L:]) + dot3(u_v[r2, HN:], wout_v[HN:, 4 * L:]), slot)
            bg.charge(T_COST)
            yield

    def wocomb_gen():
        for j in range(2):
            c1 = slice(j * L, (j + 1) * L)
            c2 = slice((2 + j) * L, (3 + j) * L)
            for r in range(HN // 32):
                top = pl.ds(r * 32, 32)
                bot = pl.ds(HN + r * 32, 32)
                b11, b12 = wout_v[top, c1].astype(F32), wout_v[top, c2].astype(F32)
                b21, b22 = wout_v[bot, c1].astype(F32), wout_v[bot, c2].astype(F32)
                for w, c in enumerate((b11 + b22, b12 - b22, b21 - b11, b11 + b12, b21 + b22)):
                    WO_v[pl.ds(w * HN + r * 32, 32), c1] = c.astype(BF16)
                yield A_COST

    def job_big(i, bg, pending, budget, every):
        a0, a1 = _blocks_of_step(i)
        KG = BIG_KG

        def lhs(j, sub, cols):
            if j == 2:
                return wsp_v[i * TM + sub:i * TM + sub + MC, cols]
            if j == 3:
                return wsp_v[i * TM + P + sub:i * TM + P + sub + MC, HK + cols.start:HK + cols.stop]
            r0 = ((i % 4) * 5 + {0: 0, 1: 1, 4: 2, 5: 3, 6: 4}[j]) * P + sub
            return Lc_v[r0:r0 + MC, cols]

        def prod(j, sub, n, acc=None):
            for kg in range(HK // KG):
                ks = slice(kg * KG, (kg + 1) * KG)
                p = _dot(lhs(j, sub, ks), R_v[j * HK + kg * KG:j * HK + (kg + 1) * KG, n * L:(n + 1) * L])
                acc = p if acc is None else acc + p
                bg.run(budget * KG / 512)
            return acc

        def tails(n):
            for _ in range(n):
                if pending:
                    next(pending.pop(0))

        def emit(a, sub, n, g):
            rows = pl.ds(a * P + sub, MC)
            lanes = slice(n * L, (n + 1) * L)
            u = z1_v[rows, lanes] * (g + bcol_v[rows, :])
            u_v[rows, lanes] = u.astype(BF16)
            bg.charge(E_COST)
            return u

        for sub in (0, MC):
            for n in range(HN // L):
                def put(w, c):
                    UL_v[pl.ds(((i % 4) * 5 + w) * P + sub, MC), n * L:(n + 1) * L] = c.astype(BF16)

                if ORDER == 0:
                    m2 = prod(1, sub, n)
                    m4 = prod(3, sub, n)
                    u21 = emit(a1, sub, n, m2 + m4)
                    m3 = prod(2, sub, n)
                    t22 = m3 - m2
                    m5 = prod(4, sub, n)
                    u12 = emit(a0, sub, n + HN // L, m3 + m5)
                    t11 = m4 - m5
                    m1 = prod(0, sub, n)
                    u11 = emit(a0, sub, n, prod(6, sub, n, t11 + m1))
                    u22 = emit(a1, sub, n + HN // L, prod(5, sub, n, t22 + m1))
                    for w, c in enumerate((u11 + u22, u21 + u22, u11 + u12, u21 - u11, u12 - u22)):
                        put(w, c)
                else:
                    m1 = prod(0, sub, n)
                    t11 = prod(6, sub, n, m1)
                    m4 = prod(3, sub, n)
                    t11 = t11 + m4
                    m5 = prod(4, sub, n)
                    u11 = emit(a0, sub, n, t11 - m5)
                    m2 = prod(1, sub, n)
                    u21 = emit(a1, sub, n, m2 + m4)
                    put(3, u21 - u11)
                    t22 = m1 - m2
                    m3 = prod(2, sub, n)
                    u12 = emit(a0, sub, n + HN // L, m3 + m5)
                    put(2, u11 + u12)
                    u22 = emit(a1, sub, n + HN // L, prod(5, sub, n, t22 + m3))
                    put(0, u11 + u22)
                    put(1, u21 + u22)
                    put(4, u12 - u22)
                bg.charge(U_COST)
                tails(every.pop(0))

    if _ONLY is not None:
        for r_ in (xn_u, XL_u, WB_u, UL_u, WO_u, z1_v, R_u, Lc_u, zf_v, zg_v, kv_u, u_u, X_v, H_v, G_v, Z_u, kf_v):
            c_ = pltpu.make_async_copy(r_, r_, sem_small.at[0])
            c_.start()
            c_.wait()

    cp_x(0).start()
    cp_win(0).start()
    cp_x(1).start()
    for c in range(1, 5):
        cp_win(c).start()
    cp_x(2).start()
    start(cp_small())

    kk = _odd_freq(jax.lax.broadcasted_iota(jnp.int32, (P, P), 0))
    nn = jax.lax.broadcasted_iota(jnp.int32, (P, P), 1)
    fc, fs = _cos_sin((kk * (4 * nn - 127)) & 2047)
    for g in range(P // 8):
        F_v[g * 16:(g + 1) * 16, 0:P] = jnp.concatenate(
            [fc[g * 8:(g + 1) * 8], -fs[g * 8:(g + 1) * 8]], axis=0).astype(BF16)
    fc, fs = _cos_sin((kk * (-127)) & 2047)
    ph_v[0] = fc
    ph_v[1] = fs
    kk = _odd_freq(jax.lax.broadcasted_iota(jnp.int32, (MC, P), 1))
    mm = jax.lax.broadcasted_iota(jnp.int32, (MC, P), 0)
    ic, is_ = _cos_sin((kk * (4 * mm + 2)) & 2047)
    Fi_v[:, 0:P] = (ic * (1.0 / (P * GA))).astype(BF16)
    Fi_v[:, P:2 * P] = (is_ * (1.0 / (P * GA))).astype(BF16)
    kf_v[:, 0:8, :] = jnp.zeros((D // L, 8, L), F32)

    cp_x(0).wait()
    for s in range(TM // 16):
        ln_x(0, s)

    def small_setup():
        sk = sk_in[...].astype(F32)
        for t in range(4):
            sk_v[t] = jnp.broadcast_to(sk[t:t + 1], (8, D))
        drow = d_in[...].astype(F32).reshape(1, D)
        for l in range(D // L):
            lanes = slice(l * L, (l + 1) * L)
            dre = ph_v[0] * drow[:, lanes]
            dim = ph_v[1] * drow[:, lanes]
            H_v[0, 0, 0:64, lanes] = -dim[0:64]
            H_v[0, 0, 64:P, lanes] = dim[64:P]
            H_v[0, 1, 0:64, lanes] = -dre[0:64]
            H_v[0, 1, 64:P, lanes] = dre[64:P]

    def bcol_task(t, j, tie):
        brow = b_in[...].astype(F32).reshape(1, S)[:, j * P:(j + 1) * P] * (0.25 / GA) + tie[0:1]
        bcol_v[j * P:(j + 1) * P, :] = jnp.broadcast_to(brow, (P, P)).T

    LAG = 2

    def interleave(*lists):
        out = []
        for j in range(max(len(a) for a in lists)):
            for a in lists:
                out += a[j:j + 1]
        return out

    def p1_first(c):
        bg = _Background()
        todo = []
        if c == 3:
            todo = tasks(ln_z2, 0)
            bg.add(wcomb_gen(range(3)))
        if c == 4:
            todo = tasks(ln_x2, 2, 8)
            bg.add(wcomb_gen(range(3, 6)))
            small_setup()
        tied = _Tied(todo, 20)
        if c == 0:
            for s in range(TM // 16):
                ln_x(1, s)
        for t in range(2):
            for m in range(TM // MC):
                job_z(t, m, range(*WIN_CHUNKS[c]), bg, (80, 40), tied)
        bg.drain()
        assert not tied.tasks

    for c in range(5):
        cp_win(c).wait()
        if c == 0:
            cp_x(1).wait()
        if c == 2:
            start(cp_conv(0))
            cp_x(3).start()
        if c == 4:
            cp_x(2).wait()
            wait(cp_small())
            cp_x(4).start()
            cp_x(5).start()
        block(lambda c=c: p1_first(c), f'p1_f{c}')

    def p1_dma(g):
        if g == 0:
            wait(cp_conv(0))
            cp_x(3).wait()
            start(cp_conv(1))
            cp_x(6).start()
            cp_x(7).start()
            start(cp_conv(2))
        if g == 1:
            wait(cp_conv(1))
            cp_x(4).wait()
            cp_x(5).wait()
            start(cp_conv(3))
            start(cp_conv(4))
        if g == 2:
            wait(cp_conv(2))
            wait(cp_conv(3))
            cp_x(6).wait()
            cp_x(7).wait()
            start(cp_conv(5))
            cp_wout().start()
            start(cp_wsp(0))
            start(cp_wsp(1))
        if g == 3:
            wait(cp_conv(4))
            wait(cp_conv(5))
            cp_wout().wait()
            wait(cp_wsp(0))
            start(cp_conv(6))
            start(cp_wsp(2))
            start(cp_conv(7))

    def take(gen, n):
        for _ in range(n):
            yield next(gen)

    def p1_step(i):
        bg = _Background()
        dft = _Background()
        t = i - LAG
        xg = P1_XG[i]
        kv = kv_gen(t)
        nx, nz, nh = KV_SPLIT if xg is not None else (0, KV_SPLIT[0] + KV_SPLIT[1], KV_SPLIT[2])
        dft.add(take(kv, nx))
        bg.add(take(kv, nz))
        hbg = _Background()
        hbg.add(take(kv, nh))
        zb = nz * KV_COST / 48.0
        extra = 0
        if i == 6:
            bg.add(wocomb_gen())
            bg.add(acomb_gen(0, range(3)))
            extra = 42
        if i == 7:
            bg.add(acomb_gen(0, range(3, 8)))
            extra = 24
        last = i == NT - 1
        z2t = tasks(ln_z2, i - 1)
        todo = interleave(*([tasks(ln_x2, t_, 8) for t_ in P1_LNX[i]] + [z2t[0::2], z2t[1::2]] +
                            [tasks(bcol_task, 0) if i == 2 else []]))
        tied = _Tied(todo, 24 if last else TIED_N)
        if xg is not None:
            dft.run(KV_COST)
            job_x(xg, dft, (nx - 1) * KV_COST / 10.0)
            dft.drain()
        for p in range(2):
            for j in range(FH // L):
                job_zs(i, p, j, bg, (1.6 * zb + extra, 0.5 * zb + extra), tied)
            assert not tied.tasks or (p == 0 and not last)
            if p == 0 and last:
                tied = _Tied(tasks(ln_z2, i, 8), 22)
        if last:
            for s in range(8, 16):
                ln_z2(i, s)
        bg.drain()
        job_h(t, hbg, nh * KV_COST / 10.0)
        hbg.drain()

    def p1_block(g):
        for i in P1_GROUPS[g]:
            p1_step(i)

    for g in range(len(P1_GROUPS)):
        p1_dma(g)
        block(lambda g=g: p1_block(g), f'p1_g{g}')

    groups = P2_GROUPS
    NG = len(groups)

    def p2_dma(gi):
        if gi >= 2:
            for i in groups[gi - 2]:
                start(cp_out(i))
        if gi >= 3:
            for i in groups[gi - 3]:
                wait(cp_out(i))
        if gi + 2 < NG:
            for i in groups[gi + 2]:
                start(cp_wsp(i))
        if gi < 2:
            wait(cp_conv(NT - 2 + gi))
        if gi + 1 < NG:
            for i in groups[gi + 1]:
                wait(cp_wsp(i))

    def tails_of(i, bg, budget):
        return [tail_gen(i, bg, budget)] * 20

    def p2_block(gi):
        bg = _Background()
        steps = groups[gi]
        tb = [0.0]
        pending = [t_ for i in (groups[gi - 1] if gi > 0 else []) for t_ in tails_of(i, bg, tb)]
        total = sum(a + 1 for i in steps for a in _blocks_of_step(i)) * 40 * 16
        total += len(steps) * (24 * E_COST + 6 * U_COST) + len(pending) * T_COST
        slots = 84 * len(steps) + TAIL_W * len(pending)
        bg.add(freq_gen(_blocks_of_step(steps[0])[0]))
        if gi < 2:
            bg.add(kv_gen(NT - 2 + gi))
            total += 20 * KV_COST
            slots += 10
        for t in P2_XG[gi]:
            slots += 10
        if gi + 1 < NG:
            for i in groups[gi + 1]:
                bg.add(acomb_gen(i))
                total += 32 * A_COST
        for i in steps[1:]:
            bg.add(freq_gen(_blocks_of_step(i)[0]))
        budget = tb[0] = total / (slots + 1.0)
        bg.run(budget)
        for t in P2_XG[gi]:
            job_x(t, bg, budget)
        if gi < 2:
            job_h(NT - 2 + gi, bg, budget)
        units = [4, 4, 2, 4, 4, 2] * (len(pending) // 20)
        every = [0] * (6 * len(steps))
        for j, n in enumerate(units):
            every[min(len(every) - 1, j * len(every) // len(units))] += n
        for i in steps:
            job_big(i, bg, pending, budget, every)
        for t_ in pending:
            next(t_)
        bg.drain()

    for gi in range(NG):
        p2_dma(gi)
        block(lambda gi=gi: p2_block(gi), f'p2_{gi}')

    def cp_last(upper):
        a0 = _blocks_of_step(NT - 1)[0]
        return [pltpu.make_async_copy(o_v.at[pl.ds(r, MC)], o_hbm.at[0, pl.ds(r, MC)], sem_out.at[(NT - 1) % 5])
                for r in ((a0 + w) * P + (MC if upper else 0) for w in range(2))]

    def p2_last():
        for j, t_ in enumerate(tails_of(NT - 1, _Background(), [0.0])):
            next(t_)
            if j == 9:
                start(cp_last(True))

    p2_dma(NG)
    block(p2_last, 'p2_last')
    start(cp_last(False))
    for i in groups[NG - 2]:
        wait(cp_out(i))
    wait(cp_last(True))
    wait(cp_last(False))
    if _ONLY is not None:
        for r_ in (xn_u, XL_u, WB_u, UL_u, WO_u, z1_v, R_u, Lc_u, zf_v, zg_v, kv_u, u_u, X_v, H_v, G_v, Z_u, kf_v):
            c_ = pltpu.make_async_copy(r_, r_, sem_small.at[0])
            c_.start()
            c_.wait()


@jax.jit
def pallas_recurrent_scan__ssm_conv_h3__mixer_gmlp__prompt_kernel(
    A_q: jax.Array,
    A_k: jax.Array,
    A_v: jax.Array,
    A_shift_k: jax.Array,
    A_ssm_k: jax.Array,
    A_ssm_D: jax.Array,
    B_x: jax.Array,
    B_w_in: jax.Array,
    B_w_sp: jax.Array,
    B_b_sp: jax.Array,
    B_w_out: jax.Array,
):
    del B_x
    hbm = pl.BlockSpec(memory_space=pl.ANY)

    def bf16_buf(*shape):
        return pltpu.VMEM(shape[:-2] + (shape[-2] // 2, shape[-1]), U32)

    return pl.pallas_call(
        _kernel,
        out_shape=jax.ShapeDtypeStruct((1, S, D), BF16),
        in_specs=[hbm] * 10,
        out_specs=hbm,
        scratch_shapes=[
            bf16_buf(S, D),
            bf16_buf(S, D),
            bf16_buf(S, D),
            bf16_buf(NT, D, TM),
            bf16_buf(D, 2 * FH),
            bf16_buf(S, S),
            bf16_buf(FH, D),
            pltpu.VMEM((S, D), BF16),
            pltpu.VMEM((4, D), BF16),
            pltpu.VMEM((D,), BF16),
            pltpu.VMEM((S,), BF16),
            bf16_buf(S, D),
            bf16_buf(4 * 5 * P, KH),
            bf16_buf(5 * KH, FH),
            bf16_buf(4 * 5 * P, HN),
            bf16_buf(5 * HN, 2 * L),
            pltpu.VMEM((S, FH), F32),
            bf16_buf(7 * HK, HN),
            bf16_buf(4 * 5 * P, HK),
            pltpu.VMEM((HK, FH), F32),
            pltpu.VMEM((3, TM, FH), F32),
            bf16_buf(S, D),
            bf16_buf(S, FH),
            pltpu.VMEM((NB, 2, P, D), F32),
            pltpu.VMEM((2, 2, P, D), F32),
            pltpu.VMEM((NB, 2, P, D), F32),
            bf16_buf(NB * 2 * P, D),
            pltpu.VMEM((2, D // L, MC, L), F32),
            bf16_buf(2 * P, 2 * P),
            bf16_buf(MC, 2 * P),
            pltpu.VMEM((S, L), F32),
            pltpu.VMEM((2, P, L), F32),
            pltpu.VMEM((4, 8, D), F32),
            pltpu.VMEM((D // L, S + 8, L), F32),
            pltpu.SemaphoreType.DMA((1,)),
            pltpu.SemaphoreType.DMA((5,)),
            pltpu.SemaphoreType.DMA((4,)),
            pltpu.SemaphoreType.DMA((5,)),
            pltpu.SemaphoreType.DMA((5,)),
            pltpu.SemaphoreType.DMA((5,)),
        ],
        compiler_params=pltpu.CompilerParams(vmem_limit_bytes=116 * 1024 * 1024, disable_semaphore_checks=True),
    )(A_q, A_k, A_v, A_shift_k.T, A_ssm_k, A_ssm_D, B_w_in, B_w_sp, B_b_sp, B_w_out)
```

```python
import math

import jax
import jax.numpy as jnp
import jax.experimental.pallas as pl
import jax.experimental.pallas.tpu as pltpu

S = 2048
D = 640
FH = 768
P = 128
NB = S // P
TM = 256
NT = S // TM
MC = 64
L = 128
HK = S // 2
KH = 256
HN = FH // 2
P1_GROUPS = ((2,), (3,), (4, 5), (6, 7))
P1_XG = {2: None, 3: 0, 4: 1, 5: None, 6: 2, 7: 3}
P1_LNX = {2: (3,), 3: (4, 5), 4: (6,), 5: (7,), 6: (), 7: ()}
P2_XG = ((4, 5), (6,), (7,), (), ())
P2_GROUPS = ((0,), (1, 2), (3, 4), (5, 6), (7,))
STEP_BLOCKS = ((6, 7), (8, 9), (4, 5), (12, 13), (2, 3), (14, 15), (0, 1), (10, 11))
KV_COST, G_COST, A_COST = 110, 36, 56
E_COST, U_COST, T_COST, TAIL_W = 24, 90, 90, 1.6
BIG_KG = 512
TIE_X = False
DFT_B = (130, 80)
Z_B0, Z_B1 = 60, 10
TIED_N = 42
ORDER = 1
ZS_MID = 0.0
H_SPLIT = ((0, 2), (2, 4), (4, 5))
KV_SPLIT = (12, 4, 4)
F_TIED = (20, 20, 18, 20, 20)
F_B = (80, 40)
FR = 16
KV_ROWS = 64
WIN_CHUNKS = ((6, 7), (7, 9), (9, 12), (0, 3), (3, 6))
EPS = 1e-5
F32 = jnp.float32
BF16 = jnp.bfloat16
U32 = jnp.uint32
GELU_C = math.sqrt(2.0 / math.pi)
GA = (GELU_C * 0.044715) ** (1.0 / 3.0)
NT_DIMS = (((1,), (1,)), ((), ()))
_ONLY = None


def _dot(a, b):
    return jnp.dot(a, b, preferred_element_type=F32)


def _cos_sin(m):
    q = (m + 256) >> 9
    x = (m - (q << 9)).astype(F32) * (2.0 * math.pi / 2048.0)
    x2 = x * x
    s = x * (1.0 + x2 * (-1.0 / 6 + x2 * (1.0 / 120 + x2 * (-1.0 / 5040 + x2 * (1.0 / 362880)))))
    c = 1.0 + x2 * (-0.5 + x2 * (1.0 / 24 + x2 * (-1.0 / 720 + x2 * (1.0 / 40320 - x2 * (1.0 / 3628800)))))
    swap = (q & 1) == 1
    c0 = jnp.where(swap, s, c)
    s0 = jnp.where(swap, c, s)
    cos = jnp.where(((q + 1) & 2) == 2, -c0, c0)
    sin = jnp.where((q & 2) == 2, -s0, s0)
    return cos, sin


def _odd_freq(r):
    return jnp.where(r < 64, 4 * r + 1, 4 * r - 253)


def _gelu_scaled(z):
    return z + z * jnp.tanh(z * (GELU_C / GA + z * z))


def _signzero(z):
    bits = jax.lax.bitcast_convert_type(z, U32) & jnp.uint32(0x80000000)
    return jax.lax.bitcast_convert_type(bits, F32)


def _ln(x, eps, tie=None, scale=None):
    n = x.shape[-1]
    cols = [x[:, j * L:(j + 1) * L] for j in range(n // L)]
    s1 = cols[0]
    s2 = cols[0] * cols[0]
    for c in cols[1:]:
        s1 = s1 + c
        s2 = s2 + c * c
    if tie is not None:
        s1 = s1 + tie
        s2 = s2 + tie
    m = jnp.sum(s1, axis=-1, keepdims=True) * (1.0 / n)
    v = jnp.maximum(jnp.sum(s2, axis=-1, keepdims=True) * (1.0 / n) - m * m, 0.0)
    rs = jax.lax.rsqrt(v + eps)
    if scale is not None:
        rs = rs * scale
    return (x - m) * rs


def _blocks_of_step(i):
    return STEP_BLOCKS[i]


class _Background:
    def __init__(self):
        self.q = []
        self.credit = 0.0

    def add(self, gen):
        self.q.append(gen)

    def run(self, budget):
        self.credit += budget
        while self.q and self.credit > 0:
            try:
                self.credit -= next(self.q[0])
            except StopIteration:
                self.q.pop(0)
        if not self.q:
            self.credit = 0.0

    def charge(self, cost):
        self.credit -= cost

    def drain(self):
        while self.q:
            self.run(1e9)


class _Tied:
    def __init__(self, tasks, npieces):
        self.tasks = list(tasks)
        self.rate = len(self.tasks) / float(npieces)
        self.credit = 0.999

    def run(self, z):
        self.credit += self.rate
        n = 0
        while self.tasks and self.credit >= 1.0:
            self.tasks.pop(0)(_signzero(z[0:16]))
            self.credit -= 1.0
            n += 1
        return n


def _kernel(q_hbm, k_hbm, v_hbm, sk_hbm, h_hbm, d_hbm, win_hbm, wsp_hbm, b_hbm, wout_hbm,
            o_hbm,
            x_u, k_u, v_u, h_u, win_u, wsp_u, wout_u, o_v, sk_in, d_in, b_in,
            xn_u, XL_u, WB_u, UL_u, WO_u, z1_v, R_u, Lc_u, zf_v, zg_v, kv_u, u_u, X_v, H_v, G_v, Z_u, yl_v, F_u, Fi_u, bcol_v, ph_v, sk_v, kf_v,
            sem_small, sem_x, sem_conv, sem_wsp, sem_w, sem_out):
    x_v, k_v, v_v, h_v, win_v, wsp_v, wout_v, xn_v, XL_v, WB_v, UL_v, WO_v, R_v, Lc_v, kv_v, u_v, Z_v, F_v, Fi_v = [
        r.bitcast(BF16) for r in (x_u, k_u, v_u, h_u, win_u, wsp_u, wout_u, xn_u, XL_u, WB_u, UL_u, WO_u, R_u, Lc_u, kv_u, u_u, Z_u, F_u,
                                  Fi_u)]

    def cp_small():
        return [pltpu.make_async_copy(s_, d_, sem_small.at[0])
                for s_, d_ in ((d_hbm, d_in), (sk_hbm, sk_in), (b_hbm, b_in))]

    def cp_x(t):
        return pltpu.make_async_copy(q_hbm.at[0, pl.ds(t * TM, TM)], x_v.at[pl.ds(t * TM, TM)], sem_x.at[t % 5])

    def cp_conv(t):
        rows = pl.ds(t * TM, TM)
        sem = sem_conv.at[t % 4]
        return [pltpu.make_async_copy(h_hbm.at[:, rows], h_v.at[t], sem),
                pltpu.make_async_copy(k_hbm.at[0, rows], k_v.at[rows], sem),
                pltpu.make_async_copy(v_hbm.at[0, rows], v_v.at[rows], sem)]

    def cp_wsp(i, which=(0, 1)):
        return [pltpu.make_async_copy(wsp_hbm.at[pl.ds(_blocks_of_step(i)[half] * P, P)],
                                      wsp_v.at[pl.ds(i * TM + half * P, P)], sem_wsp.at[i % 5]) for half in which]

    def cp_win(c):
        lo, hi = WIN_CHUNKS[c]
        cols = pl.ds(lo * L, (hi - lo) * L)
        return pltpu.make_async_copy(win_hbm.at[:, cols], win_v.at[:, cols], sem_w.at[c])

    def cp_wout():
        return pltpu.make_async_copy(wout_hbm, wout_v, sem_w.at[0])

    def cp_out(i):
        rows = pl.ds(_blocks_of_step(i)[0] * P, TM)
        return [pltpu.make_async_copy(o_v.at[rows], o_hbm.at[0, rows], sem_out.at[i % 5])]

    def start(cs):
        for c in cs:
            c.start()

    def wait(cs):
        for c in cs:
            c.wait()

    def block(fn, name):
        def body(it):
            fn()
            return it + 1

        if _ONLY is None or name in _ONLY:
            jax.lax.while_loop(lambda it: it < 1, body, jnp.int32(0))

    def ln_x(t, s, tie=None):
        rows = pl.ds(t * TM + s * 16, 16)
        y = _ln(x_v[rows, :].astype(F32), EPS, tie, GA)
        xn_v[rows, :] = y.astype(BF16)
        return y

    def ln_x2(t, s, tie):
        p, q = s // 4, s % 4
        y1 = ln_x(t, 8 * p + q, tie)
        y2 = ln_x(t, 8 * p + 4 + q, tie)
        a11, a12, a21, a22 = y1[:, :KH], y1[:, KH:2 * KH], y2[:, :KH], y2[:, KH:2 * KH]
        r0 = (t % 4) * 5 * P + p * MC + q * 16
        for j, c in enumerate((a11 + a22, a21 + a22, a11 + a12, a21 - a11, a12 - a22)):
            XL_v[pl.ds(r0 + j * P, 16), :] = c.astype(BF16)

    def wcomb_gen(cols):
        for j in cols:
            c1 = slice(j * L, (j + 1) * L)
            c2 = slice(FH + j * L, FH + (j + 1) * L)
            for r in range(KH // 32):
                top = pl.ds(r * 32, 32)
                bot = pl.ds(KH + r * 32, 32)
                b11, b12 = win_v[top, c1].astype(F32), win_v[top, c2].astype(F32)
                b21, b22 = win_v[bot, c1].astype(F32), win_v[bot, c2].astype(F32)
                for w, c in enumerate((b11 + b22, b12 - b22, b21 - b11, b11 + b12, b21 + b22)):
                    WB_v[pl.ds(w * KH + r * 32, 32), c1] = c.astype(BF16)
                yield A_COST

    def ln_z2(t, s, tie=None):
        y = _ln(zg_v[t % 3, s * 16:(s + 1) * 16, :], 4.0 * GA * GA * EPS, tie, 0.25 / GA)
        lo, hi = y[:, :HN], y[:, HN:]
        r = (t * TM + s * 16) % HK
        rows = pl.ds(r, 16)
        if t < NT // 2:
            zf_v[rows, :] = y
            R_v[pl.ds(1 * HK + r, 16), :] = lo.astype(BF16)
            R_v[pl.ds(5 * HK + r, 16), :] = (lo + hi).astype(BF16)
        else:
            b11, b12 = zf_v[rows, :HN], zf_v[rows, HN:]
            R_v[pl.ds(0 * HK + r, 16), :] = (b11 + hi).astype(BF16)
            R_v[pl.ds(2 * HK + r, 16), :] = (b12 - hi).astype(BF16)
            R_v[pl.ds(3 * HK + r, 16), :] = (lo - b11).astype(BF16)
            R_v[pl.ds(4 * HK + r, 16), :] = hi.astype(BF16)
            R_v[pl.ds(6 * HK + r, 16), :] = (lo + hi).astype(BF16)

    def acomb_gen(i, groups=range(P // 16)):
        for r in groups:
            for c in range(HK // 256):
                top = pl.ds(i * TM + r * 16, 16)
                bot = pl.ds(i * TM + P + r * 16, 16)
                c1 = slice(c * 256, (c + 1) * 256)
                c2 = slice(HK + c * 256, HK + (c + 1) * 256)
                a11 = wsp_v[top, c1].astype(F32)
                a12 = wsp_v[top, c2].astype(F32)
                a21 = wsp_v[bot, c1].astype(F32)
                a22 = wsp_v[bot, c2].astype(F32)
                r0 = (i % 4) * 5 * P + r * 16
                Lc_v[pl.ds(r0 + 0 * P, 16), c1] = (a11 + a22).astype(BF16)
                Lc_v[pl.ds(r0 + 1 * P, 16), c1] = (a21 + a22).astype(BF16)
                Lc_v[pl.ds(r0 + 2 * P, 16), c1] = (a11 + a12).astype(BF16)
                Lc_v[pl.ds(r0 + 3 * P, 16), c1] = (a21 - a11).astype(BF16)
                Lc_v[pl.ds(r0 + 4 * P, 16), c1] = (a12 - a22).astype(BF16)
                yield A_COST

    def tasks(fn, t, n=TM // 16):
        return [lambda tie, s=s: fn(t, s, tie) for s in range(n)]

    def kv_gen(t):
        for m in range(TM // KV_ROWS):
            r = t * TM + m * KV_ROWS
            for l in range(D // L):
                lanes = slice(l * L, (l + 1) * L)
                kf = k_v[pl.ds(r, KV_ROWS), lanes].astype(F32)
                kf_v[l, pl.ds(r + 8, KV_ROWS), :] = kf
                ks = kf * sk_v[0, 0:1, lanes]
                for tap in range(1, 4):
                    ks = ks + kf_v[l, pl.ds(r + 8 - tap, KV_ROWS), :] * sk_v[tap, 0:1, lanes]
                kv = ks * v_v[pl.ds(r, KV_ROWS), lanes].astype(F32)
                kv_v[pl.ds(r, KV_ROWS), lanes] = kv.astype(BF16)
                yield KV_COST * KV_ROWS / 64

    def freq_gen(a):
        def cmac(acc, x, g):
            pr = x[0] * g[0] - x[1] * g[1]
            pi = x[0] * g[1] + x[1] * g[0]
            return (pr, pi) if acc is None else (acc[0] + pr, acc[1] + pi)

        for r in range(P // 16):
            for l in range(D // L):
                lanes = slice(l * L, (l + 1) * L)
                res = []
                for sub in range(16 // FR):
                    rows = pl.ds(r * 16 + sub * FR, FR)
                    lo = hi = None
                    g = (G_v[a + 1, 0, rows, lanes], G_v[a + 1, 1, rows, lanes])
                    for c in range(a + 2):
                        x = (X_v[c, 0, rows, lanes], X_v[c, 1, rows, lanes])
                        hi = cmac(hi, x, g)
                        if c <= a:
                            g = (G_v[a - c, 0, rows, lanes], G_v[a - c, 1, rows, lanes])
                            lo = cmac(lo, x, g)
                            yield 2 * FR
                    res.append((lo, hi))
                for w in range(2):
                    for part in range(2):
                        Z_v[pl.ds((a + w) * 2 * P + part * P + r * 16, 16), lanes] = jnp.concatenate(
                            [z[w][part] for z in res], axis=0).astype(BF16)
                yield 20

    def job_x(t, bg, budget):
        for j in (2 * t, 2 * t + 1):
            for half in range(2):
                r = _dot(F_v[half * P:(half + 1) * P, 0:P], kv_v[j * P:(j + 1) * P, :]).reshape(8, 2, 8, D)
                for part in range(2):
                    X_v[j, part, half * 64:(half + 1) * 64, :] = r[:, part].reshape(64, D)
                bg.run(budget * 2.5)

    def job_h(t, bg, budget):
        for half in range(2):
            rows = pl.ds(half * 64, 64)
            for l0, l1 in H_SPLIT:
                w = (l1 - l0) * L
                lanes = slice(l0 * L, l1 * L)
                rhs = jnp.concatenate([h_v[t, lanes, 0:P], h_v[t, lanes, P:2 * P]], axis=0)
                r = jax.lax.dot_general(F_v[half * P:(half + 1) * P, 0:P], rhs, NT_DIMS,
                                        preferred_element_type=F32).reshape(8, 2, 8, 2 * w)
                re, im = r[:, 0].reshape(64, 2 * w), r[:, 1].reshape(64, 2 * w)
                prev = (H_v[t % 2, 0, rows, lanes], H_v[t % 2, 1, rows, lanes])
                for j in range(2):
                    cur = (re[:, j * w:(j + 1) * w], im[:, j * w:(j + 1) * w])
                    G_v[2 * t + j, 0, rows, lanes] = cur[0] + prev[1] if half else cur[0] - prev[1]
                    G_v[2 * t + j, 1, rows, lanes] = cur[1] - prev[0] if half else cur[1] + prev[0]
                    prev = cur
                if t + 1 < NT:
                    H_v[(t + 1) % 2, 0, rows, lanes] = prev[0]
                    H_v[(t + 1) % 2, 1, rows, lanes] = prev[1]
                bg.run(budget * (l1 - l0))

    def z_out(t, m, n, pre, bg, budget, tied):
        z = _gelu_scaled(pre)
        if n < FH // L:
            z1_v[pl.ds(t * TM + m * MC, MC), n * L:(n + 1) * L] = z
        else:
            zg_v[t % 3, m * MC:(m + 1) * MC, n * L - FH:(n + 1) * L - FH] = z
        ntask = tied.run(z)
        bg.run(budget[1] if ntask else budget[0])

    def job_z(t, m, cols, bg, budget, tied):
        for n in cols:
            z_out(t, m, n, _dot(xn_v[pl.ds(t * TM + m * MC, MC), :], win_v[:, n * L:(n + 1) * L]), bg, budget, tied)

    def job_zs(t, p, j, bg, budget, tied):
        r1 = pl.ds(t * TM + p * P, MC)
        r2 = pl.ds(t * TM + p * P + MC, MC)
        c1 = slice(j * L, (j + 1) * L)
        c2 = slice(FH + j * L, FH + (j + 1) * L)

        def xl(w):
            r0 = (t % 4) * 5 * P + w * P + p * MC
            return XL_v[r0:r0 + MC, :]

        def wb(w):
            return WB_v[w * KH:(w + 1) * KH, c1]

        def rem(rows, cols):
            return _dot(xn_v[rows, 2 * KH:], win_v[2 * KH:, cols])

        def dot2(a, b):
            r = _dot(a, b)
            bg.run(mid)
            return r

        mid = ZS_MID * budget[0]
        budget = (budget[0] - 1.75 * mid, budget[1] - 1.75 * mid)
        m2 = dot2(xl(1), win_v[0:KH, c1])
        m4 = dot2(xn_v[r2, KH:2 * KH], wb(2))
        z_out(t, 2 * p + 1, j, m2 + m4 + rem(r2, c1), bg, budget, tied)
        m3 = dot2(xn_v[r1, 0:KH], wb(1))
        m5 = dot2(xl(2), win_v[KH:2 * KH, c2])
        z_out(t, 2 * p, 6 + j, m3 + m5 + rem(r1, c2), bg, budget, tied)
        t11, t22 = m4 - m5, m3 - m2
        m1 = dot2(xl(0), wb(0))
        t11, t22 = t11 + m1, t22 + m1
        z_out(t, 2 * p, j, t11 + dot2(xl(4), wb(4)) + rem(r1, c1), bg, budget, tied)
        z_out(t, 2 * p + 1, 6 + j, t22 + dot2(xl(3), wb(3)) + rem(r2, c2), bg, budget, tied)

    rev8 = 7 - jax.lax.broadcasted_iota(jnp.int32, (8, L), 0)

    def finish(a, upper, n, hh, slot):
        rows = pl.ds(a * P + (MC if upper else 0), MC)
        lanes = slice(n * L, (n + 1) * L)
        if upper:
            ya = _dot(Fi_v[:, 0:P], Z_v[a * 2 * P:a * 2 * P + P, lanes])
            yb = _dot(Fi_v[:, P:2 * P], Z_v[a * 2 * P + P:(a + 1) * 2 * P, lanes])
            slot(0.5)
            y = ya - yb
            lo = ya + yb
            for j in range(MC // 8):
                yl_v[a % 2, n, (7 - j) * 8:(8 - j) * 8, :] = jnp.take_along_axis(lo[j * 8:(j + 1) * 8], rev8, axis=0)
        else:
            y = yl_v[a % 2, n]
        gate = hh + hh * jnp.tanh(hh)
        s = xn_v[rows, lanes].astype(F32) * y
        o_v[rows, lanes] = (x_v[rows, lanes].astype(F32) + s * gate).astype(BF16)

    def tail_gen(i, bg, budget):
        a0, a1 = _blocks_of_step(i)

        def slot(w):
            bg.run(w * budget[0])

        def dot3(a, b):
            r = _dot(a, b)
            slot(0.75)
            return r

        for upper in (True, False):
            sub = MC if upper else 0
            r1 = pl.ds(a0 * P + sub, MC)
            r2 = pl.ds(a1 * P + sub, MC)

            def ul(w):
                r0 = ((i % 4) * 5 + w) * P + sub
                return UL_v[r0:r0 + MC, :]

            for j in range(2):
                c1 = slice(j * L, (j + 1) * L)
                c2 = slice((2 + j) * L, (3 + j) * L)

                def wo(w):
                    return WO_v[w * HN:(w + 1) * HN, c1]

                m2 = dot3(ul(1), wout_v[0:HN, c1])
                m4 = dot3(u_v[r2, HN:], wo(2))
                finish(a1, upper, j, m2 + m4, slot)
                bg.charge(T_COST)
                yield
                m3 = dot3(u_v[r1, 0:HN], wo(1))
                m5 = dot3(ul(2), wout_v[HN:, c2])
                finish(a0, upper, 2 + j, m3 + m5, slot)
                bg.charge(T_COST)
                yield
                m1 = dot3(ul(0), wo(0))
                finish(a0, upper, j, (m4 - m5) + m1 + dot3(ul(4), wo(4)), slot)
                bg.charge(T_COST)
                yield
                finish(a1, upper, 2 + j, (m3 - m2) + m1 + dot3(ul(3), wo(3)), slot)
                bg.charge(T_COST)
                yield
            finish(a0, upper, 4, dot3(u_v[r1, 0:HN], wout_v[0:HN, 4 * L:]) + dot3(u_v[r1, HN:], wout_v[HN:, 4 * L:]), slot)
            bg.charge(T_COST)
            yield
            finish(a1, upper, 4, dot3(u_v[r2, 0:HN], wout_v[0:HN, 4 * L:]) + dot3(u_v[r2, HN:], wout_v[HN:, 4 * L:]), slot)
            bg.charge(T_COST)
            yield

    def wocomb_gen():
        for j in range(2):
            c1 = slice(j * L, (j + 1) * L)
            c2 = slice((2 + j) * L, (3 + j) * L)
            for r in range(HN // 32):
                top = pl.ds(r * 32, 32)
                bot = pl.ds(HN + r * 32, 32)
                b11, b12 = wout_v[top, c1].astype(F32), wout_v[top, c2].astype(F32)
                b21, b22 = wout_v[bot, c1].astype(F32), wout_v[bot, c2].astype(F32)
                for w, c in enumerate((b11 + b22, b12 - b22, b21 - b11, b11 + b12, b21 + b22)):
                    WO_v[pl.ds(w * HN + r * 32, 32), c1] = c.astype(BF16)
                yield A_COST

    def job_big(i, bg, pending, budget, every):
        a0, a1 = _blocks_of_step(i)
        KG = BIG_KG

        def lhs(j, sub, cols):
            if j == 2:
                return wsp_v[i * TM + sub:i * TM + sub + MC, cols]
            if j == 3:
                return wsp_v[i * TM + P + sub:i * TM + P + sub + MC, HK + cols.start:HK + cols.stop]
            r0 = ((i % 4) * 5 + {0: 0, 1: 1, 4: 2, 5: 3, 6: 4}[j]) * P + sub
            return Lc_v[r0:r0 + MC, cols]

        def prod(j, sub, n, acc=None):
            for kg in range(HK // KG):
                ks = slice(kg * KG, (kg + 1) * KG)
                p = _dot(lhs(j, sub, ks), R_v[j * HK + kg * KG:j * HK + (kg + 1) * KG, n * L:(n + 1) * L])
                acc = p if acc is None else acc + p
                bg.run(budget * KG / 512)
            return acc

        def tails(n):
            for _ in range(n):
                if pending:
                    next(pending.pop(0))

        def emit(a, sub, n, g):
            rows = pl.ds(a * P + sub, MC)
            lanes = slice(n * L, (n + 1) * L)
            u = z1_v[rows, lanes] * (g + bcol_v[rows, :])
            u_v[rows, lanes] = u.astype(BF16)
            bg.charge(E_COST)
            return u

        for sub in (0, MC):
            for n in range(HN // L):
                def put(w, c):
                    UL_v[pl.ds(((i % 4) * 5 + w) * P + sub, MC), n * L:(n + 1) * L] = c.astype(BF16)

                if ORDER == 0:
                    m2 = prod(1, sub, n)
                    m4 = prod(3, sub, n)
                    u21 = emit(a1, sub, n, m2 + m4)
                    m3 = prod(2, sub, n)
                    t22 = m3 - m2
                    m5 = prod(4, sub, n)
                    u12 = emit(a0, sub, n + HN // L, m3 + m5)
                    t11 = m4 - m5
                    m1 = prod(0, sub, n)
                    u11 = emit(a0, sub, n, prod(6, sub, n, t11 + m1))
                    u22 = emit(a1, sub, n + HN // L, prod(5, sub, n, t22 + m1))
                    for w, c in enumerate((u11 + u22, u21 + u22, u11 + u12, u21 - u11, u12 - u22)):
                        put(w, c)
                else:
                    m1 = prod(0, sub, n)
                    t11 = prod(6, sub, n, m1)
                    m4 = prod(3, sub, n)
                    t11 = t11 + m4
                    m5 = prod(4, sub, n)
                    u11 = emit(a0, sub, n, t11 - m5)
                    m2 = prod(1, sub, n)
                    u21 = emit(a1, sub, n, m2 + m4)
                    put(3, u21 - u11)
                    t22 = m1 - m2
                    m3 = prod(2, sub, n)
                    u12 = emit(a0, sub, n + HN // L, m3 + m5)
                    put(2, u11 + u12)
                    u22 = emit(a1, sub, n + HN // L, prod(5, sub, n, t22 + m3))
                    put(0, u11 + u22)
                    put(1, u21 + u22)
                    put(4, u12 - u22)
                bg.charge(U_COST)
                tails(every.pop(0))

    if _ONLY is not None:
        for r_ in (xn_u, XL_u, WB_u, UL_u, WO_u, z1_v, R_u, Lc_u, zf_v, zg_v, kv_u, u_u, X_v, H_v, G_v, Z_u, kf_v, bcol_v):
            c_ = pltpu.make_async_copy(r_, r_, sem_small.at[0])
            c_.start()
            c_.wait()

    cp_x(0).start()
    cp_win(0).start()
    cp_x(1).start()
    cp_win(1).start()
    start(cp_small())
    for c in range(2, 5):
        cp_win(c).start()
    cp_x(2).start()

    kk = _odd_freq(jax.lax.broadcasted_iota(jnp.int32, (P, P), 0))
    nn = jax.lax.broadcasted_iota(jnp.int32, (P, P), 1)
    fc, fs = _cos_sin((kk * (4 * nn - 127)) & 2047)
    for g in range(P // 8):
        F_v[g * 16:(g + 1) * 16, 0:P] = jnp.concatenate(
            [fc[g * 8:(g + 1) * 8], -fs[g * 8:(g + 1) * 8]], axis=0).astype(BF16)
    fc, fs = _cos_sin((kk * (-127)) & 2047)
    ph_v[0] = fc
    ph_v[1] = fs
    kk = _odd_freq(jax.lax.broadcasted_iota(jnp.int32, (MC, P), 1))
    mm = jax.lax.broadcasted_iota(jnp.int32, (MC, P), 0)
    ic, is_ = _cos_sin((kk * (4 * mm + 2)) & 2047)
    Fi_v[:, 0:P] = (ic * (1.0 / (P * GA))).astype(BF16)
    Fi_v[:, P:2 * P] = (is_ * (1.0 / (P * GA))).astype(BF16)
    kf_v[:, 0:8, :] = jnp.zeros((D // L, 8, L), F32)

    cp_x(0).wait()
    for s in range(TM // 16):
        ln_x(0, s)

    def small_setup():
        sk = sk_in[...].astype(F32)
        for t in range(4):
            sk_v[t] = jnp.broadcast_to(sk[t:t + 1], (8, D))
        drow = d_in[...].astype(F32).reshape(1, D)
        for l in range(D // L):
            lanes = slice(l * L, (l + 1) * L)
            dre = ph_v[0] * drow[:, lanes]
            dim = ph_v[1] * drow[:, lanes]
            H_v[0, 0, 0:64, lanes] = -dim[0:64]
            H_v[0, 0, 64:P, lanes] = dim[64:P]
            H_v[0, 1, 0:64, lanes] = -dre[0:64]
            H_v[0, 1, 64:P, lanes] = dre[64:P]

    def bcol_task(t, j, tie):
        brow = b_in[...].astype(F32).reshape(1, S)[:, j * P:(j + 1) * P] * (0.25 / GA) + tie[0:1]
        bcol_v[j * P:(j + 1) * P, :] = jnp.broadcast_to(brow, (P, P)).T

    LAG = 2

    def interleave(*lists):
        out = []
        for j in range(max(len(a) for a in lists)):
            for a in lists:
                out += a[j:j + 1]
        return out

    def p1_first(c):
        bg = _Background()
        todo = []
        if c == 2:
            todo = tasks(bcol_task, 0)
            small_setup()
        if c == 3:
            todo = tasks(ln_z2, 0)
            bg.add(wcomb_gen(range(3)))
        if c == 4:
            todo = tasks(ln_x2, 2, 8)
            bg.add(wcomb_gen(range(3, 6)))
        tied = _Tied(todo, F_TIED[c])
        if c == 0:
            for s in range(TM // 16):
                ln_x(1, s)
        for t in range(2):
            for m in range(TM // MC):
                job_z(t, m, range(*WIN_CHUNKS[c]), bg, F_B, tied)
        bg.drain()
        assert not tied.tasks

    for c in range(5):
        cp_win(c).wait()
        if c == 0:
            cp_x(1).wait()
        if c == 2:
            wait(cp_small())
            start(cp_conv(0))
            cp_x(3).start()
        if c == 4:
            cp_x(2).wait()
            cp_x(4).start()
            cp_x(5).start()
        block(lambda c=c: p1_first(c), f'p1_f{c}')

    def p1_dma(g):
        if g == 0:
            wait(cp_conv(0))
            cp_x(3).wait()
            start(cp_conv(1))
            cp_x(6).start()
            cp_x(7).start()
            start(cp_conv(2))
        if g == 1:
            wait(cp_conv(1))
            cp_x(4).wait()
            cp_x(5).wait()
            start(cp_conv(3))
            start(cp_conv(4))
        if g == 2:
            wait(cp_conv(2))
            wait(cp_conv(3))
            cp_x(6).wait()
            cp_x(7).wait()
            start(cp_conv(5))
            cp_wout().start()
            start(cp_wsp(0))
            start(cp_wsp(1))
        if g == 3:
            wait(cp_conv(4))
            wait(cp_conv(5))
            cp_wout().wait()
            wait(cp_wsp(0))
            start(cp_conv(6))
            start(cp_wsp(2))
            start(cp_conv(7))

    def take(gen, n):
        for _ in range(n):
            yield next(gen)

    def p1_step(i):
        bg = _Background()
        dft = _Background()
        t = i - LAG
        xg = P1_XG[i]
        kv = kv_gen(t)
        nx, nz, nh = KV_SPLIT if xg is not None else (0, KV_SPLIT[0] + KV_SPLIT[1], KV_SPLIT[2])
        dft.add(take(kv, nx))
        bg.add(take(kv, nz))
        hbg = _Background()
        hbg.add(take(kv, nh))
        zb = nz * KV_COST / 48.0
        extra = 0
        if i == 6:
            bg.add(wocomb_gen())
            bg.add(acomb_gen(0, range(3)))
            extra = 42
        if i == 7:
            bg.add(acomb_gen(0, range(3, 8)))
            extra = 24
        last = i == NT - 1
        z2t = tasks(ln_z2, i - 1)
        todo = interleave(*([tasks(ln_x2, t_, 8) for t_ in P1_LNX[i]] + [z2t[0::2], z2t[1::2]]))
        tied = _Tied(todo, 24 if last else TIED_N)
        if xg is not None:
            dft.run(KV_COST)
            job_x(xg, dft, (nx - 1) * KV_COST / 10.0)
            dft.drain()
        for p in range(2):
            for j in range(FH // L):
                job_zs(i, p, j, bg, (1.6 * zb + extra, 0.5 * zb + extra), tied)
            assert not tied.tasks or (p == 0 and not last)
            if p == 0 and last:
                tied = _Tied(tasks(ln_z2, i, 8), 22)
        if last:
            for s in range(8, 16):
                ln_z2(i, s)
        bg.drain()
        job_h(t, hbg, nh * KV_COST / 10.0)
        hbg.drain()

    def p1_block(g):
        for i in P1_GROUPS[g]:
            p1_step(i)

    for g in range(len(P1_GROUPS)):
        p1_dma(g)
        block(lambda g=g: p1_block(g), f'p1_g{g}')

    groups = P2_GROUPS
    NG = len(groups)

    def p2_dma(gi):
        if gi >= 2:
            for i in groups[gi - 2]:
                start(cp_out(i))
        if gi >= 3:
            for i in groups[gi - 3]:
                wait(cp_out(i))
        if gi + 2 < NG:
            for i in groups[gi + 2]:
                start(cp_wsp(i))
        if gi < 2:
            wait(cp_conv(NT - 2 + gi))
        if gi + 1 < NG:
            for i in groups[gi + 1]:
                wait(cp_wsp(i))

    def tails_of(i, bg, budget):
        return [tail_gen(i, bg, budget)] * 20

    def p2_block(gi):
        bg = _Background()
        steps = groups[gi]
        tb = [0.0]
        pending = [t_ for i in (groups[gi - 1] if gi > 0 else []) for t_ in tails_of(i, bg, tb)]
        total = sum(a + 1 for i in steps for a in _blocks_of_step(i)) * 40 * 16
        total += len(steps) * (24 * E_COST + 6 * U_COST) + len(pending) * T_COST
        slots = 84 * len(steps) + TAIL_W * len(pending)
        bg.add(freq_gen(_blocks_of_step(steps[0])[0]))
        if gi < 2:
            bg.add(kv_gen(NT - 2 + gi))
            total += 20 * KV_COST
            slots += 10
        for t in P2_XG[gi]:
            slots += 10
        if gi + 1 < NG:
            for i in groups[gi + 1]:
                bg.add(acomb_gen(i))
                total += 32 * A_COST
        for i in steps[1:]:
            bg.add(freq_gen(_blocks_of_step(i)[0]))
        budget = tb[0] = total / (slots + 1.0)
        bg.run(budget)
        for t in P2_XG[gi]:
            job_x(t, bg, budget)
        if gi < 2:
            job_h(NT - 2 + gi, bg, budget)
        units = [4, 4, 2, 4, 4, 2] * (len(pending) // 20)
        every = [0] * (6 * len(steps))
        for j, n in enumerate(units):
            every[min(len(every) - 1, j * len(every) // len(units))] += n
        for i in steps:
            job_big(i, bg, pending, budget, every)
        for t_ in pending:
            next(t_)
        bg.drain()

    for gi in range(NG):
        p2_dma(gi)
        block(lambda gi=gi: p2_block(gi), f'p2_{gi}')

    def cp_last(upper):
        a0 = _blocks_of_step(NT - 1)[0]
        return [pltpu.make_async_copy(o_v.at[pl.ds(r, MC)], o_hbm.at[0, pl.ds(r, MC)], sem_out.at[(NT - 1) % 5])
                for r in ((a0 + w) * P + (MC if upper else 0) for w in range(2))]

    def p2_last():
        for j, t_ in enumerate(tails_of(NT - 1, _Background(), [0.0])):
            next(t_)
            if j == 9:
                start(cp_last(True))

    p2_dma(NG)
    block(p2_last, 'p2_last')
    start(cp_last(False))
    for i in groups[NG - 2]:
        wait(cp_out(i))
    wait(cp_last(True))
    wait(cp_last(False))
    if _ONLY is not None:
        for r_ in (xn_u, XL_u, WB_u, UL_u, WO_u, z1_v, R_u, Lc_u, zf_v, zg_v, kv_u, u_u, X_v, H_v, G_v, Z_u, kf_v, bcol_v):
            c_ = pltpu.make_async_copy(r_, r_, sem_small.at[0])
            c_.start()
            c_.wait()


@jax.jit
def pallas_recurrent_scan__ssm_conv_h3__mixer_gmlp__prompt_kernel(
    A_q: jax.Array,
    A_k: jax.Array,
    A_v: jax.Array,
    A_shift_k: jax.Array,
    A_ssm_k: jax.Array,
    A_ssm_D: jax.Array,
    B_x: jax.Array,
    B_w_in: jax.Array,
    B_w_sp: jax.Array,
    B_b_sp: jax.Array,
    B_w_out: jax.Array,
):
    del B_x
    hbm = pl.BlockSpec(memory_space=pl.ANY)

    def bf16_buf(*shape):
        return pltpu.VMEM(shape[:-2] + (shape[-2] // 2, shape[-1]), U32)

    return pl.pallas_call(
        _kernel,
        out_shape=jax.ShapeDtypeStruct((1, S, D), BF16),
        in_specs=[hbm] * 10,
        out_specs=hbm,
        scratch_shapes=[
            bf16_buf(S, D),
            bf16_buf(S, D),
            bf16_buf(S, D),
            bf16_buf(NT, D, TM),
            bf16_buf(D, 2 * FH),
            bf16_buf(S, S),
            bf16_buf(FH, D),
            pltpu.VMEM((S, D), BF16),
            pltpu.VMEM((4, D), BF16),
            pltpu.VMEM((D,), BF16),
            pltpu.VMEM((S,), BF16),
            bf16_buf(S, D),
            bf16_buf(4 * 5 * P, KH),
            bf16_buf(5 * KH, FH),
            bf16_buf(4 * 5 * P, HN),
            bf16_buf(5 * HN, 2 * L),
            pltpu.VMEM((S, FH), F32),
            bf16_buf(7 * HK, HN),
            bf16_buf(4 * 5 * P, HK),
            pltpu.VMEM((HK, FH), F32),
            pltpu.VMEM((3, TM, FH), F32),
            bf16_buf(S, D),
            bf16_buf(S, FH),
            pltpu.VMEM((NB, 2, P, D), F32),
            pltpu.VMEM((2, 2, P, D), F32),
            pltpu.VMEM((NB, 2, P, D), F32),
            bf16_buf(NB * 2 * P, D),
            pltpu.VMEM((2, D // L, MC, L), F32),
            bf16_buf(2 * P, 2 * P),
            bf16_buf(MC, 2 * P),
            pltpu.VMEM((S, L), F32),
            pltpu.VMEM((2, P, L), F32),
            pltpu.VMEM((4, 8, D), F32),
            pltpu.VMEM((D // L, S + 8, L), F32),
            pltpu.SemaphoreType.DMA((1,)),
            pltpu.SemaphoreType.DMA((5,)),
            pltpu.SemaphoreType.DMA((4,)),
            pltpu.SemaphoreType.DMA((5,)),
            pltpu.SemaphoreType.DMA((5,)),
            pltpu.SemaphoreType.DMA((5,)),
        ],
        compiler_params=pltpu.CompilerParams(vmem_limit_bytes=116 * 1024 * 1024, disable_semaphore_checks=True),
    )(A_q, A_k, A_v, A_shift_k.T, A_ssm_k, A_ssm_D, B_w_in, B_w_sp, B_b_sp, B_w_out)
```

```python
import math

import jax
import jax.numpy as jnp
import jax.experimental.pallas as pl
import jax.experimental.pallas.tpu as pltpu

S = 2048
D = 640
FH = 768
P = 128
NB = S // P
TM = 256
NT = S // TM
MC = 64
L = 128
HK = S // 2
KH = 256
HN = FH // 2
P1_GROUPS = ((2,), (3,), (4, 5), (6, 7))
P1_XG = {2: None, 3: 0, 4: 1, 5: None, 6: 2, 7: 3}
P1_LNX = {2: (3,), 3: (4, 5), 4: (6,), 5: (7,), 6: (), 7: ()}
P2_XG = ((4, 5), (6,), (7,), ())
P2_GROUPS = ((0,), (1, 2), (3, 4, 5), (6, 7))
STEP_BLOCKS = ((6, 7), (8, 9), (4, 5), (12, 13), (10, 11), (0, 1), (14, 15), (2, 3))
KV_COST, G_COST, A_COST = 110, 36, 56
E_COST, U_COST, T_COST, TAIL_W = 24, 90, 90, 1.6
BIG_KG = 512
TIE_X = False
DFT_B = (130, 80)
Z_B0, Z_B1 = 60, 10
TIED_N = 42
ORDER = 1
ZS_MID = 0.0
H_SPLIT = ((0, 2), (2, 4), (4, 5))
KV_SPLIT = (12, 4, 4)
F_TIED = (20, 20, 18, 20, 20)
F_B = (80, 40)
FR = 16
KV_ROWS = 64
WIN_CHUNKS = ((6, 7), (7, 9), (9, 12), (0, 3), (3, 6))
EPS = 1e-5
F32 = jnp.float32
BF16 = jnp.bfloat16
U32 = jnp.uint32
GELU_C = math.sqrt(2.0 / math.pi)
GA = (GELU_C * 0.044715) ** (1.0 / 3.0)
NT_DIMS = (((1,), (1,)), ((), ()))
_ONLY = None


def _dot(a, b):
    return jnp.dot(a, b, preferred_element_type=F32)


def _cos_sin(m):
    q = (m + 256) >> 9
    x = (m - (q << 9)).astype(F32) * (2.0 * math.pi / 2048.0)
    x2 = x * x
    s = x * (1.0 + x2 * (-1.0 / 6 + x2 * (1.0 / 120 + x2 * (-1.0 / 5040 + x2 * (1.0 / 362880)))))
    c = 1.0 + x2 * (-0.5 + x2 * (1.0 / 24 + x2 * (-1.0 / 720 + x2 * (1.0 / 40320 - x2 * (1.0 / 3628800)))))
    swap = (q & 1) == 1
    c0 = jnp.where(swap, s, c)
    s0 = jnp.where(swap, c, s)
    cos = jnp.where(((q + 1) & 2) == 2, -c0, c0)
    sin = jnp.where((q & 2) == 2, -s0, s0)
    return cos, sin


def _odd_freq(r):
    return jnp.where(r < 64, 4 * r + 1, 4 * r - 253)


def _gelu_scaled(z):
    return z + z * jnp.tanh(z * (GELU_C / GA + z * z))


def _signzero(z):
    bits = jax.lax.bitcast_convert_type(z, U32) & jnp.uint32(0x80000000)
    return jax.lax.bitcast_convert_type(bits, F32)


def _ln(x, eps, tie=None, scale=None):
    n = x.shape[-1]
    cols = [x[:, j * L:(j + 1) * L] for j in range(n // L)]
    s1 = cols[0]
    s2 = cols[0] * cols[0]
    for c in cols[1:]:
        s1 = s1 + c
        s2 = s2 + c * c
    if tie is not None:
        s1 = s1 + tie
        s2 = s2 + tie
    m = jnp.sum(s1, axis=-1, keepdims=True) * (1.0 / n)
    v = jnp.maximum(jnp.sum(s2, axis=-1, keepdims=True) * (1.0 / n) - m * m, 0.0)
    rs = jax.lax.rsqrt(v + eps)
    if scale is not None:
        rs = rs * scale
    return (x - m) * rs


def _blocks_of_step(i):
    return STEP_BLOCKS[i]


class _Background:
    def __init__(self):
        self.q = []
        self.credit = 0.0

    def add(self, gen):
        self.q.append(gen)

    def run(self, budget):
        self.credit += budget
        while self.q and self.credit > 0:
            try:
                self.credit -= next(self.q[0])
            except StopIteration:
                self.q.pop(0)
        if not self.q:
            self.credit = 0.0

    def charge(self, cost):
        self.credit -= cost

    def drain(self):
        while self.q:
            self.run(1e9)


class _Tied:
    def __init__(self, tasks, npieces):
        self.tasks = list(tasks)
        self.rate = len(self.tasks) / float(npieces)
        self.credit = 0.999

    def run(self, z):
        self.credit += self.rate
        n = 0
        while self.tasks and self.credit >= 1.0:
            self.tasks.pop(0)(_signzero(z[0:16]))
            self.credit -= 1.0
            n += 1
        return n


def _kernel(q_hbm, k_hbm, v_hbm, sk_hbm, h_hbm, d_hbm, win_hbm, wsp_hbm, b_hbm, wout_hbm,
            o_hbm,
            x_u, k_u, v_u, h_u, win_u, wsp_u, wout_u, o_v, sk_in, d_in, b_in,
            xn_u, XL_u, WB_u, UL_u, WO_u, z1_v, R_u, Lc_u, zf_v, zg_v, kv_u, u_u, X_v, H_v, G_v, Z_u, yl_v, F_u, Fi_u, bcol_v, ph_v, sk_v, kf_v,
            sem_small, sem_x, sem_conv, sem_wsp, sem_w, sem_out):
    x_v, k_v, v_v, h_v, win_v, wsp_v, wout_v, xn_v, XL_v, WB_v, UL_v, WO_v, R_v, Lc_v, kv_v, u_v, Z_v, F_v, Fi_v = [
        r.bitcast(BF16) for r in (x_u, k_u, v_u, h_u, win_u, wsp_u, wout_u, xn_u, XL_u, WB_u, UL_u, WO_u, R_u, Lc_u, kv_u, u_u, Z_u, F_u,
                                  Fi_u)]

    def cp_small():
        return [pltpu.make_async_copy(s_, d_, sem_small.at[0])
                for s_, d_ in ((d_hbm, d_in), (sk_hbm, sk_in), (b_hbm, b_in))]

    def cp_x(t, n=1):
        rows = pl.ds(t * TM, n * TM)
        return pltpu.make_async_copy(q_hbm.at[0, rows], x_v.at[rows], sem_x.at[t])

    def cp_conv(t, n=1):
        rows = pl.ds(t * TM, n * TM)
        sem = sem_conv.at[t]
        return [pltpu.make_async_copy(h_hbm.at[:, rows], h_v.at[:, rows], sem),
                pltpu.make_async_copy(k_hbm.at[0, rows], k_v.at[rows], sem),
                pltpu.make_async_copy(v_hbm.at[0, rows], v_v.at[rows], sem)]

    def cp_wsp(i):
        return [pltpu.make_async_copy(wsp_hbm.at[pl.ds(_blocks_of_step(i)[0] * P, TM)],
                                      wsp_v.at[pl.ds(i * TM, TM)], sem_wsp.at[i])]

    def cp_win(c):
        lo, hi = WIN_CHUNKS[c]
        cols = pl.ds(lo * L, (hi - lo) * L)
        return pltpu.make_async_copy(win_hbm.at[:, cols], win_v.at[:, cols], sem_w.at[c])

    def cp_wout():
        return pltpu.make_async_copy(wout_hbm, wout_v, sem_w.at[0])

    def cp_out(i):
        rows = pl.ds(_blocks_of_step(i)[0] * P, TM)
        return [pltpu.make_async_copy(o_v.at[rows], o_hbm.at[0, rows], sem_out.at[i])]

    def start(cs):
        for c in cs:
            c.start()

    def wait(cs):
        for c in cs:
            c.wait()

    def block(fn, name):
        def body(it):
            fn()
            return it + 1

        if _ONLY is None or name in _ONLY:
            jax.lax.while_loop(lambda it: it < 1, body, jnp.int32(0))

    def ln_x(t, s, tie=None):
        rows = pl.ds(t * TM + s * 16, 16)
        y = _ln(x_v[rows, :].astype(F32), EPS, tie, GA)
        xn_v[rows, :] = y.astype(BF16)
        return y

    def ln_x2(t, s, tie):
        p, q = s // 4, s % 4
        y1 = ln_x(t, 8 * p + q, tie)
        y2 = ln_x(t, 8 * p + 4 + q, tie)
        a11, a12, a21, a22 = y1[:, :KH], y1[:, KH:2 * KH], y2[:, :KH], y2[:, KH:2 * KH]
        r0 = (t % 4) * 5 * P + p * MC + q * 16
        for j, c in enumerate((a11 + a22, a21 + a22, a11 + a12, a21 - a11, a12 - a22)):
            XL_v[pl.ds(r0 + j * P, 16), :] = c.astype(BF16)

    def wcomb_gen(cols):
        for j in cols:
            c1 = slice(j * L, (j + 1) * L)
            c2 = slice(FH + j * L, FH + (j + 1) * L)
            for r in range(KH // 32):
                top = pl.ds(r * 32, 32)
                bot = pl.ds(KH + r * 32, 32)
                b11, b12 = win_v[top, c1].astype(F32), win_v[top, c2].astype(F32)
                b21, b22 = win_v[bot, c1].astype(F32), win_v[bot, c2].astype(F32)
                for w, c in enumerate((b11 + b22, b12 - b22, b21 - b11, b11 + b12, b21 + b22)):
                    WB_v[pl.ds(w * KH + r * 32, 32), c1] = c.astype(BF16)
                yield A_COST

    def ln_z2(t, s, tie=None):
        y = _ln(zg_v[t % 3, s * 16:(s + 1) * 16, :], 4.0 * GA * GA * EPS, tie, 0.25 / GA)
        lo, hi = y[:, :HN], y[:, HN:]
        r = (t * TM + s * 16) % HK
        rows = pl.ds(r, 16)
        if t < NT // 2:
            zf_v[rows, :] = y
            R_v[pl.ds(1 * HK + r, 16), :] = lo.astype(BF16)
            R_v[pl.ds(5 * HK + r, 16), :] = (lo + hi).astype(BF16)
        else:
            b11, b12 = zf_v[rows, :HN], zf_v[rows, HN:]
            R_v[pl.ds(0 * HK + r, 16), :] = (b11 + hi).astype(BF16)
            R_v[pl.ds(2 * HK + r, 16), :] = (b12 - hi).astype(BF16)
            R_v[pl.ds(3 * HK + r, 16), :] = (lo - b11).astype(BF16)
            R_v[pl.ds(4 * HK + r, 16), :] = hi.astype(BF16)
            R_v[pl.ds(6 * HK + r, 16), :] = (lo + hi).astype(BF16)

    def acomb_gen(i, groups=range(P // 16)):
        for r in groups:
            for c in range(HK // 256):
                top = pl.ds(i * TM + r * 16, 16)
                bot = pl.ds(i * TM + P + r * 16, 16)
                c1 = slice(c * 256, (c + 1) * 256)
                c2 = slice(HK + c * 256, HK + (c + 1) * 256)
                a11 = wsp_v[top, c1].astype(F32)
                a12 = wsp_v[top, c2].astype(F32)
                a21 = wsp_v[bot, c1].astype(F32)
                a22 = wsp_v[bot, c2].astype(F32)
                r0 = (i % 5) * 5 * P + r * 16
                Lc_v[pl.ds(r0 + 0 * P, 16), c1] = (a11 + a22).astype(BF16)
                Lc_v[pl.ds(r0 + 1 * P, 16), c1] = (a21 + a22).astype(BF16)
                Lc_v[pl.ds(r0 + 2 * P, 16), c1] = (a11 + a12).astype(BF16)
                Lc_v[pl.ds(r0 + 3 * P, 16), c1] = (a21 - a11).astype(BF16)
                Lc_v[pl.ds(r0 + 4 * P, 16), c1] = (a12 - a22).astype(BF16)
                yield A_COST

    def tasks(fn, t, n=TM // 16):
        return [lambda tie, s=s: fn(t, s, tie) for s in range(n)]

    def kv_gen(t):
        for m in range(TM // KV_ROWS):
            r = t * TM + m * KV_ROWS
            for l in range(D // L):
                lanes = slice(l * L, (l + 1) * L)
                kf = k_v[pl.ds(r, KV_ROWS), lanes].astype(F32)
                kf_v[l, pl.ds(r + 8, KV_ROWS), :] = kf
                ks = kf * sk_v[0, 0:1, lanes]
                for tap in range(1, 4):
                    ks = ks + kf_v[l, pl.ds(r + 8 - tap, KV_ROWS), :] * sk_v[tap, 0:1, lanes]
                kv = ks * v_v[pl.ds(r, KV_ROWS), lanes].astype(F32)
                kv_v[pl.ds(r, KV_ROWS), lanes] = kv.astype(BF16)
                yield KV_COST * KV_ROWS / 64

    def freq_gen(a):
        def cmac(acc, x, g):
            pr = x[0] * g[0] - x[1] * g[1]
            pi = x[0] * g[1] + x[1] * g[0]
            return (pr, pi) if acc is None else (acc[0] + pr, acc[1] + pi)

        for r in range(P // 16):
            for l in range(D // L):
                lanes = slice(l * L, (l + 1) * L)
                res = []
                for sub in range(16 // FR):
                    rows = pl.ds(r * 16 + sub * FR, FR)
                    lo = hi = None
                    g = (G_v[a + 1, 0, rows, lanes], G_v[a + 1, 1, rows, lanes])
                    for c in range(a + 2):
                        x = (X_v[c, 0, rows, lanes], X_v[c, 1, rows, lanes])
                        hi = cmac(hi, x, g)
                        if c <= a:
                            g = (G_v[a - c, 0, rows, lanes], G_v[a - c, 1, rows, lanes])
                            lo = cmac(lo, x, g)
                            yield 2 * FR
                    res.append((lo, hi))
                for w in range(2):
                    for part in range(2):
                        Z_v[pl.ds((a + w) * 2 * P + part * P + r * 16, 16), lanes] = jnp.concatenate(
                            [z[w][part] for z in res], axis=0).astype(BF16)
                yield 20

    def job_x(t, bg, budget):
        for j in (2 * t, 2 * t + 1):
            for half in range(2):
                r = _dot(F_v[half * P:(half + 1) * P, 0:P], kv_v[j * P:(j + 1) * P, :]).reshape(8, 2, 8, D)
                for part in range(2):
                    X_v[j, part, half * 64:(half + 1) * 64, :] = r[:, part].reshape(64, D)
                bg.run(budget * 2.5)

    def job_h(t, bg, budget):
        for half in range(2):
            rows = pl.ds(half * 64, 64)
            for l0, l1 in H_SPLIT:
                w = (l1 - l0) * L
                lanes = slice(l0 * L, l1 * L)
                rhs = jnp.concatenate([h_v[lanes, t * TM:t * TM + P], h_v[lanes, t * TM + P:(t + 1) * TM]], axis=0)
                r = jax.lax.dot_general(F_v[half * P:(half + 1) * P, 0:P], rhs, NT_DIMS,
                                        preferred_element_type=F32).reshape(8, 2, 8, 2 * w)
                re, im = r[:, 0].reshape(64, 2 * w), r[:, 1].reshape(64, 2 * w)
                prev = (H_v[t % 2, 0, rows, lanes], H_v[t % 2, 1, rows, lanes])
                for j in range(2):
                    cur = (re[:, j * w:(j + 1) * w], im[:, j * w:(j + 1) * w])
                    G_v[2 * t + j, 0, rows, lanes] = cur[0] + prev[1] if half else cur[0] - prev[1]
                    G_v[2 * t + j, 1, rows, lanes] = cur[1] - prev[0] if half else cur[1] + prev[0]
                    prev = cur
                if t + 1 < NT:
                    H_v[(t + 1) % 2, 0, rows, lanes] = prev[0]
                    H_v[(t + 1) % 2, 1, rows, lanes] = prev[1]
                bg.run(budget * (l1 - l0))

    def z_out(t, m, n, pre, bg, budget, tied):
        z = _gelu_scaled(pre)
        if n < FH // L:
            z1_v[pl.ds(t * TM + m * MC, MC), n * L:(n + 1) * L] = z
        else:
            zg_v[t % 3, m * MC:(m + 1) * MC, n * L - FH:(n + 1) * L - FH] = z
        ntask = tied.run(z)
        bg.run(budget[1] if ntask else budget[0])

    def job_z(t, m, cols, bg, budget, tied):
        for n in cols:
            z_out(t, m, n, _dot(xn_v[pl.ds(t * TM + m * MC, MC), :], win_v[:, n * L:(n + 1) * L]), bg, budget, tied)

    def job_zs(t, p, j, bg, budget, tied):
        r1 = pl.ds(t * TM + p * P, MC)
        r2 = pl.ds(t * TM + p * P + MC, MC)
        c1 = slice(j * L, (j + 1) * L)
        c2 = slice(FH + j * L, FH + (j + 1) * L)

        def xl(w):
            r0 = (t % 4) * 5 * P + w * P + p * MC
            return XL_v[r0:r0 + MC, :]

        def wb(w):
            return WB_v[w * KH:(w + 1) * KH, c1]

        def rem(rows, cols):
            return _dot(xn_v[rows, 2 * KH:], win_v[2 * KH:, cols])

        def dot2(a, b):
            r = _dot(a, b)
            bg.run(mid)
            return r

        mid = ZS_MID * budget[0]
        budget = (budget[0] - 1.75 * mid, budget[1] - 1.75 * mid)
        m2 = dot2(xl(1), win_v[0:KH, c1])
        m4 = dot2(xn_v[r2, KH:2 * KH], wb(2))
        z_out(t, 2 * p + 1, j, m2 + m4 + rem(r2, c1), bg, budget, tied)
        m3 = dot2(xn_v[r1, 0:KH], wb(1))
        m5 = dot2(xl(2), win_v[KH:2 * KH, c2])
        z_out(t, 2 * p, 6 + j, m3 + m5 + rem(r1, c2), bg, budget, tied)
        t11, t22 = m4 - m5, m3 - m2
        m1 = dot2(xl(0), wb(0))
        t11, t22 = t11 + m1, t22 + m1
        z_out(t, 2 * p, j, t11 + dot2(xl(4), wb(4)) + rem(r1, c1), bg, budget, tied)
        z_out(t, 2 * p + 1, 6 + j, t22 + dot2(xl(3), wb(3)) + rem(r2, c2), bg, budget, tied)

    rev8 = 7 - jax.lax.broadcasted_iota(jnp.int32, (8, L), 0)

    def finish(a, upper, n, hh, slot):
        rows = pl.ds(a * P + (MC if upper else 0), MC)
        lanes = slice(n * L, (n + 1) * L)
        if upper:
            ya = _dot(Fi_v[:, 0:P], Z_v[a * 2 * P:a * 2 * P + P, lanes])
            yb = _dot(Fi_v[:, P:2 * P], Z_v[a * 2 * P + P:(a + 1) * 2 * P, lanes])
            slot(0.5)
            y = ya - yb
            lo = ya + yb
            for j in range(MC // 8):
                yl_v[a % 2, n, (7 - j) * 8:(8 - j) * 8, :] = jnp.take_along_axis(lo[j * 8:(j + 1) * 8], rev8, axis=0)
        else:
            y = yl_v[a % 2, n]
        gate = hh + hh * jnp.tanh(hh)
        s = xn_v[rows, lanes].astype(F32) * y
        o_v[rows, lanes] = (x_v[rows, lanes].astype(F32) + s * gate).astype(BF16)

    def tail_gen(i, bg, budget):
        a0, a1 = _blocks_of_step(i)

        def slot(w):
            bg.run(w * budget[0])

        def dot3(a, b):
            r = _dot(a, b)
            slot(0.75)
            return r

        for upper in (True, False):
            sub = MC if upper else 0
            r1 = pl.ds(a0 * P + sub, MC)
            r2 = pl.ds(a1 * P + sub, MC)

            def ul(w):
                r0 = ((i % 5) * 5 + w) * P + sub
                return UL_v[r0:r0 + MC, :]

            for j in range(2):
                c1 = slice(j * L, (j + 1) * L)
                c2 = slice((2 + j) * L, (3 + j) * L)

                def wo(w):
                    return WO_v[w * HN:(w + 1) * HN, c1]

                m2 = dot3(ul(1), wout_v[0:HN, c1])
                m4 = dot3(u_v[r2, HN:], wo(2))
                finish(a1, upper, j, m2 + m4, slot)
                bg.charge(T_COST)
                yield
                m3 = dot3(u_v[r1, 0:HN], wo(1))
                m5 = dot3(ul(2), wout_v[HN:, c2])
                finish(a0, upper, 2 + j, m3 + m5, slot)
                bg.charge(T_COST)
                yield
                m1 = dot3(ul(0), wo(0))
                finish(a0, upper, j, (m4 - m5) + m1 + dot3(ul(4), wo(4)), slot)
                bg.charge(T_COST)
                yield
                finish(a1, upper, 2 + j, (m3 - m2) + m1 + dot3(ul(3), wo(3)), slot)
                bg.charge(T_COST)
                yield
            finish(a0, upper, 4, dot3(u_v[r1, 0:HN], wout_v[0:HN, 4 * L:]) + dot3(u_v[r1, HN:], wout_v[HN:, 4 * L:]), slot)
            bg.charge(T_COST)
            yield
            finish(a1, upper, 4, dot3(u_v[r2, 0:HN], wout_v[0:HN, 4 * L:]) + dot3(u_v[r2, HN:], wout_v[HN:, 4 * L:]), slot)
            bg.charge(T_COST)
            yield

    def wocomb_gen():
        for j in range(2):
            c1 = slice(j * L, (j + 1) * L)
            c2 = slice((2 + j) * L, (3 + j) * L)
            for r in range(HN // 32):
                top = pl.ds(r * 32, 32)
                bot = pl.ds(HN + r * 32, 32)
                b11, b12 = wout_v[top, c1].astype(F32), wout_v[top, c2].astype(F32)
                b21, b22 = wout_v[bot, c1].astype(F32), wout_v[bot, c2].astype(F32)
                for w, c in enumerate((b11 + b22, b12 - b22, b21 - b11, b11 + b12, b21 + b22)):
                    WO_v[pl.ds(w * HN + r * 32, 32), c1] = c.astype(BF16)
                yield A_COST

    def job_big(i, bg, pending, budget, every):
        a0, a1 = _blocks_of_step(i)
        KG = BIG_KG

        def lhs(j, sub, cols):
            if j == 2:
                return wsp_v[i * TM + sub:i * TM + sub + MC, cols]
            if j == 3:
                return wsp_v[i * TM + P + sub:i * TM + P + sub + MC, HK + cols.start:HK + cols.stop]
            r0 = ((i % 5) * 5 + {0: 0, 1: 1, 4: 2, 5: 3, 6: 4}[j]) * P + sub
            return Lc_v[r0:r0 + MC, cols]

        def prod(j, sub, n, acc=None):
            for kg in range(HK // KG):
                ks = slice(kg * KG, (kg + 1) * KG)
                p = _dot(lhs(j, sub, ks), R_v[j * HK + kg * KG:j * HK + (kg + 1) * KG, n * L:(n + 1) * L])
                acc = p if acc is None else acc + p
                bg.run(budget * KG / 512)
            return acc

        def tails(n):
            for _ in range(n):
                if pending:
                    next(pending.pop(0))

        def emit(a, sub, n, g):
            rows = pl.ds(a * P + sub, MC)
            lanes = slice(n * L, (n + 1) * L)
            u = z1_v[rows, lanes] * (g + bcol_v[rows, :])
            u_v[rows, lanes] = u.astype(BF16)
            bg.charge(E_COST)
            return u

        for sub in (0, MC):
            for n in range(HN // L):
                def put(w, c):
                    UL_v[pl.ds(((i % 5) * 5 + w) * P + sub, MC), n * L:(n + 1) * L] = c.astype(BF16)

                if ORDER == 0:
                    m2 = prod(1, sub, n)
                    m4 = prod(3, sub, n)
                    u21 = emit(a1, sub, n, m2 + m4)
                    m3 = prod(2, sub, n)
                    t22 = m3 - m2
                    m5 = prod(4, sub, n)
                    u12 = emit(a0, sub, n + HN // L, m3 + m5)
                    t11 = m4 - m5
                    m1 = prod(0, sub, n)
                    u11 = emit(a0, sub, n, prod(6, sub, n, t11 + m1))
                    u22 = emit(a1, sub, n + HN // L, prod(5, sub, n, t22 + m1))
                    for w, c in enumerate((u11 + u22, u21 + u22, u11 + u12, u21 - u11, u12 - u22)):
                        put(w, c)
                else:
                    m1 = prod(0, sub, n)
                    t11 = prod(6, sub, n, m1)
                    m4 = prod(3, sub, n)
                    t11 = t11 + m4
                    m5 = prod(4, sub, n)
                    u11 = emit(a0, sub, n, t11 - m5)
                    m2 = prod(1, sub, n)
                    u21 = emit(a1, sub, n, m2 + m4)
                    put(3, u21 - u11)
                    t22 = m1 - m2
                    m3 = prod(2, sub, n)
                    u12 = emit(a0, sub, n + HN // L, m3 + m5)
                    put(2, u11 + u12)
                    u22 = emit(a1, sub, n + HN // L, prod(5, sub, n, t22 + m3))
                    put(0, u11 + u22)
                    put(1, u21 + u22)
                    put(4, u12 - u22)
                bg.charge(U_COST)
                tails(every.pop(0))

    if _ONLY is not None:
        for r_ in (xn_u, XL_u, WB_u, UL_u, WO_u, z1_v, R_u, Lc_u, zf_v, zg_v, kv_u, u_u, X_v, H_v, G_v, Z_u, kf_v, bcol_v):
            c_ = pltpu.make_async_copy(r_, r_, sem_small.at[0])
            c_.start()
            c_.wait()

    cp_x(0).start()
    cp_win(0).start()
    cp_x(1).start()
    cp_win(1).start()
    start(cp_small())
    for c in range(2, 5):
        cp_win(c).start()
    cp_x(2).start()

    kk = _odd_freq(jax.lax.broadcasted_iota(jnp.int32, (P, P), 0))
    nn = jax.lax.broadcasted_iota(jnp.int32, (P, P), 1)
    fc, fs = _cos_sin((kk * (4 * nn - 127)) & 2047)
    for g in range(P // 8):
        F_v[g * 16:(g + 1) * 16, 0:P] = jnp.concatenate(
            [fc[g * 8:(g + 1) * 8], -fs[g * 8:(g + 1) * 8]], axis=0).astype(BF16)
    fc, fs = _cos_sin((kk * (-127)) & 2047)
    ph_v[0] = fc
    ph_v[1] = fs
    kk = _odd_freq(jax.lax.broadcasted_iota(jnp.int32, (MC, P), 1))
    mm = jax.lax.broadcasted_iota(jnp.int32, (MC, P), 0)
    ic, is_ = _cos_sin((kk * (4 * mm + 2)) & 2047)
    Fi_v[:, 0:P] = (ic * (1.0 / (P * GA))).astype(BF16)
    Fi_v[:, P:2 * P] = (is_ * (1.0 / (P * GA))).astype(BF16)
    kf_v[:, 0:8, :] = jnp.zeros((D // L, 8, L), F32)

    cp_x(0).wait()
    for s in range(TM // 16):
        ln_x(0, s)

    def small_setup():
        sk = sk_in[...].astype(F32)
        for t in range(4):
            sk_v[t] = jnp.broadcast_to(sk[t:t + 1], (8, D))
        drow = d_in[...].astype(F32).reshape(1, D)
        for l in range(D // L):
            lanes = slice(l * L, (l + 1) * L)
            dre = ph_v[0] * drow[:, lanes]
            dim = ph_v[1] * drow[:, lanes]
            H_v[0, 0, 0:64, lanes] = -dim[0:64]
            H_v[0, 0, 64:P, lanes] = dim[64:P]
            H_v[0, 1, 0:64, lanes] = -dre[0:64]
            H_v[0, 1, 64:P, lanes] = dre[64:P]

    def bcol_task(t, j, tie):
        brow = b_in[...].astype(F32).reshape(1, S)[:, j * P:(j + 1) * P] * (0.25 / GA) + tie[0:1]
        bcol_v[j * P:(j + 1) * P, :] = jnp.broadcast_to(brow, (P, P)).T

    LAG = 2

    def interleave(*lists):
        out = []
        for j in range(max(len(a) for a in lists)):
            for a in lists:
                out += a[j:j + 1]
        return out

    def p1_first(c):
        bg = _Background()
        todo = []
        if c == 2:
            todo = tasks(bcol_task, 0)
            small_setup()
        if c == 3:
            todo = tasks(ln_z2, 0)
            bg.add(wcomb_gen(range(3)))
        if c == 4:
            todo = tasks(ln_x2, 2, 8)
            bg.add(wcomb_gen(range(3, 6)))
        tied = _Tied(todo, F_TIED[c])
        if c == 0:
            for s in range(TM // 16):
                ln_x(1, s)
        for t in range(2):
            for m in range(TM // MC):
                job_z(t, m, range(*WIN_CHUNKS[c]), bg, F_B, tied)
        bg.drain()
        assert not tied.tasks

    for c in range(5):
        cp_win(c).wait()
        if c == 0:
            cp_x(1).wait()
        if c == 2:
            wait(cp_small())
            start(cp_conv(0))
            cp_x(3).start()
        if c == 4:
            cp_x(2).wait()
            cp_x(4, 2).start()
        block(lambda c=c: p1_first(c), f'p1_f{c}')

    def p1_dma(g):
        if g == 0:
            wait(cp_conv(0))
            cp_x(3).wait()
            start(cp_conv(1))
            cp_x(6, 2).start()
            start(cp_conv(2, 2))
        if g == 1:
            wait(cp_conv(1))
            cp_x(4, 2).wait()
            start(cp_conv(4, 2))
            cp_wout().start()
            start(cp_wsp(0))
            start(cp_wsp(1))
        if g == 2:
            wait(cp_conv(2, 2))
            cp_x(6, 2).wait()
        if g == 3:
            wait(cp_conv(4, 2))
            cp_wout().wait()
            wait(cp_wsp(0))
            start(cp_wsp(2))
            start(cp_conv(6, 2))
            for i in (3, 4, 5):
                start(cp_wsp(i))

    def take(gen, n):
        for _ in range(n):
            yield next(gen)

    def p1_step(i):
        bg = _Background()
        dft = _Background()
        t = i - LAG
        xg = P1_XG[i]
        kv = kv_gen(t)
        nx, nz, nh = KV_SPLIT if xg is not None else (0, KV_SPLIT[0] + KV_SPLIT[1], KV_SPLIT[2])
        dft.add(take(kv, nx))
        bg.add(take(kv, nz))
        hbg = _Background()
        hbg.add(take(kv, nh))
        zb = nz * KV_COST / 48.0
        extra = 0
        if i == 6:
            bg.add(wocomb_gen())
            bg.add(acomb_gen(0, range(3)))
            extra = 42
        if i == 7:
            bg.add(acomb_gen(0, range(3, 8)))
            extra = 24
        last = i == NT - 1
        z2t = tasks(ln_z2, i - 1)
        todo = interleave(*([tasks(ln_x2, t_, 8) for t_ in P1_LNX[i]] + [z2t[0::2], z2t[1::2]]))
        tied = _Tied(todo, 24 if last else TIED_N)
        if xg is not None:
            dft.run(KV_COST)
            job_x(xg, dft, (nx - 1) * KV_COST / 10.0)
            dft.drain()
        for p in range(2):
            for j in range(FH // L):
                job_zs(i, p, j, bg, (1.6 * zb + extra, 0.5 * zb + extra), tied)
            assert not tied.tasks or (p == 0 and not last)
            if p == 0 and last:
                tied = _Tied(tasks(ln_z2, i, 8), 22)
        if last:
            for s in range(8, 16):
                ln_z2(i, s)
        bg.drain()
        job_h(t, hbg, nh * KV_COST / 10.0)
        hbg.drain()

    def p1_block(g):
        for i in P1_GROUPS[g]:
            p1_step(i)

    for g in range(len(P1_GROUPS)):
        p1_dma(g)
        block(lambda g=g: p1_block(g), f'p1_g{g}')

    groups = P2_GROUPS
    NG = len(groups)

    def p2_dma(gi):
        if gi >= 2:
            for i in groups[gi - 2]:
                start(cp_out(i))
        if gi >= 3:
            for i in groups[gi - 3]:
                wait(cp_out(i))
        if gi == 1:
            for i in (6, 7):
                start(cp_wsp(i))
        if gi == 0:
            wait(cp_conv(6, 2))
        if gi + 1 < NG:
            for i in groups[gi + 1]:
                wait(cp_wsp(i))

    def tails_of(i, bg, budget):
        return [tail_gen(i, bg, budget)] * 20

    def p2_block(gi):
        bg = _Background()
        steps = groups[gi]
        tb = [0.0]
        pending = [t_ for i in (groups[gi - 1] if gi > 0 else []) for t_ in tails_of(i, bg, tb)]
        total = sum(a + 1 for i in steps for a in _blocks_of_step(i)) * 40 * 16
        total += len(steps) * (24 * E_COST + 6 * U_COST) + len(pending) * T_COST
        slots = 84 * len(steps) + TAIL_W * len(pending)
        bg.add(freq_gen(_blocks_of_step(steps[0])[0]))
        if gi < 2:
            bg.add(kv_gen(NT - 2 + gi))
            total += 20 * KV_COST
            slots += 10
        for t in P2_XG[gi]:
            slots += 10
        if gi + 1 < NG:
            for i in groups[gi + 1]:
                bg.add(acomb_gen(i))
                total += 32 * A_COST
        for i in steps[1:]:
            bg.add(freq_gen(_blocks_of_step(i)[0]))
        budget = tb[0] = total / (slots + 1.0)
        bg.run(budget)
        for t in P2_XG[gi]:
            job_x(t, bg, budget)
        if gi < 2:
            job_h(NT - 2 + gi, bg, budget)
        units = [4, 4, 2, 4, 4, 2] * (len(pending) // 20)
        every = [0] * (6 * len(steps))
        for j, n in enumerate(units):
            every[min(len(every) - 1, j * len(every) // len(units))] += n
        for i in steps:
            job_big(i, bg, pending, budget, every)
        for t_ in pending:
            next(t_)
        bg.drain()

    for gi in range(NG):
        p2_dma(gi)
        block(lambda gi=gi: p2_block(gi), f'p2_{gi}')

    def cp_last(upper):
        a0 = _blocks_of_step(NT - 1)[0]
        return [pltpu.make_async_copy(o_v.at[pl.ds(r, MC)], o_hbm.at[0, pl.ds(r, MC)], sem_out.at[NT - 1])
                for r in ((a0 + w) * P + (MC if upper else 0) for w in range(2))]

    def p2_last():
        for i in groups[NG - 1]:
            for j, t_ in enumerate(tails_of(i, _Background(), [0.0])):
                next(t_)
                if i < NT - 1 and j == 19:
                    start(cp_out(i))
                if i == NT - 1 and j == 9:
                    start(cp_last(True))

    p2_dma(NG)
    block(p2_last, 'p2_last')
    start(cp_last(False))
    for i in groups[NG - 2] + groups[NG - 1][:-1]:
        wait(cp_out(i))
    wait(cp_last(True))
    wait(cp_last(False))
    if _ONLY is not None:
        for r_ in (xn_u, XL_u, WB_u, UL_u, WO_u, z1_v, R_u, Lc_u, zf_v, zg_v, kv_u, u_u, X_v, H_v, G_v, Z_u, kf_v, bcol_v):
            c_ = pltpu.make_async_copy(r_, r_, sem_small.at[0])
            c_.start()
            c_.wait()


@jax.jit
def pallas_recurrent_scan__ssm_conv_h3__mixer_gmlp__prompt_kernel(
    A_q: jax.Array,
    A_k: jax.Array,
    A_v: jax.Array,
    A_shift_k: jax.Array,
    A_ssm_k: jax.Array,
    A_ssm_D: jax.Array,
    B_x: jax.Array,
    B_w_in: jax.Array,
    B_w_sp: jax.Array,
    B_b_sp: jax.Array,
    B_w_out: jax.Array,
):
    del B_x
    hbm = pl.BlockSpec(memory_space=pl.ANY)

    def bf16_buf(*shape):
        return pltpu.VMEM(shape[:-2] + (shape[-2] // 2, shape[-1]), U32)

    return pl.pallas_call(
        _kernel,
        out_shape=jax.ShapeDtypeStruct((1, S, D), BF16),
        in_specs=[hbm] * 10,
        out_specs=hbm,
        scratch_shapes=[
            bf16_buf(S, D),
            bf16_buf(S, D),
            bf16_buf(S, D),
            bf16_buf(D, S),
            bf16_buf(D, 2 * FH),
            bf16_buf(S, S),
            bf16_buf(FH, D),
            pltpu.VMEM((S, D), BF16),
            pltpu.VMEM((4, D), BF16),
            pltpu.VMEM((D,), BF16),
            pltpu.VMEM((S,), BF16),
            bf16_buf(S, D),
            bf16_buf(4 * 5 * P, KH),
            bf16_buf(5 * KH, FH),
            bf16_buf(5 * 5 * P, HN),
            bf16_buf(5 * HN, 2 * L),
            pltpu.VMEM((S, FH), F32),
            bf16_buf(7 * HK, HN),
            bf16_buf(5 * 5 * P, HK),
            pltpu.VMEM((HK, FH), F32),
            pltpu.VMEM((3, TM, FH), F32),
            bf16_buf(S, D),
            bf16_buf(S, FH),
            pltpu.VMEM((NB, 2, P, D), F32),
            pltpu.VMEM((2, 2, P, D), F32),
            pltpu.VMEM((NB, 2, P, D), F32),
            bf16_buf(NB * 2 * P, D),
            pltpu.VMEM((2, D // L, MC, L), F32),
            bf16_buf(2 * P, 2 * P),
            bf16_buf(MC, 2 * P),
            pltpu.VMEM((S, L), F32),
            pltpu.VMEM((2, P, L), F32),
            pltpu.VMEM((4, 8, D), F32),
            pltpu.VMEM((D // L, S + 8, L), F32),
            pltpu.SemaphoreType.DMA((1,)),
            pltpu.SemaphoreType.DMA((NT,)),
            pltpu.SemaphoreType.DMA((NT,)),
            pltpu.SemaphoreType.DMA((NT,)),
            pltpu.SemaphoreType.DMA((5,)),
            pltpu.SemaphoreType.DMA((NT,)),
        ],
        compiler_params=pltpu.CompilerParams(vmem_limit_bytes=116 * 1024 * 1024, disable_semaphore_checks=True),
    )(A_q, A_k, A_v, A_shift_k.T, A_ssm_k, A_ssm_D, B_w_in, B_w_sp, B_b_sp, B_w_out)
```

```python
import math

import jax
import jax.numpy as jnp
import jax.experimental.pallas as pl
import jax.experimental.pallas.tpu as pltpu

S = 2048
D = 640
FH = 768
P = 128
NB = S // P
TM = 256
NT = S // TM
MC = 64
L = 128
HK = S // 2
KH = 256
HN = FH // 2
EPS = 1e-5
F32 = jnp.float32
BF16 = jnp.bfloat16
U32 = jnp.uint32
GELU_C = math.sqrt(2.0 / math.pi)
GA = (GELU_C * 0.044715) ** (1.0 / 3.0)
NT_DIMS = (((1,), (1,)), ((), ()))

WIN_CHUNKS = ((6, 7), (7, 9), (9, 12), (0, 3), (3, 6))
P1_GROUPS = ((2,), (3,), (4, 5), (6, 7))
P1_X = {2: None, 3: 0, 4: 1, 5: None, 6: 2, 7: 3}
P1_LNX = {2: (3,), 3: (4, 5), 4: (6,), 5: (7,), 6: (), 7: ()}
P2_GROUPS = ((0,), (1, 2), (3, 4, 5), (6, 7))
P2_X = ((4, 5), (6,), (7,), ())
STEP_BLOCKS = ((6, 7), (8, 9), (4, 5), (12, 13), (10, 11), (0, 1), (14, 15), (2, 3))
KV_COST, A_COST = 110, 56
E_COST, U_COST, T_COST, TAIL_W = 24, 90, 90, 1.6
KV_SPLIT = (12, 4, 4)
H_SPLIT = ((0, 2), (2, 4), (4, 5))
TIED_N = 42
F_TIED = (20, 20, 18, 20, 20)
_ONLY = None


def _dot(a, b):
    return jnp.dot(a, b, preferred_element_type=F32)


def _cos_sin(m):
    q = (m + 256) >> 9
    x = (m - (q << 9)).astype(F32) * (2.0 * math.pi / 2048.0)
    x2 = x * x
    s = x * (1.0 + x2 * (-1.0 / 6 + x2 * (1.0 / 120 + x2 * (-1.0 / 5040 + x2 * (1.0 / 362880)))))
    c = 1.0 + x2 * (-0.5 + x2 * (1.0 / 24 + x2 * (-1.0 / 720 + x2 * (1.0 / 40320 - x2 * (1.0 / 3628800)))))
    swap = (q & 1) == 1
    c0 = jnp.where(swap, s, c)
    s0 = jnp.where(swap, c, s)
    cos = jnp.where(((q + 1) & 2) == 2, -c0, c0)
    sin = jnp.where((q & 2) == 2, -s0, s0)
    return cos, sin


def _odd_freq(r):
    return jnp.where(r < 64, 4 * r + 1, 4 * r - 253)


def _gelu_scaled(z):
    return z + z * jnp.tanh(z * (GELU_C / GA + z * z))


def _signzero(z):
    bits = jax.lax.bitcast_convert_type(z, U32) & jnp.uint32(0x80000000)
    return jax.lax.bitcast_convert_type(bits, F32)


def _ln(x, eps, tie=None, scale=None):
    n = x.shape[-1]
    cols = [x[:, j * L:(j + 1) * L] for j in range(n // L)]
    s1 = cols[0]
    s2 = cols[0] * cols[0]
    for c in cols[1:]:
        s1 = s1 + c
        s2 = s2 + c * c
    if tie is not None:
        s1 = s1 + tie
        s2 = s2 + tie
    m = jnp.sum(s1, axis=-1, keepdims=True) * (1.0 / n)
    v = jnp.maximum(jnp.sum(s2, axis=-1, keepdims=True) * (1.0 / n) - m * m, 0.0)
    rs = jax.lax.rsqrt(v + eps)
    if scale is not None:
        rs = rs * scale
    return (x - m) * rs


def _blocks_of_step(i):
    return STEP_BLOCKS[i]


class _Background:
    def __init__(self):
        self.q = []
        self.credit = 0.0

    def add(self, gen):
        self.q.append(gen)

    def run(self, budget):
        self.credit += budget
        while self.q and self.credit > 0:
            try:
                self.credit -= next(self.q[0])
            except StopIteration:
                self.q.pop(0)
        if not self.q:
            self.credit = 0.0

    def charge(self, cost):
        self.credit -= cost

    def drain(self):
        while self.q:
            self.run(1e9)


class _Tied:
    def __init__(self, tasks, npieces):
        self.tasks = list(tasks)
        self.rate = len(self.tasks) / float(npieces)
        self.credit = 0.999

    def run(self, z):
        self.credit += self.rate
        n = 0
        while self.tasks and self.credit >= 1.0:
            self.tasks.pop(0)(_signzero(z[0:16]))
            self.credit -= 1.0
            n += 1
        return n


def _kernel(q_hbm, k_hbm, v_hbm, sk_hbm, h_hbm, d_hbm, win_hbm, wsp_hbm, b_hbm, wout_hbm,
            o_hbm,
            x_u, k_u, v_u, h_u, win_u, wsp_u, wout_u, o_v, sk_in, d_in, b_in,
            xn_u, XL_u, WB_u, UL_u, WO_u, z1_v, R_u, Lc_u, zf_v, zg_v, kv_u, u_u, X_v, H_v, G_v, Z_u,
            yl_v, F_u, Fi_u, bcol_v, ph_v, sk_v, kf_v,
            sem_small, sem_x, sem_conv, sem_wsp, sem_w, sem_out):
    (x_v, k_v, v_v, h_v, win_v, wsp_v, wout_v, xn_v, XL_v, WB_v, UL_v, WO_v, R_v, Lc_v, kv_v, u_v, Z_v,
     F_v, Fi_v) = [r.bitcast(BF16) for r in (x_u, k_u, v_u, h_u, win_u, wsp_u, wout_u, xn_u, XL_u, WB_u, UL_u,
                                             WO_u, R_u, Lc_u, kv_u, u_u, Z_u, F_u, Fi_u)]

    def cp_small():
        return [pltpu.make_async_copy(s_, d_, sem_small.at[0])
                for s_, d_ in ((d_hbm, d_in), (sk_hbm, sk_in), (b_hbm, b_in))]

    def cp_x(t, n=1):
        rows = pl.ds(t * TM, n * TM)
        return pltpu.make_async_copy(q_hbm.at[0, rows], x_v.at[rows], sem_x.at[t])

    def cp_conv(t, n=1):
        rows = pl.ds(t * TM, n * TM)
        sem = sem_conv.at[t]
        return [pltpu.make_async_copy(h_hbm.at[:, rows], h_v.at[:, rows], sem),
                pltpu.make_async_copy(k_hbm.at[0, rows], k_v.at[rows], sem),
                pltpu.make_async_copy(v_hbm.at[0, rows], v_v.at[rows], sem)]

    def cp_wsp(i):
        return [pltpu.make_async_copy(wsp_hbm.at[pl.ds(_blocks_of_step(i)[0] * P, TM)],
                                      wsp_v.at[pl.ds(i * TM, TM)], sem_wsp.at[i])]

    def cp_win(c):
        lo, hi = WIN_CHUNKS[c]
        cols = pl.ds(lo * L, (hi - lo) * L)
        return pltpu.make_async_copy(win_hbm.at[:, cols], win_v.at[:, cols], sem_w.at[c])

    def cp_wout():
        return pltpu.make_async_copy(wout_hbm, wout_v, sem_w.at[0])

    def cp_out(i):
        rows = pl.ds(_blocks_of_step(i)[0] * P, TM)
        return [pltpu.make_async_copy(o_v.at[rows], o_hbm.at[0, rows], sem_out.at[i])]

    def start(cs):
        for c in cs:
            c.start()

    def wait(cs):
        for c in cs:
            c.wait()

    def block(fn, name):
        def body(it):
            fn()
            return it + 1

        if _ONLY is None or name in _ONLY:
            jax.lax.while_loop(lambda it: it < 1, body, jnp.int32(0))

    def ln_x(t, s, tie=None):
        rows = pl.ds(t * TM + s * 16, 16)
        y = _ln(x_v[rows, :].astype(F32), EPS, tie, GA)
        xn_v[rows, :] = y.astype(BF16)
        return y

    def ln_x2(t, s, tie):
        p, q = s // 4, s % 4
        y1 = ln_x(t, 8 * p + q, tie)
        y2 = ln_x(t, 8 * p + 4 + q, tie)
        a11, a12, a21, a22 = y1[:, :KH], y1[:, KH:2 * KH], y2[:, :KH], y2[:, KH:2 * KH]
        r0 = (t % 4) * 5 * P + p * MC + q * 16
        for j, c in enumerate((a11 + a22, a21 + a22, a11 + a12, a21 - a11, a12 - a22)):
            XL_v[pl.ds(r0 + j * P, 16), :] = c.astype(BF16)

    def wcomb_gen(cols):
        for j in cols:
            c1 = slice(j * L, (j + 1) * L)
            c2 = slice(FH + j * L, FH + (j + 1) * L)
            for r in range(KH // 32):
                top = pl.ds(r * 32, 32)
                bot = pl.ds(KH + r * 32, 32)
                b11, b12 = win_v[top, c1].astype(F32), win_v[top, c2].astype(F32)
                b21, b22 = win_v[bot, c1].astype(F32), win_v[bot, c2].astype(F32)
                for w, c in enumerate((b11 + b22, b12 - b22, b21 - b11, b11 + b12, b21 + b22)):
                    WB_v[pl.ds(w * KH + r * 32, 32), c1] = c.astype(BF16)
                yield A_COST

    def ln_z2(t, s, tie=None):
        y = _ln(zg_v[t % 3, s * 16:(s + 1) * 16, :], 4.0 * GA * GA * EPS, tie, 0.25 / GA)
        lo, hi = y[:, :HN], y[:, HN:]
        r = (t * TM + s * 16) % HK
        rows = pl.ds(r, 16)
        if t < NT // 2:
            zf_v[rows, :] = y
            R_v[pl.ds(1 * HK + r, 16), :] = lo.astype(BF16)
            R_v[pl.ds(5 * HK + r, 16), :] = (lo + hi).astype(BF16)
        else:
            b11, b12 = zf_v[rows, :HN], zf_v[rows, HN:]
            R_v[pl.ds(0 * HK + r, 16), :] = (b11 + hi).astype(BF16)
            R_v[pl.ds(2 * HK + r, 16), :] = (b12 - hi).astype(BF16)
            R_v[pl.ds(3 * HK + r, 16), :] = (lo - b11).astype(BF16)
            R_v[pl.ds(4 * HK + r, 16), :] = hi.astype(BF16)
            R_v[pl.ds(6 * HK + r, 16), :] = (lo + hi).astype(BF16)

    def acomb_gen(i, groups=range(P // 16)):
        for r in groups:
            for c in range(HK // 256):
                top = pl.ds(i * TM + r * 16, 16)
                bot = pl.ds(i * TM + P + r * 16, 16)
                c1 = slice(c * 256, (c + 1) * 256)
                c2 = slice(HK + c * 256, HK + (c + 1) * 256)
                a11 = wsp_v[top, c1].astype(F32)
                a12 = wsp_v[top, c2].astype(F32)
                a21 = wsp_v[bot, c1].astype(F32)
                a22 = wsp_v[bot, c2].astype(F32)
                r0 = (i % 5) * 5 * P + r * 16
                Lc_v[pl.ds(r0 + 0 * P, 16), c1] = (a11 + a22).astype(BF16)
                Lc_v[pl.ds(r0 + 1 * P, 16), c1] = (a21 + a22).astype(BF16)
                Lc_v[pl.ds(r0 + 2 * P, 16), c1] = (a11 + a12).astype(BF16)
                Lc_v[pl.ds(r0 + 3 * P, 16), c1] = (a21 - a11).astype(BF16)
                Lc_v[pl.ds(r0 + 4 * P, 16), c1] = (a12 - a22).astype(BF16)
                yield A_COST

    def tasks(fn, t, n=TM // 16):
        return [lambda tie, s=s: fn(t, s, tie) for s in range(n)]

    def kv_gen(t):
        for m in range(TM // MC):
            r = t * TM + m * MC
            for l in range(D // L):
                lanes = slice(l * L, (l + 1) * L)
                kf = k_v[pl.ds(r, MC), lanes].astype(F32)
                kf_v[l, pl.ds(r + 8, MC), :] = kf
                ks = kf * sk_v[0, 0:1, lanes]
                for tap in range(1, 4):
                    ks = ks + kf_v[l, pl.ds(r + 8 - tap, MC), :] * sk_v[tap, 0:1, lanes]
                kv = ks * v_v[pl.ds(r, MC), lanes].astype(F32)
                kv_v[pl.ds(r, MC), lanes] = kv.astype(BF16)
                yield KV_COST

    def freq_gen(a):
        def cmac(acc, x, g):
            pr = x[0] * g[0] - x[1] * g[1]
            pi = x[0] * g[1] + x[1] * g[0]
            return (pr, pi) if acc is None else (acc[0] + pr, acc[1] + pi)

        for r in range(P // 16):
            rows = pl.ds(r * 16, 16)
            for l in range(D // L):
                lanes = slice(l * L, (l + 1) * L)
                lo = hi = None
                g = (G_v[a + 1, 0, rows, lanes], G_v[a + 1, 1, rows, lanes])
                for c in range(a + 2):
                    x = (X_v[c, 0, rows, lanes], X_v[c, 1, rows, lanes])
                    hi = cmac(hi, x, g)
                    if c <= a:
                        g = (G_v[a - c, 0, rows, lanes], G_v[a - c, 1, rows, lanes])
                        lo = cmac(lo, x, g)
                        yield 32
                for w, z in enumerate((lo, hi)):
                    for part in range(2):
                        Z_v[pl.ds((a + w) * 2 * P + part * P + r * 16, 16), lanes] = z[part].astype(BF16)
                yield 20

    def job_x(t, bg, budget):
        for j in (2 * t, 2 * t + 1):
            for half in range(2):
                r = _dot(F_v[half * P:(half + 1) * P, 0:P], kv_v[j * P:(j + 1) * P, :]).reshape(8, 2, 8, D)
                for part in range(2):
                    X_v[j, part, half * 64:(half + 1) * 64, :] = r[:, part].reshape(64, D)
                bg.run(budget * 2.5)

    def job_h(t, bg, budget):
        for half in range(2):
            rows = pl.ds(half * 64, 64)
            for l0, l1 in H_SPLIT:
                w = (l1 - l0) * L
                lanes = slice(l0 * L, l1 * L)
                rhs = jnp.concatenate([h_v[lanes, t * TM:t * TM + P], h_v[lanes, t * TM + P:(t + 1) * TM]], axis=0)
                r = jax.lax.dot_general(F_v[half * P:(half + 1) * P, 0:P], rhs, NT_DIMS,
                                        preferred_element_type=F32).reshape(8, 2, 8, 2 * w)
                re, im = r[:, 0].reshape(64, 2 * w), r[:, 1].reshape(64, 2 * w)
                prev = (H_v[t % 2, 0, rows, lanes], H_v[t % 2, 1, rows, lanes])
                for j in range(2):
                    cur = (re[:, j * w:(j + 1) * w], im[:, j * w:(j + 1) * w])
                    G_v[2 * t + j, 0, rows, lanes] = cur[0] + prev[1] if half else cur[0] - prev[1]
                    G_v[2 * t + j, 1, rows, lanes] = cur[1] - prev[0] if half else cur[1] + prev[0]
                    prev = cur
                if t + 1 < NT:
                    H_v[(t + 1) % 2, 0, rows, lanes] = prev[0]
                    H_v[(t + 1) % 2, 1, rows, lanes] = prev[1]
                bg.run(budget * (l1 - l0))

    def z_out(t, m, n, pre, bg, budget, tied):
        z = _gelu_scaled(pre)
        if n < FH // L:
            z1_v[pl.ds(t * TM + m * MC, MC), n * L:(n + 1) * L] = z
        else:
            zg_v[t % 3, m * MC:(m + 1) * MC, n * L - FH:(n + 1) * L - FH] = z
        ntask = tied.run(z)
        bg.run(budget[1] if ntask else budget[0])

    def job_z(t, m, cols, bg, budget, tied):
        for n in cols:
            z_out(t, m, n, _dot(xn_v[pl.ds(t * TM + m * MC, MC), :], win_v[:, n * L:(n + 1) * L]), bg, budget, tied)

    def job_zs(t, p, j, bg, budget, tied):
        r1 = pl.ds(t * TM + p * P, MC)
        r2 = pl.ds(t * TM + p * P + MC, MC)
        c1 = slice(j * L, (j + 1) * L)
        c2 = slice(FH + j * L, FH + (j + 1) * L)

        def xl(w):
            r0 = (t % 4) * 5 * P + w * P + p * MC
            return XL_v[r0:r0 + MC, :]

        def wb(w):
            return WB_v[w * KH:(w + 1) * KH, c1]

        def rem(rows, cols):
            return _dot(xn_v[rows, 2 * KH:], win_v[2 * KH:, cols])

        m2 = _dot(xl(1), win_v[0:KH, c1])
        m4 = _dot(xn_v[r2, KH:2 * KH], wb(2))
        z_out(t, 2 * p + 1, j, m2 + m4 + rem(r2, c1), bg, budget, tied)
        m3 = _dot(xn_v[r1, 0:KH], wb(1))
        m5 = _dot(xl(2), win_v[KH:2 * KH, c2])
        z_out(t, 2 * p, 6 + j, m3 + m5 + rem(r1, c2), bg, budget, tied)
        t11, t22 = m4 - m5, m3 - m2
        m1 = _dot(xl(0), wb(0))
        t11, t22 = t11 + m1, t22 + m1
        z_out(t, 2 * p, j, t11 + _dot(xl(4), wb(4)) + rem(r1, c1), bg, budget, tied)
        z_out(t, 2 * p + 1, 6 + j, t22 + _dot(xl(3), wb(3)) + rem(r2, c2), bg, budget, tied)

    rev8 = 7 - jax.lax.broadcasted_iota(jnp.int32, (8, L), 0)

    def finish(a, upper, n, hh, slot):
        rows = pl.ds(a * P + (MC if upper else 0), MC)
        lanes = slice(n * L, (n + 1) * L)
        if upper:
            ya = _dot(Fi_v[:, 0:P], Z_v[a * 2 * P:a * 2 * P + P, lanes])
            yb = _dot(Fi_v[:, P:2 * P], Z_v[a * 2 * P + P:(a + 1) * 2 * P, lanes])
            slot(0.5)
            y = ya - yb
            lo = ya + yb
            for j in range(MC // 8):
                yl_v[a % 2, n, (7 - j) * 8:(8 - j) * 8, :] = jnp.take_along_axis(lo[j * 8:(j + 1) * 8], rev8, axis=0)
        else:
            y = yl_v[a % 2, n]
        gate = hh + hh * jnp.tanh(hh)
        s = xn_v[rows, lanes].astype(F32) * y
        o_v[rows, lanes] = (x_v[rows, lanes].astype(F32) + s * gate).astype(BF16)

    def tail_gen(i, bg, budget):
        a0, a1 = _blocks_of_step(i)

        def slot(w):
            bg.run(w * budget[0])

        def dot3(a, b):
            r = _dot(a, b)
            slot(0.75)
            return r

        for upper in (True, False):
            sub = MC if upper else 0
            r1 = pl.ds(a0 * P + sub, MC)
            r2 = pl.ds(a1 * P + sub, MC)

            def ul(w):
                r0 = ((i % 5) * 5 + w) * P + sub
                return UL_v[r0:r0 + MC, :]

            for j in range(2):
                c1 = slice(j * L, (j + 1) * L)
                c2 = slice((2 + j) * L, (3 + j) * L)

                def wo(w):
                    return WO_v[w * HN:(w + 1) * HN, c1]

                m2 = dot3(ul(1), wout_v[0:HN, c1])
                m4 = dot3(u_v[r2, HN:], wo(2))
                finish(a1, upper, j, m2 + m4, slot)
                bg.charge(T_COST)
                yield
                m3 = dot3(u_v[r1, 0:HN], wo(1))
                m5 = dot3(ul(2), wout_v[HN:, c2])
                finish(a0, upper, 2 + j, m3 + m5, slot)
                bg.charge(T_COST)
                yield
                m1 = dot3(ul(0), wo(0))
                finish(a0, upper, j, (m4 - m5) + m1 + dot3(ul(4), wo(4)), slot)
                bg.charge(T_COST)
                yield
                finish(a1, upper, 2 + j, (m3 - m2) + m1 + dot3(ul(3), wo(3)), slot)
                bg.charge(T_COST)
                yield
            for a, r in ((a0, r1), (a1, r2)):
                finish(a, upper, 4, dot3(u_v[r, 0:HN], wout_v[0:HN, 4 * L:]) + dot3(u_v[r, HN:], wout_v[HN:, 4 * L:]),
                       slot)
                bg.charge(T_COST)
                yield

    def wocomb_gen():
        for j in range(2):
            c1 = slice(j * L, (j + 1) * L)
            c2 = slice((2 + j) * L, (3 + j) * L)
            for r in range(HN // 32):
                top = pl.ds(r * 32, 32)
                bot = pl.ds(HN + r * 32, 32)
                b11, b12 = wout_v[top, c1].astype(F32), wout_v[top, c2].astype(F32)
                b21, b22 = wout_v[bot, c1].astype(F32), wout_v[bot, c2].astype(F32)
                for w, c in enumerate((b11 + b22, b12 - b22, b21 - b11, b11 + b12, b21 + b22)):
                    WO_v[pl.ds(w * HN + r * 32, 32), c1] = c.astype(BF16)
                yield A_COST

    def job_big(i, bg, pending, budget, every):
        a0, a1 = _blocks_of_step(i)
        KG = 512

        def lhs(j, sub, cols):
            if j == 2:
                return wsp_v[i * TM + sub:i * TM + sub + MC, cols]
            if j == 3:
                return wsp_v[i * TM + P + sub:i * TM + P + sub + MC, HK + cols.start:HK + cols.stop]
            r0 = ((i % 5) * 5 + {0: 0, 1: 1, 4: 2, 5: 3, 6: 4}[j]) * P + sub
            return Lc_v[r0:r0 + MC, cols]

        def prod(j, sub, n, acc=None):
            for kg in range(HK // KG):
                ks = slice(kg * KG, (kg + 1) * KG)
                p = _dot(lhs(j, sub, ks), R_v[j * HK + kg * KG:j * HK + (kg + 1) * KG, n * L:(n + 1) * L])
                acc = p if acc is None else acc + p
                bg.run(budget)
            return acc

        def tails(n):
            for _ in range(n):
                if pending:
                    next(pending.pop(0))

        def emit(a, sub, n, g):
            rows = pl.ds(a * P + sub, MC)
            lanes = slice(n * L, (n + 1) * L)
            u = z1_v[rows, lanes] * (g + bcol_v[rows, :])
            u_v[rows, lanes] = u.astype(BF16)
            bg.charge(E_COST)
            return u

        for sub in (0, MC):
            for n in range(HN // L):
                def put(w, c):
                    UL_v[pl.ds(((i % 5) * 5 + w) * P + sub, MC), n * L:(n + 1) * L] = c.astype(BF16)

                m1 = prod(0, sub, n)
                t11 = prod(6, sub, n, m1)
                m4 = prod(3, sub, n)
                t11 = t11 + m4
                m5 = prod(4, sub, n)
                u11 = emit(a0, sub, n, t11 - m5)
                m2 = prod(1, sub, n)
                u21 = emit(a1, sub, n, m2 + m4)
                put(3, u21 - u11)
                t22 = m1 - m2
                m3 = prod(2, sub, n)
                u12 = emit(a0, sub, n + HN // L, m3 + m5)
                put(2, u11 + u12)
                u22 = emit(a1, sub, n + HN // L, prod(5, sub, n, t22 + m3))
                put(0, u11 + u22)
                put(1, u21 + u22)
                put(4, u12 - u22)
                bg.charge(U_COST)
                tails(every.pop(0))

    def debug_keep_alive():
        if _ONLY is not None:
            for r_ in (xn_u, XL_u, WB_u, UL_u, WO_u, z1_v, R_u, Lc_u, zf_v, zg_v, kv_u, u_u, X_v, H_v, G_v, Z_u,
                       kf_v, bcol_v):
                c_ = pltpu.make_async_copy(r_, r_, sem_small.at[0])
                c_.start()
                c_.wait()

    debug_keep_alive()

    cp_x(0).start()
    cp_win(0).start()
    cp_x(1).start()
    cp_win(1).start()
    start(cp_small())
    for c in range(2, 5):
        cp_win(c).start()
    cp_x(2).start()

    kk = _odd_freq(jax.lax.broadcasted_iota(jnp.int32, (P, P), 0))
    nn = jax.lax.broadcasted_iota(jnp.int32, (P, P), 1)
    fc, fs = _cos_sin((kk * (4 * nn - 127)) & 2047)
    for g in range(P // 8):
        F_v[g * 16:(g + 1) * 16, 0:P] = jnp.concatenate(
            [fc[g * 8:(g + 1) * 8], -fs[g * 8:(g + 1) * 8]], axis=0).astype(BF16)
    fc, fs = _cos_sin((kk * (-127)) & 2047)
    ph_v[0] = fc
    ph_v[1] = fs
    kk = _odd_freq(jax.lax.broadcasted_iota(jnp.int32, (MC, P), 1))
    mm = jax.lax.broadcasted_iota(jnp.int32, (MC, P), 0)
    ic, is_ = _cos_sin((kk * (4 * mm + 2)) & 2047)
    Fi_v[:, 0:P] = (ic * (1.0 / (P * GA))).astype(BF16)
    Fi_v[:, P:2 * P] = (is_ * (1.0 / (P * GA))).astype(BF16)
    kf_v[:, 0:8, :] = jnp.zeros((D // L, 8, L), F32)

    cp_x(0).wait()
    for s in range(TM // 16):
        ln_x(0, s)

    def small_setup():
        sk = sk_in[...].astype(F32)
        for t in range(4):
            sk_v[t] = jnp.broadcast_to(sk[t:t + 1], (8, D))
        drow = d_in[...].astype(F32).reshape(1, D)
        for l in range(D // L):
            lanes = slice(l * L, (l + 1) * L)
            dre = ph_v[0] * drow[:, lanes]
            dim = ph_v[1] * drow[:, lanes]
            H_v[0, 0, 0:64, lanes] = -dim[0:64]
            H_v[0, 0, 64:P, lanes] = dim[64:P]
            H_v[0, 1, 0:64, lanes] = -dre[0:64]
            H_v[0, 1, 64:P, lanes] = dre[64:P]

    def bcol_task(t, j, tie):
        brow = b_in[...].astype(F32).reshape(1, S)[:, j * P:(j + 1) * P] * (0.25 / GA) + tie[0:1]
        bcol_v[j * P:(j + 1) * P, :] = jnp.broadcast_to(brow, (P, P)).T

    LAG = 2

    def interleave(*lists):
        out = []
        for j in range(max(len(a) for a in lists)):
            for a in lists:
                out += a[j:j + 1]
        return out

    def p1_first(c):
        bg = _Background()
        todo = []
        if c == 2:
            todo = tasks(bcol_task, 0)
            small_setup()
        if c == 3:
            todo = tasks(ln_z2, 0)
            bg.add(wcomb_gen(range(3)))
        if c == 4:
            todo = tasks(ln_x2, 2, 8)
            bg.add(wcomb_gen(range(3, 6)))
        tied = _Tied(todo, F_TIED[c])
        if c == 0:
            for s in range(TM // 16):
                ln_x(1, s)
        for t in range(2):
            for m in range(TM // MC):
                job_z(t, m, range(*WIN_CHUNKS[c]), bg, (80, 40), tied)
        bg.drain()
        assert not tied.tasks

    for c in range(5):
        cp_win(c).wait()
        if c == 0:
            cp_x(1).wait()
        if c == 2:
            wait(cp_small())
            start(cp_conv(0))
            cp_x(3).start()
        if c == 4:
            cp_x(2).wait()
            cp_x(4, 2).start()
        block(lambda c=c: p1_first(c), f'p1_f{c}')

    def p1_dma(g):
        if g == 0:
            wait(cp_conv(0))
            cp_x(3).wait()
            start(cp_conv(1))
            cp_x(6, 2).start()
            start(cp_conv(2, 2))
        if g == 1:
            wait(cp_conv(1))
            cp_x(4, 2).wait()
            start(cp_conv(4, 2))
            cp_wout().start()
            start(cp_wsp(0))
            start(cp_wsp(1))
        if g == 2:
            wait(cp_conv(2, 2))
            cp_x(6, 2).wait()
        if g == 3:
            wait(cp_conv(4, 2))
            cp_wout().wait()
            wait(cp_wsp(0))
            start(cp_wsp(2))
            start(cp_conv(6, 2))
            for i in (3, 4, 5):
                start(cp_wsp(i))

    def take(gen, n):
        for _ in range(n):
            yield next(gen)

    def p1_step(i):
        bg = _Background()
        dft = _Background()
        t = i - LAG
        xg = P1_X[i]
        kv = kv_gen(t)
        nx, nz, nh = KV_SPLIT if xg is not None else (0, KV_SPLIT[0] + KV_SPLIT[1], KV_SPLIT[2])
        dft.add(take(kv, nx))
        bg.add(take(kv, nz))
        hbg = _Background()
        hbg.add(take(kv, nh))
        zb = nz * KV_COST / 48.0
        extra = 0
        if i == 6:
            bg.add(wocomb_gen())
            bg.add(acomb_gen(0, range(3)))
            extra = 42
        if i == 7:
            bg.add(acomb_gen(0, range(3, 8)))
            extra = 24
        last = i == NT - 1
        z2t = tasks(ln_z2, i - 1)
        todo = interleave(*([tasks(ln_x2, t_, 8) for t_ in P1_LNX[i]] + [z2t[0::2], z2t[1::2]]))
        tied = _Tied(todo, 24 if last else TIED_N)
        if xg is not None:
            dft.run(KV_COST)
            job_x(xg, dft, (nx - 1) * KV_COST / 10.0)
            dft.drain()
        for p in range(2):
            for j in range(FH // L):
                job_zs(i, p, j, bg, (1.6 * zb + extra, 0.5 * zb + extra), tied)
            assert not tied.tasks or (p == 0 and not last)
            if p == 0 and last:
                tied = _Tied(tasks(ln_z2, i, 8), 22)
        if last:
            for s in range(8, 16):
                ln_z2(i, s)
        bg.drain()
        job_h(t, hbg, nh * KV_COST / 10.0)
        hbg.drain()

    def p1_block(g):
        for i in P1_GROUPS[g]:
            p1_step(i)

    for g in range(len(P1_GROUPS)):
        p1_dma(g)
        block(lambda g=g: p1_block(g), f'p1_g{g}')

    groups = P2_GROUPS
    NG = len(groups)

    def p2_dma(gi):
        if gi >= 2:
            for i in groups[gi - 2]:
                start(cp_out(i))
        if gi >= 3:
            for i in groups[gi - 3]:
                wait(cp_out(i))
        if gi == 1:
            for i in (6, 7):
                start(cp_wsp(i))
        if gi == 0:
            wait(cp_conv(6, 2))
        if gi + 1 < NG:
            for i in groups[gi + 1]:
                wait(cp_wsp(i))

    def tails_of(i, bg, budget):
        return [tail_gen(i, bg, budget)] * 20

    def p2_block(gi):
        bg = _Background()
        steps = groups[gi]
        tb = [0.0]
        pending = [t_ for i in (groups[gi - 1] if gi > 0 else []) for t_ in tails_of(i, bg, tb)]
        total = sum(a + 1 for i in steps for a in _blocks_of_step(i)) * 40 * 16
        total += len(steps) * (24 * E_COST + 6 * U_COST) + len(pending) * T_COST
        slots = 84 * len(steps) + TAIL_W * len(pending)
        bg.add(freq_gen(_blocks_of_step(steps[0])[0]))
        if gi < 2:
            bg.add(kv_gen(NT - 2 + gi))
            total += 20 * KV_COST
            slots += 10
        for t in P2_X[gi]:
            slots += 10
        if gi + 1 < NG:
            for i in groups[gi + 1]:
                bg.add(acomb_gen(i))
                total += 32 * A_COST
        for i in steps[1:]:
            bg.add(freq_gen(_blocks_of_step(i)[0]))
        budget = tb[0] = total / slots
        bg.run(budget)
        for t in P2_X[gi]:
            job_x(t, bg, budget)
        if gi < 2:
            job_h(NT - 2 + gi, bg, budget)
        units = [4, 4, 2, 4, 4, 2] * (len(pending) // 20)
        every = [0] * (6 * len(steps))
        for j, n in enumerate(units):
            every[min(len(every) - 1, j * len(every) // len(units))] += n
        for i in steps:
            job_big(i, bg, pending, budget, every)
        for t_ in pending:
            next(t_)
        bg.drain()

    for gi in range(NG):
        p2_dma(gi)
        block(lambda gi=gi: p2_block(gi), f'p2_{gi}')

    def cp_last(upper):
        a0 = _blocks_of_step(NT - 1)[0]
        return [pltpu.make_async_copy(o_v.at[pl.ds(r, MC)], o_hbm.at[0, pl.ds(r, MC)], sem_out.at[NT - 1])
                for r in ((a0 + w) * P + (MC if upper else 0) for w in range(2))]

    def p2_last():
        for i in groups[NG - 1]:
            for j, t_ in enumerate(tails_of(i, _Background(), [0.0])):
                next(t_)
                if i < NT - 1 and j == 19:
                    start(cp_out(i))
                if i == NT - 1 and j == 9:
                    start(cp_last(True))

    p2_dma(NG)
    block(p2_last, 'p2_last')
    start(cp_last(False))
    for i in groups[NG - 2] + groups[NG - 1][:-1]:
        wait(cp_out(i))
    wait(cp_last(True))
    wait(cp_last(False))
    debug_keep_alive()


@jax.jit
def pallas_recurrent_scan__ssm_conv_h3__mixer_gmlp__prompt_kernel(
    A_q: jax.Array,
    A_k: jax.Array,
    A_v: jax.Array,
    A_shift_k: jax.Array,
    A_ssm_k: jax.Array,
    A_ssm_D: jax.Array,
    B_x: jax.Array,
    B_w_in: jax.Array,
    B_w_sp: jax.Array,
    B_b_sp: jax.Array,
    B_w_out: jax.Array,
):
    del B_x
    hbm = pl.BlockSpec(memory_space=pl.ANY)

    def bf16_buf(*shape):
        return pltpu.VMEM(shape[:-2] + (shape[-2] // 2, shape[-1]), U32)

    return pl.pallas_call(
        _kernel,
        out_shape=jax.ShapeDtypeStruct((1, S, D), BF16),
        in_specs=[hbm] * 10,
        out_specs=hbm,
        scratch_shapes=[
            bf16_buf(S, D),
            bf16_buf(S, D),
            bf16_buf(S, D),
            bf16_buf(D, S),
            bf16_buf(D, 2 * FH),
            bf16_buf(S, S),
            bf16_buf(FH, D),
            pltpu.VMEM((S, D), BF16),
            pltpu.VMEM((4, D), BF16),
            pltpu.VMEM((D,), BF16),
            pltpu.VMEM((S,), BF16),
            bf16_buf(S, D),
            bf16_buf(4 * 5 * P, KH),
            bf16_buf(5 * KH, FH),
            bf16_buf(5 * 5 * P, HN),
            bf16_buf(5 * HN, 2 * L),
            pltpu.VMEM((S, FH), F32),
            bf16_buf(7 * HK, HN),
            bf16_buf(5 * 5 * P, HK),
            pltpu.VMEM((HK, FH), F32),
            pltpu.VMEM((3, TM, FH), F32),
            bf16_buf(S, D),
            bf16_buf(S, FH),
            pltpu.VMEM((NB, 2, P, D), F32),
            pltpu.VMEM((2, 2, P, D), F32),
            pltpu.VMEM((NB, 2, P, D), F32),
            bf16_buf(NB * 2 * P, D),
            pltpu.VMEM((2, D // L, MC, L), F32),
            bf16_buf(2 * P, 2 * P),
            bf16_buf(MC, 2 * P),
            pltpu.VMEM((S, L), F32),
            pltpu.VMEM((2, P, L), F32),
            pltpu.VMEM((4, 8, D), F32),
            pltpu.VMEM((D // L, S + 8, L), F32),
            pltpu.SemaphoreType.DMA((1,)),
            pltpu.SemaphoreType.DMA((NT,)),
            pltpu.SemaphoreType.DMA((NT,)),
            pltpu.SemaphoreType.DMA((NT,)),
            pltpu.SemaphoreType.DMA((5,)),
            pltpu.SemaphoreType.DMA((NT,)),
        ],
        compiler_params=pltpu.CompilerParams(vmem_limit_bytes=116 * 1024 * 1024, disable_semaphore_checks=True),
    )(A_q, A_k, A_v, A_shift_k.T, A_ssm_k, A_ssm_D, B_w_in, B_w_sp, B_b_sp, B_w_out)
```

```python
import math

import jax
import jax.numpy as jnp
import jax.experimental.pallas as pl
import jax.experimental.pallas.tpu as pltpu

S = 2048
D = 640
FH = 768
P = 128
NB = S // P
TM = 256
NT = S // TM
MC = 64
L = 128
HK = S // 2
KH = 256
HN = FH // 2
EPS = 1e-5
F32 = jnp.float32
BF16 = jnp.bfloat16
U32 = jnp.uint32
GELU_C = math.sqrt(2.0 / math.pi)
GA = (GELU_C * 0.044715) ** (1.0 / 3.0)
NT_DIMS = (((1,), (1,)), ((), ()))

WIN_CHUNKS = ((6, 7), (7, 9), (9, 12), (0, 3), (3, 6))
P1_GROUPS = ((2,), (3,), (4, 5), (6, 7))
P1_X = {2: None, 3: 0, 4: 1, 5: None, 6: 2, 7: 3}
P1_LNX = {2: (3,), 3: (4, 5), 4: (6,), 5: (7,), 6: (), 7: ()}
P2_GROUPS = ((0,), (1, 2), (3, 4, 5), (6, 7))
P2_X = ((4, 5), (6,), (7,), ())
STEP_BLOCKS = ((6, 7), (8, 9), (4, 5), (12, 13), (10, 11), (0, 1), (14, 15), (2, 3))
KV_COST, A_COST = 110, 56
E_COST, U_COST, T_COST, TAIL_W = 24, 90, 90, 1.6
KV_SPLIT = (12, 4, 4)
H_SPLIT = ((0, 2), (2, 4), (4, 5))
TIED_N = 42
F_TIED = (20, 20, 18, 20, 20)
_ONLY = None


def _dot(a, b):
    return jnp.dot(a, b, preferred_element_type=F32)


def _cos_sin(m):
    q = (m + 256) >> 9
    x = (m - (q << 9)).astype(F32) * (2.0 * math.pi / 2048.0)
    x2 = x * x
    s = x * (1.0 + x2 * (-1.0 / 6 + x2 * (1.0 / 120 + x2 * (-1.0 / 5040 + x2 * (1.0 / 362880)))))
    c = 1.0 + x2 * (-0.5 + x2 * (1.0 / 24 + x2 * (-1.0 / 720 + x2 * (1.0 / 40320 - x2 * (1.0 / 3628800)))))
    swap = (q & 1) == 1
    c0 = jnp.where(swap, s, c)
    s0 = jnp.where(swap, c, s)
    cos = jnp.where(((q + 1) & 2) == 2, -c0, c0)
    sin = jnp.where((q & 2) == 2, -s0, s0)
    return cos, sin


def _odd_freq(r):
    return jnp.where(r < 64, 4 * r + 1, 4 * r - 253)


def _gelu_scaled(z):
    return z + z * jnp.tanh(z * (GELU_C / GA + z * z))


def _signzero(z):
    bits = jax.lax.bitcast_convert_type(z, U32) & jnp.uint32(0x80000000)
    return jax.lax.bitcast_convert_type(bits, F32)


def _ln(x, eps, tie=None, scale=None):
    n = x.shape[-1]
    cols = [x[:, j * L:(j + 1) * L] for j in range(n // L)]
    s1 = cols[0]
    s2 = cols[0] * cols[0]
    for c in cols[1:]:
        s1 = s1 + c
        s2 = s2 + c * c
    if tie is not None:
        s1 = s1 + tie
        s2 = s2 + tie
    m = jnp.sum(s1, axis=-1, keepdims=True) * (1.0 / n)
    v = jnp.maximum(jnp.sum(s2, axis=-1, keepdims=True) * (1.0 / n) - m * m, 0.0)
    rs = jax.lax.rsqrt(v + eps)
    if scale is not None:
        rs = rs * scale
    return (x - m) * rs


def _blocks_of_step(i):
    return STEP_BLOCKS[i]


class _Background:
    def __init__(self):
        self.q = []
        self.credit = 0.0

    def add(self, gen):
        self.q.append(gen)

    def run(self, budget):
        self.credit += budget
        while self.q and self.credit > 0:
            try:
                self.credit -= next(self.q[0])
            except StopIteration:
                self.q.pop(0)
        if not self.q:
            self.credit = 0.0

    def charge(self, cost):
        self.credit -= cost

    def drain(self):
        while self.q:
            self.run(1e9)


class _Tied:
    def __init__(self, tasks, npieces):
        self.tasks = list(tasks)
        self.rate = len(self.tasks) / float(npieces)
        self.credit = 0.999

    def run(self, z):
        self.credit += self.rate
        n = 0
        while self.tasks and self.credit >= 1.0:
            self.tasks.pop(0)(_signzero(z[0:16]))
            self.credit -= 1.0
            n += 1
        return n


def _kernel(q_hbm, k_hbm, v_hbm, sk_hbm, h_hbm, d_hbm, win_hbm, wsp_hbm, b_hbm, wout_hbm,
            o_hbm,
            x_u, k_u, v_u, h_u, win_u, wsp_u, wout_u, o_v, sk_in, d_in, b_in,
            xn_u, XL_u, WB_u, UL_u, WO_u, z1_v, R_u, Lc_u, zf_v, zg_v, kv_u, u_u, X_v, H_v, G_v, Z_u,
            yl_v, F_u, Fi_u, bcol_v, ph_v, sk_v, kf_v,
            sem_small, sem_x, sem_conv, sem_wsp, sem_w, sem_out):
    (x_v, k_v, v_v, h_v, win_v, wsp_v, wout_v, xn_v, XL_v, WB_v, UL_v, WO_v, R_v, Lc_v, kv_v, u_v, Z_v,
     F_v, Fi_v) = [r.bitcast(BF16) for r in (x_u, k_u, v_u, h_u, win_u, wsp_u, wout_u, xn_u, XL_u, WB_u, UL_u,
                                             WO_u, R_u, Lc_u, kv_u, u_u, Z_u, F_u, Fi_u)]

    def cp_small():
        return [pltpu.make_async_copy(s_, d_, sem_small.at[0])
                for s_, d_ in ((d_hbm, d_in), (sk_hbm, sk_in), (b_hbm, b_in))]

    def cp_x(t, n=1):
        rows = pl.ds(t * TM, n * TM)
        return pltpu.make_async_copy(q_hbm.at[0, rows], x_v.at[rows], sem_x.at[t])

    def cp_conv(t, n=1):
        rows = pl.ds(t * TM, n * TM)
        sem = sem_conv.at[t]
        return [pltpu.make_async_copy(h_hbm.at[:, rows], h_v.at[:, rows], sem),
                pltpu.make_async_copy(k_hbm.at[0, rows], k_v.at[rows], sem),
                pltpu.make_async_copy(v_hbm.at[0, rows], v_v.at[rows], sem)]

    def cp_wsp(i):
        return [pltpu.make_async_copy(wsp_hbm.at[pl.ds(_blocks_of_step(i)[0] * P, TM)],
                                      wsp_v.at[pl.ds(i * TM, TM)], sem_wsp.at[i])]

    def cp_win(c):
        lo, hi = WIN_CHUNKS[c]
        cols = pl.ds(lo * L, (hi - lo) * L)
        return pltpu.make_async_copy(win_hbm.at[:, cols], win_v.at[:, cols], sem_w.at[c])

    def cp_wout():
        return pltpu.make_async_copy(wout_hbm, wout_v, sem_w.at[0])

    def cp_out(i):
        rows = pl.ds(_blocks_of_step(i)[0] * P, TM)
        return [pltpu.make_async_copy(o_v.at[rows], o_hbm.at[0, rows], sem_out.at[i])]

    def start(cs):
        for c in cs:
            c.start()

    def wait(cs):
        for c in cs:
            c.wait()

    def block(fn, name):
        def body(it):
            fn()
            return it + 1

        if _ONLY is None or name in _ONLY:
            jax.lax.while_loop(lambda it: it < 1, body, jnp.int32(0))

    def ln_x(t, s, tie=None):
        rows = pl.ds(t * TM + s * 16, 16)
        y = _ln(x_v[rows, :].astype(F32), EPS, tie, GA)
        xn_v[rows, :] = y.astype(BF16)
        return y

    def ln_x2(t, s, tie):
        p, q = s // 4, s % 4
        y1 = ln_x(t, 8 * p + q, tie)
        y2 = ln_x(t, 8 * p + 4 + q, tie)
        a11, a12, a21, a22 = y1[:, :KH], y1[:, KH:2 * KH], y2[:, :KH], y2[:, KH:2 * KH]
        r0 = (t % 4) * 5 * P + p * MC + q * 16
        for j, c in enumerate((a11 + a22, a21 + a22, a11 + a12, a21 - a11, a12 - a22)):
            XL_v[pl.ds(r0 + j * P, 16), :] = c.astype(BF16)

    def wcomb_gen(cols):
        for j in cols:
            c1 = slice(j * L, (j + 1) * L)
            c2 = slice(FH + j * L, FH + (j + 1) * L)
            for r in range(KH // 32):
                top = pl.ds(r * 32, 32)
                bot = pl.ds(KH + r * 32, 32)
                b11, b12 = win_v[top, c1].astype(F32), win_v[top, c2].astype(F32)
                b21, b22 = win_v[bot, c1].astype(F32), win_v[bot, c2].astype(F32)
                for w, c in enumerate((b11 + b22, b12 - b22, b21 - b11, b11 + b12, b21 + b22)):
                    WB_v[pl.ds(w * KH + r * 32, 32), c1] = c.astype(BF16)
                yield A_COST

    def ln_z2(t, s, tie=None):
        y = _ln(zg_v[t % 3, s * 16:(s + 1) * 16, :], 4.0 * GA * GA * EPS, tie, 0.25 / GA)
        lo, hi = y[:, :HN], y[:, HN:]
        r = (t * TM + s * 16) % HK
        rows = pl.ds(r, 16)
        if t < NT // 2:
            zf_v[rows, :] = y
            R_v[pl.ds(1 * HK + r, 16), :] = lo.astype(BF16)
            R_v[pl.ds(5 * HK + r, 16), :] = (lo + hi).astype(BF16)
        else:
            b11, b12 = zf_v[rows, :HN], zf_v[rows, HN:]
            R_v[pl.ds(0 * HK + r, 16), :] = (b11 + hi).astype(BF16)
            R_v[pl.ds(2 * HK + r, 16), :] = (b12 - hi).astype(BF16)
            R_v[pl.ds(3 * HK + r, 16), :] = (lo - b11).astype(BF16)
            R_v[pl.ds(4 * HK + r, 16), :] = hi.astype(BF16)
            R_v[pl.ds(6 * HK + r, 16), :] = (lo + hi).astype(BF16)

    def acomb_gen(i, groups=range(P // 16)):
        for r in groups:
            for c in range(HK // 256):
                top = pl.ds(i * TM + r * 16, 16)
                bot = pl.ds(i * TM + P + r * 16, 16)
                c1 = slice(c * 256, (c + 1) * 256)
                c2 = slice(HK + c * 256, HK + (c + 1) * 256)
                a11 = wsp_v[top, c1].astype(F32)
                a12 = wsp_v[top, c2].astype(F32)
                a21 = wsp_v[bot, c1].astype(F32)
                a22 = wsp_v[bot, c2].astype(F32)
                r0 = (i % 5) * 5 * P + r * 16
                Lc_v[pl.ds(r0 + 0 * P, 16), c1] = (a11 + a22).astype(BF16)
                Lc_v[pl.ds(r0 + 1 * P, 16), c1] = (a21 + a22).astype(BF16)
                Lc_v[pl.ds(r0 + 2 * P, 16), c1] = (a11 + a12).astype(BF16)
                Lc_v[pl.ds(r0 + 3 * P, 16), c1] = (a21 - a11).astype(BF16)
                Lc_v[pl.ds(r0 + 4 * P, 16), c1] = (a12 - a22).astype(BF16)
                yield A_COST

    def tasks(fn, t, n=TM // 16):
        return [lambda tie, s=s: fn(t, s, tie) for s in range(n)]

    def kv_gen(t):
        for m in range(TM // MC):
            r = t * TM + m * MC
            for l in range(D // L):
                lanes = slice(l * L, (l + 1) * L)
                kf = k_v[pl.ds(r, MC), lanes].astype(F32)
                kf_v[l, pl.ds(r + 8, MC), :] = kf
                ks = kf * sk_v[0, 0:1, lanes]
                for tap in range(1, 4):
                    ks = ks + kf_v[l, pl.ds(r + 8 - tap, MC), :] * sk_v[tap, 0:1, lanes]
                kv = ks * v_v[pl.ds(r, MC), lanes].astype(F32)
                kv_v[pl.ds(r, MC), lanes] = kv.astype(BF16)
                yield KV_COST

    def freq_gen(a):
        def cmac(acc, x, g):
            pr = x[0] * g[0] - x[1] * g[1]
            pi = x[0] * g[1] + x[1] * g[0]
            return (pr, pi) if acc is None else (acc[0] + pr, acc[1] + pi)

        for r in range(P // 16):
            rows = pl.ds(r * 16, 16)
            for l in range(D // L):
                lanes = slice(l * L, (l + 1) * L)
                lo = hi = None
                g = (G_v[a + 1, 0, rows, lanes], G_v[a + 1, 1, rows, lanes])
                for c in range(a + 2):
                    x = (X_v[c, 0, rows, lanes], X_v[c, 1, rows, lanes])
                    hi = cmac(hi, x, g)
                    if c <= a:
                        g = (G_v[a - c, 0, rows, lanes], G_v[a - c, 1, rows, lanes])
                        lo = cmac(lo, x, g)
                        yield 32
                for w, z in enumerate((lo, hi)):
                    for part in range(2):
                        Z_v[pl.ds((a + w) * 2 * P + part * P + r * 16, 16), lanes] = z[part].astype(BF16)
                yield 20

    def job_x(t, bg, budget):
        for j in (2 * t, 2 * t + 1):
            for half in range(2):
                r = _dot(F_v[half * P:(half + 1) * P, 0:P], kv_v[j * P:(j + 1) * P, :]).reshape(8, 2, 8, D)
                for part in range(2):
                    X_v[j, part, half * 64:(half + 1) * 64, :] = r[:, part].reshape(64, D)
                bg.run(budget * 2.5)

    def job_h(t, bg, budget):
        for half in range(2):
            rows = pl.ds(half * 64, 64)
            for l0, l1 in H_SPLIT:
                w = (l1 - l0) * L
                lanes = slice(l0 * L, l1 * L)
                rhs = jnp.concatenate([h_v[lanes, t * TM:t * TM + P], h_v[lanes, t * TM + P:(t + 1) * TM]], axis=0)
                r = jax.lax.dot_general(F_v[half * P:(half + 1) * P, 0:P], rhs, NT_DIMS,
                                        preferred_element_type=F32).reshape(8, 2, 8, 2 * w)
                re, im = r[:, 0].reshape(64, 2 * w), r[:, 1].reshape(64, 2 * w)
                prev = (H_v[t % 2, 0, rows, lanes], H_v[t % 2, 1, rows, lanes])
                for j in range(2):
                    cur = (re[:, j * w:(j + 1) * w], im[:, j * w:(j + 1) * w])
                    G_v[2 * t + j, 0, rows, lanes] = cur[0] + prev[1] if half else cur[0] - prev[1]
                    G_v[2 * t + j, 1, rows, lanes] = cur[1] - prev[0] if half else cur[1] + prev[0]
                    prev = cur
                if t + 1 < NT:
                    H_v[(t + 1) % 2, 0, rows, lanes] = prev[0]
                    H_v[(t + 1) % 2, 1, rows, lanes] = prev[1]
                bg.run(budget * (l1 - l0))

    def z_out(t, m, n, pre, bg, budget, tied):
        z = _gelu_scaled(pre)
        if n < FH // L:
            z1_v[pl.ds(t * TM + m * MC, MC), n * L:(n + 1) * L] = z
        else:
            zg_v[t % 3, m * MC:(m + 1) * MC, n * L - FH:(n + 1) * L - FH] = z
        ntask = tied.run(z)
        bg.run(budget[1] if ntask else budget[0])

    def job_z(t, m, cols, bg, budget, tied):
        for n in cols:
            z_out(t, m, n, _dot(xn_v[pl.ds(t * TM + m * MC, MC), :], win_v[:, n * L:(n + 1) * L]), bg, budget, tied)

    def job_zs(t, p, j, bg, budget, tied):
        r1 = pl.ds(t * TM + p * P, MC)
        r2 = pl.ds(t * TM + p * P + MC, MC)
        c1 = slice(j * L, (j + 1) * L)
        c2 = slice(FH + j * L, FH + (j + 1) * L)

        def xl(w):
            r0 = (t % 4) * 5 * P + w * P + p * MC
            return XL_v[r0:r0 + MC, :]

        def wb(w):
            return WB_v[w * KH:(w + 1) * KH, c1]

        def rem(rows, cols):
            return _dot(xn_v[rows, 2 * KH:], win_v[2 * KH:, cols])

        m2 = _dot(xl(1), win_v[0:KH, c1])
        m4 = _dot(xn_v[r2, KH:2 * KH], wb(2))
        z_out(t, 2 * p + 1, j, m2 + m4 + rem(r2, c1), bg, budget, tied)
        m3 = _dot(xn_v[r1, 0:KH], wb(1))
        m5 = _dot(xl(2), win_v[KH:2 * KH, c2])
        z_out(t, 2 * p, 6 + j, m3 + m5 + rem(r1, c2), bg, budget, tied)
        t11, t22 = m4 - m5, m3 - m2
        m1 = _dot(xl(0), wb(0))
        t11, t22 = t11 + m1, t22 + m1
        z_out(t, 2 * p, j, t11 + _dot(xl(4), wb(4)) + rem(r1, c1), bg, budget, tied)
        z_out(t, 2 * p + 1, 6 + j, t22 + _dot(xl(3), wb(3)) + rem(r2, c2), bg, budget, tied)

    rev8 = 7 - jax.lax.broadcasted_iota(jnp.int32, (8, L), 0)

    def finish(a, upper, n, hh, slot):
        rows = pl.ds(a * P + (MC if upper else 0), MC)
        lanes = slice(n * L, (n + 1) * L)
        if upper:
            ya = _dot(Fi_v[:, 0:P], Z_v[a * 2 * P:a * 2 * P + P, lanes])
            yb = _dot(Fi_v[:, P:2 * P], Z_v[a * 2 * P + P:(a + 1) * 2 * P, lanes])
            slot(0.5)
            y = ya - yb
            lo = ya + yb
            for j in range(MC // 8):
                yl_v[a % 2, n, (7 - j) * 8:(8 - j) * 8, :] = jnp.take_along_axis(lo[j * 8:(j + 1) * 8], rev8, axis=0)
        else:
            y = yl_v[a % 2, n]
        gate = hh + hh * jnp.tanh(hh)
        s = xn_v[rows, lanes].astype(F32) * y
        o_v[rows, lanes] = (x_v[rows, lanes].astype(F32) + s * gate).astype(BF16)

    def tail_gen(i, bg, budget):
        a0, a1 = _blocks_of_step(i)

        def slot(w):
            bg.run(w * budget[0])

        def dot3(a, b):
            r = _dot(a, b)
            slot(0.75)
            return r

        for upper in (True, False):
            sub = MC if upper else 0
            r1 = pl.ds(a0 * P + sub, MC)
            r2 = pl.ds(a1 * P + sub, MC)

            def ul(w):
                r0 = ((i % 5) * 5 + w) * P + sub
                return UL_v[r0:r0 + MC, :]

            for j in range(2):
                c1 = slice(j * L, (j + 1) * L)
                c2 = slice((2 + j) * L, (3 + j) * L)

                def wo(w):
                    return WO_v[w * HN:(w + 1) * HN, c1]

                m2 = dot3(ul(1), wout_v[0:HN, c1])
                m4 = dot3(u_v[r2, HN:], wo(2))
                finish(a1, upper, j, m2 + m4, slot)
                bg.charge(T_COST)
                yield
                m3 = dot3(u_v[r1, 0:HN], wo(1))
                m5 = dot3(ul(2), wout_v[HN:, c2])
                finish(a0, upper, 2 + j, m3 + m5, slot)
                bg.charge(T_COST)
                yield
                m1 = dot3(ul(0), wo(0))
                finish(a0, upper, j, (m4 - m5) + m1 + dot3(ul(4), wo(4)), slot)
                bg.charge(T_COST)
                yield
                finish(a1, upper, 2 + j, (m3 - m2) + m1 + dot3(ul(3), wo(3)), slot)
                bg.charge(T_COST)
                yield
            for a, r in ((a0, r1), (a1, r2)):
                finish(a, upper, 4, dot3(u_v[r, 0:HN], wout_v[0:HN, 4 * L:]) + dot3(u_v[r, HN:], wout_v[HN:, 4 * L:]),
                       slot)
                bg.charge(T_COST)
                yield

    def wocomb_gen():
        for j in range(2):
            c1 = slice(j * L, (j + 1) * L)
            c2 = slice((2 + j) * L, (3 + j) * L)
            for r in range(HN // 32):
                top = pl.ds(r * 32, 32)
                bot = pl.ds(HN + r * 32, 32)
                b11, b12 = wout_v[top, c1].astype(F32), wout_v[top, c2].astype(F32)
                b21, b22 = wout_v[bot, c1].astype(F32), wout_v[bot, c2].astype(F32)
                for w, c in enumerate((b11 + b22, b12 - b22, b21 - b11, b11 + b12, b21 + b22)):
                    WO_v[pl.ds(w * HN + r * 32, 32), c1] = c.astype(BF16)
                yield A_COST

    def job_big(i, bg, pending, budget, every):
        a0, a1 = _blocks_of_step(i)
        KG = 512

        def lhs(j, sub, cols):
            if j == 2:
                return wsp_v[i * TM + sub:i * TM + sub + MC, cols]
            if j == 3:
                return wsp_v[i * TM + P + sub:i * TM + P + sub + MC, HK + cols.start:HK + cols.stop]
            r0 = ((i % 5) * 5 + {0: 0, 1: 1, 4: 2, 5: 3, 6: 4}[j]) * P + sub
            return Lc_v[r0:r0 + MC, cols]

        def prod(j, sub, n, acc=None):
            for kg in range(HK // KG):
                ks = slice(kg * KG, (kg + 1) * KG)
                p = _dot(lhs(j, sub, ks), R_v[j * HK + kg * KG:j * HK + (kg + 1) * KG, n * L:(n + 1) * L])
                acc = p if acc is None else acc + p
                bg.run(budget)
            return acc

        def tails(n):
            for _ in range(n):
                if pending:
                    next(pending.pop(0))

        def emit(a, sub, n, g):
            rows = pl.ds(a * P + sub, MC)
            lanes = slice(n * L, (n + 1) * L)
            u = z1_v[rows, lanes] * (g + bcol_v[rows, :])
            u_v[rows, lanes] = u.astype(BF16)
            bg.charge(E_COST)
            return u

        for sub in (0, MC):
            for n in range(HN // L):
                def put(w, c):
                    UL_v[pl.ds(((i % 5) * 5 + w) * P + sub, MC), n * L:(n + 1) * L] = c.astype(BF16)

                m1 = prod(0, sub, n)
                t11 = prod(6, sub, n, m1)
                m4 = prod(3, sub, n)
                t11 = t11 + m4
                m5 = prod(4, sub, n)
                u11 = emit(a0, sub, n, t11 - m5)
                m2 = prod(1, sub, n)
                u21 = emit(a1, sub, n, m2 + m4)
                put(3, u21 - u11)
                t22 = m1 - m2
                m3 = prod(2, sub, n)
                u12 = emit(a0, sub, n + HN // L, m3 + m5)
                put(2, u11 + u12)
                u22 = emit(a1, sub, n + HN // L, prod(5, sub, n, t22 + m3))
                put(0, u11 + u22)
                put(1, u21 + u22)
                put(4, u12 - u22)
                bg.charge(U_COST)
                tails(every.pop(0))

    def debug_keep_alive():
        if _ONLY is not None:
            for r_ in (xn_u, XL_u, WB_u, UL_u, WO_u, z1_v, R_u, Lc_u, zf_v, zg_v, kv_u, u_u, X_v, H_v, G_v, Z_u,
                       kf_v, bcol_v):
                c_ = pltpu.make_async_copy(r_, r_, sem_small.at[0])
                c_.start()
                c_.wait()

    debug_keep_alive()

    cp_x(0).start()
    cp_win(0).start()
    cp_x(1).start()
    cp_win(1).start()
    start(cp_small())
    for c in range(2, 5):
        cp_win(c).start()
    cp_x(2).start()

    kk = _odd_freq(jax.lax.broadcasted_iota(jnp.int32, (P, P), 0))
    nn = jax.lax.broadcasted_iota(jnp.int32, (P, P), 1)
    fc, fs = _cos_sin((kk * (4 * nn - 127)) & 2047)
    for g in range(P // 8):
        F_v[g * 16:(g + 1) * 16, 0:P] = jnp.concatenate(
            [fc[g * 8:(g + 1) * 8], -fs[g * 8:(g + 1) * 8]], axis=0).astype(BF16)
    fc, fs = _cos_sin((kk * (-127)) & 2047)
    ph_v[0] = fc
    ph_v[1] = fs
    kk = _odd_freq(jax.lax.broadcasted_iota(jnp.int32, (MC, P), 1))
    mm = jax.lax.broadcasted_iota(jnp.int32, (MC, P), 0)
    ic, is_ = _cos_sin((kk * (4 * mm + 2)) & 2047)
    Fi_v[:, 0:P] = (ic * (1.0 / (P * GA))).astype(BF16)
    Fi_v[:, P:2 * P] = (is_ * (1.0 / (P * GA))).astype(BF16)
    kf_v[:, 0:8, :] = jnp.zeros((D // L, 8, L), F32)

    cp_x(0).wait()
    for s in range(TM // 16):
        ln_x(0, s)

    def small_setup():
        sk = sk_in[...].astype(F32)
        for t in range(4):
            sk_v[t] = jnp.broadcast_to(sk[t:t + 1], (8, D))
        drow = d_in[...].astype(F32).reshape(1, D)
        for l in range(D // L):
            lanes = slice(l * L, (l + 1) * L)
            dre = ph_v[0] * drow[:, lanes]
            dim = ph_v[1] * drow[:, lanes]
            H_v[0, 0, 0:64, lanes] = -dim[0:64]
            H_v[0, 0, 64:P, lanes] = dim[64:P]
            H_v[0, 1, 0:64, lanes] = -dre[0:64]
            H_v[0, 1, 64:P, lanes] = dre[64:P]

    def bcol_task(t, j, tie):
        brow = b_in[...].astype(F32).reshape(1, S)[:, j * P:(j + 1) * P] * (0.25 / GA) + tie[0:1]
        bcol_v[j * P:(j + 1) * P, :] = jnp.broadcast_to(brow, (P, P)).T

    LAG = 2

    def interleave(*lists):
        out = []
        for j in range(max(len(a) for a in lists)):
            for a in lists:
                out += a[j:j + 1]
        return out

    def p1_first(c):
        bg = _Background()
        todo = []
        if c == 2:
            todo = tasks(bcol_task, 0)
            small_setup()
        if c == 3:
            todo = tasks(ln_z2, 0)
            bg.add(wcomb_gen(range(3)))
        if c == 4:
            todo = tasks(ln_x2, 2, 8)
            bg.add(wcomb_gen(range(3, 6)))
        tied = _Tied(todo, F_TIED[c])
        if c == 0:
            for s in range(TM // 16):
                ln_x(1, s)
        for t in range(2):
            for m in range(TM // MC):
                job_z(t, m, range(*WIN_CHUNKS[c]), bg, (80, 40), tied)
        bg.drain()
        assert not tied.tasks

    for c in range(5):
        cp_win(c).wait()
        if c == 0:
            cp_x(1).wait()
        if c == 2:
            wait(cp_small())
            start(cp_conv(0))
            cp_x(3).start()
        if c == 4:
            cp_x(2).wait()
            cp_x(4, 2).start()
        block(lambda c=c: p1_first(c), f'p1_f{c}')

    def p1_dma(g):
        if g == 0:
            wait(cp_conv(0))
            cp_x(3).wait()
            start(cp_conv(1))
            cp_x(6, 2).start()
            start(cp_conv(2, 2))
        if g == 1:
            wait(cp_conv(1))
            cp_x(4, 2).wait()
            start(cp_conv(4, 2))
            cp_wout().start()
            start(cp_wsp(0))
            start(cp_wsp(1))
        if g == 2:
            wait(cp_conv(2, 2))
            cp_x(6, 2).wait()
        if g == 3:
            wait(cp_conv(4, 2))
            cp_wout().wait()
            wait(cp_wsp(0))
            start(cp_wsp(2))
            start(cp_conv(6, 2))
            for i in (3, 4, 5):
                start(cp_wsp(i))

    def take(gen, n):
        for _ in range(n):
            yield next(gen)

    def p1_step(i):
        bg = _Background()
        dft = _Background()
        t = i - LAG
        xg = P1_X[i]
        kv = kv_gen(t)
        nx, nz, nh = KV_SPLIT if xg is not None else (0, KV_SPLIT[0] + KV_SPLIT[1], KV_SPLIT[2])
        dft.add(take(kv, nx))
        bg.add(take(kv, nz))
        hbg = _Background()
        hbg.add(take(kv, nh))
        zb = nz * KV_COST / 48.0
        extra = 0
        if i == 6:
            bg.add(wocomb_gen())
            bg.add(acomb_gen(0, range(3)))
            extra = 42
        if i == 7:
            bg.add(acomb_gen(0, range(3, 8)))
            extra = 24
        last = i == NT - 1
        z2t = tasks(ln_z2, i - 1)
        todo = interleave(*([tasks(ln_x2, t_, 8) for t_ in P1_LNX[i]] + [z2t[0::2], z2t[1::2]]))
        tied = _Tied(todo, 24 if last else TIED_N)
        if xg is not None:
            dft.run(KV_COST)
            job_x(xg, dft, (nx - 1) * KV_COST / 10.0)
            dft.drain()
        for p in range(2):
            for j in range(FH // L):
                job_zs(i, p, j, bg, (1.6 * zb + extra, 0.5 * zb + extra), tied)
            assert not tied.tasks or (p == 0 and not last)
            if p == 0 and last:
                tied = _Tied(tasks(ln_z2, i, 8), 22)
        if last:
            for s in range(8, 16):
                ln_z2(i, s)
        bg.drain()
        job_h(t, hbg, nh * KV_COST / 10.0)
        hbg.drain()

    def p1_block(g):
        for i in P1_GROUPS[g]:
            p1_step(i)

    for g in range(len(P1_GROUPS)):
        p1_dma(g)
        block(lambda g=g: p1_block(g), f'p1_g{g}')

    groups = P2_GROUPS
    NG = len(groups)

    def p2_dma(gi):
        if gi >= 2:
            for i in groups[gi - 2]:
                start(cp_out(i))
        if gi >= 3:
            for i in groups[gi - 3]:
                wait(cp_out(i))
        if gi == 1:
            for i in (6, 7):
                start(cp_wsp(i))
        if gi == 0:
            wait(cp_conv(6, 2))
        if gi + 1 < NG:
            for i in groups[gi + 1]:
                wait(cp_wsp(i))

    def tails_of(i, bg, budget):
        return [tail_gen(i, bg, budget)] * 20

    def p2_block(gi):
        bg = _Background()
        steps = groups[gi]
        tb = [0.0]
        pending = [t_ for i in (groups[gi - 1] if gi > 0 else []) for t_ in tails_of(i, bg, tb)]
        total = sum(a + 1 for i in steps for a in _blocks_of_step(i)) * 40 * 16
        total += len(steps) * (24 * E_COST + 6 * U_COST) + len(pending) * T_COST
        slots = 84 * len(steps) + TAIL_W * len(pending)
        bg.add(freq_gen(_blocks_of_step(steps[0])[0]))
        if gi < 2:
            bg.add(kv_gen(NT - 2 + gi))
            total += 20 * KV_COST
            slots += 10
        for t in P2_X[gi]:
            slots += 10
        if gi + 1 < NG:
            for i in groups[gi + 1]:
                bg.add(acomb_gen(i))
                total += 32 * A_COST
        for i in steps[1:]:
            bg.add(freq_gen(_blocks_of_step(i)[0]))
        budget = tb[0] = total / slots
        bg.run(budget)
        for t in P2_X[gi]:
            job_x(t, bg, budget)
        if gi < 2:
            job_h(NT - 2 + gi, bg, budget)
        units = [4, 4, 2, 4, 4, 2] * (len(pending) // 20)
        every = [0] * (6 * len(steps))
        for j, n in enumerate(units):
            every[min(len(every) - 1, j * len(every) // len(units))] += n
        for i in steps:
            job_big(i, bg, pending, budget, every)
        for t_ in pending:
            next(t_)
        bg.drain()

    for gi in range(NG):
        p2_dma(gi)
        block(lambda gi=gi: p2_block(gi), f'p2_{gi}')

    def cp_last(part):
        a0 = _blocks_of_step(NT - 1)[0]
        sub, cols = ((MC, pl.ds(0, D)), (0, pl.ds(0, 4 * L)), (0, pl.ds(4 * L, L)))[part]
        return [pltpu.make_async_copy(o_v.at[pl.ds(r, MC), cols], o_hbm.at[0, pl.ds(r, MC), cols],
                                      sem_out.at[NT - 1]) for r in (a0 * P + sub, (a0 + 1) * P + sub)]

    def p2_last():
        for i in groups[NG - 1]:
            for j, t_ in enumerate(tails_of(i, _Background(), [0.0])):
                next(t_)
                if i < NT - 1 and j == 19:
                    start(cp_out(i))
                if i == NT - 1 and j in (9, 17):
                    start(cp_last(j // 10))

    p2_dma(NG)
    block(p2_last, 'p2_last')
    start(cp_last(2))
    for i in groups[NG - 2] + groups[NG - 1][:-1]:
        wait(cp_out(i))
    for part in range(3):
        wait(cp_last(part))
    debug_keep_alive()


@jax.jit
def pallas_recurrent_scan__ssm_conv_h3__mixer_gmlp__prompt_kernel(
    A_q: jax.Array,
    A_k: jax.Array,
    A_v: jax.Array,
    A_shift_k: jax.Array,
    A_ssm_k: jax.Array,
    A_ssm_D: jax.Array,
    B_x: jax.Array,
    B_w_in: jax.Array,
    B_w_sp: jax.Array,
    B_b_sp: jax.Array,
    B_w_out: jax.Array,
):
    del B_x
    hbm = pl.BlockSpec(memory_space=pl.ANY)

    def bf16_buf(*shape):
        return pltpu.VMEM(shape[:-2] + (shape[-2] // 2, shape[-1]), U32)

    return pl.pallas_call(
        _kernel,
        out_shape=jax.ShapeDtypeStruct((1, S, D), BF16),
        in_specs=[hbm] * 10,
        out_specs=hbm,
        scratch_shapes=[
            bf16_buf(S, D),
            bf16_buf(S, D),
            bf16_buf(S, D),
            bf16_buf(D, S),
            bf16_buf(D, 2 * FH),
            bf16_buf(S, S),
            bf16_buf(FH, D),
            pltpu.VMEM((S, D), BF16),
            pltpu.VMEM((4, D), BF16),
            pltpu.VMEM((D,), BF16),
            pltpu.VMEM((S,), BF16),
            bf16_buf(S, D),
            bf16_buf(4 * 5 * P, KH),
            bf16_buf(5 * KH, FH),
            bf16_buf(5 * 5 * P, HN),
            bf16_buf(5 * HN, 2 * L),
            pltpu.VMEM((S, FH), F32),
            bf16_buf(7 * HK, HN),
            bf16_buf(5 * 5 * P, HK),
            pltpu.VMEM((HK, FH), F32),
            pltpu.VMEM((3, TM, FH), F32),
            bf16_buf(S, D),
            bf16_buf(S, FH),
            pltpu.VMEM((NB, 2, P, D), F32),
            pltpu.VMEM((2, 2, P, D), F32),
            pltpu.VMEM((NB, 2, P, D), F32),
            bf16_buf(NB * 2 * P, D),
            pltpu.VMEM((2, D // L, MC, L), F32),
            bf16_buf(2 * P, 2 * P),
            bf16_buf(MC, 2 * P),
            pltpu.VMEM((S, L), F32),
            pltpu.VMEM((2, P, L), F32),
            pltpu.VMEM((4, 8, D), F32),
            pltpu.VMEM((D // L, S + 8, L), F32),
            pltpu.SemaphoreType.DMA((1,)),
            pltpu.SemaphoreType.DMA((NT,)),
            pltpu.SemaphoreType.DMA((NT,)),
            pltpu.SemaphoreType.DMA((NT,)),
            pltpu.SemaphoreType.DMA((5,)),
            pltpu.SemaphoreType.DMA((NT,)),
        ],
        compiler_params=pltpu.CompilerParams(vmem_limit_bytes=116 * 1024 * 1024, disable_semaphore_checks=True),
    )(A_q, A_k, A_v, A_shift_k.T, A_ssm_k, A_ssm_D, B_w_in, B_w_sp, B_b_sp, B_w_out)
```

```python
import math

import jax
import jax.numpy as jnp
import jax.experimental.pallas as pl
import jax.experimental.pallas.tpu as pltpu

S = 2048
D = 640
FH = 768
P = 128
NB = S // P
TM = 256
NT = S // TM
MC = 64
L = 128
HK = S // 2
KH = 256
HN = FH // 2
EPS = 1e-5
F32 = jnp.float32
BF16 = jnp.bfloat16
U32 = jnp.uint32
GELU_C = math.sqrt(2.0 / math.pi)
GA = (GELU_C * 0.044715) ** (1.0 / 3.0)
NT_DIMS = (((1,), (1,)), ((), ()))

WIN_CHUNKS = ((6, 7), (7, 9), (9, 12), (0, 3), (3, 6))
X_DMAS = ((0,), (1,), (2,), (3,), (4, 5), (6, 7))
CONV_DMAS = ((0,), (1,), (2, 3), (4, 5), (6, 7))
P1_GROUPS = ((2,), (3,), (4, 5), (6, 7))
P1_X = {2: None, 3: 0, 4: 1, 5: None, 6: 2, 7: 3}
P1_LNX = {2: (3,), 3: (4, 5), 4: (6,), 5: (7,), 6: (), 7: ()}
P2_GROUPS = ((0,), (1, 2), (3, 4, 5), (6, 7))
P2_X = ((4, 5), (6,), (7,), ())
STEP_BLOCKS = ((6, 7), (8, 9), (4, 5), (12, 13), (10, 11), (0, 1), (14, 15), (2, 3))
KV_COST, A_COST = 110, 56
E_COST, U_COST, T_COST, TAIL_W = 24, 90, 90, 1.6
KV_SPLIT = (12, 4, 4)
H_SPLIT = ((0, 2), (2, 4), (4, 5))
TIED_N = 42
F_TIED = (20, 20, 18, 20, 20)
_ONLY = None


def _dot(a, b):
    return jnp.dot(a, b, preferred_element_type=F32)


def _cos_sin(m):
    q = (m + 256) >> 9
    x = (m - (q << 9)).astype(F32) * (2.0 * math.pi / 2048.0)
    x2 = x * x
    s = x * (1.0 + x2 * (-1.0 / 6 + x2 * (1.0 / 120 + x2 * (-1.0 / 5040 + x2 * (1.0 / 362880)))))
    c = 1.0 + x2 * (-0.5 + x2 * (1.0 / 24 + x2 * (-1.0 / 720 + x2 * (1.0 / 40320 - x2 * (1.0 / 3628800)))))
    swap = (q & 1) == 1
    c0 = jnp.where(swap, s, c)
    s0 = jnp.where(swap, c, s)
    cos = jnp.where(((q + 1) & 2) == 2, -c0, c0)
    sin = jnp.where((q & 2) == 2, -s0, s0)
    return cos, sin


def _odd_freq(r):
    return jnp.where(r < 64, 4 * r + 1, 4 * r - 253)


def _gelu_scaled(z):
    return z + z * jnp.tanh(z * (GELU_C / GA + z * z))


def _signzero(z):
    bits = jax.lax.bitcast_convert_type(z, U32) & jnp.uint32(0x80000000)
    return jax.lax.bitcast_convert_type(bits, F32)


def _ln(x, eps, tie=None, scale=None):
    n = x.shape[-1]
    cols = [x[:, j * L:(j + 1) * L] for j in range(n // L)]
    s1 = cols[0]
    s2 = cols[0] * cols[0]
    for c in cols[1:]:
        s1 = s1 + c
        s2 = s2 + c * c
    if tie is not None:
        s1 = s1 + tie
        s2 = s2 + tie
    m = jnp.sum(s1, axis=-1, keepdims=True) * (1.0 / n)
    v = jnp.maximum(jnp.sum(s2, axis=-1, keepdims=True) * (1.0 / n) - m * m, 0.0)
    rs = jax.lax.rsqrt(v + eps)
    if scale is not None:
        rs = rs * scale
    return (x - m) * rs


def _blocks_of_step(i):
    return STEP_BLOCKS[i]


class _Background:
    def __init__(self):
        self.q = []
        self.credit = 0.0

    def add(self, gen):
        self.q.append(gen)

    def run(self, budget):
        self.credit += budget
        while self.q and self.credit > 0:
            try:
                self.credit -= next(self.q[0])
            except StopIteration:
                self.q.pop(0)
        if not self.q:
            self.credit = 0.0

    def charge(self, cost):
        self.credit -= cost

    def drain(self):
        while self.q:
            self.run(1e9)


class _Tied:
    def __init__(self, tasks, npieces):
        self.tasks = list(tasks)
        self.rate = len(self.tasks) / float(npieces)
        self.credit = 0.999

    def run(self, z):
        self.credit += self.rate
        n = 0
        while self.tasks and self.credit >= 1.0:
            self.tasks.pop(0)(_signzero(z[0:16]))
            self.credit -= 1.0
            n += 1
        return n


def _kernel(q_hbm, k_hbm, v_hbm, sk_hbm, h_hbm, d_hbm, win_hbm, wsp_hbm, b_hbm, wout_hbm,
            o_hbm,
            x_us, k_us, v_us, h_us, win_us, wsp_us, wout_u, o_v, sk_in, d_in, b_in,
            xn_u, XL_u, WB_u, UL_u, WO_u, z1_v, R_u, Lc_u, zf_v, zg_v, kv_u, u_u, X_v, H_v, G_v, Z_u,
            yl_v, F_u, Fi_u, bcol_v, ph_v, sk_v, kf_v,
            sem_small, sem_x, sem_conv, sem_wsp, sem_w, sem_out):
    (wout_v, xn_v, XL_v, WB_v, UL_v, WO_v, R_v, Lc_v, kv_v, u_v, Z_v, F_v, Fi_v) = [
        r.bitcast(BF16) for r in (wout_u, xn_u, XL_u, WB_u, UL_u, WO_u, R_u, Lc_u, kv_u, u_u, Z_u, F_u, Fi_u)]
    x_vs = {g[0]: r.bitcast(BF16) for g, r in zip(X_DMAS, x_us)}
    k_vs, v_vs, h_vs = [{g[0]: r.bitcast(BF16) for g, r in zip(CONV_DMAS, rs)} for rs in (k_us, v_us, h_us)]
    wsp_vs = [r.bitcast(BF16) for r in wsp_us]
    win_vs = [r.bitcast(BF16) for r in win_us]

    def win(rows, n):
        c = [lo <= n < hi for lo, hi in WIN_CHUNKS].index(True)
        n -= WIN_CHUNKS[c][0]
        return win_vs[c][rows, n * L:(n + 1) * L]

    def locate(bufs, row):
        t0 = max(t for t in bufs if t * TM <= row)
        return bufs[t0], row - t0 * TM

    def rows_of(bufs, row, n, lanes=slice(None)):
        buf, r = locate(bufs, row)
        return buf[r:r + n, lanes]

    def cp_small():
        return [pltpu.make_async_copy(s_, d_, sem_small.at[0])
                for s_, d_ in ((d_hbm, d_in), (sk_hbm, sk_in), (b_hbm, b_in))]

    def cp_x(t):
        return pltpu.make_async_copy(q_hbm.at[0, pl.ds(t * TM, x_vs[t].shape[0])], x_vs[t], sem_x.at[t])

    def cp_conv(t):
        rows = pl.ds(t * TM, k_vs[t].shape[0])
        sem = sem_conv.at[t]
        return [pltpu.make_async_copy(h_hbm.at[:, rows], h_vs[t], sem),
                pltpu.make_async_copy(k_hbm.at[0, rows], k_vs[t], sem),
                pltpu.make_async_copy(v_hbm.at[0, rows], v_vs[t], sem)]

    def cp_wsp(i):
        return [pltpu.make_async_copy(wsp_hbm.at[pl.ds(_blocks_of_step(i)[0] * P, TM)], wsp_vs[i], sem_wsp.at[i])]

    def cp_win(c):
        lo, hi = WIN_CHUNKS[c]
        w = (hi - lo) * L
        return pltpu.make_async_copy(win_hbm.at[:, pl.ds(lo * L, w)], win_vs[c].at[:, pl.ds(0, w)], sem_w.at[c])

    def cp_wout():
        return pltpu.make_async_copy(wout_hbm, wout_v, sem_w.at[0])

    def cp_out(i):
        rows = pl.ds(_blocks_of_step(i)[0] * P, TM)
        return [pltpu.make_async_copy(o_v.at[rows], o_hbm.at[0, rows], sem_out.at[i])]

    def start(cs):
        for c in cs:
            c.start()

    def wait(cs):
        for c in cs:
            c.wait()

    def block(fn, name):
        def body(it):
            fn()
            return it + 1

        if _ONLY is None or name in _ONLY:
            jax.lax.while_loop(lambda it: it < 1, body, jnp.int32(0))

    def ln_x(t, s, tie=None):
        rows = pl.ds(t * TM + s * 16, 16)
        y = _ln(rows_of(x_vs, t * TM + s * 16, 16).astype(F32), EPS, tie, GA)
        xn_v[rows, :] = y.astype(BF16)
        return y

    def ln_x2(t, s, tie):
        p, q = s // 4, s % 4
        y1 = ln_x(t, 8 * p + q, tie)
        y2 = ln_x(t, 8 * p + 4 + q, tie)
        a11, a12, a21, a22 = y1[:, :KH], y1[:, KH:2 * KH], y2[:, :KH], y2[:, KH:2 * KH]
        r0 = (t % 4) * 5 * P + p * MC + q * 16
        for j, c in enumerate((a11 + a22, a21 + a22, a11 + a12, a21 - a11, a12 - a22)):
            XL_v[pl.ds(r0 + j * P, 16), :] = c.astype(BF16)

    def wcomb_gen(cols):
        for j in cols:
            c1 = slice(j * L, (j + 1) * L)
            for r in range(KH // 32):
                top = pl.ds(r * 32, 32)
                bot = pl.ds(KH + r * 32, 32)
                b11, b12 = win(top, j).astype(F32), win(top, 6 + j).astype(F32)
                b21, b22 = win(bot, j).astype(F32), win(bot, 6 + j).astype(F32)
                for w, c in enumerate((b11 + b22, b12 - b22, b21 - b11, b11 + b12, b21 + b22)):
                    WB_v[pl.ds(w * KH + r * 32, 32), c1] = c.astype(BF16)
                yield A_COST

    def ln_z2(t, s, tie=None):
        y = _ln(zg_v[t % 3, s * 16:(s + 1) * 16, :], 4.0 * GA * GA * EPS, tie, 0.25 / GA)
        lo, hi = y[:, :HN], y[:, HN:]
        r = (t * TM + s * 16) % HK
        rows = pl.ds(r, 16)
        if t < NT // 2:
            zf_v[rows, :] = y
            R_v[pl.ds(1 * HK + r, 16), :] = lo.astype(BF16)
            R_v[pl.ds(5 * HK + r, 16), :] = (lo + hi).astype(BF16)
        else:
            b11, b12 = zf_v[rows, :HN], zf_v[rows, HN:]
            R_v[pl.ds(0 * HK + r, 16), :] = (b11 + hi).astype(BF16)
            R_v[pl.ds(2 * HK + r, 16), :] = (b12 - hi).astype(BF16)
            R_v[pl.ds(3 * HK + r, 16), :] = (lo - b11).astype(BF16)
            R_v[pl.ds(4 * HK + r, 16), :] = hi.astype(BF16)
            R_v[pl.ds(6 * HK + r, 16), :] = (lo + hi).astype(BF16)

    def acomb_gen(i, groups=range(P // 16)):
        for r in groups:
            for c in range(HK // 256):
                top = pl.ds(r * 16, 16)
                bot = pl.ds(P + r * 16, 16)
                c1 = slice(c * 256, (c + 1) * 256)
                c2 = slice(HK + c * 256, HK + (c + 1) * 256)
                a11 = wsp_vs[i][top, c1].astype(F32)
                a12 = wsp_vs[i][top, c2].astype(F32)
                a21 = wsp_vs[i][bot, c1].astype(F32)
                a22 = wsp_vs[i][bot, c2].astype(F32)
                r0 = (i % 5) * 5 * P + r * 16
                Lc_v[pl.ds(r0 + 0 * P, 16), c1] = (a11 + a22).astype(BF16)
                Lc_v[pl.ds(r0 + 1 * P, 16), c1] = (a21 + a22).astype(BF16)
                Lc_v[pl.ds(r0 + 2 * P, 16), c1] = (a11 + a12).astype(BF16)
                Lc_v[pl.ds(r0 + 3 * P, 16), c1] = (a21 - a11).astype(BF16)
                Lc_v[pl.ds(r0 + 4 * P, 16), c1] = (a12 - a22).astype(BF16)
                yield A_COST

    def tasks(fn, t, n=TM // 16):
        return [lambda tie, s=s: fn(t, s, tie) for s in range(n)]

    def kv_gen(t):
        for m in range(TM // MC):
            r = t * TM + m * MC
            for l in range(D // L):
                lanes = slice(l * L, (l + 1) * L)
                kf = rows_of(k_vs, r, MC, lanes).astype(F32)
                kf_v[l, pl.ds(r + 8, MC), :] = kf
                ks = kf * sk_v[0, 0:1, lanes]
                for tap in range(1, 4):
                    ks = ks + kf_v[l, pl.ds(r + 8 - tap, MC), :] * sk_v[tap, 0:1, lanes]
                kv = ks * rows_of(v_vs, r, MC, lanes).astype(F32)
                kv_v[pl.ds(r, MC), lanes] = kv.astype(BF16)
                yield KV_COST

    def freq_gen(a):
        def cmac(acc, x, g):
            pr = x[0] * g[0] - x[1] * g[1]
            pi = x[0] * g[1] + x[1] * g[0]
            return (pr, pi) if acc is None else (acc[0] + pr, acc[1] + pi)

        for r in range(P // 16):
            rows = pl.ds(r * 16, 16)
            for l in range(D // L):
                lanes = slice(l * L, (l + 1) * L)
                lo = hi = None
                g = (G_v[a + 1, 0, rows, lanes], G_v[a + 1, 1, rows, lanes])
                for c in range(a + 2):
                    x = (X_v[c, 0, rows, lanes], X_v[c, 1, rows, lanes])
                    hi = cmac(hi, x, g)
                    if c <= a:
                        g = (G_v[a - c, 0, rows, lanes], G_v[a - c, 1, rows, lanes])
                        lo = cmac(lo, x, g)
                        yield 32
                for w, z in enumerate((lo, hi)):
                    for part in range(2):
                        Z_v[pl.ds((a + w) * 2 * P + part * P + r * 16, 16), lanes] = z[part].astype(BF16)
                yield 20

    def job_x(t, bg, budget):
        for j in (2 * t, 2 * t + 1):
            for half in range(2):
                r = _dot(F_v[half * P:(half + 1) * P, 0:P], kv_v[j * P:(j + 1) * P, :]).reshape(8, 2, 8, D)
                for part in range(2):
                    X_v[j, part, half * 64:(half + 1) * 64, :] = r[:, part].reshape(64, D)
                bg.run(budget * 2.5)

    def job_h(t, bg, budget):
        h_v, c0 = locate(h_vs, t * TM)
        for half in range(2):
            rows = pl.ds(half * 64, 64)
            for l0, l1 in H_SPLIT:
                w = (l1 - l0) * L
                lanes = slice(l0 * L, l1 * L)
                rhs = jnp.concatenate([h_v[lanes, c0:c0 + P], h_v[lanes, c0 + P:c0 + TM]], axis=0)
                r = jax.lax.dot_general(F_v[half * P:(half + 1) * P, 0:P], rhs, NT_DIMS,
                                        preferred_element_type=F32).reshape(8, 2, 8, 2 * w)
                re, im = r[:, 0].reshape(64, 2 * w), r[:, 1].reshape(64, 2 * w)
                prev = (H_v[t % 2, 0, rows, lanes], H_v[t % 2, 1, rows, lanes])
                for j in range(2):
                    cur = (re[:, j * w:(j + 1) * w], im[:, j * w:(j + 1) * w])
                    G_v[2 * t + j, 0, rows, lanes] = cur[0] + prev[1] if half else cur[0] - prev[1]
                    G_v[2 * t + j, 1, rows, lanes] = cur[1] - prev[0] if half else cur[1] + prev[0]
                    prev = cur
                if t + 1 < NT:
                    H_v[(t + 1) % 2, 0, rows, lanes] = prev[0]
                    H_v[(t + 1) % 2, 1, rows, lanes] = prev[1]
                bg.run(budget * (l1 - l0))

    def z_out(t, m, n, pre, bg, budget, tied):
        z = _gelu_scaled(pre)
        if n < FH // L:
            z1_v[pl.ds(t * TM + m * MC, MC), n * L:(n + 1) * L] = z
        else:
            zg_v[t % 3, m * MC:(m + 1) * MC, n * L - FH:(n + 1) * L - FH] = z
        ntask = tied.run(z)
        bg.run(budget[1] if ntask else budget[0])

    def job_z(t, m, cols, bg, budget, tied):
        for n in cols:
            z_out(t, m, n, _dot(xn_v[pl.ds(t * TM + m * MC, MC), :], win(slice(None), n)), bg, budget, tied)

    def job_zs(t, p, j, bg, budget, tied):
        r1 = pl.ds(t * TM + p * P, MC)
        r2 = pl.ds(t * TM + p * P + MC, MC)
        c1 = slice(j * L, (j + 1) * L)

        def xl(w):
            r0 = (t % 4) * 5 * P + w * P + p * MC
            return XL_v[r0:r0 + MC, :]

        def wb(w):
            return WB_v[w * KH:(w + 1) * KH, c1]

        def rem(rows, n):
            return _dot(xn_v[rows, 2 * KH:], win(slice(2 * KH, D), n))

        m2 = _dot(xl(1), win(slice(0, KH), j))
        m4 = _dot(xn_v[r2, KH:2 * KH], wb(2))
        z_out(t, 2 * p + 1, j, m2 + m4 + rem(r2, j), bg, budget, tied)
        m3 = _dot(xn_v[r1, 0:KH], wb(1))
        m5 = _dot(xl(2), win(slice(KH, 2 * KH), 6 + j))
        z_out(t, 2 * p, 6 + j, m3 + m5 + rem(r1, 6 + j), bg, budget, tied)
        t11, t22 = m4 - m5, m3 - m2
        m1 = _dot(xl(0), wb(0))
        t11, t22 = t11 + m1, t22 + m1
        z_out(t, 2 * p, j, t11 + _dot(xl(4), wb(4)) + rem(r1, j), bg, budget, tied)
        z_out(t, 2 * p + 1, 6 + j, t22 + _dot(xl(3), wb(3)) + rem(r2, 6 + j), bg, budget, tied)

    rev8 = 7 - jax.lax.broadcasted_iota(jnp.int32, (8, L), 0)

    def finish(a, upper, n, hh, slot):
        rows = pl.ds(a * P + (MC if upper else 0), MC)
        lanes = slice(n * L, (n + 1) * L)
        if upper:
            ya = _dot(Fi_v[:, 0:P], Z_v[a * 2 * P:a * 2 * P + P, lanes])
            yb = _dot(Fi_v[:, P:2 * P], Z_v[a * 2 * P + P:(a + 1) * 2 * P, lanes])
            slot(0.5)
            y = ya - yb
            lo = ya + yb
            for j in range(MC // 8):
                yl_v[a % 2, n, (7 - j) * 8:(8 - j) * 8, :] = jnp.take_along_axis(lo[j * 8:(j + 1) * 8], rev8, axis=0)
        else:
            y = yl_v[a % 2, n]
        gate = hh + hh * jnp.tanh(hh)
        s = xn_v[rows, lanes].astype(F32) * y
        x = rows_of(x_vs, a * P + (MC if upper else 0), MC, lanes).astype(F32)
        o_v[rows, lanes] = (x + s * gate).astype(BF16)

    def tail_gen(i, bg, budget):
        a0, a1 = _blocks_of_step(i)

        def slot(w):
            bg.run(w * budget[0])

        def dot3(a, b):
            r = _dot(a, b)
            slot(0.75)
            return r

        for upper in (True, False):
            sub = MC if upper else 0
            r1 = pl.ds(a0 * P + sub, MC)
            r2 = pl.ds(a1 * P + sub, MC)

            def ul(w):
                r0 = ((i % 5) * 5 + w) * P + sub
                return UL_v[r0:r0 + MC, :]

            for j in range(2):
                c1 = slice(j * L, (j + 1) * L)
                c2 = slice((2 + j) * L, (3 + j) * L)

                def wo(w):
                    return WO_v[w * HN:(w + 1) * HN, c1]

                m2 = dot3(ul(1), wout_v[0:HN, c1])
                m4 = dot3(u_v[r2, HN:], wo(2))
                finish(a1, upper, j, m2 + m4, slot)
                bg.charge(T_COST)
                yield
                m3 = dot3(u_v[r1, 0:HN], wo(1))
                m5 = dot3(ul(2), wout_v[HN:, c2])
                finish(a0, upper, 2 + j, m3 + m5, slot)
                bg.charge(T_COST)
                yield
                m1 = dot3(ul(0), wo(0))
                finish(a0, upper, j, (m4 - m5) + m1 + dot3(ul(4), wo(4)), slot)
                bg.charge(T_COST)
                yield
                finish(a1, upper, 2 + j, (m3 - m2) + m1 + dot3(ul(3), wo(3)), slot)
                bg.charge(T_COST)
                yield
            for a, r in ((a0, r1), (a1, r2)):
                finish(a, upper, 4, dot3(u_v[r, 0:HN], wout_v[0:HN, 4 * L:]) + dot3(u_v[r, HN:], wout_v[HN:, 4 * L:]),
                       slot)
                bg.charge(T_COST)
                yield

    def wocomb_gen():
        for j in range(2):
            c1 = slice(j * L, (j + 1) * L)
            c2 = slice((2 + j) * L, (3 + j) * L)
            for r in range(HN // 32):
                top = pl.ds(r * 32, 32)
                bot = pl.ds(HN + r * 32, 32)
                b11, b12 = wout_v[top, c1].astype(F32), wout_v[top, c2].astype(F32)
                b21, b22 = wout_v[bot, c1].astype(F32), wout_v[bot, c2].astype(F32)
                for w, c in enumerate((b11 + b22, b12 - b22, b21 - b11, b11 + b12, b21 + b22)):
                    WO_v[pl.ds(w * HN + r * 32, 32), c1] = c.astype(BF16)
                yield A_COST

    def job_big(i, bg, pending, budget, every):
        a0, a1 = _blocks_of_step(i)
        KG = 512

        def lhs(j, sub, cols):
            if j == 2:
                return wsp_vs[i][sub:sub + MC, cols]
            if j == 3:
                return wsp_vs[i][P + sub:P + sub + MC, HK + cols.start:HK + cols.stop]
            r0 = ((i % 5) * 5 + {0: 0, 1: 1, 4: 2, 5: 3, 6: 4}[j]) * P + sub
            return Lc_v[r0:r0 + MC, cols]

        def prod(j, sub, n, acc=None):
            for kg in range(HK // KG):
                ks = slice(kg * KG, (kg + 1) * KG)
                p = _dot(lhs(j, sub, ks), R_v[j * HK + kg * KG:j * HK + (kg + 1) * KG, n * L:(n + 1) * L])
                acc = p if acc is None else acc + p
                bg.run(budget)
            return acc

        def tails(n):
            for _ in range(n):
                if pending:
                    next(pending.pop(0))

        def emit(a, sub, n, g):
            rows = pl.ds(a * P + sub, MC)
            lanes = slice(n * L, (n + 1) * L)
            u = z1_v[rows, lanes] * (g + bcol_v[rows, :])
            u_v[rows, lanes] = u.astype(BF16)
            bg.charge(E_COST)
            return u

        for sub in (0, MC):
            for n in range(HN // L):
                def put(w, c):
                    UL_v[pl.ds(((i % 5) * 5 + w) * P + sub, MC), n * L:(n + 1) * L] = c.astype(BF16)

                m1 = prod(0, sub, n)
                t11 = prod(6, sub, n, m1)
                m4 = prod(3, sub, n)
                t11 = t11 + m4
                m5 = prod(4, sub, n)
                u11 = emit(a0, sub, n, t11 - m5)
                m2 = prod(1, sub, n)
                u21 = emit(a1, sub, n, m2 + m4)
                put(3, u21 - u11)
                t22 = m1 - m2
                m3 = prod(2, sub, n)
                u12 = emit(a0, sub, n + HN // L, m3 + m5)
                put(2, u11 + u12)
                u22 = emit(a1, sub, n + HN // L, prod(5, sub, n, t22 + m3))
                put(0, u11 + u22)
                put(1, u21 + u22)
                put(4, u12 - u22)
                bg.charge(U_COST)
                tails(every.pop(0))

    def debug_keep_alive():
        if _ONLY is not None:
            for r_ in (xn_u, XL_u, WB_u, UL_u, WO_u, z1_v, R_u, Lc_u, zf_v, zg_v, kv_u, u_u, X_v, H_v, G_v, Z_u,
                       kf_v, bcol_v):
                c_ = pltpu.make_async_copy(r_, r_, sem_small.at[0])
                c_.start()
                c_.wait()

    debug_keep_alive()

    cp_x(0).start()
    cp_win(0).start()
    cp_x(1).start()
    cp_win(1).start()
    start(cp_small())
    for c in range(2, 5):
        cp_win(c).start()
    cp_x(2).start()

    kk = _odd_freq(jax.lax.broadcasted_iota(jnp.int32, (P, P), 0))
    nn = jax.lax.broadcasted_iota(jnp.int32, (P, P), 1)
    fc, fs = _cos_sin((kk * (4 * nn - 127)) & 2047)
    for g in range(P // 8):
        F_v[g * 16:(g + 1) * 16, 0:P] = jnp.concatenate(
            [fc[g * 8:(g + 1) * 8], -fs[g * 8:(g + 1) * 8]], axis=0).astype(BF16)
    fc, fs = _cos_sin((kk * (-127)) & 2047)
    ph_v[0] = fc
    ph_v[1] = fs
    kk = _odd_freq(jax.lax.broadcasted_iota(jnp.int32, (MC, P), 1))
    mm = jax.lax.broadcasted_iota(jnp.int32, (MC, P), 0)
    ic, is_ = _cos_sin((kk * (4 * mm + 2)) & 2047)
    Fi_v[:, 0:P] = (ic * (1.0 / (P * GA))).astype(BF16)
    Fi_v[:, P:2 * P] = (is_ * (1.0 / (P * GA))).astype(BF16)
    kf_v[:, 0:8, :] = jnp.zeros((D // L, 8, L), F32)

    cp_x(0).wait()
    for s in range(TM // 16):
        ln_x(0, s)

    def small_setup():
        sk = sk_in[...].astype(F32)
        for t in range(4):
            sk_v[t] = jnp.broadcast_to(sk[t:t + 1], (8, D))
        drow = d_in[...].astype(F32).reshape(1, D)
        for l in range(D // L):
            lanes = slice(l * L, (l + 1) * L)
            dre = ph_v[0] * drow[:, lanes]
            dim = ph_v[1] * drow[:, lanes]
            H_v[0, 0, 0:64, lanes] = -dim[0:64]
            H_v[0, 0, 64:P, lanes] = dim[64:P]
            H_v[0, 1, 0:64, lanes] = -dre[0:64]
            H_v[0, 1, 64:P, lanes] = dre[64:P]

    def bcol_task(t, j, tie):
        brow = b_in[...].astype(F32).reshape(1, S)[:, j * P:(j + 1) * P] * (0.25 / GA) + tie[0:1]
        bcol_v[j * P:(j + 1) * P, :] = jnp.broadcast_to(brow, (P, P)).T

    LAG = 2

    def interleave(*lists):
        out = []
        for j in range(max(len(a) for a in lists)):
            for a in lists:
                out += a[j:j + 1]
        return out

    def p1_first(c):
        bg = _Background()
        todo = []
        if c == 2:
            todo = tasks(bcol_task, 0)
            small_setup()
        if c == 3:
            todo = tasks(ln_z2, 0)
            bg.add(wcomb_gen(range(3)))
        if c == 4:
            todo = tasks(ln_x2, 2, 8)
            bg.add(wcomb_gen(range(3, 6)))
        tied = _Tied(todo, F_TIED[c])
        if c == 0:
            for s in range(TM // 16):
                ln_x(1, s)
        for t in range(2):
            for m in range(TM // MC):
                job_z(t, m, range(*WIN_CHUNKS[c]), bg, (80, 40), tied)
        bg.drain()
        assert not tied.tasks

    for c in range(5):
        cp_win(c).wait()
        if c == 0:
            cp_x(1).wait()
        if c == 2:
            wait(cp_small())
            start(cp_conv(0))
            cp_x(3).start()
        if c == 4:
            cp_x(2).wait()
            cp_x(4).start()
        block(lambda c=c: p1_first(c), f'p1_f{c}')

    def p1_wait(g):
        if g == 0:
            wait(cp_conv(0))
            cp_x(3).wait()
        if g == 1:
            wait(cp_conv(1))
            cp_x(4).wait()
        if g == 2:
            wait(cp_conv(2))
            cp_x(6).wait()
        if g == 3:
            wait(cp_conv(4))
            cp_wout().wait()
            wait(cp_wsp(0))

    def p1_start(g):
        if g == 0:
            start(cp_conv(1))
            cp_x(6).start()
            start(cp_conv(2))
        if g == 1:
            start(cp_conv(4))
            cp_wout().start()
            start(cp_wsp(0))
            start(cp_wsp(1))
        if g == 3:
            start(cp_wsp(2))
            start(cp_conv(6))
            for i in (3, 4, 5):
                start(cp_wsp(i))

    def take(gen, n):
        for _ in range(n):
            yield next(gen)

    def p1_step(i):
        bg = _Background()
        dft = _Background()
        t = i - LAG
        xg = P1_X[i]
        kv = kv_gen(t)
        nx, nz, nh = KV_SPLIT if xg is not None else (0, KV_SPLIT[0] + KV_SPLIT[1], KV_SPLIT[2])
        dft.add(take(kv, nx))
        bg.add(take(kv, nz))
        hbg = _Background()
        hbg.add(take(kv, nh))
        zb = nz * KV_COST / 48.0
        extra = 0
        if i == 6:
            bg.add(wocomb_gen())
            bg.add(acomb_gen(0, range(3)))
            extra = 42
        if i == 7:
            bg.add(acomb_gen(0, range(3, 8)))
            extra = 24
        last = i == NT - 1
        z2t = tasks(ln_z2, i - 1)
        todo = interleave(*([tasks(ln_x2, t_, 8) for t_ in P1_LNX[i]] + [z2t[0::2], z2t[1::2]]))
        tied = _Tied(todo, 24 if last else TIED_N)
        if xg is not None:
            dft.run(KV_COST)
            job_x(xg, dft, (nx - 1) * KV_COST / 10.0)
            dft.drain()
        for p in range(2):
            for j in range(FH // L):
                job_zs(i, p, j, bg, (1.6 * zb + extra, 0.5 * zb + extra), tied)
            assert not tied.tasks or (p == 0 and not last)
            if p == 0 and last:
                tied = _Tied(tasks(ln_z2, i, 8), 22)
        if last:
            for s in range(8, 16):
                ln_z2(i, s)
        bg.drain()
        job_h(t, hbg, nh * KV_COST / 10.0)
        hbg.drain()

    def p1_block(g):
        for i in P1_GROUPS[g]:
            p1_step(i)

    for g in range(len(P1_GROUPS)):
        p1_wait(g)
        p1_start(g)
        block(lambda g=g: p1_block(g), f'p1_g{g}')

    groups = P2_GROUPS
    NG = len(groups)

    def p2_dma(gi):
        if gi >= 2:
            for i in groups[gi - 2]:
                start(cp_out(i))
        if gi >= 3:
            for i in groups[gi - 3]:
                wait(cp_out(i))
        if gi == 1:
            for i in (6, 7):
                start(cp_wsp(i))
        if gi == 0:
            wait(cp_conv(6))
        if gi + 1 < NG:
            for i in groups[gi + 1]:
                wait(cp_wsp(i))

    def tails_of(i, bg, budget):
        return [tail_gen(i, bg, budget)] * 20

    def p2_block(gi):
        bg = _Background()
        steps = groups[gi]
        tb = [0.0]
        pending = [t_ for i in (groups[gi - 1] if gi > 0 else []) for t_ in tails_of(i, bg, tb)]
        total = sum(a + 1 for i in steps for a in _blocks_of_step(i)) * 40 * 16
        total += len(steps) * (24 * E_COST + 6 * U_COST) + len(pending) * T_COST
        slots = 84 * len(steps) + TAIL_W * len(pending)
        bg.add(freq_gen(_blocks_of_step(steps[0])[0]))
        if gi < 2:
            bg.add(kv_gen(NT - 2 + gi))
            total += 20 * KV_COST
            slots += 10
        for t in P2_X[gi]:
            slots += 10
        if gi + 1 < NG:
            for i in groups[gi + 1]:
                bg.add(acomb_gen(i))
                total += 32 * A_COST
        for i in steps[1:]:
            bg.add(freq_gen(_blocks_of_step(i)[0]))
        budget = tb[0] = total / slots
        bg.run(budget)
        for t in P2_X[gi]:
            job_x(t, bg, budget)
        if gi < 2:
            job_h(NT - 2 + gi, bg, budget)
        units = [4, 4, 2, 4, 4, 2] * (len(pending) // 20)
        every = [0] * (6 * len(steps))
        for j, n in enumerate(units):
            every[min(len(every) - 1, j * len(every) // len(units))] += n
        for i in steps:
            job_big(i, bg, pending, budget, every)
        for t_ in pending:
            next(t_)
        bg.drain()

    for gi in range(NG):
        p2_dma(gi)
        block(lambda gi=gi: p2_block(gi), f'p2_{gi}')

    def cp_last(part):
        a0 = _blocks_of_step(NT - 1)[0]
        sub, cols = ((MC, pl.ds(0, D)), (0, pl.ds(0, 4 * L)), (0, pl.ds(4 * L, L)))[part]
        return [pltpu.make_async_copy(o_v.at[pl.ds(r, MC), cols], o_hbm.at[0, pl.ds(r, MC), cols],
                                      sem_out.at[NT - 1]) for r in (a0 * P + sub, (a0 + 1) * P + sub)]

    def p2_last():
        for i in groups[NG - 1]:
            for j, t_ in enumerate(tails_of(i, _Background(), [0.0])):
                next(t_)
                if i < NT - 1 and j == 19:
                    start(cp_out(i))
                if i == NT - 1 and j in (9, 17):
                    start(cp_last(j // 10))

    p2_dma(NG)
    block(p2_last, 'p2_last')
    start(cp_last(2))
    for i in groups[NG - 2] + groups[NG - 1][:-1]:
        wait(cp_out(i))
    for part in range(3):
        wait(cp_last(part))
    debug_keep_alive()


@jax.jit
def pallas_recurrent_scan__ssm_conv_h3__mixer_gmlp__prompt_kernel(
    A_q: jax.Array,
    A_k: jax.Array,
    A_v: jax.Array,
    A_shift_k: jax.Array,
    A_ssm_k: jax.Array,
    A_ssm_D: jax.Array,
    B_x: jax.Array,
    B_w_in: jax.Array,
    B_w_sp: jax.Array,
    B_b_sp: jax.Array,
    B_w_out: jax.Array,
):
    del B_x
    hbm = pl.BlockSpec(memory_space=pl.ANY)

    def bf16_buf(*shape):
        return pltpu.VMEM(shape[:-2] + (shape[-2] // 2, shape[-1]), U32)

    return pl.pallas_call(
        _kernel,
        out_shape=jax.ShapeDtypeStruct((1, S, D), BF16),
        in_specs=[hbm] * 10,
        out_specs=hbm,
        scratch_shapes=[
            [bf16_buf(len(g) * TM, D) for g in X_DMAS],
            [bf16_buf(len(g) * TM, D) for g in CONV_DMAS],
            [bf16_buf(len(g) * TM, D) for g in CONV_DMAS],
            [bf16_buf(D, len(g) * TM) for g in CONV_DMAS],
            [bf16_buf(D, max(hi - lo, 2) * L) for lo, hi in WIN_CHUNKS],
            [bf16_buf(TM, S) for _ in range(NT)],
            bf16_buf(FH, D),
            pltpu.VMEM((S, D), BF16),
            pltpu.VMEM((4, D), BF16),
            pltpu.VMEM((D,), BF16),
            pltpu.VMEM((S,), BF16),
            bf16_buf(S, D),
            bf16_buf(4 * 5 * P, KH),
            bf16_buf(5 * KH, FH),
            bf16_buf(5 * 5 * P, HN),
            bf16_buf(5 * HN, 2 * L),
            pltpu.VMEM((S, FH), F32),
            bf16_buf(7 * HK, HN),
            bf16_buf(5 * 5 * P, HK),
            pltpu.VMEM((HK, FH), F32),
            pltpu.VMEM((3, TM, FH), F32),
            bf16_buf(S, D),
            bf16_buf(S, FH),
            pltpu.VMEM((NB, 2, P, D), F32),
            pltpu.VMEM((2, 2, P, D), F32),
            pltpu.VMEM((NB, 2, P, D), F32),
            bf16_buf(NB * 2 * P, D),
            pltpu.VMEM((2, D // L, MC, L), F32),
            bf16_buf(2 * P, 2 * P),
            bf16_buf(MC, 2 * P),
            pltpu.VMEM((S, L), F32),
            pltpu.VMEM((2, P, L), F32),
            pltpu.VMEM((4, 8, D), F32),
            pltpu.VMEM((D // L, S + 8, L), F32),
            pltpu.SemaphoreType.DMA((1,)),
            pltpu.SemaphoreType.DMA((NT,)),
            pltpu.SemaphoreType.DMA((NT,)),
            pltpu.SemaphoreType.DMA((NT,)),
            pltpu.SemaphoreType.DMA((5,)),
            pltpu.SemaphoreType.DMA((NT,)),
        ],
        compiler_params=pltpu.CompilerParams(vmem_limit_bytes=116 * 1024 * 1024, disable_semaphore_checks=True),
    )(A_q, A_k, A_v, A_shift_k.T, A_ssm_k, A_ssm_D, B_w_in, B_w_sp, B_b_sp, B_w_out)
```

```python
import math

import jax
import jax.numpy as jnp
import jax.experimental.pallas as pl
import jax.experimental.pallas.tpu as pltpu

S = 2048
D = 640
FH = 768
P = 128
NB = S // P
TM = 256
NT = S // TM
MC = 64
L = 128
HK = S // 2
KH = 256
HN = FH // 2
EPS = 1e-5
F32 = jnp.float32
BF16 = jnp.bfloat16
U32 = jnp.uint32
GELU_C = math.sqrt(2.0 / math.pi)
GA = (GELU_C * 0.044715) ** (1.0 / 3.0)
NT_DIMS = (((1,), (1,)), ((), ()))

WIN_CHUNKS = ((6, 7), (7, 9), (9, 12), (0, 3), (3, 6))
X_DMAS = ((0,), (1,), (2,), (3,), (4, 5), (6, 7))
CONV_DMAS = ((0,), (1,), (2, 3), (4, 5), (6, 7))
P1_GROUPS = ((2,), (3,), (4, 5), (6, 7))
P1_X = {2: None, 3: 0, 4: 1, 5: None, 6: 2, 7: 3}
P1_LNX = {2: (3,), 3: (4, 5), 4: (6,), 5: (7,), 6: (), 7: ()}
P2_GROUPS = ((0,), (1, 2), (3, 4, 5), (6, 7))
P2_X = ((4, 5), (6,), (7,), ())
STEP_BLOCKS = ((6, 7), (8, 9), (4, 5), (12, 13), (10, 11), (0, 1), (14, 15), (2, 3))
KV_COST, A_COST = 110, 56
E_COST, U_COST, T_COST, TAIL_W = 24, 90, 90, 1.6
KV_SPLIT = {2: (0, 14, 6), 3: (12, 4, 4), 4: (12, 4, 4), 5: (0, 14, 6), 6: (12, 4, 4), 7: (12, 4, 4)}
H_SPLIT = ((0, 2), (2, 4), (4, 5))
P1_TUNE = {2: (42, 0), 3: (43, 1), 4: (42, 0), 5: (42, 0), 6: (44, 0), 7: (24, 0)}
EXTRA = (42, 24)
LAST_N = 22
P2_END = (0.0, -1.0, -1.0, 0.0)
F_TIED = (20, 20, 18, 20, 20)
_ONLY = None


def _dot(a, b):
    return jnp.dot(a, b, preferred_element_type=F32)


def _cos_sin(m):
    q = (m + 256) >> 9
    x = (m - (q << 9)).astype(F32) * (2.0 * math.pi / 2048.0)
    x2 = x * x
    s = x * (1.0 + x2 * (-1.0 / 6 + x2 * (1.0 / 120 + x2 * (-1.0 / 5040 + x2 * (1.0 / 362880)))))
    c = 1.0 + x2 * (-0.5 + x2 * (1.0 / 24 + x2 * (-1.0 / 720 + x2 * (1.0 / 40320 - x2 * (1.0 / 3628800)))))
    swap = (q & 1) == 1
    c0 = jnp.where(swap, s, c)
    s0 = jnp.where(swap, c, s)
    cos = jnp.where(((q + 1) & 2) == 2, -c0, c0)
    sin = jnp.where((q & 2) == 2, -s0, s0)
    return cos, sin


def _odd_freq(r):
    return jnp.where(r < 64, 4 * r + 1, 4 * r - 253)


def _gelu_scaled(z):
    return z + z * jnp.tanh(z * (GELU_C / GA + z * z))


def _signzero(z):
    bits = jax.lax.bitcast_convert_type(z, U32) & jnp.uint32(0x80000000)
    return jax.lax.bitcast_convert_type(bits, F32)


def _ln(x, eps, tie=None, scale=None):
    n = x.shape[-1]
    cols = [x[:, j * L:(j + 1) * L] for j in range(n // L)]
    s1 = cols[0]
    s2 = cols[0] * cols[0]
    for c in cols[1:]:
        s1 = s1 + c
        s2 = s2 + c * c
    if tie is not None:
        s1 = s1 + tie
        s2 = s2 + tie
    m = jnp.sum(s1, axis=-1, keepdims=True) * (1.0 / n)
    v = jnp.maximum(jnp.sum(s2, axis=-1, keepdims=True) * (1.0 / n) - m * m, 0.0)
    rs = jax.lax.rsqrt(v + eps)
    if scale is not None:
        rs = rs * scale
    return (x - m) * rs


def _blocks_of_step(i):
    return STEP_BLOCKS[i]


class _Background:
    def __init__(self):
        self.q = []
        self.credit = 0.0

    def add(self, gen):
        self.q.append(gen)

    def run(self, budget):
        self.credit += budget
        while self.q and self.credit > 0:
            try:
                self.credit -= next(self.q[0])
            except StopIteration:
                self.q.pop(0)
        if not self.q:
            self.credit = 0.0

    def charge(self, cost):
        self.credit -= cost

    def drain(self):
        while self.q:
            self.run(1e9)


class _Tied:
    def __init__(self, tasks, npieces):
        self.tasks = list(tasks)
        self.rate = len(self.tasks) / float(npieces)
        self.credit = 0.999

    def run(self, z):
        self.credit += self.rate
        n = 0
        while self.tasks and self.credit >= 1.0:
            self.tasks.pop(0)(_signzero(z[0:16]))
            self.credit -= 1.0
            n += 1
        return n


def _kernel(q_hbm, k_hbm, v_hbm, sk_hbm, h_hbm, d_hbm, win_hbm, wsp_hbm, b_hbm, wout_hbm,
            o_hbm,
            x_us, k_us, v_us, h_us, win_us, wsp_us, wout_u, o_v, sk_in, d_in, b_in,
            xn_u, XL_u, WB_u, UL_u, WO_u, z1_v, R_u, Lc_u, zf_v, zg_v, kv_u, u_u, X_v, H_v, G_v, Z_u,
            yl_v, F_u, Fi_u, bcol_v, ph_v, sk_v, kf_v,
            sem_small, sem_x, sem_conv, sem_wsp, sem_w, sem_out):
    (wout_v, xn_v, XL_v, WB_v, UL_v, WO_v, R_v, Lc_v, kv_v, u_v, Z_v, F_v, Fi_v) = [
        r.bitcast(BF16) for r in (wout_u, xn_u, XL_u, WB_u, UL_u, WO_u, R_u, Lc_u, kv_u, u_u, Z_u, F_u, Fi_u)]
    x_vs = {g[0]: r.bitcast(BF16) for g, r in zip(X_DMAS, x_us)}
    k_vs, v_vs, h_vs = [{g[0]: r.bitcast(BF16) for g, r in zip(CONV_DMAS, rs)} for rs in (k_us, v_us, h_us)]
    wsp_vs = [r.bitcast(BF16) for r in wsp_us]
    win_vs = [r.bitcast(BF16) for r in win_us]

    def win(rows, n):
        c = [lo <= n < hi for lo, hi in WIN_CHUNKS].index(True)
        n -= WIN_CHUNKS[c][0]
        return win_vs[c][rows, n * L:(n + 1) * L]

    def locate(bufs, row):
        t0 = max(t for t in bufs if t * TM <= row)
        return bufs[t0], row - t0 * TM

    def rows_of(bufs, row, n, lanes=slice(None)):
        buf, r = locate(bufs, row)
        return buf[r:r + n, lanes]

    def cp_small():
        return [pltpu.make_async_copy(s_, d_, sem_small.at[0])
                for s_, d_ in ((d_hbm, d_in), (sk_hbm, sk_in), (b_hbm, b_in))]

    def cp_x(t):
        return pltpu.make_async_copy(q_hbm.at[0, pl.ds(t * TM, x_vs[t].shape[0])], x_vs[t], sem_x.at[t])

    def cp_conv(t):
        rows = pl.ds(t * TM, k_vs[t].shape[0])
        sem = sem_conv.at[t]
        return [pltpu.make_async_copy(h_hbm.at[:, rows], h_vs[t], sem),
                pltpu.make_async_copy(k_hbm.at[0, rows], k_vs[t], sem),
                pltpu.make_async_copy(v_hbm.at[0, rows], v_vs[t], sem)]

    def cp_wsp(i):
        return [pltpu.make_async_copy(wsp_hbm.at[pl.ds(_blocks_of_step(i)[0] * P, TM)], wsp_vs[i], sem_wsp.at[i])]

    def cp_win(c):
        lo, hi = WIN_CHUNKS[c]
        w = (hi - lo) * L
        return pltpu.make_async_copy(win_hbm.at[:, pl.ds(lo * L, w)], win_vs[c].at[:, pl.ds(0, w)], sem_w.at[c])

    def cp_wout():
        return pltpu.make_async_copy(wout_hbm, wout_v, sem_w.at[0])

    def cp_out(i):
        rows = pl.ds(_blocks_of_step(i)[0] * P, TM)
        return [pltpu.make_async_copy(o_v.at[rows], o_hbm.at[0, rows], sem_out.at[i])]

    def start(cs):
        for c in cs:
            c.start()

    def wait(cs):
        for c in cs:
            c.wait()

    def block(fn, name):
        def body(it):
            fn()
            return it + 1

        if _ONLY is None or name in _ONLY:
            jax.lax.while_loop(lambda it: it < 1, body, jnp.int32(0))

    def ln_x(t, s, tie=None):
        rows = pl.ds(t * TM + s * 16, 16)
        y = _ln(rows_of(x_vs, t * TM + s * 16, 16).astype(F32), EPS, tie, GA)
        xn_v[rows, :] = y.astype(BF16)
        return y

    def ln_x2(t, s, tie):
        p, q = s // 4, s % 4
        y1 = ln_x(t, 8 * p + q, tie)
        y2 = ln_x(t, 8 * p + 4 + q, tie)
        a11, a12, a21, a22 = y1[:, :KH], y1[:, KH:2 * KH], y2[:, :KH], y2[:, KH:2 * KH]
        r0 = (t % 4) * 5 * P + p * MC + q * 16
        for j, c in enumerate((a11 + a22, a21 + a22, a11 + a12, a21 - a11, a12 - a22)):
            XL_v[pl.ds(r0 + j * P, 16), :] = c.astype(BF16)

    def wcomb_gen(cols):
        for j in cols:
            c1 = slice(j * L, (j + 1) * L)
            for r in range(KH // 32):
                top = pl.ds(r * 32, 32)
                bot = pl.ds(KH + r * 32, 32)
                b11, b12 = win(top, j).astype(F32), win(top, 6 + j).astype(F32)
                b21, b22 = win(bot, j).astype(F32), win(bot, 6 + j).astype(F32)
                for w, c in enumerate((b11 + b22, b12 - b22, b21 - b11, b11 + b12, b21 + b22)):
                    WB_v[pl.ds(w * KH + r * 32, 32), c1] = c.astype(BF16)
                yield A_COST

    def ln_z2(t, s, tie=None):
        y = _ln(zg_v[t % 3, s * 16:(s + 1) * 16, :], 4.0 * GA * GA * EPS, tie, 0.25 / GA)
        lo, hi = y[:, :HN], y[:, HN:]
        r = (t * TM + s * 16) % HK
        rows = pl.ds(r, 16)
        if t < NT // 2:
            zf_v[rows, :] = y
            R_v[pl.ds(1 * HK + r, 16), :] = lo.astype(BF16)
            R_v[pl.ds(5 * HK + r, 16), :] = (lo + hi).astype(BF16)
        else:
            b11, b12 = zf_v[rows, :HN], zf_v[rows, HN:]
            R_v[pl.ds(0 * HK + r, 16), :] = (b11 + hi).astype(BF16)
            R_v[pl.ds(2 * HK + r, 16), :] = (b12 - hi).astype(BF16)
            R_v[pl.ds(3 * HK + r, 16), :] = (lo - b11).astype(BF16)
            R_v[pl.ds(4 * HK + r, 16), :] = hi.astype(BF16)
            R_v[pl.ds(6 * HK + r, 16), :] = (lo + hi).astype(BF16)

    def acomb_gen(i, groups=range(P // 16)):
        for r in groups:
            for c in range(HK // 256):
                top = pl.ds(r * 16, 16)
                bot = pl.ds(P + r * 16, 16)
                c1 = slice(c * 256, (c + 1) * 256)
                c2 = slice(HK + c * 256, HK + (c + 1) * 256)
                a11 = wsp_vs[i][top, c1].astype(F32)
                a12 = wsp_vs[i][top, c2].astype(F32)
                a21 = wsp_vs[i][bot, c1].astype(F32)
                a22 = wsp_vs[i][bot, c2].astype(F32)
                r0 = (i % 5) * 5 * P + r * 16
                Lc_v[pl.ds(r0 + 0 * P, 16), c1] = (a11 + a22).astype(BF16)
                Lc_v[pl.ds(r0 + 1 * P, 16), c1] = (a21 + a22).astype(BF16)
                Lc_v[pl.ds(r0 + 2 * P, 16), c1] = (a11 + a12).astype(BF16)
                Lc_v[pl.ds(r0 + 3 * P, 16), c1] = (a21 - a11).astype(BF16)
                Lc_v[pl.ds(r0 + 4 * P, 16), c1] = (a12 - a22).astype(BF16)
                yield A_COST

    def tasks(fn, t, n=TM // 16):
        return [lambda tie, s=s: fn(t, s, tie) for s in range(n)]

    def kv_gen(t):
        for m in range(TM // MC):
            r = t * TM + m * MC
            for l in range(D // L):
                lanes = slice(l * L, (l + 1) * L)
                kf = rows_of(k_vs, r, MC, lanes).astype(F32)
                kf_v[l, pl.ds(r + 8, MC), :] = kf
                ks = kf * sk_v[0, 0:1, lanes]
                for tap in range(1, 4):
                    ks = ks + kf_v[l, pl.ds(r + 8 - tap, MC), :] * sk_v[tap, 0:1, lanes]
                kv = ks * rows_of(v_vs, r, MC, lanes).astype(F32)
                kv_v[pl.ds(r, MC), lanes] = kv.astype(BF16)
                yield KV_COST

    def freq_gen(a):
        def cmac(acc, x, g):
            pr = x[0] * g[0] - x[1] * g[1]
            pi = x[0] * g[1] + x[1] * g[0]
            return (pr, pi) if acc is None else (acc[0] + pr, acc[1] + pi)

        for r in range(P // 16):
            rows = pl.ds(r * 16, 16)
            for l in range(D // L):
                lanes = slice(l * L, (l + 1) * L)
                lo = hi = None
                g = (G_v[a + 1, 0, rows, lanes], G_v[a + 1, 1, rows, lanes])
                for c in range(a + 2):
                    x = (X_v[c, 0, rows, lanes], X_v[c, 1, rows, lanes])
                    hi = cmac(hi, x, g)
                    if c <= a:
                        g = (G_v[a - c, 0, rows, lanes], G_v[a - c, 1, rows, lanes])
                        lo = cmac(lo, x, g)
                        yield 32
                for w, z in enumerate((lo, hi)):
                    for part in range(2):
                        Z_v[pl.ds((a + w) * 2 * P + part * P + r * 16, 16), lanes] = z[part].astype(BF16)
                yield 20

    def job_x(t, bg, budget):
        for j in (2 * t, 2 * t + 1):
            for half in range(2):
                r = _dot(F_v[half * P:(half + 1) * P, 0:P], kv_v[j * P:(j + 1) * P, :]).reshape(8, 2, 8, D)
                for part in range(2):
                    X_v[j, part, half * 64:(half + 1) * 64, :] = r[:, part].reshape(64, D)
                bg.run(budget * 2.5)

    def job_h(t, bg, budget):
        h_v, c0 = locate(h_vs, t * TM)
        for half in range(2):
            rows = pl.ds(half * 64, 64)
            for l0, l1 in H_SPLIT:
                w = (l1 - l0) * L
                lanes = slice(l0 * L, l1 * L)
                rhs = jnp.concatenate([h_v[lanes, c0:c0 + P], h_v[lanes, c0 + P:c0 + TM]], axis=0)
                r = jax.lax.dot_general(F_v[half * P:(half + 1) * P, 0:P], rhs, NT_DIMS,
                                        preferred_element_type=F32).reshape(8, 2, 8, 2 * w)
                re, im = r[:, 0].reshape(64, 2 * w), r[:, 1].reshape(64, 2 * w)
                prev = (H_v[t % 2, 0, rows, lanes], H_v[t % 2, 1, rows, lanes])
                for j in range(2):
                    cur = (re[:, j * w:(j + 1) * w], im[:, j * w:(j + 1) * w])
                    G_v[2 * t + j, 0, rows, lanes] = cur[0] + prev[1] if half else cur[0] - prev[1]
                    G_v[2 * t + j, 1, rows, lanes] = cur[1] - prev[0] if half else cur[1] + prev[0]
                    prev = cur
                if t + 1 < NT:
                    H_v[(t + 1) % 2, 0, rows, lanes] = prev[0]
                    H_v[(t + 1) % 2, 1, rows, lanes] = prev[1]
                bg.run(budget * (l1 - l0))

    def z_out(t, m, n, pre, bg, budget, tied):
        z = _gelu_scaled(pre)
        if n < FH // L:
            z1_v[pl.ds(t * TM + m * MC, MC), n * L:(n + 1) * L] = z
        else:
            zg_v[t % 3, m * MC:(m + 1) * MC, n * L - FH:(n + 1) * L - FH] = z
        ntask = tied.run(z)
        bg.run(budget[1] if ntask else budget[0])

    def job_z(t, m, cols, bg, budget, tied):
        for n in cols:
            z_out(t, m, n, _dot(xn_v[pl.ds(t * TM + m * MC, MC), :], win(slice(None), n)), bg, budget, tied)

    def job_zs(t, p, j, bg, budget, tied):
        r1 = pl.ds(t * TM + p * P, MC)
        r2 = pl.ds(t * TM + p * P + MC, MC)
        c1 = slice(j * L, (j + 1) * L)

        def xl(w):
            r0 = (t % 4) * 5 * P + w * P + p * MC
            return XL_v[r0:r0 + MC, :]

        def wb(w):
            return WB_v[w * KH:(w + 1) * KH, c1]

        def rem(rows, n):
            return _dot(xn_v[rows, 2 * KH:], win(slice(2 * KH, D), n))

        m2 = _dot(xl(1), win(slice(0, KH), j))
        m4 = _dot(xn_v[r2, KH:2 * KH], wb(2))
        z_out(t, 2 * p + 1, j, m2 + m4 + rem(r2, j), bg, budget, tied)
        m3 = _dot(xn_v[r1, 0:KH], wb(1))
        m5 = _dot(xl(2), win(slice(KH, 2 * KH), 6 + j))
        z_out(t, 2 * p, 6 + j, m3 + m5 + rem(r1, 6 + j), bg, budget, tied)
        t11, t22 = m4 - m5, m3 - m2
        m1 = _dot(xl(0), wb(0))
        t11, t22 = t11 + m1, t22 + m1
        z_out(t, 2 * p, j, t11 + _dot(xl(4), wb(4)) + rem(r1, j), bg, budget, tied)
        z_out(t, 2 * p + 1, 6 + j, t22 + _dot(xl(3), wb(3)) + rem(r2, 6 + j), bg, budget, tied)

    rev8 = 7 - jax.lax.broadcasted_iota(jnp.int32, (8, L), 0)

    def finish(a, upper, n, hh, slot):
        rows = pl.ds(a * P + (MC if upper else 0), MC)
        lanes = slice(n * L, (n + 1) * L)
        if upper:
            ya = _dot(Fi_v[:, 0:P], Z_v[a * 2 * P:a * 2 * P + P, lanes])
            yb = _dot(Fi_v[:, P:2 * P], Z_v[a * 2 * P + P:(a + 1) * 2 * P, lanes])
            slot(0.5)
            y = ya - yb
            lo = ya + yb
            for j in range(MC // 8):
                yl_v[a % 2, n, (7 - j) * 8:(8 - j) * 8, :] = jnp.take_along_axis(lo[j * 8:(j + 1) * 8], rev8, axis=0)
        else:
            y = yl_v[a % 2, n]
        gate = hh + hh * jnp.tanh(hh)
        s = xn_v[rows, lanes].astype(F32) * y
        x = rows_of(x_vs, a * P + (MC if upper else 0), MC, lanes).astype(F32)
        o_v[rows, lanes] = (x + s * gate).astype(BF16)

    def tail_gen(i, bg, budget):
        a0, a1 = _blocks_of_step(i)

        def slot(w):
            bg.run(w * budget[0])

        def dot3(a, b):
            r = _dot(a, b)
            slot(0.75)
            return r

        for upper in (True, False):
            sub = MC if upper else 0
            r1 = pl.ds(a0 * P + sub, MC)
            r2 = pl.ds(a1 * P + sub, MC)

            def ul(w):
                r0 = ((i % 5) * 5 + w) * P + sub
                return UL_v[r0:r0 + MC, :]

            for j in range(2):
                c1 = slice(j * L, (j + 1) * L)
                c2 = slice((2 + j) * L, (3 + j) * L)

                def wo(w):
                    return WO_v[w * HN:(w + 1) * HN, c1]

                m2 = dot3(ul(1), wout_v[0:HN, c1])
                m4 = dot3(u_v[r2, HN:], wo(2))
                finish(a1, upper, j, m2 + m4, slot)
                bg.charge(T_COST)
                yield
                m3 = dot3(u_v[r1, 0:HN], wo(1))
                m5 = dot3(ul(2), wout_v[HN:, c2])
                finish(a0, upper, 2 + j, m3 + m5, slot)
                bg.charge(T_COST)
                yield
                m1 = dot3(ul(0), wo(0))
                finish(a0, upper, j, (m4 - m5) + m1 + dot3(ul(4), wo(4)), slot)
                bg.charge(T_COST)
                yield
                finish(a1, upper, 2 + j, (m3 - m2) + m1 + dot3(ul(3), wo(3)), slot)
                bg.charge(T_COST)
                yield
            for a, r in ((a0, r1), (a1, r2)):
                finish(a, upper, 4, dot3(u_v[r, 0:HN], wout_v[0:HN, 4 * L:]) + dot3(u_v[r, HN:], wout_v[HN:, 4 * L:]),
                       slot)
                bg.charge(T_COST)
                yield

    def wocomb_gen():
        for j in range(2):
            c1 = slice(j * L, (j + 1) * L)
            c2 = slice((2 + j) * L, (3 + j) * L)
            for r in range(HN // 32):
                top = pl.ds(r * 32, 32)
                bot = pl.ds(HN + r * 32, 32)
                b11, b12 = wout_v[top, c1].astype(F32), wout_v[top, c2].astype(F32)
                b21, b22 = wout_v[bot, c1].astype(F32), wout_v[bot, c2].astype(F32)
                for w, c in enumerate((b11 + b22, b12 - b22, b21 - b11, b11 + b12, b21 + b22)):
                    WO_v[pl.ds(w * HN + r * 32, 32), c1] = c.astype(BF16)
                yield A_COST

    def job_big(i, bg, pending, budget, every):
        a0, a1 = _blocks_of_step(i)
        KG = 512

        def lhs(j, sub, cols):
            if j == 2:
                return wsp_vs[i][sub:sub + MC, cols]
            if j == 3:
                return wsp_vs[i][P + sub:P + sub + MC, HK + cols.start:HK + cols.stop]
            r0 = ((i % 5) * 5 + {0: 0, 1: 1, 4: 2, 5: 3, 6: 4}[j]) * P + sub
            return Lc_v[r0:r0 + MC, cols]

        def prod(j, sub, n, acc=None):
            for kg in range(HK // KG):
                ks = slice(kg * KG, (kg + 1) * KG)
                p = _dot(lhs(j, sub, ks), R_v[j * HK + kg * KG:j * HK + (kg + 1) * KG, n * L:(n + 1) * L])
                acc = p if acc is None else acc + p
                bg.run(budget)
            return acc

        def tails(n):
            for _ in range(n):
                if pending:
                    next(pending.pop(0))

        def emit(a, sub, n, g):
            rows = pl.ds(a * P + sub, MC)
            lanes = slice(n * L, (n + 1) * L)
            u = z1_v[rows, lanes] * (g + bcol_v[rows, :])
            u_v[rows, lanes] = u.astype(BF16)
            bg.charge(E_COST)
            return u

        for sub in (0, MC):
            for n in range(HN // L):
                def put(w, c):
                    UL_v[pl.ds(((i % 5) * 5 + w) * P + sub, MC), n * L:(n + 1) * L] = c.astype(BF16)

                m1 = prod(0, sub, n)
                t11 = prod(6, sub, n, m1)
                m4 = prod(3, sub, n)
                t11 = t11 + m4
                m5 = prod(4, sub, n)
                u11 = emit(a0, sub, n, t11 - m5)
                m2 = prod(1, sub, n)
                u21 = emit(a1, sub, n, m2 + m4)
                put(3, u21 - u11)
                t22 = m1 - m2
                m3 = prod(2, sub, n)
                u12 = emit(a0, sub, n + HN // L, m3 + m5)
                put(2, u11 + u12)
                u22 = emit(a1, sub, n + HN // L, prod(5, sub, n, t22 + m3))
                put(0, u11 + u22)
                put(1, u21 + u22)
                put(4, u12 - u22)
                bg.charge(U_COST)
                tails(every.pop(0))

    def debug_keep_alive():
        if _ONLY is not None:
            for r_ in (xn_u, XL_u, WB_u, UL_u, WO_u, z1_v, R_u, Lc_u, zf_v, zg_v, kv_u, u_u, X_v, H_v, G_v, Z_u,
                       kf_v, bcol_v):
                c_ = pltpu.make_async_copy(r_, r_, sem_small.at[0])
                c_.start()
                c_.wait()

    debug_keep_alive()

    cp_x(0).start()
    cp_win(0).start()
    cp_x(1).start()
    cp_win(1).start()
    start(cp_small())
    for c in range(2, 5):
        cp_win(c).start()
    cp_x(2).start()

    kk = _odd_freq(jax.lax.broadcasted_iota(jnp.int32, (P, P), 0))
    nn = jax.lax.broadcasted_iota(jnp.int32, (P, P), 1)
    fc, fs = _cos_sin((kk * (4 * nn - 127)) & 2047)
    for g in range(P // 8):
        F_v[g * 16:(g + 1) * 16, 0:P] = jnp.concatenate(
            [fc[g * 8:(g + 1) * 8], -fs[g * 8:(g + 1) * 8]], axis=0).astype(BF16)
    fc, fs = _cos_sin((kk * (-127)) & 2047)
    ph_v[0] = fc
    ph_v[1] = fs
    kk = _odd_freq(jax.lax.broadcasted_iota(jnp.int32, (MC, P), 1))
    mm = jax.lax.broadcasted_iota(jnp.int32, (MC, P), 0)
    ic, is_ = _cos_sin((kk * (4 * mm + 2)) & 2047)
    Fi_v[:, 0:P] = (ic * (1.0 / (P * GA))).astype(BF16)
    Fi_v[:, P:2 * P] = (is_ * (1.0 / (P * GA))).astype(BF16)
    kf_v[:, 0:8, :] = jnp.zeros((D // L, 8, L), F32)

    cp_x(0).wait()
    for s in range(TM // 16):
        ln_x(0, s)

    def small_setup():
        sk = sk_in[...].astype(F32)
        for t in range(4):
            sk_v[t] = jnp.broadcast_to(sk[t:t + 1], (8, D))
        drow = d_in[...].astype(F32).reshape(1, D)
        for l in range(D // L):
            lanes = slice(l * L, (l + 1) * L)
            dre = ph_v[0] * drow[:, lanes]
            dim = ph_v[1] * drow[:, lanes]
            H_v[0, 0, 0:64, lanes] = -dim[0:64]
            H_v[0, 0, 64:P, lanes] = dim[64:P]
            H_v[0, 1, 0:64, lanes] = -dre[0:64]
            H_v[0, 1, 64:P, lanes] = dre[64:P]

    def bcol_task(t, j, tie):
        brow = b_in[...].astype(F32).reshape(1, S)[:, j * P:(j + 1) * P] * (0.25 / GA) + tie[0:1]
        bcol_v[j * P:(j + 1) * P, :] = jnp.broadcast_to(brow, (P, P)).T

    LAG = 2

    def interleave(*lists):
        out = []
        for j in range(max(len(a) for a in lists)):
            for a in lists:
                out += a[j:j + 1]
        return out

    def p1_first(c):
        bg = _Background()
        todo = []
        if c == 2:
            todo = tasks(bcol_task, 0)
            small_setup()
        if c == 3:
            todo = tasks(ln_z2, 0)
            bg.add(wcomb_gen(range(3)))
        if c == 4:
            todo = tasks(ln_x2, 2, 8)
            bg.add(wcomb_gen(range(3, 6)))
        tied = _Tied(todo, F_TIED[c])
        if c == 0:
            for s in range(TM // 16):
                ln_x(1, s)
        for t in range(2):
            for m in range(TM // MC):
                job_z(t, m, range(*WIN_CHUNKS[c]), bg, (80, 40), tied)
        bg.drain()
        assert not tied.tasks

    for c in range(5):
        cp_win(c).wait()
        if c == 0:
            cp_x(1).wait()
        if c == 2:
            wait(cp_small())
            start(cp_conv(0))
            cp_x(3).start()
        if c == 4:
            cp_x(2).wait()
            cp_x(4).start()
        block(lambda c=c: p1_first(c), f'p1_f{c}')

    def p1_wait(g):
        if g == 0:
            wait(cp_conv(0))
            cp_x(3).wait()
        if g == 1:
            wait(cp_conv(1))
            cp_x(4).wait()
        if g == 2:
            wait(cp_conv(2))
            cp_x(6).wait()
        if g == 3:
            wait(cp_conv(4))
            cp_wout().wait()
            wait(cp_wsp(0))

    def p1_start(g):
        if g == 0:
            start(cp_conv(1))
            cp_x(6).start()
            start(cp_conv(2))
        if g == 1:
            start(cp_conv(4))
            cp_wout().start()
            start(cp_wsp(0))
            start(cp_wsp(1))
        if g == 3:
            start(cp_wsp(2))
            start(cp_conv(6))
            for i in (3, 4, 5):
                start(cp_wsp(i))

    def take(gen, n):
        for _ in range(n):
            yield next(gen)

    def p1_step(i):
        bg = _Background()
        dft = _Background()
        t = i - LAG
        xg = P1_X[i]
        kv = kv_gen(t)
        nx, nz, nh = KV_SPLIT[i]
        dft.add(take(kv, nx))
        bg.add(take(kv, nz))
        hbg = _Background()
        hbg.add(take(kv, nh))
        zb = nz * KV_COST / 48.0
        extra = 0
        if i == 6:
            bg.add(wocomb_gen())
            bg.add(acomb_gen(0, range(3)))
            extra = EXTRA[0]
        if i == 7:
            bg.add(acomb_gen(0, range(3, 8)))
            extra = EXTRA[1]
        last = i == NT - 1
        z2t = tasks(ln_z2, i - 1)
        xt = [tasks(ln_x2, t_, 8) for t_ in P1_LNX[i]]
        if P1_TUNE[i][1]:
            todo = interleave(*([z2t[0::2]] + xt + [z2t[1::2]]))
        else:
            todo = interleave(*(xt + [z2t[0::2], z2t[1::2]]))
        tied = _Tied(todo, P1_TUNE[i][0])
        if xg is not None:
            dft.run(KV_COST)
            job_x(xg, dft, (nx - 1) * KV_COST / 10.0)
            dft.drain()
        for p in range(2):
            for j in range(FH // L):
                job_zs(i, p, j, bg, (1.6 * zb + extra, 0.5 * zb + extra), tied)
            assert not tied.tasks or (p == 0 and not last)
            if p == 0 and last:
                tied = _Tied(tasks(ln_z2, i, 8), LAST_N)
        if last:
            for s in range(8, 16):
                ln_z2(i, s)
        bg.drain()
        job_h(t, hbg, nh * KV_COST / 10.0)
        hbg.drain()

    def p1_block(g):
        for i in P1_GROUPS[g]:
            p1_step(i)

    for g in range(len(P1_GROUPS)):
        p1_wait(g)
        p1_start(g)
        block(lambda g=g: p1_block(g), f'p1_g{g}')

    groups = P2_GROUPS
    NG = len(groups)

    def p2_dma(gi):
        if gi >= 2:
            for i in groups[gi - 2]:
                start(cp_out(i))
        if gi >= 3:
            for i in groups[gi - 3]:
                wait(cp_out(i))
        if gi == 1:
            for i in (6, 7):
                start(cp_wsp(i))
        if gi == 0:
            wait(cp_conv(6))
        if gi + 1 < NG:
            for i in groups[gi + 1]:
                wait(cp_wsp(i))

    def tails_of(i, bg, budget):
        return [tail_gen(i, bg, budget)] * 20

    def p2_block(gi):
        bg = _Background()
        steps = groups[gi]
        tb = [0.0]
        pending = [t_ for i in (groups[gi - 1] if gi > 0 else []) for t_ in tails_of(i, bg, tb)]
        total = sum(a + 1 for i in steps for a in _blocks_of_step(i)) * 40 * 16
        total += len(steps) * (24 * E_COST + 6 * U_COST) + len(pending) * T_COST
        slots = 84 * len(steps) + TAIL_W * len(pending)
        bg.add(freq_gen(_blocks_of_step(steps[0])[0]))
        if gi < 2:
            bg.add(kv_gen(NT - 2 + gi))
            total += 20 * KV_COST
            slots += 10
        for t in P2_X[gi]:
            slots += 10
        if gi + 1 < NG:
            for i in groups[gi + 1]:
                bg.add(acomb_gen(i))
                total += 32 * A_COST
        for i in steps[1:]:
            bg.add(freq_gen(_blocks_of_step(i)[0]))
        budget = tb[0] = total / (slots + P2_END[gi])
        bg.run(budget)
        for t in P2_X[gi]:
            job_x(t, bg, budget)
        if gi < 2:
            job_h(NT - 2 + gi, bg, budget)
        units = [4, 4, 2, 4, 4, 2] * (len(pending) // 20)
        every = [0] * (6 * len(steps))
        for j, n in enumerate(units):
            every[min(len(every) - 1, j * len(every) // len(units))] += n
        for i in steps:
            job_big(i, bg, pending, budget, every)
        for t_ in pending:
            next(t_)
        bg.drain()

    for gi in range(NG):
        p2_dma(gi)
        block(lambda gi=gi: p2_block(gi), f'p2_{gi}')

    def cp_last(part):
        a0 = _blocks_of_step(NT - 1)[0]
        sub, cols = ((MC, pl.ds(0, D)), (0, pl.ds(0, 4 * L)), (0, pl.ds(4 * L, L)))[part]
        return [pltpu.make_async_copy(o_v.at[pl.ds(r, MC), cols], o_hbm.at[0, pl.ds(r, MC), cols],
                                      sem_out.at[NT - 1]) for r in (a0 * P + sub, (a0 + 1) * P + sub)]

    def p2_last():
        for i in groups[NG - 1]:
            for j, t_ in enumerate(tails_of(i, _Background(), [0.0])):
                next(t_)
                if i < NT - 1 and j == 19:
                    start(cp_out(i))
                if i == NT - 1 and j in (9, 17):
                    start(cp_last(j // 10))

    p2_dma(NG)
    block(p2_last, 'p2_last')
    start(cp_last(2))
    for i in groups[NG - 2] + groups[NG - 1][:-1]:
        wait(cp_out(i))
    for part in range(3):
        wait(cp_last(part))
    debug_keep_alive()


@jax.jit
def pallas_recurrent_scan__ssm_conv_h3__mixer_gmlp__prompt_kernel(
    A_q: jax.Array,
    A_k: jax.Array,
    A_v: jax.Array,
    A_shift_k: jax.Array,
    A_ssm_k: jax.Array,
    A_ssm_D: jax.Array,
    B_x: jax.Array,
    B_w_in: jax.Array,
    B_w_sp: jax.Array,
    B_b_sp: jax.Array,
    B_w_out: jax.Array,
):
    del B_x
    hbm = pl.BlockSpec(memory_space=pl.ANY)

    def bf16_buf(*shape):
        return pltpu.VMEM(shape[:-2] + (shape[-2] // 2, shape[-1]), U32)

    return pl.pallas_call(
        _kernel,
        out_shape=jax.ShapeDtypeStruct((1, S, D), BF16),
        in_specs=[hbm] * 10,
        out_specs=hbm,
        scratch_shapes=[
            [bf16_buf(len(g) * TM, D) for g in X_DMAS],
            [bf16_buf(len(g) * TM, D) for g in CONV_DMAS],
            [bf16_buf(len(g) * TM, D) for g in CONV_DMAS],
            [bf16_buf(D, len(g) * TM) for g in CONV_DMAS],
            [bf16_buf(D, max(hi - lo, 2) * L) for lo, hi in WIN_CHUNKS],
            [bf16_buf(TM, S) for _ in range(NT)],
            bf16_buf(FH, D),
            pltpu.VMEM((S, D), BF16),
            pltpu.VMEM((4, D), BF16),
            pltpu.VMEM((D,), BF16),
            pltpu.VMEM((S,), BF16),
            bf16_buf(S, D),
            bf16_buf(4 * 5 * P, KH),
            bf16_buf(5 * KH, FH),
            bf16_buf(5 * 5 * P, HN),
            bf16_buf(5 * HN, 2 * L),
            pltpu.VMEM((S, FH), F32),
            bf16_buf(7 * HK, HN),
            bf16_buf(5 * 5 * P, HK),
            pltpu.VMEM((HK, FH), F32),
            pltpu.VMEM((3, TM, FH), F32),
            bf16_buf(S, D),
            bf16_buf(S, FH),
            pltpu.VMEM((NB, 2, P, D), F32),
            pltpu.VMEM((2, 2, P, D), F32),
            pltpu.VMEM((NB, 2, P, D), F32),
            bf16_buf(NB * 2 * P, D),
            pltpu.VMEM((2, D // L, MC, L), F32),
            bf16_buf(2 * P, 2 * P),
            bf16_buf(MC, 2 * P),
            pltpu.VMEM((S, L), F32),
            pltpu.VMEM((2, P, L), F32),
            pltpu.VMEM((4, 8, D), F32),
            pltpu.VMEM((D // L, S + 8, L), F32),
            pltpu.SemaphoreType.DMA((1,)),
            pltpu.SemaphoreType.DMA((NT,)),
            pltpu.SemaphoreType.DMA((NT,)),
            pltpu.SemaphoreType.DMA((NT,)),
            pltpu.SemaphoreType.DMA((5,)),
            pltpu.SemaphoreType.DMA((NT,)),
        ],
        compiler_params=pltpu.CompilerParams(vmem_limit_bytes=116 * 1024 * 1024, disable_semaphore_checks=True),
    )(A_q, A_k, A_v, A_shift_k.T, A_ssm_k, A_ssm_D, B_w_in, B_w_sp, B_b_sp, B_w_out)
```

```python
import math

import jax
import jax.numpy as jnp
import jax.experimental.pallas as pl
import jax.experimental.pallas.tpu as pltpu

S = 2048
D = 640
FH = 768
P = 128
NB = S // P
TM = 256
NT = S // TM
MC = 64
L = 128
HK = S // 2
KH = 256
HN = FH // 2
EPS = 1e-5
F32 = jnp.float32
BF16 = jnp.bfloat16
U32 = jnp.uint32
GELU_C = math.sqrt(2.0 / math.pi)
GA = (GELU_C * 0.044715) ** (1.0 / 3.0)
NT_DIMS = (((1,), (1,)), ((), ()))

WIN_CHUNKS = ((6, 7), (7, 9), (9, 12), (0, 3), (3, 6))
X_DMAS = ((0,), (1,), (2,), (3,), (4, 5), (6, 7))
CONV_DMAS = ((0,), (1,), (2, 3), (4, 5), (6, 7))
P1_GROUPS = ((2,), (3,), (4, 5), (6, 7))
P1_X = {2: None, 3: 0, 4: 1, 5: None, 6: 2, 7: 3}
P1_LNX = {2: (3,), 3: (4, 5), 4: (6,), 5: (7,), 6: (), 7: ()}
P2_GROUPS = ((0,), (1, 2), (3, 4, 5), (6, 7))
P2_X = ((4, 5), (6,), (7,), ())
STEP_BLOCKS = ((6, 7), (8, 9), (4, 5), (12, 13), (10, 11), (0, 1), (14, 15), (2, 3))
KV_COST, A_COST = 110, 56
E_COST, U_COST, T_COST, TAIL_W = 24, 90, 90, 1.6
KV_SPLIT = {2: (0, 14, 6), 3: (12, 4, 4), 4: (12, 4, 4), 5: (0, 14, 6), 6: (12, 4, 4), 7: (12, 4, 4)}
H_SPLIT = ((0, 2), (2, 4), (4, 5))
P1_TUNE = {2: (42, 0), 3: (43, 1), 4: (42, 0), 5: (42, 0), 6: (44, 0), 7: (24, 0)}
EXTRA = (42, 24)
LAST_N = 22
P2_END = (0.0, -1.0, -1.0, 0.0)
F_TIED = (20, 20, 18, 20, 20)
_ONLY = None


def _dot(a, b):
    return jnp.dot(a, b, preferred_element_type=F32)


def _cos_sin(m):
    q = (m + 256) >> 9
    x = (m - (q << 9)).astype(F32) * (2.0 * math.pi / 2048.0)
    x2 = x * x
    s = x * (1.0 + x2 * (-1.0 / 6 + x2 * (1.0 / 120 + x2 * (-1.0 / 5040 + x2 * (1.0 / 362880)))))
    c = 1.0 + x2 * (-0.5 + x2 * (1.0 / 24 + x2 * (-1.0 / 720 + x2 * (1.0 / 40320 - x2 * (1.0 / 3628800)))))
    swap = (q & 1) == 1
    c0 = jnp.where(swap, s, c)
    s0 = jnp.where(swap, c, s)
    cos = jnp.where(((q + 1) & 2) == 2, -c0, c0)
    sin = jnp.where((q & 2) == 2, -s0, s0)
    return cos, sin


def _odd_freq(r):
    return jnp.where(r < 64, 4 * r + 1, 4 * r - 253)


def _gelu_scaled(z):
    return z + z * jnp.tanh(z * (GELU_C / GA + z * z))


def _signzero(z):
    bits = jax.lax.bitcast_convert_type(z, U32) & jnp.uint32(0x80000000)
    return jax.lax.bitcast_convert_type(bits, F32)


def _ln(x, eps, tie=None, scale=None):
    n = x.shape[-1]
    cols = [x[:, j * L:(j + 1) * L] for j in range(n // L)]
    s1 = cols[0]
    s2 = cols[0] * cols[0]
    for c in cols[1:]:
        s1 = s1 + c
        s2 = s2 + c * c
    if tie is not None:
        s1 = s1 + tie
        s2 = s2 + tie
    m = jnp.sum(s1, axis=-1, keepdims=True) * (1.0 / n)
    v = jnp.maximum(jnp.sum(s2, axis=-1, keepdims=True) * (1.0 / n) - m * m, 0.0)
    rs = jax.lax.rsqrt(v + eps)
    if scale is not None:
        rs = rs * scale
    return (x - m) * rs


def _blocks_of_step(i):
    return STEP_BLOCKS[i]


class _Background:
    def __init__(self):
        self.q = []
        self.credit = 0.0

    def add(self, gen):
        self.q.append(gen)

    def run(self, budget):
        self.credit += budget
        while self.q and self.credit > 0:
            try:
                self.credit -= next(self.q[0])
            except StopIteration:
                self.q.pop(0)
        if not self.q:
            self.credit = 0.0

    def charge(self, cost):
        self.credit -= cost

    def drain(self):
        while self.q:
            self.run(1e9)


class _Tied:
    def __init__(self, tasks, npieces):
        self.tasks = list(tasks)
        self.rate = len(self.tasks) / float(npieces)
        self.credit = 0.999

    def run(self, z):
        self.credit += self.rate
        n = 0
        while self.tasks and self.credit >= 1.0:
            self.tasks.pop(0)(_signzero(z[0:16]))
            self.credit -= 1.0
            n += 1
        return n


def _kernel(q_hbm, k_hbm, v_hbm, sk_hbm, h_hbm, d_hbm, win_hbm, wsp_hbm, b_hbm, wout_hbm,
            o_hbm,
            x_us, k_us, v_us, h_us, win_us, wsp_us, wout_u, o_v, sk_in, d_in, b_in,
            xn_u, XL_u, WB_u, UL_u, WO_u, z1_v, R_u, Lc_u, zf_v, zg_v, kv_u, u_u, X_v, H_v, G_v, Z_u,
            yl_v, F_u, Fi_u, bcol_v, ph_v, sk_v, kf_v,
            sem_small, sem_x, sem_conv, sem_wsp, sem_w, sem_out):
    (wout_v, xn_v, XL_v, WB_v, UL_v, WO_v, R_v, Lc_v, kv_v, u_v, Z_v, F_v, Fi_v) = [
        r.bitcast(BF16) for r in (wout_u, xn_u, XL_u, WB_u, UL_u, WO_u, R_u, Lc_u, kv_u, u_u, Z_u, F_u, Fi_u)]
    x_vs = {g[0]: r.bitcast(BF16) for g, r in zip(X_DMAS, x_us)}
    k_vs, v_vs, h_vs = [{g[0]: r.bitcast(BF16) for g, r in zip(CONV_DMAS, rs)} for rs in (k_us, v_us, h_us)]
    wsp_vs = [r.bitcast(BF16) for r in wsp_us]
    win_vs = [r.bitcast(BF16) for r in win_us]

    def win(rows, n):
        c = [lo <= n < hi for lo, hi in WIN_CHUNKS].index(True)
        n -= WIN_CHUNKS[c][0]
        return win_vs[c][rows, n * L:(n + 1) * L]

    def locate(bufs, row):
        t0 = max(t for t in bufs if t * TM <= row)
        return bufs[t0], row - t0 * TM

    def rows_of(bufs, row, n, lanes=slice(None)):
        buf, r = locate(bufs, row)
        return buf[r:r + n, lanes]

    def cp_small():
        return [pltpu.make_async_copy(s_, d_, sem_small.at[0])
                for s_, d_ in ((d_hbm, d_in), (sk_hbm, sk_in), (b_hbm, b_in))]

    def cp_x(t):
        return pltpu.make_async_copy(q_hbm.at[0, pl.ds(t * TM, x_vs[t].shape[0])], x_vs[t], sem_x.at[t])

    def cp_conv(t):
        rows = pl.ds(t * TM, k_vs[t].shape[0])
        sem = sem_conv.at[t]
        return [pltpu.make_async_copy(h_hbm.at[:, rows], h_vs[t], sem),
                pltpu.make_async_copy(k_hbm.at[0, rows], k_vs[t], sem),
                pltpu.make_async_copy(v_hbm.at[0, rows], v_vs[t], sem)]

    def cp_wsp(i):
        return [pltpu.make_async_copy(wsp_hbm.at[pl.ds(_blocks_of_step(i)[0] * P, TM)], wsp_vs[i], sem_wsp.at[i])]

    def cp_win(c):
        lo, hi = WIN_CHUNKS[c]
        w = (hi - lo) * L
        return pltpu.make_async_copy(win_hbm.at[:, pl.ds(lo * L, w)], win_vs[c].at[:, pl.ds(0, w)], sem_w.at[c])

    def cp_wout():
        return pltpu.make_async_copy(wout_hbm, wout_v, sem_w.at[0])

    def cp_out(i):
        rows = pl.ds(_blocks_of_step(i)[0] * P, TM)
        return [pltpu.make_async_copy(o_v.at[rows], o_hbm.at[0, rows], sem_out.at[i])]

    def start(cs):
        for c in cs:
            c.start()

    def wait(cs):
        for c in cs:
            c.wait()

    def block(fn, name):
        def body(it):
            fn()
            return it + 1

        if _ONLY is None or name in _ONLY:
            jax.lax.while_loop(lambda it: it < 1, body, jnp.int32(0))

    def ln_x(t, s, tie=None):
        rows = pl.ds(t * TM + s * 16, 16)
        y = _ln(rows_of(x_vs, t * TM + s * 16, 16).astype(F32), EPS, tie, GA)
        xn_v[rows, :] = y.astype(BF16)
        return y

    def ln_x2(t, s, tie):
        p, q = s // 4, s % 4
        y1 = ln_x(t, 8 * p + q, tie)
        y2 = ln_x(t, 8 * p + 4 + q, tie)
        a11, a12, a21, a22 = y1[:, :KH], y1[:, KH:2 * KH], y2[:, :KH], y2[:, KH:2 * KH]
        r0 = (t % 4) * 5 * P + p * MC + q * 16
        for j, c in enumerate((a11 + a22, a21 + a22, a11 + a12, a21 - a11, a12 - a22)):
            XL_v[pl.ds(r0 + j * P, 16), :] = c.astype(BF16)

    def wcomb_gen(cols):
        for j in cols:
            c1 = slice(j * L, (j + 1) * L)
            for r in range(KH // 32):
                top = pl.ds(r * 32, 32)
                bot = pl.ds(KH + r * 32, 32)
                b11, b12 = win(top, j).astype(F32), win(top, 6 + j).astype(F32)
                b21, b22 = win(bot, j).astype(F32), win(bot, 6 + j).astype(F32)
                for w, c in enumerate((b11 + b22, b12 - b22, b21 - b11, b11 + b12, b21 + b22)):
                    WB_v[pl.ds(w * KH + r * 32, 32), c1] = c.astype(BF16)
                yield A_COST

    def ln_z2(t, s, tie=None):
        y = _ln(zg_v[t % 3, s * 16:(s + 1) * 16, :], 4.0 * GA * GA * EPS, tie, 0.25 / GA)
        lo, hi = y[:, :HN], y[:, HN:]
        r = (t * TM + s * 16) % HK
        rows = pl.ds(r, 16)
        if t < NT // 2:
            zf_v[rows, :] = y
            R_v[pl.ds(1 * HK + r, 16), :] = lo.astype(BF16)
            R_v[pl.ds(5 * HK + r, 16), :] = (lo + hi).astype(BF16)
        else:
            b11, b12 = zf_v[rows, :HN], zf_v[rows, HN:]
            R_v[pl.ds(0 * HK + r, 16), :] = (b11 + hi).astype(BF16)
            R_v[pl.ds(2 * HK + r, 16), :] = (b12 - hi).astype(BF16)
            R_v[pl.ds(3 * HK + r, 16), :] = (lo - b11).astype(BF16)
            R_v[pl.ds(4 * HK + r, 16), :] = hi.astype(BF16)
            R_v[pl.ds(6 * HK + r, 16), :] = (lo + hi).astype(BF16)

    def acomb_gen(i, groups=range(P // 16)):
        for r in groups:
            for c in range(HK // 256):
                top = pl.ds(r * 16, 16)
                bot = pl.ds(P + r * 16, 16)
                c1 = slice(c * 256, (c + 1) * 256)
                c2 = slice(HK + c * 256, HK + (c + 1) * 256)
                a11 = wsp_vs[i][top, c1].astype(F32)
                a12 = wsp_vs[i][top, c2].astype(F32)
                a21 = wsp_vs[i][bot, c1].astype(F32)
                a22 = wsp_vs[i][bot, c2].astype(F32)
                r0 = (i % 5) * 5 * P + r * 16
                Lc_v[pl.ds(r0 + 0 * P, 16), c1] = (a11 + a22).astype(BF16)
                Lc_v[pl.ds(r0 + 1 * P, 16), c1] = (a21 + a22).astype(BF16)
                Lc_v[pl.ds(r0 + 2 * P, 16), c1] = (a11 + a12).astype(BF16)
                Lc_v[pl.ds(r0 + 3 * P, 16), c1] = (a21 - a11).astype(BF16)
                Lc_v[pl.ds(r0 + 4 * P, 16), c1] = (a12 - a22).astype(BF16)
                yield A_COST

    def tasks(fn, t, n=TM // 16):
        return [lambda tie, s=s: fn(t, s, tie) for s in range(n)]

    def kv_gen(t):
        for m in range(TM // MC):
            r = t * TM + m * MC
            for l in range(D // L):
                lanes = slice(l * L, (l + 1) * L)
                kf = rows_of(k_vs, r, MC, lanes).astype(F32)
                kf_v[l, pl.ds(r + 8, MC), :] = kf
                ks = kf * sk_v[0, 0:1, lanes]
                for tap in range(1, 4):
                    ks = ks + kf_v[l, pl.ds(r + 8 - tap, MC), :] * sk_v[tap, 0:1, lanes]
                kv = ks * rows_of(v_vs, r, MC, lanes).astype(F32)
                kv_v[pl.ds(r, MC), lanes] = kv.astype(BF16)
                yield KV_COST

    def freq_gen(a):
        def cmac(acc, x, g):
            pr = x[0] * g[0] - x[1] * g[1]
            pi = x[0] * g[1] + x[1] * g[0]
            return (pr, pi) if acc is None else (acc[0] + pr, acc[1] + pi)

        for r in range(P // 16):
            rows = pl.ds(r * 16, 16)
            for l in range(D // L):
                lanes = slice(l * L, (l + 1) * L)
                lo = hi = None
                g = (G_v[a + 1, 0, rows, lanes], G_v[a + 1, 1, rows, lanes])
                for c in range(a + 2):
                    x = (X_v[c, 0, rows, lanes], X_v[c, 1, rows, lanes])
                    hi = cmac(hi, x, g)
                    if c <= a:
                        g = (G_v[a - c, 0, rows, lanes], G_v[a - c, 1, rows, lanes])
                        lo = cmac(lo, x, g)
                        yield 32
                for w, z in enumerate((lo, hi)):
                    for part in range(2):
                        Z_v[pl.ds((a + w) * 2 * P + part * P + r * 16, 16), lanes] = z[part].astype(BF16)
                yield 20

    def job_x(t, bg, budget):
        for j in (2 * t, 2 * t + 1):
            for half in range(2):
                r = _dot(F_v[half * P:(half + 1) * P, 0:P], kv_v[j * P:(j + 1) * P, :]).reshape(8, 2, 8, D)
                for part in range(2):
                    X_v[j, part, half * 64:(half + 1) * 64, :] = r[:, part].reshape(64, D)
                bg.run(budget * 2.5)

    def job_h(t, bg, budget):
        h_v, c0 = locate(h_vs, t * TM)
        for half in range(2):
            rows = pl.ds(half * 64, 64)
            for l0, l1 in H_SPLIT:
                w = (l1 - l0) * L
                lanes = slice(l0 * L, l1 * L)
                rhs = jnp.concatenate([h_v[lanes, c0:c0 + P], h_v[lanes, c0 + P:c0 + TM]], axis=0)
                r = jax.lax.dot_general(F_v[half * P:(half + 1) * P, 0:P], rhs, NT_DIMS,
                                        preferred_element_type=F32).reshape(8, 2, 8, 2 * w)
                re, im = r[:, 0].reshape(64, 2 * w), r[:, 1].reshape(64, 2 * w)
                prev = (H_v[t % 2, 0, rows, lanes], H_v[t % 2, 1, rows, lanes])
                for j in range(2):
                    cur = (re[:, j * w:(j + 1) * w], im[:, j * w:(j + 1) * w])
                    G_v[2 * t + j, 0, rows, lanes] = cur[0] + prev[1] if half else cur[0] - prev[1]
                    G_v[2 * t + j, 1, rows, lanes] = cur[1] - prev[0] if half else cur[1] + prev[0]
                    prev = cur
                if t + 1 < NT:
                    H_v[(t + 1) % 2, 0, rows, lanes] = prev[0]
                    H_v[(t + 1) % 2, 1, rows, lanes] = prev[1]
                bg.run(budget * (l1 - l0))

    def z_out(t, m, n, pre, bg, budget, tied):
        z = _gelu_scaled(pre)
        if n < FH // L:
            z1_v[pl.ds(t * TM + m * MC, MC), n * L:(n + 1) * L] = z
        else:
            zg_v[t % 3, m * MC:(m + 1) * MC, n * L - FH:(n + 1) * L - FH] = z
        ntask = tied.run(z)
        bg.run(budget[1] if ntask else budget[0])

    def job_z(t, m, cols, bg, budget, tied):
        for n in cols:
            z_out(t, m, n, _dot(xn_v[pl.ds(t * TM + m * MC, MC), :], win(slice(None), n)), bg, budget, tied)

    def job_zs(t, p, j, bg, budget, tied):
        r1 = pl.ds(t * TM + p * P, MC)
        r2 = pl.ds(t * TM + p * P + MC, MC)
        c1 = slice(j * L, (j + 1) * L)

        def xl(w):
            r0 = (t % 4) * 5 * P + w * P + p * MC
            return XL_v[r0:r0 + MC, :]

        def wb(w):
            return WB_v[w * KH:(w + 1) * KH, c1]

        def rem(rows, n):
            return _dot(xn_v[rows, 2 * KH:], win(slice(2 * KH, D), n))

        m2 = _dot(xl(1), win(slice(0, KH), j))
        m4 = _dot(xn_v[r2, KH:2 * KH], wb(2))
        z_out(t, 2 * p + 1, j, m2 + m4 + rem(r2, j), bg, budget, tied)
        m3 = _dot(xn_v[r1, 0:KH], wb(1))
        m5 = _dot(xl(2), win(slice(KH, 2 * KH), 6 + j))
        z_out(t, 2 * p, 6 + j, m3 + m5 + rem(r1, 6 + j), bg, budget, tied)
        t11, t22 = m4 - m5, m3 - m2
        m1 = _dot(xl(0), wb(0))
        t11, t22 = t11 + m1, t22 + m1
        z_out(t, 2 * p, j, t11 + _dot(xl(4), wb(4)) + rem(r1, j), bg, budget, tied)
        z_out(t, 2 * p + 1, 6 + j, t22 + _dot(xl(3), wb(3)) + rem(r2, 6 + j), bg, budget, tied)

    rev8 = 7 - jax.lax.broadcasted_iota(jnp.int32, (8, L), 0)

    def finish(a, upper, n, hh, slot):
        rows = pl.ds(a * P + (MC if upper else 0), MC)
        lanes = slice(n * L, (n + 1) * L)
        if upper:
            ya = _dot(Fi_v[:, 0:P], Z_v[a * 2 * P:a * 2 * P + P, lanes])
            yb = _dot(Fi_v[:, P:2 * P], Z_v[a * 2 * P + P:(a + 1) * 2 * P, lanes])
            slot(0.5)
            y = ya - yb
            lo = ya + yb
            for j in range(MC // 8):
                yl_v[a % 2, n, (7 - j) * 8:(8 - j) * 8, :] = jnp.take_along_axis(lo[j * 8:(j + 1) * 8], rev8, axis=0)
        else:
            y = yl_v[a % 2, n]
        gate = hh + hh * jnp.tanh(hh)
        s = xn_v[rows, lanes].astype(F32) * y
        x = rows_of(x_vs, a * P + (MC if upper else 0), MC, lanes).astype(F32)
        o_v[rows, lanes] = (x + s * gate).astype(BF16)

    def tail_gen(i, bg, budget):
        a0, a1 = _blocks_of_step(i)

        def slot(w):
            bg.run(w * budget[0])

        def dot3(a, b):
            r = _dot(a, b)
            slot(0.75)
            return r

        for upper in (True, False):
            sub = MC if upper else 0
            r1 = pl.ds(a0 * P + sub, MC)
            r2 = pl.ds(a1 * P + sub, MC)

            def ul(w):
                r0 = ((i % 5) * 5 + w) * P + sub
                return UL_v[r0:r0 + MC, :]

            for j in range(2):
                c1 = slice(j * L, (j + 1) * L)
                c2 = slice((2 + j) * L, (3 + j) * L)

                def wo(w):
                    return WO_v[w * HN:(w + 1) * HN, c1]

                m2 = dot3(ul(1), wout_v[0:HN, c1])
                m4 = dot3(u_v[r2, HN:], wo(2))
                finish(a1, upper, j, m2 + m4, slot)
                bg.charge(T_COST)
                yield
                m3 = dot3(u_v[r1, 0:HN], wo(1))
                m5 = dot3(ul(2), wout_v[HN:, c2])
                finish(a0, upper, 2 + j, m3 + m5, slot)
                bg.charge(T_COST)
                yield
                m1 = dot3(ul(0), wo(0))
                finish(a0, upper, j, (m4 - m5) + m1 + dot3(ul(4), wo(4)), slot)
                bg.charge(T_COST)
                yield
                finish(a1, upper, 2 + j, (m3 - m2) + m1 + dot3(ul(3), wo(3)), slot)
                bg.charge(T_COST)
                yield
            for a, r in ((a0, r1), (a1, r2)):
                finish(a, upper, 4, dot3(u_v[r, 0:HN], wout_v[0:HN, 4 * L:]) + dot3(u_v[r, HN:], wout_v[HN:, 4 * L:]),
                       slot)
                bg.charge(T_COST)
                yield

    def wocomb_gen():
        for j in range(2):
            c1 = slice(j * L, (j + 1) * L)
            c2 = slice((2 + j) * L, (3 + j) * L)
            for r in range(HN // 32):
                top = pl.ds(r * 32, 32)
                bot = pl.ds(HN + r * 32, 32)
                b11, b12 = wout_v[top, c1].astype(F32), wout_v[top, c2].astype(F32)
                b21, b22 = wout_v[bot, c1].astype(F32), wout_v[bot, c2].astype(F32)
                for w, c in enumerate((b11 + b22, b12 - b22, b21 - b11, b11 + b12, b21 + b22)):
                    WO_v[pl.ds(w * HN + r * 32, 32), c1] = c.astype(BF16)
                yield A_COST

    def job_big(i, bg, pending, budget, every):
        a0, a1 = _blocks_of_step(i)
        KG = 512

        def lhs(j, sub, cols):
            if j == 2:
                return wsp_vs[i][sub:sub + MC, cols]
            if j == 3:
                return wsp_vs[i][P + sub:P + sub + MC, HK + cols.start:HK + cols.stop]
            r0 = ((i % 5) * 5 + {0: 0, 1: 1, 4: 2, 5: 3, 6: 4}[j]) * P + sub
            return Lc_v[r0:r0 + MC, cols]

        def prod(j, sub, n, acc=None):
            for kg in range(HK // KG):
                ks = slice(kg * KG, (kg + 1) * KG)
                p = _dot(lhs(j, sub, ks), R_v[j * HK + kg * KG:j * HK + (kg + 1) * KG, n * L:(n + 1) * L])
                acc = p if acc is None else acc + p
                bg.run(budget)
            return acc

        def tails(n):
            for _ in range(n):
                if pending:
                    next(pending.pop(0))

        def emit(a, sub, n, g):
            rows = pl.ds(a * P + sub, MC)
            lanes = slice(n * L, (n + 1) * L)
            u = z1_v[rows, lanes] * (g + bcol_v[rows, :])
            u_v[rows, lanes] = u.astype(BF16)
            bg.charge(E_COST)
            return u

        for sub in (0, MC):
            for n in range(HN // L):
                def put(w, c):
                    UL_v[pl.ds(((i % 5) * 5 + w) * P + sub, MC), n * L:(n + 1) * L] = c.astype(BF16)

                m1 = prod(0, sub, n)
                t11 = prod(6, sub, n, m1)
                m4 = prod(3, sub, n)
                t11 = t11 + m4
                m5 = prod(4, sub, n)
                u11 = emit(a0, sub, n, t11 - m5)
                m2 = prod(1, sub, n)
                u21 = emit(a1, sub, n, m2 + m4)
                put(3, u21 - u11)
                t22 = m1 - m2
                m3 = prod(2, sub, n)
                u12 = emit(a0, sub, n + HN // L, m3 + m5)
                put(2, u11 + u12)
                u22 = emit(a1, sub, n + HN // L, prod(5, sub, n, t22 + m3))
                put(0, u11 + u22)
                put(1, u21 + u22)
                put(4, u12 - u22)
                bg.charge(U_COST)
                tails(every.pop(0))

    def debug_keep_alive():
        if _ONLY is not None:
            for r_ in (xn_u, XL_u, WB_u, UL_u, WO_u, z1_v, R_u, Lc_u, zf_v, zg_v, kv_u, u_u, X_v, H_v, G_v, Z_u,
                       kf_v, bcol_v):
                c_ = pltpu.make_async_copy(r_, r_, sem_small.at[0])
                c_.start()
                c_.wait()

    debug_keep_alive()

    cp_x(0).start()
    cp_win(0).start()
    cp_x(1).start()
    cp_win(1).start()
    start(cp_small())
    for c in range(2, 5):
        cp_win(c).start()
    cp_x(2).start()

    kk = _odd_freq(jax.lax.broadcasted_iota(jnp.int32, (P, P), 0))
    nn = jax.lax.broadcasted_iota(jnp.int32, (P, P), 1)
    fc, fs = _cos_sin((kk * (4 * nn - 127)) & 2047)
    for g in range(P // 8):
        F_v[g * 16:(g + 1) * 16, 0:P] = jnp.concatenate(
            [fc[g * 8:(g + 1) * 8], -fs[g * 8:(g + 1) * 8]], axis=0).astype(BF16)
    fc, fs = _cos_sin((kk * (-127)) & 2047)
    ph_v[0] = fc
    ph_v[1] = fs
    kk = _odd_freq(jax.lax.broadcasted_iota(jnp.int32, (MC, P), 1))
    mm = jax.lax.broadcasted_iota(jnp.int32, (MC, P), 0)
    ic, is_ = _cos_sin((kk * (4 * mm + 2)) & 2047)
    Fi_v[:, 0:P] = (ic * (1.0 / (P * GA))).astype(BF16)
    Fi_v[:, P:2 * P] = (is_ * (1.0 / (P * GA))).astype(BF16)
    kf_v[:, 0:8, :] = jnp.zeros((D // L, 8, L), F32)

    cp_x(0).wait()
    for s in range(TM // 16):
        ln_x(0, s)

    def small_setup():
        sk = sk_in[...].astype(F32)
        for t in range(4):
            sk_v[t] = jnp.broadcast_to(sk[t:t + 1], (8, D))
        drow = d_in[...].astype(F32).reshape(1, D)
        for l in range(D // L):
            lanes = slice(l * L, (l + 1) * L)
            dre = ph_v[0] * drow[:, lanes]
            dim = ph_v[1] * drow[:, lanes]
            H_v[0, 0, 0:64, lanes] = -dim[0:64]
            H_v[0, 0, 64:P, lanes] = dim[64:P]
            H_v[0, 1, 0:64, lanes] = -dre[0:64]
            H_v[0, 1, 64:P, lanes] = dre[64:P]

    def bcol_task(t, j, tie):
        brow = b_in[...].astype(F32).reshape(1, S)[:, j * P:(j + 1) * P] * (0.25 / GA) + tie[0:1]
        bcol_v[j * P:(j + 1) * P, :] = jnp.broadcast_to(brow, (P, P)).T

    LAG = 2

    def interleave(*lists):
        out = []
        for j in range(max(len(a) for a in lists)):
            for a in lists:
                out += a[j:j + 1]
        return out

    def p1_first(c):
        bg = _Background()
        todo = []
        if c == 2:
            todo = tasks(bcol_task, 0)
            small_setup()
        if c == 3:
            todo = tasks(ln_z2, 0)
            bg.add(wcomb_gen(range(3)))
        if c == 4:
            todo = tasks(ln_x2, 2, 8)
            bg.add(wcomb_gen(range(3, 6)))
        tied = _Tied(todo, F_TIED[c])
        if c == 0:
            for s in range(TM // 16):
                ln_x(1, s)
        for t in range(2):
            for m in range(TM // MC):
                job_z(t, m, range(*WIN_CHUNKS[c]), bg, (80, 40), tied)
        bg.drain()
        assert not tied.tasks

    for c in range(5):
        cp_win(c).wait()
        if c == 0:
            cp_x(1).wait()
        if c == 2:
            wait(cp_small())
            start(cp_conv(0))
            cp_x(3).start()
        if c == 4:
            cp_x(2).wait()
            cp_x(4).start()
        block(lambda c=c: p1_first(c), f'p1_f{c}')

    def p1_wait(g):
        if g == 0:
            wait(cp_conv(0))
            cp_x(3).wait()
        if g == 1:
            wait(cp_conv(1))
            cp_x(4).wait()
        if g == 2:
            wait(cp_conv(2))
            cp_x(6).wait()
        if g == 3:
            wait(cp_conv(4))
            cp_wout().wait()
            wait(cp_wsp(0))

    def p1_start(g):
        if g == 0:
            start(cp_conv(1))
            cp_x(6).start()
            start(cp_conv(2))
        if g == 1:
            start(cp_conv(4))
            cp_wout().start()
            start(cp_wsp(0))
            start(cp_wsp(1))
        if g == 3:
            start(cp_wsp(2))
            start(cp_conv(6))
            for i in (3, 4, 5):
                start(cp_wsp(i))

    def take(gen, n):
        for _ in range(n):
            yield next(gen)

    def p1_step(i):
        bg = _Background()
        dft = _Background()
        t = i - LAG
        xg = P1_X[i]
        kv = kv_gen(t)
        nx, nz, nh = KV_SPLIT[i]
        dft.add(take(kv, nx))
        bg.add(take(kv, nz))
        hbg = _Background()
        hbg.add(take(kv, nh))
        zb = nz * KV_COST / 48.0
        extra = 0
        if i == 6:
            bg.add(wocomb_gen())
            bg.add(acomb_gen(0, range(3)))
            extra = EXTRA[0]
        if i == 7:
            bg.add(acomb_gen(0, range(3, 8)))
            extra = EXTRA[1]
        last = i == NT - 1
        z2t = tasks(ln_z2, i - 1)
        xt = [tasks(ln_x2, t_, 8) for t_ in P1_LNX[i]]
        if P1_TUNE[i][1]:
            todo = interleave(*([z2t[0::2]] + xt + [z2t[1::2]]))
        else:
            todo = interleave(*(xt + [z2t[0::2], z2t[1::2]]))
        tied = _Tied(todo, P1_TUNE[i][0])
        if xg is not None:
            dft.run(KV_COST)
            job_x(xg, dft, (nx - 1) * KV_COST / 10.0)
            dft.drain()
        for p in range(2):
            for j in range(FH // L):
                job_zs(i, p, j, bg, (1.6 * zb + extra, 0.5 * zb + extra), tied)
            assert not tied.tasks or (p == 0 and not last)
            if p == 0 and last:
                tied = _Tied(tasks(ln_z2, i, 8), LAST_N)
        if last:
            for s in range(8, 16):
                ln_z2(i, s)
        bg.drain()
        job_h(t, hbg, nh * KV_COST / 10.0)
        hbg.drain()

    def p1_block(g):
        for i in P1_GROUPS[g]:
            p1_step(i)

    for g in range(len(P1_GROUPS)):
        p1_wait(g)
        p1_start(g)
        block(lambda g=g: p1_block(g), f'p1_g{g}')

    groups = P2_GROUPS
    NG = len(groups)

    def p2_dma(gi):
        if gi >= 2:
            for i in groups[gi - 2]:
                start(cp_out(i))
        if gi >= 3:
            for i in groups[gi - 3]:
                wait(cp_out(i))
        if gi == 1:
            for i in (6, 7):
                start(cp_wsp(i))
        if gi == 0:
            wait(cp_conv(6))
        if gi + 1 < NG:
            for i in groups[gi + 1]:
                wait(cp_wsp(i))

    def tails_of(i, bg, budget):
        return [tail_gen(i, bg, budget)] * 20

    def p2_block(gi):
        bg = _Background()
        steps = groups[gi]
        tb = [0.0]
        pending = [t_ for i in (groups[gi - 1] if gi > 0 else []) for t_ in tails_of(i, bg, tb)]
        total = sum(a + 1 for i in steps for a in _blocks_of_step(i)) * 40 * 16
        total += len(steps) * (24 * E_COST + 6 * U_COST) + len(pending) * T_COST
        slots = 84 * len(steps) + TAIL_W * len(pending)
        bg.add(freq_gen(_blocks_of_step(steps[0])[0]))
        if gi < 2:
            bg.add(kv_gen(NT - 2 + gi))
            total += 20 * KV_COST
            slots += 10
        for t in P2_X[gi]:
            slots += 10
        if gi + 1 < NG:
            for i in groups[gi + 1]:
                bg.add(acomb_gen(i))
                total += 32 * A_COST
        for i in steps[1:]:
            bg.add(freq_gen(_blocks_of_step(i)[0]))
        budget = tb[0] = total / (slots + P2_END[gi])
        bg.run(budget)
        for t in P2_X[gi]:
            job_x(t, bg, budget)
        if gi < 2:
            job_h(NT - 2 + gi, bg, budget)
        units = [4, 4, 2, 4, 4, 2] * (len(pending) // 20)
        every = [0] * (6 * len(steps))
        for j, n in enumerate(units):
            every[min(len(every) - 1, j * len(every) // len(units))] += n
        for i in steps:
            job_big(i, bg, pending, budget, every)
        for t_ in pending:
            next(t_)
        bg.drain()

    for gi in range(NG):
        p2_dma(gi)
        block(lambda gi=gi: p2_block(gi), f'p2_{gi}')

    def cp_last(part):
        a0 = _blocks_of_step(NT - 1)[0]
        sub, cols = ((MC, pl.ds(0, D)), (0, pl.ds(0, 4 * L)), (0, pl.ds(4 * L, L)))[part]
        return [pltpu.make_async_copy(o_v.at[pl.ds(r, MC), cols], o_hbm.at[0, pl.ds(r, MC), cols],
                                      sem_out.at[NT - 1]) for r in (a0 * P + sub, (a0 + 1) * P + sub)]

    def p2_last():
        for i in groups[NG - 1]:
            for j, t_ in enumerate(tails_of(i, _Background(), [0.0])):
                next(t_)
                if i < NT - 1 and j == 19:
                    start(cp_out(i))
                if i == NT - 1 and j in (9, 17):
                    start(cp_last(j // 10))

    p2_dma(NG)
    block(p2_last, 'p2_last')
    start(cp_last(2))
    for i in groups[NG - 2] + groups[NG - 1][:-1]:
        wait(cp_out(i))
    for part in range(3):
        wait(cp_last(part))
    debug_keep_alive()


def _compiler_params():
    vmem = 116 * 1024 * 1024
    try:
        return pltpu.CompilerParams(vmem_limit_bytes=vmem, disable_semaphore_checks=True)
    except TypeError:
        return pltpu.CompilerParams(vmem_limit_bytes=vmem)


@jax.jit
def pallas_recurrent_scan__ssm_conv_h3__mixer_gmlp__prompt_kernel(
    A_q: jax.Array,
    A_k: jax.Array,
    A_v: jax.Array,
    A_shift_k: jax.Array,
    A_ssm_k: jax.Array,
    A_ssm_D: jax.Array,
    B_x: jax.Array,
    B_w_in: jax.Array,
    B_w_sp: jax.Array,
    B_b_sp: jax.Array,
    B_w_out: jax.Array,
):
    del B_x
    hbm = pl.BlockSpec(memory_space=pl.ANY)

    def bf16_buf(*shape):
        return pltpu.VMEM(shape[:-2] + (shape[-2] // 2, shape[-1]), U32)

    return pl.pallas_call(
        _kernel,
        out_shape=jax.ShapeDtypeStruct((1, S, D), BF16),
        in_specs=[hbm] * 10,
        out_specs=hbm,
        scratch_shapes=[
            [bf16_buf(len(g) * TM, D) for g in X_DMAS],
            [bf16_buf(len(g) * TM, D) for g in CONV_DMAS],
            [bf16_buf(len(g) * TM, D) for g in CONV_DMAS],
            [bf16_buf(D, len(g) * TM) for g in CONV_DMAS],
            [bf16_buf(D, max(hi - lo, 2) * L) for lo, hi in WIN_CHUNKS],
            [bf16_buf(TM, S) for _ in range(NT)],
            bf16_buf(FH, D),
            pltpu.VMEM((S, D), BF16),
            pltpu.VMEM((4, D), BF16),
            pltpu.VMEM((D,), BF16),
            pltpu.VMEM((S,), BF16),
            bf16_buf(S, D),
            bf16_buf(4 * 5 * P, KH),
            bf16_buf(5 * KH, FH),
            bf16_buf(5 * 5 * P, HN),
            bf16_buf(5 * HN, 2 * L),
            pltpu.VMEM((S, FH), F32),
            bf16_buf(7 * HK, HN),
            bf16_buf(5 * 5 * P, HK),
            pltpu.VMEM((HK, FH), F32),
            pltpu.VMEM((3, TM, FH), F32),
            bf16_buf(S, D),
            bf16_buf(S, FH),
            pltpu.VMEM((NB, 2, P, D), F32),
            pltpu.VMEM((2, 2, P, D), F32),
            pltpu.VMEM((NB, 2, P, D), F32),
            bf16_buf(NB * 2 * P, D),
            pltpu.VMEM((2, D // L, MC, L), F32),
            bf16_buf(2 * P, 2 * P),
            bf16_buf(MC, 2 * P),
            pltpu.VMEM((S, L), F32),
            pltpu.VMEM((2, P, L), F32),
            pltpu.VMEM((4, 8, D), F32),
            pltpu.VMEM((D // L, S + 8, L), F32),
            pltpu.SemaphoreType.DMA((1,)),
            pltpu.SemaphoreType.DMA((NT,)),
            pltpu.SemaphoreType.DMA((NT,)),
            pltpu.SemaphoreType.DMA((NT,)),
            pltpu.SemaphoreType.DMA((5,)),
            pltpu.SemaphoreType.DMA((NT,)),
        ],
        compiler_params=_compiler_params(),
    )(A_q, A_k, A_v, A_shift_k.T, A_ssm_k, A_ssm_D, B_w_in, B_w_sp, B_b_sp, B_w_out)
```

```python
import math

import jax
import jax.numpy as jnp
import jax.experimental.pallas as pl
import jax.experimental.pallas.tpu as pltpu

S = 2048
D = 640
FH = 768
P = 128
NB = S // P
TM = 256
NT = S // TM
MC = 64
L = 128
HK = S // 2
KQ = 512
A2_COST = 34
L1_USE = {0: ((0, 1, True, False), (3, 1, True, False)), 6: ((0, 1, False, False),), 3: ((0, 1, False, False), (2, 1, True, False)),
          4: ((0, -1, False, True), (1, 1, True, False)), 1: ((2, 1, False, True), (3, -1, False, False)),
          2: ((1, 1, False, True), (3, 1, False, False)), 5: ((3, 1, False, True),)}
KH = 256
HN = FH // 2
EPS = 1e-5
F32 = jnp.float32
BF16 = jnp.bfloat16
U32 = jnp.uint32
GELU_C = math.sqrt(2.0 / math.pi)
GA = (GELU_C * 0.044715) ** (1.0 / 3.0)
NT_DIMS = (((1,), (1,)), ((), ()))

WIN_CHUNKS = ((6, 7), (7, 9), (9, 12), (0, 3), (3, 6))
X_DMAS = ((0,), (1,), (2,), (3,), (4, 5), (6, 7))
CONV_DMAS = ((0,), (1,), (2, 3), (4, 5), (6, 7))
P1_GROUPS = ((2,), (3,), (4, 5), (6, 7))
P1_X = {2: None, 3: 0, 4: 1, 5: None, 6: 2, 7: 3}
P1_LNX = {2: (3,), 3: (4, 5), 4: (6,), 5: (7,), 6: (), 7: ()}
P2_GROUPS = ((0,), (1, 2), (3, 4, 5), (6, 7))
P2_X = ((4, 5), (6,), (7,), ())
STEP_BLOCKS = ((2, 3), (6, 7), (4, 5), (12, 13), (10, 11), (0, 1), (14, 15), (8, 9))
KV_COST, A_COST = 110, 56
E_COST, U_COST, T_COST, TAIL_W = 24, 90, 90, 1.6
KV_SPLIT = {2: (0, 14, 6), 3: (12, 4, 4), 4: (12, 4, 4), 5: (0, 14, 6), 6: (12, 4, 4), 7: (12, 4, 4)}
H_SPLIT = ((0, 2), (2, 4), (4, 5))
P1_TUNE = {2: (42, 0), 3: (43, 1), 4: (42, 0), 5: (42, 0), 6: (44, 0), 7: (24, 0)}
EXTRA = (52, 52)
LAST_N = 22
P2_END = (0.0, -1.0, -1.0, 0.0)
F_TIED = (20, 20, 18, 20, 20)
_ONLY = None


def _dot(a, b):
    return jnp.dot(a, b, preferred_element_type=F32)


def _cos_sin(m):
    q = (m + 256) >> 9
    x = (m - (q << 9)).astype(F32) * (2.0 * math.pi / 2048.0)
    x2 = x * x
    s = x * (1.0 + x2 * (-1.0 / 6 + x2 * (1.0 / 120 + x2 * (-1.0 / 5040 + x2 * (1.0 / 362880)))))
    c = 1.0 + x2 * (-0.5 + x2 * (1.0 / 24 + x2 * (-1.0 / 720 + x2 * (1.0 / 40320 - x2 * (1.0 / 3628800)))))
    swap = (q & 1) == 1
    c0 = jnp.where(swap, s, c)
    s0 = jnp.where(swap, c, s)
    cos = jnp.where(((q + 1) & 2) == 2, -c0, c0)
    sin = jnp.where((q & 2) == 2, -s0, s0)
    return cos, sin


def _odd_freq(r):
    return jnp.where(r < 64, 4 * r + 1, 4 * r - 253)


def _gelu_scaled(z):
    return z + z * jnp.tanh(z * (GELU_C / GA + z * z))


def _signzero(z):
    bits = jax.lax.bitcast_convert_type(z, U32) & jnp.uint32(0x80000000)
    return jax.lax.bitcast_convert_type(bits, F32)


def _ln(x, eps, tie=None, scale=None):
    n = x.shape[-1]
    cols = [x[:, j * L:(j + 1) * L] for j in range(n // L)]
    s1 = cols[0]
    s2 = cols[0] * cols[0]
    for c in cols[1:]:
        s1 = s1 + c
        s2 = s2 + c * c
    if tie is not None:
        s1 = s1 + tie
        s2 = s2 + tie
    m = jnp.sum(s1, axis=-1, keepdims=True) * (1.0 / n)
    v = jnp.maximum(jnp.sum(s2, axis=-1, keepdims=True) * (1.0 / n) - m * m, 0.0)
    rs = jax.lax.rsqrt(v + eps)
    if scale is not None:
        rs = rs * scale
    return (x - m) * rs


def _blocks_of_step(i):
    return STEP_BLOCKS[i]


class _Background:
    def __init__(self):
        self.q = []
        self.credit = 0.0

    def add(self, gen):
        self.q.append(gen)

    def run(self, budget):
        self.credit += budget
        while self.q and self.credit > 0:
            try:
                self.credit -= next(self.q[0])
            except StopIteration:
                self.q.pop(0)
        if not self.q:
            self.credit = 0.0

    def charge(self, cost):
        self.credit -= cost

    def drain(self):
        while self.q:
            self.run(1e9)


class _Tied:
    def __init__(self, tasks, npieces):
        self.tasks = list(tasks)
        self.rate = len(self.tasks) / float(npieces)
        self.credit = 0.999

    def run(self, z):
        self.credit += self.rate
        n = 0
        while self.tasks and self.credit >= 1.0:
            self.tasks.pop(0)(_signzero(z[0:16]))
            self.credit -= 1.0
            n += 1
        return n


def _kernel(q_hbm, k_hbm, v_hbm, sk_hbm, h_hbm, d_hbm, win_hbm, wsp_hbm, b_hbm, wout_hbm,
            o_hbm,
            x_us, k_us, v_us, h_us, win_us, wsp_us, wout_u, o_v, sk_in, d_in, b_in,
            xn_u, XL_u, WB_u, UL_u, WO_u, z1_v, R_u, Lc_u, L2_u, R2_u, C_v, zf_v, zg_v, kv_u, u_u, X_v, H_v, G_v, Z_u,
            yl_v, F_u, Fi_u, bcol_v, ph_v, sk_v, kf_v,
            sem_small, sem_x, sem_conv, sem_wsp, sem_w, sem_out):
    (wout_v, xn_v, XL_v, WB_v, UL_v, WO_v, R_v, Lc_v, L2_v, R2_v, kv_v, u_v, Z_v, F_v, Fi_v) = [
        r.bitcast(BF16) for r in (wout_u, xn_u, XL_u, WB_u, UL_u, WO_u, R_u, Lc_u, L2_u, R2_u, kv_u, u_u, Z_u, F_u, Fi_u)]
    x_vs = {g[0]: r.bitcast(BF16) for g, r in zip(X_DMAS, x_us)}
    k_vs, v_vs, h_vs = [{g[0]: r.bitcast(BF16) for g, r in zip(CONV_DMAS, rs)} for rs in (k_us, v_us, h_us)]
    wsp_vs = [r.bitcast(BF16) for r in wsp_us]
    win_vs = [r.bitcast(BF16) for r in win_us]

    def win(rows, n):
        c = [lo <= n < hi for lo, hi in WIN_CHUNKS].index(True)
        n -= WIN_CHUNKS[c][0]
        return win_vs[c][rows, n * L:(n + 1) * L]

    def locate(bufs, row):
        t0 = max(t for t in bufs if t * TM <= row)
        return bufs[t0], row - t0 * TM

    def rows_of(bufs, row, n, lanes=slice(None)):
        buf, r = locate(bufs, row)
        return buf[r:r + n, lanes]

    def cp_small():
        return [pltpu.make_async_copy(s_, d_, sem_small.at[0])
                for s_, d_ in ((d_hbm, d_in), (sk_hbm, sk_in), (b_hbm, b_in))]

    def cp_x(t):
        return pltpu.make_async_copy(q_hbm.at[0, pl.ds(t * TM, x_vs[t].shape[0])], x_vs[t], sem_x.at[t])

    def cp_conv(t):
        rows = pl.ds(t * TM, k_vs[t].shape[0])
        sem = sem_conv.at[t]
        return [pltpu.make_async_copy(h_hbm.at[:, rows], h_vs[t], sem),
                pltpu.make_async_copy(k_hbm.at[0, rows], k_vs[t], sem),
                pltpu.make_async_copy(v_hbm.at[0, rows], v_vs[t], sem)]

    def cp_wsp(i):
        return [pltpu.make_async_copy(wsp_hbm.at[pl.ds(_blocks_of_step(i)[0] * P, TM)], wsp_vs[i], sem_wsp.at[i])]

    def cp_win(c):
        lo, hi = WIN_CHUNKS[c]
        w = (hi - lo) * L
        return pltpu.make_async_copy(win_hbm.at[:, pl.ds(lo * L, w)], win_vs[c].at[:, pl.ds(0, w)], sem_w.at[c])

    def cp_wout():
        return pltpu.make_async_copy(wout_hbm, wout_v, sem_w.at[0])

    def cp_out(i):
        rows = pl.ds(_blocks_of_step(i)[0] * P, TM)
        return [pltpu.make_async_copy(o_v.at[rows], o_hbm.at[0, rows], sem_out.at[i])]

    def start(cs):
        for c in cs:
            c.start()

    def wait(cs):
        for c in cs:
            c.wait()

    def block(fn, name):
        def body(it):
            fn()
            return it + 1

        if _ONLY is None or name in _ONLY:
            jax.lax.while_loop(lambda it: it < 1, body, jnp.int32(0))

    def ln_x(t, s, tie=None):
        rows = pl.ds(t * TM + s * 16, 16)
        y = _ln(rows_of(x_vs, t * TM + s * 16, 16).astype(F32), EPS, tie, GA)
        xn_v[rows, :] = y.astype(BF16)
        return y

    def ln_x2(t, s, tie):
        p, q = s // 4, s % 4
        y1 = ln_x(t, 8 * p + q, tie)
        y2 = ln_x(t, 8 * p + 4 + q, tie)
        a11, a12, a21, a22 = y1[:, :KH], y1[:, KH:2 * KH], y2[:, :KH], y2[:, KH:2 * KH]
        r0 = (t % 4) * 5 * P + p * MC + q * 16
        for j, c in enumerate((a11 + a22, a21 + a22, a11 + a12, a21 - a11, a12 - a22)):
            XL_v[pl.ds(r0 + j * P, 16), :] = c.astype(BF16)

    def wcomb_gen(cols):
        for j in cols:
            c1 = slice(j * L, (j + 1) * L)
            for r in range(KH // 32):
                top = pl.ds(r * 32, 32)
                bot = pl.ds(KH + r * 32, 32)
                b11, b12 = win(top, j).astype(F32), win(top, 6 + j).astype(F32)
                b21, b22 = win(bot, j).astype(F32), win(bot, 6 + j).astype(F32)
                for w, c in enumerate((b11 + b22, b12 - b22, b21 - b11, b11 + b12, b21 + b22)):
                    WB_v[pl.ds(w * KH + r * 32, 32), c1] = c.astype(BF16)
                yield A_COST

    def ln_z2(t, s, tie=None):
        y = _ln(zg_v[t % 3, s * 16:(s + 1) * 16, :], 4.0 * GA * GA * EPS, tie, 0.25 / GA)
        lo, hi = y[:, :HN], y[:, HN:]
        r = (t * TM + s * 16) % HK
        rows = pl.ds(r, 16)
        if t < NT // 2:
            zf_v[rows, :] = y
            R_v[pl.ds(1 * HK + r, 16), :] = lo.astype(BF16)
            R_v[pl.ds(5 * HK + r, 16), :] = (lo + hi).astype(BF16)
        else:
            b11, b12 = zf_v[rows, :HN], zf_v[rows, HN:]
            R_v[pl.ds(0 * HK + r, 16), :] = (b11 + hi).astype(BF16)
            R_v[pl.ds(2 * HK + r, 16), :] = (b12 - hi).astype(BF16)
            R_v[pl.ds(3 * HK + r, 16), :] = (lo - b11).astype(BF16)
            R_v[pl.ds(4 * HK + r, 16), :] = hi.astype(BF16)
            R_v[pl.ds(6 * HK + r, 16), :] = (lo + hi).astype(BF16)

    def acomb_gen(i, groups=range(P // 16)):
        for r in groups:
            for c in range(HK // 256):
                top = pl.ds(r * 16, 16)
                bot = pl.ds(P + r * 16, 16)
                c1 = slice(c * 256, (c + 1) * 256)
                c2 = slice(HK + c * 256, HK + (c + 1) * 256)
                a11 = wsp_vs[i][top, c1].astype(F32)
                a12 = wsp_vs[i][top, c2].astype(F32)
                a21 = wsp_vs[i][bot, c1].astype(F32)
                a22 = wsp_vs[i][bot, c2].astype(F32)
                r0 = (i % 5) * 5 * P + r * 16
                Lc_v[pl.ds(r0 + 0 * P, 16), c1] = (a11 + a22).astype(BF16)
                Lc_v[pl.ds(r0 + 1 * P, 16), c1] = (a21 + a22).astype(BF16)
                Lc_v[pl.ds(r0 + 2 * P, 16), c1] = (a11 + a12).astype(BF16)
                Lc_v[pl.ds(r0 + 3 * P, 16), c1] = (a21 - a11).astype(BF16)
                Lc_v[pl.ds(r0 + 4 * P, 16), c1] = (a12 - a22).astype(BF16)
                yield A_COST

    def acomb2_gen(i):
        for r in range(MC // 16):
            for c in range(KQ // L):
                quad = {}

                def w(b, H):
                    if (b, H) not in quad:
                        quad[b, H] = [[wsp_vs[i][pl.ds(b * P + s_ * MC + r * 16, 16),
                                                 H * HK + kh * KQ + c * L:H * HK + kh * KQ + (c + 1) * L].astype(F32)
                                       for kh in range(2)] for s_ in range(2)]
                    return quad[b, H]

                for j, slot, (p_, q_, sign) in ((2, None, ((0, 0), None, 0)), (0, 0, ((0, 0), (1, 1), 1)),
                                                (3, None, ((1, 1), None, 0)), (1, 1, ((1, 0), (1, 1), 1)),
                                                (5, 3, ((1, 0), (0, 0), -1)), (4, 2, ((0, 0), (0, 1), 1)),
                                                (6, 4, ((0, 1), (1, 1), -1))):
                    a = w(*p_)
                    if q_ is not None:
                        b_ = w(*q_)
                        a = [[a[s_][kh] + b_[s_][kh] if sign > 0 else a[s_][kh] - b_[s_][kh] for kh in range(2)]
                             for s_ in range(2)]
                        for s_ in range(2):
                            for kh in range(2):
                                Lc_v[pl.ds(((i % 5) * 5 + slot) * P + s_ * MC + r * 16, 16),
                                     kh * KQ + c * L:kh * KQ + (c + 1) * L] = a[s_][kh].astype(BF16)
                    for w2, v_ in enumerate((a[0][0] + a[1][1], a[1][0] + a[1][1], a[0][0] + a[0][1],
                                             a[1][0] - a[0][0], a[0][1] - a[1][1])):
                        L2_v[pl.ds((((i % 5) * 7 + j) * 5 + w2) * MC + r * 16, 16), c * L:(c + 1) * L] = v_.astype(BF16)
                    yield A2_COST

    def bcomb2_gen(js):
        for j in js:
            for r in range(KQ // 32):
                top = pl.ds(j * HK + r * 32, 32)
                bot = pl.ds(j * HK + KQ + r * 32, 32)
                b11, b12 = R_v[top, 0:L].astype(F32), R_v[top, L:2 * L].astype(F32)
                b21, b22 = R_v[bot, 0:L].astype(F32), R_v[bot, L:2 * L].astype(F32)
                for w, c in enumerate((b11 + b22, b12 - b22, b21 - b11, b11 + b12, b21 + b22)):
                    R2_v[pl.ds((j * 3 + w // 2) * KQ + r * 32, 32), (w % 2) * L:(w % 2 + 1) * L] = c.astype(BF16)
                yield A_COST

    def tasks(fn, t, n=TM // 16):
        return [lambda tie, s=s: fn(t, s, tie) for s in range(n)]

    def kv_gen(t):
        for m in range(TM // MC):
            r = t * TM + m * MC
            for l in range(D // L):
                lanes = slice(l * L, (l + 1) * L)
                kf = rows_of(k_vs, r, MC, lanes).astype(F32)
                kf_v[l, pl.ds(r + 8, MC), :] = kf
                ks = kf * sk_v[0, 0:1, lanes]
                for tap in range(1, 4):
                    ks = ks + kf_v[l, pl.ds(r + 8 - tap, MC), :] * sk_v[tap, 0:1, lanes]
                kv = ks * rows_of(v_vs, r, MC, lanes).astype(F32)
                kv_v[pl.ds(r, MC), lanes] = kv.astype(BF16)
                yield KV_COST

    def freq_gen(a):
        def cmac(acc, x, g):
            pr = x[0] * g[0] - x[1] * g[1]
            pi = x[0] * g[1] + x[1] * g[0]
            return (pr, pi) if acc is None else (acc[0] + pr, acc[1] + pi)

        for r in range(P // 16):
            rows = pl.ds(r * 16, 16)
            for l in range(D // L):
                lanes = slice(l * L, (l + 1) * L)
                lo = hi = None
                g = (G_v[a + 1, 0, rows, lanes], G_v[a + 1, 1, rows, lanes])
                for c in range(a + 2):
                    x = (X_v[c, 0, rows, lanes], X_v[c, 1, rows, lanes])
                    hi = cmac(hi, x, g)
                    if c <= a:
                        g = (G_v[a - c, 0, rows, lanes], G_v[a - c, 1, rows, lanes])
                        lo = cmac(lo, x, g)
                        yield 32
                for w, z in enumerate((lo, hi)):
                    for part in range(2):
                        Z_v[pl.ds((a + w) * 2 * P + part * P + r * 16, 16), lanes] = z[part].astype(BF16)
                yield 20

    def job_x(t, bg, budget):
        for j in (2 * t, 2 * t + 1):
            for half in range(2):
                r = _dot(F_v[half * P:(half + 1) * P, 0:P], kv_v[j * P:(j + 1) * P, :]).reshape(8, 2, 8, D)
                for part in range(2):
                    X_v[j, part, half * 64:(half + 1) * 64, :] = r[:, part].reshape(64, D)
                bg.run(budget * 2.5)

    def job_h(t, bg, budget):
        h_v, c0 = locate(h_vs, t * TM)
        for half in range(2):
            rows = pl.ds(half * 64, 64)
            for l0, l1 in H_SPLIT:
                w = (l1 - l0) * L
                lanes = slice(l0 * L, l1 * L)
                rhs = jnp.concatenate([h_v[lanes, c0:c0 + P], h_v[lanes, c0 + P:c0 + TM]], axis=0)
                r = jax.lax.dot_general(F_v[half * P:(half + 1) * P, 0:P], rhs, NT_DIMS,
                                        preferred_element_type=F32).reshape(8, 2, 8, 2 * w)
                re, im = r[:, 0].reshape(64, 2 * w), r[:, 1].reshape(64, 2 * w)
                prev = (H_v[t % 2, 0, rows, lanes], H_v[t % 2, 1, rows, lanes])
                for j in range(2):
                    cur = (re[:, j * w:(j + 1) * w], im[:, j * w:(j + 1) * w])
                    G_v[2 * t + j, 0, rows, lanes] = cur[0] + prev[1] if half else cur[0] - prev[1]
                    G_v[2 * t + j, 1, rows, lanes] = cur[1] - prev[0] if half else cur[1] + prev[0]
                    prev = cur
                if t + 1 < NT:
                    H_v[(t + 1) % 2, 0, rows, lanes] = prev[0]
                    H_v[(t + 1) % 2, 1, rows, lanes] = prev[1]
                bg.run(budget * (l1 - l0))

    def z_out(t, m, n, pre, bg, budget, tied):
        z = _gelu_scaled(pre)
        if n < FH // L:
            z1_v[pl.ds(t * TM + m * MC, MC), n * L:(n + 1) * L] = z
        else:
            zg_v[t % 3, m * MC:(m + 1) * MC, n * L - FH:(n + 1) * L - FH] = z
        ntask = tied.run(z)
        bg.run(budget[1] if ntask else budget[0])

    def job_z(t, m, cols, bg, budget, tied):
        for n in cols:
            z_out(t, m, n, _dot(xn_v[pl.ds(t * TM + m * MC, MC), :], win(slice(None), n)), bg, budget, tied)

    def job_zs(t, p, j, bg, budget, tied):
        r1 = pl.ds(t * TM + p * P, MC)
        r2 = pl.ds(t * TM + p * P + MC, MC)
        c1 = slice(j * L, (j + 1) * L)

        def xl(w):
            r0 = (t % 4) * 5 * P + w * P + p * MC
            return XL_v[r0:r0 + MC, :]

        def wb(w):
            return WB_v[w * KH:(w + 1) * KH, c1]

        def rem(rows, n):
            return _dot(xn_v[rows, 2 * KH:], win(slice(2 * KH, D), n))

        m2 = _dot(xl(1), win(slice(0, KH), j))
        m4 = _dot(xn_v[r2, KH:2 * KH], wb(2))
        z_out(t, 2 * p + 1, j, m2 + m4 + rem(r2, j), bg, budget, tied)
        m3 = _dot(xn_v[r1, 0:KH], wb(1))
        m5 = _dot(xl(2), win(slice(KH, 2 * KH), 6 + j))
        z_out(t, 2 * p, 6 + j, m3 + m5 + rem(r1, 6 + j), bg, budget, tied)
        t11, t22 = m4 - m5, m3 - m2
        m1 = _dot(xl(0), wb(0))
        t11, t22 = t11 + m1, t22 + m1
        z_out(t, 2 * p, j, t11 + _dot(xl(4), wb(4)) + rem(r1, j), bg, budget, tied)
        z_out(t, 2 * p + 1, 6 + j, t22 + _dot(xl(3), wb(3)) + rem(r2, 6 + j), bg, budget, tied)

    rev8 = 7 - jax.lax.broadcasted_iota(jnp.int32, (8, L), 0)

    def finish(a, upper, n, hh, slot):
        rows = pl.ds(a * P + (MC if upper else 0), MC)
        lanes = slice(n * L, (n + 1) * L)
        if upper:
            ya = _dot(Fi_v[:, 0:P], Z_v[a * 2 * P:a * 2 * P + P, lanes])
            yb = _dot(Fi_v[:, P:2 * P], Z_v[a * 2 * P + P:(a + 1) * 2 * P, lanes])
            slot(0.5)
            y = ya - yb
            lo = ya + yb
            for j in range(MC // 8):
                yl_v[a % 2, n, (7 - j) * 8:(8 - j) * 8, :] = jnp.take_along_axis(lo[j * 8:(j + 1) * 8], rev8, axis=0)
        else:
            y = yl_v[a % 2, n]
        gate = hh + hh * jnp.tanh(hh)
        s = xn_v[rows, lanes].astype(F32) * y
        x = rows_of(x_vs, a * P + (MC if upper else 0), MC, lanes).astype(F32)
        o_v[rows, lanes] = (x + s * gate).astype(BF16)

    def tail_gen(i, bg, budget):
        a0, a1 = _blocks_of_step(i)

        def slot(w):
            bg.run(w * budget[0])

        def dot3(a, b):
            r = _dot(a, b)
            slot(0.75)
            return r

        for upper in (True, False):
            sub = MC if upper else 0
            r1 = pl.ds(a0 * P + sub, MC)
            r2 = pl.ds(a1 * P + sub, MC)

            def ul(w):
                r0 = ((i % 5) * 5 + w) * P + sub
                return UL_v[r0:r0 + MC, :]

            for j in range(2):
                c1 = slice(j * L, (j + 1) * L)
                c2 = slice((2 + j) * L, (3 + j) * L)

                def wo(w):
                    return WO_v[w * HN:(w + 1) * HN, c1]

                m2 = dot3(ul(1), wout_v[0:HN, c1])
                m4 = dot3(u_v[r2, HN:], wo(2))
                finish(a1, upper, j, m2 + m4, slot)
                bg.charge(T_COST)
                yield
                m3 = dot3(u_v[r1, 0:HN], wo(1))
                m5 = dot3(ul(2), wout_v[HN:, c2])
                finish(a0, upper, 2 + j, m3 + m5, slot)
                bg.charge(T_COST)
                yield
                m1 = dot3(ul(0), wo(0))
                finish(a0, upper, j, (m4 - m5) + m1 + dot3(ul(4), wo(4)), slot)
                bg.charge(T_COST)
                yield
                finish(a1, upper, 2 + j, (m3 - m2) + m1 + dot3(ul(3), wo(3)), slot)
                bg.charge(T_COST)
                yield
            for a, r in ((a0, r1), (a1, r2)):
                finish(a, upper, 4, dot3(u_v[r, 0:HN], wout_v[0:HN, 4 * L:]) + dot3(u_v[r, HN:], wout_v[HN:, 4 * L:]),
                       slot)
                bg.charge(T_COST)
                yield

    def wocomb_gen():
        for j in range(2):
            c1 = slice(j * L, (j + 1) * L)
            c2 = slice((2 + j) * L, (3 + j) * L)
            for r in range(HN // 32):
                top = pl.ds(r * 32, 32)
                bot = pl.ds(HN + r * 32, 32)
                b11, b12 = wout_v[top, c1].astype(F32), wout_v[top, c2].astype(F32)
                b21, b22 = wout_v[bot, c1].astype(F32), wout_v[bot, c2].astype(F32)
                for w, c in enumerate((b11 + b22, b12 - b22, b21 - b11, b11 + b12, b21 + b22)):
                    WO_v[pl.ds(w * HN + r * 32, 32), c1] = c.astype(BF16)
                yield A_COST

    def job_big(i, bg, pending, budget, every):
        a0, a1 = _blocks_of_step(i)
        KG = 512

        def lhs(j, sub, cols):
            if j == 2:
                return wsp_vs[i][sub:sub + MC, cols]
            if j == 3:
                return wsp_vs[i][P + sub:P + sub + MC, HK + cols.start:HK + cols.stop]
            r0 = ((i % 5) * 5 + {0: 0, 1: 1, 4: 2, 5: 3, 6: 4}[j]) * P + sub
            return Lc_v[r0:r0 + MC, cols]

        def prod(j, sub, n, acc=None):
            for kg in range(HK // KG):
                ks = slice(kg * KG, (kg + 1) * KG)
                p = _dot(lhs(j, sub, ks), R_v[j * HK + kg * KG:j * HK + (kg + 1) * KG, n * L:(n + 1) * L])
                acc = p if acc is None else acc + p
                bg.run(budget)
            return acc

        def tails(n):
            for _ in range(n):
                if pending:
                    next(pending.pop(0))

        def emit(a, sub, n, g):
            rows = pl.ds(a * P + sub, MC)
            lanes = slice(n * L, (n + 1) * L)
            u = z1_v[rows, lanes] * (g + bcol_v[rows, :])
            u_v[rows, lanes] = u.astype(BF16)
            bg.charge(E_COST)
            return u

        if i > 0:
            def piece(a, b, acc=None):
                p = _dot(a, b)
                bg.run(budget)
                return p if acc is None else acc + p

            def cslot(k, s_, n):
                return pl.ds(((k * 2 + s_) * 2 + n) * MC, MC)

            us = {}

            def contribute(j, s_, n, m):
                for k, sign, first, last in L1_USE[j]:
                    cs = cslot(k, s_, n)
                    v_ = m if first else (C_v[cs, :] + m if sign > 0 else C_v[cs, :] - m)
                    if last:
                        u = emit((a0, a0, a1, a1)[k], s_ * MC, n + (k % 2) * (HN // L), v_)
                        us[k, s_, n] = True
                        v_ = u
                        if k == 3:
                            u11, u12, u21 = C_v[cslot(0, s_, n), :], C_v[cslot(1, s_, n), :], C_v[cslot(2, s_, n), :]
                            for w, c in enumerate((u11 + u, u21 + u, u11 + u12, u21 - u11, u12 - u)):
                                UL_v[pl.ds(((i % 5) * 5 + w) * P + s_ * MC, MC), n * L:(n + 1) * L] = c.astype(BF16)
                            bg.charge(U_COST)
                            continue
                    C_v[cs, :] = v_

            for j in (0, 6, 3, 4, 1, 2, 5):
                def l2(w):
                    r0 = (((i % 5) * 7 + j) * 5 + w) * MC
                    return L2_v[r0:r0 + MC, :]

                def r2(w):
                    r0 = (j * 3 + w // 2) * KQ
                    return R2_v[r0:r0 + KQ, (w % 2) * L:(w % 2 + 1) * L]

                def rq(kh, n):
                    return R_v[j * HK + kh * KQ:j * HK + (kh + 1) * KQ, n * L:(n + 1) * L]

                p1 = piece(l2(0), r2(0))
                t11 = piece(l2(4), r2(4), p1)
                p4 = piece(lhs(j, MC, slice(KQ, 2 * KQ)), r2(2))
                t11 = t11 + p4
                p5 = piece(l2(2), rq(1, 1))
                contribute(j, 0, 0, t11 - p5)
                p2 = piece(l2(1), rq(0, 0))
                contribute(j, 1, 0, p2 + p4)
                t22 = p1 - p2
                p3 = piece(lhs(j, 0, slice(0, KQ)), r2(1))
                contribute(j, 0, 1, p3 + p5)
                contribute(j, 1, 1, piece(l2(3), r2(3), t22 + p3))
                tails(every.pop(0))

        for sub in (0, MC):
            for n in (range(HN // L) if i == 0 else (2,)):
                def put(w, c):
                    UL_v[pl.ds(((i % 5) * 5 + w) * P + sub, MC), n * L:(n + 1) * L] = c.astype(BF16)

                m1 = prod(0, sub, n)
                t11 = prod(6, sub, n, m1)
                m4 = prod(3, sub, n)
                t11 = t11 + m4
                m5 = prod(4, sub, n)
                u11 = emit(a0, sub, n, t11 - m5)
                m2 = prod(1, sub, n)
                u21 = emit(a1, sub, n, m2 + m4)
                put(3, u21 - u11)
                t22 = m1 - m2
                m3 = prod(2, sub, n)
                u12 = emit(a0, sub, n + HN // L, m3 + m5)
                put(2, u11 + u12)
                u22 = emit(a1, sub, n + HN // L, prod(5, sub, n, t22 + m3))
                put(0, u11 + u22)
                put(1, u21 + u22)
                put(4, u12 - u22)
                bg.charge(U_COST)
                tails(every.pop(0))

    def debug_keep_alive():
        if _ONLY is not None:
            for r_ in (xn_u, XL_u, WB_u, UL_u, WO_u, z1_v, R_u, Lc_u, L2_u, R2_u, C_v, zf_v, zg_v, kv_u, u_u, X_v, H_v, G_v, Z_u,
                       kf_v, bcol_v):
                c_ = pltpu.make_async_copy(r_, r_, sem_small.at[0])
                c_.start()
                c_.wait()

    debug_keep_alive()

    cp_x(0).start()
    cp_win(0).start()
    cp_x(1).start()
    cp_win(1).start()
    start(cp_small())
    for c in range(2, 5):
        cp_win(c).start()
    cp_x(2).start()

    kk = _odd_freq(jax.lax.broadcasted_iota(jnp.int32, (P, P), 0))
    nn = jax.lax.broadcasted_iota(jnp.int32, (P, P), 1)
    fc, fs = _cos_sin((kk * (4 * nn - 127)) & 2047)
    for g in range(P // 8):
        F_v[g * 16:(g + 1) * 16, 0:P] = jnp.concatenate(
            [fc[g * 8:(g + 1) * 8], -fs[g * 8:(g + 1) * 8]], axis=0).astype(BF16)
    fc, fs = _cos_sin((kk * (-127)) & 2047)
    ph_v[0] = fc
    ph_v[1] = fs
    kk = _odd_freq(jax.lax.broadcasted_iota(jnp.int32, (MC, P), 1))
    mm = jax.lax.broadcasted_iota(jnp.int32, (MC, P), 0)
    ic, is_ = _cos_sin((kk * (4 * mm + 2)) & 2047)
    Fi_v[:, 0:P] = (ic * (1.0 / (P * GA))).astype(BF16)
    Fi_v[:, P:2 * P] = (is_ * (1.0 / (P * GA))).astype(BF16)
    kf_v[:, 0:8, :] = jnp.zeros((D // L, 8, L), F32)

    cp_x(0).wait()
    for s in range(TM // 16):
        ln_x(0, s)

    def small_setup():
        sk = sk_in[...].astype(F32)
        for t in range(4):
            sk_v[t] = jnp.broadcast_to(sk[t:t + 1], (8, D))
        drow = d_in[...].astype(F32).reshape(1, D)
        for l in range(D // L):
            lanes = slice(l * L, (l + 1) * L)
            dre = ph_v[0] * drow[:, lanes]
            dim = ph_v[1] * drow[:, lanes]
            H_v[0, 0, 0:64, lanes] = -dim[0:64]
            H_v[0, 0, 64:P, lanes] = dim[64:P]
            H_v[0, 1, 0:64, lanes] = -dre[0:64]
            H_v[0, 1, 64:P, lanes] = dre[64:P]

    def bcol_task(t, j, tie):
        brow = b_in[...].astype(F32).reshape(1, S)[:, j * P:(j + 1) * P] * (0.25 / GA) + tie[0:1]
        bcol_v[j * P:(j + 1) * P, :] = jnp.broadcast_to(brow, (P, P)).T

    LAG = 2

    def interleave(*lists):
        out = []
        for j in range(max(len(a) for a in lists)):
            for a in lists:
                out += a[j:j + 1]
        return out

    def p1_first(c):
        bg = _Background()
        todo = []
        if c == 2:
            todo = tasks(bcol_task, 0)
            small_setup()
        if c == 3:
            todo = tasks(ln_z2, 0)
            bg.add(wcomb_gen(range(3)))
        if c == 4:
            todo = tasks(ln_x2, 2, 8)
            bg.add(wcomb_gen(range(3, 6)))
        tied = _Tied(todo, F_TIED[c])
        if c == 0:
            for s in range(TM // 16):
                ln_x(1, s)
        for t in range(2):
            for m in range(TM // MC):
                job_z(t, m, range(*WIN_CHUNKS[c]), bg, (80, 40), tied)
        bg.drain()
        assert not tied.tasks

    for c in range(5):
        cp_win(c).wait()
        if c == 0:
            cp_x(1).wait()
        if c == 2:
            wait(cp_small())
            start(cp_conv(0))
            cp_x(3).start()
        if c == 4:
            cp_x(2).wait()
            cp_x(4).start()
        block(lambda c=c: p1_first(c), f'p1_f{c}')

    def p1_wait(g):
        if g == 0:
            wait(cp_conv(0))
            cp_x(3).wait()
        if g == 1:
            wait(cp_conv(1))
            cp_x(4).wait()
        if g == 2:
            wait(cp_conv(2))
            cp_x(6).wait()
        if g == 3:
            wait(cp_conv(4))
            cp_wout().wait()
            wait(cp_wsp(0))

    def p1_start(g):
        if g == 0:
            start(cp_conv(1))
            cp_x(6).start()
            start(cp_conv(2))
        if g == 1:
            start(cp_conv(4))
            cp_wout().start()
            start(cp_wsp(0))
            start(cp_wsp(1))
        if g == 3:
            start(cp_wsp(2))
            start(cp_conv(6))
            for i in (3, 4, 5):
                start(cp_wsp(i))

    def take(gen, n):
        for _ in range(n):
            yield next(gen)

    def p1_step(i):
        bg = _Background()
        dft = _Background()
        t = i - LAG
        xg = P1_X[i]
        kv = kv_gen(t)
        nx, nz, nh = KV_SPLIT[i]
        dft.add(take(kv, nx))
        bg.add(take(kv, nz))
        hbg = _Background()
        hbg.add(take(kv, nh))
        zb = nz * KV_COST / 48.0
        extra = 0
        if i == 6:
            bg.add(wocomb_gen())
            bg.add(acomb_gen(0, range(5)))
            extra = EXTRA[0]
        if i == 7:
            bg.add(acomb_gen(0, range(5, 8)))
            bg.add(bcomb2_gen((1, 5)))
            extra = EXTRA[1]
        last = i == NT - 1
        z2t = tasks(ln_z2, i - 1)
        xt = [tasks(ln_x2, t_, 8) for t_ in P1_LNX[i]]
        if P1_TUNE[i][1]:
            todo = interleave(*([z2t[0::2]] + xt + [z2t[1::2]]))
        else:
            todo = interleave(*(xt + [z2t[0::2], z2t[1::2]]))
        tied = _Tied(todo, P1_TUNE[i][0])
        if xg is not None:
            dft.run(KV_COST)
            job_x(xg, dft, (nx - 1) * KV_COST / 10.0)
            dft.drain()
        for p in range(2):
            for j in range(FH // L):
                job_zs(i, p, j, bg, (1.6 * zb + extra, 0.5 * zb + extra), tied)
            assert not tied.tasks or (p == 0 and not last)
            if p == 0 and last:
                tied = _Tied(tasks(ln_z2, i, 8), LAST_N)
        if last:
            for s in range(8, 16):
                ln_z2(i, s)
        bg.drain()
        job_h(t, hbg, nh * KV_COST / 10.0)
        hbg.drain()

    def p1_block(g):
        for i in P1_GROUPS[g]:
            p1_step(i)

    for g in range(len(P1_GROUPS)):
        p1_wait(g)
        p1_start(g)
        block(lambda g=g: p1_block(g), f'p1_g{g}')

    groups = P2_GROUPS
    NG = len(groups)

    def p2_dma(gi):
        if gi >= 2:
            for i in groups[gi - 2]:
                start(cp_out(i))
        if gi >= 3:
            for i in groups[gi - 3]:
                wait(cp_out(i))
        if gi == 1:
            for i in (6, 7):
                start(cp_wsp(i))
        if gi == 0:
            wait(cp_conv(6))
        if gi + 1 < NG:
            for i in groups[gi + 1]:
                wait(cp_wsp(i))

    def tails_of(i, bg, budget):
        return [tail_gen(i, bg, budget)] * 20

    def p2_block(gi):
        bg = _Background()
        steps = groups[gi]
        tb = [0.0]
        pending = [t_ for i in (groups[gi - 1] if gi > 0 else []) for t_ in tails_of(i, bg, tb)]
        total = sum(a + 1 for i in steps for a in _blocks_of_step(i)) * 40 * 16
        total += len(steps) * (24 * E_COST + 6 * U_COST) + len(pending) * T_COST
        slots = sum(84 if i == 0 else 77 for i in steps) + TAIL_W * len(pending)
        bg.add(freq_gen(_blocks_of_step(steps[0])[0]))
        if gi == 0:
            bg.add(bcomb2_gen((0, 2, 3, 4, 6)))
            total += 5 * 16 * A_COST
        if gi < 2:
            bg.add(kv_gen(NT - 2 + gi))
            total += 20 * KV_COST
            slots += 10
        for t in P2_X[gi]:
            slots += 10
        if gi + 1 < NG:
            for i in groups[gi + 1]:
                bg.add(acomb2_gen(i))
                total += 16 * 7 * A2_COST
        for i in steps[1:]:
            bg.add(freq_gen(_blocks_of_step(i)[0]))
        budget = tb[0] = total / (slots + P2_END[gi])
        bg.run(budget)
        for t in P2_X[gi]:
            job_x(t, bg, budget)
        if gi < 2:
            job_h(NT - 2 + gi, bg, budget)
        units = [4, 4, 2, 4, 4, 2] * (len(pending) // 20)
        every = [0] * sum(6 if i == 0 else 9 for i in steps)
        for j, n in enumerate(units):
            every[min(len(every) - 1, j * len(every) // len(units))] += n
        for i in steps:
            job_big(i, bg, pending, budget, every)
        for t_ in pending:
            next(t_)
        bg.drain()

    for gi in range(NG):
        p2_dma(gi)
        block(lambda gi=gi: p2_block(gi), f'p2_{gi}')

    def cp_last(part):
        a0 = _blocks_of_step(NT - 1)[0]
        sub, cols = ((MC, pl.ds(0, D)), (0, pl.ds(0, 4 * L)), (0, pl.ds(4 * L, L)))[part]
        return [pltpu.make_async_copy(o_v.at[pl.ds(r, MC), cols], o_hbm.at[0, pl.ds(r, MC), cols],
                                      sem_out.at[NT - 1]) for r in (a0 * P + sub, (a0 + 1) * P + sub)]

    def p2_last():
        for i in groups[NG - 1]:
            for j, t_ in enumerate(tails_of(i, _Background(), [0.0])):
                next(t_)
                if i < NT - 1 and j == 19:
                    start(cp_out(i))
                if i == NT - 1 and j in (9, 17):
                    start(cp_last(j // 10))

    p2_dma(NG)
    block(p2_last, 'p2_last')
    start(cp_last(2))
    for i in groups[NG - 2] + groups[NG - 1][:-1]:
        wait(cp_out(i))
    for part in range(3):
        wait(cp_last(part))
    debug_keep_alive()


def _compiler_params():
    vmem = 124 * 1024 * 1024
    try:
        return pltpu.CompilerParams(vmem_limit_bytes=vmem, disable_semaphore_checks=True)
    except TypeError:
        return pltpu.CompilerParams(vmem_limit_bytes=vmem)


@jax.jit
def pallas_recurrent_scan__ssm_conv_h3__mixer_gmlp__prompt_kernel(
    A_q: jax.Array,
    A_k: jax.Array,
    A_v: jax.Array,
    A_shift_k: jax.Array,
    A_ssm_k: jax.Array,
    A_ssm_D: jax.Array,
    B_x: jax.Array,
    B_w_in: jax.Array,
    B_w_sp: jax.Array,
    B_b_sp: jax.Array,
    B_w_out: jax.Array,
):
    del B_x
    hbm = pl.BlockSpec(memory_space=pl.ANY)

    def bf16_buf(*shape):
        return pltpu.VMEM(shape[:-2] + (shape[-2] // 2, shape[-1]), U32)

    return pl.pallas_call(
        _kernel,
        out_shape=jax.ShapeDtypeStruct((1, S, D), BF16),
        in_specs=[hbm] * 10,
        out_specs=hbm,
        scratch_shapes=[
            [bf16_buf(len(g) * TM, D) for g in X_DMAS],
            [bf16_buf(len(g) * TM, D) for g in CONV_DMAS],
            [bf16_buf(len(g) * TM, D) for g in CONV_DMAS],
            [bf16_buf(D, len(g) * TM) for g in CONV_DMAS],
            [bf16_buf(D, max(hi - lo, 2) * L) for lo, hi in WIN_CHUNKS],
            [bf16_buf(TM, S) for _ in range(NT)],
            bf16_buf(FH, D),
            pltpu.VMEM((S, D), BF16),
            pltpu.VMEM((4, D), BF16),
            pltpu.VMEM((D,), BF16),
            pltpu.VMEM((S,), BF16),
            bf16_buf(S, D),
            bf16_buf(4 * 5 * P, KH),
            bf16_buf(5 * KH, FH),
            bf16_buf(5 * 5 * P, HN),
            bf16_buf(5 * HN, 2 * L),
            pltpu.VMEM((S, FH), F32),
            bf16_buf(7 * HK, HN),
            bf16_buf(5 * 5 * P, HK),
            bf16_buf(5 * 35 * MC, KQ),
            bf16_buf(21 * KQ, 2 * L),
            pltpu.VMEM((16 * MC, L), F32),
            pltpu.VMEM((HK, FH), F32),
            pltpu.VMEM((3, TM, FH), F32),
            bf16_buf(S, D),
            bf16_buf(S, FH),
            pltpu.VMEM((NB, 2, P, D), F32),
            pltpu.VMEM((2, 2, P, D), F32),
            pltpu.VMEM((NB, 2, P, D), F32),
            bf16_buf(NB * 2 * P, D),
            pltpu.VMEM((2, D // L, MC, L), F32),
            bf16_buf(2 * P, 2 * P),
            bf16_buf(MC, 2 * P),
            pltpu.VMEM((S, L), F32),
            pltpu.VMEM((2, P, L), F32),
            pltpu.VMEM((4, 8, D), F32),
            pltpu.VMEM((D // L, S + 8, L), F32),
            pltpu.SemaphoreType.DMA((1,)),
            pltpu.SemaphoreType.DMA((NT,)),
            pltpu.SemaphoreType.DMA((NT,)),
            pltpu.SemaphoreType.DMA((NT,)),
            pltpu.SemaphoreType.DMA((5,)),
            pltpu.SemaphoreType.DMA((NT,)),
        ],
        compiler_params=_compiler_params(),
    )(A_q, A_k, A_v, A_shift_k.T, A_ssm_k, A_ssm_D, B_w_in, B_w_sp, B_b_sp, B_w_out)
```

```python
import math

import jax
import jax.numpy as jnp
import jax.experimental.pallas as pl
import jax.experimental.pallas.tpu as pltpu

S = 2048
D = 640
FH = 768
P = 128
NB = S // P
TM = 256
NT = S // TM
MC = 64
L = 128
HK = S // 2
KQ = 512
A2_COST = 34
FR = 8
L2_ORDER = 1
TAIL_EAGER = True
A2_ORDER = (2, 0, 3, 1, 5, 4, 6)
L1_USE = {0: ((0, 1, True, False), (3, 1, True, False)), 6: ((0, 1, False, False),), 3: ((0, 1, False, False), (2, 1, True, False)),
          4: ((0, -1, False, True), (1, 1, True, False)), 1: ((2, 1, False, True), (3, -1, False, False)),
          2: ((1, 1, False, True), (3, 1, False, False)), 5: ((3, 1, False, True),)}
KH = 256
HN = FH // 2
EPS = 1e-5
F32 = jnp.float32
BF16 = jnp.bfloat16
U32 = jnp.uint32
GELU_C = math.sqrt(2.0 / math.pi)
GA = (GELU_C * 0.044715) ** (1.0 / 3.0)
NT_DIMS = (((1,), (1,)), ((), ()))

WIN_CHUNKS = ((6, 7), (7, 9), (9, 12), (0, 3), (3, 6))
X_DMAS = ((0,), (1,), (2,), (3,), (4, 5), (6, 7))
CONV_DMAS = ((0,), (1,), (2, 3), (4, 5), (6, 7))
P1_GROUPS = ((2,), (3,), (4, 5), (6, 7))
P1_X = {2: None, 3: 0, 4: 1, 5: None, 6: 2, 7: 3}
P1_LNX = {2: (3,), 3: (4, 5), 4: (6,), 5: (7,), 6: (), 7: ()}
P2_GROUPS = ((0,), (1, 2), (3, 4, 5), (6, 7))
P2_X = ((4, 5), (6,), (7,), ())
STEP_BLOCKS = ((2, 3), (6, 7), (4, 5), (12, 13), (10, 11), (0, 1), (14, 15), (8, 9))
KV_COST, A_COST = 110, 56
E_COST, U_COST, T_COST, TAIL_W = 24, 90, 90, 1.6
KV_SPLIT = {2: (0, 14, 6), 3: (12, 4, 4), 4: (12, 4, 4), 5: (0, 14, 6), 6: (12, 4, 4), 7: (12, 4, 4)}
H_SPLIT = ((0, 2), (2, 4), (4, 5))
P1_TUNE = {2: (42, 0), 3: (43, 1), 4: (42, 0), 5: (42, 0), 6: (44, 0), 7: (24, 0)}
EXTRA = (52, 52)
LAST_N = 22
P2_END = (0.0, -1.0, -1.0, 0.0)
F_TIED = (20, 20, 18, 20, 20)
_ONLY = None


def _dot(a, b):
    return jnp.dot(a, b, preferred_element_type=F32)


def _cos_sin(m):
    q = (m + 256) >> 9
    x = (m - (q << 9)).astype(F32) * (2.0 * math.pi / 2048.0)
    x2 = x * x
    s = x * (1.0 + x2 * (-1.0 / 6 + x2 * (1.0 / 120 + x2 * (-1.0 / 5040 + x2 * (1.0 / 362880)))))
    c = 1.0 + x2 * (-0.5 + x2 * (1.0 / 24 + x2 * (-1.0 / 720 + x2 * (1.0 / 40320 - x2 * (1.0 / 3628800)))))
    swap = (q & 1) == 1
    c0 = jnp.where(swap, s, c)
    s0 = jnp.where(swap, c, s)
    cos = jnp.where(((q + 1) & 2) == 2, -c0, c0)
    sin = jnp.where((q & 2) == 2, -s0, s0)
    return cos, sin


def _odd_freq(r):
    return jnp.where(r < 64, 4 * r + 1, 4 * r - 253)


def _gelu_scaled(z):
    return z + z * jnp.tanh(z * (GELU_C / GA + z * z))


def _signzero(z):
    bits = jax.lax.bitcast_convert_type(z, U32) & jnp.uint32(0x80000000)
    return jax.lax.bitcast_convert_type(bits, F32)


def _ln(x, eps, tie=None, scale=None):
    n = x.shape[-1]
    cols = [x[:, j * L:(j + 1) * L] for j in range(n // L)]
    s1 = cols[0]
    s2 = cols[0] * cols[0]
    for c in cols[1:]:
        s1 = s1 + c
        s2 = s2 + c * c
    if tie is not None:
        s1 = s1 + tie
        s2 = s2 + tie
    m = jnp.sum(s1, axis=-1, keepdims=True) * (1.0 / n)
    v = jnp.maximum(jnp.sum(s2, axis=-1, keepdims=True) * (1.0 / n) - m * m, 0.0)
    rs = jax.lax.rsqrt(v + eps)
    if scale is not None:
        rs = rs * scale
    return (x - m) * rs


def _blocks_of_step(i):
    return STEP_BLOCKS[i]


class _Background:
    def __init__(self):
        self.q = []
        self.credit = 0.0

    def add(self, gen):
        self.q.append(gen)

    def run(self, budget):
        self.credit += budget
        while self.q and self.credit > 0:
            try:
                self.credit -= next(self.q[0])
            except StopIteration:
                self.q.pop(0)
        if not self.q:
            self.credit = 0.0

    def charge(self, cost):
        self.credit -= cost

    def drain(self):
        while self.q:
            self.run(1e9)


class _Tied:
    def __init__(self, tasks, npieces):
        self.tasks = list(tasks)
        self.rate = len(self.tasks) / float(npieces)
        self.credit = 0.999

    def run(self, z):
        self.credit += self.rate
        n = 0
        while self.tasks and self.credit >= 1.0:
            self.tasks.pop(0)(_signzero(z[0:16]))
            self.credit -= 1.0
            n += 1
        return n


def _kernel(q_hbm, k_hbm, v_hbm, sk_hbm, h_hbm, d_hbm, win_hbm, wsp_hbm, b_hbm, wout_hbm,
            o_hbm,
            x_us, k_us, v_us, h_us, win_us, wsp_us, wout_u, o_v, sk_in, d_in, b_in,
            xn_u, XL_u, WB_u, UL_u, WO_u, z1_v, R_u, Lc_u, L2_u, R2_u, C_v, zf_v, zg_v, kv_u, u_u, X_v, H_v, G_v, Z_u,
            yl_v, F_u, Fi_u, bcol_v, ph_v, sk_v, kf_v,
            sem_small, sem_x, sem_conv, sem_wsp, sem_w, sem_out):
    (wout_v, xn_v, XL_v, WB_v, UL_v, WO_v, R_v, Lc_v, L2_v, R2_v, kv_v, u_v, Z_v, F_v, Fi_v) = [
        r.bitcast(BF16) for r in (wout_u, xn_u, XL_u, WB_u, UL_u, WO_u, R_u, Lc_u, L2_u, R2_u, kv_u, u_u, Z_u, F_u, Fi_u)]
    x_vs = {g[0]: r.bitcast(BF16) for g, r in zip(X_DMAS, x_us)}
    k_vs, v_vs, h_vs = [{g[0]: r.bitcast(BF16) for g, r in zip(CONV_DMAS, rs)} for rs in (k_us, v_us, h_us)]
    wsp_vs = [r.bitcast(BF16) for r in wsp_us]
    win_vs = [r.bitcast(BF16) for r in win_us]

    def win(rows, n):
        c = [lo <= n < hi for lo, hi in WIN_CHUNKS].index(True)
        n -= WIN_CHUNKS[c][0]
        return win_vs[c][rows, n * L:(n + 1) * L]

    def locate(bufs, row):
        t0 = max(t for t in bufs if t * TM <= row)
        return bufs[t0], row - t0 * TM

    def rows_of(bufs, row, n, lanes=slice(None)):
        buf, r = locate(bufs, row)
        return buf[r:r + n, lanes]

    def cp_small():
        return [pltpu.make_async_copy(s_, d_, sem_small.at[0])
                for s_, d_ in ((d_hbm, d_in), (sk_hbm, sk_in), (b_hbm, b_in))]

    def cp_x(t):
        return pltpu.make_async_copy(q_hbm.at[0, pl.ds(t * TM, x_vs[t].shape[0])], x_vs[t], sem_x.at[t])

    def cp_conv(t):
        rows = pl.ds(t * TM, k_vs[t].shape[0])
        sem = sem_conv.at[t]
        return [pltpu.make_async_copy(h_hbm.at[:, rows], h_vs[t], sem),
                pltpu.make_async_copy(k_hbm.at[0, rows], k_vs[t], sem),
                pltpu.make_async_copy(v_hbm.at[0, rows], v_vs[t], sem)]

    def cp_wsp(i):
        return [pltpu.make_async_copy(wsp_hbm.at[pl.ds(_blocks_of_step(i)[0] * P, TM)], wsp_vs[i], sem_wsp.at[i])]

    def cp_win(c):
        lo, hi = WIN_CHUNKS[c]
        w = (hi - lo) * L
        return pltpu.make_async_copy(win_hbm.at[:, pl.ds(lo * L, w)], win_vs[c].at[:, pl.ds(0, w)], sem_w.at[c])

    def cp_wout():
        return pltpu.make_async_copy(wout_hbm, wout_v, sem_w.at[0])

    def cp_out(i):
        rows = pl.ds(_blocks_of_step(i)[0] * P, TM)
        return [pltpu.make_async_copy(o_v.at[rows], o_hbm.at[0, rows], sem_out.at[i])]

    def start(cs):
        for c in cs:
            c.start()

    def wait(cs):
        for c in cs:
            c.wait()

    def block(fn, name):
        def body(it):
            fn()
            return it + 1

        if _ONLY is None or name in _ONLY:
            jax.lax.while_loop(lambda it: it < 1, body, jnp.int32(0))

    def ln_x(t, s, tie=None):
        rows = pl.ds(t * TM + s * 16, 16)
        y = _ln(rows_of(x_vs, t * TM + s * 16, 16).astype(F32), EPS, tie, GA)
        xn_v[rows, :] = y.astype(BF16)
        return y

    def ln_x2(t, s, tie):
        p, q = s // 4, s % 4
        y1 = ln_x(t, 8 * p + q, tie)
        y2 = ln_x(t, 8 * p + 4 + q, tie)
        a11, a12, a21, a22 = y1[:, :KH], y1[:, KH:2 * KH], y2[:, :KH], y2[:, KH:2 * KH]
        r0 = (t % 4) * 5 * P + p * MC + q * 16
        for j, c in enumerate((a11 + a22, a21 + a22, a11 + a12, a21 - a11, a12 - a22)):
            XL_v[pl.ds(r0 + j * P, 16), :] = c.astype(BF16)

    def wcomb_gen(cols):
        for j in cols:
            c1 = slice(j * L, (j + 1) * L)
            for r in range(KH // 32):
                top = pl.ds(r * 32, 32)
                bot = pl.ds(KH + r * 32, 32)
                b11, b12 = win(top, j).astype(F32), win(top, 6 + j).astype(F32)
                b21, b22 = win(bot, j).astype(F32), win(bot, 6 + j).astype(F32)
                for w, c in enumerate((b11 + b22, b12 - b22, b21 - b11, b11 + b12, b21 + b22)):
                    WB_v[pl.ds(w * KH + r * 32, 32), c1] = c.astype(BF16)
                yield A_COST

    def ln_z2(t, s, tie=None):
        y = _ln(zg_v[t % 3, s * 16:(s + 1) * 16, :], 4.0 * GA * GA * EPS, tie, 0.25 / GA)
        lo, hi = y[:, :HN], y[:, HN:]
        r = (t * TM + s * 16) % HK
        rows = pl.ds(r, 16)
        if t < NT // 2:
            zf_v[rows, :] = y
            R_v[pl.ds(1 * HK + r, 16), :] = lo.astype(BF16)
            R_v[pl.ds(5 * HK + r, 16), :] = (lo + hi).astype(BF16)
        else:
            b11, b12 = zf_v[rows, :HN], zf_v[rows, HN:]
            R_v[pl.ds(0 * HK + r, 16), :] = (b11 + hi).astype(BF16)
            R_v[pl.ds(2 * HK + r, 16), :] = (b12 - hi).astype(BF16)
            R_v[pl.ds(3 * HK + r, 16), :] = (lo - b11).astype(BF16)
            R_v[pl.ds(4 * HK + r, 16), :] = hi.astype(BF16)
            R_v[pl.ds(6 * HK + r, 16), :] = (lo + hi).astype(BF16)

    def acomb_gen(i, groups=range(P // 16)):
        for r in groups:
            for c in range(HK // 256):
                top = pl.ds(r * 16, 16)
                bot = pl.ds(P + r * 16, 16)
                c1 = slice(c * 256, (c + 1) * 256)
                c2 = slice(HK + c * 256, HK + (c + 1) * 256)
                a11 = wsp_vs[i][top, c1].astype(F32)
                a12 = wsp_vs[i][top, c2].astype(F32)
                a21 = wsp_vs[i][bot, c1].astype(F32)
                a22 = wsp_vs[i][bot, c2].astype(F32)
                r0 = (i % 5) * 5 * P + r * 16
                Lc_v[pl.ds(r0 + 0 * P, 16), c1] = (a11 + a22).astype(BF16)
                Lc_v[pl.ds(r0 + 1 * P, 16), c1] = (a21 + a22).astype(BF16)
                Lc_v[pl.ds(r0 + 2 * P, 16), c1] = (a11 + a12).astype(BF16)
                Lc_v[pl.ds(r0 + 3 * P, 16), c1] = (a21 - a11).astype(BF16)
                Lc_v[pl.ds(r0 + 4 * P, 16), c1] = (a12 - a22).astype(BF16)
                yield A_COST

    def acomb2_gen(i):
        for r in range(MC // 16):
            for c in range(KQ // L):
                quad = {}

                def w(b, H):
                    if (b, H) not in quad:
                        quad[b, H] = [[wsp_vs[i][pl.ds(b * P + s_ * MC + r * 16, 16),
                                                 H * HK + kh * KQ + c * L:H * HK + kh * KQ + (c + 1) * L].astype(F32)
                                       for kh in range(2)] for s_ in range(2)]
                    return quad[b, H]

                spec = {2: (None, (0, 0), None, 0), 0: (0, (0, 0), (1, 1), 1), 3: (None, (1, 1), None, 0),
                        1: (1, (1, 0), (1, 1), 1), 5: (3, (1, 0), (0, 0), -1), 4: (2, (0, 0), (0, 1), 1),
                        6: (4, (0, 1), (1, 1), -1)}
                for j in A2_ORDER:
                    slot, p_, q_, sign = spec[j]
                    a = w(*p_)
                    if q_ is not None:
                        b_ = w(*q_)
                        a = [[a[s_][kh] + b_[s_][kh] if sign > 0 else a[s_][kh] - b_[s_][kh] for kh in range(2)]
                             for s_ in range(2)]
                        for s_ in range(2):
                            for kh in range(2):
                                Lc_v[pl.ds(((i % 5) * 5 + slot) * P + s_ * MC + r * 16, 16),
                                     kh * KQ + c * L:kh * KQ + (c + 1) * L] = a[s_][kh].astype(BF16)
                    for w2, v_ in enumerate((a[0][0] + a[1][1], a[1][0] + a[1][1], a[0][0] + a[0][1],
                                             a[1][0] - a[0][0], a[0][1] - a[1][1])):
                        L2_v[pl.ds((((i % 5) * 7 + j) * 5 + w2) * MC + r * 16, 16), c * L:(c + 1) * L] = v_.astype(BF16)
                    yield A2_COST

    def bcomb2_gen(js):
        for j in js:
            for r in range(KQ // 32):
                top = pl.ds(j * HK + r * 32, 32)
                bot = pl.ds(j * HK + KQ + r * 32, 32)
                b11, b12 = R_v[top, 0:L].astype(F32), R_v[top, L:2 * L].astype(F32)
                b21, b22 = R_v[bot, 0:L].astype(F32), R_v[bot, L:2 * L].astype(F32)
                for w, c in enumerate((b11 + b22, b12 - b22, b21 - b11, b11 + b12, b21 + b22)):
                    R2_v[pl.ds((j * 3 + w // 2) * KQ + r * 32, 32), (w % 2) * L:(w % 2 + 1) * L] = c.astype(BF16)
                yield A_COST

    def tasks(fn, t, n=TM // 16):
        return [lambda tie, s=s: fn(t, s, tie) for s in range(n)]

    def kv_gen(t):
        for m in range(TM // MC):
            r = t * TM + m * MC
            for l in range(D // L):
                lanes = slice(l * L, (l + 1) * L)
                kf = rows_of(k_vs, r, MC, lanes).astype(F32)
                kf_v[l, pl.ds(r + 8, MC), :] = kf
                ks = kf * sk_v[0, 0:1, lanes]
                for tap in range(1, 4):
                    ks = ks + kf_v[l, pl.ds(r + 8 - tap, MC), :] * sk_v[tap, 0:1, lanes]
                kv = ks * rows_of(v_vs, r, MC, lanes).astype(F32)
                kv_v[pl.ds(r, MC), lanes] = kv.astype(BF16)
                yield KV_COST

    def freq_gen(a):
        def cmac(acc, x, g):
            pr = x[0] * g[0] - x[1] * g[1]
            pi = x[0] * g[1] + x[1] * g[0]
            return (pr, pi) if acc is None else (acc[0] + pr, acc[1] + pi)

        for r in range(P // 16):
            for l in range(D // L):
                lanes = slice(l * L, (l + 1) * L)
                res = []
                for sub in range(16 // FR):
                    rows = pl.ds(r * 16 + sub * FR, FR)
                    lo = hi = None
                    g = (G_v[a + 1, 0, rows, lanes], G_v[a + 1, 1, rows, lanes])
                    for c in range(a + 2):
                        x = (X_v[c, 0, rows, lanes], X_v[c, 1, rows, lanes])
                        hi = cmac(hi, x, g)
                        if c <= a:
                            g = (G_v[a - c, 0, rows, lanes], G_v[a - c, 1, rows, lanes])
                            lo = cmac(lo, x, g)
                            yield 2 * FR
                    res.append((lo, hi))
                for w in range(2):
                    for part in range(2):
                        Z_v[pl.ds((a + w) * 2 * P + part * P + r * 16, 16), lanes] = jnp.concatenate(
                            [z[w][part] for z in res], axis=0).astype(BF16)
                yield 20

    def job_x(t, bg, budget):
        for j in (2 * t, 2 * t + 1):
            for half in range(2):
                r = _dot(F_v[half * P:(half + 1) * P, 0:P], kv_v[j * P:(j + 1) * P, :]).reshape(8, 2, 8, D)
                for part in range(2):
                    X_v[j, part, half * 64:(half + 1) * 64, :] = r[:, part].reshape(64, D)
                bg.run(budget * 2.5)

    def job_h(t, bg, budget):
        h_v, c0 = locate(h_vs, t * TM)
        for half in range(2):
            rows = pl.ds(half * 64, 64)
            for l0, l1 in H_SPLIT:
                w = (l1 - l0) * L
                lanes = slice(l0 * L, l1 * L)
                rhs = jnp.concatenate([h_v[lanes, c0:c0 + P], h_v[lanes, c0 + P:c0 + TM]], axis=0)
                r = jax.lax.dot_general(F_v[half * P:(half + 1) * P, 0:P], rhs, NT_DIMS,
                                        preferred_element_type=F32).reshape(8, 2, 8, 2 * w)
                re, im = r[:, 0].reshape(64, 2 * w), r[:, 1].reshape(64, 2 * w)
                prev = (H_v[t % 2, 0, rows, lanes], H_v[t % 2, 1, rows, lanes])
                for j in range(2):
                    cur = (re[:, j * w:(j + 1) * w], im[:, j * w:(j + 1) * w])
                    G_v[2 * t + j, 0, rows, lanes] = cur[0] + prev[1] if half else cur[0] - prev[1]
                    G_v[2 * t + j, 1, rows, lanes] = cur[1] - prev[0] if half else cur[1] + prev[0]
                    prev = cur
                if t + 1 < NT:
                    H_v[(t + 1) % 2, 0, rows, lanes] = prev[0]
                    H_v[(t + 1) % 2, 1, rows, lanes] = prev[1]
                bg.run(budget * (l1 - l0))

    def z_out(t, m, n, pre, bg, budget, tied):
        z = _gelu_scaled(pre)
        if n < FH // L:
            z1_v[pl.ds(t * TM + m * MC, MC), n * L:(n + 1) * L] = z
        else:
            zg_v[t % 3, m * MC:(m + 1) * MC, n * L - FH:(n + 1) * L - FH] = z
        ntask = tied.run(z)
        bg.run(budget[1] if ntask else budget[0])

    def job_z(t, m, cols, bg, budget, tied):
        for n in cols:
            z_out(t, m, n, _dot(xn_v[pl.ds(t * TM + m * MC, MC), :], win(slice(None), n)), bg, budget, tied)

    def job_zs(t, p, j, bg, budget, tied):
        r1 = pl.ds(t * TM + p * P, MC)
        r2 = pl.ds(t * TM + p * P + MC, MC)
        c1 = slice(j * L, (j + 1) * L)

        def xl(w):
            r0 = (t % 4) * 5 * P + w * P + p * MC
            return XL_v[r0:r0 + MC, :]

        def wb(w):
            return WB_v[w * KH:(w + 1) * KH, c1]

        def rem(rows, n):
            return _dot(xn_v[rows, 2 * KH:], win(slice(2 * KH, D), n))

        m2 = _dot(xl(1), win(slice(0, KH), j))
        m4 = _dot(xn_v[r2, KH:2 * KH], wb(2))
        z_out(t, 2 * p + 1, j, m2 + m4 + rem(r2, j), bg, budget, tied)
        m3 = _dot(xn_v[r1, 0:KH], wb(1))
        m5 = _dot(xl(2), win(slice(KH, 2 * KH), 6 + j))
        z_out(t, 2 * p, 6 + j, m3 + m5 + rem(r1, 6 + j), bg, budget, tied)
        t11, t22 = m4 - m5, m3 - m2
        m1 = _dot(xl(0), wb(0))
        t11, t22 = t11 + m1, t22 + m1
        z_out(t, 2 * p, j, t11 + _dot(xl(4), wb(4)) + rem(r1, j), bg, budget, tied)
        z_out(t, 2 * p + 1, 6 + j, t22 + _dot(xl(3), wb(3)) + rem(r2, 6 + j), bg, budget, tied)

    rev8 = 7 - jax.lax.broadcasted_iota(jnp.int32, (8, L), 0)

    def finish(a, upper, n, hh, slot):
        rows = pl.ds(a * P + (MC if upper else 0), MC)
        lanes = slice(n * L, (n + 1) * L)
        if upper:
            ya = _dot(Fi_v[:, 0:P], Z_v[a * 2 * P:a * 2 * P + P, lanes])
            yb = _dot(Fi_v[:, P:2 * P], Z_v[a * 2 * P + P:(a + 1) * 2 * P, lanes])
            slot(0.5)
            y = ya - yb
            lo = ya + yb
            for j in range(MC // 8):
                yl_v[a % 2, n, (7 - j) * 8:(8 - j) * 8, :] = jnp.take_along_axis(lo[j * 8:(j + 1) * 8], rev8, axis=0)
        else:
            y = yl_v[a % 2, n]
        gate = hh + hh * jnp.tanh(hh)
        s = xn_v[rows, lanes].astype(F32) * y
        x = rows_of(x_vs, a * P + (MC if upper else 0), MC, lanes).astype(F32)
        o_v[rows, lanes] = (x + s * gate).astype(BF16)

    def tail_gen(i, bg, budget):
        a0, a1 = _blocks_of_step(i)

        def slot(w):
            bg.run(w * budget[0])

        def dot3(a, b):
            r = _dot(a, b)
            slot(0.75)
            return r

        for upper in (True, False):
            sub = MC if upper else 0
            r1 = pl.ds(a0 * P + sub, MC)
            r2 = pl.ds(a1 * P + sub, MC)

            def ul(w):
                r0 = ((i % 5) * 5 + w) * P + sub
                return UL_v[r0:r0 + MC, :]

            for j in range(2):
                c1 = slice(j * L, (j + 1) * L)
                c2 = slice((2 + j) * L, (3 + j) * L)

                def wo(w):
                    return WO_v[w * HN:(w + 1) * HN, c1]

                m2 = dot3(ul(1), wout_v[0:HN, c1])
                m4 = dot3(u_v[r2, HN:], wo(2))
                finish(a1, upper, j, m2 + m4, slot)
                bg.charge(T_COST)
                yield
                m3 = dot3(u_v[r1, 0:HN], wo(1))
                m5 = dot3(ul(2), wout_v[HN:, c2])
                finish(a0, upper, 2 + j, m3 + m5, slot)
                bg.charge(T_COST)
                yield
                if TAIL_EAGER:
                    t11, t22 = m4 - m5, m3 - m2
                m1 = dot3(ul(0), wo(0))
                if TAIL_EAGER:
                    t11, t22 = t11 + m1, t22 + m1
                else:
                    t11, t22 = (m4 - m5) + m1, None
                finish(a0, upper, j, t11 + dot3(ul(4), wo(4)), slot)
                bg.charge(T_COST)
                yield
                if not TAIL_EAGER:
                    t22 = (m3 - m2) + m1
                finish(a1, upper, 2 + j, t22 + dot3(ul(3), wo(3)), slot)
                bg.charge(T_COST)
                yield
            for a, r in ((a0, r1), (a1, r2)):
                finish(a, upper, 4, dot3(u_v[r, 0:HN], wout_v[0:HN, 4 * L:]) + dot3(u_v[r, HN:], wout_v[HN:, 4 * L:]),
                       slot)
                bg.charge(T_COST)
                yield

    def wocomb_gen():
        for j in range(2):
            c1 = slice(j * L, (j + 1) * L)
            c2 = slice((2 + j) * L, (3 + j) * L)
            for r in range(HN // 32):
                top = pl.ds(r * 32, 32)
                bot = pl.ds(HN + r * 32, 32)
                b11, b12 = wout_v[top, c1].astype(F32), wout_v[top, c2].astype(F32)
                b21, b22 = wout_v[bot, c1].astype(F32), wout_v[bot, c2].astype(F32)
                for w, c in enumerate((b11 + b22, b12 - b22, b21 - b11, b11 + b12, b21 + b22)):
                    WO_v[pl.ds(w * HN + r * 32, 32), c1] = c.astype(BF16)
                yield A_COST

    def job_big(i, bg, pending, budget, every):
        a0, a1 = _blocks_of_step(i)
        KG = 512

        def lhs(j, sub, cols):
            if j == 2:
                return wsp_vs[i][sub:sub + MC, cols]
            if j == 3:
                return wsp_vs[i][P + sub:P + sub + MC, HK + cols.start:HK + cols.stop]
            r0 = ((i % 5) * 5 + {0: 0, 1: 1, 4: 2, 5: 3, 6: 4}[j]) * P + sub
            return Lc_v[r0:r0 + MC, cols]

        def prod(j, sub, n, acc=None):
            for kg in range(HK // KG):
                ks = slice(kg * KG, (kg + 1) * KG)
                p = _dot(lhs(j, sub, ks), R_v[j * HK + kg * KG:j * HK + (kg + 1) * KG, n * L:(n + 1) * L])
                acc = p if acc is None else acc + p
                bg.run(budget)
            return acc

        def tails(n):
            for _ in range(n):
                if pending:
                    next(pending.pop(0))

        def emit(a, sub, n, g):
            rows = pl.ds(a * P + sub, MC)
            lanes = slice(n * L, (n + 1) * L)
            u = z1_v[rows, lanes] * (g + bcol_v[rows, :])
            u_v[rows, lanes] = u.astype(BF16)
            bg.charge(E_COST)
            return u

        if i > 0:
            def piece(a, b, acc=None):
                p = _dot(a, b)
                bg.run(budget)
                return p if acc is None else acc + p

            def cslot(k, s_, n):
                return pl.ds(((k * 2 + s_) * 2 + n) * MC, MC)

            us = {}

            def contribute(j, s_, n, m):
                for k, sign, first, last in L1_USE[j]:
                    cs = cslot(k, s_, n)
                    v_ = m if first else (C_v[cs, :] + m if sign > 0 else C_v[cs, :] - m)
                    if last:
                        u = emit((a0, a0, a1, a1)[k], s_ * MC, n + (k % 2) * (HN // L), v_)
                        us[k, s_, n] = True
                        v_ = u
                        if k == 3:
                            u11, u12, u21 = C_v[cslot(0, s_, n), :], C_v[cslot(1, s_, n), :], C_v[cslot(2, s_, n), :]
                            for w, c in enumerate((u11 + u, u21 + u, u11 + u12, u21 - u11, u12 - u)):
                                UL_v[pl.ds(((i % 5) * 5 + w) * P + s_ * MC, MC), n * L:(n + 1) * L] = c.astype(BF16)
                            bg.charge(U_COST)
                            continue
                    C_v[cs, :] = v_

            for j in (0, 6, 3, 4, 1, 2, 5):
                def l2(w):
                    r0 = (((i % 5) * 7 + j) * 5 + w) * MC
                    return L2_v[r0:r0 + MC, :]

                def r2(w):
                    r0 = (j * 3 + w // 2) * KQ
                    return R2_v[r0:r0 + KQ, (w % 2) * L:(w % 2 + 1) * L]

                def rq(kh, n):
                    return R_v[j * HK + kh * KQ:j * HK + (kh + 1) * KQ, n * L:(n + 1) * L]

                if L2_ORDER == 0:
                    p1 = piece(l2(0), r2(0))
                    t11 = piece(l2(4), r2(4), p1)
                    p4 = piece(lhs(j, MC, slice(KQ, 2 * KQ)), r2(2))
                    t11 = t11 + p4
                    p5 = piece(l2(2), rq(1, 1))
                    contribute(j, 0, 0, t11 - p5)
                    p2 = piece(l2(1), rq(0, 0))
                    contribute(j, 1, 0, p2 + p4)
                    t22 = p1 - p2
                    p3 = piece(lhs(j, 0, slice(0, KQ)), r2(1))
                    contribute(j, 0, 1, p3 + p5)
                    contribute(j, 1, 1, piece(l2(3), r2(3), t22 + p3))
                else:
                    p2 = piece(l2(1), rq(0, 0))
                    p4 = piece(lhs(j, MC, slice(KQ, 2 * KQ)), r2(2))
                    contribute(j, 1, 0, p2 + p4)
                    p3 = piece(lhs(j, 0, slice(0, KQ)), r2(1))
                    t22 = p3 - p2
                    p5 = piece(l2(2), rq(1, 1))
                    contribute(j, 0, 1, p3 + p5)
                    t11 = p4 - p5
                    p1 = piece(l2(0), r2(0))
                    t11, t22 = t11 + p1, t22 + p1
                    contribute(j, 0, 0, piece(l2(4), r2(4), t11))
                    contribute(j, 1, 1, piece(l2(3), r2(3), t22))
                tails(every.pop(0))

        for sub in (0, MC):
            for n in (range(HN // L) if i == 0 else (2,)):
                def put(w, c):
                    UL_v[pl.ds(((i % 5) * 5 + w) * P + sub, MC), n * L:(n + 1) * L] = c.astype(BF16)

                m1 = prod(0, sub, n)
                t11 = prod(6, sub, n, m1)
                m4 = prod(3, sub, n)
                t11 = t11 + m4
                m5 = prod(4, sub, n)
                u11 = emit(a0, sub, n, t11 - m5)
                m2 = prod(1, sub, n)
                u21 = emit(a1, sub, n, m2 + m4)
                put(3, u21 - u11)
                t22 = m1 - m2
                m3 = prod(2, sub, n)
                u12 = emit(a0, sub, n + HN // L, m3 + m5)
                put(2, u11 + u12)
                u22 = emit(a1, sub, n + HN // L, prod(5, sub, n, t22 + m3))
                put(0, u11 + u22)
                put(1, u21 + u22)
                put(4, u12 - u22)
                bg.charge(U_COST)
                tails(every.pop(0))

    def debug_keep_alive():
        if _ONLY is not None:
            for r_ in (xn_u, XL_u, WB_u, UL_u, WO_u, z1_v, R_u, Lc_u, L2_u, R2_u, C_v, zf_v, zg_v, kv_u, u_u, X_v, H_v, G_v, Z_u,
                       kf_v, bcol_v):
                c_ = pltpu.make_async_copy(r_, r_, sem_small.at[0])
                c_.start()
                c_.wait()

    debug_keep_alive()

    cp_x(0).start()
    cp_win(0).start()
    cp_x(1).start()
    cp_win(1).start()
    start(cp_small())
    for c in range(2, 5):
        cp_win(c).start()
    cp_x(2).start()

    kk = _odd_freq(jax.lax.broadcasted_iota(jnp.int32, (P, P), 0))
    nn = jax.lax.broadcasted_iota(jnp.int32, (P, P), 1)
    fc, fs = _cos_sin((kk * (4 * nn - 127)) & 2047)
    for g in range(P // 8):
        F_v[g * 16:(g + 1) * 16, 0:P] = jnp.concatenate(
            [fc[g * 8:(g + 1) * 8], -fs[g * 8:(g + 1) * 8]], axis=0).astype(BF16)
    fc, fs = _cos_sin((kk * (-127)) & 2047)
    ph_v[0] = fc
    ph_v[1] = fs
    kk = _odd_freq(jax.lax.broadcasted_iota(jnp.int32, (MC, P), 1))
    mm = jax.lax.broadcasted_iota(jnp.int32, (MC, P), 0)
    ic, is_ = _cos_sin((kk * (4 * mm + 2)) & 2047)
    Fi_v[:, 0:P] = (ic * (1.0 / (P * GA))).astype(BF16)
    Fi_v[:, P:2 * P] = (is_ * (1.0 / (P * GA))).astype(BF16)
    kf_v[:, 0:8, :] = jnp.zeros((D // L, 8, L), F32)

    cp_x(0).wait()
    for s in range(TM // 16):
        ln_x(0, s)

    def small_setup():
        sk = sk_in[...].astype(F32)
        for t in range(4):
            sk_v[t] = jnp.broadcast_to(sk[t:t + 1], (8, D))
        drow = d_in[...].astype(F32).reshape(1, D)
        for l in range(D // L):
            lanes = slice(l * L, (l + 1) * L)
            dre = ph_v[0] * drow[:, lanes]
            dim = ph_v[1] * drow[:, lanes]
            H_v[0, 0, 0:64, lanes] = -dim[0:64]
            H_v[0, 0, 64:P, lanes] = dim[64:P]
            H_v[0, 1, 0:64, lanes] = -dre[0:64]
            H_v[0, 1, 64:P, lanes] = dre[64:P]

    def bcol_task(t, j, tie):
        brow = b_in[...].astype(F32).reshape(1, S)[:, j * P:(j + 1) * P] * (0.25 / GA) + tie[0:1]
        bcol_v[j * P:(j + 1) * P, :] = jnp.broadcast_to(brow, (P, P)).T

    LAG = 2

    def interleave(*lists):
        out = []
        for j in range(max(len(a) for a in lists)):
            for a in lists:
                out += a[j:j + 1]
        return out

    def p1_first(c):
        bg = _Background()
        todo = []
        if c == 2:
            todo = tasks(bcol_task, 0)
            small_setup()
        if c == 3:
            todo = tasks(ln_z2, 0)
            bg.add(wcomb_gen(range(3)))
        if c == 4:
            todo = tasks(ln_x2, 2, 8)
            bg.add(wcomb_gen(range(3, 6)))
        tied = _Tied(todo, F_TIED[c])
        if c == 0:
            for s in range(TM // 16):
                ln_x(1, s)
        for t in range(2):
            for m in range(TM // MC):
                job_z(t, m, range(*WIN_CHUNKS[c]), bg, (80, 40), tied)
        bg.drain()
        assert not tied.tasks

    for c in range(5):
        cp_win(c).wait()
        if c == 0:
            cp_x(1).wait()
        if c == 2:
            wait(cp_small())
            start(cp_conv(0))
            cp_x(3).start()
        if c == 4:
            cp_x(2).wait()
            cp_x(4).start()
        block(lambda c=c: p1_first(c), f'p1_f{c}')

    def p1_wait(g):
        if g == 0:
            wait(cp_conv(0))
            cp_x(3).wait()
        if g == 1:
            wait(cp_conv(1))
            cp_x(4).wait()
        if g == 2:
            wait(cp_conv(2))
            cp_x(6).wait()
        if g == 3:
            wait(cp_conv(4))
            cp_wout().wait()
            wait(cp_wsp(0))

    def p1_start(g):
        if g == 0:
            start(cp_conv(1))
            cp_x(6).start()
            start(cp_conv(2))
        if g == 1:
            start(cp_conv(4))
            cp_wout().start()
            start(cp_wsp(0))
            start(cp_wsp(1))
        if g == 3:
            start(cp_wsp(2))
            start(cp_conv(6))
            for i in (3, 4, 5):
                start(cp_wsp(i))

    def take(gen, n):
        for _ in range(n):
            yield next(gen)

    def p1_step(i):
        bg = _Background()
        dft = _Background()
        t = i - LAG
        xg = P1_X[i]
        kv = kv_gen(t)
        nx, nz, nh = KV_SPLIT[i]
        dft.add(take(kv, nx))
        bg.add(take(kv, nz))
        hbg = _Background()
        hbg.add(take(kv, nh))
        zb = nz * KV_COST / 48.0
        extra = 0
        if i == 6:
            bg.add(wocomb_gen())
            bg.add(acomb_gen(0, range(5)))
            extra = EXTRA[0]
        if i == 7:
            bg.add(acomb_gen(0, range(5, 8)))
            bg.add(bcomb2_gen((1, 5)))
            extra = EXTRA[1]
        last = i == NT - 1
        z2t = tasks(ln_z2, i - 1)
        xt = [tasks(ln_x2, t_, 8) for t_ in P1_LNX[i]]
        if P1_TUNE[i][1]:
            todo = interleave(*([z2t[0::2]] + xt + [z2t[1::2]]))
        else:
            todo = interleave(*(xt + [z2t[0::2], z2t[1::2]]))
        tied = _Tied(todo, P1_TUNE[i][0])
        if xg is not None:
            dft.run(KV_COST)
            job_x(xg, dft, (nx - 1) * KV_COST / 10.0)
            dft.drain()
        for p in range(2):
            for j in range(FH // L):
                job_zs(i, p, j, bg, (1.6 * zb + extra, 0.5 * zb + extra), tied)
            assert not tied.tasks or (p == 0 and not last)
            if p == 0 and last:
                tied = _Tied(tasks(ln_z2, i, 8), LAST_N)
        if last:
            for s in range(8, 16):
                ln_z2(i, s)
        bg.drain()
        job_h(t, hbg, nh * KV_COST / 10.0)
        hbg.drain()

    def p1_block(g):
        for i in P1_GROUPS[g]:
            p1_step(i)

    for g in range(len(P1_GROUPS)):
        p1_wait(g)
        p1_start(g)
        block(lambda g=g: p1_block(g), f'p1_g{g}')

    groups = P2_GROUPS
    NG = len(groups)

    def p2_dma(gi):
        if gi >= 2:
            for i in groups[gi - 2]:
                start(cp_out(i))
        if gi >= 3:
            for i in groups[gi - 3]:
                wait(cp_out(i))
        if gi == 1:
            for i in (6, 7):
                start(cp_wsp(i))
        if gi == 0:
            wait(cp_conv(6))
        if gi + 1 < NG:
            for i in groups[gi + 1]:
                wait(cp_wsp(i))

    def tails_of(i, bg, budget):
        return [tail_gen(i, bg, budget)] * 20

    def p2_block(gi):
        bg = _Background()
        steps = groups[gi]
        tb = [0.0]
        pending = [t_ for i in (groups[gi - 1] if gi > 0 else []) for t_ in tails_of(i, bg, tb)]
        total = sum(a + 1 for i in steps for a in _blocks_of_step(i)) * 40 * 16
        total += len(steps) * (24 * E_COST + 6 * U_COST) + len(pending) * T_COST
        slots = sum(84 if i == 0 else 77 for i in steps) + TAIL_W * len(pending)
        bg.add(freq_gen(_blocks_of_step(steps[0])[0]))
        if gi == 0:
            bg.add(bcomb2_gen((0, 2, 3, 4, 6)))
            total += 5 * 16 * A_COST
        if gi < 2:
            bg.add(kv_gen(NT - 2 + gi))
            total += 20 * KV_COST
            slots += 10
        for t in P2_X[gi]:
            slots += 10
        if gi + 1 < NG:
            for i in groups[gi + 1]:
                bg.add(acomb2_gen(i))
                total += 16 * 7 * A2_COST
        for i in steps[1:]:
            bg.add(freq_gen(_blocks_of_step(i)[0]))
        budget = tb[0] = total / (slots + P2_END[gi])
        bg.run(budget)
        for t in P2_X[gi]:
            job_x(t, bg, budget)
        if gi < 2:
            job_h(NT - 2 + gi, bg, budget)
        units = [4, 4, 2, 4, 4, 2] * (len(pending) // 20)
        every = [0] * sum(6 if i == 0 else 9 for i in steps)
        for j, n in enumerate(units):
            every[min(len(every) - 1, j * len(every) // len(units))] += n
        for i in steps:
            job_big(i, bg, pending, budget, every)
        for t_ in pending:
            next(t_)
        bg.drain()

    for gi in range(NG):
        p2_dma(gi)
        block(lambda gi=gi: p2_block(gi), f'p2_{gi}')

    def cp_last(part):
        a0 = _blocks_of_step(NT - 1)[0]
        sub, cols = ((MC, pl.ds(0, D)), (0, pl.ds(0, 4 * L)), (0, pl.ds(4 * L, L)))[part]
        return [pltpu.make_async_copy(o_v.at[pl.ds(r, MC), cols], o_hbm.at[0, pl.ds(r, MC), cols],
                                      sem_out.at[NT - 1]) for r in (a0 * P + sub, (a0 + 1) * P + sub)]

    def p2_last():
        for i in groups[NG - 1]:
            for j, t_ in enumerate(tails_of(i, _Background(), [0.0])):
                next(t_)
                if i < NT - 1 and j == 19:
                    start(cp_out(i))
                if i == NT - 1 and j in (9, 17):
                    start(cp_last(j // 10))

    p2_dma(NG)
    block(p2_last, 'p2_last')
    start(cp_last(2))
    for i in groups[NG - 2] + groups[NG - 1][:-1]:
        wait(cp_out(i))
    for part in range(3):
        wait(cp_last(part))
    debug_keep_alive()


def _compiler_params():
    vmem = 124 * 1024 * 1024
    try:
        return pltpu.CompilerParams(vmem_limit_bytes=vmem, disable_semaphore_checks=True)
    except TypeError:
        return pltpu.CompilerParams(vmem_limit_bytes=vmem)


@jax.jit
def pallas_recurrent_scan__ssm_conv_h3__mixer_gmlp__prompt_kernel(
    A_q: jax.Array,
    A_k: jax.Array,
    A_v: jax.Array,
    A_shift_k: jax.Array,
    A_ssm_k: jax.Array,
    A_ssm_D: jax.Array,
    B_x: jax.Array,
    B_w_in: jax.Array,
    B_w_sp: jax.Array,
    B_b_sp: jax.Array,
    B_w_out: jax.Array,
):
    del B_x
    hbm = pl.BlockSpec(memory_space=pl.ANY)

    def bf16_buf(*shape):
        return pltpu.VMEM(shape[:-2] + (shape[-2] // 2, shape[-1]), U32)

    return pl.pallas_call(
        _kernel,
        out_shape=jax.ShapeDtypeStruct((1, S, D), BF16),
        in_specs=[hbm] * 10,
        out_specs=hbm,
        scratch_shapes=[
            [bf16_buf(len(g) * TM, D) for g in X_DMAS],
            [bf16_buf(len(g) * TM, D) for g in CONV_DMAS],
            [bf16_buf(len(g) * TM, D) for g in CONV_DMAS],
            [bf16_buf(D, len(g) * TM) for g in CONV_DMAS],
            [bf16_buf(D, max(hi - lo, 2) * L) for lo, hi in WIN_CHUNKS],
            [bf16_buf(TM, S) for _ in range(NT)],
            bf16_buf(FH, D),
            pltpu.VMEM((S, D), BF16),
            pltpu.VMEM((4, D), BF16),
            pltpu.VMEM((D,), BF16),
            pltpu.VMEM((S,), BF16),
            bf16_buf(S, D),
            bf16_buf(4 * 5 * P, KH),
            bf16_buf(5 * KH, FH),
            bf16_buf(5 * 5 * P, HN),
            bf16_buf(5 * HN, 2 * L),
            pltpu.VMEM((S, FH), F32),
            bf16_buf(7 * HK, HN),
            bf16_buf(5 * 5 * P, HK),
            bf16_buf(5 * 35 * MC, KQ),
            bf16_buf(21 * KQ, 2 * L),
            pltpu.VMEM((16 * MC, L), F32),
            pltpu.VMEM((HK, FH), F32),
            pltpu.VMEM((3, TM, FH), F32),
            bf16_buf(S, D),
            bf16_buf(S, FH),
            pltpu.VMEM((NB, 2, P, D), F32),
            pltpu.VMEM((2, 2, P, D), F32),
            pltpu.VMEM((NB, 2, P, D), F32),
            bf16_buf(NB * 2 * P, D),
            pltpu.VMEM((2, D // L, MC, L), F32),
            bf16_buf(2 * P, 2 * P),
            bf16_buf(MC, 2 * P),
            pltpu.VMEM((S, L), F32),
            pltpu.VMEM((2, P, L), F32),
            pltpu.VMEM((4, 8, D), F32),
            pltpu.VMEM((D // L, S + 8, L), F32),
            pltpu.SemaphoreType.DMA((1,)),
            pltpu.SemaphoreType.DMA((NT,)),
            pltpu.SemaphoreType.DMA((NT,)),
            pltpu.SemaphoreType.DMA((NT,)),
            pltpu.SemaphoreType.DMA((5,)),
            pltpu.SemaphoreType.DMA((NT,)),
        ],
        compiler_params=_compiler_params(),
    )(A_q, A_k, A_v, A_shift_k.T, A_ssm_k, A_ssm_D, B_w_in, B_w_sp, B_b_sp, B_w_out)
```

```python
import math

import jax
import jax.numpy as jnp
import jax.experimental.pallas as pl
import jax.experimental.pallas.tpu as pltpu

S = 2048
D = 640
FH = 768
P = 128
NB = S // P
TM = 256
NT = S // TM
MC = 64
L = 128
HK = S // 2
KQ = HK // 2
KH = 256
HN = FH // 2
EPS = 1e-5
F32 = jnp.float32
BF16 = jnp.bfloat16
U32 = jnp.uint32
GELU_C = math.sqrt(2.0 / math.pi)
GA = (GELU_C * 0.044715) ** (1.0 / 3.0)
NT_DIMS = (((1,), (1,)), ((), ()))

WIN_CHUNKS = ((6, 7), (7, 9), (9, 12), (0, 3), (3, 6))
X_DMAS = ((0,), (1,), (2,), (3,), (4, 5), (6, 7))
CONV_DMAS = ((0,), (1,), (2, 3), (4, 5), (6, 7))
P1_GROUPS = ((2,), (3,), (4, 5), (6, 7))
P1_X = {2: None, 3: 0, 4: 1, 5: None, 6: 2, 7: 3}
P1_LNX = {2: (3,), 3: (4, 5), 4: (6,), 5: (7,), 6: (), 7: ()}
P2_GROUPS = ((0,), (1, 2), (3, 4, 5), (6, 7))
P2_X = ((4, 5), (6,), (7,), ())
STEP_BLOCKS = ((2, 3), (6, 7), (4, 5), (12, 13), (10, 11), (0, 1), (14, 15), (8, 9))
KV_COST, A_COST, A2_COST = 110, 56, 34
E_COST, U_COST, T_COST, TAIL_W = 24, 90, 90, 1.6
KV_SPLIT = {2: (0, 14, 6), 3: (12, 4, 4), 4: (12, 4, 4), 5: (0, 14, 6), 6: (12, 4, 4), 7: (12, 4, 4)}
FR = 8
L1_USE = {0: ((0, 1, True, False), (3, 1, True, False)), 6: ((0, 1, False, False),),
          3: ((0, 1, False, False), (2, 1, True, False)), 4: ((0, -1, False, True), (1, 1, True, False)),
          1: ((2, 1, False, True), (3, -1, False, False)), 2: ((1, 1, False, True), (3, 1, False, False)),
          5: ((3, 1, False, True),)}
H_SPLIT = ((0, 2), (2, 4), (4, 5))
P1_TUNE = {2: (42, 0), 3: (43, 1), 4: (42, 0), 5: (42, 0), 6: (44, 0), 7: (24, 0)}
EXTRA = (52, 52)
LAST_N = 22
P2_END = (0.0, -1.0, -1.0, 0.0)
F_TIED = (20, 20, 18, 20, 20)
_ONLY = None


def _dot(a, b):
    return jnp.dot(a, b, preferred_element_type=F32)


def _cos_sin(m):
    q = (m + 256) >> 9
    x = (m - (q << 9)).astype(F32) * (2.0 * math.pi / 2048.0)
    x2 = x * x
    s = x * (1.0 + x2 * (-1.0 / 6 + x2 * (1.0 / 120 + x2 * (-1.0 / 5040 + x2 * (1.0 / 362880)))))
    c = 1.0 + x2 * (-0.5 + x2 * (1.0 / 24 + x2 * (-1.0 / 720 + x2 * (1.0 / 40320 - x2 * (1.0 / 3628800)))))
    swap = (q & 1) == 1
    c0 = jnp.where(swap, s, c)
    s0 = jnp.where(swap, c, s)
    cos = jnp.where(((q + 1) & 2) == 2, -c0, c0)
    sin = jnp.where((q & 2) == 2, -s0, s0)
    return cos, sin


def _odd_freq(r):
    return jnp.where(r < 64, 4 * r + 1, 4 * r - 253)


def _gelu_scaled(z):
    return z + z * jnp.tanh(z * (GELU_C / GA + z * z))


def _signzero(z):
    bits = jax.lax.bitcast_convert_type(z, U32) & jnp.uint32(0x80000000)
    return jax.lax.bitcast_convert_type(bits, F32)


def _ln(x, eps, tie=None, scale=None):
    n = x.shape[-1]
    cols = [x[:, j * L:(j + 1) * L] for j in range(n // L)]
    s1 = cols[0]
    s2 = cols[0] * cols[0]
    for c in cols[1:]:
        s1 = s1 + c
        s2 = s2 + c * c
    if tie is not None:
        s1 = s1 + tie
        s2 = s2 + tie
    m = jnp.sum(s1, axis=-1, keepdims=True) * (1.0 / n)
    v = jnp.maximum(jnp.sum(s2, axis=-1, keepdims=True) * (1.0 / n) - m * m, 0.0)
    rs = jax.lax.rsqrt(v + eps)
    if scale is not None:
        rs = rs * scale
    return (x - m) * rs


def _blocks_of_step(i):
    return STEP_BLOCKS[i]


class _Background:
    def __init__(self):
        self.q = []
        self.credit = 0.0

    def add(self, gen):
        self.q.append(gen)

    def run(self, budget):
        self.credit += budget
        while self.q and self.credit > 0:
            try:
                self.credit -= next(self.q[0])
            except StopIteration:
                self.q.pop(0)
        if not self.q:
            self.credit = 0.0

    def charge(self, cost):
        self.credit -= cost

    def drain(self):
        while self.q:
            self.run(1e9)


class _Tied:
    def __init__(self, tasks, npieces):
        self.tasks = list(tasks)
        self.rate = len(self.tasks) / float(npieces)
        self.credit = 0.999

    def run(self, z):
        self.credit += self.rate
        n = 0
        while self.tasks and self.credit >= 1.0:
            self.tasks.pop(0)(_signzero(z[0:16]))
            self.credit -= 1.0
            n += 1
        return n


def _kernel(q_hbm, k_hbm, v_hbm, sk_hbm, h_hbm, d_hbm, win_hbm, wsp_hbm, b_hbm, wout_hbm,
            o_hbm,
            x_us, k_us, v_us, h_us, win_us, wsp_us, wout_u, o_v, sk_in, d_in, b_in,
            xn_u, XL_u, WB_u, UL_u, WO_u, z1_v, R_u, Lc_u, L2_u, R2_u, C_v, zf_v, zg_v, kv_u, u_u, X_v, H_v, G_v, Z_u,
            yl_v, F_u, Fi_u, bcol_v, ph_v, sk_v, kf_v,
            sem_small, sem_x, sem_conv, sem_wsp, sem_w, sem_out):
    (wout_v, xn_v, XL_v, WB_v, UL_v, WO_v, R_v, Lc_v, L2_v, R2_v, kv_v, u_v, Z_v, F_v, Fi_v) = [
        r.bitcast(BF16) for r in (wout_u, xn_u, XL_u, WB_u, UL_u, WO_u, R_u, Lc_u, L2_u, R2_u, kv_u, u_u, Z_u, F_u, Fi_u)]
    x_vs = {g[0]: r.bitcast(BF16) for g, r in zip(X_DMAS, x_us)}
    k_vs, v_vs, h_vs = [{g[0]: r.bitcast(BF16) for g, r in zip(CONV_DMAS, rs)} for rs in (k_us, v_us, h_us)]
    wsp_vs = [r.bitcast(BF16) for r in wsp_us]
    win_vs = [r.bitcast(BF16) for r in win_us]

    def win(rows, n):
        c = [lo <= n < hi for lo, hi in WIN_CHUNKS].index(True)
        n -= WIN_CHUNKS[c][0]
        return win_vs[c][rows, n * L:(n + 1) * L]

    def locate(bufs, row):
        t0 = max(t for t in bufs if t * TM <= row)
        return bufs[t0], row - t0 * TM

    def rows_of(bufs, row, n, lanes=slice(None)):
        buf, r = locate(bufs, row)
        return buf[r:r + n, lanes]

    def cp_small():
        return [pltpu.make_async_copy(s_, d_, sem_small.at[0])
                for s_, d_ in ((d_hbm, d_in), (sk_hbm, sk_in), (b_hbm, b_in))]

    def cp_x(t):
        return pltpu.make_async_copy(q_hbm.at[0, pl.ds(t * TM, x_vs[t].shape[0])], x_vs[t], sem_x.at[t])

    def cp_conv(t):
        rows = pl.ds(t * TM, k_vs[t].shape[0])
        sem = sem_conv.at[t]
        return [pltpu.make_async_copy(h_hbm.at[:, rows], h_vs[t], sem),
                pltpu.make_async_copy(k_hbm.at[0, rows], k_vs[t], sem),
                pltpu.make_async_copy(v_hbm.at[0, rows], v_vs[t], sem)]

    def cp_wsp(i):
        return [pltpu.make_async_copy(wsp_hbm.at[pl.ds(_blocks_of_step(i)[0] * P, TM)], wsp_vs[i], sem_wsp.at[i])]

    def cp_win(c):
        lo, hi = WIN_CHUNKS[c]
        w = (hi - lo) * L
        return pltpu.make_async_copy(win_hbm.at[:, pl.ds(lo * L, w)], win_vs[c].at[:, pl.ds(0, w)], sem_w.at[c])

    def cp_wout():
        return pltpu.make_async_copy(wout_hbm, wout_v, sem_w.at[0])

    def cp_out(i):
        rows = pl.ds(_blocks_of_step(i)[0] * P, TM)
        return [pltpu.make_async_copy(o_v.at[rows], o_hbm.at[0, rows], sem_out.at[i])]

    def start(cs):
        for c in cs:
            c.start()

    def wait(cs):
        for c in cs:
            c.wait()

    def block(fn, name):
        def body(it):
            fn()
            return it + 1

        if _ONLY is None or name in _ONLY:
            jax.lax.while_loop(lambda it: it < 1, body, jnp.int32(0))

    def ln_x(t, s, tie=None):
        rows = pl.ds(t * TM + s * 16, 16)
        y = _ln(rows_of(x_vs, t * TM + s * 16, 16).astype(F32), EPS, tie, GA)
        xn_v[rows, :] = y.astype(BF16)
        return y

    def ln_x2(t, s, tie):
        p, q = s // 4, s % 4
        y1 = ln_x(t, 8 * p + q, tie)
        y2 = ln_x(t, 8 * p + 4 + q, tie)
        a11, a12, a21, a22 = y1[:, :KH], y1[:, KH:2 * KH], y2[:, :KH], y2[:, KH:2 * KH]
        r0 = (t % 4) * 5 * P + p * MC + q * 16
        for j, c in enumerate((a11 + a22, a21 + a22, a11 + a12, a21 - a11, a12 - a22)):
            XL_v[pl.ds(r0 + j * P, 16), :] = c.astype(BF16)

    def wcomb_gen(cols):
        for j in cols:
            c1 = slice(j * L, (j + 1) * L)
            for r in range(KH // 32):
                top = pl.ds(r * 32, 32)
                bot = pl.ds(KH + r * 32, 32)
                b11, b12 = win(top, j).astype(F32), win(top, 6 + j).astype(F32)
                b21, b22 = win(bot, j).astype(F32), win(bot, 6 + j).astype(F32)
                for w, c in enumerate((b11 + b22, b12 - b22, b21 - b11, b11 + b12, b21 + b22)):
                    WB_v[pl.ds(w * KH + r * 32, 32), c1] = c.astype(BF16)
                yield A_COST

    def ln_z2(t, s, tie=None):
        y = _ln(zg_v[t % 3, s * 16:(s + 1) * 16, :], 4.0 * GA * GA * EPS, tie, 0.25 / GA)
        lo, hi = y[:, :HN], y[:, HN:]
        r = (t * TM + s * 16) % HK
        rows = pl.ds(r, 16)
        if t < NT // 2:
            zf_v[rows, :] = y
            R_v[pl.ds(1 * HK + r, 16), :] = lo.astype(BF16)
            R_v[pl.ds(5 * HK + r, 16), :] = (lo + hi).astype(BF16)
        else:
            b11, b12 = zf_v[rows, :HN], zf_v[rows, HN:]
            R_v[pl.ds(0 * HK + r, 16), :] = (b11 + hi).astype(BF16)
            R_v[pl.ds(2 * HK + r, 16), :] = (b12 - hi).astype(BF16)
            R_v[pl.ds(3 * HK + r, 16), :] = (lo - b11).astype(BF16)
            R_v[pl.ds(4 * HK + r, 16), :] = hi.astype(BF16)
            R_v[pl.ds(6 * HK + r, 16), :] = (lo + hi).astype(BF16)

    def acomb_gen(i, groups=range(P // 16)):
        for r in groups:
            for c in range(HK // 256):
                top = pl.ds(r * 16, 16)
                bot = pl.ds(P + r * 16, 16)
                c1 = slice(c * 256, (c + 1) * 256)
                c2 = slice(HK + c * 256, HK + (c + 1) * 256)
                a11 = wsp_vs[i][top, c1].astype(F32)
                a12 = wsp_vs[i][top, c2].astype(F32)
                a21 = wsp_vs[i][bot, c1].astype(F32)
                a22 = wsp_vs[i][bot, c2].astype(F32)
                r0 = (i % 5) * 5 * P + r * 16
                Lc_v[pl.ds(r0 + 0 * P, 16), c1] = (a11 + a22).astype(BF16)
                Lc_v[pl.ds(r0 + 1 * P, 16), c1] = (a21 + a22).astype(BF16)
                Lc_v[pl.ds(r0 + 2 * P, 16), c1] = (a11 + a12).astype(BF16)
                Lc_v[pl.ds(r0 + 3 * P, 16), c1] = (a21 - a11).astype(BF16)
                Lc_v[pl.ds(r0 + 4 * P, 16), c1] = (a12 - a22).astype(BF16)
                yield A_COST

    def acomb2_gen(i):
        for r in range(MC // 16):
            for c in range(KQ // L):
                quad = {}

                def w(b, H):
                    if (b, H) not in quad:
                        quad[b, H] = [[wsp_vs[i][pl.ds(b * P + s_ * MC + r * 16, 16),
                                                 H * HK + kh * KQ + c * L:H * HK + kh * KQ + (c + 1) * L].astype(F32)
                                       for kh in range(2)] for s_ in range(2)]
                    return quad[b, H]

                spec = {2: (None, (0, 0), None, 0), 0: (0, (0, 0), (1, 1), 1), 3: (None, (1, 1), None, 0),
                        1: (1, (1, 0), (1, 1), 1), 5: (3, (1, 0), (0, 0), -1), 4: (2, (0, 0), (0, 1), 1),
                        6: (4, (0, 1), (1, 1), -1)}
                for j in (2, 0, 3, 1, 5, 4, 6):
                    slot, p_, q_, sign = spec[j]
                    a = w(*p_)
                    if q_ is not None:
                        b_ = w(*q_)
                        a = [[a[s_][kh] + b_[s_][kh] if sign > 0 else a[s_][kh] - b_[s_][kh] for kh in range(2)]
                             for s_ in range(2)]
                        for s_ in range(2):
                            for kh in range(2):
                                Lc_v[pl.ds(((i % 5) * 5 + slot) * P + s_ * MC + r * 16, 16),
                                     kh * KQ + c * L:kh * KQ + (c + 1) * L] = a[s_][kh].astype(BF16)
                    for w2, v_ in enumerate((a[0][0] + a[1][1], a[1][0] + a[1][1], a[0][0] + a[0][1],
                                             a[1][0] - a[0][0], a[0][1] - a[1][1])):
                        L2_v[pl.ds((((i % 5) * 7 + j) * 5 + w2) * MC + r * 16, 16), c * L:(c + 1) * L] = v_.astype(BF16)
                    yield A2_COST

    def bcomb2_gen(js):
        for j in js:
            for r in range(KQ // 16):
                top = pl.ds(j * HK + r * 16, 16)
                bot = pl.ds(j * HK + KQ + r * 16, 16)
                b11, b12 = R_v[top, 0:L].astype(F32), R_v[top, L:2 * L].astype(F32)
                b21, b22 = R_v[bot, 0:L].astype(F32), R_v[bot, L:2 * L].astype(F32)
                for w, c in enumerate((b11 + b22, b12 - b22, b21 - b11, b11 + b12, b21 + b22)):
                    R2_v[pl.ds((j * 3 + w // 2) * KQ + r * 16, 16), (w % 2) * L:(w % 2 + 1) * L] = c.astype(BF16)
                yield A_COST / 2

    def tasks(fn, t, n=TM // 16):
        return [lambda tie, s=s: fn(t, s, tie) for s in range(n)]

    def kv_gen(t):
        for m in range(TM // MC):
            r = t * TM + m * MC
            for l in range(D // L):
                lanes = slice(l * L, (l + 1) * L)
                kf = rows_of(k_vs, r, MC, lanes).astype(F32)
                kf_v[l, pl.ds(r + 8, MC), :] = kf
                ks = kf * sk_v[0, 0:1, lanes]
                for tap in range(1, 4):
                    ks = ks + kf_v[l, pl.ds(r + 8 - tap, MC), :] * sk_v[tap, 0:1, lanes]
                kv = ks * rows_of(v_vs, r, MC, lanes).astype(F32)
                kv_v[pl.ds(r, MC), lanes] = kv.astype(BF16)
                yield KV_COST

    def freq_gen(a):
        def cmac(acc, x, g):
            pr = x[0] * g[0] - x[1] * g[1]
            pi = x[0] * g[1] + x[1] * g[0]
            return (pr, pi) if acc is None else (acc[0] + pr, acc[1] + pi)

        for r in range(P // 16):
            for l in range(D // L):
                lanes = slice(l * L, (l + 1) * L)
                res = []
                for sub in range(16 // FR):
                    rows = pl.ds(r * 16 + sub * FR, FR)
                    lo = hi = None
                    g = (G_v[a + 1, 0, rows, lanes], G_v[a + 1, 1, rows, lanes])
                    for c in range(a + 2):
                        x = (X_v[c, 0, rows, lanes], X_v[c, 1, rows, lanes])
                        hi = cmac(hi, x, g)
                        if c <= a:
                            g = (G_v[a - c, 0, rows, lanes], G_v[a - c, 1, rows, lanes])
                            lo = cmac(lo, x, g)
                            yield 2 * FR
                    res.append((lo, hi))
                for w in range(2):
                    for part in range(2):
                        Z_v[pl.ds((a + w) * 2 * P + part * P + r * 16, 16), lanes] = jnp.concatenate(
                            [z[w][part] for z in res], axis=0).astype(BF16)
                yield 20

    def job_x(t, bg, budget):
        for j in (2 * t, 2 * t + 1):
            for half in range(2):
                r = _dot(F_v[half * P:(half + 1) * P, 0:P], kv_v[j * P:(j + 1) * P, :]).reshape(8, 2, 8, D)
                for part in range(2):
                    X_v[j, part, half * 64:(half + 1) * 64, :] = r[:, part].reshape(64, D)
                bg.run(budget * 2.5)

    def job_h(t, bg, budget):
        h_v, c0 = locate(h_vs, t * TM)
        for half in range(2):
            rows = pl.ds(half * 64, 64)
            for l0, l1 in H_SPLIT:
                w = (l1 - l0) * L
                lanes = slice(l0 * L, l1 * L)
                rhs = jnp.concatenate([h_v[lanes, c0:c0 + P], h_v[lanes, c0 + P:c0 + TM]], axis=0)
                r = jax.lax.dot_general(F_v[half * P:(half + 1) * P, 0:P], rhs, NT_DIMS,
                                        preferred_element_type=F32).reshape(8, 2, 8, 2 * w)
                re, im = r[:, 0].reshape(64, 2 * w), r[:, 1].reshape(64, 2 * w)
                prev = (H_v[t % 2, 0, rows, lanes], H_v[t % 2, 1, rows, lanes])
                for j in range(2):
                    cur = (re[:, j * w:(j + 1) * w], im[:, j * w:(j + 1) * w])
                    G_v[2 * t + j, 0, rows, lanes] = cur[0] + prev[1] if half else cur[0] - prev[1]
                    G_v[2 * t + j, 1, rows, lanes] = cur[1] - prev[0] if half else cur[1] + prev[0]
                    prev = cur
                if t + 1 < NT:
                    H_v[(t + 1) % 2, 0, rows, lanes] = prev[0]
                    H_v[(t + 1) % 2, 1, rows, lanes] = prev[1]
                bg.run(budget * (l1 - l0))

    def z_out(t, m, n, pre, bg, budget, tied):
        z = _gelu_scaled(pre)
        if n < FH // L:
            z1_v[pl.ds(t * TM + m * MC, MC), n * L:(n + 1) * L] = z
        else:
            zg_v[t % 3, m * MC:(m + 1) * MC, n * L - FH:(n + 1) * L - FH] = z
        ntask = tied.run(z)
        bg.run(budget[1] if ntask else budget[0])

    def job_z(t, m, cols, bg, budget, tied):
        for n in cols:
            z_out(t, m, n, _dot(xn_v[pl.ds(t * TM + m * MC, MC), :], win(slice(None), n)), bg, budget, tied)

    def job_zs(t, p, j, bg, budget, tied):
        r1 = pl.ds(t * TM + p * P, MC)
        r2 = pl.ds(t * TM + p * P + MC, MC)
        c1 = slice(j * L, (j + 1) * L)

        def xl(w):
            r0 = (t % 4) * 5 * P + w * P + p * MC
            return XL_v[r0:r0 + MC, :]

        def wb(w):
            return WB_v[w * KH:(w + 1) * KH, c1]

        def rem(rows, n):
            return _dot(xn_v[rows, 2 * KH:], win(slice(2 * KH, D), n))

        m2 = _dot(xl(1), win(slice(0, KH), j))
        m4 = _dot(xn_v[r2, KH:2 * KH], wb(2))
        z_out(t, 2 * p + 1, j, m2 + m4 + rem(r2, j), bg, budget, tied)
        m3 = _dot(xn_v[r1, 0:KH], wb(1))
        m5 = _dot(xl(2), win(slice(KH, 2 * KH), 6 + j))
        z_out(t, 2 * p, 6 + j, m3 + m5 + rem(r1, 6 + j), bg, budget, tied)
        t11, t22 = m4 - m5, m3 - m2
        m1 = _dot(xl(0), wb(0))
        t11, t22 = t11 + m1, t22 + m1
        z_out(t, 2 * p, j, t11 + _dot(xl(4), wb(4)) + rem(r1, j), bg, budget, tied)
        z_out(t, 2 * p + 1, 6 + j, t22 + _dot(xl(3), wb(3)) + rem(r2, 6 + j), bg, budget, tied)

    rev8 = 7 - jax.lax.broadcasted_iota(jnp.int32, (8, L), 0)

    def finish(a, upper, n, hh, slot):
        rows = pl.ds(a * P + (MC if upper else 0), MC)
        lanes = slice(n * L, (n + 1) * L)
        if upper:
            ya = _dot(Fi_v[:, 0:P], Z_v[a * 2 * P:a * 2 * P + P, lanes])
            yb = _dot(Fi_v[:, P:2 * P], Z_v[a * 2 * P + P:(a + 1) * 2 * P, lanes])
            slot(0.5)
            y = ya - yb
            lo = ya + yb
            for j in range(MC // 8):
                yl_v[a % 2, n, (7 - j) * 8:(8 - j) * 8, :] = jnp.take_along_axis(lo[j * 8:(j + 1) * 8], rev8, axis=0)
        else:
            y = yl_v[a % 2, n]
        gate = hh + hh * jnp.tanh(hh)
        s = xn_v[rows, lanes].astype(F32) * y
        x = rows_of(x_vs, a * P + (MC if upper else 0), MC, lanes).astype(F32)
        o_v[rows, lanes] = (x + s * gate).astype(BF16)

    def tail_gen(i, bg, budget):
        a0, a1 = _blocks_of_step(i)

        def slot(w):
            bg.run(w * budget[0])

        def dot3(a, b):
            r = _dot(a, b)
            slot(0.75)
            return r

        for upper in (True, False):
            sub = MC if upper else 0
            r1 = pl.ds(a0 * P + sub, MC)
            r2 = pl.ds(a1 * P + sub, MC)

            def ul(w):
                r0 = ((i % 5) * 5 + w) * P + sub
                return UL_v[r0:r0 + MC, :]

            for j in range(2):
                c1 = slice(j * L, (j + 1) * L)
                c2 = slice((2 + j) * L, (3 + j) * L)

                def wo(w):
                    return WO_v[w * HN:(w + 1) * HN, c1]

                m2 = dot3(ul(1), wout_v[0:HN, c1])
                m4 = dot3(u_v[r2, HN:], wo(2))
                finish(a1, upper, j, m2 + m4, slot)
                bg.charge(T_COST)
                yield
                m3 = dot3(u_v[r1, 0:HN], wo(1))
                m5 = dot3(ul(2), wout_v[HN:, c2])
                finish(a0, upper, 2 + j, m3 + m5, slot)
                bg.charge(T_COST)
                yield
                t11, t22 = m4 - m5, m3 - m2
                m1 = dot3(ul(0), wo(0))
                t11, t22 = t11 + m1, t22 + m1
                finish(a0, upper, j, t11 + dot3(ul(4), wo(4)), slot)
                bg.charge(T_COST)
                yield
                finish(a1, upper, 2 + j, t22 + dot3(ul(3), wo(3)), slot)
                bg.charge(T_COST)
                yield
            for a, r in ((a0, r1), (a1, r2)):
                finish(a, upper, 4, dot3(u_v[r, 0:HN], wout_v[0:HN, 4 * L:]) + dot3(u_v[r, HN:], wout_v[HN:, 4 * L:]),
                       slot)
                bg.charge(T_COST)
                yield

    def wocomb_gen():
        for j in range(2):
            c1 = slice(j * L, (j + 1) * L)
            c2 = slice((2 + j) * L, (3 + j) * L)
            for r in range(HN // 32):
                top = pl.ds(r * 32, 32)
                bot = pl.ds(HN + r * 32, 32)
                b11, b12 = wout_v[top, c1].astype(F32), wout_v[top, c2].astype(F32)
                b21, b22 = wout_v[bot, c1].astype(F32), wout_v[bot, c2].astype(F32)
                for w, c in enumerate((b11 + b22, b12 - b22, b21 - b11, b11 + b12, b21 + b22)):
                    WO_v[pl.ds(w * HN + r * 32, 32), c1] = c.astype(BF16)
                yield A_COST

    def job_big(i, bg, pending, budget, every):
        a0, a1 = _blocks_of_step(i)
        KG = 512

        def lhs(j, sub, cols):
            if j == 2:
                return wsp_vs[i][sub:sub + MC, cols]
            if j == 3:
                return wsp_vs[i][P + sub:P + sub + MC, HK + cols.start:HK + cols.stop]
            r0 = ((i % 5) * 5 + {0: 0, 1: 1, 4: 2, 5: 3, 6: 4}[j]) * P + sub
            return Lc_v[r0:r0 + MC, cols]

        def prod(j, sub, n, acc=None):
            for kg in range(HK // KG):
                ks = slice(kg * KG, (kg + 1) * KG)
                p = _dot(lhs(j, sub, ks), R_v[j * HK + kg * KG:j * HK + (kg + 1) * KG, n * L:(n + 1) * L])
                acc = p if acc is None else acc + p
                bg.run(budget)
            return acc

        def tails(n):
            for _ in range(n):
                if pending:
                    next(pending.pop(0))

        def emit(a, sub, n, g):
            rows = pl.ds(a * P + sub, MC)
            lanes = slice(n * L, (n + 1) * L)
            u = z1_v[rows, lanes] * (g + bcol_v[rows, :])
            u_v[rows, lanes] = u.astype(BF16)
            bg.charge(E_COST)
            return u

        if i > 0:
            def piece(a, b, acc=None):
                p = _dot(a, b)
                bg.run(budget)
                return p if acc is None else acc + p

            def cslot(k, s_, n):
                return pl.ds(((k * 2 + s_) * 2 + n) * MC, MC)

            def contribute(j, s_, n, m):
                for k, sign, first, last in L1_USE[j]:
                    cs = cslot(k, s_, n)
                    v_ = m if first else (C_v[cs, :] + m if sign > 0 else C_v[cs, :] - m)
                    if last:
                        u = emit((a0, a0, a1, a1)[k], s_ * MC, n + (k % 2) * (HN // L), v_)
                        v_ = u
                        if k == 3:
                            u11, u12, u21 = C_v[cslot(0, s_, n), :], C_v[cslot(1, s_, n), :], C_v[cslot(2, s_, n), :]
                            for w, c in enumerate((u11 + u, u21 + u, u11 + u12, u21 - u11, u12 - u)):
                                UL_v[pl.ds(((i % 5) * 5 + w) * P + s_ * MC, MC), n * L:(n + 1) * L] = c.astype(BF16)
                            bg.charge(U_COST)
                            continue
                    C_v[cs, :] = v_

            for j in (0, 6, 3, 4, 1, 2, 5):
                def l2(w):
                    r0 = (((i % 5) * 7 + j) * 5 + w) * MC
                    return L2_v[r0:r0 + MC, :]

                def r2(w):
                    r0 = (j * 3 + w // 2) * KQ
                    return R2_v[r0:r0 + KQ, (w % 2) * L:(w % 2 + 1) * L]

                def rq(kh, n):
                    return R_v[j * HK + kh * KQ:j * HK + (kh + 1) * KQ, n * L:(n + 1) * L]

                p2 = piece(l2(1), rq(0, 0))
                p4 = piece(lhs(j, MC, slice(KQ, 2 * KQ)), r2(2))
                contribute(j, 1, 0, p2 + p4)
                p3 = piece(lhs(j, 0, slice(0, KQ)), r2(1))
                t22 = p3 - p2
                p5 = piece(l2(2), rq(1, 1))
                contribute(j, 0, 1, p3 + p5)
                t11 = p4 - p5
                p1 = piece(l2(0), r2(0))
                t11, t22 = t11 + p1, t22 + p1
                contribute(j, 0, 0, piece(l2(4), r2(4), t11))
                contribute(j, 1, 1, piece(l2(3), r2(3), t22))
                tails(every.pop(0))

        for sub in (0, MC):
            for n in (range(HN // L) if i == 0 else (2,)):
                def put(w, c):
                    UL_v[pl.ds(((i % 5) * 5 + w) * P + sub, MC), n * L:(n + 1) * L] = c.astype(BF16)

                m1 = prod(0, sub, n)
                t11 = prod(6, sub, n, m1)
                m4 = prod(3, sub, n)
                t11 = t11 + m4
                m5 = prod(4, sub, n)
                u11 = emit(a0, sub, n, t11 - m5)
                m2 = prod(1, sub, n)
                u21 = emit(a1, sub, n, m2 + m4)
                put(3, u21 - u11)
                t22 = m1 - m2
                m3 = prod(2, sub, n)
                u12 = emit(a0, sub, n + HN // L, m3 + m5)
                put(2, u11 + u12)
                u22 = emit(a1, sub, n + HN // L, prod(5, sub, n, t22 + m3))
                put(0, u11 + u22)
                put(1, u21 + u22)
                put(4, u12 - u22)
                bg.charge(U_COST)
                tails(every.pop(0))

    def debug_keep_alive():
        if _ONLY is not None:
            for r_ in (xn_u, XL_u, WB_u, UL_u, WO_u, z1_v, R_u, Lc_u, L2_u, R2_u, C_v, zf_v, zg_v, kv_u, u_u, X_v, H_v, G_v, Z_u,
                       kf_v, bcol_v):
                c_ = pltpu.make_async_copy(r_, r_, sem_small.at[0])
                c_.start()
                c_.wait()

    debug_keep_alive()

    cp_x(0).start()
    cp_win(0).start()
    cp_x(1).start()
    cp_win(1).start()
    start(cp_small())
    for c in range(2, 5):
        cp_win(c).start()
    cp_x(2).start()

    kk = _odd_freq(jax.lax.broadcasted_iota(jnp.int32, (P, P), 0))
    nn = jax.lax.broadcasted_iota(jnp.int32, (P, P), 1)
    fc, fs = _cos_sin((kk * (4 * nn - 127)) & 2047)
    for g in range(P // 8):
        F_v[g * 16:(g + 1) * 16, 0:P] = jnp.concatenate(
            [fc[g * 8:(g + 1) * 8], -fs[g * 8:(g + 1) * 8]], axis=0).astype(BF16)
    fc, fs = _cos_sin((kk * (-127)) & 2047)
    ph_v[0] = fc
    ph_v[1] = fs
    kk = _odd_freq(jax.lax.broadcasted_iota(jnp.int32, (MC, P), 1))
    mm = jax.lax.broadcasted_iota(jnp.int32, (MC, P), 0)
    ic, is_ = _cos_sin((kk * (4 * mm + 2)) & 2047)
    Fi_v[:, 0:P] = (ic * (1.0 / (P * GA))).astype(BF16)
    Fi_v[:, P:2 * P] = (is_ * (1.0 / (P * GA))).astype(BF16)
    kf_v[:, 0:8, :] = jnp.zeros((D // L, 8, L), F32)

    cp_x(0).wait()
    for s in range(TM // 16):
        ln_x(0, s)

    def small_setup():
        sk = sk_in[...].astype(F32)
        for t in range(4):
            sk_v[t] = jnp.broadcast_to(sk[t:t + 1], (8, D))
        drow = d_in[...].astype(F32).reshape(1, D)
        for l in range(D // L):
            lanes = slice(l * L, (l + 1) * L)
            dre = ph_v[0] * drow[:, lanes]
            dim = ph_v[1] * drow[:, lanes]
            H_v[0, 0, 0:64, lanes] = -dim[0:64]
            H_v[0, 0, 64:P, lanes] = dim[64:P]
            H_v[0, 1, 0:64, lanes] = -dre[0:64]
            H_v[0, 1, 64:P, lanes] = dre[64:P]

    def bcol_task(t, j, tie):
        brow = b_in[...].astype(F32).reshape(1, S)[:, j * P:(j + 1) * P] * (0.25 / GA) + tie[0:1]
        bcol_v[j * P:(j + 1) * P, :] = jnp.broadcast_to(brow, (P, P)).T

    LAG = 2

    def interleave(*lists):
        out = []
        for j in range(max(len(a) for a in lists)):
            for a in lists:
                out += a[j:j + 1]
        return out

    def p1_first(c):
        bg = _Background()
        todo = []
        if c == 2:
            todo = tasks(bcol_task, 0)
            small_setup()
        if c == 3:
            todo = tasks(ln_z2, 0)
            bg.add(wcomb_gen(range(3)))
        if c == 4:
            todo = tasks(ln_x2, 2, 8)
            bg.add(wcomb_gen(range(3, 6)))
        tied = _Tied(todo, F_TIED[c])
        if c == 0:
            for s in range(TM // 16):
                ln_x(1, s)
        for t in range(2):
            for m in range(TM // MC):
                job_z(t, m, range(*WIN_CHUNKS[c]), bg, (80, 40), tied)
        bg.drain()
        assert not tied.tasks

    for c in range(5):
        cp_win(c).wait()
        if c == 0:
            cp_x(1).wait()
        if c == 2:
            wait(cp_small())
            start(cp_conv(0))
            cp_x(3).start()
        if c == 4:
            cp_x(2).wait()
            cp_x(4).start()
        block(lambda c=c: p1_first(c), f'p1_f{c}')

    def p1_wait(g):
        if g == 0:
            wait(cp_conv(0))
            cp_x(3).wait()
        if g == 1:
            wait(cp_conv(1))
            cp_x(4).wait()
        if g == 2:
            wait(cp_conv(2))
            cp_x(6).wait()
        if g == 3:
            wait(cp_conv(4))
            cp_wout().wait()
            wait(cp_wsp(0))

    def p1_start(g):
        if g == 0:
            start(cp_conv(1))
            cp_x(6).start()
            start(cp_conv(2))
        if g == 1:
            start(cp_conv(4))
            cp_wout().start()
            start(cp_wsp(0))
            start(cp_wsp(1))
        if g == 3:
            start(cp_wsp(2))
            start(cp_conv(6))
            for i in (3, 4, 5):
                start(cp_wsp(i))

    def take(gen, n):
        for _ in range(n):
            yield next(gen)

    def p1_step(i):
        bg = _Background()
        dft = _Background()
        t = i - LAG
        xg = P1_X[i]
        kv = kv_gen(t)
        nx, nz, nh = KV_SPLIT[i]
        dft.add(take(kv, nx))
        bg.add(take(kv, nz))
        hbg = _Background()
        hbg.add(take(kv, nh))
        zb = nz * KV_COST / 48.0
        extra = 0
        if i == 6:
            bg.add(wocomb_gen())
            bg.add(acomb_gen(0, range(5)))
            extra = EXTRA[0]
        if i == 7:
            bg.add(acomb_gen(0, range(5, 8)))
            bg.add(bcomb2_gen((1, 5)))
            extra = EXTRA[1]
        last = i == NT - 1
        z2t = tasks(ln_z2, i - 1)
        xt = [tasks(ln_x2, t_, 8) for t_ in P1_LNX[i]]
        if P1_TUNE[i][1]:
            todo = interleave(*([z2t[0::2]] + xt + [z2t[1::2]]))
        else:
            todo = interleave(*(xt + [z2t[0::2], z2t[1::2]]))
        tied = _Tied(todo, P1_TUNE[i][0])
        if xg is not None:
            dft.run(KV_COST)
            job_x(xg, dft, (nx - 1) * KV_COST / 10.0)
            dft.drain()
        for p in range(2):
            for j in range(FH // L):
                job_zs(i, p, j, bg, (1.6 * zb + extra, 0.5 * zb + extra), tied)
            assert not tied.tasks or (p == 0 and not last)
            if p == 0 and last:
                tied = _Tied(tasks(ln_z2, i, 8), LAST_N)
        if last:
            for s in range(8, 16):
                ln_z2(i, s)
        bg.drain()
        job_h(t, hbg, nh * KV_COST / 10.0)
        hbg.drain()

    def p1_block(g):
        for i in P1_GROUPS[g]:
            p1_step(i)

    for g in range(len(P1_GROUPS)):
        p1_wait(g)
        p1_start(g)
        block(lambda g=g: p1_block(g), f'p1_g{g}')

    groups = P2_GROUPS
    NG = len(groups)

    def p2_dma(gi):
        if gi >= 2:
            for i in groups[gi - 2]:
                start(cp_out(i))
        if gi >= 3:
            for i in groups[gi - 3]:
                wait(cp_out(i))
        if gi == 1:
            for i in (6, 7):
                start(cp_wsp(i))
        if gi == 0:
            wait(cp_conv(6))
        if gi + 1 < NG:
            for i in groups[gi + 1]:
                wait(cp_wsp(i))

    def tails_of(i, bg, budget):
        return [tail_gen(i, bg, budget)] * 20

    def p2_block(gi):
        bg = _Background()
        steps = groups[gi]
        tb = [0.0]
        pending = [t_ for i in (groups[gi - 1] if gi > 0 else []) for t_ in tails_of(i, bg, tb)]
        total = sum(a + 1 for i in steps for a in _blocks_of_step(i)) * 40 * 16
        total += len(steps) * (24 * E_COST + 6 * U_COST) + len(pending) * T_COST
        slots = sum(84 if i == 0 else 77 for i in steps) + TAIL_W * len(pending)
        bg.add(freq_gen(_blocks_of_step(steps[0])[0]))
        if gi == 0:
            bg.add(bcomb2_gen((0, 2, 3, 4, 6)))
            total += 5 * 16 * A_COST
        if gi < 2:
            bg.add(kv_gen(NT - 2 + gi))
            total += 20 * KV_COST
            slots += 10
        for t in P2_X[gi]:
            slots += 10
        if gi + 1 < NG:
            for i in groups[gi + 1]:
                bg.add(acomb2_gen(i))
                total += 16 * 7 * A2_COST
        for i in steps[1:]:
            bg.add(freq_gen(_blocks_of_step(i)[0]))
        budget = tb[0] = total / (slots + P2_END[gi])
        bg.run(budget)
        for t in P2_X[gi]:
            job_x(t, bg, budget)
        if gi < 2:
            job_h(NT - 2 + gi, bg, budget)
        units = [4, 4, 2, 4, 4, 2] * (len(pending) // 20)
        every = [0] * sum(6 if i == 0 else 9 for i in steps)
        for j, n in enumerate(units):
            every[min(len(every) - 1, j * len(every) // len(units))] += n
        for i in steps:
            job_big(i, bg, pending, budget, every)
        for t_ in pending:
            next(t_)
        bg.drain()

    for gi in range(NG):
        p2_dma(gi)
        block(lambda gi=gi: p2_block(gi), f'p2_{gi}')

    def cp_last(part):
        a0 = _blocks_of_step(NT - 1)[0]
        sub, cols = ((MC, pl.ds(0, D)), (0, pl.ds(0, 4 * L)), (0, pl.ds(4 * L, L)))[part]
        return [pltpu.make_async_copy(o_v.at[pl.ds(r, MC), cols], o_hbm.at[0, pl.ds(r, MC), cols],
                                      sem_out.at[NT - 1]) for r in (a0 * P + sub, (a0 + 1) * P + sub)]

    def p2_last():
        for i in groups[NG - 1]:
            for j, t_ in enumerate(tails_of(i, _Background(), [0.0])):
                next(t_)
                if i < NT - 1 and j == 19:
                    start(cp_out(i))
                if i == NT - 1 and j in (9, 17):
                    start(cp_last(j // 10))

    p2_dma(NG)
    block(p2_last, 'p2_last')
    start(cp_last(2))
    for i in groups[NG - 2] + groups[NG - 1][:-1]:
        wait(cp_out(i))
    for part in range(3):
        wait(cp_last(part))
    debug_keep_alive()


def _compiler_params():
    vmem = 124 * 1024 * 1024
    try:
        return pltpu.CompilerParams(vmem_limit_bytes=vmem, disable_semaphore_checks=True)
    except TypeError:
        return pltpu.CompilerParams(vmem_limit_bytes=vmem)


@jax.jit
def pallas_recurrent_scan__ssm_conv_h3__mixer_gmlp__prompt_kernel(
    A_q: jax.Array,
    A_k: jax.Array,
    A_v: jax.Array,
    A_shift_k: jax.Array,
    A_ssm_k: jax.Array,
    A_ssm_D: jax.Array,
    B_x: jax.Array,
    B_w_in: jax.Array,
    B_w_sp: jax.Array,
    B_b_sp: jax.Array,
    B_w_out: jax.Array,
):
    del B_x
    hbm = pl.BlockSpec(memory_space=pl.ANY)

    def bf16_buf(*shape):
        return pltpu.VMEM(shape[:-2] + (shape[-2] // 2, shape[-1]), U32)

    return pl.pallas_call(
        _kernel,
        out_shape=jax.ShapeDtypeStruct((1, S, D), BF16),
        in_specs=[hbm] * 10,
        out_specs=hbm,
        scratch_shapes=[
            [bf16_buf(len(g) * TM, D) for g in X_DMAS],
            [bf16_buf(len(g) * TM, D) for g in CONV_DMAS],
            [bf16_buf(len(g) * TM, D) for g in CONV_DMAS],
            [bf16_buf(D, len(g) * TM) for g in CONV_DMAS],
            [bf16_buf(D, max(hi - lo, 2) * L) for lo, hi in WIN_CHUNKS],
            [bf16_buf(TM, S) for _ in range(NT)],
            bf16_buf(FH, D),
            pltpu.VMEM((S, D), BF16),
            pltpu.VMEM((4, D), BF16),
            pltpu.VMEM((D,), BF16),
            pltpu.VMEM((S,), BF16),
            bf16_buf(S, D),
            bf16_buf(4 * 5 * P, KH),
            bf16_buf(5 * KH, FH),
            bf16_buf(5 * 5 * P, HN),
            bf16_buf(5 * HN, 2 * L),
            pltpu.VMEM((S, FH), F32),
            bf16_buf(7 * HK, HN),
            bf16_buf(5 * 5 * P, HK),
            bf16_buf(5 * 35 * MC, KQ),
            bf16_buf(21 * KQ, 2 * L),
            pltpu.VMEM((16 * MC, L), F32),
            pltpu.VMEM((HK, FH), F32),
            pltpu.VMEM((3, TM, FH), F32),
            bf16_buf(S, D),
            bf16_buf(S, FH),
            pltpu.VMEM((NB, 2, P, D), F32),
            pltpu.VMEM((2, 2, P, D), F32),
            pltpu.VMEM((NB, 2, P, D), F32),
            bf16_buf(NB * 2 * P, D),
            pltpu.VMEM((2, D // L, MC, L), F32),
            bf16_buf(2 * P, 2 * P),
            bf16_buf(MC, 2 * P),
            pltpu.VMEM((S, L), F32),
            pltpu.VMEM((2, P, L), F32),
            pltpu.VMEM((4, 8, D), F32),
            pltpu.VMEM((D // L, S + 8, L), F32),
            pltpu.SemaphoreType.DMA((1,)),
            pltpu.SemaphoreType.DMA((NT,)),
            pltpu.SemaphoreType.DMA((NT,)),
            pltpu.SemaphoreType.DMA((NT,)),
            pltpu.SemaphoreType.DMA((5,)),
            pltpu.SemaphoreType.DMA((NT,)),
        ],
        compiler_params=_compiler_params(),
    )(A_q, A_k, A_v, A_shift_k.T, A_ssm_k, A_ssm_D, B_w_in, B_w_sp, B_b_sp, B_w_out)
```

```python
import math

import jax
import jax.numpy as jnp
import jax.experimental.pallas as pl
import jax.experimental.pallas.tpu as pltpu

S = 2048
D = 640
FH = 768
P = 128
NB = S // P
TM = 256
NT = S // TM
MC = 64
L = 128
HK = S // 2
KQ = HK // 2
KH = 256
HN = FH // 2
EPS = 1e-5
F32 = jnp.float32
BF16 = jnp.bfloat16
U32 = jnp.uint32
GELU_C = math.sqrt(2.0 / math.pi)
GA = (GELU_C * 0.044715) ** (1.0 / 3.0)
NT_DIMS = (((1,), (1,)), ((), ()))

WIN_CHUNKS = ((6, 7), (7, 9), (9, 12), (0, 3), (3, 6))
X_DMAS = ((0,), (1,), (2,), (3,), (4, 5), (6, 7))
CONV_DMAS = ((0,), (1,), (2, 3), (4, 5), (6, 7))
P1_GROUPS = ((2,), (3,), (4, 5), (6, 7))
P1_X = {2: None, 3: 0, 4: 1, 5: None, 6: 2, 7: 3}
P1_LNX = {2: (3,), 3: (4, 5), 4: (6,), 5: (7,), 6: (), 7: ()}
P2_GROUPS = ((0,), (1, 2), (3, 4, 5), (6, 7))
P2_X = ((4, 5), (6,), (7,), ())
STEP_BLOCKS = ((2, 3), (6, 7), (4, 5), (12, 13), (10, 11), (0, 1), (14, 15), (8, 9))
KV_COST, A_COST, A2_COST = 110, 56, 34
E_COST, U_COST, T_COST, TAIL_W = 24, 90, 90, 1.6
KV_SPLIT = {2: (0, 14, 6), 3: (12, 4, 4), 4: (12, 4, 4), 5: (0, 14, 6), 6: (12, 4, 4), 7: (12, 4, 4)}
FR = 8
L1_USE = {0: ((0, 1, True, False), (3, 1, True, False)), 6: ((0, 1, False, False),),
          3: ((0, 1, False, False), (2, 1, True, False)), 4: ((0, -1, False, True), (1, 1, True, False)),
          1: ((2, 1, False, True), (3, -1, False, False)), 2: ((1, 1, False, True), (3, 1, False, False)),
          5: ((3, 1, False, True),)}
H_SPLIT = ((0, 2), (2, 4), (4, 5))
P1_TUNE = {2: (42, 0), 3: (43, 1), 4: (42, 0), 5: (42, 0), 6: (44, 0), 7: (24, 0)}
EXTRA = (52, 52)
LAST_N = 22
P2_END = (0.0, -1.0, -1.0, 0.0)
F_TIED = (20, 20, 18, 20, 20)
_ONLY = None


def _dot(a, b):
    return jnp.dot(a, b, preferred_element_type=F32)


def _sums_left(a11, a12, a21, a22):
    add, sub = jax.lax.add, jax.lax.sub
    return jnp.concatenate((add(a11, a22), add(a21, a22), add(a11, a12), sub(a21, a11), sub(a12, a22)),
                           axis=1).astype(BF16)


def _sums_right(b11, b12, b21, b22):
    add, sub = jax.lax.add, jax.lax.sub
    return jnp.concatenate((add(b11, b22), sub(b12, b22), sub(b21, b11), add(b11, b12), add(b21, b22)),
                           axis=1).astype(BF16)


def _cos_sin(m):
    q = (m + 256) >> 9
    x = (m - (q << 9)).astype(F32) * (2.0 * math.pi / 2048.0)
    x2 = x * x
    s = x * (1.0 + x2 * (-1.0 / 6 + x2 * (1.0 / 120 + x2 * (-1.0 / 5040 + x2 * (1.0 / 362880)))))
    c = 1.0 + x2 * (-0.5 + x2 * (1.0 / 24 + x2 * (-1.0 / 720 + x2 * (1.0 / 40320 - x2 * (1.0 / 3628800)))))
    swap = (q & 1) == 1
    c0 = jnp.where(swap, s, c)
    s0 = jnp.where(swap, c, s)
    cos = jnp.where(((q + 1) & 2) == 2, -c0, c0)
    sin = jnp.where((q & 2) == 2, -s0, s0)
    return cos, sin


def _odd_freq(r):
    return jnp.where(r < 64, 4 * r + 1, 4 * r - 253)


def _gelu_scaled(z):
    return z + z * jnp.tanh(z * (GELU_C / GA + z * z))


def _signzero(z):
    bits = jax.lax.bitcast_convert_type(z, U32) & jnp.uint32(0x80000000)
    return jax.lax.bitcast_convert_type(bits, F32)


def _ln(x, eps, tie=None, scale=None):
    n = x.shape[-1]
    cols = [x[:, j * L:(j + 1) * L] for j in range(n // L)]
    s1 = cols[0]
    s2 = cols[0] * cols[0]
    for c in cols[1:]:
        s1 = s1 + c
        s2 = s2 + c * c
    if tie is not None:
        s1 = s1 + tie
        s2 = s2 + tie
    m = jnp.sum(s1, axis=-1, keepdims=True) * (1.0 / n)
    v = jnp.maximum(jnp.sum(s2, axis=-1, keepdims=True) * (1.0 / n) - m * m, 0.0)
    rs = jax.lax.rsqrt(v + eps)
    if scale is not None:
        rs = rs * scale
    return (x - m) * rs


def _blocks_of_step(i):
    return STEP_BLOCKS[i]


class _Background:
    def __init__(self):
        self.q = []
        self.credit = 0.0

    def add(self, gen):
        self.q.append(gen)

    def run(self, budget):
        self.credit += budget
        while self.q and self.credit > 0:
            try:
                self.credit -= next(self.q[0])
            except StopIteration:
                self.q.pop(0)
        if not self.q:
            self.credit = 0.0

    def charge(self, cost):
        self.credit -= cost

    def drain(self):
        while self.q:
            self.run(1e9)


class _Tied:
    def __init__(self, tasks, npieces):
        self.tasks = list(tasks)
        self.rate = len(self.tasks) / float(npieces)
        self.credit = 0.999

    def run(self, z):
        self.credit += self.rate
        n = 0
        while self.tasks and self.credit >= 1.0:
            self.tasks.pop(0)(_signzero(z[0:16]))
            self.credit -= 1.0
            n += 1
        return n


def _kernel(q_hbm, k_hbm, v_hbm, sk_hbm, h_hbm, d_hbm, win_hbm, wsp_hbm, b_hbm, wout_hbm,
            o_hbm,
            x_us, k_us, v_us, h_us, win_us, wsp_us, wout_u, o_v, sk_in, d_in, b_in,
            xn_u, XL_u, WB_u, UL_u, WO_u, z1_v, R_u, Lc_u, L2_u, R2_u, C_v, zf_v, zg_v, kv_u, u_u, X_v, H_v, G_v, Z_u,
            yl_v, F_u, Fi_u, bcol_v, ph_v, sk_v, kf_v,
            sem_small, sem_x, sem_conv, sem_wsp, sem_w, sem_out):
    (wout_v, xn_v, XL_v, WB_v, UL_v, WO_v, R_v, Lc_v, L2_v, R2_v, kv_v, u_v, Z_v, F_v, Fi_v) = [
        r.bitcast(BF16) for r in (wout_u, xn_u, XL_u, WB_u, UL_u, WO_u, R_u, Lc_u, L2_u, R2_u, kv_u, u_u, Z_u, F_u, Fi_u)]
    x_vs = {g[0]: r.bitcast(BF16) for g, r in zip(X_DMAS, x_us)}
    k_vs, v_vs, h_vs = [{g[0]: r.bitcast(BF16) for g, r in zip(CONV_DMAS, rs)} for rs in (k_us, v_us, h_us)]
    wsp_vs = [r.bitcast(BF16) for r in wsp_us]
    win_vs = [r.bitcast(BF16) for r in win_us]

    def win(rows, n):
        c = [lo <= n < hi for lo, hi in WIN_CHUNKS].index(True)
        n -= WIN_CHUNKS[c][0]
        return win_vs[c][rows, n * L:(n + 1) * L]

    def locate(bufs, row):
        t0 = max(t for t in bufs if t * TM <= row)
        return bufs[t0], row - t0 * TM

    def rows_of(bufs, row, n, lanes=slice(None)):
        buf, r = locate(bufs, row)
        return buf[r:r + n, lanes]

    def cp_small():
        return [pltpu.make_async_copy(s_, d_, sem_small.at[0])
                for s_, d_ in ((d_hbm, d_in), (sk_hbm, sk_in), (b_hbm, b_in))]

    def cp_x(t):
        return pltpu.make_async_copy(q_hbm.at[0, pl.ds(t * TM, x_vs[t].shape[0])], x_vs[t], sem_x.at[t])

    def cp_conv(t):
        rows = pl.ds(t * TM, k_vs[t].shape[0])
        sem = sem_conv.at[t]
        return [pltpu.make_async_copy(h_hbm.at[:, rows], h_vs[t], sem),
                pltpu.make_async_copy(k_hbm.at[0, rows], k_vs[t], sem),
                pltpu.make_async_copy(v_hbm.at[0, rows], v_vs[t], sem)]

    def cp_wsp(i):
        return [pltpu.make_async_copy(wsp_hbm.at[pl.ds(_blocks_of_step(i)[0] * P, TM)], wsp_vs[i], sem_wsp.at[i])]

    def cp_win(c):
        lo, hi = WIN_CHUNKS[c]
        w = (hi - lo) * L
        return pltpu.make_async_copy(win_hbm.at[:, pl.ds(lo * L, w)], win_vs[c].at[:, pl.ds(0, w)], sem_w.at[c])

    def cp_wout():
        return pltpu.make_async_copy(wout_hbm, wout_v, sem_w.at[0])

    def cp_out(i):
        rows = pl.ds(_blocks_of_step(i)[0] * P, TM)
        return [pltpu.make_async_copy(o_v.at[rows], o_hbm.at[0, rows], sem_out.at[i])]

    def start(cs):
        for c in cs:
            c.start()

    def wait(cs):
        for c in cs:
            c.wait()

    def block(fn, name):
        def body(it):
            fn()
            return it + 1

        if _ONLY is None or name in _ONLY:
            jax.lax.while_loop(lambda it: it < 1, body, jnp.int32(0))

    def ln_x(t, s, tie=None):
        rows = pl.ds(t * TM + s * 16, 16)
        y = _ln(rows_of(x_vs, t * TM + s * 16, 16).astype(F32), EPS, tie, GA)
        xn_v[rows, :] = y.astype(BF16)
        return y

    def ln_x2(t, s, tie):
        p, q = s // 4, s % 4
        y1 = ln_x(t, 8 * p + q, tie)
        y2 = ln_x(t, 8 * p + 4 + q, tie)
        a11, a12, a21, a22 = y1[:, :KH], y1[:, KH:2 * KH], y2[:, :KH], y2[:, KH:2 * KH]
        XL_v[pl.ds((t % 4) * P + p * MC + q * 16, 16), :] = _sums_left(a11, a12, a21, a22)

    def wcomb_gen(cols):
        for j in cols:
            for r in range(KH // 32):
                top = pl.ds(r * 32, 32)
                bot = pl.ds(KH + r * 32, 32)
                b11, b12 = win(top, j).astype(F32), win(top, 6 + j).astype(F32)
                b21, b22 = win(bot, j).astype(F32), win(bot, 6 + j).astype(F32)
                WB_v[top, j * 5 * L:(j + 1) * 5 * L] = _sums_right(b11, b12, b21, b22)
                yield A_COST

    def ln_z2(t, s, tie=None):
        y = _ln(zg_v[t % 3, s * 16:(s + 1) * 16, :], 4.0 * GA * GA * EPS, tie, 0.25 / GA)
        lo, hi = y[:, :HN], y[:, HN:]
        rows = pl.ds((t * TM + s * 16) % HK, 16)
        if t < NT // 2:
            zf_v[rows, :] = y
            R_v[rows, 0:2 * HN] = jnp.concatenate((lo, lo + hi), axis=1).astype(BF16)
        else:
            b11, b12 = zf_v[rows, :HN], zf_v[rows, HN:]
            R_v[rows, 2 * HN:] = jnp.concatenate((b11 + hi, b12 - hi, lo - b11, hi, lo + hi), axis=1).astype(BF16)

    def r1(j, rows, n):
        c0 = {1: 0, 5: 1, 0: 2, 2: 3, 3: 4, 4: 5, 6: 6}[j] * HN + n * L
        return R_v[rows, c0:c0 + L]

    def acomb_gen(i, groups=range(P // 16)):
        for r in groups:
            for c in range(HK // 256):
                top = pl.ds(r * 16, 16)
                bot = pl.ds(P + r * 16, 16)
                c1 = slice(c * 256, (c + 1) * 256)
                c2 = slice(HK + c * 256, HK + (c + 1) * 256)
                a11 = wsp_vs[i][top, c1].astype(F32)
                a12 = wsp_vs[i][top, c2].astype(F32)
                a21 = wsp_vs[i][bot, c1].astype(F32)
                a22 = wsp_vs[i][bot, c2].astype(F32)
                r0 = (i % 5) * 5 * P + (r % 4 * 2 + r // 4) * 16
                Lc_v[pl.ds(r0 + 0 * P, 16), c1] = (a11 + a22).astype(BF16)
                Lc_v[pl.ds(r0 + 1 * P, 16), c1] = (a21 + a22).astype(BF16)
                Lc_v[pl.ds(r0 + 2 * P, 16), c1] = (a11 + a12).astype(BF16)
                Lc_v[pl.ds(r0 + 3 * P, 16), c1] = (a21 - a11).astype(BF16)
                Lc_v[pl.ds(r0 + 4 * P, 16), c1] = (a12 - a22).astype(BF16)
                yield A_COST

    def acomb2_gen(i):
        for r in range(MC // 16):
            for c in range(KQ // L):
                quad = {}

                def w(b, H):
                    if (b, H) not in quad:
                        quad[b, H] = [[wsp_vs[i][pl.ds(b * P + s_ * MC + r * 16, 16),
                                                 H * HK + kh * KQ + c * L:H * HK + kh * KQ + (c + 1) * L].astype(F32)
                                       for kh in range(2)] for s_ in range(2)]
                    return quad[b, H]

                spec = {2: (None, (0, 0), None, 0), 0: (0, (0, 0), (1, 1), 1), 3: (None, (1, 1), None, 0),
                        1: (1, (1, 0), (1, 1), 1), 5: (3, (1, 0), (0, 0), -1), 4: (2, (0, 0), (0, 1), 1),
                        6: (4, (0, 1), (1, 1), -1)}
                for j in (2, 0, 3, 1, 5, 4, 6):
                    slot, p_, q_, sign = spec[j]
                    a = w(*p_)
                    if q_ is not None:
                        b_ = w(*q_)
                        op = jax.lax.add if sign > 0 else jax.lax.sub
                        a = [[op(a[s_][kh], b_[s_][kh]) for kh in range(2)] for s_ in range(2)]
                        for kh in range(2):
                            Lc_v[pl.ds(((i % 5) * 5 + slot) * P + r * 32, 32),
                                 kh * KQ + c * L:kh * KQ + (c + 1) * L] = jnp.concatenate(
                                     (a[0][kh], a[1][kh]), axis=0).astype(BF16)
                    L2_v[pl.ds(((i % 5) * 7 + j) * MC + r * 16, 16), c * 5 * L:(c + 1) * 5 * L] = _sums_left(
                        a[0][0], a[0][1], a[1][0], a[1][1])
                    yield A2_COST

    def bcomb2_gen(js):
        for j in js:
            for r in range(KQ // 16):
                top = pl.ds(r * 16, 16)
                bot = pl.ds(KQ + r * 16, 16)
                R2_v[pl.ds(j * KQ + r * 16, 16), :] = _sums_right(
                    *[r1(j, rows, n).astype(F32) for rows in (top, bot) for n in range(2)])
                yield A_COST / 2

    def tasks(fn, t, n=TM // 16):
        return [lambda tie, s=s: fn(t, s, tie) for s in range(n)]

    def kv_gen(t):
        for m in range(TM // MC):
            r = t * TM + m * MC
            for l in range(D // L):
                lanes = slice(l * L, (l + 1) * L)
                kf = rows_of(k_vs, r, MC, lanes).astype(F32)
                kf_v[l, pl.ds(r + 8, MC), :] = kf
                ks = kf * sk_v[0, 0:1, lanes]
                for tap in range(1, 4):
                    ks = ks + kf_v[l, pl.ds(r + 8 - tap, MC), :] * sk_v[tap, 0:1, lanes]
                kv = ks * rows_of(v_vs, r, MC, lanes).astype(F32)
                kv_v[pl.ds(r, MC), lanes] = kv.astype(BF16)
                yield KV_COST

    def freq_gen(a):
        def cmac(acc, x, g):
            mul, add = jax.lax.mul, jax.lax.add
            pr = jax.lax.sub(mul(x[0], g[0]), mul(x[1], g[1]))
            pi = add(mul(x[0], g[1]), mul(x[1], g[0]))
            return (pr, pi) if acc is None else (add(acc[0], pr), add(acc[1], pi))

        for r in range(P // 16):
            for l in range(D // L):
                lanes = slice(l * L, (l + 1) * L)
                res = []
                for sub in range(16 // FR):
                    rows = pl.ds(r * 16 + sub * FR, FR)
                    lo = hi = None
                    g = (G_v[a + 1, 0, rows, lanes], G_v[a + 1, 1, rows, lanes])
                    for c in range(a + 2):
                        x = (X_v[c, 0, rows, lanes], X_v[c, 1, rows, lanes])
                        hi = cmac(hi, x, g)
                        if c <= a:
                            g = (G_v[a - c, 0, rows, lanes], G_v[a - c, 1, rows, lanes])
                            lo = cmac(lo, x, g)
                            yield 2 * FR
                    res.append((lo, hi))
                Z_v[pl.ds(a // 2 * P + r * 16, 16), l * 4 * L:(l + 1) * 4 * L] = jnp.concatenate(
                    [jnp.concatenate([z[0][0], z[0][1], z[1][0], z[1][1]], axis=1) for z in res], axis=0).astype(BF16)
                yield 20

    def job_x(t, bg, budget):
        for j in (2 * t, 2 * t + 1):
            for half in range(2):
                r = _dot(F_v[half * P:(half + 1) * P, 0:P], kv_v[j * P:(j + 1) * P, :]).reshape(8, 2, 8, D)
                for part in range(2):
                    X_v[j, part, half * 64:(half + 1) * 64, :] = r[:, part].reshape(64, D)
                bg.run(budget * 2.5)

    def job_h(t, bg, budget):
        h_v, c0 = locate(h_vs, t * TM)
        for half in range(2):
            rows = pl.ds(half * 64, 64)
            for l0, l1 in H_SPLIT:
                w = (l1 - l0) * L
                lanes = slice(l0 * L, l1 * L)
                rhs = jnp.concatenate([h_v[lanes, c0:c0 + P], h_v[lanes, c0 + P:c0 + TM]], axis=0)
                r = jax.lax.dot_general(F_v[half * P:(half + 1) * P, 0:P], rhs, NT_DIMS,
                                        preferred_element_type=F32).reshape(8, 2, 8, 2 * w)
                re, im = r[:, 0].reshape(64, 2 * w), r[:, 1].reshape(64, 2 * w)
                prev = (H_v[t % 2, 0, rows, lanes], H_v[t % 2, 1, rows, lanes])
                for j in range(2):
                    cur = (re[:, j * w:(j + 1) * w], im[:, j * w:(j + 1) * w])
                    G_v[2 * t + j, 0, rows, lanes] = cur[0] + prev[1] if half else cur[0] - prev[1]
                    G_v[2 * t + j, 1, rows, lanes] = cur[1] - prev[0] if half else cur[1] + prev[0]
                    prev = cur
                if t + 1 < NT:
                    H_v[(t + 1) % 2, 0, rows, lanes] = prev[0]
                    H_v[(t + 1) % 2, 1, rows, lanes] = prev[1]
                bg.run(budget * (l1 - l0))

    def z_out(t, m, n, pre, bg, budget, tied):
        z = _gelu_scaled(pre)
        if n < FH // L:
            z1_v[pl.ds(t * TM + m * MC, MC), n * L:(n + 1) * L] = z
        else:
            zg_v[t % 3, m * MC:(m + 1) * MC, n * L - FH:(n + 1) * L - FH] = z
        ntask = tied.run(z)
        bg.run(budget[1] if ntask else budget[0])

    def job_z(t, m, cols, bg, budget, tied):
        for n in cols:
            z_out(t, m, n, _dot(xn_v[pl.ds(t * TM + m * MC, MC), :], win(slice(None), n)), bg, budget, tied)

    def job_zs(t, p, j, bg, budget, tied):
        r1 = pl.ds(t * TM + p * P, MC)
        r2 = pl.ds(t * TM + p * P + MC, MC)

        def xl(w):
            r0 = (t % 4) * P + p * MC
            return XL_v[r0:r0 + MC, w * KH:(w + 1) * KH]

        def wb(w):
            return WB_v[:, (j * 5 + w) * L:(j * 5 + w + 1) * L]

        def rem(rows, n):
            return _dot(xn_v[rows, 2 * KH:], win(slice(2 * KH, D), n))

        m2 = _dot(xl(1), win(slice(0, KH), j))
        m4 = _dot(xn_v[r2, KH:2 * KH], wb(2))
        z_out(t, 2 * p + 1, j, m2 + m4 + rem(r2, j), bg, budget, tied)
        m3 = _dot(xn_v[r1, 0:KH], wb(1))
        m5 = _dot(xl(2), win(slice(KH, 2 * KH), 6 + j))
        z_out(t, 2 * p, 6 + j, m3 + m5 + rem(r1, 6 + j), bg, budget, tied)
        t11, t22 = m4 - m5, m3 - m2
        m1 = _dot(xl(0), wb(0))
        t11, t22 = t11 + m1, t22 + m1
        z_out(t, 2 * p, j, t11 + _dot(xl(4), wb(4)) + rem(r1, j), bg, budget, tied)
        z_out(t, 2 * p + 1, 6 + j, t22 + _dot(xl(3), wb(3)) + rem(r2, 6 + j), bg, budget, tied)

    rev8 = 7 - jax.lax.broadcasted_iota(jnp.int32, (8, L), 0)

    def finish(a, upper, n, hh, slot):
        rows = pl.ds(a * P + (MC if upper else 0), MC)
        lanes = slice(n * L, (n + 1) * L)
        if upper:
            zc = (n * 4 + a % 2 * 2) * L
            ya = _dot(Fi_v[:, 0:P], Z_v[a // 2 * P:(a // 2 + 1) * P, zc:zc + L])
            yb = _dot(Fi_v[:, P:2 * P], Z_v[a // 2 * P:(a // 2 + 1) * P, zc + L:zc + 2 * L])
            slot(0.5)
            y = ya - yb
            lo = ya + yb
            for j in range(MC // 8):
                yl_v[a % 2, n, (7 - j) * 8:(8 - j) * 8, :] = jnp.take_along_axis(lo[j * 8:(j + 1) * 8], rev8, axis=0)
        else:
            y = yl_v[a % 2, n]
        gate = hh + hh * jnp.tanh(hh)
        s = xn_v[rows, lanes].astype(F32) * y
        x = rows_of(x_vs, a * P + (MC if upper else 0), MC, lanes).astype(F32)
        o_v[rows, lanes] = (x + s * gate).astype(BF16)

    def tail_gen(i, bg, budget):
        a0, a1 = _blocks_of_step(i)

        def slot(w):
            bg.run(w * budget[0])

        def dot3(a, b):
            r = _dot(a, b)
            slot(0.75)
            return r

        for upper in (True, False):
            sub = MC if upper else 0
            r1 = pl.ds(a0 * P + sub, MC)
            r2 = pl.ds(a1 * P + sub, MC)

            def ul(w):
                allw = UL_v[(i % 5) * P + sub:(i % 5) * P + sub + MC, :]
                return jnp.concatenate([allw[:, (n * 5 + w) * L:(n * 5 + w + 1) * L] for n in range(HN // L)], axis=1)

            for j in range(2):
                c1 = slice(j * L, (j + 1) * L)
                c2 = slice((2 + j) * L, (3 + j) * L)

                def wo(w):
                    return WO_v[:, (j * 5 + w) * L:(j * 5 + w + 1) * L]

                m2 = dot3(ul(1), wout_v[0:HN, c1])
                m4 = dot3(u_v[r2, HN:], wo(2))
                finish(a1, upper, j, m2 + m4, slot)
                bg.charge(T_COST)
                yield
                m3 = dot3(u_v[r1, 0:HN], wo(1))
                m5 = dot3(ul(2), wout_v[HN:, c2])
                finish(a0, upper, 2 + j, m3 + m5, slot)
                bg.charge(T_COST)
                yield
                t11, t22 = m4 - m5, m3 - m2
                m1 = dot3(ul(0), wo(0))
                t11, t22 = t11 + m1, t22 + m1
                finish(a0, upper, j, t11 + dot3(ul(4), wo(4)), slot)
                bg.charge(T_COST)
                yield
                finish(a1, upper, 2 + j, t22 + dot3(ul(3), wo(3)), slot)
                bg.charge(T_COST)
                yield
            for a, r in ((a0, r1), (a1, r2)):
                finish(a, upper, 4, dot3(u_v[r, 0:HN], wout_v[0:HN, 4 * L:]) + dot3(u_v[r, HN:], wout_v[HN:, 4 * L:]),
                       slot)
                bg.charge(T_COST)
                yield

    def wocomb_gen():
        for j in range(2):
            c1 = slice(j * L, (j + 1) * L)
            c2 = slice((2 + j) * L, (3 + j) * L)
            for r in range(HN // 32):
                top = pl.ds(r * 32, 32)
                bot = pl.ds(HN + r * 32, 32)
                b11, b12 = wout_v[top, c1].astype(F32), wout_v[top, c2].astype(F32)
                b21, b22 = wout_v[bot, c1].astype(F32), wout_v[bot, c2].astype(F32)
                WO_v[top, j * 5 * L:(j + 1) * 5 * L] = _sums_right(b11, b12, b21, b22)
                yield A_COST

    def job_big(i, bg, pending, budget, every):
        a0, a1 = _blocks_of_step(i)
        KG = 512

        def lhs(j, sub, cols):
            if j == 2:
                return wsp_vs[i][sub:sub + MC, cols]
            if j == 3:
                return wsp_vs[i][P + sub:P + sub + MC, HK + cols.start:HK + cols.stop]
            r0 = ((i % 5) * 5 + {0: 0, 1: 1, 4: 2, 5: 3, 6: 4}[j]) * P
            both = Lc_v[r0:r0 + P, cols]
            return jnp.concatenate([both[q * 32 + sub // 4:q * 32 + sub // 4 + 16] for q in range(4)], axis=0)

        def prod(j, sub, n, acc=None):
            for kg in range(HK // KG):
                ks = slice(kg * KG, (kg + 1) * KG)
                p = _dot(lhs(j, sub, ks), r1(j, ks, n))
                acc = p if acc is None else acc + p
                bg.run(budget)
            return acc

        def tails(n):
            for _ in range(n):
                if pending:
                    next(pending.pop(0))

        def emit(a, sub, n, g):
            rows = pl.ds(a * P + sub, MC)
            lanes = slice(n * L, (n + 1) * L)
            u = z1_v[rows, lanes] * (g + bcol_v[rows, :])
            u_v[rows, lanes] = u.astype(BF16)
            bg.charge(E_COST)
            return u

        if i > 0:
            def piece(a, b, acc=None):
                p = _dot(a, b)
                bg.run(budget)
                return p if acc is None else acc + p

            def cslot(k, s_, n):
                return pl.ds(((k * 2 + s_) * 2 + n) * MC, MC)

            def contribute(j, s_, n, m):
                for k, sign, first, last in L1_USE[j]:
                    cs = cslot(k, s_, n)
                    v_ = m if first else (C_v[cs, :] + m if sign > 0 else C_v[cs, :] - m)
                    if last:
                        u = emit((a0, a0, a1, a1)[k], s_ * MC, n + (k % 2) * (HN // L), v_)
                        v_ = u
                        if k == 3:
                            u11, u12, u21 = C_v[cslot(0, s_, n), :], C_v[cslot(1, s_, n), :], C_v[cslot(2, s_, n), :]
                            UL_v[pl.ds((i % 5) * P + s_ * MC, MC), n * 5 * L:(n + 1) * 5 * L] = _sums_left(
                                u11, u12, u21, u)
                            bg.charge(U_COST)
                            continue
                    C_v[cs, :] = v_

            for j in (0, 6, 3, 4, 1, 2, 5):
                def l2(w):
                    r0 = ((i % 5) * 7 + j) * MC
                    allw = L2_v[r0:r0 + MC, :]
                    return jnp.concatenate([allw[:, (c * 5 + w) * L:(c * 5 + w + 1) * L] for c in range(KQ // L)],
                                           axis=1)

                def r2(w):
                    return R2_v[j * KQ:(j + 1) * KQ, w * L:(w + 1) * L]

                def rq(kh, n):
                    return r1(j, slice(kh * KQ, (kh + 1) * KQ), n)

                p2 = piece(l2(1), rq(0, 0))
                p4 = piece(lhs(j, MC, slice(KQ, 2 * KQ)), r2(2))
                contribute(j, 1, 0, p2 + p4)
                p3 = piece(lhs(j, 0, slice(0, KQ)), r2(1))
                t22 = p3 - p2
                p5 = piece(l2(2), rq(1, 1))
                contribute(j, 0, 1, p3 + p5)
                t11 = p4 - p5
                p1 = piece(l2(0), r2(0))
                t11, t22 = t11 + p1, t22 + p1
                contribute(j, 0, 0, piece(l2(4), r2(4), t11))
                contribute(j, 1, 1, piece(l2(3), r2(3), t22))
                tails(every.pop(0))

        for sub in (0, MC):
            for n in (range(HN // L) if i == 0 else (2,)):
                def put(w, c):
                    UL_v[pl.ds((i % 5) * P + sub, MC), (n * 5 + w) * L:(n * 5 + w + 1) * L] = c.astype(BF16)

                m1 = prod(0, sub, n)
                t11 = prod(6, sub, n, m1)
                m4 = prod(3, sub, n)
                t11 = t11 + m4
                m5 = prod(4, sub, n)
                u11 = emit(a0, sub, n, t11 - m5)
                m2 = prod(1, sub, n)
                u21 = emit(a1, sub, n, m2 + m4)
                put(3, u21 - u11)
                t22 = m1 - m2
                m3 = prod(2, sub, n)
                u12 = emit(a0, sub, n + HN // L, m3 + m5)
                put(2, u11 + u12)
                u22 = emit(a1, sub, n + HN // L, prod(5, sub, n, t22 + m3))
                put(0, u11 + u22)
                put(1, u21 + u22)
                put(4, u12 - u22)
                bg.charge(U_COST)
                tails(every.pop(0))

    def debug_keep_alive():
        if _ONLY is not None:
            for r_ in (xn_u, XL_u, WB_u, UL_u, WO_u, z1_v, R_u, Lc_u, L2_u, R2_u, C_v, zf_v, zg_v, kv_u, u_u, X_v, H_v, G_v, Z_u,
                       kf_v, bcol_v):
                c_ = pltpu.make_async_copy(r_, r_, sem_small.at[0])
                c_.start()
                c_.wait()

    debug_keep_alive()

    cp_x(0).start()
    cp_win(0).start()
    cp_x(1).start()
    cp_win(1).start()
    start(cp_small())
    for c in range(2, 5):
        cp_win(c).start()
    cp_x(2).start()

    kk = _odd_freq(jax.lax.broadcasted_iota(jnp.int32, (P, P), 0))
    nn = jax.lax.broadcasted_iota(jnp.int32, (P, P), 1)
    fc, fs = _cos_sin((kk * (4 * nn - 127)) & 2047)
    for g in range(P // 8):
        F_v[g * 16:(g + 1) * 16, 0:P] = jnp.concatenate(
            [fc[g * 8:(g + 1) * 8], -fs[g * 8:(g + 1) * 8]], axis=0).astype(BF16)
    fc, fs = _cos_sin((kk * (-127)) & 2047)
    ph_v[0] = fc
    ph_v[1] = fs
    kk = _odd_freq(jax.lax.broadcasted_iota(jnp.int32, (MC, P), 1))
    mm = jax.lax.broadcasted_iota(jnp.int32, (MC, P), 0)
    ic, is_ = _cos_sin((kk * (4 * mm + 2)) & 2047)
    Fi_v[:, 0:P] = (ic * (1.0 / (P * GA))).astype(BF16)
    Fi_v[:, P:2 * P] = (is_ * (1.0 / (P * GA))).astype(BF16)
    kf_v[:, 0:8, :] = jnp.zeros((D // L, 8, L), F32)

    cp_x(0).wait()
    for s in range(TM // 16):
        ln_x(0, s)

    def small_setup():
        sk = sk_in[...].astype(F32)
        for t in range(4):
            sk_v[t] = jnp.broadcast_to(sk[t:t + 1], (8, D))
        drow = d_in[...].astype(F32).reshape(1, D)
        for l in range(D // L):
            lanes = slice(l * L, (l + 1) * L)
            dre = ph_v[0] * drow[:, lanes]
            dim = ph_v[1] * drow[:, lanes]
            H_v[0, 0, 0:64, lanes] = -dim[0:64]
            H_v[0, 0, 64:P, lanes] = dim[64:P]
            H_v[0, 1, 0:64, lanes] = -dre[0:64]
            H_v[0, 1, 64:P, lanes] = dre[64:P]

    def bcol_task(t, j, tie):
        brow = b_in[...].astype(F32).reshape(1, S)[:, j * P:(j + 1) * P] * (0.25 / GA) + tie[0:1]
        bcol_v[j * P:(j + 1) * P, :] = jnp.broadcast_to(brow, (P, P)).T

    LAG = 2

    def interleave(*lists):
        out = []
        for j in range(max(len(a) for a in lists)):
            for a in lists:
                out += a[j:j + 1]
        return out

    def p1_first(c):
        bg = _Background()
        todo = []
        if c == 2:
            todo = tasks(bcol_task, 0)
            small_setup()
        if c == 3:
            todo = tasks(ln_z2, 0)
            bg.add(wcomb_gen(range(3)))
        if c == 4:
            todo = tasks(ln_x2, 2, 8)
            bg.add(wcomb_gen(range(3, 6)))
        tied = _Tied(todo, F_TIED[c])
        if c == 0:
            for s in range(TM // 16):
                ln_x(1, s)
        for t in range(2):
            for m in range(TM // MC):
                job_z(t, m, range(*WIN_CHUNKS[c]), bg, (80, 40), tied)
        bg.drain()
        assert not tied.tasks

    for c in range(5):
        cp_win(c).wait()
        if c == 0:
            cp_x(1).wait()
        if c == 2:
            wait(cp_small())
            start(cp_conv(0))
            cp_x(3).start()
        if c == 4:
            cp_x(2).wait()
            cp_x(4).start()
        block(lambda c=c: p1_first(c), f'p1_f{c}')

    def p1_wait(g):
        if g == 0:
            wait(cp_conv(0))
            cp_x(3).wait()
        if g == 1:
            wait(cp_conv(1))
            cp_x(4).wait()
        if g == 2:
            wait(cp_conv(2))
            cp_x(6).wait()
        if g == 3:
            wait(cp_conv(4))
            cp_wout().wait()
            wait(cp_wsp(0))

    def p1_start(g):
        if g == 0:
            start(cp_conv(1))
            cp_x(6).start()
            start(cp_conv(2))
        if g == 1:
            start(cp_conv(4))
            cp_wout().start()
            start(cp_wsp(0))
            start(cp_wsp(1))
        if g == 3:
            start(cp_wsp(2))
            start(cp_conv(6))
            for i in (3, 4, 5):
                start(cp_wsp(i))

    def take(gen, n):
        for _ in range(n):
            yield next(gen)

    def p1_step(i):
        bg = _Background()
        dft = _Background()
        t = i - LAG
        xg = P1_X[i]
        kv = kv_gen(t)
        nx, nz, nh = KV_SPLIT[i]
        dft.add(take(kv, nx))
        bg.add(take(kv, nz))
        hbg = _Background()
        hbg.add(take(kv, nh))
        zb = nz * KV_COST / 48.0
        extra = 0
        if i == 6:
            bg.add(wocomb_gen())
            bg.add(acomb_gen(0, range(5)))
            extra = EXTRA[0]
        if i == 7:
            bg.add(acomb_gen(0, range(5, 8)))
            bg.add(bcomb2_gen((1, 5)))
            extra = EXTRA[1]
        last = i == NT - 1
        z2t = tasks(ln_z2, i - 1)
        xt = [tasks(ln_x2, t_, 8) for t_ in P1_LNX[i]]
        if P1_TUNE[i][1]:
            todo = interleave(*([z2t[0::2]] + xt + [z2t[1::2]]))
        else:
            todo = interleave(*(xt + [z2t[0::2], z2t[1::2]]))
        tied = _Tied(todo, P1_TUNE[i][0])
        if xg is not None:
            dft.run(KV_COST)
            job_x(xg, dft, (nx - 1) * KV_COST / 10.0)
            dft.drain()
        for p in range(2):
            for j in range(FH // L):
                job_zs(i, p, j, bg, (1.6 * zb + extra, 0.5 * zb + extra), tied)
            assert not tied.tasks or (p == 0 and not last)
            if p == 0 and last:
                tied = _Tied(tasks(ln_z2, i, 8), LAST_N)
        if last:
            for s in range(8, 16):
                ln_z2(i, s)
        bg.drain()
        job_h(t, hbg, nh * KV_COST / 10.0)
        hbg.drain()

    def p1_block(g):
        for i in P1_GROUPS[g]:
            p1_step(i)

    for g in range(len(P1_GROUPS)):
        p1_wait(g)
        p1_start(g)
        block(lambda g=g: p1_block(g), f'p1_g{g}')

    groups = P2_GROUPS
    NG = len(groups)

    def p2_dma(gi):
        if gi >= 2:
            for i in groups[gi - 2]:
                start(cp_out(i))
        if gi >= 3:
            for i in groups[gi - 3]:
                wait(cp_out(i))
        if gi == 1:
            for i in (6, 7):
                start(cp_wsp(i))
        if gi == 0:
            wait(cp_conv(6))
        if gi + 1 < NG:
            for i in groups[gi + 1]:
                wait(cp_wsp(i))

    def tails_of(i, bg, budget):
        return [tail_gen(i, bg, budget)] * 20

    def p2_block(gi):
        bg = _Background()
        steps = groups[gi]
        tb = [0.0]
        pending = [t_ for i in (groups[gi - 1] if gi > 0 else []) for t_ in tails_of(i, bg, tb)]
        total = sum(a + 1 for i in steps for a in _blocks_of_step(i)) * 40 * 16
        total += len(steps) * (24 * E_COST + 6 * U_COST) + len(pending) * T_COST
        slots = sum(84 if i == 0 else 77 for i in steps) + TAIL_W * len(pending)
        bg.add(freq_gen(_blocks_of_step(steps[0])[0]))
        if gi == 0:
            bg.add(bcomb2_gen((0, 2, 3, 4, 6)))
            total += 5 * 16 * A_COST
        if gi < 2:
            bg.add(kv_gen(NT - 2 + gi))
            total += 20 * KV_COST
            slots += 10
        for t in P2_X[gi]:
            slots += 10
        if gi + 1 < NG:
            for i in groups[gi + 1]:
                bg.add(acomb2_gen(i))
                total += 16 * 7 * A2_COST
        for i in steps[1:]:
            bg.add(freq_gen(_blocks_of_step(i)[0]))
        budget = tb[0] = total / (slots + P2_END[gi])
        bg.run(budget)
        for t in P2_X[gi]:
            job_x(t, bg, budget)
        if gi < 2:
            job_h(NT - 2 + gi, bg, budget)
        units = [4, 4, 2, 4, 4, 2] * (len(pending) // 20)
        every = [0] * sum(6 if i == 0 else 9 for i in steps)
        for j, n in enumerate(units):
            every[min(len(every) - 1, j * len(every) // len(units))] += n
        for i in steps:
            job_big(i, bg, pending, budget, every)
        for t_ in pending:
            next(t_)
        bg.drain()

    for gi in range(NG):
        p2_dma(gi)
        block(lambda gi=gi: p2_block(gi), f'p2_{gi}')

    def cp_last(part):
        a0 = _blocks_of_step(NT - 1)[0]
        sub, cols = ((MC, pl.ds(0, D)), (0, pl.ds(0, 4 * L)), (0, pl.ds(4 * L, L)))[part]
        return [pltpu.make_async_copy(o_v.at[pl.ds(r, MC), cols], o_hbm.at[0, pl.ds(r, MC), cols],
                                      sem_out.at[NT - 1]) for r in (a0 * P + sub, (a0 + 1) * P + sub)]

    def p2_last():
        for i in groups[NG - 1]:
            for j, t_ in enumerate(tails_of(i, _Background(), [0.0])):
                next(t_)
                if i < NT - 1 and j == 19:
                    start(cp_out(i))
                if i == NT - 1 and j in (9, 17):
                    start(cp_last(j // 10))

    p2_dma(NG)
    block(p2_last, 'p2_last')
    start(cp_last(2))
    for i in groups[NG - 2] + groups[NG - 1][:-1]:
        wait(cp_out(i))
    for part in range(3):
        wait(cp_last(part))
    debug_keep_alive()


def _compiler_params():
    vmem = 116 * 1024 * 1024
    try:
        return pltpu.CompilerParams(vmem_limit_bytes=vmem, disable_semaphore_checks=True)
    except TypeError:
        return pltpu.CompilerParams(vmem_limit_bytes=vmem)


@jax.jit
def pallas_recurrent_scan__ssm_conv_h3__mixer_gmlp__prompt_kernel(
    A_q: jax.Array,
    A_k: jax.Array,
    A_v: jax.Array,
    A_shift_k: jax.Array,
    A_ssm_k: jax.Array,
    A_ssm_D: jax.Array,
    B_x: jax.Array,
    B_w_in: jax.Array,
    B_w_sp: jax.Array,
    B_b_sp: jax.Array,
    B_w_out: jax.Array,
):
    del B_x
    hbm = pl.BlockSpec(memory_space=pl.ANY)

    def bf16_buf(*shape):
        return pltpu.VMEM(shape[:-2] + (shape[-2] // 2, shape[-1]), U32)

    return pl.pallas_call(
        _kernel,
        out_shape=jax.ShapeDtypeStruct((1, S, D), BF16),
        in_specs=[hbm] * 10,
        out_specs=hbm,
        scratch_shapes=[
            [bf16_buf(len(g) * TM, D) for g in X_DMAS],
            [bf16_buf(len(g) * TM, D) for g in CONV_DMAS],
            [bf16_buf(len(g) * TM, D) for g in CONV_DMAS],
            [bf16_buf(D, len(g) * TM) for g in CONV_DMAS],
            [bf16_buf(D, max(hi - lo, 2) * L) for lo, hi in WIN_CHUNKS],
            [bf16_buf(TM, S) for _ in range(NT)],
            bf16_buf(FH, D),
            pltpu.VMEM((S, D), BF16),
            pltpu.VMEM((4, D), BF16),
            pltpu.VMEM((D,), BF16),
            pltpu.VMEM((S,), BF16),
            bf16_buf(S, D),
            bf16_buf(4 * P, 5 * KH),
            bf16_buf(KH, 5 * FH),
            bf16_buf(5 * P, 5 * HN),
            bf16_buf(HN, 10 * L),
            pltpu.VMEM((S, FH), F32),
            bf16_buf(HK, 7 * HN),
            bf16_buf(5 * 5 * P, HK),
            bf16_buf(5 * 7 * MC, 5 * KQ),
            bf16_buf(7 * KQ, 5 * L),
            pltpu.VMEM((16 * MC, L), F32),
            pltpu.VMEM((HK, FH), F32),
            pltpu.VMEM((3, TM, FH), F32),
            bf16_buf(S, D),
            bf16_buf(S, FH),
            pltpu.VMEM((NB, 2, P, D), F32),
            pltpu.VMEM((2, 2, P, D), F32),
            pltpu.VMEM((NB, 2, P, D), F32),
            bf16_buf(NB // 2 * P, 4 * D),
            pltpu.VMEM((2, D // L, MC, L), F32),
            bf16_buf(2 * P, 2 * P),
            bf16_buf(MC, 2 * P),
            pltpu.VMEM((S, L), F32),
            pltpu.VMEM((2, P, L), F32),
            pltpu.VMEM((4, 8, D), F32),
            pltpu.VMEM((D // L, S + 8, L), F32),
            pltpu.SemaphoreType.DMA((1,)),
            pltpu.SemaphoreType.DMA((NT,)),
            pltpu.SemaphoreType.DMA((NT,)),
            pltpu.SemaphoreType.DMA((NT,)),
            pltpu.SemaphoreType.DMA((5,)),
            pltpu.SemaphoreType.DMA((NT,)),
        ],
        compiler_params=_compiler_params(),
    )(A_q, A_k, A_v, A_shift_k.T, A_ssm_k, A_ssm_D, B_w_in, B_w_sp, B_b_sp, B_w_out)
```

```python
import math

import jax
import jax.numpy as jnp
import jax.experimental.pallas as pl
import jax.experimental.pallas.tpu as pltpu

S = 2048
D = 640
FH = 768
P = 128
NB = S // P
TM = 256
NT = S // TM
MC = 64
L = 128
HK = S // 2
KQ = HK // 2
KH = 256
HN = FH // 2
EPS = 1e-5
F32 = jnp.float32
BF16 = jnp.bfloat16
U32 = jnp.uint32
GELU_C = math.sqrt(2.0 / math.pi)
GA = (GELU_C * 0.044715) ** (1.0 / 3.0)
NT_DIMS = (((1,), (1,)), ((), ()))

WIN_CHUNKS = ((6, 7), (7, 9), (9, 12), (0, 3), (3, 6))
X_DMAS = ((0,), (1,), (2,), (3,), (4, 5), (6, 7))
CONV_DMAS = ((0,), (1,), (2, 3), (4, 5), (6, 7))
P1_GROUPS = ((2,), (3,), (4, 5), (6, 7))
P1_X = {2: None, 3: 0, 4: 1, 5: None, 6: 2, 7: 3}
P1_LNX = {2: (3,), 3: (4, 5), 4: (6,), 5: (7,), 6: (), 7: ()}
P2_GROUPS = ((0,), (1, 2), (3, 4, 5), (6, 7))
P2_X = ((4, 5), (6,), (7,), ())
STEP_BLOCKS = ((2, 3), (6, 7), (4, 5), (12, 13), (10, 11), (0, 1), (14, 15), (8, 9))
KV_COST, A_COST, A2_COST = 110, 56, 34
E_COST, U_COST, T_COST, TAIL_W = 24, 90, 90, 1.6
KV_SPLIT = {2: (0, 14, 6), 3: (12, 4, 4), 4: (12, 4, 4), 5: (0, 14, 6), 6: (12, 4, 4), 7: (12, 4, 4)}
FR = 8
L1_USE = {0: ((0, 1, True, False), (3, 1, True, False)), 6: ((0, 1, False, False),),
          3: ((0, 1, False, False), (2, 1, True, False)), 4: ((0, -1, False, True), (1, 1, True, False)),
          1: ((2, 1, False, True), (3, -1, False, False)), 2: ((1, 1, False, True), (3, 1, False, False)),
          5: ((3, 1, False, True),)}
H_SPLIT = ((0, 2), (2, 4), (4, 5))
FINE = tuple((l, l + 1) for l in range(D // L))
P1_TUNE = {2: (42, 0), 3: (43, 1), 4: (42, 0), 5: (42, 0), 6: (44, 0), 7: (24, 0)}
EXTRA = (52, 52)
LAST_N = 22
P2_END = (0.0, -1.0, -1.0, 0.0)
F_TIED = (20, 20, 18, 20, 20)
_ONLY = None


def _dot(a, b):
    return jnp.dot(a, b, preferred_element_type=F32)


def _sums_left(a11, a12, a21, a22):
    add, sub = jax.lax.add, jax.lax.sub
    return jnp.concatenate((add(a11, a22), add(a21, a22), add(a11, a12), sub(a21, a11), sub(a12, a22)),
                           axis=1).astype(BF16)


def _sums_right(b11, b12, b21, b22):
    add, sub = jax.lax.add, jax.lax.sub
    return jnp.concatenate((add(b11, b22), sub(b12, b22), sub(b21, b11), add(b11, b12), add(b21, b22)),
                           axis=1).astype(BF16)


def _cos_sin(m):
    q = (m + 256) >> 9
    x = (m - (q << 9)).astype(F32) * (2.0 * math.pi / 2048.0)
    x2 = x * x
    s = x * (1.0 + x2 * (-1.0 / 6 + x2 * (1.0 / 120 + x2 * (-1.0 / 5040 + x2 * (1.0 / 362880)))))
    c = 1.0 + x2 * (-0.5 + x2 * (1.0 / 24 + x2 * (-1.0 / 720 + x2 * (1.0 / 40320 - x2 * (1.0 / 3628800)))))
    swap = (q & 1) == 1
    c0 = jnp.where(swap, s, c)
    s0 = jnp.where(swap, c, s)
    cos = jnp.where(((q + 1) & 2) == 2, -c0, c0)
    sin = jnp.where((q & 2) == 2, -s0, s0)
    return cos, sin


def _odd_freq(r):
    return jnp.where(r < 64, 4 * r + 1, 4 * r - 253)


def _gelu_scaled(z):
    return z + z * jnp.tanh(z * (GELU_C / GA + z * z))


def _signzero(z):
    bits = jax.lax.bitcast_convert_type(z, U32) & jnp.uint32(0x80000000)
    return jax.lax.bitcast_convert_type(bits, F32)


def _ln(x, eps, tie=None, scale=None):
    n = x.shape[-1]
    cols = [x[:, j * L:(j + 1) * L] for j in range(n // L)]
    s1 = cols[0]
    s2 = cols[0] * cols[0]
    for c in cols[1:]:
        s1 = s1 + c
        s2 = s2 + c * c
    if tie is not None:
        s1 = s1 + tie
        s2 = s2 + tie
    m = jnp.sum(s1, axis=-1, keepdims=True) * (1.0 / n)
    v = jnp.maximum(jnp.sum(s2, axis=-1, keepdims=True) * (1.0 / n) - m * m, 0.0)
    rs = jax.lax.rsqrt(v + eps)
    if scale is not None:
        rs = rs * scale
    return (x - m) * rs


def _blocks_of_step(i):
    return STEP_BLOCKS[i]


class _Background:
    def __init__(self):
        self.q = []
        self.credit = 0.0

    def add(self, gen):
        self.q.append(gen)

    def run(self, budget):
        self.credit += budget
        while self.q and self.credit > 0:
            try:
                self.credit -= next(self.q[0])
            except StopIteration:
                self.q.pop(0)
        if not self.q:
            self.credit = 0.0

    def charge(self, cost):
        self.credit -= cost

    def drain(self):
        while self.q:
            self.run(1e9)


class _Tied:
    def __init__(self, tasks, npieces):
        self.tasks = list(tasks)
        self.rate = len(self.tasks) / float(npieces)
        self.credit = 0.999

    def run(self, z):
        self.credit += self.rate
        n = 0
        while self.tasks and self.credit >= 1.0:
            self.tasks.pop(0)(_signzero(z[0:16]))
            self.credit -= 1.0
            n += 1
        return n


def _kernel(q_hbm, k_hbm, v_hbm, sk_hbm, h_hbm, d_hbm, win_hbm, wsp_hbm, b_hbm, wout_hbm,
            o_hbm,
            x_us, k_us, v_us, h_us, win_us, wsp_us, wout_u, o_v, sk_in, d_in, b_in,
            xn_u, XL_u, WB_u, UL_u, WO_u, z1_v, R_u, Lc_u, L2_u, R2_u, C_v, zf_v, zg_v, kv_u, u_u, X_v, H_v, G_v, Z_u,
            yl_v, F_u, Fi_u, bcol_v, ph_v, sk_v, kf_v,
            sem_small, sem_x, sem_conv, sem_wsp, sem_w, sem_out):
    (wout_v, xn_v, XL_v, WB_v, UL_v, WO_v, R_v, Lc_v, L2_v, R2_v, kv_v, u_v, Z_v, F_v, Fi_v) = [
        r.bitcast(BF16) for r in (wout_u, xn_u, XL_u, WB_u, UL_u, WO_u, R_u, Lc_u, L2_u, R2_u, kv_u, u_u, Z_u, F_u, Fi_u)]
    x_vs = {g[0]: r.bitcast(BF16) for g, r in zip(X_DMAS, x_us)}
    k_vs, v_vs, h_vs = [{g[0]: r.bitcast(BF16) for g, r in zip(CONV_DMAS, rs)} for rs in (k_us, v_us, h_us)]
    wsp_vs = [r.bitcast(BF16) for r in wsp_us]
    win_vs = [r.bitcast(BF16) for r in win_us]

    def win(rows, n):
        c = [lo <= n < hi for lo, hi in WIN_CHUNKS].index(True)
        n -= WIN_CHUNKS[c][0]
        return win_vs[c][rows, n * L:(n + 1) * L]

    def locate(bufs, row):
        t0 = max(t for t in bufs if t * TM <= row)
        return bufs[t0], row - t0 * TM

    def rows_of(bufs, row, n, lanes=slice(None)):
        buf, r = locate(bufs, row)
        return buf[r:r + n, lanes]

    def cp_small():
        return [pltpu.make_async_copy(s_, d_, sem_small.at[0])
                for s_, d_ in ((d_hbm, d_in), (sk_hbm, sk_in), (b_hbm, b_in))]

    def cp_x(t):
        return pltpu.make_async_copy(q_hbm.at[0, pl.ds(t * TM, x_vs[t].shape[0])], x_vs[t], sem_x.at[t])

    def cp_conv(t):
        rows = pl.ds(t * TM, k_vs[t].shape[0])
        sem = sem_conv.at[t]
        return [pltpu.make_async_copy(h_hbm.at[:, rows], h_vs[t], sem),
                pltpu.make_async_copy(k_hbm.at[0, rows], k_vs[t], sem),
                pltpu.make_async_copy(v_hbm.at[0, rows], v_vs[t], sem)]

    def cp_wsp(i):
        return [pltpu.make_async_copy(wsp_hbm.at[pl.ds(_blocks_of_step(i)[0] * P, TM)], wsp_vs[i], sem_wsp.at[i])]

    def cp_win(c):
        lo, hi = WIN_CHUNKS[c]
        w = (hi - lo) * L
        return pltpu.make_async_copy(win_hbm.at[:, pl.ds(lo * L, w)], win_vs[c].at[:, pl.ds(0, w)], sem_w.at[c])

    def cp_wout():
        return pltpu.make_async_copy(wout_hbm, wout_v, sem_w.at[0])

    def cp_out(i):
        rows = pl.ds(_blocks_of_step(i)[0] * P, TM)
        return [pltpu.make_async_copy(o_v.at[rows], o_hbm.at[0, rows], sem_out.at[i])]

    def start(cs):
        for c in cs:
            c.start()

    def wait(cs):
        for c in cs:
            c.wait()

    def block(fn, name):
        def body(it):
            fn()
            return it + 1

        if _ONLY is None or name in _ONLY:
            jax.lax.while_loop(lambda it: it < 1, body, jnp.int32(0))

    def ln_x(t, s, tie=None):
        rows = pl.ds(t * TM + s * 16, 16)
        y = _ln(rows_of(x_vs, t * TM + s * 16, 16).astype(F32), EPS, tie, GA)
        xn_v[rows, :] = y.astype(BF16)
        return y

    def ln_x2(t, s, tie):
        p, q = s // 4, s % 4
        y1 = ln_x(t, 8 * p + q, tie)
        y2 = ln_x(t, 8 * p + 4 + q, tie)
        a11, a12, a21, a22 = y1[:, :KH], y1[:, KH:2 * KH], y2[:, :KH], y2[:, KH:2 * KH]
        XL_v[pl.ds((t % 4) * P + p * MC + q * 16, 16), :] = _sums_left(a11, a12, a21, a22)

    def wcomb_gen(cols):
        for j in cols:
            for r in range(KH // 32):
                top = pl.ds(r * 32, 32)
                bot = pl.ds(KH + r * 32, 32)
                b11, b12 = win(top, j).astype(F32), win(top, 6 + j).astype(F32)
                b21, b22 = win(bot, j).astype(F32), win(bot, 6 + j).astype(F32)
                WB_v[top, j * 5 * L:(j + 1) * 5 * L] = _sums_right(b11, b12, b21, b22)
                yield A_COST

    def ln_z2(t, s, tie=None):
        y = _ln(zg_v[t % 3, s * 16:(s + 1) * 16, :], 4.0 * GA * GA * EPS, tie, 0.25 / GA)
        lo, hi = y[:, :HN], y[:, HN:]
        rows = pl.ds((t * TM + s * 16) % HK, 16)
        if t < NT // 2:
            zf_v[rows, :] = y
            R_v[rows, 0:2 * HN] = jnp.concatenate((lo, lo + hi), axis=1).astype(BF16)
        else:
            b11, b12 = zf_v[rows, :HN], zf_v[rows, HN:]
            R_v[rows, 2 * HN:] = jnp.concatenate((b11 + hi, b12 - hi, lo - b11, hi, lo + hi), axis=1).astype(BF16)

    def r1(j, rows, n):
        c0 = {1: 0, 5: 1, 0: 2, 2: 3, 3: 4, 4: 5, 6: 6}[j] * HN + n * L
        return R_v[rows, c0:c0 + L]

    def acomb_gen(i, groups=range(P // 16)):
        for r in groups:
            for c in range(HK // 256):
                top = pl.ds(r * 16, 16)
                bot = pl.ds(P + r * 16, 16)
                c1 = slice(c * 256, (c + 1) * 256)
                c2 = slice(HK + c * 256, HK + (c + 1) * 256)
                a11 = wsp_vs[i][top, c1].astype(F32)
                a12 = wsp_vs[i][top, c2].astype(F32)
                a21 = wsp_vs[i][bot, c1].astype(F32)
                a22 = wsp_vs[i][bot, c2].astype(F32)
                r0 = (i % 5) * 5 * P + (r % 4 * 2 + r // 4) * 16
                Lc_v[pl.ds(r0 + 0 * P, 16), c1] = (a11 + a22).astype(BF16)
                Lc_v[pl.ds(r0 + 1 * P, 16), c1] = (a21 + a22).astype(BF16)
                Lc_v[pl.ds(r0 + 2 * P, 16), c1] = (a11 + a12).astype(BF16)
                Lc_v[pl.ds(r0 + 3 * P, 16), c1] = (a21 - a11).astype(BF16)
                Lc_v[pl.ds(r0 + 4 * P, 16), c1] = (a12 - a22).astype(BF16)
                yield A_COST

    def acomb2_gen(i):
        for r in range(MC // 16):
            for c in range(KQ // L):
                quad = {}

                def w(b, H):
                    if (b, H) not in quad:
                        quad[b, H] = [[wsp_vs[i][pl.ds(b * P + s_ * MC + r * 16, 16),
                                                 H * HK + kh * KQ + c * L:H * HK + kh * KQ + (c + 1) * L].astype(F32)
                                       for kh in range(2)] for s_ in range(2)]
                    return quad[b, H]

                spec = {2: (None, (0, 0), None, 0), 0: (0, (0, 0), (1, 1), 1), 3: (None, (1, 1), None, 0),
                        1: (1, (1, 0), (1, 1), 1), 5: (3, (1, 0), (0, 0), -1), 4: (2, (0, 0), (0, 1), 1),
                        6: (4, (0, 1), (1, 1), -1)}
                for j in (2, 0, 3, 1, 5, 4, 6):
                    slot, p_, q_, sign = spec[j]
                    a = w(*p_)
                    if q_ is not None:
                        b_ = w(*q_)
                        op = jax.lax.add if sign > 0 else jax.lax.sub
                        a = [[op(a[s_][kh], b_[s_][kh]) for kh in range(2)] for s_ in range(2)]
                        for kh in range(2):
                            Lc_v[pl.ds(((i % 5) * 5 + slot) * P + r * 32, 32),
                                 kh * KQ + c * L:kh * KQ + (c + 1) * L] = jnp.concatenate(
                                     (a[0][kh], a[1][kh]), axis=0).astype(BF16)
                    L2_v[pl.ds(((i % 5) * 7 + j) * MC + r * 16, 16), c * 5 * L:(c + 1) * 5 * L] = _sums_left(
                        a[0][0], a[0][1], a[1][0], a[1][1])
                    yield A2_COST

    def bcomb2_gen(js):
        for j in js:
            for r in range(KQ // 16):
                top = pl.ds(r * 16, 16)
                bot = pl.ds(KQ + r * 16, 16)
                R2_v[pl.ds(j * KQ + r * 16, 16), :] = _sums_right(
                    *[r1(j, rows, n).astype(F32) for rows in (top, bot) for n in range(2)])
                yield A_COST / 2

    def tasks(fn, t, n=TM // 16):
        return [lambda tie, s=s: fn(t, s, tie) for s in range(n)]

    def kv_gen(t):
        for m in range(TM // MC):
            r = t * TM + m * MC
            for l in range(D // L):
                lanes = slice(l * L, (l + 1) * L)
                kf = rows_of(k_vs, r, MC, lanes).astype(F32)
                kf_v[l, pl.ds(r + 8, MC), :] = kf
                ks = kf * sk_v[0, 0:1, lanes]
                for tap in range(1, 4):
                    ks = ks + kf_v[l, pl.ds(r + 8 - tap, MC), :] * sk_v[tap, 0:1, lanes]
                kv = ks * rows_of(v_vs, r, MC, lanes).astype(F32)
                kv_v[pl.ds(r, MC), lanes] = kv.astype(BF16)
                yield KV_COST

    def freq_gen(a):
        def cmac(acc, x, g):
            mul, add = jax.lax.mul, jax.lax.add
            pr = jax.lax.sub(mul(x[0], g[0]), mul(x[1], g[1]))
            pi = add(mul(x[0], g[1]), mul(x[1], g[0]))
            return (pr, pi) if acc is None else (add(acc[0], pr), add(acc[1], pi))

        for r in range(P // 16):
            for l in range(D // L):
                lanes = slice(l * L, (l + 1) * L)
                res = []
                for sub in range(16 // FR):
                    rows = pl.ds(r * 16 + sub * FR, FR)
                    lo = hi = None
                    g = (G_v[a + 1, 0, rows, lanes], G_v[a + 1, 1, rows, lanes])
                    for c in range(a + 2):
                        x = (X_v[c, 0, rows, lanes], X_v[c, 1, rows, lanes])
                        hi = cmac(hi, x, g)
                        if c <= a:
                            g = (G_v[a - c, 0, rows, lanes], G_v[a - c, 1, rows, lanes])
                            lo = cmac(lo, x, g)
                            yield 2 * FR
                    res.append((lo, hi))
                Z_v[pl.ds(a // 2 * P + r * 16, 16), l * 4 * L:(l + 1) * 4 * L] = jnp.concatenate(
                    [jnp.concatenate([z[0][0], z[0][1], z[1][0], z[1][1]], axis=1) for z in res], axis=0).astype(BF16)
                yield 20

    def job_x(t, bg, budget, split=((0, 5),)):
        for j in (2 * t, 2 * t + 1):
            for half in range(2):
                for l0, l1 in split:
                    w, lanes = (l1 - l0) * L, slice(l0 * L, l1 * L)
                    r = _dot(F_v[half * P:(half + 1) * P, 0:P], kv_v[j * P:(j + 1) * P, lanes]).reshape(8, 2, 8, w)
                    for part in range(2):
                        X_v[j, part, half * 64:(half + 1) * 64, lanes] = r[:, part].reshape(64, w)
                    bg.run(budget * (l1 - l0) / 2)

    def job_h(t, bg, budget, split=H_SPLIT):
        h_v, c0 = locate(h_vs, t * TM)
        for half in range(2):
            rows = pl.ds(half * 64, 64)
            for l0, l1 in split:
                w = (l1 - l0) * L
                lanes = slice(l0 * L, l1 * L)
                rhs = jnp.concatenate([h_v[lanes, c0:c0 + P], h_v[lanes, c0 + P:c0 + TM]], axis=0)
                r = jax.lax.dot_general(F_v[half * P:(half + 1) * P, 0:P], rhs, NT_DIMS,
                                        preferred_element_type=F32).reshape(8, 2, 8, 2 * w)
                re, im = r[:, 0].reshape(64, 2 * w), r[:, 1].reshape(64, 2 * w)
                prev = (H_v[t % 2, 0, rows, lanes], H_v[t % 2, 1, rows, lanes])
                for j in range(2):
                    cur = (re[:, j * w:(j + 1) * w], im[:, j * w:(j + 1) * w])
                    G_v[2 * t + j, 0, rows, lanes] = cur[0] + prev[1] if half else cur[0] - prev[1]
                    G_v[2 * t + j, 1, rows, lanes] = cur[1] - prev[0] if half else cur[1] + prev[0]
                    prev = cur
                if t + 1 < NT:
                    H_v[(t + 1) % 2, 0, rows, lanes] = prev[0]
                    H_v[(t + 1) % 2, 1, rows, lanes] = prev[1]
                bg.run(budget * (l1 - l0))

    def z_out(t, m, n, pre, bg, budget, tied):
        z = _gelu_scaled(pre)
        if n < FH // L:
            z1_v[pl.ds(t * TM + m * MC, MC), n * L:(n + 1) * L] = z
        else:
            zg_v[t % 3, m * MC:(m + 1) * MC, n * L - FH:(n + 1) * L - FH] = z
        ntask = tied.run(z)
        bg.run(budget[1] if ntask else budget[0])

    def job_z(t, m, cols, bg, budget, tied):
        for n in cols:
            z_out(t, m, n, _dot(xn_v[pl.ds(t * TM + m * MC, MC), :], win(slice(None), n)), bg, budget, tied)

    def job_zs(t, p, j, bg, budget, tied):
        r1 = pl.ds(t * TM + p * P, MC)
        r2 = pl.ds(t * TM + p * P + MC, MC)

        def xl(w):
            r0 = (t % 4) * P + p * MC
            return XL_v[r0:r0 + MC, w * KH:(w + 1) * KH]

        def wb(w):
            return WB_v[:, (j * 5 + w) * L:(j * 5 + w + 1) * L]

        def rem(rows, n):
            return _dot(xn_v[rows, 2 * KH:], win(slice(2 * KH, D), n))

        m2 = _dot(xl(1), win(slice(0, KH), j))
        m4 = _dot(xn_v[r2, KH:2 * KH], wb(2))
        z_out(t, 2 * p + 1, j, m2 + m4 + rem(r2, j), bg, budget, tied)
        m3 = _dot(xn_v[r1, 0:KH], wb(1))
        m5 = _dot(xl(2), win(slice(KH, 2 * KH), 6 + j))
        z_out(t, 2 * p, 6 + j, m3 + m5 + rem(r1, 6 + j), bg, budget, tied)
        t11, t22 = m4 - m5, m3 - m2
        m1 = _dot(xl(0), wb(0))
        t11, t22 = t11 + m1, t22 + m1
        z_out(t, 2 * p, j, t11 + _dot(xl(4), wb(4)) + rem(r1, j), bg, budget, tied)
        z_out(t, 2 * p + 1, 6 + j, t22 + _dot(xl(3), wb(3)) + rem(r2, 6 + j), bg, budget, tied)

    rev8 = 7 - jax.lax.broadcasted_iota(jnp.int32, (8, L), 0)

    def finish(a, upper, n, hh, slot):
        rows = pl.ds(a * P + (MC if upper else 0), MC)
        lanes = slice(n * L, (n + 1) * L)
        if upper:
            zc = (n * 4 + a % 2 * 2) * L
            ya = _dot(Fi_v[:, 0:P], Z_v[a // 2 * P:(a // 2 + 1) * P, zc:zc + L])
            yb = _dot(Fi_v[:, P:2 * P], Z_v[a // 2 * P:(a // 2 + 1) * P, zc + L:zc + 2 * L])
            slot(0.5)
            y = ya - yb
            lo = ya + yb
            for j in range(MC // 8):
                yl_v[a % 2, n, (7 - j) * 8:(8 - j) * 8, :] = jnp.take_along_axis(lo[j * 8:(j + 1) * 8], rev8, axis=0)
        else:
            y = yl_v[a % 2, n]
        gate = hh + hh * jnp.tanh(hh)
        s = xn_v[rows, lanes].astype(F32) * y
        x = rows_of(x_vs, a * P + (MC if upper else 0), MC, lanes).astype(F32)
        o_v[rows, lanes] = (x + s * gate).astype(BF16)

    def tail_gen(i, bg, budget):
        a0, a1 = _blocks_of_step(i)

        def slot(w):
            bg.run(w * budget[0])

        def dot3(a, b):
            r = _dot(a, b)
            slot(0.75)
            return r

        for upper in (True, False):
            sub = MC if upper else 0
            r1 = pl.ds(a0 * P + sub, MC)
            r2 = pl.ds(a1 * P + sub, MC)

            def ul(w):
                allw = UL_v[(i % 5) * P + sub:(i % 5) * P + sub + MC, :]
                return jnp.concatenate([allw[:, (n * 5 + w) * L:(n * 5 + w + 1) * L] for n in range(HN // L)], axis=1)

            for j in range(2):
                c1 = slice(j * L, (j + 1) * L)
                c2 = slice((2 + j) * L, (3 + j) * L)

                def wo(w):
                    return WO_v[:, (j * 5 + w) * L:(j * 5 + w + 1) * L]

                m2 = dot3(ul(1), wout_v[0:HN, c1])
                m4 = dot3(u_v[r2, HN:], wo(2))
                finish(a1, upper, j, m2 + m4, slot)
                bg.charge(T_COST)
                yield
                m3 = dot3(u_v[r1, 0:HN], wo(1))
                m5 = dot3(ul(2), wout_v[HN:, c2])
                finish(a0, upper, 2 + j, m3 + m5, slot)
                bg.charge(T_COST)
                yield
                t11, t22 = m4 - m5, m3 - m2
                m1 = dot3(ul(0), wo(0))
                t11, t22 = t11 + m1, t22 + m1
                finish(a0, upper, j, t11 + dot3(ul(4), wo(4)), slot)
                bg.charge(T_COST)
                yield
                finish(a1, upper, 2 + j, t22 + dot3(ul(3), wo(3)), slot)
                bg.charge(T_COST)
                yield
            for a, r in ((a0, r1), (a1, r2)):
                finish(a, upper, 4, dot3(u_v[r, 0:HN], wout_v[0:HN, 4 * L:]) + dot3(u_v[r, HN:], wout_v[HN:, 4 * L:]),
                       slot)
                bg.charge(T_COST)
                yield

    def wocomb_gen():
        for j in range(2):
            c1 = slice(j * L, (j + 1) * L)
            c2 = slice((2 + j) * L, (3 + j) * L)
            for r in range(HN // 32):
                top = pl.ds(r * 32, 32)
                bot = pl.ds(HN + r * 32, 32)
                b11, b12 = wout_v[top, c1].astype(F32), wout_v[top, c2].astype(F32)
                b21, b22 = wout_v[bot, c1].astype(F32), wout_v[bot, c2].astype(F32)
                WO_v[top, j * 5 * L:(j + 1) * 5 * L] = _sums_right(b11, b12, b21, b22)
                yield A_COST

    def job_big(i, bg, pending, budget, every):
        a0, a1 = _blocks_of_step(i)
        KG = 512

        def lhs(j, sub, cols):
            if j == 2:
                return wsp_vs[i][sub:sub + MC, cols]
            if j == 3:
                return wsp_vs[i][P + sub:P + sub + MC, HK + cols.start:HK + cols.stop]
            r0 = ((i % 5) * 5 + {0: 0, 1: 1, 4: 2, 5: 3, 6: 4}[j]) * P
            both = Lc_v[r0:r0 + P, cols]
            return jnp.concatenate([both[q * 32 + sub // 4:q * 32 + sub // 4 + 16] for q in range(4)], axis=0)

        def prod(j, sub, n, acc=None):
            for kg in range(HK // KG):
                ks = slice(kg * KG, (kg + 1) * KG)
                p = _dot(lhs(j, sub, ks), r1(j, ks, n))
                acc = p if acc is None else p + acc
                bg.run(budget)
            return acc

        def tails(n):
            for _ in range(n):
                if pending:
                    next(pending.pop(0))

        def emit(a, sub, n, g):
            rows = pl.ds(a * P + sub, MC)
            lanes = slice(n * L, (n + 1) * L)
            u = z1_v[rows, lanes] * (g + bcol_v[rows, :])
            u_v[rows, lanes] = u.astype(BF16)
            bg.charge(E_COST)
            return u

        if i > 0:
            def piece(a, b, acc=None):
                p = _dot(a, b)
                bg.run(budget)
                return p if acc is None else acc + p

            def cslot(k, s_, n):
                return pl.ds(((k * 2 + s_) * 2 + n) * MC, MC)

            def contribute(j, s_, n, m):
                for k, sign, first, last in L1_USE[j]:
                    cs = cslot(k, s_, n)
                    v_ = m if first else (C_v[cs, :] + m if sign > 0 else C_v[cs, :] - m)
                    if last:
                        u = emit((a0, a0, a1, a1)[k], s_ * MC, n + (k % 2) * (HN // L), v_)
                        v_ = u
                        if k == 3:
                            u11, u12, u21 = C_v[cslot(0, s_, n), :], C_v[cslot(1, s_, n), :], C_v[cslot(2, s_, n), :]
                            UL_v[pl.ds((i % 5) * P + s_ * MC, MC), n * 5 * L:(n + 1) * 5 * L] = _sums_left(
                                u11, u12, u21, u)
                            bg.charge(U_COST)
                            continue
                    C_v[cs, :] = v_

            for j in (0, 6, 3, 4, 1, 2, 5):
                def l2(w):
                    r0 = ((i % 5) * 7 + j) * MC
                    allw = L2_v[r0:r0 + MC, :]
                    return jnp.concatenate([allw[:, (c * 5 + w) * L:(c * 5 + w + 1) * L] for c in range(KQ // L)],
                                           axis=1)

                def r2(w):
                    return R2_v[j * KQ:(j + 1) * KQ, w * L:(w + 1) * L]

                def rq(kh, n):
                    return r1(j, slice(kh * KQ, (kh + 1) * KQ), n)

                p2 = piece(l2(1), rq(0, 0))
                p4 = piece(lhs(j, MC, slice(KQ, 2 * KQ)), r2(2))
                contribute(j, 1, 0, p2 + p4)
                p3 = piece(lhs(j, 0, slice(0, KQ)), r2(1))
                t22 = p3 - p2
                p5 = piece(l2(2), rq(1, 1))
                contribute(j, 0, 1, p3 + p5)
                t11 = p4 - p5
                p1 = piece(l2(0), r2(0))
                t11, t22 = t11 + p1, t22 + p1
                contribute(j, 0, 0, piece(l2(4), r2(4), t11))
                contribute(j, 1, 1, piece(l2(3), r2(3), t22))
                tails(every.pop(0))

        for sub in (0, MC):
            for n in (range(HN // L) if i == 0 else (2,)):
                def put(w, c):
                    UL_v[pl.ds((i % 5) * P + sub, MC), (n * 5 + w) * L:(n * 5 + w + 1) * L] = c.astype(BF16)

                m1 = prod(0, sub, n)
                t11 = prod(6, sub, n, m1)
                m4 = prod(3, sub, n)
                t11 = t11 + m4
                m5 = prod(4, sub, n)
                u11 = emit(a0, sub, n, t11 - m5)
                m2 = prod(1, sub, n)
                u21 = emit(a1, sub, n, m2 + m4)
                put(3, u21 - u11)
                t22 = m1 - m2
                m3 = prod(2, sub, n)
                u12 = emit(a0, sub, n + HN // L, m3 + m5)
                put(2, u11 + u12)
                u22 = emit(a1, sub, n + HN // L, prod(5, sub, n, t22 + m3))
                put(0, u11 + u22)
                put(1, u21 + u22)
                put(4, u12 - u22)
                bg.charge(U_COST)
                tails(every.pop(0))

    def debug_keep_alive():
        if _ONLY is not None:
            for r_ in (xn_u, XL_u, WB_u, UL_u, WO_u, z1_v, R_u, Lc_u, L2_u, R2_u, C_v, zf_v, zg_v, kv_u, u_u, X_v, H_v, G_v, Z_u,
                       kf_v, bcol_v):
                c_ = pltpu.make_async_copy(r_, r_, sem_small.at[0])
                c_.start()
                c_.wait()

    debug_keep_alive()

    cp_x(0).start()
    cp_win(0).start()
    cp_x(1).start()
    cp_win(1).start()
    start(cp_small())
    for c in range(2, 5):
        cp_win(c).start()
    cp_x(2).start()

    kk = _odd_freq(jax.lax.broadcasted_iota(jnp.int32, (P, P), 0))
    nn = jax.lax.broadcasted_iota(jnp.int32, (P, P), 1)
    fc, fs = _cos_sin((kk * (4 * nn - 127)) & 2047)
    for g in range(P // 8):
        F_v[g * 16:(g + 1) * 16, 0:P] = jnp.concatenate(
            [fc[g * 8:(g + 1) * 8], -fs[g * 8:(g + 1) * 8]], axis=0).astype(BF16)
    fc, fs = _cos_sin((kk * (-127)) & 2047)
    ph_v[0] = fc
    ph_v[1] = fs
    kk = _odd_freq(jax.lax.broadcasted_iota(jnp.int32, (MC, P), 1))
    mm = jax.lax.broadcasted_iota(jnp.int32, (MC, P), 0)
    ic, is_ = _cos_sin((kk * (4 * mm + 2)) & 2047)
    Fi_v[:, 0:P] = (ic * (1.0 / (P * GA))).astype(BF16)
    Fi_v[:, P:2 * P] = (is_ * (1.0 / (P * GA))).astype(BF16)
    kf_v[:, 0:8, :] = jnp.zeros((D // L, 8, L), F32)

    cp_x(0).wait()
    for s in range(TM // 16):
        ln_x(0, s)

    def small_setup():
        sk = sk_in[...].astype(F32)
        for t in range(4):
            sk_v[t] = jnp.broadcast_to(sk[t:t + 1], (8, D))
        drow = d_in[...].astype(F32).reshape(1, D)
        for l in range(D // L):
            lanes = slice(l * L, (l + 1) * L)
            dre = ph_v[0] * drow[:, lanes]
            dim = ph_v[1] * drow[:, lanes]
            H_v[0, 0, 0:64, lanes] = -dim[0:64]
            H_v[0, 0, 64:P, lanes] = dim[64:P]
            H_v[0, 1, 0:64, lanes] = -dre[0:64]
            H_v[0, 1, 64:P, lanes] = dre[64:P]

    def bcol_task(t, j, tie):
        brow = b_in[...].astype(F32).reshape(1, S)[:, j * P:(j + 1) * P] * (0.25 / GA) + tie[0:1]
        bcol_v[j * P:(j + 1) * P, :] = jnp.broadcast_to(brow, (P, P)).T

    LAG = 2

    def interleave(*lists):
        out = []
        for j in range(max(len(a) for a in lists)):
            for a in lists:
                out += a[j:j + 1]
        return out

    def p1_first(c):
        bg = _Background()
        todo = []
        if c == 2:
            todo = tasks(bcol_task, 0)
            small_setup()
        if c == 3:
            todo = tasks(ln_z2, 0)
            bg.add(wcomb_gen(range(3)))
        if c == 4:
            todo = tasks(ln_x2, 2, 8)
            bg.add(wcomb_gen(range(3, 6)))
        tied = _Tied(todo, F_TIED[c])
        if c == 0:
            for s in range(TM // 16):
                ln_x(1, s)
        for t in range(2):
            for m in range(TM // MC):
                job_z(t, m, range(*WIN_CHUNKS[c]), bg, (80, 40), tied)
        bg.drain()
        assert not tied.tasks

    for c in range(5):
        cp_win(c).wait()
        if c == 0:
            cp_x(1).wait()
        if c == 2:
            wait(cp_small())
            start(cp_conv(0))
            cp_x(3).start()
        if c == 4:
            cp_x(2).wait()
            cp_x(4).start()
        block(lambda c=c: p1_first(c), f'p1_f{c}')

    def p1_wait(g):
        if g == 0:
            wait(cp_conv(0))
            cp_x(3).wait()
        if g == 1:
            wait(cp_conv(1))
            cp_x(4).wait()
        if g == 2:
            wait(cp_conv(2))
            cp_x(6).wait()
        if g == 3:
            wait(cp_conv(4))
            cp_wout().wait()
            wait(cp_wsp(0))

    def p1_start(g):
        if g == 0:
            start(cp_conv(1))
            cp_x(6).start()
            start(cp_conv(2))
        if g == 1:
            start(cp_conv(4))
            cp_wout().start()
            start(cp_wsp(0))
            start(cp_wsp(1))
        if g == 3:
            start(cp_wsp(2))
            start(cp_conv(6))
            for i in (3, 4, 5):
                start(cp_wsp(i))

    def take(gen, n):
        for _ in range(n):
            yield next(gen)

    def p1_step(i):
        bg = _Background()
        dft = _Background()
        t = i - LAG
        xg = P1_X[i]
        kv = kv_gen(t)
        nx, nz, nh = KV_SPLIT[i]
        dft.add(take(kv, nx))
        bg.add(take(kv, nz))
        hbg = _Background()
        hbg.add(take(kv, nh))
        zb = nz * KV_COST / 48.0
        extra = 0
        if i == 6:
            bg.add(wocomb_gen())
            bg.add(acomb_gen(0, range(5)))
            extra = EXTRA[0]
        if i == 7:
            bg.add(acomb_gen(0, range(5, 8)))
            bg.add(bcomb2_gen((1, 5)))
            extra = EXTRA[1]
        last = i == NT - 1
        z2t = tasks(ln_z2, i - 1)
        xt = [tasks(ln_x2, t_, 8) for t_ in P1_LNX[i]]
        if P1_TUNE[i][1]:
            todo = interleave(*([z2t[0::2]] + xt + [z2t[1::2]]))
        else:
            todo = interleave(*(xt + [z2t[0::2], z2t[1::2]]))
        tied = _Tied(todo, P1_TUNE[i][0])
        if xg is not None:
            dft.run(KV_COST)
            job_x(xg, dft, (nx - 1) * KV_COST / 10.0)
            dft.drain()
        for p in range(2):
            for j in range(FH // L):
                job_zs(i, p, j, bg, (1.6 * zb + extra, 0.5 * zb + extra), tied)
            assert not tied.tasks or (p == 0 and not last)
            if p == 0 and last:
                tied = _Tied(tasks(ln_z2, i, 8), LAST_N)
        if last:
            for s in range(8, 16):
                ln_z2(i, s)
        bg.drain()
        job_h(t, hbg, nh * KV_COST / 10.0)
        hbg.drain()

    def p1_block(g):
        for i in P1_GROUPS[g]:
            p1_step(i)

    for g in range(len(P1_GROUPS)):
        p1_wait(g)
        p1_start(g)
        block(lambda g=g: p1_block(g), f'p1_g{g}')

    groups = P2_GROUPS
    NG = len(groups)

    def p2_dma(gi):
        if gi >= 2:
            for i in groups[gi - 2]:
                start(cp_out(i))
        if gi >= 3:
            for i in groups[gi - 3]:
                wait(cp_out(i))
        if gi == 1:
            for i in (6, 7):
                start(cp_wsp(i))
        if gi == 0:
            wait(cp_conv(6))
        if gi + 1 < NG:
            for i in groups[gi + 1]:
                wait(cp_wsp(i))

    def tails_of(i, bg, budget):
        return [tail_gen(i, bg, budget)] * 20

    def p2_block(gi):
        bg = _Background()
        steps = groups[gi]
        tb = [0.0]
        pending = [t_ for i in (groups[gi - 1] if gi > 0 else []) for t_ in tails_of(i, bg, tb)]
        total = sum(a + 1 for i in steps for a in _blocks_of_step(i)) * 40 * 16
        total += len(steps) * (24 * E_COST + 6 * U_COST) + len(pending) * T_COST
        slots = sum(84 if i == 0 else 77 for i in steps) + TAIL_W * len(pending)
        bg.add(freq_gen(_blocks_of_step(steps[0])[0]))
        if gi == 0:
            bg.add(bcomb2_gen((0, 2, 3, 4, 6)))
            total += 5 * 16 * A_COST
        if gi < 2:
            bg.add(kv_gen(NT - 2 + gi))
            total += 20 * KV_COST
            slots += 10
        for t in P2_X[gi]:
            slots += 10
        if gi + 1 < NG:
            for i in groups[gi + 1]:
                bg.add(acomb2_gen(i))
                total += 16 * 7 * A2_COST
        for i in steps[1:]:
            bg.add(freq_gen(_blocks_of_step(i)[0]))
        budget = tb[0] = total / (slots + P2_END[gi])
        bg.run(budget)
        for t in P2_X[gi]:
            job_x(t, bg, budget, FINE)
        if gi < 2:
            job_h(NT - 2 + gi, bg, budget, FINE)
        units = [4, 4, 2, 4, 4, 2] * (len(pending) // 20)
        every = [0] * sum(6 if i == 0 else 9 for i in steps)
        for j, n in enumerate(units):
            every[min(len(every) - 1, j * len(every) // len(units))] += n
        for i in steps:
            job_big(i, bg, pending, budget, every)
        for t_ in pending:
            next(t_)
        bg.drain()

    for gi in range(NG):
        p2_dma(gi)
        block(lambda gi=gi: p2_block(gi), f'p2_{gi}')

    def cp_last(part):
        a0 = _blocks_of_step(NT - 1)[0]
        sub, cols = ((MC, pl.ds(0, D)), (0, pl.ds(0, 4 * L)), (0, pl.ds(4 * L, L)))[part]
        return [pltpu.make_async_copy(o_v.at[pl.ds(r, MC), cols], o_hbm.at[0, pl.ds(r, MC), cols],
                                      sem_out.at[NT - 1]) for r in (a0 * P + sub, (a0 + 1) * P + sub)]

    def p2_last():
        for i in groups[NG - 1]:
            for j, t_ in enumerate(tails_of(i, _Background(), [0.0])):
                next(t_)
                if i < NT - 1 and j == 19:
                    start(cp_out(i))
                if i == NT - 1 and j in (9, 17):
                    start(cp_last(j // 10))

    p2_dma(NG)
    block(p2_last, 'p2_last')
    start(cp_last(2))
    for i in groups[NG - 2] + groups[NG - 1][:-1]:
        wait(cp_out(i))
    for part in range(3):
        wait(cp_last(part))
    debug_keep_alive()


def _compiler_params():
    vmem = 116 * 1024 * 1024
    try:
        return pltpu.CompilerParams(vmem_limit_bytes=vmem, disable_semaphore_checks=True)
    except TypeError:
        return pltpu.CompilerParams(vmem_limit_bytes=vmem)


@jax.jit
def pallas_recurrent_scan__ssm_conv_h3__mixer_gmlp__prompt_kernel(
    A_q: jax.Array,
    A_k: jax.Array,
    A_v: jax.Array,
    A_shift_k: jax.Array,
    A_ssm_k: jax.Array,
    A_ssm_D: jax.Array,
    B_x: jax.Array,
    B_w_in: jax.Array,
    B_w_sp: jax.Array,
    B_b_sp: jax.Array,
    B_w_out: jax.Array,
):
    del B_x
    hbm = pl.BlockSpec(memory_space=pl.ANY)

    def bf16_buf(*shape):
        return pltpu.VMEM(shape[:-2] + (shape[-2] // 2, shape[-1]), U32)

    return pl.pallas_call(
        _kernel,
        out_shape=jax.ShapeDtypeStruct((1, S, D), BF16),
        in_specs=[hbm] * 10,
        out_specs=hbm,
        scratch_shapes=[
            [bf16_buf(len(g) * TM, D) for g in X_DMAS],
            [bf16_buf(len(g) * TM, D) for g in CONV_DMAS],
            [bf16_buf(len(g) * TM, D) for g in CONV_DMAS],
            [bf16_buf(D, len(g) * TM) for g in CONV_DMAS],
            [bf16_buf(D, max(hi - lo, 2) * L) for lo, hi in WIN_CHUNKS],
            [bf16_buf(TM, S) for _ in range(NT)],
            bf16_buf(FH, D),
            pltpu.VMEM((S, D), BF16),
            pltpu.VMEM((4, D), BF16),
            pltpu.VMEM((D,), BF16),
            pltpu.VMEM((S,), BF16),
            bf16_buf(S, D),
            bf16_buf(4 * P, 5 * KH),
            bf16_buf(KH, 5 * FH),
            bf16_buf(5 * P, 5 * HN),
            bf16_buf(HN, 10 * L),
            pltpu.VMEM((S, FH), F32),
            bf16_buf(HK, 7 * HN),
            bf16_buf(5 * 5 * P, HK),
            bf16_buf(5 * 7 * MC, 5 * KQ),
            bf16_buf(7 * KQ, 5 * L),
            pltpu.VMEM((16 * MC, L), F32),
            pltpu.VMEM((HK, FH), F32),
            pltpu.VMEM((3, TM, FH), F32),
            bf16_buf(S, D),
            bf16_buf(S, FH),
            pltpu.VMEM((NB, 2, P, D), F32),
            pltpu.VMEM((2, 2, P, D), F32),
            pltpu.VMEM((NB, 2, P, D), F32),
            bf16_buf(NB // 2 * P, 4 * D),
            pltpu.VMEM((2, D // L, MC, L), F32),
            bf16_buf(2 * P, 2 * P),
            bf16_buf(MC, 2 * P),
            pltpu.VMEM((S, L), F32),
            pltpu.VMEM((2, P, L), F32),
            pltpu.VMEM((4, 8, D), F32),
            pltpu.VMEM((D // L, S + 8, L), F32),
            pltpu.SemaphoreType.DMA((1,)),
            pltpu.SemaphoreType.DMA((NT,)),
            pltpu.SemaphoreType.DMA((NT,)),
            pltpu.SemaphoreType.DMA((NT,)),
            pltpu.SemaphoreType.DMA((5,)),
            pltpu.SemaphoreType.DMA((NT,)),
        ],
        compiler_params=_compiler_params(),
    )(A_q, A_k, A_v, A_shift_k.T, A_ssm_k, A_ssm_D, B_w_in, B_w_sp, B_b_sp, B_w_out)
```

```python
import math

import jax
import jax.numpy as jnp
import jax.experimental.pallas as pl
import jax.experimental.pallas.tpu as pltpu

S = 2048
D = 640
FH = 768
P = 128
NB = S // P
TM = 256
NT = S // TM
MC = 64
L = 128
HK = S // 2
KQ = HK // 2
KH = 256
HN = FH // 2
EPS = 1e-5
F32 = jnp.float32
BF16 = jnp.bfloat16
U32 = jnp.uint32
GELU_C = math.sqrt(2.0 / math.pi)
GA = (GELU_C * 0.044715) ** (1.0 / 3.0)
NT_DIMS = (((1,), (1,)), ((), ()))

WIN_CHUNKS = ((6, 7), (7, 9), (9, 12), (0, 3), (3, 6))
X_DMAS = ((0,), (1,), (2,), (3,), (4, 5), (6, 7))
CONV_DMAS = ((0,), (1,), (2, 3), (4, 5), (6, 7))
P1_GROUPS = ((2,), (3,), (4, 5), (6, 7))
P1_X = {2: None, 3: 0, 4: 1, 5: None, 6: 2, 7: 3}
P1_LNX = {2: (3,), 3: (4, 5), 4: (6,), 5: (7,), 6: (), 7: ()}
P2_GROUPS = ((0,), (1, 2), (3, 4, 5), (6, 7))
P2_X = ((4, 5), (6,), (7,), ())
STEP_BLOCKS = ((2, 3), (6, 7), (4, 5), (12, 13), (10, 11), (0, 1), (14, 15), (8, 9))
KV_COST, A_COST, A2_COST = 110, 56, 34
E_COST, U_COST, T_COST, TAIL_W = 24, 90, 90, 1.6
KV_SPLIT = {2: (0, 14, 6), 3: (12, 4, 4), 4: (12, 4, 4), 5: (0, 14, 6), 6: (12, 4, 4), 7: (12, 4, 4)}
FR = 8
L1_USE = {0: ((0, 1, True, False), (3, 1, True, False)), 6: ((0, 1, False, False),),
          3: ((0, 1, False, False), (2, 1, True, False)), 4: ((0, -1, False, True), (1, 1, True, False)),
          1: ((2, 1, False, True), (3, -1, False, False)), 2: ((1, 1, False, True), (3, 1, False, False)),
          5: ((3, 1, False, True),)}
H_SPLIT = ((0, 2), (2, 4), (4, 5))
FINE = tuple((l, l + 1) for l in range(D // L))
P1_TUNE = {2: (40, 0), 3: (44, 0), 4: (42, 0), 5: (42, 0), 6: (44, 0), 7: (24, 0)}
EXTRA = (52, 52)
LAST_N = 22
P2_END = (0.0, -1.0, -1.0, 0.0)
F_TIED = (20, 20, 18, 20, 20)
_ONLY = None


def _dot(a, b):
    return jnp.dot(a, b, preferred_element_type=F32)


def _sums_left(a11, a12, a21, a22):
    add, sub = jax.lax.add, jax.lax.sub
    return jnp.concatenate((add(a11, a22), add(a21, a22), add(a11, a12), sub(a21, a11), sub(a12, a22)),
                           axis=1).astype(BF16)


def _sums_right(b11, b12, b21, b22):
    add, sub = jax.lax.add, jax.lax.sub
    return jnp.concatenate((add(b11, b22), sub(b12, b22), sub(b21, b11), add(b11, b12), add(b21, b22)),
                           axis=1).astype(BF16)


def _cos_sin(m):
    q = (m + 256) >> 9
    x = (m - (q << 9)).astype(F32) * (2.0 * math.pi / 2048.0)
    x2 = x * x
    s = x * (1.0 + x2 * (-1.0 / 6 + x2 * (1.0 / 120 + x2 * (-1.0 / 5040 + x2 * (1.0 / 362880)))))
    c = 1.0 + x2 * (-0.5 + x2 * (1.0 / 24 + x2 * (-1.0 / 720 + x2 * (1.0 / 40320 - x2 * (1.0 / 3628800)))))
    swap = (q & 1) == 1
    c0 = jnp.where(swap, s, c)
    s0 = jnp.where(swap, c, s)
    cos = jnp.where(((q + 1) & 2) == 2, -c0, c0)
    sin = jnp.where((q & 2) == 2, -s0, s0)
    return cos, sin


def _odd_freq(r):
    return jnp.where(r < 64, 4 * r + 1, 4 * r - 253)


def _gelu_scaled(z):
    return z + z * jnp.tanh(z * (GELU_C / GA + z * z))


def _signzero(z):
    bits = jax.lax.bitcast_convert_type(z, U32) & jnp.uint32(0x80000000)
    return jax.lax.bitcast_convert_type(bits, F32)


def _ln(x, eps, tie=None, scale=None):
    n = x.shape[-1]
    cols = [x[:, j * L:(j + 1) * L] for j in range(n // L)]
    s1 = cols[0]
    s2 = cols[0] * cols[0]
    for c in cols[1:]:
        s1 = s1 + c
        s2 = s2 + c * c
    if tie is not None:
        s1 = s1 + tie
        s2 = s2 + tie
    m = jnp.sum(s1, axis=-1, keepdims=True) * (1.0 / n)
    v = jnp.maximum(jnp.sum(s2, axis=-1, keepdims=True) * (1.0 / n) - m * m, 0.0)
    rs = jax.lax.rsqrt(v + eps)
    if scale is not None:
        rs = rs * scale
    return (x - m) * rs


def _blocks_of_step(i):
    return STEP_BLOCKS[i]


class _Background:
    def __init__(self):
        self.q = []
        self.credit = 0.0

    def add(self, gen):
        self.q.append(gen)

    def run(self, budget):
        self.credit += budget
        while self.q and self.credit > 0:
            try:
                self.credit -= next(self.q[0])
            except StopIteration:
                self.q.pop(0)
        if not self.q:
            self.credit = 0.0

    def charge(self, cost):
        self.credit -= cost

    def drain(self):
        while self.q:
            self.run(1e9)


class _Tied:
    def __init__(self, tasks, npieces):
        self.tasks = list(tasks)
        self.rate = len(self.tasks) / float(npieces)
        self.credit = 0.999

    def run(self, z):
        self.credit += self.rate
        n = 0
        while self.tasks and self.credit >= 1.0:
            self.tasks.pop(0)(_signzero(z[0:16]))
            self.credit -= 1.0
            n += 1
        return n


def _kernel(q_hbm, k_hbm, v_hbm, sk_hbm, h_hbm, d_hbm, win_hbm, wsp_hbm, b_hbm, wout_hbm,
            o_hbm,
            x_us, k_us, v_us, h_us, win_us, wsp_us, wout_u, o_v, sk_in, d_in, b_in,
            xn_u, XL_u, WB_u, UL_u, WO_u, z1_v, R_u, Lc_u, L2_u, R2_u, C_v, zf_v, zg_v, kv_u, u_u, X_v, H_v, G_v, Z_u,
            yl_v, F_u, Fi_u, bcol_v, ph_v, sk_v, kf_v,
            sem_small, sem_x, sem_conv, sem_wsp, sem_w, sem_out):
    (wout_v, xn_v, XL_v, WB_v, UL_v, WO_v, R_v, Lc_v, L2_v, R2_v, kv_v, u_v, Z_v, F_v, Fi_v) = [
        r.bitcast(BF16) for r in (wout_u, xn_u, XL_u, WB_u, UL_u, WO_u, R_u, Lc_u, L2_u, R2_u, kv_u, u_u, Z_u, F_u, Fi_u)]
    x_vs = {g[0]: r.bitcast(BF16) for g, r in zip(X_DMAS, x_us)}
    k_vs, v_vs, h_vs = [{g[0]: r.bitcast(BF16) for g, r in zip(CONV_DMAS, rs)} for rs in (k_us, v_us, h_us)]
    wsp_vs = [r.bitcast(BF16) for r in wsp_us]
    win_vs = [r.bitcast(BF16) for r in win_us]

    def win(rows, n):
        c = [lo <= n < hi for lo, hi in WIN_CHUNKS].index(True)
        n -= WIN_CHUNKS[c][0]
        return win_vs[c][rows, n * L:(n + 1) * L]

    def locate(bufs, row):
        t0 = max(t for t in bufs if t * TM <= row)
        return bufs[t0], row - t0 * TM

    def rows_of(bufs, row, n, lanes=slice(None)):
        buf, r = locate(bufs, row)
        return buf[r:r + n, lanes]

    def cp_small():
        return [pltpu.make_async_copy(s_, d_, sem_small.at[0])
                for s_, d_ in ((d_hbm, d_in), (sk_hbm, sk_in), (b_hbm, b_in))]

    def cp_x(t):
        return pltpu.make_async_copy(q_hbm.at[0, pl.ds(t * TM, x_vs[t].shape[0])], x_vs[t], sem_x.at[t])

    def cp_conv(t):
        rows = pl.ds(t * TM, k_vs[t].shape[0])
        sem = sem_conv.at[t]
        return [pltpu.make_async_copy(h_hbm.at[:, rows], h_vs[t], sem),
                pltpu.make_async_copy(k_hbm.at[0, rows], k_vs[t], sem),
                pltpu.make_async_copy(v_hbm.at[0, rows], v_vs[t], sem)]

    def cp_wsp(i):
        return [pltpu.make_async_copy(wsp_hbm.at[pl.ds(_blocks_of_step(i)[0] * P, TM)], wsp_vs[i], sem_wsp.at[i])]

    def cp_win(c):
        lo, hi = WIN_CHUNKS[c]
        w = (hi - lo) * L
        return pltpu.make_async_copy(win_hbm.at[:, pl.ds(lo * L, w)], win_vs[c].at[:, pl.ds(0, w)], sem_w.at[c])

    def cp_wout():
        return pltpu.make_async_copy(wout_hbm, wout_v, sem_w.at[0])

    def cp_out(i):
        rows = pl.ds(_blocks_of_step(i)[0] * P, TM)
        return [pltpu.make_async_copy(o_v.at[rows], o_hbm.at[0, rows], sem_out.at[i])]

    def start(cs):
        for c in cs:
            c.start()

    def wait(cs):
        for c in cs:
            c.wait()

    def block(fn, name):
        def body(it):
            fn()
            return it + 1

        if _ONLY is None or name in _ONLY:
            jax.lax.while_loop(lambda it: it < 1, body, jnp.int32(0))

    def ln_x(t, s, tie=None):
        rows = pl.ds(t * TM + s * 16, 16)
        y = _ln(rows_of(x_vs, t * TM + s * 16, 16).astype(F32), EPS, tie, GA)
        xn_v[rows, :] = y.astype(BF16)
        return y

    def ln_x2_tasks(t):
        held = {}

        def first(s, tie):
            held[s] = ln_x(t, 8 * (s // 4) + s % 4, tie)

        def second(s, tie):
            p, q = s // 4, s % 4
            y1, y2 = held.pop(s), ln_x(t, 8 * p + 4 + q, tie)
            XL_v[pl.ds((t % 4) * P + p * MC + q * 16, 16), :] = _sums_left(
                y1[:, :KH], y1[:, KH:2 * KH], y2[:, :KH], y2[:, KH:2 * KH])

        return [[lambda tie, s=s: first(s, tie) for s in range(8)],
                [lambda tie, s=s: second(s, tie) for s in range(8)]]

    def wcomb_gen(cols):
        for j in cols:
            for r in range(KH // 32):
                top = pl.ds(r * 32, 32)
                bot = pl.ds(KH + r * 32, 32)
                b11, b12 = win(top, j).astype(F32), win(top, 6 + j).astype(F32)
                b21, b22 = win(bot, j).astype(F32), win(bot, 6 + j).astype(F32)
                WB_v[top, j * 5 * L:(j + 1) * 5 * L] = _sums_right(b11, b12, b21, b22)
                yield A_COST

    def ln_z2(t, s, tie=None):
        y = _ln(zg_v[t % 3, s * 16:(s + 1) * 16, :], 4.0 * GA * GA * EPS, tie, 0.25 / GA)
        lo, hi = y[:, :HN], y[:, HN:]
        rows = pl.ds((t * TM + s * 16) % HK, 16)
        if t < NT // 2:
            zf_v[rows, :] = y
            R_v[rows, 0:2 * HN] = jnp.concatenate((lo, lo + hi), axis=1).astype(BF16)
        else:
            b11, b12 = zf_v[rows, :HN], zf_v[rows, HN:]
            R_v[rows, 2 * HN:] = jnp.concatenate((b11 + hi, b12 - hi, lo - b11, hi, lo + hi), axis=1).astype(BF16)

    def r1(j, rows, n):
        c0 = {1: 0, 5: 1, 0: 2, 2: 3, 3: 4, 4: 5, 6: 6}[j] * HN + n * L
        return R_v[rows, c0:c0 + L]

    def acomb_gen(i, groups=range(P // 16)):
        for r in groups:
            for c in range(HK // 256):
                top = pl.ds(r * 16, 16)
                bot = pl.ds(P + r * 16, 16)
                c1 = slice(c * 256, (c + 1) * 256)
                c2 = slice(HK + c * 256, HK + (c + 1) * 256)
                a11 = wsp_vs[i][top, c1].astype(F32)
                a12 = wsp_vs[i][top, c2].astype(F32)
                a21 = wsp_vs[i][bot, c1].astype(F32)
                a22 = wsp_vs[i][bot, c2].astype(F32)
                r0 = (i % 5) * 5 * P + (r % 4 * 2 + r // 4) * 16
                Lc_v[pl.ds(r0 + 0 * P, 16), c1] = (a11 + a22).astype(BF16)
                Lc_v[pl.ds(r0 + 1 * P, 16), c1] = (a21 + a22).astype(BF16)
                Lc_v[pl.ds(r0 + 2 * P, 16), c1] = (a11 + a12).astype(BF16)
                Lc_v[pl.ds(r0 + 3 * P, 16), c1] = (a21 - a11).astype(BF16)
                Lc_v[pl.ds(r0 + 4 * P, 16), c1] = (a12 - a22).astype(BF16)
                yield A_COST

    def acomb2_gen(i):
        for r in range(MC // 16):
            for c in range(KQ // L):
                quad = {}

                def w(b, H):
                    if (b, H) not in quad:
                        quad[b, H] = [[wsp_vs[i][pl.ds(b * P + s_ * MC + r * 16, 16),
                                                 H * HK + kh * KQ + c * L:H * HK + kh * KQ + (c + 1) * L].astype(F32)
                                       for kh in range(2)] for s_ in range(2)]
                    return quad[b, H]

                spec = {2: (None, (0, 0), None, 0), 0: (0, (0, 0), (1, 1), 1), 3: (None, (1, 1), None, 0),
                        1: (1, (1, 0), (1, 1), 1), 5: (3, (1, 0), (0, 0), -1), 4: (2, (0, 0), (0, 1), 1),
                        6: (4, (0, 1), (1, 1), -1)}
                for j in (2, 0, 3, 1, 5, 4, 6):
                    slot, p_, q_, sign = spec[j]
                    a = w(*p_)
                    if q_ is not None:
                        b_ = w(*q_)
                        op = jax.lax.add if sign > 0 else jax.lax.sub
                        a = [[op(a[s_][kh], b_[s_][kh]) for kh in range(2)] for s_ in range(2)]
                        for kh in range(2):
                            Lc_v[pl.ds(((i % 5) * 5 + slot) * P + r * 32, 32),
                                 kh * KQ + c * L:kh * KQ + (c + 1) * L] = jnp.concatenate(
                                     (a[0][kh], a[1][kh]), axis=0).astype(BF16)
                    L2_v[pl.ds(((i % 5) * 7 + j) * MC + r * 16, 16), c * 5 * L:(c + 1) * 5 * L] = _sums_left(
                        a[0][0], a[0][1], a[1][0], a[1][1])
                    yield A2_COST

    def bcomb2_gen(js):
        for j in js:
            for r in range(KQ // 16):
                top = pl.ds(r * 16, 16)
                bot = pl.ds(KQ + r * 16, 16)
                R2_v[pl.ds(j * KQ + r * 16, 16), :] = _sums_right(
                    *[r1(j, rows, n).astype(F32) for rows in (top, bot) for n in range(2)])
                yield A_COST / 2

    def tasks(fn, t, n=TM // 16):
        return [lambda tie, s=s: fn(t, s, tie) for s in range(n)]

    def kv_gen(t):
        for m in range(TM // MC):
            r = t * TM + m * MC
            for l in range(D // L):
                lanes = slice(l * L, (l + 1) * L)
                kf = rows_of(k_vs, r, MC, lanes).astype(F32)
                kf_v[l, pl.ds(r + 8, MC), :] = kf
                ks = kf * sk_v[0, 0:1, lanes]
                for tap in range(1, 4):
                    ks = ks + kf_v[l, pl.ds(r + 8 - tap, MC), :] * sk_v[tap, 0:1, lanes]
                kv = ks * rows_of(v_vs, r, MC, lanes).astype(F32)
                kv_v[pl.ds(r, MC), lanes] = kv.astype(BF16)
                yield KV_COST

    def freq_gen(a):
        def cmac(acc, x, g):
            mul, add = jax.lax.mul, jax.lax.add
            pr = jax.lax.sub(mul(x[0], g[0]), mul(x[1], g[1]))
            pi = add(mul(x[0], g[1]), mul(x[1], g[0]))
            return (pr, pi) if acc is None else (add(acc[0], pr), add(acc[1], pi))

        for r in range(P // 16):
            for l in range(D // L):
                lanes = slice(l * L, (l + 1) * L)
                res = []
                for sub in range(16 // FR):
                    rows = pl.ds(r * 16 + sub * FR, FR)
                    lo = hi = None
                    g = (G_v[a + 1, 0, rows, lanes], G_v[a + 1, 1, rows, lanes])
                    for c in range(a + 2):
                        x = (X_v[c, 0, rows, lanes], X_v[c, 1, rows, lanes])
                        hi = cmac(hi, x, g)
                        if c <= a:
                            g = (G_v[a - c, 0, rows, lanes], G_v[a - c, 1, rows, lanes])
                            lo = cmac(lo, x, g)
                            yield 2 * FR
                    res.append((lo, hi))
                Z_v[pl.ds(a // 2 * P + r * 16, 16), l * 4 * L:(l + 1) * 4 * L] = jnp.concatenate(
                    [jnp.concatenate([z[0][0], z[0][1], z[1][0], z[1][1]], axis=1) for z in res], axis=0).astype(BF16)
                yield 20

    def job_x(t, bg, budget, split=((0, 5),)):
        for j in (2 * t, 2 * t + 1):
            for half in range(2):
                for l0, l1 in split:
                    w, lanes = (l1 - l0) * L, slice(l0 * L, l1 * L)
                    r = _dot(F_v[half * P:(half + 1) * P, 0:P], kv_v[j * P:(j + 1) * P, lanes]).reshape(8, 2, 8, w)
                    for part in range(2):
                        X_v[j, part, half * 64:(half + 1) * 64, lanes] = r[:, part].reshape(64, w)
                    bg.run(budget * (l1 - l0) / 2)

    def job_h(t, bg, budget, split=H_SPLIT):
        h_v, c0 = locate(h_vs, t * TM)
        for half in range(2):
            rows = pl.ds(half * 64, 64)
            for l0, l1 in split:
                w = (l1 - l0) * L
                lanes = slice(l0 * L, l1 * L)
                rhs = jnp.concatenate([h_v[lanes, c0:c0 + P], h_v[lanes, c0 + P:c0 + TM]], axis=0)
                r = jax.lax.dot_general(F_v[half * P:(half + 1) * P, 0:P], rhs, NT_DIMS,
                                        preferred_element_type=F32).reshape(8, 2, 8, 2 * w)
                re, im = r[:, 0].reshape(64, 2 * w), r[:, 1].reshape(64, 2 * w)
                prev = (H_v[t % 2, 0, rows, lanes], H_v[t % 2, 1, rows, lanes])
                for j in range(2):
                    cur = (re[:, j * w:(j + 1) * w], im[:, j * w:(j + 1) * w])
                    G_v[2 * t + j, 0, rows, lanes] = cur[0] + prev[1] if half else cur[0] - prev[1]
                    G_v[2 * t + j, 1, rows, lanes] = cur[1] - prev[0] if half else cur[1] + prev[0]
                    prev = cur
                if t + 1 < NT:
                    H_v[(t + 1) % 2, 0, rows, lanes] = prev[0]
                    H_v[(t + 1) % 2, 1, rows, lanes] = prev[1]
                bg.run(budget * (l1 - l0))

    def z_out(t, m, n, pre, bg, budget, tied):
        z = _gelu_scaled(pre)
        if n < FH // L:
            z1_v[pl.ds(t * TM + m * MC, MC), n * L:(n + 1) * L] = z
        else:
            zg_v[t % 3, m * MC:(m + 1) * MC, n * L - FH:(n + 1) * L - FH] = z
        ntask = tied.run(z)
        bg.run(budget[1] if ntask else budget[0])

    def job_z(t, m, cols, bg, budget, tied):
        for n in cols:
            z_out(t, m, n, _dot(xn_v[pl.ds(t * TM + m * MC, MC), :], win(slice(None), n)), bg, budget, tied)

    def job_zs(t, p, j, bg, budget, tied):
        r1 = pl.ds(t * TM + p * P, MC)
        r2 = pl.ds(t * TM + p * P + MC, MC)

        def xl(w):
            r0 = (t % 4) * P + p * MC
            return XL_v[r0:r0 + MC, w * KH:(w + 1) * KH]

        def wb(w):
            return WB_v[:, (j * 5 + w) * L:(j * 5 + w + 1) * L]

        def rem(rows, n):
            return _dot(xn_v[rows, 2 * KH:], win(slice(2 * KH, D), n))

        m2 = _dot(xl(1), win(slice(0, KH), j))
        m4 = _dot(xn_v[r2, KH:2 * KH], wb(2))
        z_out(t, 2 * p + 1, j, m2 + m4 + rem(r2, j), bg, budget, tied)
        m3 = _dot(xn_v[r1, 0:KH], wb(1))
        m5 = _dot(xl(2), win(slice(KH, 2 * KH), 6 + j))
        z_out(t, 2 * p, 6 + j, m3 + m5 + rem(r1, 6 + j), bg, budget, tied)
        t11, t22 = m4 - m5, m3 - m2
        m1 = _dot(xl(0), wb(0))
        t11, t22 = t11 + m1, t22 + m1
        z_out(t, 2 * p, j, t11 + _dot(xl(4), wb(4)) + rem(r1, j), bg, budget, tied)
        z_out(t, 2 * p + 1, 6 + j, t22 + _dot(xl(3), wb(3)) + rem(r2, 6 + j), bg, budget, tied)

    rev8 = 7 - jax.lax.broadcasted_iota(jnp.int32, (8, L), 0)

    def finish(a, upper, n, hh, slot):
        rows = pl.ds(a * P + (MC if upper else 0), MC)
        lanes = slice(n * L, (n + 1) * L)
        if upper:
            zc = (n * 4 + a % 2 * 2) * L
            ya = _dot(Fi_v[:, 0:P], Z_v[a // 2 * P:(a // 2 + 1) * P, zc:zc + L])
            yb = _dot(Fi_v[:, P:2 * P], Z_v[a // 2 * P:(a // 2 + 1) * P, zc + L:zc + 2 * L])
            slot(0.5)
            y = ya - yb
            lo = ya + yb
            for j in range(MC // 8):
                yl_v[a % 2, n, (7 - j) * 8:(8 - j) * 8, :] = jnp.take_along_axis(lo[j * 8:(j + 1) * 8], rev8, axis=0)
        else:
            y = yl_v[a % 2, n]
        gate = hh + hh * jnp.tanh(hh)
        s = xn_v[rows, lanes].astype(F32) * y
        x = rows_of(x_vs, a * P + (MC if upper else 0), MC, lanes).astype(F32)
        o_v[rows, lanes] = (x + s * gate).astype(BF16)

    def tail_gen(i, bg, budget):
        a0, a1 = _blocks_of_step(i)

        def slot(w):
            bg.run(w * budget[0])

        def dot3(a, b):
            r = _dot(a, b)
            slot(0.75)
            return r

        for upper in (True, False):
            sub = MC if upper else 0
            r1 = pl.ds(a0 * P + sub, MC)
            r2 = pl.ds(a1 * P + sub, MC)

            def ul(w):
                allw = UL_v[(i % 5) * P + sub:(i % 5) * P + sub + MC, :]
                return jnp.concatenate([allw[:, (n * 5 + w) * L:(n * 5 + w + 1) * L] for n in range(HN // L)], axis=1)

            for j in range(2):
                c1 = slice(j * L, (j + 1) * L)
                c2 = slice((2 + j) * L, (3 + j) * L)

                def wo(w):
                    return WO_v[:, (j * 5 + w) * L:(j * 5 + w + 1) * L]

                m2 = dot3(ul(1), wout_v[0:HN, c1])
                m4 = dot3(u_v[r2, HN:], wo(2))
                finish(a1, upper, j, m2 + m4, slot)
                bg.charge(T_COST)
                yield
                m3 = dot3(u_v[r1, 0:HN], wo(1))
                m5 = dot3(ul(2), wout_v[HN:, c2])
                finish(a0, upper, 2 + j, m3 + m5, slot)
                bg.charge(T_COST)
                yield
                t11, t22 = m4 - m5, m3 - m2
                m1 = dot3(ul(0), wo(0))
                t11, t22 = t11 + m1, t22 + m1
                finish(a0, upper, j, t11 + dot3(ul(4), wo(4)), slot)
                bg.charge(T_COST)
                yield
                finish(a1, upper, 2 + j, t22 + dot3(ul(3), wo(3)), slot)
                bg.charge(T_COST)
                yield
            for a, r in ((a0, r1), (a1, r2)):
                finish(a, upper, 4, dot3(u_v[r, 0:HN], wout_v[0:HN, 4 * L:]) + dot3(u_v[r, HN:], wout_v[HN:, 4 * L:]),
                       slot)
                bg.charge(T_COST)
                yield

    def wocomb_gen():
        for j in range(2):
            c1 = slice(j * L, (j + 1) * L)
            c2 = slice((2 + j) * L, (3 + j) * L)
            for r in range(HN // 32):
                top = pl.ds(r * 32, 32)
                bot = pl.ds(HN + r * 32, 32)
                b11, b12 = wout_v[top, c1].astype(F32), wout_v[top, c2].astype(F32)
                b21, b22 = wout_v[bot, c1].astype(F32), wout_v[bot, c2].astype(F32)
                WO_v[top, j * 5 * L:(j + 1) * 5 * L] = _sums_right(b11, b12, b21, b22)
                yield A_COST

    def job_big(i, bg, pending, budget, every):
        a0, a1 = _blocks_of_step(i)
        KG = 512

        def lhs(j, sub, cols):
            if j == 2:
                return wsp_vs[i][sub:sub + MC, cols]
            if j == 3:
                return wsp_vs[i][P + sub:P + sub + MC, HK + cols.start:HK + cols.stop]
            r0 = ((i % 5) * 5 + {0: 0, 1: 1, 4: 2, 5: 3, 6: 4}[j]) * P
            both = Lc_v[r0:r0 + P, cols]
            return jnp.concatenate([both[q * 32 + sub // 4:q * 32 + sub // 4 + 16] for q in range(4)], axis=0)

        def prod(j, sub, n, acc=None):
            for kg in range(HK // KG):
                ks = slice(kg * KG, (kg + 1) * KG)
                p = _dot(lhs(j, sub, ks), r1(j, ks, n))
                acc = p if acc is None else p + acc
                bg.run(budget)
            return acc

        def tails(n):
            for _ in range(n):
                if pending:
                    next(pending.pop(0))

        def emit(a, sub, n, g):
            rows = pl.ds(a * P + sub, MC)
            lanes = slice(n * L, (n + 1) * L)
            u = z1_v[rows, lanes] * (g + bcol_v[rows, :])
            u_v[rows, lanes] = u.astype(BF16)
            bg.charge(E_COST)
            return u

        if i > 0:
            def piece(a, b, acc=None):
                p = _dot(a, b)
                bg.run(budget)
                return p if acc is None else acc + p

            def cslot(k, s_, n):
                return pl.ds(((k * 2 + s_) * 2 + n) * MC, MC)

            def contribute(j, s_, n, m):
                for k, sign, first, last in L1_USE[j]:
                    cs = cslot(k, s_, n)
                    v_ = m if first else (C_v[cs, :] + m if sign > 0 else C_v[cs, :] - m)
                    if last:
                        u = emit((a0, a0, a1, a1)[k], s_ * MC, n + (k % 2) * (HN // L), v_)
                        v_ = u
                        if k == 3:
                            u11, u12, u21 = C_v[cslot(0, s_, n), :], C_v[cslot(1, s_, n), :], C_v[cslot(2, s_, n), :]
                            UL_v[pl.ds((i % 5) * P + s_ * MC, MC), n * 5 * L:(n + 1) * 5 * L] = _sums_left(
                                u11, u12, u21, u)
                            bg.charge(U_COST)
                            continue
                    C_v[cs, :] = v_

            for j in (0, 6, 3, 4, 1, 2, 5):
                def l2(w):
                    r0 = ((i % 5) * 7 + j) * MC
                    allw = L2_v[r0:r0 + MC, :]
                    return jnp.concatenate([allw[:, (c * 5 + w) * L:(c * 5 + w + 1) * L] for c in range(KQ // L)],
                                           axis=1)

                def r2(w):
                    return R2_v[j * KQ:(j + 1) * KQ, w * L:(w + 1) * L]

                def rq(kh, n):
                    return r1(j, slice(kh * KQ, (kh + 1) * KQ), n)

                p2 = piece(l2(1), rq(0, 0))
                p4 = piece(lhs(j, MC, slice(KQ, 2 * KQ)), r2(2))
                contribute(j, 1, 0, p2 + p4)
                p3 = piece(lhs(j, 0, slice(0, KQ)), r2(1))
                t22 = p3 - p2
                p5 = piece(l2(2), rq(1, 1))
                contribute(j, 0, 1, p3 + p5)
                t11 = p4 - p5
                p1 = piece(l2(0), r2(0))
                t11, t22 = t11 + p1, t22 + p1
                contribute(j, 0, 0, piece(l2(4), r2(4), t11))
                contribute(j, 1, 1, piece(l2(3), r2(3), t22))
                tails(every.pop(0))

        for sub in (0, MC):
            for n in (range(HN // L) if i == 0 else (2,)):
                def put(w, c):
                    UL_v[pl.ds((i % 5) * P + sub, MC), (n * 5 + w) * L:(n * 5 + w + 1) * L] = c.astype(BF16)

                m1 = prod(0, sub, n)
                t11 = prod(6, sub, n, m1)
                m4 = prod(3, sub, n)
                t11 = t11 + m4
                m5 = prod(4, sub, n)
                u11 = emit(a0, sub, n, t11 - m5)
                m2 = prod(1, sub, n)
                u21 = emit(a1, sub, n, m2 + m4)
                put(3, u21 - u11)
                t22 = m1 - m2
                m3 = prod(2, sub, n)
                u12 = emit(a0, sub, n + HN // L, m3 + m5)
                put(2, u11 + u12)
                u22 = emit(a1, sub, n + HN // L, prod(5, sub, n, t22 + m3))
                put(0, u11 + u22)
                put(1, u21 + u22)
                put(4, u12 - u22)
                bg.charge(U_COST)
                tails(every.pop(0))

    def debug_keep_alive():
        if _ONLY is not None:
            for r_ in (xn_u, XL_u, WB_u, UL_u, WO_u, z1_v, R_u, Lc_u, L2_u, R2_u, C_v, zf_v, zg_v, kv_u, u_u, X_v, H_v, G_v, Z_u,
                       kf_v, bcol_v):
                c_ = pltpu.make_async_copy(r_, r_, sem_small.at[0])
                c_.start()
                c_.wait()

    debug_keep_alive()

    cp_x(0).start()
    cp_win(0).start()
    cp_x(1).start()
    cp_win(1).start()
    start(cp_small())
    for c in range(2, 5):
        cp_win(c).start()
    cp_x(2).start()

    kk = _odd_freq(jax.lax.broadcasted_iota(jnp.int32, (P, P), 0))
    nn = jax.lax.broadcasted_iota(jnp.int32, (P, P), 1)
    fc, fs = _cos_sin((kk * (4 * nn - 127)) & 2047)
    for g in range(P // 8):
        F_v[g * 16:(g + 1) * 16, 0:P] = jnp.concatenate(
            [fc[g * 8:(g + 1) * 8], -fs[g * 8:(g + 1) * 8]], axis=0).astype(BF16)
    fc, fs = _cos_sin((kk * (-127)) & 2047)
    ph_v[0] = fc
    ph_v[1] = fs
    kk = _odd_freq(jax.lax.broadcasted_iota(jnp.int32, (MC, P), 1))
    mm = jax.lax.broadcasted_iota(jnp.int32, (MC, P), 0)
    ic, is_ = _cos_sin((kk * (4 * mm + 2)) & 2047)
    Fi_v[:, 0:P] = (ic * (1.0 / (P * GA))).astype(BF16)
    Fi_v[:, P:2 * P] = (is_ * (1.0 / (P * GA))).astype(BF16)
    kf_v[:, 0:8, :] = jnp.zeros((D // L, 8, L), F32)

    cp_x(0).wait()
    for s in range(TM // 16):
        ln_x(0, s)

    def small_setup():
        sk = sk_in[...].astype(F32)
        for t in range(4):
            sk_v[t] = jnp.broadcast_to(sk[t:t + 1], (8, D))
        drow = d_in[...].astype(F32).reshape(1, D)
        for l in range(D // L):
            lanes = slice(l * L, (l + 1) * L)
            dre = ph_v[0] * drow[:, lanes]
            dim = ph_v[1] * drow[:, lanes]
            H_v[0, 0, 0:64, lanes] = -dim[0:64]
            H_v[0, 0, 64:P, lanes] = dim[64:P]
            H_v[0, 1, 0:64, lanes] = -dre[0:64]
            H_v[0, 1, 64:P, lanes] = dre[64:P]

    def bcol_task(t, j, tie):
        brow = b_in[...].astype(F32).reshape(1, S)[:, j * P:(j + 1) * P] * (0.25 / GA) + tie[0:1]
        bcol_v[j * P:(j + 1) * P, :] = jnp.broadcast_to(brow, (P, P)).T

    LAG = 2

    def interleave(*lists):
        out = []
        for j in range(max(len(a) for a in lists)):
            for a in lists:
                out += a[j:j + 1]
        return out

    def p1_first(c):
        bg = _Background()
        todo = []
        if c == 2:
            todo = tasks(bcol_task, 0)
            small_setup()
        if c == 3:
            todo = tasks(ln_z2, 0)
            bg.add(wcomb_gen(range(3)))
        if c == 4:
            todo = interleave(*ln_x2_tasks(2))
            bg.add(wcomb_gen(range(3, 6)))
        tied = _Tied(todo, F_TIED[c])
        if c == 0:
            for s in range(TM // 16):
                ln_x(1, s)
        for t in range(2):
            for m in range(TM // MC):
                job_z(t, m, range(*WIN_CHUNKS[c]), bg, (80, 40), tied)
        bg.drain()
        assert not tied.tasks

    for c in range(5):
        cp_win(c).wait()
        if c == 0:
            cp_x(1).wait()
        if c == 2:
            wait(cp_small())
            start(cp_conv(0))
            cp_x(3).start()
        if c == 4:
            cp_x(2).wait()
            cp_x(4).start()
        block(lambda c=c: p1_first(c), f'p1_f{c}')

    def p1_wait(g):
        if g == 0:
            wait(cp_conv(0))
            cp_x(3).wait()
        if g == 1:
            wait(cp_conv(1))
            cp_x(4).wait()
        if g == 2:
            wait(cp_conv(2))
            cp_x(6).wait()
        if g == 3:
            wait(cp_conv(4))
            cp_wout().wait()
            wait(cp_wsp(0))

    def p1_start(g):
        if g == 0:
            start(cp_conv(1))
            cp_x(6).start()
            start(cp_conv(2))
        if g == 1:
            start(cp_conv(4))
            cp_wout().start()
            start(cp_wsp(0))
            start(cp_wsp(1))
        if g == 3:
            start(cp_wsp(2))
            start(cp_conv(6))
            for i in (3, 4, 5):
                start(cp_wsp(i))

    def take(gen, n):
        for _ in range(n):
            yield next(gen)

    def p1_step(i):
        bg = _Background()
        dft = _Background()
        t = i - LAG
        xg = P1_X[i]
        kv = kv_gen(t)
        nx, nz, nh = KV_SPLIT[i]
        dft.add(take(kv, nx))
        bg.add(take(kv, nz))
        hbg = _Background()
        hbg.add(take(kv, nh))
        zb = nz * KV_COST / 48.0
        extra = 0
        if i == 6:
            bg.add(wocomb_gen())
            bg.add(acomb_gen(0, range(5)))
            extra = EXTRA[0]
        if i == 7:
            bg.add(acomb_gen(0, range(5, 8)))
            bg.add(bcomb2_gen((1, 5)))
            extra = EXTRA[1]
        last = i == NT - 1
        z2t = tasks(ln_z2, i - 1)
        xt = [l_ for t_ in P1_LNX[i] for l_ in ln_x2_tasks(t_)]
        if P1_TUNE[i][1]:
            todo = interleave(*([z2t[0::2]] + xt + [z2t[1::2]]))
        else:
            todo = interleave(*(xt + [z2t[0::2], z2t[1::2]]))
        tied = _Tied(todo, P1_TUNE[i][0])
        if xg is not None:
            dft.run(KV_COST)
            job_x(xg, dft, (nx - 1) * KV_COST / 10.0)
            dft.drain()
        for p in range(2):
            for j in range(FH // L):
                job_zs(i, p, j, bg, (1.6 * zb + extra, 0.5 * zb + extra), tied)
            assert not tied.tasks or (p == 0 and not last)
            if p == 0 and last:
                tied = _Tied(tasks(ln_z2, i, 8), LAST_N)
        if last:
            for s in range(8, 16):
                ln_z2(i, s)
        bg.drain()
        job_h(t, hbg, nh * KV_COST / 10.0)
        hbg.drain()

    def p1_block(g):
        for i in P1_GROUPS[g]:
            p1_step(i)

    for g in range(len(P1_GROUPS)):
        p1_wait(g)
        p1_start(g)
        block(lambda g=g: p1_block(g), f'p1_g{g}')

    groups = P2_GROUPS
    NG = len(groups)

    def p2_dma(gi):
        if gi >= 2:
            for i in groups[gi - 2]:
                start(cp_out(i))
        if gi >= 3:
            for i in groups[gi - 3]:
                wait(cp_out(i))
        if gi == 1:
            for i in (6, 7):
                start(cp_wsp(i))
        if gi == 0:
            wait(cp_conv(6))
        if gi + 1 < NG:
            for i in groups[gi + 1]:
                wait(cp_wsp(i))

    def tails_of(i, bg, budget):
        return [tail_gen(i, bg, budget)] * 20

    def p2_block(gi):
        bg = _Background()
        steps = groups[gi]
        tb = [0.0]
        pending = [t_ for i in (groups[gi - 1] if gi > 0 else []) for t_ in tails_of(i, bg, tb)]
        total = sum(a + 1 for i in steps for a in _blocks_of_step(i)) * 40 * 16
        total += len(steps) * (24 * E_COST + 6 * U_COST) + len(pending) * T_COST
        slots = sum(84 if i == 0 else 77 for i in steps) + TAIL_W * len(pending)
        bg.add(freq_gen(_blocks_of_step(steps[0])[0]))
        if gi == 0:
            bg.add(bcomb2_gen((0, 2, 3, 4, 6)))
            total += 5 * 16 * A_COST
        if gi < 2:
            bg.add(kv_gen(NT - 2 + gi))
            total += 20 * KV_COST
            slots += 10
        for t in P2_X[gi]:
            slots += 10
        if gi + 1 < NG:
            for i in groups[gi + 1]:
                bg.add(acomb2_gen(i))
                total += 16 * 7 * A2_COST
        for i in steps[1:]:
            bg.add(freq_gen(_blocks_of_step(i)[0]))
        budget = tb[0] = total / (slots + P2_END[gi])
        bg.run(budget)
        for t in P2_X[gi]:
            job_x(t, bg, budget, FINE)
        if gi < 2:
            job_h(NT - 2 + gi, bg, budget, FINE)
        units = [4, 4, 2, 4, 4, 2] * (len(pending) // 20)
        every = [0] * sum(6 if i == 0 else 9 for i in steps)
        for j, n in enumerate(units):
            every[min(len(every) - 1, j * len(every) // len(units))] += n
        for i in steps:
            job_big(i, bg, pending, budget, every)
        for t_ in pending:
            next(t_)
        bg.drain()

    for gi in range(NG):
        p2_dma(gi)
        block(lambda gi=gi: p2_block(gi), f'p2_{gi}')

    def cp_last(part):
        a0 = _blocks_of_step(NT - 1)[0]
        sub, cols = ((MC, pl.ds(0, D)), (0, pl.ds(0, 4 * L)), (0, pl.ds(4 * L, L)))[part]
        return [pltpu.make_async_copy(o_v.at[pl.ds(r, MC), cols], o_hbm.at[0, pl.ds(r, MC), cols],
                                      sem_out.at[NT - 1]) for r in (a0 * P + sub, (a0 + 1) * P + sub)]

    def p2_last():
        for i in groups[NG - 1]:
            for j, t_ in enumerate(tails_of(i, _Background(), [0.0])):
                next(t_)
                if i < NT - 1 and j == 19:
                    start(cp_out(i))
                if i == NT - 1 and j in (9, 17):
                    start(cp_last(j // 10))

    p2_dma(NG)
    block(p2_last, 'p2_last')
    start(cp_last(2))
    for i in groups[NG - 2] + groups[NG - 1][:-1]:
        wait(cp_out(i))
    for part in range(3):
        wait(cp_last(part))
    debug_keep_alive()


def _compiler_params():
    vmem = 116 * 1024 * 1024
    try:
        return pltpu.CompilerParams(vmem_limit_bytes=vmem, disable_semaphore_checks=True)
    except TypeError:
        return pltpu.CompilerParams(vmem_limit_bytes=vmem)


@jax.jit
def pallas_recurrent_scan__ssm_conv_h3__mixer_gmlp__prompt_kernel(
    A_q: jax.Array,
    A_k: jax.Array,
    A_v: jax.Array,
    A_shift_k: jax.Array,
    A_ssm_k: jax.Array,
    A_ssm_D: jax.Array,
    B_x: jax.Array,
    B_w_in: jax.Array,
    B_w_sp: jax.Array,
    B_b_sp: jax.Array,
    B_w_out: jax.Array,
):
    del B_x
    hbm = pl.BlockSpec(memory_space=pl.ANY)

    def bf16_buf(*shape):
        return pltpu.VMEM(shape[:-2] + (shape[-2] // 2, shape[-1]), U32)

    return pl.pallas_call(
        _kernel,
        out_shape=jax.ShapeDtypeStruct((1, S, D), BF16),
        in_specs=[hbm] * 10,
        out_specs=hbm,
        scratch_shapes=[
            [bf16_buf(len(g) * TM, D) for g in X_DMAS],
            [bf16_buf(len(g) * TM, D) for g in CONV_DMAS],
            [bf16_buf(len(g) * TM, D) for g in CONV_DMAS],
            [bf16_buf(D, len(g) * TM) for g in CONV_DMAS],
            [bf16_buf(D, max(hi - lo, 2) * L) for lo, hi in WIN_CHUNKS],
            [bf16_buf(TM, S) for _ in range(NT)],
            bf16_buf(FH, D),
            pltpu.VMEM((S, D), BF16),
            pltpu.VMEM((4, D), BF16),
            pltpu.VMEM((D,), BF16),
            pltpu.VMEM((S,), BF16),
            bf16_buf(S, D),
            bf16_buf(4 * P, 5 * KH),
            bf16_buf(KH, 5 * FH),
            bf16_buf(5 * P, 5 * HN),
            bf16_buf(HN, 10 * L),
            pltpu.VMEM((S, FH), F32),
            bf16_buf(HK, 7 * HN),
            bf16_buf(5 * 5 * P, HK),
            bf16_buf(5 * 7 * MC, 5 * KQ),
            bf16_buf(7 * KQ, 5 * L),
            pltpu.VMEM((16 * MC, L), F32),
            pltpu.VMEM((HK, FH), F32),
            pltpu.VMEM((3, TM, FH), F32),
            bf16_buf(S, D),
            bf16_buf(S, FH),
            pltpu.VMEM((NB, 2, P, D), F32),
            pltpu.VMEM((2, 2, P, D), F32),
            pltpu.VMEM((NB, 2, P, D), F32),
            bf16_buf(NB // 2 * P, 4 * D),
            pltpu.VMEM((2, D // L, MC, L), F32),
            bf16_buf(2 * P, 2 * P),
            bf16_buf(MC, 2 * P),
            pltpu.VMEM((S, L), F32),
            pltpu.VMEM((2, P, L), F32),
            pltpu.VMEM((4, 8, D), F32),
            pltpu.VMEM((D // L, S + 8, L), F32),
            pltpu.SemaphoreType.DMA((1,)),
            pltpu.SemaphoreType.DMA((NT,)),
            pltpu.SemaphoreType.DMA((NT,)),
            pltpu.SemaphoreType.DMA((NT,)),
            pltpu.SemaphoreType.DMA((5,)),
            pltpu.SemaphoreType.DMA((NT,)),
        ],
        compiler_params=_compiler_params(),
    )(A_q, A_k, A_v, A_shift_k.T, A_ssm_k, A_ssm_D, B_w_in, B_w_sp, B_b_sp, B_w_out)
```

```python
import math

import jax
import jax.numpy as jnp
import jax.experimental.pallas as pl
import jax.experimental.pallas.tpu as pltpu

S = 2048
D = 640
FH = 768
P = 128
NB = S // P
TM = 256
NT = S // TM
MC = 64
L = 128
HK = S // 2
KQ = HK // 2
KH = 256
HN = FH // 2
EPS = 1e-5
F32 = jnp.float32
BF16 = jnp.bfloat16
U32 = jnp.uint32
GELU_C = math.sqrt(2.0 / math.pi)
GA = (GELU_C * 0.044715) ** (1.0 / 3.0)
NT_DIMS = (((1,), (1,)), ((), ()))

WIN_CHUNKS = ((6, 7), (7, 9), (9, 12), (0, 3), (3, 6))
X_DMAS = ((0,), (1,), (2,), (3,), (4, 5), (6, 7))
CONV_DMAS = ((0,), (1,), (2, 3), (4, 5), (6, 7))
P1_GROUPS = ((2,), (3,), (4, 5), (6, 7))
P1_X = {2: None, 3: 0, 4: 1, 5: None, 6: 2, 7: 3}
P1_LNX = {2: (3,), 3: (4, 5), 4: (6,), 5: (7,), 6: (), 7: ()}
P2_GROUPS = ((0,), (1, 2), (3, 4, 5), (6, 7))
P2_X = ((4, 5), (6,), (7,), ())
STEP_BLOCKS = ((2, 3), (6, 7), (4, 5), (12, 13), (10, 11), (0, 1), (14, 15), (8, 9))
KV_COST, A_COST, A2_COST = 110, 56, 34
E_COST, U_COST, T_COST, TAIL_W = 24, 90, 90, 1.6
KV_SPLIT = {2: (0, 14, 6), 3: (12, 4, 4), 4: (12, 4, 4), 5: (0, 14, 6), 6: (12, 4, 4), 7: (12, 4, 4)}
FR = 8
L1_USE = {0: ((0, 1, True, False), (3, 1, True, False)), 6: ((0, 1, False, False),),
          3: ((0, 1, False, False), (2, 1, True, False)), 4: ((0, -1, False, True), (1, 1, True, False)),
          1: ((2, 1, False, True), (3, -1, False, False)), 2: ((1, 1, False, True), (3, 1, False, False)),
          5: ((3, 1, False, True),)}
H_SPLIT = ((0, 2), (2, 4), (4, 5))
FINE = tuple((l, l + 1) for l in range(D // L))
P1_TUNE = {2: (40, 0), 3: (44, 0), 4: (42, 0), 5: (42, 0), 6: (44, 0), 7: (24, 0)}
EXTRA = (52, 52)
LAST_N = 22
P2_END = (0.0, -1.0, -1.0, 0.0)
F_TIED = (20, 20, 18, 20, 20)
_ONLY = None


def _dot(a, b):
    return jnp.dot(a, b, preferred_element_type=F32)


def _sums_left(a11, a12, a21, a22):
    add, sub = jax.lax.add, jax.lax.sub
    return jnp.concatenate((add(a11, a22), add(a21, a22), add(a11, a12), sub(a21, a11), sub(a12, a22)),
                           axis=1).astype(BF16)


def _sums_right(b11, b12, b21, b22):
    add, sub = jax.lax.add, jax.lax.sub
    return jnp.concatenate((add(b11, b22), sub(b12, b22), sub(b21, b11), add(b11, b12), add(b21, b22)),
                           axis=1).astype(BF16)


def _cos_sin(m):
    q = (m + 256) >> 9
    x = (m - (q << 9)).astype(F32) * (2.0 * math.pi / 2048.0)
    x2 = x * x
    s = x * (1.0 + x2 * (-1.0 / 6 + x2 * (1.0 / 120 + x2 * (-1.0 / 5040 + x2 * (1.0 / 362880)))))
    c = 1.0 + x2 * (-0.5 + x2 * (1.0 / 24 + x2 * (-1.0 / 720 + x2 * (1.0 / 40320 - x2 * (1.0 / 3628800)))))
    swap = (q & 1) == 1
    c0 = jnp.where(swap, s, c)
    s0 = jnp.where(swap, c, s)
    cos = jnp.where(((q + 1) & 2) == 2, -c0, c0)
    sin = jnp.where((q & 2) == 2, -s0, s0)
    return cos, sin


def _odd_freq(r):
    return jnp.where(r < 64, 4 * r + 1, 4 * r - 253)


def _gelu_scaled(z):
    return z + z * jnp.tanh(z * (GELU_C / GA + z * z))


def _signzero(z):
    bits = jax.lax.bitcast_convert_type(z, U32) & jnp.uint32(0x80000000)
    return jax.lax.bitcast_convert_type(bits, F32)


def _ln(x, eps, tie=None, scale=None):
    n = x.shape[-1]
    cols = [x[:, j * L:(j + 1) * L] for j in range(n // L)]
    s1 = cols[0]
    s2 = cols[0] * cols[0]
    for c in cols[1:]:
        s1 = s1 + c
        s2 = s2 + c * c
    if tie is not None:
        s1 = s1 + tie
        s2 = s2 + tie
    m = jnp.sum(s1, axis=-1, keepdims=True) * (1.0 / n)
    v = jnp.maximum(jnp.sum(s2, axis=-1, keepdims=True) * (1.0 / n) - m * m, 0.0)
    rs = jax.lax.rsqrt(v + eps)
    if scale is not None:
        rs = rs * scale
    return (x - m) * rs


def _blocks_of_step(i):
    return STEP_BLOCKS[i]


class _Background:
    def __init__(self):
        self.q = []
        self.credit = 0.0

    def add(self, gen):
        self.q.append(gen)

    def run(self, budget):
        self.credit += budget
        while self.q and self.credit > 0:
            try:
                self.credit -= next(self.q[0])
            except StopIteration:
                self.q.pop(0)
        if not self.q:
            self.credit = 0.0

    def charge(self, cost):
        self.credit -= cost

    def drain(self):
        while self.q:
            self.run(1e9)


class _Tied:
    def __init__(self, tasks, npieces):
        self.tasks = list(tasks)
        self.rate = len(self.tasks) / float(npieces)
        self.credit = 0.999

    def run(self, z):
        self.credit += self.rate
        n = 0
        while self.tasks and self.credit >= 1.0:
            self.tasks.pop(0)(_signzero(z[0:16]))
            self.credit -= 1.0
            n += 1
        return n


def _kernel(q_hbm, k_hbm, v_hbm, sk_hbm, h_hbm, d_hbm, win_hbm, wsp_hbm, b_hbm, wout_hbm,
            o_hbm,
            x_us, k_us, v_us, h_us, win_us, wsp_us, wout_u, o_v, sk_in, d_in, b_in,
            xn_u, XL_u, WB_u, UL_u, WO_u, z1_v, R_u, Lc_u, L2_u, R2_u, C_v, zf_v, zg_v, kv_u, u_u, X_v, H_v, G_v, Z_u,
            yl_v, F_u, Fi_u, bcol_v, ph_v, sk_v, kf_v,
            sem_small, sem_x, sem_conv, sem_wsp, sem_w, sem_out):
    (wout_v, xn_v, XL_v, WB_v, UL_v, WO_v, R_v, Lc_v, L2_v, R2_v, kv_v, u_v, Z_v, F_v, Fi_v) = [
        r.bitcast(BF16) for r in (wout_u, xn_u, XL_u, WB_u, UL_u, WO_u, R_u, Lc_u, L2_u, R2_u, kv_u, u_u, Z_u, F_u, Fi_u)]
    x_vs = {g[0]: r.bitcast(BF16) for g, r in zip(X_DMAS, x_us)}
    k_vs, v_vs, h_vs = [{g[0]: r.bitcast(BF16) for g, r in zip(CONV_DMAS, rs)} for rs in (k_us, v_us, h_us)]
    wsp_vs = [r.bitcast(BF16) for r in wsp_us]
    win_vs = [r.bitcast(BF16) for r in win_us]

    def win(rows, n):
        c = [lo <= n < hi for lo, hi in WIN_CHUNKS].index(True)
        n -= WIN_CHUNKS[c][0]
        return win_vs[c][rows, n * L:(n + 1) * L]

    def locate(bufs, row):
        t0 = max(t for t in bufs if t * TM <= row)
        return bufs[t0], row - t0 * TM

    def rows_of(bufs, row, n, lanes=slice(None)):
        buf, r = locate(bufs, row)
        return buf[r:r + n, lanes]

    def cp_small():
        return [pltpu.make_async_copy(s_, d_, sem_small.at[0])
                for s_, d_ in ((d_hbm, d_in), (sk_hbm, sk_in), (b_hbm, b_in))]

    def cp_x(t):
        return pltpu.make_async_copy(q_hbm.at[0, pl.ds(t * TM, x_vs[t].shape[0])], x_vs[t], sem_x.at[t])

    def cp_conv(t):
        rows = pl.ds(t * TM, k_vs[t].shape[0])
        sem = sem_conv.at[t]
        return [pltpu.make_async_copy(h_hbm.at[:, rows], h_vs[t], sem),
                pltpu.make_async_copy(k_hbm.at[0, rows], k_vs[t], sem),
                pltpu.make_async_copy(v_hbm.at[0, rows], v_vs[t], sem)]

    def cp_wsp(i):
        return [pltpu.make_async_copy(wsp_hbm.at[pl.ds(_blocks_of_step(i)[0] * P, TM)], wsp_vs[i], sem_wsp.at[i])]

    def cp_win(c):
        lo, hi = WIN_CHUNKS[c]
        w = (hi - lo) * L
        return pltpu.make_async_copy(win_hbm.at[:, pl.ds(lo * L, w)], win_vs[c].at[:, pl.ds(0, w)], sem_w.at[c])

    def cp_wout():
        return pltpu.make_async_copy(wout_hbm, wout_v, sem_w.at[5])

    def cp_out(i):
        rows = pl.ds(_blocks_of_step(i)[0] * P, TM)
        return [pltpu.make_async_copy(o_v.at[rows], o_hbm.at[0, rows], sem_out.at[i])]

    def start(cs):
        for c in cs:
            c.start()

    def wait(cs):
        for c in cs:
            c.wait()

    def block(fn, name):
        def body(it):
            fn()
            return it + 1

        if _ONLY is None or name in _ONLY:
            jax.lax.while_loop(lambda it: it < 1, body, jnp.int32(0))

    def ln_x(t, s, tie=None):
        rows = pl.ds(t * TM + s * 16, 16)
        y = _ln(rows_of(x_vs, t * TM + s * 16, 16).astype(F32), EPS, tie, GA)
        xn_v[rows, :] = y.astype(BF16)
        return y

    def ln_x2_tasks(t):
        held = {}

        def first(s, tie):
            held[s] = ln_x(t, 8 * (s // 4) + s % 4, tie)

        def second(s, tie):
            p, q = s // 4, s % 4
            y1, y2 = held.pop(s), ln_x(t, 8 * p + 4 + q, tie)
            XL_v[pl.ds((t % 4) * P + p * MC + q * 16, 16), :] = _sums_left(
                y1[:, :KH], y1[:, KH:2 * KH], y2[:, :KH], y2[:, KH:2 * KH])

        return [[lambda tie, s=s: first(s, tie) for s in range(8)],
                [lambda tie, s=s: second(s, tie) for s in range(8)]]

    def wcomb_gen(cols):
        for j in cols:
            for r in range(KH // 32):
                top = pl.ds(r * 32, 32)
                bot = pl.ds(KH + r * 32, 32)
                b11, b12 = win(top, j).astype(F32), win(top, 6 + j).astype(F32)
                b21, b22 = win(bot, j).astype(F32), win(bot, 6 + j).astype(F32)
                WB_v[top, j * 5 * L:(j + 1) * 5 * L] = _sums_right(b11, b12, b21, b22)
                yield A_COST

    def ln_z2(t, s, tie=None):
        y = _ln(zg_v[t % 3, s * 16:(s + 1) * 16, :], 4.0 * GA * GA * EPS, tie, 0.25 / GA)
        lo, hi = y[:, :HN], y[:, HN:]
        rows = pl.ds((t * TM + s * 16) % HK, 16)
        if t < NT // 2:
            zf_v[rows, :] = y
            R_v[rows, 0:2 * HN] = jnp.concatenate((lo, lo + hi), axis=1).astype(BF16)
        else:
            b11, b12 = zf_v[rows, :HN], zf_v[rows, HN:]
            R_v[rows, 2 * HN:] = jnp.concatenate((b11 + hi, b12 - hi, lo - b11, hi, lo + hi), axis=1).astype(BF16)

    def r1(j, rows, n):
        c0 = {1: 0, 5: 1, 0: 2, 2: 3, 3: 4, 4: 5, 6: 6}[j] * HN + n * L
        return R_v[rows, c0:c0 + L]

    def acomb_gen(i, groups=range(P // 16)):
        for r in groups:
            for c in range(HK // 256):
                top = pl.ds(r * 16, 16)
                bot = pl.ds(P + r * 16, 16)
                c1 = slice(c * 256, (c + 1) * 256)
                c2 = slice(HK + c * 256, HK + (c + 1) * 256)
                a11 = wsp_vs[i][top, c1].astype(F32)
                a12 = wsp_vs[i][top, c2].astype(F32)
                a21 = wsp_vs[i][bot, c1].astype(F32)
                a22 = wsp_vs[i][bot, c2].astype(F32)
                r0 = (i % 5) * 5 * P + (r % 4 * 2 + r // 4) * 16
                Lc_v[pl.ds(r0 + 0 * P, 16), c1] = (a11 + a22).astype(BF16)
                Lc_v[pl.ds(r0 + 1 * P, 16), c1] = (a21 + a22).astype(BF16)
                Lc_v[pl.ds(r0 + 2 * P, 16), c1] = (a11 + a12).astype(BF16)
                Lc_v[pl.ds(r0 + 3 * P, 16), c1] = (a21 - a11).astype(BF16)
                Lc_v[pl.ds(r0 + 4 * P, 16), c1] = (a12 - a22).astype(BF16)
                yield A_COST

    def acomb2_gen(i):
        for r in range(MC // 16):
            for c in range(KQ // L):
                quad = {}

                def w(b, H):
                    if (b, H) not in quad:
                        quad[b, H] = [[wsp_vs[i][pl.ds(b * P + s_ * MC + r * 16, 16),
                                                 H * HK + kh * KQ + c * L:H * HK + kh * KQ + (c + 1) * L].astype(F32)
                                       for kh in range(2)] for s_ in range(2)]
                    return quad[b, H]

                spec = {2: (None, (0, 0), None, 0), 0: (0, (0, 0), (1, 1), 1), 3: (None, (1, 1), None, 0),
                        1: (1, (1, 0), (1, 1), 1), 5: (3, (1, 0), (0, 0), -1), 4: (2, (0, 0), (0, 1), 1),
                        6: (4, (0, 1), (1, 1), -1)}
                for j in (2, 0, 3, 1, 5, 4, 6):
                    slot, p_, q_, sign = spec[j]
                    a = w(*p_)
                    if q_ is not None:
                        b_ = w(*q_)
                        op = jax.lax.add if sign > 0 else jax.lax.sub
                        a = [[op(a[s_][kh], b_[s_][kh]) for kh in range(2)] for s_ in range(2)]
                        for kh in range(2):
                            Lc_v[pl.ds(((i % 5) * 5 + slot) * P + r * 32, 32),
                                 kh * KQ + c * L:kh * KQ + (c + 1) * L] = jnp.concatenate(
                                     (a[0][kh], a[1][kh]), axis=0).astype(BF16)
                    L2_v[pl.ds(((i % 5) * 7 + j) * MC + r * 16, 16), c * 5 * L:(c + 1) * 5 * L] = _sums_left(
                        a[0][0], a[0][1], a[1][0], a[1][1])
                    yield A2_COST

    def bcomb2_gen(js):
        for j in js:
            for r in range(KQ // 16):
                top = pl.ds(r * 16, 16)
                bot = pl.ds(KQ + r * 16, 16)
                R2_v[pl.ds(j * KQ + r * 16, 16), :] = _sums_right(
                    *[r1(j, rows, n).astype(F32) for rows in (top, bot) for n in range(2)])
                yield A_COST / 2

    def tasks(fn, t, n=TM // 16):
        return [lambda tie, s=s: fn(t, s, tie) for s in range(n)]

    def kv_gen(t):
        for m in range(TM // MC):
            r = t * TM + m * MC
            for l in range(D // L):
                lanes = slice(l * L, (l + 1) * L)
                kf = rows_of(k_vs, r, MC, lanes).astype(F32)
                kf_v[l, pl.ds(r + 8, MC), :] = kf
                ks = kf * sk_v[0, 0:1, lanes]
                for tap in range(1, 4):
                    ks = ks + kf_v[l, pl.ds(r + 8 - tap, MC), :] * sk_v[tap, 0:1, lanes]
                kv = ks * rows_of(v_vs, r, MC, lanes).astype(F32)
                kv_v[pl.ds(r, MC), lanes] = kv.astype(BF16)
                yield KV_COST

    def freq_gen(a):
        def cmac(acc, x, g):
            mul, add = jax.lax.mul, jax.lax.add
            pr = jax.lax.sub(mul(x[0], g[0]), mul(x[1], g[1]))
            pi = add(mul(x[0], g[1]), mul(x[1], g[0]))
            return (pr, pi) if acc is None else (add(acc[0], pr), add(acc[1], pi))

        for r in range(P // 16):
            for l in range(D // L):
                lanes = slice(l * L, (l + 1) * L)
                res = []
                for sub in range(16 // FR):
                    rows = pl.ds(r * 16 + sub * FR, FR)
                    lo = hi = None
                    g = (G_v[a + 1, 0, rows, lanes], G_v[a + 1, 1, rows, lanes])
                    for c in range(a + 2):
                        x = (X_v[c, 0, rows, lanes], X_v[c, 1, rows, lanes])
                        hi = cmac(hi, x, g)
                        if c <= a:
                            g = (G_v[a - c, 0, rows, lanes], G_v[a - c, 1, rows, lanes])
                            lo = cmac(lo, x, g)
                            yield 2 * FR
                    res.append((lo, hi))
                Z_v[pl.ds(a // 2 * P + r * 16, 16), l * 4 * L:(l + 1) * 4 * L] = jnp.concatenate(
                    [jnp.concatenate([z[0][0], z[0][1], z[1][0], z[1][1]], axis=1) for z in res], axis=0).astype(BF16)
                yield 20

    def job_x(t, bg, budget, split=((0, 5),)):
        for j in (2 * t, 2 * t + 1):
            for half in range(2):
                for l0, l1 in split:
                    w, lanes = (l1 - l0) * L, slice(l0 * L, l1 * L)
                    r = _dot(F_v[half * P:(half + 1) * P, 0:P], kv_v[j * P:(j + 1) * P, lanes]).reshape(8, 2, 8, w)
                    for part in range(2):
                        X_v[j, part, half * 64:(half + 1) * 64, lanes] = r[:, part].reshape(64, w)
                    bg.run(budget * (l1 - l0) / 2)

    def job_h(t, bg, budget, split=H_SPLIT):
        h_v, c0 = locate(h_vs, t * TM)
        for half in range(2):
            rows = pl.ds(half * 64, 64)
            for l0, l1 in split:
                w = (l1 - l0) * L
                lanes = slice(l0 * L, l1 * L)
                rhs = jnp.concatenate([h_v[lanes, c0:c0 + P], h_v[lanes, c0 + P:c0 + TM]], axis=0)
                r = jax.lax.dot_general(F_v[half * P:(half + 1) * P, 0:P], rhs, NT_DIMS,
                                        preferred_element_type=F32).reshape(8, 2, 8, 2 * w)
                re, im = r[:, 0].reshape(64, 2 * w), r[:, 1].reshape(64, 2 * w)
                prev = (H_v[t % 2, 0, rows, lanes], H_v[t % 2, 1, rows, lanes])
                for j in range(2):
                    cur = (re[:, j * w:(j + 1) * w], im[:, j * w:(j + 1) * w])
                    G_v[2 * t + j, 0, rows, lanes] = cur[0] + prev[1] if half else cur[0] - prev[1]
                    G_v[2 * t + j, 1, rows, lanes] = cur[1] - prev[0] if half else cur[1] + prev[0]
                    prev = cur
                if t + 1 < NT:
                    H_v[(t + 1) % 2, 0, rows, lanes] = prev[0]
                    H_v[(t + 1) % 2, 1, rows, lanes] = prev[1]
                bg.run(budget * (l1 - l0))

    def z_out(t, m, n, pre, bg, budget, tied):
        z = _gelu_scaled(pre)
        if n < FH // L:
            z1_v[pl.ds(t * TM + m * MC, MC), n * L:(n + 1) * L] = z
        else:
            zg_v[t % 3, m * MC:(m + 1) * MC, n * L - FH:(n + 1) * L - FH] = z
        ntask = tied.run(z)
        bg.run(budget[1] if ntask else budget[0])

    def job_z(t, m, cols, bg, budget, tied):
        for n in cols:
            z_out(t, m, n, _dot(xn_v[pl.ds(t * TM + m * MC, MC), :], win(slice(None), n)), bg, budget, tied)

    def job_zs(t, p, j, bg, budget, tied):
        r1 = pl.ds(t * TM + p * P, MC)
        r2 = pl.ds(t * TM + p * P + MC, MC)

        def xl(w):
            r0 = (t % 4) * P + p * MC
            return XL_v[r0:r0 + MC, w * KH:(w + 1) * KH]

        def wb(w):
            return WB_v[:, (j * 5 + w) * L:(j * 5 + w + 1) * L]

        def rem(rows, n):
            return _dot(xn_v[rows, 2 * KH:], win(slice(2 * KH, D), n))

        m2 = _dot(xl(1), win(slice(0, KH), j))
        m4 = _dot(xn_v[r2, KH:2 * KH], wb(2))
        z_out(t, 2 * p + 1, j, m2 + m4 + rem(r2, j), bg, budget, tied)
        m3 = _dot(xn_v[r1, 0:KH], wb(1))
        m5 = _dot(xl(2), win(slice(KH, 2 * KH), 6 + j))
        z_out(t, 2 * p, 6 + j, m3 + m5 + rem(r1, 6 + j), bg, budget, tied)
        t11, t22 = m4 - m5, m3 - m2
        m1 = _dot(xl(0), wb(0))
        t11, t22 = t11 + m1, t22 + m1
        z_out(t, 2 * p, j, t11 + _dot(xl(4), wb(4)) + rem(r1, j), bg, budget, tied)
        z_out(t, 2 * p + 1, 6 + j, t22 + _dot(xl(3), wb(3)) + rem(r2, 6 + j), bg, budget, tied)

    rev8 = 7 - jax.lax.broadcasted_iota(jnp.int32, (8, L), 0)

    def finish(a, upper, n, hh, slot):
        rows = pl.ds(a * P + (MC if upper else 0), MC)
        lanes = slice(n * L, (n + 1) * L)
        if upper:
            zc = (n * 4 + a % 2 * 2) * L
            ya = _dot(Fi_v[:, 0:P], Z_v[a // 2 * P:(a // 2 + 1) * P, zc:zc + L])
            yb = _dot(Fi_v[:, P:2 * P], Z_v[a // 2 * P:(a // 2 + 1) * P, zc + L:zc + 2 * L])
            slot(0.5)
            y = ya - yb
            lo = ya + yb
            for j in range(MC // 8):
                yl_v[a % 2, n, (7 - j) * 8:(8 - j) * 8, :] = jnp.take_along_axis(lo[j * 8:(j + 1) * 8], rev8, axis=0)
        else:
            y = yl_v[a % 2, n]
        gate = hh + hh * jnp.tanh(hh)
        s = xn_v[rows, lanes].astype(F32) * y
        x = rows_of(x_vs, a * P + (MC if upper else 0), MC, lanes).astype(F32)
        o_v[rows, lanes] = (x + s * gate).astype(BF16)

    def tail_gen(i, bg, budget):
        a0, a1 = _blocks_of_step(i)

        def slot(w):
            bg.run(w * budget[0])

        def dot3(a, b):
            r = _dot(a, b)
            slot(0.75)
            return r

        for upper in (True, False):
            sub = MC if upper else 0
            r1 = pl.ds(a0 * P + sub, MC)
            r2 = pl.ds(a1 * P + sub, MC)

            def ul(w):
                allw = UL_v[(i % 5) * P + sub:(i % 5) * P + sub + MC, :]
                return jnp.concatenate([allw[:, (n * 5 + w) * L:(n * 5 + w + 1) * L] for n in range(HN // L)], axis=1)

            for j in range(2):
                c1 = slice(j * L, (j + 1) * L)
                c2 = slice((2 + j) * L, (3 + j) * L)

                def wo(w):
                    return WO_v[:, (j * 5 + w) * L:(j * 5 + w + 1) * L]

                m2 = dot3(ul(1), wout_v[0:HN, c1])
                m4 = dot3(u_v[r2, HN:], wo(2))
                finish(a1, upper, j, m2 + m4, slot)
                bg.charge(T_COST)
                yield
                m3 = dot3(u_v[r1, 0:HN], wo(1))
                m5 = dot3(ul(2), wout_v[HN:, c2])
                finish(a0, upper, 2 + j, m3 + m5, slot)
                bg.charge(T_COST)
                yield
                t11, t22 = m4 - m5, m3 - m2
                m1 = dot3(ul(0), wo(0))
                t11, t22 = t11 + m1, t22 + m1
                finish(a0, upper, j, t11 + dot3(ul(4), wo(4)), slot)
                bg.charge(T_COST)
                yield
                finish(a1, upper, 2 + j, t22 + dot3(ul(3), wo(3)), slot)
                bg.charge(T_COST)
                yield
            for a, r in ((a0, r1), (a1, r2)):
                finish(a, upper, 4, dot3(u_v[r, 0:HN], wout_v[0:HN, 4 * L:]) + dot3(u_v[r, HN:], wout_v[HN:, 4 * L:]),
                       slot)
                bg.charge(T_COST)
                yield

    def wocomb_gen():
        for j in range(2):
            c1 = slice(j * L, (j + 1) * L)
            c2 = slice((2 + j) * L, (3 + j) * L)
            for r in range(HN // 32):
                top = pl.ds(r * 32, 32)
                bot = pl.ds(HN + r * 32, 32)
                b11, b12 = wout_v[top, c1].astype(F32), wout_v[top, c2].astype(F32)
                b21, b22 = wout_v[bot, c1].astype(F32), wout_v[bot, c2].astype(F32)
                WO_v[top, j * 5 * L:(j + 1) * 5 * L] = _sums_right(b11, b12, b21, b22)
                yield A_COST

    def job_big(i, bg, pending, budget, every):
        a0, a1 = _blocks_of_step(i)
        KG = 512

        def lhs(j, sub, cols):
            if j == 2:
                return wsp_vs[i][sub:sub + MC, cols]
            if j == 3:
                return wsp_vs[i][P + sub:P + sub + MC, HK + cols.start:HK + cols.stop]
            r0 = ((i % 5) * 5 + {0: 0, 1: 1, 4: 2, 5: 3, 6: 4}[j]) * P
            both = Lc_v[r0:r0 + P, cols]
            return jnp.concatenate([both[q * 32 + sub // 4:q * 32 + sub // 4 + 16] for q in range(4)], axis=0)

        def prod(j, sub, n, acc=None):
            for kg in range(HK // KG):
                ks = slice(kg * KG, (kg + 1) * KG)
                p = _dot(lhs(j, sub, ks), r1(j, ks, n))
                acc = p if acc is None else p + acc
                bg.run(budget)
            return acc

        def tails(n):
            for _ in range(n):
                if pending:
                    next(pending.pop(0))

        def emit(a, sub, n, g):
            rows = pl.ds(a * P + sub, MC)
            lanes = slice(n * L, (n + 1) * L)
            u = z1_v[rows, lanes] * (g + bcol_v[rows, :])
            u_v[rows, lanes] = u.astype(BF16)
            bg.charge(E_COST)
            return u

        if i > 0:
            def piece(a, b, acc=None):
                p = _dot(a, b)
                bg.run(budget)
                return p if acc is None else acc + p

            def cslot(k, s_, n):
                return pl.ds(((k * 2 + s_) * 2 + n) * MC, MC)

            def contribute(j, s_, n, m):
                for k, sign, first, last in L1_USE[j]:
                    cs = cslot(k, s_, n)
                    v_ = m if first else (C_v[cs, :] + m if sign > 0 else C_v[cs, :] - m)
                    if last:
                        u = emit((a0, a0, a1, a1)[k], s_ * MC, n + (k % 2) * (HN // L), v_)
                        v_ = u
                        if k == 3:
                            u11, u12, u21 = C_v[cslot(0, s_, n), :], C_v[cslot(1, s_, n), :], C_v[cslot(2, s_, n), :]
                            UL_v[pl.ds((i % 5) * P + s_ * MC, MC), n * 5 * L:(n + 1) * 5 * L] = _sums_left(
                                u11, u12, u21, u)
                            bg.charge(U_COST)
                            continue
                    C_v[cs, :] = v_

            for j in (0, 6, 3, 4, 1, 2, 5):
                def l2(w):
                    r0 = ((i % 5) * 7 + j) * MC
                    allw = L2_v[r0:r0 + MC, :]
                    return jnp.concatenate([allw[:, (c * 5 + w) * L:(c * 5 + w + 1) * L] for c in range(KQ // L)],
                                           axis=1)

                def r2(w):
                    return R2_v[j * KQ:(j + 1) * KQ, w * L:(w + 1) * L]

                def rq(kh, n):
                    return r1(j, slice(kh * KQ, (kh + 1) * KQ), n)

                p2 = piece(l2(1), rq(0, 0))
                p4 = piece(lhs(j, MC, slice(KQ, 2 * KQ)), r2(2))
                contribute(j, 1, 0, p2 + p4)
                p3 = piece(lhs(j, 0, slice(0, KQ)), r2(1))
                t22 = p3 - p2
                p5 = piece(l2(2), rq(1, 1))
                contribute(j, 0, 1, p3 + p5)
                t11 = p4 - p5
                p1 = piece(l2(0), r2(0))
                t11, t22 = t11 + p1, t22 + p1
                contribute(j, 0, 0, piece(l2(4), r2(4), t11))
                contribute(j, 1, 1, piece(l2(3), r2(3), t22))
                tails(every.pop(0))

        for sub in (0, MC):
            for n in (range(HN // L) if i == 0 else (2,)):
                def put(w, c):
                    UL_v[pl.ds((i % 5) * P + sub, MC), (n * 5 + w) * L:(n * 5 + w + 1) * L] = c.astype(BF16)

                m1 = prod(0, sub, n)
                t11 = prod(6, sub, n, m1)
                m4 = prod(3, sub, n)
                t11 = t11 + m4
                m5 = prod(4, sub, n)
                u11 = emit(a0, sub, n, t11 - m5)
                m2 = prod(1, sub, n)
                u21 = emit(a1, sub, n, m2 + m4)
                put(3, u21 - u11)
                t22 = m1 - m2
                m3 = prod(2, sub, n)
                u12 = emit(a0, sub, n + HN // L, m3 + m5)
                put(2, u11 + u12)
                u22 = emit(a1, sub, n + HN // L, prod(5, sub, n, t22 + m3))
                put(0, u11 + u22)
                put(1, u21 + u22)
                put(4, u12 - u22)
                bg.charge(U_COST)
                tails(every.pop(0))

    def debug_keep_alive():
        if _ONLY is not None:
            for r_ in (xn_u, XL_u, WB_u, UL_u, WO_u, z1_v, R_u, Lc_u, L2_u, R2_u, C_v, zf_v, zg_v, kv_u, u_u, X_v, H_v, G_v, Z_u,
                       kf_v, bcol_v):
                c_ = pltpu.make_async_copy(r_, r_, sem_small.at[0])
                c_.start()
                c_.wait()

    debug_keep_alive()

    cp_x(0).start()
    cp_win(0).start()
    cp_x(1).start()
    cp_win(1).start()
    start(cp_small())
    for c in range(2, 5):
        cp_win(c).start()
    cp_x(2).start()

    kk = _odd_freq(jax.lax.broadcasted_iota(jnp.int32, (P, P), 0))
    nn = jax.lax.broadcasted_iota(jnp.int32, (P, P), 1)
    fc, fs = _cos_sin((kk * (4 * nn - 127)) & 2047)
    for g in range(P // 8):
        F_v[g * 16:(g + 1) * 16, 0:P] = jnp.concatenate(
            [fc[g * 8:(g + 1) * 8], -fs[g * 8:(g + 1) * 8]], axis=0).astype(BF16)
    fc, fs = _cos_sin((kk * (-127)) & 2047)
    ph_v[0] = fc
    ph_v[1] = fs
    kk = _odd_freq(jax.lax.broadcasted_iota(jnp.int32, (MC, P), 1))
    mm = jax.lax.broadcasted_iota(jnp.int32, (MC, P), 0)
    ic, is_ = _cos_sin((kk * (4 * mm + 2)) & 2047)
    Fi_v[:, 0:P] = (ic * (1.0 / (P * GA))).astype(BF16)
    Fi_v[:, P:2 * P] = (is_ * (1.0 / (P * GA))).astype(BF16)
    kf_v[:, 0:8, :] = jnp.zeros((D // L, 8, L), F32)

    cp_x(0).wait()
    for s in range(TM // 16):
        ln_x(0, s)
    start(cp_conv(0) + [cp_x(3), cp_x(4)] + cp_conv(1) + [cp_x(6)] + cp_conv(2) + cp_conv(4) + [cp_wout()])
    start(cp_wsp(0) + cp_wsp(1) + cp_wsp(2) + cp_conv(6))
    for i in range(3, NT):
        start(cp_wsp(i))

    def small_setup():
        sk = sk_in[...].astype(F32)
        for t in range(4):
            sk_v[t] = jnp.broadcast_to(sk[t:t + 1], (8, D))
        drow = d_in[...].astype(F32).reshape(1, D)
        for l in range(D // L):
            lanes = slice(l * L, (l + 1) * L)
            dre = ph_v[0] * drow[:, lanes]
            dim = ph_v[1] * drow[:, lanes]
            H_v[0, 0, 0:64, lanes] = -dim[0:64]
            H_v[0, 0, 64:P, lanes] = dim[64:P]
            H_v[0, 1, 0:64, lanes] = -dre[0:64]
            H_v[0, 1, 64:P, lanes] = dre[64:P]

    def bcol_task(t, j, tie):
        brow = b_in[...].astype(F32).reshape(1, S)[:, j * P:(j + 1) * P] * (0.25 / GA) + tie[0:1]
        bcol_v[j * P:(j + 1) * P, :] = jnp.broadcast_to(brow, (P, P)).T

    LAG = 2

    def interleave(*lists):
        out = []
        for j in range(max(len(a) for a in lists)):
            for a in lists:
                out += a[j:j + 1]
        return out

    def p1_first(c):
        bg = _Background()
        todo = []
        if c == 2:
            todo = tasks(bcol_task, 0)
            small_setup()
        if c == 3:
            todo = tasks(ln_z2, 0)
            bg.add(wcomb_gen(range(3)))
        if c == 4:
            todo = interleave(*ln_x2_tasks(2))
            bg.add(wcomb_gen(range(3, 6)))
        tied = _Tied(todo, F_TIED[c])
        if c == 0:
            for s in range(TM // 16):
                ln_x(1, s)
        for t in range(2):
            for m in range(TM // MC):
                job_z(t, m, range(*WIN_CHUNKS[c]), bg, (80, 40), tied)
        bg.drain()
        assert not tied.tasks

    for c in range(5):
        cp_win(c).wait()
        if c == 0:
            cp_x(1).wait()
        if c == 2:
            wait(cp_small())
        if c == 4:
            cp_x(2).wait()
        block(lambda c=c: p1_first(c), f'p1_f{c}')

    def p1_wait(g):
        if g == 0:
            wait(cp_conv(0))
            cp_x(3).wait()
        if g == 1:
            wait(cp_conv(1))
            cp_x(4).wait()
        if g == 2:
            wait(cp_conv(2))
            cp_x(6).wait()
        if g == 3:
            wait(cp_conv(4))
            cp_wout().wait()
            wait(cp_wsp(0))

    def take(gen, n):
        for _ in range(n):
            yield next(gen)

    def p1_step(i):
        bg = _Background()
        dft = _Background()
        t = i - LAG
        xg = P1_X[i]
        kv = kv_gen(t)
        nx, nz, nh = KV_SPLIT[i]
        dft.add(take(kv, nx))
        bg.add(take(kv, nz))
        hbg = _Background()
        hbg.add(take(kv, nh))
        zb = nz * KV_COST / 48.0
        extra = 0
        if i == 6:
            bg.add(wocomb_gen())
            bg.add(acomb_gen(0, range(5)))
            extra = EXTRA[0]
        if i == 7:
            bg.add(acomb_gen(0, range(5, 8)))
            bg.add(bcomb2_gen((1, 5)))
            extra = EXTRA[1]
        last = i == NT - 1
        z2t = tasks(ln_z2, i - 1)
        xt = [l_ for t_ in P1_LNX[i] for l_ in ln_x2_tasks(t_)]
        if P1_TUNE[i][1]:
            todo = interleave(*([z2t[0::2]] + xt + [z2t[1::2]]))
        else:
            todo = interleave(*(xt + [z2t[0::2], z2t[1::2]]))
        tied = _Tied(todo, P1_TUNE[i][0])
        if xg is not None:
            dft.run(KV_COST)
            job_x(xg, dft, (nx - 1) * KV_COST / 10.0)
            dft.drain()
        for p in range(2):
            for j in range(FH // L):
                job_zs(i, p, j, bg, (1.6 * zb + extra, 0.5 * zb + extra), tied)
            assert not tied.tasks or (p == 0 and not last)
            if p == 0 and last:
                tied = _Tied(tasks(ln_z2, i, 8), LAST_N)
        if last:
            for s in range(8, 16):
                ln_z2(i, s)
        bg.drain()
        job_h(t, hbg, nh * KV_COST / 10.0)
        hbg.drain()

    def p1_block(g):
        for i in P1_GROUPS[g]:
            p1_step(i)

    for g in range(len(P1_GROUPS)):
        p1_wait(g)
        block(lambda g=g: p1_block(g), f'p1_g{g}')

    groups = P2_GROUPS
    NG = len(groups)

    def p2_dma(gi):
        if gi >= 2:
            for i in groups[gi - 2]:
                start(cp_out(i))
        if gi >= 3:
            for i in groups[gi - 3]:
                wait(cp_out(i))
        if gi == 0:
            wait(cp_conv(6))
        if gi + 1 < NG:
            for i in groups[gi + 1]:
                wait(cp_wsp(i))

    def tails_of(i, bg, budget):
        return [tail_gen(i, bg, budget)] * 20

    def p2_block(gi):
        bg = _Background()
        steps = groups[gi]
        tb = [0.0]
        pending = [t_ for i in (groups[gi - 1] if gi > 0 else []) for t_ in tails_of(i, bg, tb)]
        total = sum(a + 1 for i in steps for a in _blocks_of_step(i)) * 40 * 16
        total += len(steps) * (24 * E_COST + 6 * U_COST) + len(pending) * T_COST
        slots = sum(84 if i == 0 else 77 for i in steps) + TAIL_W * len(pending)
        bg.add(freq_gen(_blocks_of_step(steps[0])[0]))
        if gi == 0:
            bg.add(bcomb2_gen((0, 2, 3, 4, 6)))
            total += 5 * 16 * A_COST
        if gi < 2:
            bg.add(kv_gen(NT - 2 + gi))
            total += 20 * KV_COST
            slots += 10
        for t in P2_X[gi]:
            slots += 10
        if gi + 1 < NG:
            for i in groups[gi + 1]:
                bg.add(acomb2_gen(i))
                total += 16 * 7 * A2_COST
        for i in steps[1:]:
            bg.add(freq_gen(_blocks_of_step(i)[0]))
        budget = tb[0] = total / (slots + P2_END[gi])
        bg.run(budget)
        for t in P2_X[gi]:
            job_x(t, bg, budget, FINE)
        if gi < 2:
            job_h(NT - 2 + gi, bg, budget, FINE)
        units = [4, 4, 2, 4, 4, 2] * (len(pending) // 20)
        every = [0] * sum(6 if i == 0 else 9 for i in steps)
        for j, n in enumerate(units):
            every[min(len(every) - 1, j * len(every) // len(units))] += n
        for i in steps:
            job_big(i, bg, pending, budget, every)
        for t_ in pending:
            next(t_)
        bg.drain()

    for gi in range(NG):
        p2_dma(gi)
        block(lambda gi=gi: p2_block(gi), f'p2_{gi}')

    def cp_last(part):
        a0 = _blocks_of_step(NT - 1)[0]
        sub, cols = ((MC, pl.ds(0, D)), (0, pl.ds(0, 4 * L)), (0, pl.ds(4 * L, L)))[part]
        return [pltpu.make_async_copy(o_v.at[pl.ds(r, MC), cols], o_hbm.at[0, pl.ds(r, MC), cols],
                                      sem_out.at[NT - 1]) for r in (a0 * P + sub, (a0 + 1) * P + sub)]

    def p2_last():
        for i in groups[NG - 1]:
            for j, t_ in enumerate(tails_of(i, _Background(), [0.0])):
                next(t_)
                if i < NT - 1 and j == 19:
                    start(cp_out(i))
                if i == NT - 1 and j in (9, 17):
                    start(cp_last(j // 10))

    p2_dma(NG)
    block(p2_last, 'p2_last')
    start(cp_last(2))
    for i in groups[NG - 2] + groups[NG - 1][:-1]:
        wait(cp_out(i))
    for part in range(3):
        wait(cp_last(part))
    debug_keep_alive()


def _compiler_params():
    vmem = 116 * 1024 * 1024
    try:
        return pltpu.CompilerParams(vmem_limit_bytes=vmem, disable_semaphore_checks=True)
    except TypeError:
        return pltpu.CompilerParams(vmem_limit_bytes=vmem)


@jax.jit
def pallas_recurrent_scan__ssm_conv_h3__mixer_gmlp__prompt_kernel(
    A_q: jax.Array,
    A_k: jax.Array,
    A_v: jax.Array,
    A_shift_k: jax.Array,
    A_ssm_k: jax.Array,
    A_ssm_D: jax.Array,
    B_x: jax.Array,
    B_w_in: jax.Array,
    B_w_sp: jax.Array,
    B_b_sp: jax.Array,
    B_w_out: jax.Array,
):
    del B_x
    hbm = pl.BlockSpec(memory_space=pl.ANY)

    def bf16_buf(*shape):
        return pltpu.VMEM(shape[:-2] + (shape[-2] // 2, shape[-1]), U32)

    return pl.pallas_call(
        _kernel,
        out_shape=jax.ShapeDtypeStruct((1, S, D), BF16),
        in_specs=[hbm] * 10,
        out_specs=hbm,
        scratch_shapes=[
            [bf16_buf(len(g) * TM, D) for g in X_DMAS],
            [bf16_buf(len(g) * TM, D) for g in CONV_DMAS],
            [bf16_buf(len(g) * TM, D) for g in CONV_DMAS],
            [bf16_buf(D, len(g) * TM) for g in CONV_DMAS],
            [bf16_buf(D, max(hi - lo, 2) * L) for lo, hi in WIN_CHUNKS],
            [bf16_buf(TM, S) for _ in range(NT)],
            bf16_buf(FH, D),
            pltpu.VMEM((S, D), BF16),
            pltpu.VMEM((4, D), BF16),
            pltpu.VMEM((D,), BF16),
            pltpu.VMEM((S,), BF16),
            bf16_buf(S, D),
            bf16_buf(4 * P, 5 * KH),
            bf16_buf(KH, 5 * FH),
            bf16_buf(5 * P, 5 * HN),
            bf16_buf(HN, 10 * L),
            pltpu.VMEM((S, FH), F32),
            bf16_buf(HK, 7 * HN),
            bf16_buf(5 * 5 * P, HK),
            bf16_buf(5 * 7 * MC, 5 * KQ),
            bf16_buf(7 * KQ, 5 * L),
            pltpu.VMEM((16 * MC, L), F32),
            pltpu.VMEM((HK, FH), F32),
            pltpu.VMEM((3, TM, FH), F32),
            bf16_buf(S, D),
            bf16_buf(S, FH),
            pltpu.VMEM((NB, 2, P, D), F32),
            pltpu.VMEM((2, 2, P, D), F32),
            pltpu.VMEM((NB, 2, P, D), F32),
            bf16_buf(NB // 2 * P, 4 * D),
            pltpu.VMEM((2, D // L, MC, L), F32),
            bf16_buf(2 * P, 2 * P),
            bf16_buf(MC, 2 * P),
            pltpu.VMEM((S, L), F32),
            pltpu.VMEM((2, P, L), F32),
            pltpu.VMEM((4, 8, D), F32),
            pltpu.VMEM((D // L, S + 8, L), F32),
            pltpu.SemaphoreType.DMA((1,)),
            pltpu.SemaphoreType.DMA((NT,)),
            pltpu.SemaphoreType.DMA((NT,)),
            pltpu.SemaphoreType.DMA((NT,)),
            pltpu.SemaphoreType.DMA((6,)),
            pltpu.SemaphoreType.DMA((NT,)),
        ],
        compiler_params=_compiler_params(),
    )(A_q, A_k, A_v, A_shift_k.T, A_ssm_k, A_ssm_D, B_w_in, B_w_sp, B_b_sp, B_w_out)
```
